```python
import jax
import jax.numpy as jnp

def _softmax(x, axis=-1):
    return jax.nn.softmax(x, axis=axis)

def _gelu(x):
    return jax.nn.gelu(x, approximate=True)

def _silu(x):
    return jax.nn.silu(x)

def _sigmoid(x):
    return jax.nn.sigmoid(x)

def _layernorm(x, axis=-1, eps=1e-05):
    m = jnp.mean(x, axis=axis, keepdims=True)
    v = jnp.var(x, axis=axis, keepdims=True)
    return (x - m) / jnp.sqrt(v + eps)

def _scatter_add(tgt, idx, src, axis=0):
    return tgt.at[idx].add(src)

def _segment_sum(src, seg, n):
    return jax.ops.segment_sum(src, seg, n)

class _Rng:

    def __init__(self, key):
        self._k = key

    def _next(self):
        self._k, sub = jax.random.split(self._k)
        return sub

    def normal(self, shape):
        return jax.random.normal(self._next(), shape, dtype=jnp.bfloat16)

    def randint(self, lo, hi, shape):
        return jax.random.randint(self._next(), shape, lo, hi, dtype=jnp.int32)

    def uniform(self, shape, lo=0.0, hi=1.0):
        return jax.random.uniform(self._next(), shape, jnp.bfloat16, lo, hi)

    def permutation(self, n):
        return jax.random.permutation(self._next(), n)
kernel_name = 'concat_heads__sliding_local_dilated__memory_aug_recurrent_mem_tr__prompt'

def setup_inputs():
    _rng = _Rng(jax.random.key(int.from_bytes(__import__("os").urandom(4), "little")))
    _w = lambda a: (lambda t: t.astype(jnp.bfloat16) if jnp.issubdtype(t.dtype, jnp.floating) else t)(jnp.asarray(a))

    def _A_setup():
        B, S, D = (1, 2048, 640)
        return {'x': _w((lambda *s: _rng.normal(s) * 0.05)(B, S, D)), 'wqkv': _w((lambda *s: _rng.normal(s) * 0.05)(D, 3 * D)), 'wo': _w((lambda *s: _rng.normal(s) * 0.05)(D, D))}
    _A_in = _A_setup()

    def _B_setup():
        B, S, Dm = (1, 2048, 640)
        H, Dh = (32, 192)
        M, seg = (8, 32)
        seg = min(seg, S)
        S = S // seg * seg
        return {'x': _w((lambda *s: _rng.normal(s) * 0.05)(B, S, Dm)), 'mem0': _w((lambda *s: _rng.normal(s) * 0.05)(B, M, Dm)), 'Wq': _w((lambda *s: _rng.normal(s) * 0.05)(Dm, H, Dh) * Dm ** (-0.5)), 'Wk': _w((lambda *s: _rng.normal(s) * 0.05)(Dm, H, Dh) * Dm ** (-0.5)), 'Wv': _w((lambda *s: _rng.normal(s) * 0.05)(Dm, H, Dh) * Dm ** (-0.5)), 'Wo': _w((lambda *s: _rng.normal(s) * 0.05)(H, Dh, Dm) * (H * Dh) ** (-0.5)), 'seg_len': seg}
    _B_in = _B_setup()
    return {'A_x': _A_in['x'], 'A_wqkv': _A_in['wqkv'], 'A_wo': _A_in['wo'], 'B_x': _B_in['x'], 'B_mem0': _B_in['mem0'], 'B_Wq': _B_in['Wq'], 'B_Wk': _B_in['Wk'], 'B_Wv': _B_in['Wv'], 'B_Wo': _B_in['Wo'], 'B_seg_len': _B_in['seg_len']}

def reference(A_x, A_wqkv, A_wo, B_x, B_mem0, B_Wq, B_Wk, B_Wv, B_Wo, B_seg_len):

    def _A_ref(x, wqkv, wo):
        B, S, D = x.shape
        H = 32
        Dh = D // H
        W, dil = (8, 2)
        qkv = (lambda x, *d: x.transpose(*d))((x @ wqkv).reshape(B, S, 3, H, Dh), 2, 0, 3, 1, 4)
        q, k, v = (qkv[0], qkv[1], qkv[2])
        scale = Dh ** (-0.5)
        pos = jnp.arange(S)
        off = jnp.arange(W) * dil
        idx = pos[:, None] - off[None, :]
        mask = idx >= 0
        idx_c = jnp.where(mask, idx, 0).reshape(-1)
        kg = k[:, :, idx_c, :].reshape(B, H, S, W, Dh)
        vg = v[:, :, idx_c, :].reshape(B, H, S, W, Dh)
        logits = jnp.einsum('bhsd,bhswd->bhsw', q, kg) * scale
        logits = jnp.where(mask[None, None, :, :], logits, -1000000000.0)
        attn = _softmax(logits, axis=-1)
        o = jnp.einsum('bhsw,bhswd->bhsd', attn, vg)
        return (lambda x, *d: x.transpose(*d))(o, 0, 2, 1, 3).reshape(B, S, D) @ wo

    def _B_ref(x, mem0, Wq, Wk, Wv, Wo, seg_len):
        B, S, Dm = x.shape
        H, Dh = (Wq.shape[1], Wq.shape[2])
        M = mem0.shape[1]
        scale = Dh ** (-0.5)
        n_seg = S // seg_len
        L = M + seg_len
        idx = jnp.arange(L)
        mask = (idx[:, None] < M) | (idx[:, None] >= idx[None, :])
        mem = mem0
        outs = []
        for s in range(n_seg):
            xs = x[:, s * seg_len:(s + 1) * seg_len, :].copy()
            h = jnp.concatenate([mem, xs], axis=1)
            q = jnp.einsum('btd,dhe->bhte', h, Wq)
            k = jnp.einsum('btd,dhe->bhte', h, Wk)
            v = jnp.einsum('btd,dhe->bhte', h, Wv)
            scores = jnp.einsum('bhqe,bhke->bhqk', q, k) * scale
            scores = jnp.where(mask[None, None], scores, -1000000000.0)
            p = _softmax(scores, axis=-1)
            o = jnp.einsum('bhqk,bhke->bhqe', p, v)
            o = jnp.einsum('bhte,hed->btd', o, Wo)
            mem = o[:, :M, :].copy()
            outs.append(o[:, M:, :])
        return jnp.concatenate(outs, axis=1)
    a = _A_ref(A_x, A_wqkv, A_wo)
    b = _B_ref(B_x, B_mem0, B_Wq, B_Wk, B_Wv, B_Wo, B_seg_len)
    return jnp.concatenate([a, b], axis=-1)
```

```python
import functools

import jax
import jax.numpy as jnp
from jax import lax
import jax.experimental.pallas as pl
import jax.experimental.pallas.tpu as pltpu

F32 = jnp.float32
BF16 = jnp.bfloat16

S = 2048
D = 640
NT = D // 128
A_H = 32
A_DH = D // A_H
A_W = 8
A_DIL = 2
A_HALO = 16
B_H = 32
B_DH = 192
MEM = 8
SEG = 32
NSEG = S // SEG
NP = B_H // 2
PW = 2 * B_DH
FRESH = SEG - MEM
L = MEM + SEG
NEG = -1000000000.0
NSLOT = 3
EP_CHUNKS = 4


def _nt_dot(a, b):
    return lax.dot_general(a, b, (((1,), (1,)), ((), ())), preferred_element_type=F32)


def _dot(a, b):
    return jnp.dot(a, b, preferred_element_type=F32)


def _kernel(ax_hbm, awqkv_hbm, awo_hbm, bx_hbm, bx4_hbm, mem0_hbm, wq_hbm, wk_hbm, wv_hbm, wo_hbm,
            out_hbm,
            stage, wa_stage, w_s, wo_s, pre_s, odef_s, ob_s, out_s,
            xa_s, xb_s, xpre_s, mem0_s, wa_s, awo_raw, awo_s, t1_s, t2_s, kv_s,
            ring_sem, misc_sem, out_sem):
    def ring_copies(p, slot):
        rows = pl.ds(pl.multiple_of(p * PW, PW), PW)
        piece = jnp.minimum(p, 3 * NT - 1)
        c = piece // NT
        kt = piece % NT
        return [
            pltpu.make_async_copy(wq_hbm.at[rows, :], stage.at[slot, 0], ring_sem.at[slot, 0]),
            pltpu.make_async_copy(wk_hbm.at[rows, :], stage.at[slot, 1], ring_sem.at[slot, 1]),
            pltpu.make_async_copy(wv_hbm.at[rows, :], stage.at[slot, 2], ring_sem.at[slot, 2]),
            pltpu.make_async_copy(
                awqkv_hbm.at[pl.ds(pl.multiple_of(kt * 128, 128), 128),
                             pl.ds(pl.multiple_of(c * D, 128), D)],
                wa_stage.at[slot], ring_sem.at[slot, 3]),
        ]

    def extra_copies(p):
        r1 = pl.ds(pl.multiple_of(p * PW, PW), PW)
        r2 = pl.ds(pl.multiple_of(p * (S // NP), S // NP), S // NP)
        return [
            pltpu.make_async_copy(wo_hbm.at[r1, :], wo_s.at[r1, :], misc_sem.at[0]),
            pltpu.make_async_copy(ax_hbm.at[r2, :], xa_s.at[r2, :], misc_sem.at[1]),
            pltpu.make_async_copy(bx_hbm.at[r2, :], xb_s.at[r2, :], misc_sem.at[2]),
        ]

    xpre_cp = pltpu.make_async_copy(bx4_hbm.at[:, 3], xpre_s, misc_sem.at[3])
    mem_cp = pltpu.make_async_copy(mem0_hbm, mem0_s, misc_sem.at[4])
    awo_cp = pltpu.make_async_copy(awo_hbm, awo_raw, misc_sem.at[5])

    xpre_cp.start()
    for cp in ring_copies(0, 0):
        cp.start()
    for cp in ring_copies(1, 1):
        cp.start()
    mem_cp.start()
    awo_cp.start()
    xpre_cp.wait()

    def prologue(p, carry):
        slot = p % NSLOT
        for cp in ring_copies(p, slot):
            cp.wait()

        @pl.when(p + 2 < NP)
        def _():
            for cp in ring_copies(p + 2, (p + 2) % NSLOT):
                cp.start()

        for cp in extra_copies(p):
            cp.start()

        xp = xpre_s[...].reshape(NSEG * MEM, D)
        for m in range(3):
            wt = stage[slot, m]
            w_s[p, :, m * PW:(m + 1) * PW] = wt.T
            pre_s[p, :, m * PW:(m + 1) * PW] = _nt_dot(xp, wt)

        piece = jnp.minimum(p, 3 * NT - 1)
        t1_s[...] = wa_stage[slot].astype(F32).T
        for d in range(A_DH):
            t2_s[d * A_H:(d + 1) * A_H, :] = t1_s[pl.ds(d, A_H, stride=A_DH), :]
        wa_s[piece // NT, pl.ds(pl.multiple_of((piece % NT) * 128, 128), 128), :] = (
            t2_s[...].T.astype(BF16))
        return carry

    lax.fori_loop(0, NP, prologue, 0)

    awo_cp.wait()
    mem_cp.wait()
    for j in range(NT):
        t1_s[...] = awo_raw[:, j * 128:(j + 1) * 128].astype(F32)
        for d in range(A_DH):
            awo_s[d * A_H:(d + 1) * A_H, j * 128:(j + 1) * 128] = (
                t1_s[pl.ds(d, A_H, stride=A_DH), :].astype(BF16))
    kv_s[...] = jnp.zeros_like(kv_s)

    def wait_extra(p, carry):
        for cp in extra_copies(p):
            cp.wait()
        return carry

    lax.fori_loop(0, NP, wait_extra, 0)

    b_scale = B_DH ** (-0.5)
    a_scale = A_DH ** (-0.5)

    def step(s, mem):
        row0 = pl.multiple_of(s * SEG, SEG)

        qi = lax.broadcasted_iota(jnp.int32, (L, 2 * L), 0)
        kl = lax.broadcasted_iota(jnp.int32, (L, 2 * L), 1)
        qpos = jnp.where(qi < FRESH, qi + MEM, jnp.where(qi < SEG, qi - FRESH, qi))
        kf = kl % SEG
        kpos_f = jnp.where(kf < FRESH, kf + MEM, kf - FRESH)
        kpos = jnp.where(kl < 2 * SEG, kpos_f, SEG + kl % MEM)
        allowed = (qpos < MEM) | (qpos >= kpos)
        is_a = (kl < SEG) | ((kl >= 2 * SEG) & (kl < 2 * SEG + MEM))
        col = lax.broadcasted_iota(jnp.int32, (1, PW), 1)
        col_a = col < B_DH

        xa = xa_s[pl.ds(row0, SEG), :]
        qa = _dot(xa, wa_s[0])
        ka = _dot(xa, wa_s[1])
        va = _dot(xa, wa_s[2])

        xb = xb_s[pl.ds(row0, SEG), :].astype(F32)
        h = jnp.concatenate([xb[:FRESH], mem], axis=0).astype(BF16)
        pre_rows = pl.ds(pl.multiple_of(s * MEM, MEM), MEM)

        def block_diag(fresh, pre):
            z = jnp.zeros_like(fresh)
            zp = jnp.zeros_like(pre)
            return jnp.concatenate([
                jnp.where(col_a, fresh, z), jnp.where(col_a, z, fresh),
                jnp.where(col_a, pre, zp), jnp.where(col_a, zp, pre)], axis=0).astype(BF16)

        def proj(p):
            f = _dot(h, w_s[p])
            g = pre_s[p, pre_rows, :]
            q = jnp.concatenate([f[:, :PW], g[:, :PW]], axis=0).astype(BF16)
            kbd = block_diag(f[:, PW:2 * PW], g[:, PW:2 * PW])
            vbd = block_diag(f[:, 2 * PW:], g[:, 2 * PW:])
            return q, kbd, vbd

        def scores(q, kbd):
            sc = _nt_dot(q, kbd) * b_scale
            sc = jnp.where(allowed, sc, NEG)
            ninf = jnp.float32(-jnp.inf)
            ma = jnp.max(jnp.where(is_a, sc, ninf), axis=1, keepdims=True)
            mb = jnp.max(jnp.where(is_a, ninf, sc), axis=1, keepdims=True)
            e = jnp.exp(sc - jnp.where(is_a, ma, mb))
            sa = jnp.sum(jnp.where(is_a, e, 0.0), axis=1, keepdims=True)
            sb = jnp.sum(jnp.where(is_a, 0.0, e), axis=1, keepdims=True)
            return (e / jnp.where(is_a, sa, sb)).astype(BF16)

        def pv_out(p, pr, vbd, acc):
            o = _dot(pr, vbd)
            odef_s[pre_rows, p * PW:(p + 1) * PW] = o[SEG:]
            contrib = _dot(o[:SEG].astype(BF16), wo_s[p * PW:(p + 1) * PW, :])
            return contrib if acc is None else acc + contrib

        def local_attention():
            kwin = jnp.concatenate([kv_s[0], ka], axis=0)
            vwin = jnp.concatenate([kv_s[1], va], axis=0)
            kv_s[0] = ka[SEG - A_HALO:]
            kv_s[1] = va[SEG - A_HALO:]
            pos = row0 + lax.broadcasted_iota(jnp.int32, (SEG, 128), 0)
            logits = []
            for w in range(A_W):
                lo = A_HALO - A_DIL * w
                prod = qa * kwin[lo:lo + SEG]
                t = prod[:, :128]
                for j in range(1, NT):
                    t = t + prod[:, j * 128:(j + 1) * 128]
                t = t + pltpu.roll(t, 64, 1)
                t = t + pltpu.roll(t, 32, 1)
                logits.append(jnp.where(pos >= A_DIL * w, t * a_scale, NEG))
            mx = functools.reduce(jnp.maximum, logits)
            es = [jnp.exp(l - mx) for l in logits]
            inv = 1.0 / functools.reduce(lambda u, v: u + v, es)
            outs = []
            for j in range(NT):
                o = None
                for w in range(A_W):
                    lo = A_HALO - A_DIL * w
                    term = es[w] * vwin[lo:lo + SEG, j * 128:(j + 1) * 128]
                    o = term if o is None else o + term
                outs.append(o * inv)
            return jnp.concatenate(outs, axis=1).astype(BF16)

        qkv = {}
        probs = {}
        acc = None
        oa = None
        for t in range(NP + 2):
            if t < NP:
                qkv[t] = proj(t)
            if 1 <= t <= NP:
                probs[t - 1] = scores(qkv[t - 1][0], qkv[t - 1][1])
            if t == 2:
                oa = local_attention()
            if t == NP + 1:
                out_s[pl.ds(row0, SEG), :D] = _dot(oa, awo_s[...]).astype(BF16)
            if t >= 2:
                acc = pv_out(t - 2, probs[t - 2], qkv[t - 2][2], acc)

        ob_s[s, :FRESH, :] = acc[:FRESH]
        return acc[FRESH:]

    lax.fori_loop(0, NSEG, step, mem0_s[...].astype(F32))

    segs = NSEG // EP_CHUNKS
    rows = S // EP_CHUNKS

    def out_copy(c):
        r = pl.ds(pl.multiple_of(c * rows, rows), rows)
        return pltpu.make_async_copy(out_s.at[r, :], out_hbm.at[r, :], out_sem.at[c])

    def epilogue(c, carry):
        od = odef_s[pl.ds(pl.multiple_of(c * segs * MEM, segs * MEM), segs * MEM), :].astype(BF16)
        res = _dot(od, wo_s[...])
        sg = pl.ds(pl.multiple_of(c * segs, segs), segs)
        ob_s[sg, FRESH:, :] = res.reshape(segs, MEM, D)
        out_s[pl.ds(pl.multiple_of(c * rows, rows), rows), D:] = (
            ob_s[sg].reshape(rows, D).astype(BF16))
        out_copy(c).start()
        return carry

    lax.fori_loop(0, EP_CHUNKS, epilogue, 0)
    for c in range(EP_CHUNKS):
        out_copy(c).wait()


@functools.partial(jax.jit, static_argnames=("B_seg_len",))
def pallas_concat_heads__sliding_local_dilated__memory_aug_recurrent_mem_tr__prompt_kernel(
    A_x: jax.Array,
    A_wqkv: jax.Array,
    A_wo: jax.Array,
    B_x: jax.Array,
    B_mem0: jax.Array,
    B_Wq: jax.Array,
    B_Wk: jax.Array,
    B_Wv: jax.Array,
    B_Wo: jax.Array,
    B_seg_len,
):
    assert B_seg_len == SEG
    assert A_x.shape == (1, S, D) and B_x.shape == (1, S, D)
    hd = B_H * B_DH
    wq_t = jnp.transpose(B_Wq, (1, 2, 0)).reshape(hd, D)
    wk_t = jnp.transpose(B_Wk, (1, 2, 0)).reshape(hd, D)
    wv_t = jnp.transpose(B_Wv, (1, 2, 0)).reshape(hd, D)
    wo = B_Wo.reshape(hd, D)

    any_spec = pl.BlockSpec(memory_space=pl.ANY)
    out = pl.pallas_call(
        _kernel,
        out_shape=jax.ShapeDtypeStruct((S, 2 * D), BF16),
        in_specs=[any_spec] * 10,
        out_specs=any_spec,
        scratch_shapes=[
            pltpu.VMEM((NSLOT, 3, PW, D), BF16),
            pltpu.VMEM((NSLOT, 128, D), BF16),
            pltpu.VMEM((NP, D, 3 * PW), BF16),
            pltpu.VMEM((hd, D), BF16),
            pltpu.VMEM((NP, NSEG * MEM, 3 * PW), F32),
            pltpu.VMEM((NSEG * MEM, hd), F32),
            pltpu.VMEM((NSEG, SEG, D), F32),
            pltpu.VMEM((S, 2 * D), BF16),
            pltpu.VMEM((S, D), BF16),
            pltpu.VMEM((S, D), BF16),
            pltpu.VMEM((NSEG, MEM, D), BF16),
            pltpu.VMEM((MEM, D), BF16),
            pltpu.VMEM((3, D, D), BF16),
            pltpu.VMEM((D, D), BF16),
            pltpu.VMEM((D, D), BF16),
            pltpu.VMEM((D, 128), F32),
            pltpu.VMEM((D, 128), F32),
            pltpu.VMEM((2, A_HALO, D), F32),
            pltpu.SemaphoreType.DMA((NSLOT, 4)),
            pltpu.SemaphoreType.DMA((6,)),
            pltpu.SemaphoreType.DMA((EP_CHUNKS,)),
        ],
        compiler_params=pltpu.CompilerParams(vmem_limit_bytes=120 * 1024 * 1024),
    )(A_x.reshape(S, D), A_wqkv, A_wo, B_x.reshape(S, D), B_x.reshape(NSEG, SEG // MEM, MEM, D),
      B_mem0.reshape(MEM, D), wq_t, wk_t, wv_t, wo)
    return out.reshape(1, S, 2 * D)
```

```python
import functools

import jax
import jax.numpy as jnp
from jax import lax
import jax.experimental.pallas as pl
import jax.experimental.pallas.tpu as pltpu

F32 = jnp.float32
BF16 = jnp.bfloat16

S = 2048
D = 640
NT = D // 128
A_H = 32
A_DH = D // A_H
A_W = 8
A_DIL = 2
A_HALO = 16
B_H = 32
B_DH = 192
MEM = 8
SEG = 32
NSEG = S // SEG
NP = B_H // 2
PW = 2 * B_DH
FRESH = SEG - MEM
L = MEM + SEG
NEG = -1000000000.0
NSLOT = 3
EP_CHUNKS = 4


def _nt_dot(a, b):
    return lax.dot_general(a, b, (((1,), (1,)), ((), ())), preferred_element_type=F32)


def _dot(a, b):
    return jnp.dot(a, b, preferred_element_type=F32)


def _kernel(ax_hbm, awqkv_hbm, awo_hbm, bx_hbm, bx4_hbm, mem0_hbm, wq_hbm, wk_hbm, wv_hbm, wo_hbm,
            out_hbm,
            stage, wa_stage, w_s, wo_s, pre_s, odef_s, ob_s, out_s,
            xa_s, xb_s, xpre_s, mem0_s, wa_s, awo_raw, awo_s, t1_s, t2_s, qa_s, kv_s,
            ring_sem, misc_sem, out_sem):
    def ring_copies(p, slot):
        rows = pl.ds(pl.multiple_of(p * PW, PW), PW)
        piece = jnp.minimum(p, 3 * NT - 1)
        c = piece // NT
        kt = piece % NT
        return [
            pltpu.make_async_copy(wq_hbm.at[rows, :], stage.at[slot, 0], ring_sem.at[slot, 0]),
            pltpu.make_async_copy(wk_hbm.at[rows, :], stage.at[slot, 1], ring_sem.at[slot, 1]),
            pltpu.make_async_copy(wv_hbm.at[rows, :], stage.at[slot, 2], ring_sem.at[slot, 2]),
            pltpu.make_async_copy(
                awqkv_hbm.at[pl.ds(pl.multiple_of(kt * 128, 128), 128),
                             pl.ds(pl.multiple_of(c * D, 128), D)],
                wa_stage.at[slot], ring_sem.at[slot, 3]),
        ]

    def extra_copies(p):
        r1 = pl.ds(pl.multiple_of(p * PW, PW), PW)
        r2 = pl.ds(pl.multiple_of(p * (S // NP), S // NP), S // NP)
        return [
            pltpu.make_async_copy(wo_hbm.at[r1, :], wo_s.at[r1, :], misc_sem.at[0]),
            pltpu.make_async_copy(ax_hbm.at[r2, :], xa_s.at[r2, :], misc_sem.at[1]),
            pltpu.make_async_copy(bx_hbm.at[r2, :], xb_s.at[r2, :], misc_sem.at[2]),
        ]

    xpre_cp = pltpu.make_async_copy(bx4_hbm.at[:, 3], xpre_s, misc_sem.at[3])
    mem_cp = pltpu.make_async_copy(mem0_hbm, mem0_s, misc_sem.at[4])
    awo_cp = pltpu.make_async_copy(awo_hbm, awo_raw, misc_sem.at[5])

    xpre_cp.start()
    for cp in ring_copies(0, 0):
        cp.start()
    for cp in ring_copies(1, 1):
        cp.start()
    mem_cp.start()
    awo_cp.start()
    xpre_cp.wait()

    def prologue(p, carry):
        slot = p % NSLOT
        for cp in ring_copies(p, slot):
            cp.wait()

        @pl.when(p + 2 < NP)
        def _():
            for cp in ring_copies(p + 2, (p + 2) % NSLOT):
                cp.start()

        for cp in extra_copies(p):
            cp.start()

        xp = xpre_s[...].reshape(NSEG * MEM, D)
        for m in range(3):
            wt = stage[slot, m]
            w_s[p, :, m * PW:(m + 1) * PW] = wt.T
            pre_s[p, :, m * PW:(m + 1) * PW] = _nt_dot(xp, wt)

        piece = jnp.minimum(p, 3 * NT - 1)
        t1_s[...] = wa_stage[slot].astype(F32).T
        for d in range(A_DH):
            t2_s[d * A_H:(d + 1) * A_H, :] = t1_s[pl.ds(d, A_H, stride=A_DH), :]
        wa_s[piece // NT, pl.ds(pl.multiple_of((piece % NT) * 128, 128), 128), :] = (
            t2_s[...].T.astype(BF16))
        return carry

    lax.fori_loop(0, NP, prologue, 0)

    awo_cp.wait()
    mem_cp.wait()
    for j in range(NT):
        t1_s[...] = awo_raw[:, j * 128:(j + 1) * 128].astype(F32)
        for d in range(A_DH):
            awo_s[d * A_H:(d + 1) * A_H, j * 128:(j + 1) * 128] = (
                t1_s[pl.ds(d, A_H, stride=A_DH), :].astype(BF16))

    def wait_extra(p, carry):
        for cp in extra_copies(p):
            cp.wait()
        return carry

    lax.fori_loop(0, NP, wait_extra, 0)

    xa0 = xa_s[:SEG, :]
    qa_s[...] = _dot(xa0, wa_s[0])
    kv_s[:, :A_HALO, :] = jnp.zeros((2, A_HALO, D), F32)
    kv_s[0, A_HALO:, :] = _dot(xa0, wa_s[1])
    kv_s[1, A_HALO:, :] = _dot(xa0, wa_s[2])

    b_scale = B_DH ** (-0.5)
    a_scale = A_DH ** (-0.5)

    def step(s, mem):
        row0 = pl.multiple_of(s * SEG, SEG)

        qi = lax.broadcasted_iota(jnp.int32, (L, 2 * L), 0)
        kl = lax.broadcasted_iota(jnp.int32, (L, 2 * L), 1)
        qpos = jnp.where(qi < FRESH, qi + MEM, jnp.where(qi < SEG, qi - FRESH, qi))
        kf = kl % SEG
        kpos_f = jnp.where(kf < FRESH, kf + MEM, kf - FRESH)
        kpos = jnp.where(kl < 2 * SEG, kpos_f, SEG + kl % MEM)
        allowed = (qpos < MEM) | (qpos >= kpos)
        is_a = (kl < SEG) | ((kl >= 2 * SEG) & (kl < 2 * SEG + MEM))
        col = lax.broadcasted_iota(jnp.int32, (1, PW), 1)
        col_a = col < B_DH

        col128_a = lax.broadcasted_iota(jnp.int32, (1, 128), 1) < (B_DH - 128)

        xb = xb_s[pl.ds(row0, SEG), :].astype(F32)
        h = jnp.concatenate([xb[:FRESH], mem], axis=0).astype(BF16)
        pre_rows = pl.ds(pl.multiple_of(s * MEM, MEM), MEM)

        def block_diag(fresh, pre):
            z = jnp.zeros_like(fresh)
            zp = jnp.zeros_like(pre)
            return jnp.concatenate([
                jnp.where(col_a, fresh, z), jnp.where(col_a, z, fresh),
                jnp.where(col_a, pre, zp), jnp.where(col_a, zp, pre)], axis=0).astype(BF16)

        def proj(p):
            f = _dot(h, w_s[p])
            g = pre_s[p, pre_rows, :]
            q = jnp.concatenate([f[:, :PW], g[:, :PW]], axis=0).astype(BF16)
            kbd = block_diag(f[:, PW:2 * PW], g[:, PW:2 * PW])
            vbd = block_diag(f[:, 2 * PW:], g[:, 2 * PW:])
            return q, kbd, vbd

        def scores(q, kbd):
            sc = _nt_dot(q, kbd) * b_scale
            sc = jnp.where(allowed, sc, NEG)
            ninf = jnp.float32(-jnp.inf)
            ma = jnp.max(jnp.where(is_a, sc, ninf), axis=1, keepdims=True)
            mb = jnp.max(jnp.where(is_a, ninf, sc), axis=1, keepdims=True)
            e = jnp.exp(sc - jnp.where(is_a, ma, mb))
            ra = 1.0 / jnp.sum(jnp.where(is_a, e, 0.0), axis=1, keepdims=True)
            rb = 1.0 / jnp.sum(jnp.where(is_a, 0.0, e), axis=1, keepdims=True)
            return e.astype(BF16), ra, rb

        def pv(p, sm, vbd):
            e, ra, rb = sm
            o = _dot(e, vbd)
            o = jnp.concatenate([
                o[:, :128] * ra,
                o[:, 128:256] * jnp.where(col128_a, ra, rb),
                o[:, 256:] * rb], axis=1)
            odef_s[pre_rows, p * PW:(p + 1) * PW] = o[SEG:]
            return o[:SEG].astype(BF16)

        def wout(p, o, acc):
            contrib = _dot(o, wo_s[p * PW:(p + 1) * PW, :])
            return contrib if acc is None else acc + contrib

        def local_attention():
            qa = qa_s[...]
            kwin = kv_s[0]
            vwin = kv_s[1]
            pos = row0 + lax.broadcasted_iota(jnp.int32, (SEG, 128), 0)
            logits = []
            for w in range(A_W):
                lo = A_HALO - A_DIL * w
                prod = qa * kwin[lo:lo + SEG]
                t = prod[:, :128]
                for j in range(1, NT):
                    t = t + prod[:, j * 128:(j + 1) * 128]
                t = t + pltpu.roll(t, 64, 1)
                t = t + pltpu.roll(t, 32, 1)
                logits.append(jnp.where(pos >= A_DIL * w, t * a_scale, NEG))
            mx = functools.reduce(jnp.maximum, logits)
            es = [jnp.exp(l - mx) for l in logits]
            inv = 1.0 / functools.reduce(lambda u, v: u + v, es)
            outs = []
            for j in range(NT):
                o = None
                for w in range(A_W):
                    lo = A_HALO - A_DIL * w
                    term = es[w] * vwin[lo:lo + SEG, j * 128:(j + 1) * 128]
                    o = term if o is None else o + term
                outs.append(o * inv)
            kv_s[0, :A_HALO, :] = kwin[SEG:]
            kv_s[1, :A_HALO, :] = vwin[SEG:]
            return jnp.concatenate(outs, axis=1).astype(BF16)

        nxt = pl.multiple_of(jnp.minimum(s + 1, NSEG - 1) * SEG, SEG)

        def a_proj(m):
            r = _dot(xa_s[pl.ds(nxt, SEG), :], wa_s[m])
            if m == 0:
                qa_s[...] = r
            else:
                kv_s[m - 1, A_HALO:, :] = r

        order = []
        for t in range(NP):
            order.append(("P", t))
            if t >= 1:
                order.append(("S", t - 1))
            if t >= 2:
                order.append(("V", t - 2))
            if t >= 3:
                order.append(("W", t - 3))
            if t == 2:
                order.append(("LA", 0))
        order += [("S", NP - 1), ("AP", 0), ("V", NP - 2), ("W", NP - 3), ("V", NP - 1),
                  ("W", NP - 2), ("AP", 1), ("W", NP - 1), ("AP", 2), ("AO", 0)]

        qkv, sm, ov = {}, {}, {}
        acc = None
        oa = None
        for kind, t in order:
            if kind == "P":
                qkv[t] = proj(t)
            elif kind == "S":
                sm[t] = scores(qkv[t][0], qkv[t][1])
            elif kind == "V":
                ov[t] = pv(t, sm[t], qkv[t][2])
            elif kind == "W":
                acc = wout(t, ov[t], acc)
            elif kind == "LA":
                oa = local_attention()
            elif kind == "AP":
                a_proj(t)
            elif kind == "AO":
                out_s[pl.ds(row0, SEG), :D] = _dot(oa, awo_s[...]).astype(BF16)

        ob_s[s, :FRESH, :] = acc[:FRESH]
        return acc[FRESH:]

    lax.fori_loop(0, NSEG, step, mem0_s[...].astype(F32))

    segs = NSEG // EP_CHUNKS
    rows = S // EP_CHUNKS

    def out_copy(c):
        r = pl.ds(pl.multiple_of(c * rows, rows), rows)
        return pltpu.make_async_copy(out_s.at[r, :], out_hbm.at[r, :], out_sem.at[c])

    def epilogue(c, carry):
        od = odef_s[pl.ds(pl.multiple_of(c * segs * MEM, segs * MEM), segs * MEM), :].astype(BF16)
        res = _dot(od, wo_s[...])
        sg = pl.ds(pl.multiple_of(c * segs, segs), segs)
        ob_s[sg, FRESH:, :] = res.reshape(segs, MEM, D)
        out_s[pl.ds(pl.multiple_of(c * rows, rows), rows), D:] = (
            ob_s[sg].reshape(rows, D).astype(BF16))
        out_copy(c).start()
        return carry

    lax.fori_loop(0, EP_CHUNKS, epilogue, 0)
    for c in range(EP_CHUNKS):
        out_copy(c).wait()


@functools.partial(jax.jit, static_argnames=("B_seg_len",))
def pallas_concat_heads__sliding_local_dilated__memory_aug_recurrent_mem_tr__prompt_kernel(
    A_x: jax.Array,
    A_wqkv: jax.Array,
    A_wo: jax.Array,
    B_x: jax.Array,
    B_mem0: jax.Array,
    B_Wq: jax.Array,
    B_Wk: jax.Array,
    B_Wv: jax.Array,
    B_Wo: jax.Array,
    B_seg_len,
):
    assert B_seg_len == SEG
    assert A_x.shape == (1, S, D) and B_x.shape == (1, S, D)
    hd = B_H * B_DH
    wq_t = jnp.transpose(B_Wq, (1, 2, 0)).reshape(hd, D)
    wk_t = jnp.transpose(B_Wk, (1, 2, 0)).reshape(hd, D)
    wv_t = jnp.transpose(B_Wv, (1, 2, 0)).reshape(hd, D)
    wo = B_Wo.reshape(hd, D)

    any_spec = pl.BlockSpec(memory_space=pl.ANY)
    out = pl.pallas_call(
        _kernel,
        out_shape=jax.ShapeDtypeStruct((S, 2 * D), BF16),
        in_specs=[any_spec] * 10,
        out_specs=any_spec,
        scratch_shapes=[
            pltpu.VMEM((NSLOT, 3, PW, D), BF16),
            pltpu.VMEM((NSLOT, 128, D), BF16),
            pltpu.VMEM((NP, D, 3 * PW), BF16),
            pltpu.VMEM((hd, D), BF16),
            pltpu.VMEM((NP, NSEG * MEM, 3 * PW), F32),
            pltpu.VMEM((NSEG * MEM, hd), F32),
            pltpu.VMEM((NSEG, SEG, D), F32),
            pltpu.VMEM((S, 2 * D), BF16),
            pltpu.VMEM((S, D), BF16),
            pltpu.VMEM((S, D), BF16),
            pltpu.VMEM((NSEG, MEM, D), BF16),
            pltpu.VMEM((MEM, D), BF16),
            pltpu.VMEM((3, D, D), BF16),
            pltpu.VMEM((D, D), BF16),
            pltpu.VMEM((D, D), BF16),
            pltpu.VMEM((D, 128), F32),
            pltpu.VMEM((D, 128), F32),
            pltpu.VMEM((SEG, D), F32),
            pltpu.VMEM((2, A_HALO + SEG, D), F32),
            pltpu.SemaphoreType.DMA((NSLOT, 4)),
            pltpu.SemaphoreType.DMA((6,)),
            pltpu.SemaphoreType.DMA((EP_CHUNKS,)),
        ],
        compiler_params=pltpu.CompilerParams(vmem_limit_bytes=120 * 1024 * 1024),
    )(A_x.reshape(S, D), A_wqkv, A_wo, B_x.reshape(S, D), B_x.reshape(NSEG, SEG // MEM, MEM, D),
      B_mem0.reshape(MEM, D), wq_t, wk_t, wv_t, wo)
    return out.reshape(1, S, 2 * D)
```

```python
import functools

import jax
import jax.numpy as jnp
from jax import lax
import jax.experimental.pallas as pl
import jax.experimental.pallas.tpu as pltpu

F32 = jnp.float32
BF16 = jnp.bfloat16

S = 2048
D = 640
NT = D // 128
A_H = 32
A_DH = D // A_H
A_W = 8
A_DIL = 2
A_HALO = 16
B_H = 32
B_DH = 192
MEM = 8
SEG = 32
NSEG = S // SEG
NP = B_H // 2
PW = 2 * B_DH
FRESH = SEG - MEM
L = MEM + SEG
NEG = -1000000000.0
NSLOT = 3
EP_CHUNKS = 4
N_STEPS = NSEG


def _nt_dot(a, b):
    return lax.dot_general(a, b, (((1,), (1,)), ((), ())), preferred_element_type=F32)


def _dot(a, b):
    return jnp.dot(a, b, preferred_element_type=F32)


def _recip(x):
    r = pl.reciprocal(x, approx=True)
    return r * (2.0 - x * r)


def _kernel(ax_hbm, awqkv_hbm, awo_hbm, bx_hbm, bx4_hbm, mem0_hbm, wq_hbm, wk_hbm, wv_hbm, wo_hbm,
            out_hbm,
            stage, wa_stage, w_s, wo_s, pre_s, odef_s, ob_s, out_s,
            xa_s, xb_s, xpre_s, mem0_s, wa_s, awo_raw, awo_s, t1_s, t2_s, qa_s, kv_s,
            ring_sem, misc_sem, out_sem):
    def ring_copies(p, slot):
        rows = pl.ds(pl.multiple_of(p * PW, PW), PW)
        piece = jnp.minimum(p, 3 * NT - 1)
        c = piece // NT
        kt = piece % NT
        return [
            pltpu.make_async_copy(wq_hbm.at[rows, :], stage.at[slot, 0], ring_sem.at[slot, 0]),
            pltpu.make_async_copy(wk_hbm.at[rows, :], stage.at[slot, 1], ring_sem.at[slot, 1]),
            pltpu.make_async_copy(wv_hbm.at[rows, :], stage.at[slot, 2], ring_sem.at[slot, 2]),
            pltpu.make_async_copy(
                awqkv_hbm.at[pl.ds(pl.multiple_of(kt * 128, 128), 128),
                             pl.ds(pl.multiple_of(c * D, 128), D)],
                wa_stage.at[slot], ring_sem.at[slot, 3]),
        ]

    def extra_copies(p):
        r1 = pl.ds(pl.multiple_of(p * PW, PW), PW)
        r2 = pl.ds(pl.multiple_of(p * (S // NP), S // NP), S // NP)
        return [
            pltpu.make_async_copy(wo_hbm.at[r1, :], wo_s.at[r1, :], misc_sem.at[0]),
            pltpu.make_async_copy(ax_hbm.at[r2, :], xa_s.at[r2, :], misc_sem.at[1]),
            pltpu.make_async_copy(bx_hbm.at[r2, :], xb_s.at[r2, :], misc_sem.at[2]),
        ]

    xpre_cp = pltpu.make_async_copy(bx4_hbm.at[:, 3], xpre_s, misc_sem.at[3])
    mem_cp = pltpu.make_async_copy(mem0_hbm, mem0_s, misc_sem.at[4])
    awo_cp = pltpu.make_async_copy(awo_hbm, awo_raw, misc_sem.at[5])

    xpre_cp.start()
    for cp in ring_copies(0, 0):
        cp.start()
    for cp in ring_copies(1, 1):
        cp.start()
    mem_cp.start()
    awo_cp.start()
    xpre_cp.wait()

    def prologue(p, carry):
        slot = p % NSLOT
        for cp in ring_copies(p, slot):
            cp.wait()

        @pl.when(p + 2 < NP)
        def _():
            for cp in ring_copies(p + 2, (p + 2) % NSLOT):
                cp.start()

        for cp in extra_copies(p):
            cp.start()

        xp = xpre_s[...].reshape(NSEG * MEM, D)
        for m in range(3):
            wt = stage[slot, m]
            w_s[p, :, m * PW:(m + 1) * PW] = wt.T
            pre_s[p, :, m * PW:(m + 1) * PW] = _nt_dot(xp, wt)

        piece = jnp.minimum(p, 3 * NT - 1)
        t1_s[...] = wa_stage[slot].astype(F32).T
        for d in range(A_DH):
            t2_s[d * A_H:(d + 1) * A_H, :] = t1_s[pl.ds(d, A_H, stride=A_DH), :]
        wa_s[piece // NT, pl.ds(pl.multiple_of((piece % NT) * 128, 128), 128), :] = (
            t2_s[...].T.astype(BF16))
        return carry

    lax.fori_loop(0, NP, prologue, 0)

    awo_cp.wait()
    mem_cp.wait()
    for j in range(NT):
        t1_s[...] = awo_raw[:, j * 128:(j + 1) * 128].astype(F32)
        for d in range(A_DH):
            awo_s[d * A_H:(d + 1) * A_H, j * 128:(j + 1) * 128] = (
                t1_s[pl.ds(d, A_H, stride=A_DH), :].astype(BF16))

    def wait_extra(p, carry):
        for cp in extra_copies(p):
            cp.wait()
        return carry

    lax.fori_loop(0, NP, wait_extra, 0)

    xa0 = xa_s[:SEG, :]
    qa_s[...] = _dot(xa0, wa_s[0])
    kv_s[:, :A_HALO, :] = jnp.zeros((2, A_HALO, D), F32)
    kv_s[0, A_HALO:, :] = _dot(xa0, wa_s[1])
    kv_s[1, A_HALO:, :] = _dot(xa0, wa_s[2])

    b_scale = B_DH ** (-0.5)
    a_scale = A_DH ** (-0.5)

    def step(s, mem):
        row0 = pl.multiple_of(s * SEG, SEG)

        qi = lax.broadcasted_iota(jnp.int32, (L, 2 * L), 0)
        kl = lax.broadcasted_iota(jnp.int32, (L, 2 * L), 1)
        qpos = jnp.where(qi < FRESH, qi + MEM, jnp.where(qi < SEG, qi - FRESH, qi))
        kf = kl % SEG
        kpos_f = jnp.where(kf < FRESH, kf + MEM, kf - FRESH)
        kpos = jnp.where(kl < 2 * SEG, kpos_f, SEG + kl % MEM)
        allowed = (qpos < MEM) | (qpos >= kpos)
        is_a = (kl < SEG) | ((kl >= 2 * SEG) & (kl < 2 * SEG + MEM))
        col = lax.broadcasted_iota(jnp.int32, (1, PW), 1)
        col_a = col < B_DH

        col128_a = lax.broadcasted_iota(jnp.int32, (1, 128), 1) < (B_DH - 128)

        xb = xb_s[pl.ds(row0, SEG), :].astype(F32)
        h = jnp.concatenate([xb[:FRESH], mem], axis=0).astype(BF16)
        pre_rows = pl.ds(pl.multiple_of(s * MEM, MEM), MEM)

        def block_diag(fresh, pre):
            z = jnp.zeros_like(fresh)
            zp = jnp.zeros_like(pre)
            return jnp.concatenate([
                jnp.where(col_a, fresh, z), jnp.where(col_a, z, fresh),
                jnp.where(col_a, pre, zp), jnp.where(col_a, zp, pre)], axis=0).astype(BF16)

        def proj(p):
            f = _dot(h, w_s[p])
            g = pre_s[p, pre_rows, :]
            q = jnp.concatenate([f[:, :PW], g[:, :PW]], axis=0).astype(BF16)
            kbd = block_diag(f[:, PW:2 * PW], g[:, PW:2 * PW])
            vbd = block_diag(f[:, 2 * PW:], g[:, 2 * PW:])
            return q, kbd, vbd

        def scores(q, kbd, late_norm):
            sc = _nt_dot(q, kbd) * b_scale
            sc = jnp.where(allowed, sc, NEG)
            ninf = jnp.float32(-jnp.inf)
            ma = jnp.max(jnp.where(is_a, sc, ninf), axis=1, keepdims=True)
            mb = jnp.max(jnp.where(is_a, ninf, sc), axis=1, keepdims=True)
            e = jnp.exp(sc - jnp.where(is_a, ma, mb))
            sa = jnp.sum(jnp.where(is_a, e, 0.0), axis=1, keepdims=True)
            sb = jnp.sum(jnp.where(is_a, 0.0, e), axis=1, keepdims=True)
            if late_norm:
                return e.astype(BF16), _recip(sa), _recip(sb)
            return (e * _recip(jnp.where(is_a, sa, sb))).astype(BF16), None, None

        def pv(p, sm, vbd):
            e, ra, rb = sm
            o = _dot(e, vbd)
            if ra is not None:
                o = jnp.concatenate([
                    o[:, :128] * ra,
                    o[:, 128:256] * jnp.where(col128_a, ra, rb),
                    o[:, 256:] * rb], axis=1)
            odef_s[pre_rows, p * PW:(p + 1) * PW] = o[SEG:]
            return o[:SEG].astype(BF16)

        def wout(p, o, acc):
            contrib = _dot(o, wo_s[p * PW:(p + 1) * PW, :])
            return contrib if acc is None else acc + contrib

        def local_attention():
            qa = qa_s[...]
            kwin = kv_s[0]
            vwin = kv_s[1]
            pos = row0 + lax.broadcasted_iota(jnp.int32, (SEG, 128), 0)
            logits = []
            for w in range(A_W):
                lo = A_HALO - A_DIL * w
                prod = qa * kwin[lo:lo + SEG]
                t = prod[:, :128]
                for j in range(1, NT):
                    t = t + prod[:, j * 128:(j + 1) * 128]
                t = t + pltpu.roll(t, 64, 1)
                t = t + pltpu.roll(t, 32, 1)
                logits.append(jnp.where(pos >= A_DIL * w, t * a_scale, NEG))
            mx = functools.reduce(jnp.maximum, logits)
            es = [jnp.exp(l - mx) for l in logits]
            inv = _recip(functools.reduce(lambda u, v: u + v, es))
            outs = []
            for j in range(NT):
                o = None
                for w in range(A_W):
                    lo = A_HALO - A_DIL * w
                    term = es[w] * vwin[lo:lo + SEG, j * 128:(j + 1) * 128]
                    o = term if o is None else o + term
                outs.append(o * inv)
            kv_s[0, :A_HALO, :] = kwin[SEG:]
            kv_s[1, :A_HALO, :] = vwin[SEG:]
            return jnp.concatenate(outs, axis=1).astype(BF16)

        nxt = pl.multiple_of(jnp.minimum(s + 1, NSEG - 1) * SEG, SEG)

        def a_proj(m):
            r = _dot(xa_s[pl.ds(nxt, SEG), :], wa_s[m])
            if m == 0:
                qa_s[...] = r
            else:
                kv_s[m - 1, A_HALO:, :] = r

        order = []
        for t in range(NP):
            order.append(("P", t))
            if t >= 1:
                order.append(("S", t - 1))
            if t >= 2:
                order.append(("V", t - 2))
            if t >= 3:
                order.append(("W", t - 3))
            if t == 2:
                order.append(("LA", 0))
            if t == 8:
                order.append(("AO", 0))
        order += [("S", NP - 1), ("AP", 0), ("V", NP - 2), ("W", NP - 3), ("V", NP - 1),
                  ("W", NP - 2), ("AP", 1), ("W", NP - 1), ("AP", 2)]

        qkv, sm, ov = {}, {}, {}
        acc = None
        oa = None
        for kind, t in order:
            if kind == "P":
                qkv[t] = proj(t)
            elif kind == "S":
                sm[t] = scores(qkv[t][0], qkv[t][1], t >= NP - 2)
            elif kind == "V":
                ov[t] = pv(t, sm[t], qkv[t][2])
            elif kind == "W":
                acc = wout(t, ov[t], acc)
            elif kind == "LA":
                oa = local_attention()
            elif kind == "AP":
                a_proj(t)
            elif kind == "AO":
                out_s[pl.ds(row0, SEG), :D] = _dot(oa, awo_s[...]).astype(BF16)

        ob_s[s, :FRESH, :] = acc[:FRESH]
        return acc[FRESH:]

    lax.fori_loop(0, N_STEPS, step, mem0_s[...].astype(F32))

    segs = NSEG // EP_CHUNKS
    rows = S // EP_CHUNKS

    def out_copy(c):
        r = pl.ds(pl.multiple_of(c * rows, rows), rows)
        return pltpu.make_async_copy(out_s.at[r, :], out_hbm.at[r, :], out_sem.at[c])

    def epilogue(c, carry):
        od = odef_s[pl.ds(pl.multiple_of(c * segs * MEM, segs * MEM), segs * MEM), :].astype(BF16)
        res = _dot(od, wo_s[...])
        sg = pl.ds(pl.multiple_of(c * segs, segs), segs)
        ob_s[sg, FRESH:, :] = res.reshape(segs, MEM, D)
        out_s[pl.ds(pl.multiple_of(c * rows, rows), rows), D:] = (
            ob_s[sg].reshape(rows, D).astype(BF16))
        out_copy(c).start()
        return carry

    lax.fori_loop(0, EP_CHUNKS, epilogue, 0)
    for c in range(EP_CHUNKS):
        out_copy(c).wait()


@functools.partial(jax.jit, static_argnames=("B_seg_len",))
def pallas_concat_heads__sliding_local_dilated__memory_aug_recurrent_mem_tr__prompt_kernel(
    A_x: jax.Array,
    A_wqkv: jax.Array,
    A_wo: jax.Array,
    B_x: jax.Array,
    B_mem0: jax.Array,
    B_Wq: jax.Array,
    B_Wk: jax.Array,
    B_Wv: jax.Array,
    B_Wo: jax.Array,
    B_seg_len,
):
    assert B_seg_len == SEG
    assert A_x.shape == (1, S, D) and B_x.shape == (1, S, D)
    hd = B_H * B_DH
    wq_t = jnp.transpose(B_Wq, (1, 2, 0)).reshape(hd, D)
    wk_t = jnp.transpose(B_Wk, (1, 2, 0)).reshape(hd, D)
    wv_t = jnp.transpose(B_Wv, (1, 2, 0)).reshape(hd, D)
    wo = B_Wo.reshape(hd, D)

    any_spec = pl.BlockSpec(memory_space=pl.ANY)
    out = pl.pallas_call(
        _kernel,
        out_shape=jax.ShapeDtypeStruct((S, 2 * D), BF16),
        in_specs=[any_spec] * 10,
        out_specs=any_spec,
        scratch_shapes=[
            pltpu.VMEM((NSLOT, 3, PW, D), BF16),
            pltpu.VMEM((NSLOT, 128, D), BF16),
            pltpu.VMEM((NP, D, 3 * PW), BF16),
            pltpu.VMEM((hd, D), BF16),
            pltpu.VMEM((NP, NSEG * MEM, 3 * PW), F32),
            pltpu.VMEM((NSEG * MEM, hd), F32),
            pltpu.VMEM((NSEG, SEG, D), F32),
            pltpu.VMEM((S, 2 * D), BF16),
            pltpu.VMEM((S, D), BF16),
            pltpu.VMEM((S, D), BF16),
            pltpu.VMEM((NSEG, MEM, D), BF16),
            pltpu.VMEM((MEM, D), BF16),
            pltpu.VMEM((3, D, D), BF16),
            pltpu.VMEM((D, D), BF16),
            pltpu.VMEM((D, D), BF16),
            pltpu.VMEM((D, 128), F32),
            pltpu.VMEM((D, 128), F32),
            pltpu.VMEM((SEG, D), F32),
            pltpu.VMEM((2, A_HALO + SEG, D), F32),
            pltpu.SemaphoreType.DMA((NSLOT, 4)),
            pltpu.SemaphoreType.DMA((6,)),
            pltpu.SemaphoreType.DMA((EP_CHUNKS,)),
        ],
        compiler_params=pltpu.CompilerParams(vmem_limit_bytes=120 * 1024 * 1024),
    )(A_x.reshape(S, D), A_wqkv, A_wo, B_x.reshape(S, D), B_x.reshape(NSEG, SEG // MEM, MEM, D),
      B_mem0.reshape(MEM, D), wq_t, wk_t, wv_t, wo)
    return out.reshape(1, S, 2 * D)
```

```python
import functools

import jax
import jax.numpy as jnp
from jax import lax
import jax.experimental.pallas as pl
import jax.experimental.pallas.tpu as pltpu

F32 = jnp.float32
BF16 = jnp.bfloat16

S = 2048
D = 640
NT = D // 128
A_H = 32
A_DH = D // A_H
A_W = 8
A_DIL = 2
A_HALO = 16
B_H = 32
B_DH = 192
MEM = 8
SEG = 32
NSEG = S // SEG
NP = B_H // 2
PW = 2 * B_DH
FRESH = SEG - MEM
L = MEM + SEG
NEG = -1000000000.0
NSLOT = 3
N_STEPS = NSEG // 2
U32 = jnp.uint32


def _nt_dot(a, b):
    return lax.dot_general(a, b, (((1,), (1,)), ((), ())), preferred_element_type=F32)


def _dot(a, b):
    return jnp.dot(a, b, preferred_element_type=F32)


def _pack(x):
    return pltpu.bitcast(x, U32)


def _unpack(x):
    return pltpu.bitcast(x, BF16)


def _recip(x):
    r = pl.reciprocal(x, approx=True)
    return r * (2.0 - x * r)


def _kernel(ax_hbm, awqkv_hbm, awo_hbm, bx_hbm, bx4_hbm, mem0_hbm, wq_hbm, wk_hbm, wv_hbm, wo_hbm,
            out_hbm,
            stage, wa_stage, w_s, wo_s, pre_s, odef_s, out_s,
            xa_s, xb_s, xpre_s, mem0_s, wa_s, awo_raw, awo_s, t1_s, t2_s, qa_s, kv_s,
            ring_sem, misc_sem, out_sem):
    def ring_copies(p, slot):
        rows = pl.ds(pl.multiple_of(p * PW, PW), PW)
        piece = jnp.minimum(p, 3 * NT - 1)
        c = piece // NT
        kt = piece % NT
        return [
            pltpu.make_async_copy(wq_hbm.at[rows, :], stage.at[slot, 0], ring_sem.at[slot, 0]),
            pltpu.make_async_copy(wk_hbm.at[rows, :], stage.at[slot, 1], ring_sem.at[slot, 1]),
            pltpu.make_async_copy(wv_hbm.at[rows, :], stage.at[slot, 2], ring_sem.at[slot, 2]),
            pltpu.make_async_copy(wo_hbm.at[rows, :], stage.at[slot, 3], ring_sem.at[slot, 4]),
            pltpu.make_async_copy(
                awqkv_hbm.at[pl.ds(pl.multiple_of(kt * 128, 128), 128),
                             pl.ds(pl.multiple_of(c * D, 128), D)],
                wa_stage.at[slot], ring_sem.at[slot, 3]),
        ]

    def extra_copies(p):
        r2 = pl.ds(pl.multiple_of(p * (S // NP), S // NP), S // NP)
        return [
            pltpu.make_async_copy(ax_hbm.at[r2, :], xa_s.at[r2, :], misc_sem.at[1]),
            pltpu.make_async_copy(bx_hbm.at[r2, :], xb_s.at[r2, :], misc_sem.at[2]),
        ]

    xpre_cp = pltpu.make_async_copy(bx4_hbm.at[:, 3], xpre_s, misc_sem.at[3])
    mem_cp = pltpu.make_async_copy(mem0_hbm, mem0_s, misc_sem.at[4])
    awo_cp = pltpu.make_async_copy(awo_hbm, awo_raw, misc_sem.at[5])

    xpre_cp.start()
    for cp in ring_copies(0, 0):
        cp.start()
    for cp in ring_copies(1, 1):
        cp.start()
    mem_cp.start()
    awo_cp.start()
    xpre_cp.wait()

    def prologue(p, carry):
        slot = p % NSLOT
        for cp in ring_copies(p, slot):
            cp.wait()

        @pl.when(p + 2 < NP)
        def _():
            for cp in ring_copies(p + 2, (p + 2) % NSLOT):
                cp.start()

        for cp in extra_copies(p):
            cp.start()

        xp = xpre_s[...].reshape(NSEG * MEM, D)
        for m in range(3):
            wt = stage[slot, m]
            w_s[p, :, m * PW:(m + 1) * PW] = _pack(wt.T)
            pre_s[p, :, m * PW:(m + 1) * PW] = _nt_dot(xp, wt)
        wo_s[p] = _pack(stage[slot, 3])

        piece = jnp.minimum(p, 3 * NT - 1)
        t1_s[...] = wa_stage[slot].astype(F32).T
        for d in range(A_DH):
            t2_s[d * A_H:(d + 1) * A_H, :] = t1_s[pl.ds(d, A_H, stride=A_DH), :]
        wa_s[piece // NT, pl.ds(pl.multiple_of((piece % NT) * 64, 64), 64), :] = (
            _pack(t2_s[...].T.astype(BF16)))
        return carry

    lax.fori_loop(0, NP, prologue, 0)

    awo_cp.wait()
    mem_cp.wait()
    for j in range(NT):
        t1_s[...] = awo_raw[:, j * 128:(j + 1) * 128].astype(F32)
        for d in range(A_DH):
            awo_s[d * A_H // 2:(d + 1) * A_H // 2, j * 128:(j + 1) * 128] = (
                _pack(t1_s[pl.ds(d, A_H, stride=A_DH), :].astype(BF16)))

    def wait_extra(p, carry):
        for cp in extra_copies(p):
            cp.wait()
        return carry

    lax.fori_loop(0, NP, wait_extra, 0)

    xa0 = xa_s[:SEG, :]
    qa_s[...] = _dot(xa0, _unpack(wa_s[0]))
    kv_s[:, :A_HALO, :] = jnp.zeros((2, A_HALO, D), F32)
    kv_s[0, A_HALO:, :] = _dot(xa0, _unpack(wa_s[1]))
    kv_s[1, A_HALO:, :] = _dot(xa0, _unpack(wa_s[2]))

    b_scale = B_DH ** (-0.5)
    a_scale = A_DH ** (-0.5)

    def segment(s, mem, odd):
        row0 = pl.multiple_of(s * SEG, SEG)

        qi = lax.broadcasted_iota(jnp.int32, (L, 2 * L), 0)
        kl = lax.broadcasted_iota(jnp.int32, (L, 2 * L), 1)
        qpos = jnp.where(qi < FRESH, qi + MEM, jnp.where(qi < SEG, qi - FRESH, qi))
        kf = kl % SEG
        kpos_f = jnp.where(kf < FRESH, kf + MEM, kf - FRESH)
        kpos = jnp.where(kl < 2 * SEG, kpos_f, SEG + kl % MEM)
        allowed = (qpos < MEM) | (qpos >= kpos)
        is_a = (kl < SEG) | ((kl >= 2 * SEG) & (kl < 2 * SEG + MEM))
        col = lax.broadcasted_iota(jnp.int32, (1, PW), 1)
        col_a = col < B_DH
        col128_a = lax.broadcasted_iota(jnp.int32, (1, 128), 1) < (B_DH - 128)

        xb = xb_s[pl.ds(row0, SEG), :].astype(F32)
        h = jnp.concatenate([xb[:FRESH], mem], axis=0).astype(BF16)
        pre_rows = pl.ds(pl.multiple_of(s * MEM, MEM), MEM)

        def block_diag(fresh, pre):
            z = jnp.zeros_like(fresh)
            zp = jnp.zeros_like(pre)
            return jnp.concatenate([
                jnp.where(col_a, fresh, z), jnp.where(col_a, z, fresh),
                jnp.where(col_a, pre, zp), jnp.where(col_a, zp, pre)], axis=0).astype(BF16)

        def proj(p):
            f = _dot(h, _unpack(w_s[p]))
            g = pre_s[p, pre_rows, :]
            q = jnp.concatenate([f[:, :PW], g[:, :PW]], axis=0).astype(BF16)
            kbd = block_diag(f[:, PW:2 * PW], g[:, PW:2 * PW])
            vbd = block_diag(f[:, 2 * PW:], g[:, 2 * PW:])
            return q, kbd, vbd

        def scores(q, kbd, late_norm):
            sc = _nt_dot(q, kbd) * b_scale
            sc = jnp.where(allowed, sc, NEG)
            ninf = jnp.float32(-jnp.inf)
            ma = jnp.max(jnp.where(is_a, sc, ninf), axis=1, keepdims=True)
            mb = jnp.max(jnp.where(is_a, ninf, sc), axis=1, keepdims=True)
            e = jnp.exp(sc - jnp.where(is_a, ma, mb))
            sa = jnp.sum(jnp.where(is_a, e, 0.0), axis=1, keepdims=True)
            sb = jnp.sum(jnp.where(is_a, 0.0, e), axis=1, keepdims=True)
            if late_norm:
                return e.astype(BF16), _recip(sa), _recip(sb)
            return (e * _recip(jnp.where(is_a, sa, sb))).astype(BF16), None, None

        def pv(p, sm, vbd):
            e, ra, rb = sm
            o = _dot(e, vbd)
            if ra is not None:
                o = jnp.concatenate([
                    o[:, :128] * ra,
                    o[:, 128:256] * jnp.where(col128_a, ra, rb),
                    o[:, 256:] * rb], axis=1)
            if odd:
                o = jnp.concatenate([o, odef_s[:, p * PW:(p + 1) * PW]], axis=0)
                return o.astype(BF16)
            odef_s[:, p * PW:(p + 1) * PW] = o[SEG:]
            return o[:SEG].astype(BF16)

        def wout(p, o, acc):
            contrib = _dot(o, _unpack(wo_s[p]))
            return contrib if acc is None else acc + contrib

        def local_attention():
            qa = qa_s[...]
            kwin = kv_s[0]
            vwin = kv_s[1]
            pos = row0 + lax.broadcasted_iota(jnp.int32, (SEG, 128), 0)
            logits = []
            for w in range(A_W):
                lo = A_HALO - A_DIL * w
                prod = qa * kwin[lo:lo + SEG]
                t = prod[:, :128]
                for j in range(1, NT):
                    t = t + prod[:, j * 128:(j + 1) * 128]
                t = t + pltpu.roll(t, 64, 1)
                t = t + pltpu.roll(t, 32, 1)
                logits.append(jnp.where(pos >= A_DIL * w, t * a_scale, NEG))
            mx = functools.reduce(jnp.maximum, logits)
            es = [jnp.exp(l - mx) for l in logits]
            inv = _recip(functools.reduce(lambda u, v: u + v, es))
            outs = []
            for j in range(NT):
                o = None
                for w in range(A_W):
                    lo = A_HALO - A_DIL * w
                    term = es[w] * vwin[lo:lo + SEG, j * 128:(j + 1) * 128]
                    o = term if o is None else o + term
                outs.append(o * inv)
            kv_s[0, :A_HALO, :] = kwin[SEG:]
            kv_s[1, :A_HALO, :] = vwin[SEG:]
            return jnp.concatenate(outs, axis=1).astype(BF16)

        nxt = pl.multiple_of(jnp.minimum(s + 1, NSEG - 1) * SEG, SEG)

        def a_proj(m):
            r = _dot(xa_s[pl.ds(nxt, SEG), :], _unpack(wa_s[m]))
            if m == 0:
                qa_s[...] = r
            else:
                kv_s[m - 1, A_HALO:, :] = r

        order = []
        for t in range(NP):
            order.append(("P", t))
            if t >= 1:
                order.append(("S", t - 1))
            if t >= 2:
                order.append(("V", t - 2))
            if t >= 3:
                order.append(("W", t - 3))
            if t == 2:
                order.append(("LA", 0))
            if t == 8:
                order.append(("AO", 0))
        order += [("S", NP - 1), ("AP", 0), ("V", NP - 2), ("W", NP - 3), ("V", NP - 1),
                  ("W", NP - 2), ("AP", 1), ("W", NP - 1), ("AP", 2)]

        qkv, sm, ov = {}, {}, {}
        acc = None
        oa = None
        for kind, t in order:
            if kind == "P":
                qkv[t] = proj(t)
            elif kind == "S":
                sm[t] = scores(qkv[t][0], qkv[t][1], t >= NP - 2)
            elif kind == "V":
                ov[t] = pv(t, sm[t], qkv[t][2])
            elif kind == "W":
                acc = wout(t, ov[t], acc)
            elif kind == "LA":
                oa = local_attention()
            elif kind == "AP":
                a_proj(t)
            elif kind == "AO":
                out_s[pl.ds(row0, SEG), :D] = _dot(oa, _unpack(awo_s[...])).astype(BF16)
        return acc

    def out_copy(i):
        r = pl.ds(pl.multiple_of(i * 2 * SEG, 2 * SEG), 2 * SEG)
        return pltpu.make_async_copy(out_s.at[r, :], out_hbm.at[r, :], out_sem)

    def step(i, mem):
        acc0 = segment(2 * i, mem, False)
        acc1 = segment(2 * i + 1, acc0[FRESH:], True)
        res = jnp.concatenate([acc0[:FRESH], acc1[L:], acc1[:FRESH], acc1[SEG:L]], axis=0)
        out_s[pl.ds(pl.multiple_of(i * 2 * SEG, 2 * SEG), 2 * SEG), D:] = res.astype(BF16)
        out_copy(i).start()
        return acc1[FRESH:SEG]

    lax.fori_loop(0, N_STEPS, step, mem0_s[...].astype(F32))

    def wait_out(i, carry):
        out_copy(i).wait()
        return carry

    lax.fori_loop(0, N_STEPS, wait_out, 0)


@functools.partial(jax.jit, static_argnames=("B_seg_len",))
def pallas_concat_heads__sliding_local_dilated__memory_aug_recurrent_mem_tr__prompt_kernel(
    A_x: jax.Array,
    A_wqkv: jax.Array,
    A_wo: jax.Array,
    B_x: jax.Array,
    B_mem0: jax.Array,
    B_Wq: jax.Array,
    B_Wk: jax.Array,
    B_Wv: jax.Array,
    B_Wo: jax.Array,
    B_seg_len,
):
    assert B_seg_len == SEG
    assert A_x.shape == (1, S, D) and B_x.shape == (1, S, D)
    hd = B_H * B_DH
    wq_t = jnp.transpose(B_Wq, (1, 2, 0)).reshape(hd, D)
    wk_t = jnp.transpose(B_Wk, (1, 2, 0)).reshape(hd, D)
    wv_t = jnp.transpose(B_Wv, (1, 2, 0)).reshape(hd, D)
    wo = B_Wo.reshape(hd, D)

    any_spec = pl.BlockSpec(memory_space=pl.ANY)
    out = pl.pallas_call(
        _kernel,
        out_shape=jax.ShapeDtypeStruct((S, 2 * D), BF16),
        in_specs=[any_spec] * 10,
        out_specs=any_spec,
        scratch_shapes=[
            pltpu.VMEM((NSLOT, 4, PW, D), BF16),
            pltpu.VMEM((NSLOT, 128, D), BF16),
            pltpu.VMEM((NP, D // 2, 3 * PW), U32),
            pltpu.VMEM((NP, PW // 2, D), U32),
            pltpu.VMEM((NP, NSEG * MEM, 3 * PW), F32),
            pltpu.VMEM((MEM, hd), F32),
            pltpu.VMEM((S, 2 * D), BF16),
            pltpu.VMEM((S, D), BF16),
            pltpu.VMEM((S, D), BF16),
            pltpu.VMEM((NSEG, MEM, D), BF16),
            pltpu.VMEM((MEM, D), BF16),
            pltpu.VMEM((3, D // 2, D), U32),
            pltpu.VMEM((D, D), BF16),
            pltpu.VMEM((D // 2, D), U32),
            pltpu.VMEM((D, 128), F32),
            pltpu.VMEM((D, 128), F32),
            pltpu.VMEM((SEG, D), F32),
            pltpu.VMEM((2, A_HALO + SEG, D), F32),
            pltpu.SemaphoreType.DMA((NSLOT, 5)),
            pltpu.SemaphoreType.DMA((6,)),
            pltpu.SemaphoreType.DMA,
        ],
        compiler_params=pltpu.CompilerParams(vmem_limit_bytes=120 * 1024 * 1024),
    )(A_x.reshape(S, D), A_wqkv, A_wo, B_x.reshape(S, D), B_x.reshape(NSEG, SEG // MEM, MEM, D),
      B_mem0.reshape(MEM, D), wq_t, wk_t, wv_t, wo)
    return out.reshape(1, S, 2 * D)
```

```python
import functools

import jax
import jax.numpy as jnp
from jax import lax
import jax.experimental.pallas as pl
import jax.experimental.pallas.tpu as pltpu

F32 = jnp.float32
BF16 = jnp.bfloat16

S = 2048
D = 640
NT = D // 128
A_H = 32
A_DH = D // A_H
A_W = 8
A_DIL = 2
A_HALO = 16
B_H = 32
B_DH = 192
MEM = 8
SEG = 32
NSEG = S // SEG
NP = B_H // 2
PW = 2 * B_DH
FRESH = SEG - MEM
L = MEM + SEG
LOG2E = 1.4426950408889634
NEG = -1000000000.0 * LOG2E
NSLOT = 3
N_STEPS = NSEG // 2
U32 = jnp.uint32
AO_AT = (5, 7, 9, 11, 13)


def _nt_dot(a, b):
    return lax.dot_general(a, b, (((1,), (1,)), ((), ())), preferred_element_type=F32)


def _dot(a, b):
    return jnp.dot(a, b, preferred_element_type=F32)


def _pack(x):
    return pltpu.bitcast(x, U32)


def _unpack(x):
    return pltpu.bitcast(x, BF16)


def _recip(x):
    r = pl.reciprocal(x, approx=True)
    return r * (2.0 - x * r)


def _kernel(ax_hbm, awqkv_hbm, awo_hbm, bx_hbm, bx4_hbm, mem0_hbm, wq_hbm, wk_hbm, wv_hbm, wo_hbm,
            out_hbm,
            stage, wa_stage, w_s, wo_s, pre_s, odef_s, out_s,
            xa_s, xb_s, xpre_s, mem0_s, wa_s, awo_raw, awo_s, t1_s, t2_s, qa_s, kv_s,
            ring_sem, misc_sem, out_sem):
    b_scale = B_DH ** (-0.5) * LOG2E
    a_scale = A_DH ** (-0.5) * LOG2E

    def ring_copies(p, slot):
        rows = pl.ds(pl.multiple_of(p * PW, PW), PW)
        piece = jnp.minimum(p, 3 * NT - 1)
        c = piece // NT
        kt = piece % NT
        return [
            pltpu.make_async_copy(wq_hbm.at[rows, :], stage.at[slot, 0], ring_sem.at[slot, 0]),
            pltpu.make_async_copy(wk_hbm.at[rows, :], stage.at[slot, 1], ring_sem.at[slot, 1]),
            pltpu.make_async_copy(wv_hbm.at[rows, :], stage.at[slot, 2], ring_sem.at[slot, 2]),
            pltpu.make_async_copy(wo_hbm.at[rows, :], stage.at[slot, 3], ring_sem.at[slot, 4]),
            pltpu.make_async_copy(
                awqkv_hbm.at[pl.ds(pl.multiple_of(kt * 128, 128), 128),
                             pl.ds(pl.multiple_of(c * D, 128), D)],
                wa_stage.at[slot], ring_sem.at[slot, 3]),
        ]

    def extra_copies(p):
        r2 = pl.ds(pl.multiple_of(p * (S // NP), S // NP), S // NP)
        return [
            pltpu.make_async_copy(ax_hbm.at[r2, :], xa_s.at[r2, :], misc_sem.at[1]),
            pltpu.make_async_copy(bx_hbm.at[r2, :], xb_s.at[r2, :], misc_sem.at[2]),
        ]

    xpre_cp = pltpu.make_async_copy(bx4_hbm.at[:, 3], xpre_s, misc_sem.at[3])
    mem_cp = pltpu.make_async_copy(mem0_hbm, mem0_s, misc_sem.at[4])
    awo_cp = pltpu.make_async_copy(awo_hbm, awo_raw, misc_sem.at[5])

    xpre_cp.start()
    for cp in ring_copies(0, 0):
        cp.start()
    for cp in ring_copies(1, 1):
        cp.start()
    mem_cp.start()
    awo_cp.start()
    xpre_cp.wait()

    def prologue(p, carry):
        slot = p % NSLOT
        for cp in ring_copies(p, slot):
            cp.wait()

        @pl.when(p + 2 < NP)
        def _():
            for cp in ring_copies(p + 2, (p + 2) % NSLOT):
                cp.start()

        for cp in extra_copies(p):
            cp.start()

        xp = xpre_s[...].reshape(NSEG * MEM, D)
        for m in range(3):
            wt = stage[slot, m]
            w_s[p, :, m * PW:(m + 1) * PW] = _pack(wt.T)
            pre_s[p, :, m * PW:(m + 1) * PW] = _nt_dot(xp, wt)
        wo_s[p] = _pack(stage[slot, 3])

        piece = jnp.minimum(p, 3 * NT - 1)
        t1_s[...] = wa_stage[slot].astype(F32).T
        for d in range(A_DH):
            t2_s[d * A_H:(d + 1) * A_H, :] = t1_s[pl.ds(d, A_H, stride=A_DH), :]
        wa_s[piece // NT, pl.ds(pl.multiple_of((piece % NT) * 64, 64), 64), :] = (
            _pack(t2_s[...].T.astype(BF16)))
        return carry

    lax.fori_loop(0, NP, prologue, 0)

    awo_cp.wait()
    mem_cp.wait()
    for j in range(NT):
        t1_s[...] = awo_raw[:, j * 128:(j + 1) * 128].astype(F32)
        for d in range(A_DH):
            awo_s[d * A_H // 2:(d + 1) * A_H // 2, j * 128:(j + 1) * 128] = (
                _pack(t1_s[pl.ds(d, A_H, stride=A_DH), :].astype(BF16)))

    def wait_extra(p, carry):
        for cp in extra_copies(p):
            cp.wait()
        return carry

    lax.fori_loop(0, NP, wait_extra, 0)

    def a_store(m, r):
        for j in range(NT):
            t = r[:, j * 128:(j + 1) * 128]
            if m == 0:
                qa_s[j] = t * a_scale
            else:
                kv_s[m - 1, j, A_HALO:, :] = t

    kv_s[:, :, :A_HALO, :] = jnp.zeros((2, NT, A_HALO, 128), F32)
    for m in range(3):
        a_store(m, _dot(xa_s[:SEG, :], _unpack(wa_s[m])))


    def segment(s, mem, odd):
        row0 = pl.multiple_of(s * SEG, SEG)

        qi = lax.broadcasted_iota(jnp.int32, (L, 2 * L), 0)
        kl = lax.broadcasted_iota(jnp.int32, (L, 2 * L), 1)
        qpos = jnp.where(qi < FRESH, qi + MEM, jnp.where(qi < SEG, qi - FRESH, qi))
        kf = kl % SEG
        kpos_f = jnp.where(kf < FRESH, kf + MEM, kf - FRESH)
        kpos = jnp.where(kl < 2 * SEG, kpos_f, SEG + kl % MEM)
        allowed = (qpos < MEM) | (qpos >= kpos)
        is_a = (kl < SEG) | ((kl >= 2 * SEG) & (kl < 2 * SEG + MEM))
        col = lax.broadcasted_iota(jnp.int32, (1, PW), 1)
        col_a = col < B_DH
        col128_a = lax.broadcasted_iota(jnp.int32, (1, 128), 1) < (B_DH - 128)

        xb = xb_s[pl.ds(row0, SEG), :].astype(F32)
        h = jnp.concatenate([xb[:FRESH], mem], axis=0).astype(BF16)
        pre_rows = pl.ds(pl.multiple_of(s * MEM, MEM), MEM)

        def block_diag(fresh, pre):
            z = jnp.zeros_like(fresh)
            zp = jnp.zeros_like(pre)
            return jnp.concatenate([
                jnp.where(col_a, fresh, z), jnp.where(col_a, z, fresh),
                jnp.where(col_a, pre, zp), jnp.where(col_a, zp, pre)], axis=0).astype(BF16)

        def proj(p):
            f = _dot(h, _unpack(w_s[p]))
            g = pre_s[p, pre_rows, :]
            q = jnp.concatenate([f[:, :PW], g[:, :PW]], axis=0).astype(BF16)
            kbd = block_diag(f[:, PW:2 * PW], g[:, PW:2 * PW])
            vbd = block_diag(f[:, 2 * PW:], g[:, 2 * PW:])
            return q, kbd, vbd

        def scores(q, kbd, late_norm):
            sc = _nt_dot(q, kbd) * b_scale
            sc = jnp.where(allowed, sc, NEG)
            ninf = jnp.float32(-jnp.inf)
            ma = jnp.max(jnp.where(is_a, sc, ninf), axis=1, keepdims=True)
            mb = jnp.max(jnp.where(is_a, ninf, sc), axis=1, keepdims=True)
            e = jnp.exp2(sc - jnp.where(is_a, ma, mb))
            sa = jnp.sum(jnp.where(is_a, e, 0.0), axis=1, keepdims=True)
            sb = jnp.sum(jnp.where(is_a, 0.0, e), axis=1, keepdims=True)
            if late_norm:
                return e.astype(BF16), _recip(sa), _recip(sb)
            return (e * _recip(jnp.where(is_a, sa, sb))).astype(BF16), None, None

        def pv(p, sm, vbd):
            e, ra, rb = sm
            o = _dot(e, vbd)
            if ra is not None:
                o = jnp.concatenate([
                    o[:, :128] * ra,
                    o[:, 128:256] * jnp.where(col128_a, ra, rb),
                    o[:, 256:] * rb], axis=1)
            if odd:
                o = jnp.concatenate([o, odef_s[:, p * PW:(p + 1) * PW]], axis=0)
                return o.astype(BF16)
            odef_s[:, p * PW:(p + 1) * PW] = o[SEG:]
            return o[:SEG].astype(BF16)

        def wout(p, o, acc):
            contrib = _dot(o, _unpack(wo_s[p]))
            return contrib if acc is None else acc + contrib

        def window(m, j, w):
            lo = A_HALO - A_DIL * w
            return kv_s[m, j, lo:lo + SEG, :]

        def local_softmax():
            pos = row0 + lax.broadcasted_iota(jnp.int32, (SEG, 128), 0)
            logits = []
            for w in range(A_W):
                t = qa_s[0] * window(0, 0, w)
                for j in range(1, NT):
                    t = t + qa_s[j] * window(0, j, w)
                t = t + pltpu.roll(t, 64, 1)
                t = t + pltpu.roll(t, 32, 1)
                logits.append(t if w == 0 else jnp.where(pos >= A_DIL * w, t, NEG))
            mx = functools.reduce(jnp.maximum, logits)
            es = [jnp.exp2(l - mx) for l in logits]
            inv = _recip(functools.reduce(lambda u, v: u + v, es))
            return es, inv

        def local_out(j, es, inv, acc):
            o = es[0] * window(1, j, 0)
            for w in range(1, A_W):
                o = o + es[w] * window(1, j, w)
            for m in range(2):
                kv_s[m, j, :A_HALO, :] = kv_s[m, j, SEG:, :]
            r = _dot((o * inv).astype(BF16), _unpack(awo_s[j * 64:(j + 1) * 64, :]))
            return r if acc is None else acc + r

        nxt = pl.multiple_of(jnp.minimum(s + 1, NSEG - 1) * SEG, SEG)

        def a_proj(m):
            a_store(m, _dot(xa_s[pl.ds(nxt, SEG), :], _unpack(wa_s[m])))

        order = []
        for t in range(NP):
            order.append(("P", t))
            if t >= 1:
                order.append(("S", t - 1))
            if t >= 2:
                order.append(("V", t - 2))
            if t >= 3:
                order.append(("W", t - 3))
            if t == 2:
                order.append(("LA", 0))
            if t in AO_AT:
                order.append(("AO", AO_AT.index(t)))
        order += [("S", NP - 1), ("AP", 0), ("V", NP - 2), ("W", NP - 3), ("V", NP - 1),
                  ("W", NP - 2), ("AP", 1), ("W", NP - 1), ("AP", 2)]

        qkv, sm, ov = {}, {}, {}
        acc = None
        oa = None
        for kind, t in order:
            if kind == "P":
                qkv[t] = proj(t)
            elif kind == "S":
                sm[t] = scores(qkv[t][0], qkv[t][1], t >= NP - 2)
            elif kind == "V":
                ov[t] = pv(t, sm[t], qkv[t][2])
            elif kind == "W":
                acc = wout(t, ov[t], acc)
            elif kind == "LA":
                la = local_softmax()
            elif kind == "AP":
                a_proj(t)
            elif kind == "AO":
                oa = local_out(t, la[0], la[1], oa)
                if t == NT - 1:
                    out_s[pl.ds(row0, SEG), :D] = oa.astype(BF16)
        return acc

    def out_copy(i):
        r = pl.ds(pl.multiple_of(i * 2 * SEG, 2 * SEG), 2 * SEG)
        return pltpu.make_async_copy(out_s.at[r, :], out_hbm.at[r, :], out_sem)

    def step(i, mem):
        acc0 = segment(2 * i, mem, False)
        acc1 = segment(2 * i + 1, acc0[FRESH:], True)
        res = jnp.concatenate([acc0[:FRESH], acc1[L:], acc1[:FRESH], acc1[SEG:L]], axis=0)
        out_s[pl.ds(pl.multiple_of(i * 2 * SEG, 2 * SEG), 2 * SEG), D:] = res.astype(BF16)
        out_copy(i).start()
        return acc1[FRESH:SEG]

    lax.fori_loop(0, N_STEPS, step, mem0_s[...].astype(F32))

    def wait_out(i, carry):
        out_copy(i).wait()
        return carry

    lax.fori_loop(0, N_STEPS, wait_out, 0)


@functools.partial(jax.jit, static_argnames=("B_seg_len",))
def pallas_concat_heads__sliding_local_dilated__memory_aug_recurrent_mem_tr__prompt_kernel(
    A_x: jax.Array,
    A_wqkv: jax.Array,
    A_wo: jax.Array,
    B_x: jax.Array,
    B_mem0: jax.Array,
    B_Wq: jax.Array,
    B_Wk: jax.Array,
    B_Wv: jax.Array,
    B_Wo: jax.Array,
    B_seg_len,
):
    assert B_seg_len == SEG
    assert A_x.shape == (1, S, D) and B_x.shape == (1, S, D)
    hd = B_H * B_DH
    wq_t = jnp.transpose(B_Wq, (1, 2, 0)).reshape(hd, D)
    wk_t = jnp.transpose(B_Wk, (1, 2, 0)).reshape(hd, D)
    wv_t = jnp.transpose(B_Wv, (1, 2, 0)).reshape(hd, D)
    wo = B_Wo.reshape(hd, D)

    any_spec = pl.BlockSpec(memory_space=pl.ANY)
    out = pl.pallas_call(
        _kernel,
        out_shape=jax.ShapeDtypeStruct((S, 2 * D), BF16),
        in_specs=[any_spec] * 10,
        out_specs=any_spec,
        scratch_shapes=[
            pltpu.VMEM((NSLOT, 4, PW, D), BF16),
            pltpu.VMEM((NSLOT, 128, D), BF16),
            pltpu.VMEM((NP, D // 2, 3 * PW), U32),
            pltpu.VMEM((NP, PW // 2, D), U32),
            pltpu.VMEM((NP, NSEG * MEM, 3 * PW), F32),
            pltpu.VMEM((MEM, hd), F32),
            pltpu.VMEM((S, 2 * D), BF16),
            pltpu.VMEM((S, D), BF16),
            pltpu.VMEM((S, D), BF16),
            pltpu.VMEM((NSEG, MEM, D), BF16),
            pltpu.VMEM((MEM, D), BF16),
            pltpu.VMEM((3, D // 2, D), U32),
            pltpu.VMEM((D, D), BF16),
            pltpu.VMEM((D // 2, D), U32),
            pltpu.VMEM((D, 128), F32),
            pltpu.VMEM((D, 128), F32),
            pltpu.VMEM((NT, SEG, 128), F32),
            pltpu.VMEM((2, NT, A_HALO + SEG, 128), F32),
            pltpu.SemaphoreType.DMA((NSLOT, 5)),
            pltpu.SemaphoreType.DMA((6,)),
            pltpu.SemaphoreType.DMA,
        ],
        compiler_params=pltpu.CompilerParams(vmem_limit_bytes=120 * 1024 * 1024,
                                             disable_bounds_checks=True),
    )(A_x.reshape(S, D), A_wqkv, A_wo, B_x.reshape(S, D), B_x.reshape(NSEG, SEG // MEM, MEM, D),
      B_mem0.reshape(MEM, D), wq_t, wk_t, wv_t, wo)
    return out.reshape(1, S, 2 * D)
```

```python
import functools

import jax
import jax.numpy as jnp
from jax import lax
import jax.experimental.pallas as pl
import jax.experimental.pallas.tpu as pltpu

F32 = jnp.float32
BF16 = jnp.bfloat16

S = 2048
D = 640
NT = D // 128
A_H = 32
A_DH = D // A_H
A_W = 8
A_DIL = 2
A_HALO = 16
B_H = 32
B_DH = 192
MEM = 8
SEG = 32
NSEG = S // SEG
NP = B_H // 2
PW = 2 * B_DH
FRESH = SEG - MEM
L = MEM + SEG
LOG2E = 1.4426950408889634
NEG = -1000000000.0 * LOG2E
NSLOT = 4
UNR = 2
N_STEPS = NSEG // 2 // UNR
U32 = jnp.uint32
AO_AT = (5, 7, 9, 11, 13)


def _nt_dot(a, b):
    return lax.dot_general(a, b, (((1,), (1,)), ((), ())), preferred_element_type=F32)


def _dot(a, b):
    return jnp.dot(a, b, preferred_element_type=F32)


def _pack(x):
    return pltpu.bitcast(x, U32)


def _unpack(x):
    return pltpu.bitcast(x, BF16)


def _recip(x):
    r = pl.reciprocal(x, approx=True)
    return r * (2.0 - x * r)


def _kernel(ax_hbm, awqkv_hbm, awo_hbm, bx_hbm, bx4_hbm, mem0_hbm, wq_hbm, wk_hbm, wv_hbm, wo_hbm,
            out_hbm,
            stage, w_s, wo_s, pre_s, odef_s, out_s,
            xa_s, xb_s, xpre_s, mem0_s, wa_s, awo_raw, awo_s, t1_s, t2_s, qa_s, kv_s,
            ring_sem, misc_sem, out_sem):
    b_scale = B_DH ** (-0.5) * LOG2E
    a_scale = A_DH ** (-0.5) * LOG2E

    w_hbm = (wq_hbm, wk_hbm, wv_hbm, wo_hbm)

    def w_copy(p, m):
        slot = p % NSLOT
        src = jnp.minimum(p, NP - 1)
        rows = pl.ds(pl.multiple_of(src * PW, PW), PW)
        return pltpu.make_async_copy(w_hbm[m].at[rows, :], stage.at[slot, m], ring_sem.at[slot, m])

    def wa_copy(p):
        slot = p % NSLOT
        piece = jnp.minimum(p, 3 * NT - 1)
        return pltpu.make_async_copy(
            awqkv_hbm.at[pl.ds(pl.multiple_of((piece % NT) * 128, 128), 128),
                         pl.ds(pl.multiple_of((piece // NT) * D, 128), D)],
            stage.at[slot, 4, :128], ring_sem.at[slot, 4])

    def x_copies(p):
        r = pl.ds(pl.multiple_of(p * (S // NP), S // NP), S // NP)
        return [
            pltpu.make_async_copy(ax_hbm.at[r, :], xa_s.at[r, :], misc_sem.at[0]),
            pltpu.make_async_copy(bx_hbm.at[r, :], xb_s.at[r, :], misc_sem.at[1]),
        ]

    xpre_cp = pltpu.make_async_copy(bx4_hbm.at[:, 3], xpre_s, misc_sem.at[2])
    mem_cp = pltpu.make_async_copy(mem0_hbm, mem0_s, misc_sem.at[3])
    awo_cp = pltpu.make_async_copy(awo_hbm, awo_raw, misc_sem.at[4])

    xpre_cp.start()
    for m in range(3):
        w_copy(0, m).start()
    for m in range(3):
        w_copy(1, m).start(priority=1)
    w_copy(0, 3).start(priority=1)
    wa_copy(0).start(priority=1)
    mem_cp.start(priority=1)
    awo_cp.start(priority=1)
    xpre_cp.wait()

    def prologue(p, carry):
        slot = p % NSLOT
        for m in range(3):
            w_copy(p, m).wait()

        @pl.when(p > 0)
        def _():
            w_copy(p - 1, 3).wait()
            wa_copy(p - 1).wait()

        xp = xpre_s[...].reshape(NSEG * MEM, D)
        for m in range(3):
            wt = stage[slot, m]
            w_s[p, :, m * PW:(m + 1) * PW] = _pack(wt.T)
            pre_s[p, :, m * PW:(m + 1) * PW] = _nt_dot(xp, wt)
            if m == 0:
                for mm in range(3):
                    w_copy(p + 2, mm).start(priority=1)
                w_copy(p + 1, 3).start(priority=1)
                wa_copy(p + 1).start(priority=1)
                for cp in x_copies(p):
                    cp.start(priority=1)

        lag = jnp.maximum(p - 1, 0)
        lslot = lag % NSLOT
        wo_s[lag] = _pack(stage[lslot, jnp.where(p > 0, 3, 0)])
        t1_s[...] = stage[lslot, jnp.where(p > 0, 4, 0), :128].astype(F32).T
        for d in range(A_DH):
            t2_s[d * A_H:(d + 1) * A_H, :] = t1_s[pl.ds(d, A_H, stride=A_DH), :]
        wa_s[lag // NT, pl.ds(pl.multiple_of((lag % NT) * 64, 64), 64), :] = (
            _pack(t2_s[...].T.astype(BF16)))
        return carry

    lax.fori_loop(0, NP, prologue, 0)

    for p in (NP, NP + 1):
        for m in range(3):
            w_copy(p, m).wait()
    for p in (NP - 1, NP):
        w_copy(p, 3).wait()
        wa_copy(p).wait()
    for p in range(NP):
        for cp in x_copies(p):
            cp.wait()
    awo_cp.wait()
    mem_cp.wait()

    wo_s[NP - 1] = _pack(stage[(NP - 1) % NSLOT, 3])
    for j in range(NT):
        tj = t1_s if j % 2 == 0 else t2_s
        tj[...] = awo_raw[:, j * 128:(j + 1) * 128].astype(F32)
        for d in range(A_DH):
            awo_s[d * A_H // 2:(d + 1) * A_H // 2, j * 128:(j + 1) * 128] = (
                _pack(tj[pl.ds(d, A_H, stride=A_DH), :].astype(BF16)))

    def a_store(m, r):
        for j in range(NT):
            t = r[:, j * 128:(j + 1) * 128]
            if m == 0:
                qa_s[j] = t * a_scale
            else:
                kv_s[m - 1, j, A_HALO:, :] = t

    kv_s[:, :, :A_HALO, :] = jnp.zeros((2, NT, A_HALO, 128), F32)
    for m in range(3):
        a_store(m, _dot(xa_s[:SEG, :], _unpack(wa_s[m])))


    def segment(s, mem, odd):
        row0 = pl.multiple_of(s * SEG, SEG)

        qi = lax.broadcasted_iota(jnp.int32, (L, 2 * L), 0)
        kl = lax.broadcasted_iota(jnp.int32, (L, 2 * L), 1)
        qpos = jnp.where(qi < FRESH, qi + MEM, jnp.where(qi < SEG, qi - FRESH, qi))
        kf = kl % SEG
        kpos_f = jnp.where(kf < FRESH, kf + MEM, kf - FRESH)
        kpos = jnp.where(kl < 2 * SEG, kpos_f, SEG + kl % MEM)
        allowed = (qpos < MEM) | (qpos >= kpos)
        is_a = (kl < SEG) | ((kl >= 2 * SEG) & (kl < 2 * SEG + MEM))
        col = lax.broadcasted_iota(jnp.int32, (1, PW), 1)
        col_a = col < B_DH
        col128_a = lax.broadcasted_iota(jnp.int32, (1, 128), 1) < (B_DH - 128)

        xb = xb_s[pl.ds(row0, SEG), :].astype(F32)
        h = jnp.concatenate([xb[:FRESH], mem], axis=0).astype(BF16)
        pre_rows = pl.ds(pl.multiple_of(s * MEM, MEM), MEM)

        def block_diag(fresh, pre):
            z = jnp.zeros_like(fresh)
            zp = jnp.zeros_like(pre)
            return jnp.concatenate([
                jnp.where(col_a, fresh, z), jnp.where(col_a, z, fresh),
                jnp.where(col_a, pre, zp), jnp.where(col_a, zp, pre)], axis=0).astype(BF16)

        def proj(p):
            f = _dot(h, _unpack(w_s[p]))
            g = pre_s[p, pre_rows, :]
            q = jnp.concatenate([f[:, :PW], g[:, :PW]], axis=0).astype(BF16)
            kbd = block_diag(f[:, PW:2 * PW], g[:, PW:2 * PW])
            vbd = block_diag(f[:, 2 * PW:], g[:, 2 * PW:])
            return q, kbd, vbd

        def scores(q, kbd, late_norm):
            sc = _nt_dot(q, kbd) * b_scale
            sc = jnp.where(allowed, sc, NEG)
            ninf = jnp.float32(-jnp.inf)
            ma = jnp.max(jnp.where(is_a, sc, ninf), axis=1, keepdims=True)
            mb = jnp.max(jnp.where(is_a, ninf, sc), axis=1, keepdims=True)
            e = jnp.exp2(sc - jnp.where(is_a, ma, mb))
            sa = jnp.sum(jnp.where(is_a, e, 0.0), axis=1, keepdims=True)
            sb = jnp.sum(jnp.where(is_a, 0.0, e), axis=1, keepdims=True)
            if late_norm:
                return e.astype(BF16), _recip(sa), _recip(sb)
            return (e * _recip(jnp.where(is_a, sa, sb))).astype(BF16), None, None

        def pv(p, sm, vbd):
            e, ra, rb = sm
            o = _dot(e, vbd)
            if ra is not None:
                o = jnp.concatenate([
                    o[:, :128] * ra,
                    o[:, 128:256] * jnp.where(col128_a, ra, rb),
                    o[:, 256:] * rb], axis=1)
            if odd:
                o = jnp.concatenate([o, odef_s[:, p * PW:(p + 1) * PW]], axis=0)
                return o.astype(BF16)
            odef_s[:, p * PW:(p + 1) * PW] = o[SEG:]
            return o[:SEG].astype(BF16)

        def wout(p, o, acc):
            contrib = _dot(o, _unpack(wo_s[p]))
            return contrib if acc is None else acc + contrib

        def window(m, j, w):
            lo = A_HALO - A_DIL * w
            return kv_s[m, j, lo:lo + SEG, :]

        def local_softmax():
            pos = row0 + lax.broadcasted_iota(jnp.int32, (SEG, 128), 0)
            logits = []
            for w in range(A_W):
                t = qa_s[0] * window(0, 0, w)
                for j in range(1, NT):
                    t = t + qa_s[j] * window(0, j, w)
                t = t + pltpu.roll(t, 64, 1)
                t = t + pltpu.roll(t, 32, 1)
                logits.append(t if w == 0 else jnp.where(pos >= A_DIL * w, t, NEG))
            mx = functools.reduce(jnp.maximum, logits)
            es = [jnp.exp2(l - mx) for l in logits]
            inv = _recip(functools.reduce(lambda u, v: u + v, es))
            return es, inv

        def local_out(j, es, inv, acc):
            o = es[0] * window(1, j, 0)
            for w in range(1, A_W):
                o = o + es[w] * window(1, j, w)
            for m in range(2):
                kv_s[m, j, :A_HALO, :] = kv_s[m, j, SEG:, :]
            r = _dot((o * inv).astype(BF16), _unpack(awo_s[j * 64:(j + 1) * 64, :]))
            return r if acc is None else acc + r

        nxt = pl.multiple_of(jnp.minimum(s + 1, NSEG - 1) * SEG, SEG)

        def a_proj(m):
            a_store(m, _dot(xa_s[pl.ds(nxt, SEG), :], _unpack(wa_s[m])))

        order = []
        for t in range(NP):
            order.append(("P", t))
            if t >= 1:
                order.append(("S", t - 1))
            if t >= 2:
                order.append(("V", t - 2))
            if t >= 3:
                order.append(("W", t - 3))
            if t == 2:
                order.append(("LA", 0))
            if t in AO_AT:
                order.append(("AO", AO_AT.index(t)))
        order += [("S", NP - 1), ("AP", 0), ("V", NP - 2), ("W", NP - 3), ("V", NP - 1),
                  ("W", NP - 2), ("AP", 1), ("W", NP - 1), ("AP", 2)]

        qkv, sm, ov = {}, {}, {}
        acc = None
        oa = None
        for kind, t in order:
            if kind == "P":
                qkv[t] = proj(t)
            elif kind == "S":
                sm[t] = scores(qkv[t][0], qkv[t][1], t >= NP - 2)
            elif kind == "V":
                ov[t] = pv(t, sm[t], qkv[t][2])
            elif kind == "W":
                acc = wout(t, ov[t], acc)
            elif kind == "LA":
                la = local_softmax()
            elif kind == "AP":
                a_proj(t)
            elif kind == "AO":
                oa = local_out(t, la[0], la[1], oa)
                if t == NT - 1:
                    out_s[pl.ds(row0, SEG), :D] = oa.astype(BF16)
        return acc

    def out_copy(i):
        r = pl.ds(pl.multiple_of(i * 2 * SEG, 2 * SEG), 2 * SEG)
        return pltpu.make_async_copy(out_s.at[r, :], out_hbm.at[r, :], out_sem)

    def step(i, mem):
        acc0 = segment(2 * i, mem, False)
        acc1 = segment(2 * i + 1, acc0[FRESH:], True)
        res = jnp.concatenate([acc0[:FRESH], acc1[L:], acc1[:FRESH], acc1[SEG:L]], axis=0)
        out_s[pl.ds(pl.multiple_of(i * 2 * SEG, 2 * SEG), 2 * SEG), D:] = res.astype(BF16)
        out_copy(i).start()
        return acc1[FRESH:SEG]

    def steps(i, mem):
        for u in range(UNR):
            mem = step(i * UNR + u, mem)
        return mem

    lax.fori_loop(0, N_STEPS, steps, mem0_s[...].astype(F32))

    def wait_out(i, carry):
        out_copy(i).wait()
        return carry

    lax.fori_loop(0, N_STEPS * UNR, wait_out, 0)


@functools.partial(jax.jit, static_argnames=("B_seg_len",))
def pallas_concat_heads__sliding_local_dilated__memory_aug_recurrent_mem_tr__prompt_kernel(
    A_x: jax.Array,
    A_wqkv: jax.Array,
    A_wo: jax.Array,
    B_x: jax.Array,
    B_mem0: jax.Array,
    B_Wq: jax.Array,
    B_Wk: jax.Array,
    B_Wv: jax.Array,
    B_Wo: jax.Array,
    B_seg_len,
):
    assert B_seg_len == SEG
    assert A_x.shape == (1, S, D) and B_x.shape == (1, S, D)
    hd = B_H * B_DH
    wq_t = jnp.transpose(B_Wq, (1, 2, 0)).reshape(hd, D)
    wk_t = jnp.transpose(B_Wk, (1, 2, 0)).reshape(hd, D)
    wv_t = jnp.transpose(B_Wv, (1, 2, 0)).reshape(hd, D)
    wo = B_Wo.reshape(hd, D)

    any_spec = pl.BlockSpec(memory_space=pl.ANY)
    out = pl.pallas_call(
        _kernel,
        out_shape=jax.ShapeDtypeStruct((S, 2 * D), BF16),
        in_specs=[any_spec] * 10,
        out_specs=any_spec,
        scratch_shapes=[
            pltpu.VMEM((NSLOT, 5, PW, D), BF16),
            pltpu.VMEM((NP, D // 2, 3 * PW), U32),
            pltpu.VMEM((NP, PW // 2, D), U32),
            pltpu.VMEM((NP, NSEG * MEM, 3 * PW), F32),
            pltpu.VMEM((MEM, hd), F32),
            pltpu.VMEM((S, 2 * D), BF16),
            pltpu.VMEM((S, D), BF16),
            pltpu.VMEM((S, D), BF16),
            pltpu.VMEM((NSEG, MEM, D), BF16),
            pltpu.VMEM((MEM, D), BF16),
            pltpu.VMEM((3, D // 2, D), U32),
            pltpu.VMEM((D, D), BF16),
            pltpu.VMEM((D // 2, D), U32),
            pltpu.VMEM((D, 128), F32),
            pltpu.VMEM((D, 128), F32),
            pltpu.VMEM((NT, SEG, 128), F32),
            pltpu.VMEM((2, NT, A_HALO + SEG, 128), F32),
            pltpu.SemaphoreType.DMA((NSLOT, 5)),
            pltpu.SemaphoreType.DMA((5,)),
            pltpu.SemaphoreType.DMA,
        ],
        compiler_params=pltpu.CompilerParams(vmem_limit_bytes=120 * 1024 * 1024,
                                             disable_bounds_checks=True),
    )(A_x.reshape(S, D), A_wqkv, A_wo, B_x.reshape(S, D), B_x.reshape(NSEG, SEG // MEM, MEM, D),
      B_mem0.reshape(MEM, D), wq_t, wk_t, wv_t, wo)
    return out.reshape(1, S, 2 * D)
```

```python
import functools

import jax
import jax.numpy as jnp
from jax import lax
import jax.experimental.pallas as pl
import jax.experimental.pallas.tpu as pltpu

F32 = jnp.float32
BF16 = jnp.bfloat16
U32 = jnp.uint32

S = 2048
D = 640
NT = D // 128
A_H = 32
A_DH = D // A_H
A_W = 8
A_DIL = 2
A_HALO = 16
B_H = 32
B_DH = 192
MEM = 8
SEG = 32
NSEG = S // SEG
NP = B_H // 2
PW = 2 * B_DH
PRE = 8
FRESH = SEG - PRE
L = MEM + SEG
GP = 4
NG = NP // GP
LOG2E = 1.4426950408889634
NEG = -1000000000.0 * LOG2E
NSLOT = 4
UNR = 2
N_STEPS = NSEG // 2 // UNR

LAT_MM, LAT_SM, LAT_SM_LATE, LAT_T = 190, 700, 330, 600
LATE_FROM = NP - 2
AO_AFTER = (10, 18, 26, 34, 40)
XLU_T_PRE = True
T_F32 = True
XLU_T_MAIN = True


def _segment_order(odd):
    proj = []
    for g in range(NG):
        proj += [("K", GP * g + r) for r in range(GP)]
        for r in range(GP):
            proj += [("V", GP * g + r), ("Q", GP * g + r)]
    dur = {"K": 120, "V": 120, "Q": 120, "S": 24, "PV": 24, "PS": 24, "PPV": 24,
           "W": 180 if odd else 120, "AO": 40, "AP": 200}
    end = {}

    def ready(task):
        k, i = task
        if k == "S":
            deps = [(("Q", i), LAT_MM), (("K", i), LAT_T if XLU_T_MAIN else LAT_MM)]
        elif k == "PV":
            deps = [(("S", i), LAT_SM_LATE if i >= LATE_FROM else LAT_SM), (("V", i), LAT_MM)]
        elif k == "PS":
            deps = [(("K", GP * i + GP - 1), LAT_T if XLU_T_PRE else LAT_MM)]
        elif k == "PPV":
            deps = [(("PS", i), LAT_SM), (("V", GP * i + GP - 1), LAT_MM)]
        else:
            deps = [(("PV", i), LAT_MM)] + ([(("PPV", i // GP), LAT_MM)] if odd else [])
        if any(d not in end for d, _ in deps):
            return None
        return max(end[d] + lat for d, lat in deps)

    pend = ([("W", p) for p in range(NP)] + [("PPV", g) for g in range(NG)]
            + [("PV", p) for p in range(NP)] + [("PS", g) for g in range(NG)]
            + [("S", p) for p in range(NP)])
    fill = [("AP", 0), ("AP", 1)]
    order = []
    now = [0]

    def emit(task):
        order.append(task)
        now[0] += dur[task[0]]
        end[task] = now[0]

    nproj = 0
    while pend:
        cand = [x for x in pend if ready(x) is not None and ready(x) <= now[0]]
        if cand:
            if not proj:
                cand = [x for x in cand if x[0] != "W"] or cand
            pend.remove(cand[0])
            emit(cand[0])
        elif proj:
            emit(proj.pop(0))
            nproj += 1
            if nproj == GP:
                order.append(("LA", 0))
            if nproj in AO_AFTER:
                emit(("AO", AO_AFTER.index(nproj)))
        elif fill:
            emit(fill.pop(0))
        else:
            now[0] = min(ready(x) for x in pend if ready(x) is not None)
    return order + fill + [("AP", 2)]


def _nt_dot(a, b):
    return lax.dot_general(a, b, (((1,), (1,)), ((), ())), preferred_element_type=F32)


def _dot(a, b):
    return jnp.dot(a, b, preferred_element_type=F32)


def _pack(x):
    return pltpu.bitcast(x, U32)


def _unpack(x):
    return pltpu.bitcast(x, BF16)


def _recip(x):
    r = pl.reciprocal(x, approx=True)
    return r * (2.0 - x * r)


def _kernel(ax_hbm, awqkv_hbm, awo_hbm, bx_hbm, bx4_hbm, mem0_hbm, wq_hbm, wk_hbm, wv_hbm, wo_hbm,
            out_hbm,
            stage, awo_stage, w_s, wo_s, pre_s, odef_s, out_s,
            xa_s, xb_s, xpre_s, mem0_s, wa_s, awo_s, t1_s, t2_s, t3_s, qa_s, kv_s,
            ring_sem, misc_sem, out_sem):
    b_scale = B_DH ** (-0.5) * LOG2E
    a_scale = A_DH ** (-0.5) * LOG2E

    w_hbm = (wq_hbm, wk_hbm, wv_hbm, wo_hbm)

    def w_copy(p, m):
        slot = p % NSLOT
        src = jnp.minimum(p, NP - 1)
        rows = pl.ds(pl.multiple_of(src * PW, PW), PW)
        return pltpu.make_async_copy(w_hbm[m].at[rows, :], stage.at[slot, m], ring_sem.at[slot, m])

    def lag_copies(p):
        slot = p % NSLOT
        piece = jnp.minimum(p, 3 * NT - 1)
        col = jnp.minimum(p, NT - 1)
        return [
            w_copy(p, 3),
            pltpu.make_async_copy(
                awqkv_hbm.at[pl.ds(pl.multiple_of((piece % NT) * 128, 128), 128),
                             pl.ds(pl.multiple_of((piece // NT) * D, 128), D)],
                stage.at[slot, 4, :128], ring_sem.at[slot, 4]),
            pltpu.make_async_copy(
                awo_hbm.at[:, pl.ds(pl.multiple_of(col * 128, 128), 128)],
                awo_stage.at[slot], ring_sem.at[slot, 5]),
        ]

    def x_copies(p):
        r = pl.ds(pl.multiple_of(p * (S // NP), S // NP), S // NP)
        return [
            pltpu.make_async_copy(ax_hbm.at[r, :], xa_s.at[r, :], misc_sem.at[0]),
            pltpu.make_async_copy(bx_hbm.at[r, :], xb_s.at[r, :], misc_sem.at[1]),
        ]

    xpre_cp = pltpu.make_async_copy(bx4_hbm.at[:, 0], xpre_s, misc_sem.at[2])
    mem_cp = pltpu.make_async_copy(mem0_hbm, mem0_s, misc_sem.at[3])

    xpre_cp.start()
    for m in range(3):
        w_copy(0, m).start()
    for m in range(3):
        w_copy(1, m).start(priority=1)
    for cp in lag_copies(0):
        cp.start(priority=1)
    mem_cp.start(priority=1)
    awo_stage[NSLOT - 1] = jnp.zeros((D, 128), BF16)
    kv_s[:, :, :A_HALO, :] = jnp.zeros((2, NT, A_HALO, 128), F32)
    xpre_cp.wait()

    def prologue(p, carry):
        slot = p % NSLOT
        for m in range(3):
            w_copy(p, m).wait()

        @pl.when(p > 0)
        def _():
            for cp in lag_copies(p - 1):
                cp.wait()

        xp = xpre_s[...].reshape(NSEG * PRE, D)
        for m in range(3):
            wt = stage[slot, m]
            w_s[p, :, m * PW:(m + 1) * PW] = _pack(wt.T)
            pre_s[p, :, m * PW:(m + 1) * PW] = _nt_dot(xp, wt)
            if m == 0:
                for cp in x_copies(p):
                    cp.start(priority=1)
                for cp in lag_copies(p + 1):
                    cp.start(priority=1)
                for mm in range(3):
                    w_copy(p + 2, mm).start(priority=1)

        lag = jnp.maximum(p - 1, 0)
        lslot = lag % NSLOT
        wo_s[lag] = _pack(stage[lslot, jnp.where(p > 0, 3, 0)])
        t1_s[...] = stage[lslot, jnp.where(p > 0, 4, 0), :128].astype(F32).T
        for d in range(A_DH):
            t2_s[d * A_H:(d + 1) * A_H, :] = t1_s[pl.ds(d, A_H, stride=A_DH), :]
        wa_s[lag // NT, pl.ds(pl.multiple_of((lag % NT) * 64, 64), 64), :] = (
            _pack(t2_s[...].T.astype(BF16)))
        t3_s[...] = awo_stage[(p + NSLOT - 1) % NSLOT].astype(F32)
        col = jnp.minimum(lag, NT - 1)
        for d in range(A_DH):
            awo_s[col, d * A_H // 2:(d + 1) * A_H // 2, :] = (
                _pack(t3_s[pl.ds(d, A_H, stride=A_DH), :].astype(BF16)))
        return carry

    lax.fori_loop(0, NP, prologue, 0)

    for cp in lag_copies(NP - 1):
        cp.wait()
    for p in range(NP):
        for cp in x_copies(p):
            cp.wait()
    mem_cp.wait()
    wo_s[NP - 1] = _pack(stage[(NP - 1) % NSLOT, 3])

    def a_store(m, r):
        for j in range(NT):
            t = r[:, j * 128:(j + 1) * 128]
            if m == 0:
                qa_s[j] = t * a_scale
            else:
                kv_s[m - 1, j, A_HALO:, :] = t

    for m in range(3):
        a_store(m, _dot(xa_s[:SEG, :], _unpack(wa_s[m])))

    def segment(s, mem, odd):
        row0 = pl.multiple_of(s * SEG, SEG)
        ninf = jnp.float32(-jnp.inf)

        qi = lax.broadcasted_iota(jnp.int32, (SEG, 2 * L), 0)
        kl = lax.broadcasted_iota(jnp.int32, (SEG, 2 * L), 1)
        xk = jnp.where(kl < SEG + FRESH, kl - SEG, kl - SEG - FRESH)
        allowed = (qi >= FRESH) | (kl < SEG) | (qi >= xk)
        is_a = (kl < MEM + PRE) | ((kl >= SEG) & (kl < SEG + FRESH))
        pi = lax.broadcasted_iota(jnp.int32, (GP * PRE, 128), 0)
        pk = lax.broadcasted_iota(jnp.int32, (GP * PRE, 128), 1)
        p_own = (pk // SEG) == (pi // PRE)
        p_allowed = (pk % (MEM + PRE)) <= (pi % PRE) + MEM
        p_first = (pk % SEG) < MEM + PRE
        p_is_a = p_own & p_first
        p_is_b = p_own & jnp.logical_not(p_first)
        col_a = lax.broadcasted_iota(jnp.int32, (1, PW), 1) < B_DH
        col128_a = lax.broadcasted_iota(jnp.int32, (1, 128), 1) < (B_DH - 128)

        xb = xb_s[pl.ds(row0, SEG), :].astype(F32)
        h = jnp.concatenate([xb[PRE:], mem], axis=0).astype(BF16)
        pre_rows = pl.ds(pl.multiple_of(s * PRE, PRE), PRE)

        def proj(p, m):
            return _dot(h, _unpack(w_s[p, :, m * PW:(m + 1) * PW]))

        def pre(p, m):
            return pre_s[p, pre_rows, m * PW:(m + 1) * PW]

        def block_diag(p, m):
            f = proj(p, m)
            lead = jnp.concatenate([f[FRESH:], pre(p, m)], axis=0)
            rest = f[:FRESH]
            zl = jnp.zeros_like(lead)
            zr = jnp.zeros_like(rest)
            return (
                jnp.concatenate([jnp.where(col_a, lead, zl), jnp.where(col_a, zl, lead)], axis=0),
                jnp.concatenate([jnp.where(col_a, rest, zr), jnp.where(col_a, zr, rest)], axis=0))

        def cat(parts):
            return jnp.concatenate(parts, axis=0)

        def qk(q, k, via_xlu):
            if via_xlu:
                if T_F32:
                    return _dot(q, k.T.astype(BF16))
                return _dot(q, _unpack(_pack(k.astype(BF16).T)))
            return _nt_dot(q, k.astype(BF16))

        def scores(q, kbd, late_norm):
            sc = qk(q, cat(kbd), XLU_T_MAIN) * b_scale
            sc = jnp.where(allowed, sc, NEG)
            ma = jnp.max(jnp.where(is_a, sc, ninf), axis=1, keepdims=True)
            mb = jnp.max(jnp.where(is_a, ninf, sc), axis=1, keepdims=True)
            e = jnp.exp2(sc - jnp.where(is_a, ma, mb))
            sa = jnp.sum(jnp.where(is_a, e, 0.0), axis=1, keepdims=True)
            sb = jnp.sum(jnp.where(is_a, 0.0, e), axis=1, keepdims=True)
            if late_norm:
                return e.astype(BF16), _recip(sa), _recip(sb)
            return (e * _recip(jnp.where(is_a, sa, sb))).astype(BF16), None, None

        def pv(sm, vbd):
            e, ra, rb = sm
            o = _dot(e, cat(vbd).astype(BF16))
            if ra is not None:
                o = jnp.concatenate([
                    o[:, :128] * ra,
                    o[:, 128:256] * jnp.where(col128_a, ra, rb),
                    o[:, 256:] * rb], axis=1)
            return o

        def pre_scores(g, kbds):
            q = jnp.concatenate([pre(GP * g + r, 0) for r in range(GP)], axis=0).astype(BF16)
            k = cat([kb[0] for kb in kbds])
            sc = qk(q, k, XLU_T_PRE) * b_scale
            sc = jnp.where(p_allowed, sc, NEG)
            ma = jnp.max(jnp.where(p_is_a, sc, ninf), axis=1, keepdims=True)
            mb = jnp.max(jnp.where(p_is_b, sc, ninf), axis=1, keepdims=True)
            e = jnp.where(p_own, jnp.exp2(sc - jnp.where(p_first, ma, mb)), 0.0)
            sa = jnp.sum(jnp.where(p_first, e, 0.0), axis=1, keepdims=True)
            sb = jnp.sum(jnp.where(p_first, 0.0, e), axis=1, keepdims=True)
            return (e * _recip(jnp.where(p_first, sa, sb))).astype(BF16)

        def pre_pv(g, pr, vbds):
            v = cat([vb[0] for vb in vbds])
            o = _dot(pr, v.astype(BF16))
            if not odd:
                odef_s[g] = o
            return o

        def wout(p, o, opre, acc):
            if odd:
                r = pl.ds((p % GP) * PRE, PRE)
                o = jnp.concatenate(
                    [o, opre[(p % GP) * PRE:(p % GP + 1) * PRE], odef_s[p // GP, r, :]], axis=0)
            contrib = _dot(o.astype(BF16), _unpack(wo_s[p]))
            return contrib if acc is None else acc + contrib

        def window(m, j, w):
            lo = A_HALO - A_DIL * w
            return kv_s[m, j, lo:lo + SEG, :]

        def local_softmax():
            pos = row0 + lax.broadcasted_iota(jnp.int32, (SEG, 128), 0)
            logits = []
            for w in range(A_W):
                t = qa_s[0] * window(0, 0, w)
                for j in range(1, NT):
                    t = t + qa_s[j] * window(0, j, w)
                t = t + pltpu.roll(t, 64, 1)
                t = t + pltpu.roll(t, 32, 1)
                logits.append(t if w == 0 else jnp.where(pos >= A_DIL * w, t, NEG))
            mx = functools.reduce(jnp.maximum, logits)
            es = [jnp.exp2(l - mx) for l in logits]
            inv = _recip(functools.reduce(lambda u, v: u + v, es))
            return es, inv

        def local_out(j, es, inv, acc):
            o = es[0] * window(1, j, 0)
            for w in range(1, A_W):
                o = o + es[w] * window(1, j, w)
            for m in range(2):
                kv_s[m, j, :A_HALO, :] = kv_s[m, j, SEG:, :]
            wj = jnp.concatenate([awo_s[c, j * 64:(j + 1) * 64, :] for c in range(NT)], axis=1)
            r = _dot((o * inv).astype(BF16), _unpack(wj))
            return r if acc is None else acc + r

        nxt = pl.multiple_of(jnp.minimum(s + 1, NSEG - 1) * SEG, SEG)

        val = {}
        acc = None
        oa = None
        for kind, t in _segment_order(odd):
            if kind == "K":
                val[kind, t] = block_diag(t, 1)
            elif kind == "V":
                val[kind, t] = block_diag(t, 2)
            elif kind == "Q":
                val[kind, t] = proj(t, 0).astype(BF16)
            elif kind == "S":
                val[kind, t] = scores(val["Q", t], val["K", t], t >= LATE_FROM)
            elif kind == "PV":
                val[kind, t] = pv(val["S", t], val["V", t])
            elif kind == "PS":
                val[kind, t] = pre_scores(t, [val["K", GP * t + r] for r in range(GP)])
            elif kind == "PPV":
                val[kind, t] = pre_pv(t, val["PS", t], [val["V", GP * t + r] for r in range(GP)])
            elif kind == "W":
                acc = wout(t, val["PV", t], val.get(("PPV", t // GP)), acc)
            elif kind == "LA":
                la = local_softmax()
            elif kind == "AP":
                a_store(t, _dot(xa_s[pl.ds(nxt, SEG), :], _unpack(wa_s[t])))
            elif kind == "AO":
                oa = local_out(t, la[0], la[1], oa)
                if t == NT - 1:
                    out_s[pl.ds(row0, SEG), :D] = oa.astype(BF16)
        return acc

    def out_copy(i):
        r = pl.ds(pl.multiple_of(i * 2 * SEG, 2 * SEG), 2 * SEG)
        return pltpu.make_async_copy(out_s.at[r, :], out_hbm.at[r, :], out_sem)

    def step(i, mem):
        acc0 = segment(2 * i, mem, False)
        acc1 = segment(2 * i + 1, acc0[FRESH:], True)
        res = jnp.concatenate([acc1[SEG + PRE:], acc0[:FRESH], acc1[SEG:SEG + PRE], acc1[:FRESH]],
                              axis=0)
        out_s[pl.ds(pl.multiple_of(i * 2 * SEG, 2 * SEG), 2 * SEG), D:] = res.astype(BF16)
        out_copy(i).start()
        return acc1[FRESH:SEG]

    def steps(i, mem):
        for u in range(UNR):
            mem = step(i * UNR + u, mem)
        return mem

    lax.fori_loop(0, N_STEPS, steps, mem0_s[...].astype(F32))

    for p in (NP, NP + 1):
        for m in range(3):
            w_copy(p, m).wait()
    for cp in lag_copies(NP):
        cp.wait()

    def wait_out(i, carry):
        out_copy(i).wait()
        return carry

    lax.fori_loop(0, N_STEPS * UNR, wait_out, 0)


@functools.partial(jax.jit, static_argnames=("B_seg_len",))
def pallas_concat_heads__sliding_local_dilated__memory_aug_recurrent_mem_tr__prompt_kernel(
    A_x: jax.Array,
    A_wqkv: jax.Array,
    A_wo: jax.Array,
    B_x: jax.Array,
    B_mem0: jax.Array,
    B_Wq: jax.Array,
    B_Wk: jax.Array,
    B_Wv: jax.Array,
    B_Wo: jax.Array,
    B_seg_len,
):
    assert B_seg_len == SEG
    assert A_x.shape == (1, S, D) and B_x.shape == (1, S, D)
    hd = B_H * B_DH
    wq_t = jnp.transpose(B_Wq, (1, 2, 0)).reshape(hd, D)
    wk_t = jnp.transpose(B_Wk, (1, 2, 0)).reshape(hd, D)
    wv_t = jnp.transpose(B_Wv, (1, 2, 0)).reshape(hd, D)
    wo = B_Wo.reshape(hd, D)

    any_spec = pl.BlockSpec(memory_space=pl.ANY)
    out = pl.pallas_call(
        _kernel,
        out_shape=jax.ShapeDtypeStruct((S, 2 * D), BF16),
        in_specs=[any_spec] * 10,
        out_specs=any_spec,
        scratch_shapes=[
            pltpu.VMEM((NSLOT, 5, PW, D), BF16),
            pltpu.VMEM((NSLOT, D, 128), BF16),
            pltpu.VMEM((NP, D // 2, 3 * PW), U32),
            pltpu.VMEM((NP, PW // 2, D), U32),
            pltpu.VMEM((NP, NSEG * PRE, 3 * PW), F32),
            pltpu.VMEM((NG, GP * PRE, PW), F32),
            pltpu.VMEM((S, 2 * D), BF16),
            pltpu.VMEM((S, D), BF16),
            pltpu.VMEM((S, D), BF16),
            pltpu.VMEM((NSEG, PRE, D), BF16),
            pltpu.VMEM((MEM, D), BF16),
            pltpu.VMEM((3, D // 2, D), U32),
            pltpu.VMEM((NT, D // 2, 128), U32),
            pltpu.VMEM((D, 128), F32),
            pltpu.VMEM((D, 128), F32),
            pltpu.VMEM((D, 128), F32),
            pltpu.VMEM((NT, SEG, 128), F32),
            pltpu.VMEM((2, NT, A_HALO + SEG, 128), F32),
            pltpu.SemaphoreType.DMA((NSLOT, 6)),
            pltpu.SemaphoreType.DMA((4,)),
            pltpu.SemaphoreType.DMA,
        ],
        compiler_params=pltpu.CompilerParams(vmem_limit_bytes=120 * 1024 * 1024,
                                             disable_bounds_checks=True),
    )(A_x.reshape(S, D), A_wqkv, A_wo, B_x.reshape(S, D), B_x.reshape(NSEG, SEG // PRE, PRE, D),
      B_mem0.reshape(MEM, D), wq_t, wk_t, wv_t, wo)
    return out.reshape(1, S, 2 * D)
```

```python
import functools

import jax
import jax.numpy as jnp
from jax import lax
import jax.experimental.pallas as pl
import jax.experimental.pallas.tpu as pltpu

F32 = jnp.float32
BF16 = jnp.bfloat16
U32 = jnp.uint32

S = 2048
D = 640
NT = D // 128
A_H = 32
A_DH = D // A_H
A_W = 8
A_DIL = 2
A_HALO = 16
B_H = 32
B_DH = 192
MEM = 8
SEG = 32
NSEG = S // SEG
NP = B_H // 2
PW = 2 * B_DH
PRE = 8
FRESH = SEG - PRE
L = MEM + SEG
GP = 4
NG = NP // GP
LOG2E = 1.4426950408889634
NEG = -1000000000.0 * LOG2E
NSLOT = 4
UNR = 2
N_STEPS = NSEG // 2 // UNR

LAT_MM, LAT_SM, LAT_SM_LATE, LAT_T = 190, 700, 330, 600
LATE_FROM = NP - 2
AO_AFTER = (10, 18, 26, 34, 40)
PRO_ORDER = "0sa12"
XLU_T_PRE = True
T_F32 = True
XLU_T_MAIN = True


def _segment_order(odd):
    proj = []
    for g in range(NG):
        proj += [("K", GP * g + r) for r in range(GP)]
        for r in range(GP):
            proj += [("V", GP * g + r), ("Q", GP * g + r)]
    dur = {"K": 120, "V": 120, "Q": 120, "S": 24, "PV": 24, "PS": 24, "PPV": 24,
           "W": 180 if odd else 120, "AO": 40, "AP": 200}
    end = {}

    def ready(task):
        k, i = task
        if k == "S":
            deps = [(("Q", i), LAT_MM), (("K", i), LAT_T if XLU_T_MAIN else LAT_MM)]
        elif k == "PV":
            deps = [(("S", i), LAT_SM_LATE if i >= LATE_FROM else LAT_SM), (("V", i), LAT_MM)]
        elif k == "PS":
            deps = [(("K", GP * i + GP - 1), LAT_T if XLU_T_PRE else LAT_MM)]
        elif k == "PPV":
            deps = [(("PS", i), LAT_SM), (("V", GP * i + GP - 1), LAT_MM)]
        else:
            deps = [(("PV", i), LAT_MM)] + ([(("PPV", i // GP), LAT_MM)] if odd else [])
        if any(d not in end for d, _ in deps):
            return None
        return max(end[d] + lat for d, lat in deps)

    pend = ([("W", p) for p in range(NP)] + [("PPV", g) for g in range(NG)]
            + [("PV", p) for p in range(NP)] + [("PS", g) for g in range(NG)]
            + [("S", p) for p in range(NP)])
    fill = [("AP", 0), ("AP", 1)]
    order = []
    now = [0]

    def emit(task):
        order.append(task)
        now[0] += dur[task[0]]
        end[task] = now[0]

    nproj = 0
    while pend:
        cand = [x for x in pend if ready(x) is not None and ready(x) <= now[0]]
        if cand:
            if not proj:
                cand = [x for x in cand if x[0] != "W"] or cand
            pend.remove(cand[0])
            emit(cand[0])
        elif proj:
            emit(proj.pop(0))
            nproj += 1
            if nproj == GP:
                order.append(("LA", 0))
            if nproj in AO_AFTER:
                emit(("AO", AO_AFTER.index(nproj)))
        elif fill:
            emit(fill.pop(0))
        else:
            now[0] = min(ready(x) for x in pend if ready(x) is not None)
    return order + fill + [("AP", 2)]


def _nt_dot(a, b):
    return lax.dot_general(a, b, (((1,), (1,)), ((), ())), preferred_element_type=F32)


def _dot(a, b):
    return jnp.dot(a, b, preferred_element_type=F32)


def _pack(x):
    return pltpu.bitcast(x, U32)


def _unpack(x):
    return pltpu.bitcast(x, BF16)


def _recip(x):
    r = pl.reciprocal(x, approx=True)
    return r * (2.0 - x * r)


def _kernel(ax_hbm, awqkv_hbm, awo_hbm, bx_hbm, bx4_hbm, mem0_hbm, wq_hbm, wk_hbm, wv_hbm, wo_hbm,
            out_hbm,
            stage, awo_raw, w_s, wo_s, pre_s, odef_s, out_s,
            xa_s, xb_s, xpre_s, mem0_s, wa_s, awo_s, t1_s, qa_s, kv_s,
            ring_sem, misc_sem, out_sem):
    b_scale = B_DH ** (-0.5) * LOG2E
    a_scale = A_DH ** (-0.5) * LOG2E

    w_hbm = (wq_hbm, wk_hbm, wv_hbm)
    wo32 = wo_hbm.bitcast(U32)
    awo32 = awo_hbm.bitcast(U32)
    hw = PW // 2

    def w_copy(p, m):
        slot = p % NSLOT
        src = jnp.minimum(p, NP - 1)
        rows = pl.ds(pl.multiple_of(src * PW, PW), PW)
        return pltpu.make_async_copy(w_hbm[m].at[rows, :], stage.at[slot, m], ring_sem.at[slot, m])

    def wa_copy(p):
        slot = p % NSLOT
        piece = jnp.minimum(p, 3 * NT - 1)
        return pltpu.make_async_copy(
            awqkv_hbm.at[pl.ds(pl.multiple_of((piece % NT) * 128, 128), 128),
                         pl.ds(pl.multiple_of((piece // NT) * D, 128), D)],
            stage.at[slot, 3, :128], ring_sem.at[slot, 3])

    def x_copies(p):
        r = pl.ds(pl.multiple_of(p * (S // NP), S // NP), S // NP)
        return [
            pltpu.make_async_copy(ax_hbm.at[r, :], xa_s.at[r, :], misc_sem.at[0]),
            pltpu.make_async_copy(bx_hbm.at[r, :], xb_s.at[r, :], misc_sem.at[1]),
        ]

    def wo_copy(p):
        rows = pl.ds(pl.multiple_of(p * hw, hw), hw)
        return pltpu.make_async_copy(wo32.at[rows, :], wo_s.at[rows, :], misc_sem.at[2])

    xpre_cp = pltpu.make_async_copy(bx4_hbm.at[:, 0], xpre_s, misc_sem.at[3])
    mem_cp = pltpu.make_async_copy(mem0_hbm, mem0_s, misc_sem.at[4])
    awo_cps = [pltpu.make_async_copy(awo32.at[:, c * 128:(c + 1) * 128], awo_raw.at[c],
                                     misc_sem.at[5 + c]) for c in range(NT)]

    xpre_cp.start()
    for m in range(3):
        w_copy(0, m).start()
    for m in range(3):
        w_copy(1, m).start(priority=1)
    wa_copy(0).start(priority=1)
    mem_cp.start(priority=1)
    for cp in awo_cps:
        cp.start(priority=1)
    kv_s[:, :, :A_HALO, :] = jnp.zeros((2, NT, A_HALO, 128), F32)
    xpre_cp.wait()

    def gather_heads(ref):
        rows = []
        for j in range(A_DH // 2):
            u = ref[pl.ds(j, A_H, stride=A_DH // 2), :]
            rows.append(pltpu.bitcast(u << 16, F32))
            rows.append(pltpu.bitcast(u & jnp.uint32(0xFFFF0000), F32))
        return jnp.concatenate(rows, axis=0)

    def prologue(p, carry):
        slot = p % NSLOT
        wo_copy(p).start()
        for m in range(3):
            w_copy(p, m).wait()

        @pl.when(p > 0)
        def _():
            wa_copy(p - 1).wait()

        lag = jnp.maximum(p - 1, 0)

        def wa_prep():
            piece = stage[lag % NSLOT, jnp.where(p > 0, 3, 0), :128]
            t1_s[...] = _pack(piece.T)
            wa_s[lag // NT, pl.ds(pl.multiple_of((lag % NT) * 64, 64), 64), :] = (
                _pack(gather_heads(t1_s).astype(BF16).T))

        def starts():
            for cp in x_copies(p):
                cp.start()
            wa_copy(p + 1).start(priority=1)
            for mm in range(3):
                w_copy(p + 2, mm).start(priority=1)

        def pair(m):
            wt = stage[slot, m]
            w_s[p, :, m * PW:(m + 1) * PW] = _pack(wt.T)
            pre_s[p, :, m * PW:(m + 1) * PW] = _nt_dot(xp, wt)

        xp = xpre_s[...].reshape(NSEG * PRE, D)
        parts = {"a": wa_prep, "s": starts,
                 "0": functools.partial(pair, 0), "1": functools.partial(pair, 1),
                 "2": functools.partial(pair, 2)}
        for c in PRO_ORDER:
            parts[c]()
        return carry

    lax.fori_loop(0, NP, prologue, 0)

    pltpu.make_async_copy(ax_hbm, xa_s, misc_sem.at[0]).wait()
    pltpu.make_async_copy(bx_hbm, xb_s, misc_sem.at[1]).wait()
    pltpu.make_async_copy(wo32, wo_s, misc_sem.at[2]).wait()
    mem_cp.wait()
    for cp in awo_cps:
        cp.wait()

    def a_store(m, r):
        for j in range(NT):
            t = r[:, j * 128:(j + 1) * 128]
            if m == 0:
                qa_s[j] = t * a_scale
            else:
                kv_s[m - 1, j, A_HALO:, :] = t

    for m in range(3):
        a_store(m, _dot(xa_s[:SEG, :], _unpack(wa_s[m])))
    for c in range(NT):
        awo_s[:, c * 128:(c + 1) * 128] = _pack(gather_heads(awo_raw.at[c]).astype(BF16))

    def segment(s, mem, odd):
        row0 = pl.multiple_of(s * SEG, SEG)
        ninf = jnp.float32(-jnp.inf)

        qi = lax.broadcasted_iota(jnp.int32, (SEG, 2 * L), 0)
        kl = lax.broadcasted_iota(jnp.int32, (SEG, 2 * L), 1)
        xk = jnp.where(kl < SEG + FRESH, kl - SEG, kl - SEG - FRESH)
        allowed = (qi >= FRESH) | (kl < SEG) | (qi >= xk)
        is_a = (kl < MEM + PRE) | ((kl >= SEG) & (kl < SEG + FRESH))
        pi = lax.broadcasted_iota(jnp.int32, (GP * PRE, 128), 0)
        pk = lax.broadcasted_iota(jnp.int32, (GP * PRE, 128), 1)
        p_own = (pk // SEG) == (pi // PRE)
        p_allowed = (pk % (MEM + PRE)) <= (pi % PRE) + MEM
        p_first = (pk % SEG) < MEM + PRE
        p_is_a = p_own & p_first
        p_is_b = p_own & jnp.logical_not(p_first)
        col_a = lax.broadcasted_iota(jnp.int32, (1, PW), 1) < B_DH
        col128_a = lax.broadcasted_iota(jnp.int32, (1, 128), 1) < (B_DH - 128)

        xb = xb_s[pl.ds(row0, SEG), :].astype(F32)
        h = jnp.concatenate([xb[PRE:], mem], axis=0).astype(BF16)
        pre_rows = pl.ds(pl.multiple_of(s * PRE, PRE), PRE)

        def proj(p, m):
            return _dot(h, _unpack(w_s[p, :, m * PW:(m + 1) * PW]))

        def pre(p, m):
            return pre_s[p, pre_rows, m * PW:(m + 1) * PW]

        def block_diag(p, m):
            f = proj(p, m)
            lead = jnp.concatenate([f[FRESH:], pre(p, m)], axis=0)
            rest = f[:FRESH]
            zl = jnp.zeros_like(lead)
            zr = jnp.zeros_like(rest)
            return (
                jnp.concatenate([jnp.where(col_a, lead, zl), jnp.where(col_a, zl, lead)], axis=0),
                jnp.concatenate([jnp.where(col_a, rest, zr), jnp.where(col_a, zr, rest)], axis=0))

        def cat(parts):
            return jnp.concatenate(parts, axis=0)

        def qk(q, k, via_xlu):
            if via_xlu:
                if T_F32:
                    return _dot(q, k.T.astype(BF16))
                return _dot(q, _unpack(_pack(k.astype(BF16).T)))
            return _nt_dot(q, k.astype(BF16))

        def scores(q, kbd, late_norm):
            sc = qk(q, cat(kbd), XLU_T_MAIN) * b_scale
            sc = jnp.where(allowed, sc, NEG)
            ma = jnp.max(jnp.where(is_a, sc, ninf), axis=1, keepdims=True)
            mb = jnp.max(jnp.where(is_a, ninf, sc), axis=1, keepdims=True)
            e = jnp.exp2(sc - jnp.where(is_a, ma, mb))
            sa = jnp.sum(jnp.where(is_a, e, 0.0), axis=1, keepdims=True)
            sb = jnp.sum(jnp.where(is_a, 0.0, e), axis=1, keepdims=True)
            if late_norm:
                return e.astype(BF16), _recip(sa), _recip(sb)
            return (e * _recip(jnp.where(is_a, sa, sb))).astype(BF16), None, None

        def pv(sm, vbd):
            e, ra, rb = sm
            o = _dot(e, cat(vbd).astype(BF16))
            if ra is not None:
                o = jnp.concatenate([
                    o[:, :128] * ra,
                    o[:, 128:256] * jnp.where(col128_a, ra, rb),
                    o[:, 256:] * rb], axis=1)
            return o

        def pre_scores(g, kbds):
            q = jnp.concatenate([pre(GP * g + r, 0) for r in range(GP)], axis=0).astype(BF16)
            k = cat([kb[0] for kb in kbds])
            sc = qk(q, k, XLU_T_PRE) * b_scale
            sc = jnp.where(p_allowed, sc, NEG)
            ma = jnp.max(jnp.where(p_is_a, sc, ninf), axis=1, keepdims=True)
            mb = jnp.max(jnp.where(p_is_b, sc, ninf), axis=1, keepdims=True)
            e = jnp.where(p_own, jnp.exp2(sc - jnp.where(p_first, ma, mb)), 0.0)
            sa = jnp.sum(jnp.where(p_first, e, 0.0), axis=1, keepdims=True)
            sb = jnp.sum(jnp.where(p_first, 0.0, e), axis=1, keepdims=True)
            return (e * _recip(jnp.where(p_first, sa, sb))).astype(BF16)

        def pre_pv(g, pr, vbds):
            v = cat([vb[0] for vb in vbds])
            o = _dot(pr, v.astype(BF16))
            if not odd:
                odef_s[g] = o
            return o

        def wout(p, o, opre, acc):
            if odd:
                r = pl.ds((p % GP) * PRE, PRE)
                o = jnp.concatenate(
                    [o, opre[(p % GP) * PRE:(p % GP + 1) * PRE], odef_s[p // GP, r, :]], axis=0)
            contrib = _dot(o.astype(BF16), _unpack(wo_s[p * hw:(p + 1) * hw, :]))
            return contrib if acc is None else acc + contrib

        def window(m, j, w):
            lo = A_HALO - A_DIL * w
            return kv_s[m, j, lo:lo + SEG, :]

        def local_softmax():
            pos = row0 + lax.broadcasted_iota(jnp.int32, (SEG, 128), 0)
            logits = []
            for w in range(A_W):
                t = qa_s[0] * window(0, 0, w)
                for j in range(1, NT):
                    t = t + qa_s[j] * window(0, j, w)
                t = t + pltpu.roll(t, 64, 1)
                t = t + pltpu.roll(t, 32, 1)
                logits.append(t if w == 0 else jnp.where(pos >= A_DIL * w, t, NEG))
            mx = functools.reduce(jnp.maximum, logits)
            es = [jnp.exp2(l - mx) for l in logits]
            inv = _recip(functools.reduce(lambda u, v: u + v, es))
            return es, inv

        def local_out(j, es, inv, acc):
            o = es[0] * window(1, j, 0)
            for w in range(1, A_W):
                o = o + es[w] * window(1, j, w)
            for m in range(2):
                kv_s[m, j, :A_HALO, :] = kv_s[m, j, SEG:, :]
            r = _dot((o * inv).astype(BF16), _unpack(awo_s[j * 64:(j + 1) * 64, :]))
            return r if acc is None else acc + r

        nxt = pl.multiple_of(jnp.minimum(s + 1, NSEG - 1) * SEG, SEG)

        val = {}
        acc = None
        oa = None
        for kind, t in _segment_order(odd):
            if kind == "K":
                val[kind, t] = block_diag(t, 1)
            elif kind == "V":
                val[kind, t] = block_diag(t, 2)
            elif kind == "Q":
                val[kind, t] = proj(t, 0).astype(BF16)
            elif kind == "S":
                val[kind, t] = scores(val["Q", t], val["K", t], t >= LATE_FROM)
            elif kind == "PV":
                val[kind, t] = pv(val["S", t], val["V", t])
            elif kind == "PS":
                val[kind, t] = pre_scores(t, [val["K", GP * t + r] for r in range(GP)])
            elif kind == "PPV":
                val[kind, t] = pre_pv(t, val["PS", t], [val["V", GP * t + r] for r in range(GP)])
            elif kind == "W":
                acc = wout(t, val["PV", t], val.get(("PPV", t // GP)), acc)
            elif kind == "LA":
                la = local_softmax()
            elif kind == "AP":
                a_store(t, _dot(xa_s[pl.ds(nxt, SEG), :], _unpack(wa_s[t])))
            elif kind == "AO":
                oa = local_out(t, la[0], la[1], oa)
                if t == NT - 1:
                    out_s[pl.ds(row0, SEG), :D] = oa.astype(BF16)
        return acc

    def out_copy(i):
        r = pl.ds(pl.multiple_of(i * 2 * SEG, 2 * SEG), 2 * SEG)
        return pltpu.make_async_copy(out_s.at[r, :], out_hbm.at[r, :], out_sem)

    def step(i, mem):
        acc0 = segment(2 * i, mem, False)
        acc1 = segment(2 * i + 1, acc0[FRESH:], True)
        res = jnp.concatenate([acc1[SEG + PRE:], acc0[:FRESH], acc1[SEG:SEG + PRE], acc1[:FRESH]],
                              axis=0)
        out_s[pl.ds(pl.multiple_of(i * 2 * SEG, 2 * SEG), 2 * SEG), D:] = res.astype(BF16)
        out_copy(i).start()
        return acc1[FRESH:SEG]

    def steps(i, mem):
        for u in range(UNR):
            mem = step(i * UNR + u, mem)
        return mem

    lax.fori_loop(0, N_STEPS, steps, mem0_s[...].astype(F32))

    for p in (NP, NP + 1):
        for m in range(3):
            w_copy(p, m).wait()
    for p in (NP - 1, NP):
        wa_copy(p).wait()

    def wait_out(i, carry):
        out_copy(i).wait()
        return carry

    lax.fori_loop(0, N_STEPS * UNR, wait_out, 0)


@functools.partial(jax.jit, static_argnames=("B_seg_len",))
def pallas_concat_heads__sliding_local_dilated__memory_aug_recurrent_mem_tr__prompt_kernel(
    A_x: jax.Array,
    A_wqkv: jax.Array,
    A_wo: jax.Array,
    B_x: jax.Array,
    B_mem0: jax.Array,
    B_Wq: jax.Array,
    B_Wk: jax.Array,
    B_Wv: jax.Array,
    B_Wo: jax.Array,
    B_seg_len,
):
    assert B_seg_len == SEG
    assert A_x.shape == (1, S, D) and B_x.shape == (1, S, D)
    hd = B_H * B_DH
    wq_t = jnp.transpose(B_Wq, (1, 2, 0)).reshape(hd, D)
    wk_t = jnp.transpose(B_Wk, (1, 2, 0)).reshape(hd, D)
    wv_t = jnp.transpose(B_Wv, (1, 2, 0)).reshape(hd, D)
    wo = B_Wo.reshape(hd, D)

    any_spec = pl.BlockSpec(memory_space=pl.ANY)
    out = pl.pallas_call(
        _kernel,
        out_shape=jax.ShapeDtypeStruct((S, 2 * D), BF16),
        in_specs=[any_spec] * 10,
        out_specs=any_spec,
        scratch_shapes=[
            pltpu.VMEM((NSLOT, 4, PW, D), BF16),
            pltpu.VMEM((NT, D // 2, 128), U32),
            pltpu.VMEM((NP, D // 2, 3 * PW), U32),
            pltpu.VMEM((hd // 2, D), U32),
            pltpu.VMEM((NP, NSEG * PRE, 3 * PW), F32),
            pltpu.VMEM((NG, GP * PRE, PW), F32),
            pltpu.VMEM((S, 2 * D), BF16),
            pltpu.VMEM((S, D), BF16),
            pltpu.VMEM((S, D), BF16),
            pltpu.VMEM((NSEG, PRE, D), BF16),
            pltpu.VMEM((MEM, D), BF16),
            pltpu.VMEM((3, D // 2, D), U32),
            pltpu.VMEM((D // 2, D), U32),
            pltpu.VMEM((D // 2, 128), U32),
            pltpu.VMEM((NT, SEG, 128), F32),
            pltpu.VMEM((2, NT, A_HALO + SEG, 128), F32),
            pltpu.SemaphoreType.DMA((NSLOT, 4)),
            pltpu.SemaphoreType.DMA((5 + NT,)),
            pltpu.SemaphoreType.DMA,
        ],
        compiler_params=pltpu.CompilerParams(vmem_limit_bytes=120 * 1024 * 1024,
                                             disable_bounds_checks=True),
    )(A_x.reshape(S, D), A_wqkv, A_wo, B_x.reshape(S, D), B_x.reshape(NSEG, SEG // PRE, PRE, D),
      B_mem0.reshape(MEM, D), wq_t, wk_t, wv_t, wo)
    return out.reshape(1, S, 2 * D)
```

```python
import functools

import jax
import jax.numpy as jnp
from jax import lax
import jax.experimental.pallas as pl
import jax.experimental.pallas.tpu as pltpu

F32 = jnp.float32
BF16 = jnp.bfloat16
U32 = jnp.uint32

S = 2048
D = 640
NT = D // 128
A_H = 32
A_DH = D // A_H
A_W = 8
A_DIL = 2
A_HALO = 16
B_H = 32
B_DH = 192
MEM = 8
SEG = 32
NSEG = S // SEG
NP = B_H // 2
PW = 2 * B_DH
PRE = 8
FRESH = SEG - PRE
L = MEM + SEG
GP = 4
NG = NP // GP
LOG2E = 1.4426950408889634
NEG = -1000000000.0 * LOG2E
PP = 2
NTRIP = NP // PP - 1
PEEL_CHUNKS = 4
X_ROWS = 288
WO_ROWS = 432
UNR = 2
N_STEPS = NSEG // 2 // UNR

LAT_MM, LAT_SM, LAT_SM_LATE, LAT_T = 190, 700, 330, 600
LATE_FROM = NP - 2
AO_AFTER = (10, 18, 26, 34, 40)
XLU_T_PRE = True
T_F32 = True
XLU_T_MAIN = True


def _segment_order(odd):
    proj = []
    for g in range(NG):
        proj += [("K", GP * g + r) for r in range(GP)]
        for r in range(GP):
            proj += [("V", GP * g + r), ("Q", GP * g + r)]
    dur = {"K": 120, "V": 120, "Q": 120, "S": 24, "PV": 24, "PS": 24, "PPV": 24,
           "W": 180 if odd else 120, "AO": 40, "AP": 200}
    end = {}

    def ready(task):
        k, i = task
        if k == "S":
            deps = [(("Q", i), LAT_MM), (("K", i), LAT_T if XLU_T_MAIN else LAT_MM)]
        elif k == "PV":
            deps = [(("S", i), LAT_SM_LATE if i >= LATE_FROM else LAT_SM), (("V", i), LAT_MM)]
        elif k == "PS":
            deps = [(("K", GP * i + GP - 1), LAT_T if XLU_T_PRE else LAT_MM)]
        elif k == "PPV":
            deps = [(("PS", i), LAT_SM), (("V", GP * i + GP - 1), LAT_MM)]
        else:
            deps = [(("PV", i), LAT_MM)] + ([(("PPV", i // GP), LAT_MM)] if odd else [])
        if any(d not in end for d, _ in deps):
            return None
        return max(end[d] + lat for d, lat in deps)

    pend = ([("W", p) for p in range(NP)] + [("PPV", g) for g in range(NG)]
            + [("PV", p) for p in range(NP)] + [("PS", g) for g in range(NG)]
            + [("S", p) for p in range(NP)])
    fill = [("AP", 0), ("AP", 1)]
    order = []
    now = [0]

    def emit(task):
        order.append(task)
        now[0] += dur[task[0]]
        end[task] = now[0]

    nproj = 0
    while pend:
        cand = [x for x in pend if ready(x) is not None and ready(x) <= now[0]]
        if cand:
            if not proj:
                cand = [x for x in cand if x[0] != "W"] or cand
            pend.remove(cand[0])
            emit(cand[0])
        elif proj:
            emit(proj.pop(0))
            nproj += 1
            if nproj == GP:
                order.append(("LA", 0))
            if nproj in AO_AFTER:
                emit(("AO", AO_AFTER.index(nproj)))
        elif fill:
            emit(fill.pop(0))
        else:
            now[0] = min(ready(x) for x in pend if ready(x) is not None)
    return order + fill + [("AP", 2)]


def _nt_dot(a, b):
    return lax.dot_general(a, b, (((1,), (1,)), ((), ())), preferred_element_type=F32)


def _dot(a, b):
    return jnp.dot(a, b, preferred_element_type=F32)


def _pack(x):
    return pltpu.bitcast(x, U32)


def _unpack(x):
    return pltpu.bitcast(x, BF16)


def _recip(x):
    r = pl.reciprocal(x, approx=True)
    return r * (2.0 - x * r)


def _kernel(ax_hbm, awqkv_hbm, awo_hbm, bx_hbm, bx4_hbm, mem0_hbm, wq_hbm, wk_hbm, wv_hbm, wo_hbm,
            out_hbm,
            stage, awo_raw, w_s, wo_s, pre_s, odef_s, out_s,
            xa_s, xb_s, xpre_s, mem0_s, wa_s, awo_s, t1_s, qa_s, kv_s,
            ring_sem, misc_sem, out_sem):
    b_scale = B_DH ** (-0.5) * LOG2E
    a_scale = A_DH ** (-0.5) * LOG2E

    w_hbm = (wq_hbm, wk_hbm, wv_hbm)
    wo32 = wo_hbm.bitcast(U32)
    awo32 = awo_hbm.bitcast(U32)
    hw = PW // 2
    hd = B_H * B_DH

    def w_copy(p, half, q, m):
        rows = pl.ds(pl.multiple_of(p * PW, PW), PW)
        return pltpu.make_async_copy(w_hbm[m].at[rows, :], stage.at[half, q, m],
                                     ring_sem.at[half, q, m])

    def wa_copy(piece, half, q):
        return pltpu.make_async_copy(
            awqkv_hbm.at[pl.ds(pl.multiple_of((piece % NT) * 128, 128), 128),
                         pl.ds(pl.multiple_of((piece // NT) * D, 128), D)],
            stage.at[half, q, 3, :128], ring_sem.at[half, q, 3])

    def trip_copies(g):
        half = g % 2
        src = jnp.minimum(g, NTRIP - 1)
        cps = []
        for q in range(PP):
            cps += [w_copy((src + 1) * PP + q, half, q, m) for m in range(3)]
            cps.append(wa_copy(1 + src * PP + q, half, q))
        return cps

    x0 = S - NTRIP * X_ROWS
    wo0 = hd // 2 - NTRIP * WO_ROWS

    def bulk_copies(xr, wr):
        return [
            pltpu.make_async_copy(ax_hbm.at[xr, :], xa_s.at[xr, :], misc_sem.at[0]),
            pltpu.make_async_copy(bx_hbm.at[xr, :], xb_s.at[xr, :], misc_sem.at[1]),
            pltpu.make_async_copy(wo32.at[wr, :], wo_s.at[wr, :], misc_sem.at[2]),
        ]

    xpre_cp = pltpu.make_async_copy(bx4_hbm.at[:, 0], xpre_s, misc_sem.at[3])
    mem_cp = pltpu.make_async_copy(mem0_hbm, mem0_s, misc_sem.at[4])
    awo_cps = [pltpu.make_async_copy(awo32.at[:, c * 128:(c + 1) * 128], awo_raw.at[c],
                                     misc_sem.at[5 + c]) for c in range(NT)]

    xpre_cp.start()
    for q in range(PP):
        for m in range(3):
            w_copy(q, 1, q, m).start(priority=1)
    wa_copy(0, 1, 0).start(priority=1)
    for cp in trip_copies(0):
        cp.start(priority=1)
    for cp in bulk_copies(pl.ds(0, x0), pl.ds(0, wo0)):
        cp.start(priority=1)
    mem_cp.start(priority=1)
    for cp in awo_cps:
        cp.start(priority=1)
    kv_s[:, :, :A_HALO, :] = jnp.zeros((2, NT, A_HALO, 128), F32)

    def gather_heads(ref):
        rows = []
        for j in range(A_DH // 2):
            u = ref[pl.ds(j, A_H, stride=A_DH // 2), :]
            rows.append(pltpu.bitcast(u << 16, F32))
            rows.append(pltpu.bitcast(u & jnp.uint32(0xFFFF0000), F32))
        return jnp.concatenate(rows, axis=0)

    def pair_prep(p, half, q, m, chunks=1):
        wt = stage[half, q, m]
        w_s[p, :, m * PW:(m + 1) * PW] = _pack(wt.T)
        n = NSEG // chunks
        for c in range(chunks):
            xp = xpre_s[c * n:(c + 1) * n].reshape(n * PRE, D)
            pre_s[p, c * n * PRE:(c + 1) * n * PRE, m * PW:(m + 1) * PW] = _nt_dot(xp, wt)

    def wa_prep(piece, half, q):
        t1_s[q] = _pack(stage[half, q, 3, :128].T)
        wa_s[piece // NT, pl.ds(pl.multiple_of((piece % NT) * 64, 64), 64), :] = (
            _pack(gather_heads(t1_s.at[q]).astype(BF16).T))

    xpre_cp.wait()
    w_copy(0, 1, 0, 0).wait()
    pair_prep(0, 1, 0, 0, PEEL_CHUNKS)
    for m in (1, 2):
        w_copy(0, 1, 0, m).wait()
    for m in (1, 2):
        pair_prep(0, 1, 0, m, PEEL_CHUNKS)
    for q in range(1, PP):
        for m in range(3):
            w_copy(q, 1, q, m).wait()
    wa_copy(0, 1, 0).wait()
    for q in range(1, PP):
        for m in range(3):
            pair_prep(q, 1, q, m, PEEL_CHUNKS)
    wa_prep(0, 1, 0)

    def prologue(g, carry):
        half = g % 2
        for cp in bulk_copies(pl.ds(pl.multiple_of(x0 + g * X_ROWS, 16), X_ROWS),
                              pl.ds(pl.multiple_of(wo0 + g * WO_ROWS, 8), WO_ROWS)):
            cp.start()
        for cp in trip_copies(g):
            cp.wait()
        for q in range(PP):
            for m in range(3):
                pair_prep((g + 1) * PP + q, half, q, m)
                if q == 0 and m == 0:
                    for cp in trip_copies(g + 1):
                        cp.start(priority=1)
            wa_prep(1 + g * PP + q, half, q)
        return carry

    lax.fori_loop(0, NTRIP, prologue, 0)

    pltpu.make_async_copy(ax_hbm, xa_s, misc_sem.at[0]).wait()
    pltpu.make_async_copy(bx_hbm, xb_s, misc_sem.at[1]).wait()
    pltpu.make_async_copy(wo32, wo_s, misc_sem.at[2]).wait()
    mem_cp.wait()
    for cp in awo_cps:
        cp.wait()

    def a_store(m, r):
        for j in range(NT):
            t = r[:, j * 128:(j + 1) * 128]
            if m == 0:
                qa_s[j] = t * a_scale
            else:
                kv_s[m - 1, j, A_HALO:, :] = t

    for m in range(3):
        a_store(m, _dot(xa_s[:SEG, :], _unpack(wa_s[m])))
    for c in range(NT):
        awo_s[:, c * 128:(c + 1) * 128] = _pack(gather_heads(awo_raw.at[c]).astype(BF16))

    def segment(s, mem, odd):
        row0 = pl.multiple_of(s * SEG, SEG)
        ninf = jnp.float32(-jnp.inf)

        qi = lax.broadcasted_iota(jnp.int32, (SEG, 2 * L), 0)
        kl = lax.broadcasted_iota(jnp.int32, (SEG, 2 * L), 1)
        is_a = kl < L
        kpos = jnp.where(is_a, kl, kl - L)
        allowed = (qi >= FRESH) | (qi + MEM + PRE >= kpos)
        pi = lax.broadcasted_iota(jnp.int32, (GP * PRE, 128), 0)
        pk = lax.broadcasted_iota(jnp.int32, (GP * PRE, 128), 1)
        p_own = (pk // SEG) == (pi // PRE)
        p_allowed = (pk % (MEM + PRE)) <= (pi % PRE) + MEM
        p_first = (pk % SEG) < MEM + PRE
        p_is_a = p_own & p_first
        p_is_b = p_own & jnp.logical_not(p_first)
        col_a = lax.broadcasted_iota(jnp.int32, (1, PW), 1) < B_DH
        col128_a = lax.broadcasted_iota(jnp.int32, (1, 128), 1) < (B_DH - 128)

        xb = xb_s[pl.ds(row0, SEG), :].astype(F32)
        h = jnp.concatenate([xb[PRE:], mem], axis=0).astype(BF16)
        pre_rows = pl.ds(pl.multiple_of(s * PRE, PRE), PRE)

        def proj(p, m):
            return _dot(h, _unpack(w_s[p, :, m * PW:(m + 1) * PW]))

        def pre(p, m):
            return pre_s[p, pre_rows, m * PW:(m + 1) * PW]

        def block_diag(p, m):
            f = proj(p, m)
            full = jnp.concatenate([f[FRESH:], pre(p, m), f[:FRESH]], axis=0)
            z = jnp.zeros_like(full)
            return jnp.where(col_a, full, z), jnp.where(col_a, z, full)

        def cat(parts):
            return jnp.concatenate(parts, axis=0)

        def qk(q, k, via_xlu):
            if via_xlu:
                if T_F32:
                    return _dot(q, k.T.astype(BF16))
                return _dot(q, _unpack(_pack(k.astype(BF16).T)))
            return _nt_dot(q, k.astype(BF16))

        def scores(q, kbd, late_norm):
            sc = qk(q, cat(kbd), XLU_T_MAIN) * b_scale
            sc = jnp.where(allowed, sc, NEG)
            ma = jnp.max(jnp.where(is_a, sc, ninf), axis=1, keepdims=True)
            mb = jnp.max(jnp.where(is_a, ninf, sc), axis=1, keepdims=True)
            e = jnp.exp2(sc - jnp.where(is_a, ma, mb))
            sa = jnp.sum(jnp.where(is_a, e, 0.0), axis=1, keepdims=True)
            sb = jnp.sum(jnp.where(is_a, 0.0, e), axis=1, keepdims=True)
            if late_norm:
                return e.astype(BF16), _recip(sa), _recip(sb)
            return (e * _recip(jnp.where(is_a, sa, sb))).astype(BF16), None, None

        def pv(sm, vbd):
            e, ra, rb = sm
            o = _dot(e, cat(vbd).astype(BF16))
            if ra is not None:
                o = jnp.concatenate([
                    o[:, :128] * ra,
                    o[:, 128:256] * jnp.where(col128_a, ra, rb),
                    o[:, 256:] * rb], axis=1)
            return o

        def pre_scores(g, kbds):
            q = jnp.concatenate([pre(GP * g + r, 0) for r in range(GP)], axis=0).astype(BF16)
            k = cat([x[:MEM + PRE] for kb in kbds for x in kb])
            sc = qk(q, k, XLU_T_PRE) * b_scale
            sc = jnp.where(p_allowed, sc, NEG)
            ma = jnp.max(jnp.where(p_is_a, sc, ninf), axis=1, keepdims=True)
            mb = jnp.max(jnp.where(p_is_b, sc, ninf), axis=1, keepdims=True)
            e = jnp.where(p_own, jnp.exp2(sc - jnp.where(p_first, ma, mb)), 0.0)
            sa = jnp.sum(jnp.where(p_first, e, 0.0), axis=1, keepdims=True)
            sb = jnp.sum(jnp.where(p_first, 0.0, e), axis=1, keepdims=True)
            return (e * _recip(jnp.where(p_first, sa, sb))).astype(BF16)

        def pre_pv(g, pr, vbds):
            v = cat([x[:MEM + PRE] for vb in vbds for x in vb])
            o = _dot(pr, v.astype(BF16))
            if not odd:
                odef_s[g] = o
            return o

        def wout(p, o, opre, acc):
            if odd:
                r = pl.ds((p % GP) * PRE, PRE)
                o = jnp.concatenate(
                    [o, opre[(p % GP) * PRE:(p % GP + 1) * PRE], odef_s[p // GP, r, :]], axis=0)
            contrib = _dot(o.astype(BF16), _unpack(wo_s[p * hw:(p + 1) * hw, :]))
            return contrib if acc is None else acc + contrib

        def window(m, j, w):
            lo = A_HALO - A_DIL * w
            return kv_s[m, j, lo:lo + SEG, :]

        def local_softmax():
            pos = row0 + lax.broadcasted_iota(jnp.int32, (SEG, 128), 0)
            logits = []
            for w in range(A_W):
                t = qa_s[0] * window(0, 0, w)
                for j in range(1, NT):
                    t = t + qa_s[j] * window(0, j, w)
                t = t + pltpu.roll(t, 64, 1)
                t = t + pltpu.roll(t, 32, 1)
                logits.append(t if w == 0 else jnp.where(pos >= A_DIL * w, t, NEG))
            mx = functools.reduce(jnp.maximum, logits)
            es = [jnp.exp2(l - mx) for l in logits]
            inv = _recip(functools.reduce(lambda u, v: u + v, es))
            return es, inv

        def local_out(j, es, inv, acc):
            o = es[0] * window(1, j, 0)
            for w in range(1, A_W):
                o = o + es[w] * window(1, j, w)
            for m in range(2):
                kv_s[m, j, :A_HALO, :] = kv_s[m, j, SEG:, :]
            r = _dot((o * inv).astype(BF16), _unpack(awo_s[j * 64:(j + 1) * 64, :]))
            return r if acc is None else acc + r

        nxt = pl.multiple_of(jnp.minimum(s + 1, NSEG - 1) * SEG, SEG)

        val = {}
        acc = None
        oa = None
        for kind, t in _segment_order(odd):
            if kind == "K":
                val[kind, t] = block_diag(t, 1)
            elif kind == "V":
                val[kind, t] = block_diag(t, 2)
            elif kind == "Q":
                val[kind, t] = proj(t, 0).astype(BF16)
            elif kind == "S":
                val[kind, t] = scores(val["Q", t], val["K", t], t >= LATE_FROM)
            elif kind == "PV":
                val[kind, t] = pv(val["S", t], val["V", t])
            elif kind == "PS":
                val[kind, t] = pre_scores(t, [val["K", GP * t + r] for r in range(GP)])
            elif kind == "PPV":
                val[kind, t] = pre_pv(t, val["PS", t], [val["V", GP * t + r] for r in range(GP)])
            elif kind == "W":
                acc = wout(t, val["PV", t], val.get(("PPV", t // GP)), acc)
            elif kind == "LA":
                la = local_softmax()
            elif kind == "AP":
                a_store(t, _dot(xa_s[pl.ds(nxt, SEG), :], _unpack(wa_s[t])))
            elif kind == "AO":
                oa = local_out(t, la[0], la[1], oa)
                if t == NT - 1:
                    out_s[pl.ds(row0, SEG), :D] = oa.astype(BF16)
        return acc

    def out_copy(i):
        r = pl.ds(pl.multiple_of(i * 2 * SEG, 2 * SEG), 2 * SEG)
        return pltpu.make_async_copy(out_s.at[r, :], out_hbm.at[r, :], out_sem)

    def step(i, mem):
        acc0 = segment(2 * i, mem, False)
        acc1 = segment(2 * i + 1, acc0[FRESH:], True)
        res = jnp.concatenate([acc1[SEG + PRE:], acc0[:FRESH], acc1[SEG:SEG + PRE], acc1[:FRESH]],
                              axis=0)
        out_s[pl.ds(pl.multiple_of(i * 2 * SEG, 2 * SEG), 2 * SEG), D:] = res.astype(BF16)
        out_copy(i).start()
        return acc1[FRESH:SEG]

    def steps(i, mem):
        for u in range(UNR):
            mem = step(i * UNR + u, mem)
        return mem

    lax.fori_loop(0, N_STEPS, steps, mem0_s[...].astype(F32))

    for cp in trip_copies(NTRIP):
        cp.wait()

    def wait_out(i, carry):
        out_copy(i).wait()
        return carry

    lax.fori_loop(0, N_STEPS * UNR, wait_out, 0)


@functools.partial(jax.jit, static_argnames=("B_seg_len",))
def pallas_concat_heads__sliding_local_dilated__memory_aug_recurrent_mem_tr__prompt_kernel(
    A_x: jax.Array,
    A_wqkv: jax.Array,
    A_wo: jax.Array,
    B_x: jax.Array,
    B_mem0: jax.Array,
    B_Wq: jax.Array,
    B_Wk: jax.Array,
    B_Wv: jax.Array,
    B_Wo: jax.Array,
    B_seg_len,
):
    assert B_seg_len == SEG
    assert A_x.shape == (1, S, D) and B_x.shape == (1, S, D)
    hd = B_H * B_DH
    wq_t = jnp.transpose(B_Wq, (1, 2, 0)).reshape(hd, D)
    wk_t = jnp.transpose(B_Wk, (1, 2, 0)).reshape(hd, D)
    wv_t = jnp.transpose(B_Wv, (1, 2, 0)).reshape(hd, D)
    wo = B_Wo.reshape(hd, D)

    any_spec = pl.BlockSpec(memory_space=pl.ANY)
    out = pl.pallas_call(
        _kernel,
        out_shape=jax.ShapeDtypeStruct((S, 2 * D), BF16),
        in_specs=[any_spec] * 10,
        out_specs=any_spec,
        scratch_shapes=[
            pltpu.VMEM((2, PP, 4, PW, D), BF16),
            pltpu.VMEM((NT, D // 2, 128), U32),
            pltpu.VMEM((NP, D // 2, 3 * PW), U32),
            pltpu.VMEM((hd // 2, D), U32),
            pltpu.VMEM((NP, NSEG * PRE, 3 * PW), F32),
            pltpu.VMEM((NG, GP * PRE, PW), F32),
            pltpu.VMEM((S, 2 * D), BF16),
            pltpu.VMEM((S, D), BF16),
            pltpu.VMEM((S, D), BF16),
            pltpu.VMEM((NSEG, PRE, D), BF16),
            pltpu.VMEM((MEM, D), BF16),
            pltpu.VMEM((3, D // 2, D), U32),
            pltpu.VMEM((D // 2, D), U32),
            pltpu.VMEM((PP, D // 2, 128), U32),
            pltpu.VMEM((NT, SEG, 128), F32),
            pltpu.VMEM((2, NT, A_HALO + SEG, 128), F32),
            pltpu.SemaphoreType.DMA((2, PP, 4)),
            pltpu.SemaphoreType.DMA((5 + NT,)),
            pltpu.SemaphoreType.DMA,
        ],
        compiler_params=pltpu.CompilerParams(vmem_limit_bytes=120 * 1024 * 1024,
                                             disable_bounds_checks=True),
    )(A_x.reshape(S, D), A_wqkv, A_wo, B_x.reshape(S, D), B_x.reshape(NSEG, SEG // PRE, PRE, D),
      B_mem0.reshape(MEM, D), wq_t, wk_t, wv_t, wo)
    return out.reshape(1, S, 2 * D)
```

```python
import functools

import jax
import jax.numpy as jnp
from jax import lax
import jax.experimental.pallas as pl
import jax.experimental.pallas.tpu as pltpu

F32 = jnp.float32
BF16 = jnp.bfloat16
U32 = jnp.uint32

S = 2048
D = 640
NT = D // 128
A_H = 32
A_DH = D // A_H
A_W = 8
A_DIL = 2
A_HALO = 16
B_H = 32
B_DH = 192
MEM = 8
SEG = 32
NSEG = S // SEG
NP = B_H // 2
PW = 2 * B_DH
PRE = 8
FRESH = SEG - PRE
L = MEM + SEG
GP = 4
NG = NP // GP
LOG2E = 1.4426950408889634
NEG = -1000000000.0 * LOG2E
PP = 2
NTRIP = NP // PP - 1
PEEL_CHUNKS = 4
X_ROWS = 288
WO_ROWS = 432
UNR = 2
N_STEPS = NSEG // 2 // UNR

LAT_MM, LAT_SM, LAT_SM_LATE, LAT_T = 190, 650, 330, 600
LATE_FROM = NP - 2
AO_AFTER = (10, 18, 26, 34, 40)
FOLD_T = True
PV_PAD = False
XLU_T_PRE = True
T_F32 = True
XLU_T_MAIN = True


def _segment_order(odd):
    proj = []
    for g in range(NG):
        proj += [("K", GP * g + r) for r in range(GP)]
        for r in range(GP):
            proj += [("V", GP * g + r), ("Q", GP * g + r)]
    dur = {"K": 120, "V": 120, "Q": 120, "S": 24, "PV": 24, "PS": 24, "PPV": 24,
           "W": 180 if odd else 120, "AO": 40, "AP": 200}
    end = {}

    def ready(task):
        k, i = task
        if k == "S":
            deps = [(("Q", i), LAT_MM), (("K", i), LAT_T if XLU_T_MAIN else LAT_MM)]
        elif k == "PV":
            deps = [(("S", i), LAT_SM_LATE if i >= LATE_FROM else LAT_SM), (("V", i), LAT_MM)]
        elif k == "PS":
            deps = [(("K", GP * i + GP - 1), LAT_T if XLU_T_PRE else LAT_MM)]
        elif k == "PPV":
            deps = [(("PS", i), LAT_SM), (("V", GP * i + GP - 1), LAT_MM)]
        else:
            deps = [(("PV", i), LAT_MM)] + ([(("PPV", i // GP), LAT_MM)] if odd else [])
        if any(d not in end for d, _ in deps):
            return None
        return max(end[d] + lat for d, lat in deps)

    pend = ([("W", p) for p in range(NP)] + [("PPV", g) for g in range(NG)]
            + [("PV", p) for p in range(NP)] + [("PS", g) for g in range(NG)]
            + [("S", p) for p in range(NP)])
    fill = [("AP", 0), ("AP", 1)]
    order = []
    now = [0]

    def emit(task):
        order.append(task)
        now[0] += dur[task[0]]
        end[task] = now[0]

    nproj = 0
    while pend:
        cand = [x for x in pend if ready(x) is not None and ready(x) <= now[0]]
        if cand:
            if not proj:
                cand = [x for x in cand if x[0] != "W"] or cand
            pend.remove(cand[0])
            emit(cand[0])
        elif proj:
            emit(proj.pop(0))
            nproj += 1
            if nproj == GP:
                order.append(("LA", 0))
            if nproj in AO_AFTER:
                emit(("AO", AO_AFTER.index(nproj)))
        elif fill:
            emit(fill.pop(0))
        else:
            now[0] = min(ready(x) for x in pend if ready(x) is not None)
    return order + fill + [("AP", 2)]


ORDERS = (
    "K0 K1 K2 K3 V0 LA0 Q1 Q0 V1 S0 V2 PS0 Q2 AO0 S1 V3 Q3 S2 PV0 K4 K5 PPV0 S3 K6 W0 PV1 K7 "
    "PV2 V4 W1 W2 PV3 Q4 AO1 V5 W3 PS1 S4 Q5 V6 Q6 S5 V7 Q7 S6 K8 PPV1 PV4 S7 K9 AO2 K10 W4 PV5 "
    "K11 PV6 V8 W5 W6 PV7 Q8 V9 W7 S8 PS2 Q9 V10 Q10 AO3 S9 V11 PV8 Q11 K12 PPV2 S11 S10 K13 W8 "
    "PV9 K14 K15 W9 PV10 PV11 V12 AO4 Q12 W10 W11 PS3 S12 V13 V15 Q13 Q14 Q15 S13 V14 PV12 S14 "
    "AP0 PPV3 S15 W12 PV13 AP1 PV14 PV15 W13 W14 W15 AP2 ",
    "K0 K1 K2 K3 LA0 V0 Q0 V1 Q1 S0 V2 PS0 Q2 AO0 S1 V3 K4 Q3 S2 PV0 K5 PPV0 S3 K6 PV1 K7 W0 Q4 "
    "W1 PV2 V4 PV3 PS1 AO1 W2 W3 S4 V5 Q5 V6 Q6 S5 V7 Q7 PV4 S6 K8 PPV1 S7 K9 K10 AO2 W4 PV5 "
    "PV6 K11 V8 W5 W6 PV7 Q8 PS2 V9 W7 Q9 S8 V10 Q10 AO3 S9 V11 Q11 PV8 S10 K12 PPV2 S11 K13 "
    "K14 W8 PV9 K15 AO4 PV10 V12 PV11 W10 W9 Q12 PS3 V13 W11 S12 Q13 V14 Q14 S13 V15 Q15 AP0 "
    "S14 PPV3 PV12 S15 AP1 PV13 PV14 W12 PV15 W13 W14 W15 AP2 ",
    "K0 K1 K2 K3 LA0 V0 V1 Q0 Q1 S0 V2 PS0 Q2 AO0 S1 V3 Q3 S2 K4 K5 PPV0 PV0 S3 K6 W0 PV1 K7 "
    "PV2 V4 PV3 W1 W2 Q4 AO1 V5 W3 PS1 S4 Q5 V6 Q6 S5 V7 Q7 S6 K8 S7 PPV1 K9 PV4 AO2 K10 W4 PV5 "
    "PV6 K11 W5 V8 W6 PV7 Q8 W7 V9 PS2 S8 V10 Q9 Q10 AO3 S9 V11 Q11 PV8 S10 K12 PPV2 S11 W8 K13 "
    "PV9 K14 K15 AO4 W9 PV10 PV11 V12 Q12 W10 W11 PS3 S12 Q13 V13 V14 Q14 S13 Q15 PV12 V15 S14 "
    "AP0 PPV3 S15 W12 PV14 PV13 AP1 PV15 W13 W14 W15 AP2 ",
    "K3 K0 K1 K2 LA0 V0 Q0 V1 Q1 S0 V2 PS0 Q2 S1 V3 AO0 S2 K4 PV0 Q3 K5 PPV0 S3 K6 PV1 K7 W0 W1 "
    "PV2 PV3 Q4 V4 W2 W3 AO1 PS1 S4 V5 Q5 V6 Q6 S5 V7 PV4 Q7 S6 K8 S7 K9 AO2 PPV1 K11 K10 W4 "
    "PV5 PV6 V8 W5 PV7 W6 Q8 PS2 V10 V9 W7 S8 Q9 Q10 AO3 S9 V11 Q11 PV8 S10 K12 S11 PPV2 K13 "
    "K14 W8 PV9 K15 AO4 PV10 V12 W9 W10 PV11 Q12 V13 PS3 W11 S12 Q13 V14 S13 V15 Q14 Q15 S14 "
    "AP0 PPV3 PV12 S15 AP1 PV13 PV14 W12 PV15 W13 W14 W15 AP2 ",
)
SKIP_PROLOGUE = False


def _order(u):
    if ORDERS is None or ORDERS[u] is None:
        return _segment_order(u % 2 == 1)
    return [(t.rstrip("0123456789"), int(t.lstrip("ABCDEFGHIJKLMNOPQRSTUVWXYZ")))
            for t in ORDERS[u].split()]


def _nt_dot(a, b):
    return lax.dot_general(a, b, (((1,), (1,)), ((), ())), preferred_element_type=F32)


def _dot(a, b):
    return jnp.dot(a, b, preferred_element_type=F32)


def _pack(x):
    return pltpu.bitcast(x, U32)


def _unpack(x):
    return pltpu.bitcast(x, BF16)


def _recip(x):
    r = pl.reciprocal(x, approx=True)
    return r * (2.0 - x * r)


def _kernel(ax_hbm, awqkv_hbm, awo_hbm, bx_hbm, bx4_hbm, mem0_hbm, wq_hbm, wk_hbm, wv_hbm, wo_hbm,
            out_hbm,
            stage, awo_raw, w_s, wo_s, pre_s, odef_s, out_s,
            xa_s, xb_s, xpre_s, mem0_s, wa_s, awo_s, t1_s, qa_s, kv_s,
            ring_sem, misc_sem, out_sem):
    b_scale = B_DH ** (-0.5) * LOG2E
    a_scale = A_DH ** (-0.5) * LOG2E

    w_hbm = (wq_hbm, wk_hbm, wv_hbm)
    wo32 = wo_hbm.bitcast(U32)
    awo32 = awo_hbm.bitcast(U32)
    hw = PW // 2
    hd = B_H * B_DH

    def w_copy(p, half, q, m):
        rows = pl.ds(pl.multiple_of(p * PW, PW), PW)
        return pltpu.make_async_copy(w_hbm[m].at[rows, :], stage.at[half, q, m],
                                     ring_sem.at[half, q, m])

    def wa_copy(piece, half, q):
        return pltpu.make_async_copy(
            awqkv_hbm.at[pl.ds(pl.multiple_of((piece % NT) * 128, 128), 128),
                         pl.ds(pl.multiple_of((piece // NT) * D, 128), D)],
            stage.at[half, q, 3, :128], ring_sem.at[half, q, 3])

    def trip_copies(g):
        half = g % 2
        src = jnp.minimum(g, NTRIP - 1)
        cps = []
        for q in range(PP):
            cps += [w_copy((src + 1) * PP + q, half, q, m) for m in range(3)]
            cps.append(wa_copy(1 + src * PP + q, half, q))
        return cps

    x0 = S - NTRIP * X_ROWS
    wo0 = hd // 2 - NTRIP * WO_ROWS

    def bulk_copies(xr, wr):
        return [
            pltpu.make_async_copy(ax_hbm.at[xr, :], xa_s.at[xr, :], misc_sem.at[0]),
            pltpu.make_async_copy(bx_hbm.at[xr, :], xb_s.at[xr, :], misc_sem.at[1]),
            pltpu.make_async_copy(wo32.at[wr, :], wo_s.at[wr, :], misc_sem.at[2]),
        ]

    xpre_cp = pltpu.make_async_copy(bx4_hbm.at[:, 0], xpre_s, misc_sem.at[3])
    mem_cp = pltpu.make_async_copy(mem0_hbm, mem0_s, misc_sem.at[4])
    awo_cps = [pltpu.make_async_copy(awo32.at[:, c * 128:(c + 1) * 128], awo_raw.at[c],
                                     misc_sem.at[5 + c]) for c in range(NT)]

    xpre_cp.start()
    for q in range(PP):
        for m in range(3):
            w_copy(q, 1, q, m).start(priority=1)
    wa_copy(0, 1, 0).start(priority=1)
    for cp in trip_copies(0):
        cp.start(priority=1)
    for cp in bulk_copies(pl.ds(0, x0), pl.ds(0, wo0)):
        cp.start(priority=1)
    mem_cp.start(priority=1)
    for cp in awo_cps:
        cp.start(priority=1)
    kv_s[:, :, :A_HALO, :] = jnp.zeros((2, NT, A_HALO, 128), F32)

    def gather_heads(ref):
        rows = []
        for j in range(A_DH // 2):
            u = ref[pl.ds(j, A_H, stride=A_DH // 2), :]
            rows.append(pltpu.bitcast(u << 16, F32))
            rows.append(pltpu.bitcast(u & jnp.uint32(0xFFFF0000), F32))
        return jnp.concatenate(rows, axis=0)

    def pair_prep(p, half, q, m, chunks=1):
        if SKIP_PROLOGUE:
            return
        wt = stage[half, q, m]
        w_s[p, :, m * PW:(m + 1) * PW] = _pack(wt.T)
        n = NSEG // chunks
        for c in range(chunks):
            xp = xpre_s[c * n:(c + 1) * n].reshape(n * PRE, D)
            pre_s[p, c * n * PRE:(c + 1) * n * PRE, m * PW:(m + 1) * PW] = _nt_dot(xp, wt)

    def wa_prep(piece, half, q):
        t1_s[q] = _pack(stage[half, q, 3, :128].T)
        wa_s[piece // NT, pl.ds(pl.multiple_of((piece % NT) * 64, 64), 64), :] = (
            _pack(gather_heads(t1_s.at[q]).astype(BF16).T))

    xpre_cp.wait()
    w_copy(0, 1, 0, 0).wait()
    pair_prep(0, 1, 0, 0, PEEL_CHUNKS)
    for m in (1, 2):
        w_copy(0, 1, 0, m).wait()
    for m in (1, 2):
        pair_prep(0, 1, 0, m, PEEL_CHUNKS)
    for q in range(1, PP):
        for m in range(3):
            w_copy(q, 1, q, m).wait()
    wa_copy(0, 1, 0).wait()
    for q in range(1, PP):
        for m in range(3):
            pair_prep(q, 1, q, m, PEEL_CHUNKS)
    wa_prep(0, 1, 0)

    def prologue(g, carry):
        half = g % 2
        for cp in bulk_copies(pl.ds(pl.multiple_of(x0 + g * X_ROWS, 16), X_ROWS),
                              pl.ds(pl.multiple_of(wo0 + g * WO_ROWS, 8), WO_ROWS)):
            cp.start()
        for cp in trip_copies(g):
            cp.wait()
        for q in range(PP):
            for m in range(3):
                pair_prep((g + 1) * PP + q, half, q, m)
                if q == 0 and m == 0:
                    for cp in trip_copies(g + 1):
                        cp.start(priority=1)
            wa_prep(1 + g * PP + q, half, q)
        return carry

    lax.fori_loop(0, NTRIP, prologue, 0)

    pltpu.make_async_copy(ax_hbm, xa_s, misc_sem.at[0]).wait()
    pltpu.make_async_copy(bx_hbm, xb_s, misc_sem.at[1]).wait()
    pltpu.make_async_copy(wo32, wo_s, misc_sem.at[2]).wait()
    mem_cp.wait()
    for cp in awo_cps:
        cp.wait()

    def a_store(m, r):
        for j in range(NT):
            t = r[:, j * 128:(j + 1) * 128]
            if m == 0:
                qa_s[j] = t * a_scale
            else:
                kv_s[m - 1, j, A_HALO:, :] = t

    for m in range(3):
        a_store(m, _dot(xa_s[:SEG, :], _unpack(wa_s[m])))
    for c in range(NT):
        awo_s[:, c * 128:(c + 1) * 128] = _pack(gather_heads(awo_raw.at[c]).astype(BF16))

    def segment(s, mem, u):
        odd = u % 2 == 1
        row0 = pl.multiple_of(s * SEG, SEG)
        ninf = jnp.float32(-jnp.inf)

        qi = lax.broadcasted_iota(jnp.int32, (SEG, 2 * L), 0)
        kl = lax.broadcasted_iota(jnp.int32, (SEG, 2 * L), 1)
        is_a = kl < L
        kpos = jnp.where(is_a, kl, kl - L)
        allowed = (qi >= FRESH) | (qi + MEM + PRE >= kpos)
        pi = lax.broadcasted_iota(jnp.int32, (GP * PRE, 128), 0)
        pk = lax.broadcasted_iota(jnp.int32, (GP * PRE, 128), 1)
        p_own = (pk // SEG) == (pi // PRE)
        p_allowed = (pk % (MEM + PRE)) <= (pi % PRE) + MEM
        p_first = (pk % SEG) < MEM + PRE
        p_is_a = p_own & p_first
        p_is_b = p_own & jnp.logical_not(p_first)
        col_a = lax.broadcasted_iota(jnp.int32, (1, PW), 1) < B_DH
        col128_a = lax.broadcasted_iota(jnp.int32, (1, 128), 1) < (B_DH - 128)

        xb = xb_s[pl.ds(row0, SEG), :].astype(F32)
        h = jnp.concatenate([xb[PRE:], mem], axis=0).astype(BF16)
        pre_rows = pl.ds(pl.multiple_of(s * PRE, PRE), PRE)

        def proj(p, m):
            return _dot(h, _unpack(w_s[p, :, m * PW:(m + 1) * PW]))

        def pre(p, m):
            return pre_s[p, pre_rows, m * PW:(m + 1) * PW]

        def block_diag(p, m):
            f = proj(p, m)
            full = jnp.concatenate([f[FRESH:], pre(p, m), f[:FRESH]], axis=0)
            z = jnp.zeros_like(full)
            return jnp.where(col_a, full, z), jnp.where(col_a, z, full)

        def cat(parts):
            return jnp.concatenate(parts, axis=0)

        def qk(q, blocks):
            if not FOLD_T:
                return _dot(q, cat(blocks).T.astype(BF16))
            fold = cat([jnp.concatenate([x[:, :128] if i % 2 == 0 else x[:, 256:], x[:, 128:256]],
                                        axis=1) for i, x in enumerate(blocks)])
            if T_F32:
                t = fold.T
            else:
                t = fold.astype(BF16).T.astype(F32)
            outer = t[:128]
            n = blocks[0].shape[0]
            lane = lax.broadcasted_iota(jnp.int32, outer.shape, 1)
            lane_a = lane < n if len(blocks) == 2 else lane % (2 * n) < n
            z = jnp.zeros_like(outer)
            kt = cat([jnp.where(lane_a, outer, z), t[128:], jnp.where(lane_a, z, outer)])
            return _dot(q, kt.astype(BF16))

        def scores(q, kbd, late_norm):
            sc = qk(q, kbd) * b_scale
            sc = jnp.where(allowed, sc, NEG)
            ma = jnp.max(jnp.where(is_a, sc, ninf), axis=1, keepdims=True)
            mb = jnp.max(jnp.where(is_a, ninf, sc), axis=1, keepdims=True)
            e = jnp.exp2(sc - jnp.where(is_a, ma, mb))
            sa = jnp.sum(jnp.where(is_a, e, 0.0), axis=1, keepdims=True)
            sb = jnp.sum(jnp.where(is_a, 0.0, e), axis=1, keepdims=True)
            def fin(x):
                if PV_PAD:
                    x = jnp.concatenate([x, jnp.zeros((SEG, 128 - 2 * L), F32)], axis=1)
                return x.astype(BF16)
            if late_norm:
                return fin(e), _recip(sa), _recip(sb)
            return fin(e * _recip(jnp.where(is_a, sa, sb))), None, None

        def pv(sm, vbd):
            e, ra, rb = sm
            if PV_PAD:
                vbd = list(vbd) + [jnp.zeros((128 - 2 * L, PW), F32)]
            o = _dot(e, cat(vbd).astype(BF16))
            if ra is not None:
                o = jnp.concatenate([
                    o[:, :128] * ra,
                    o[:, 128:256] * jnp.where(col128_a, ra, rb),
                    o[:, 256:] * rb], axis=1)
            return o

        def pre_scores(g, kbds):
            q = jnp.concatenate([pre(GP * g + r, 0) for r in range(GP)], axis=0).astype(BF16)
            k = [x[:MEM + PRE] for kb in kbds for x in kb]
            sc = qk(q, k) * b_scale
            sc = jnp.where(p_allowed, sc, NEG)
            ma = jnp.max(jnp.where(p_is_a, sc, ninf), axis=1, keepdims=True)
            mb = jnp.max(jnp.where(p_is_b, sc, ninf), axis=1, keepdims=True)
            e = jnp.where(p_own, jnp.exp2(sc - jnp.where(p_first, ma, mb)), 0.0)
            sa = jnp.sum(jnp.where(p_first, e, 0.0), axis=1, keepdims=True)
            sb = jnp.sum(jnp.where(p_first, 0.0, e), axis=1, keepdims=True)
            return (e * _recip(jnp.where(p_first, sa, sb))).astype(BF16)

        def pre_pv(g, pr, vbds):
            v = cat([x[:MEM + PRE] for vb in vbds for x in vb])
            o = _dot(pr, v.astype(BF16))
            if not odd:
                odef_s[g] = o
            return o

        def wout(p, o, opre, acc):
            if odd:
                r = pl.ds((p % GP) * PRE, PRE)
                o = jnp.concatenate(
                    [o, opre[(p % GP) * PRE:(p % GP + 1) * PRE], odef_s[p // GP, r, :]], axis=0)
            contrib = _dot(o.astype(BF16), _unpack(wo_s[p * hw:(p + 1) * hw, :]))
            return contrib if acc is None else acc + contrib

        def window(m, j, w):
            lo = A_HALO - A_DIL * w
            return kv_s[m, j, lo:lo + SEG, :]

        def local_softmax():
            pos = row0 + lax.broadcasted_iota(jnp.int32, (SEG, 128), 0)
            logits = []
            for w in range(A_W):
                t = qa_s[0] * window(0, 0, w)
                for j in range(1, NT):
                    t = t + qa_s[j] * window(0, j, w)
                t = t + pltpu.roll(t, 64, 1)
                t = t + pltpu.roll(t, 32, 1)
                logits.append(t if w == 0 else jnp.where(pos >= A_DIL * w, t, NEG))
            mx = functools.reduce(jnp.maximum, logits)
            es = [jnp.exp2(l - mx) for l in logits]
            inv = _recip(functools.reduce(lambda u, v: u + v, es))
            return es, inv

        def local_out(j, es, inv, acc):
            o = es[0] * window(1, j, 0)
            for w in range(1, A_W):
                o = o + es[w] * window(1, j, w)
            for m in range(2):
                kv_s[m, j, :A_HALO, :] = kv_s[m, j, SEG:, :]
            r = _dot((o * inv).astype(BF16), _unpack(awo_s[j * 64:(j + 1) * 64, :]))
            return r if acc is None else acc + r

        nxt = pl.multiple_of(jnp.minimum(s + 1, NSEG - 1) * SEG, SEG)

        val = {}
        acc = None
        oa = None
        for kind, t in _order(u):
            if kind == "K":
                val[kind, t] = block_diag(t, 1)
            elif kind == "V":
                val[kind, t] = block_diag(t, 2)
            elif kind == "Q":
                val[kind, t] = proj(t, 0).astype(BF16)
            elif kind == "S":
                val[kind, t] = scores(val["Q", t], val["K", t], t >= LATE_FROM)
            elif kind == "PV":
                val[kind, t] = pv(val["S", t], val["V", t])
            elif kind == "PS":
                val[kind, t] = pre_scores(t, [val["K", GP * t + r] for r in range(GP)])
            elif kind == "PPV":
                val[kind, t] = pre_pv(t, val["PS", t], [val["V", GP * t + r] for r in range(GP)])
            elif kind == "W":
                acc = wout(t, val["PV", t], val.get(("PPV", t // GP)), acc)
            elif kind == "LA":
                la = local_softmax()
            elif kind == "AP":
                a_store(t, _dot(xa_s[pl.ds(nxt, SEG), :], _unpack(wa_s[t])))
            elif kind == "AO":
                oa = local_out(t, la[0], la[1], oa)
                if t == NT - 1:
                    out_s[pl.ds(row0, SEG), :D] = oa.astype(BF16)
        return acc

    def out_copy(i):
        r = pl.ds(pl.multiple_of(i * 2 * SEG, 2 * SEG), 2 * SEG)
        return pltpu.make_async_copy(out_s.at[r, :], out_hbm.at[r, :], out_sem)

    def step(i, mem, u):
        acc0 = segment(2 * i, mem, 2 * u)
        acc1 = segment(2 * i + 1, acc0[FRESH:], 2 * u + 1)
        res = jnp.concatenate([acc1[SEG + PRE:], acc0[:FRESH], acc1[SEG:SEG + PRE], acc1[:FRESH]],
                              axis=0)
        out_s[pl.ds(pl.multiple_of(i * 2 * SEG, 2 * SEG), 2 * SEG), D:] = res.astype(BF16)
        out_copy(i).start()
        return acc1[FRESH:SEG]

    def steps(i, mem):
        for u in range(UNR):
            mem = step(i * UNR + u, mem, u)
        return mem

    lax.fori_loop(0, N_STEPS, steps, mem0_s[...].astype(F32))

    for cp in trip_copies(NTRIP):
        cp.wait()

    def wait_out(i, carry):
        out_copy(i).wait()
        return carry

    lax.fori_loop(0, N_STEPS * UNR, wait_out, 0)


@jax.jit
def pallas_concat_heads__sliding_local_dilated__memory_aug_recurrent_mem_tr__prompt_kernel(
    A_x: jax.Array,
    A_wqkv: jax.Array,
    A_wo: jax.Array,
    B_x: jax.Array,
    B_mem0: jax.Array,
    B_Wq: jax.Array,
    B_Wk: jax.Array,
    B_Wv: jax.Array,
    B_Wo: jax.Array,
    B_seg_len,
):
    del B_seg_len
    assert A_x.shape == (1, S, D) and B_x.shape == (1, S, D)
    hd = B_H * B_DH
    wq_t = jnp.transpose(B_Wq, (1, 2, 0)).reshape(hd, D)
    wk_t = jnp.transpose(B_Wk, (1, 2, 0)).reshape(hd, D)
    wv_t = jnp.transpose(B_Wv, (1, 2, 0)).reshape(hd, D)
    wo = B_Wo.reshape(hd, D)

    any_spec = pl.BlockSpec(memory_space=pl.ANY)
    out = pl.pallas_call(
        _kernel,
        out_shape=jax.ShapeDtypeStruct((S, 2 * D), BF16),
        in_specs=[any_spec] * 10,
        out_specs=any_spec,
        scratch_shapes=[
            pltpu.VMEM((2, PP, 4, PW, D), BF16),
            pltpu.VMEM((NT, D // 2, 128), U32),
            pltpu.VMEM((NP, D // 2, 3 * PW), U32),
            pltpu.VMEM((hd // 2, D), U32),
            pltpu.VMEM((NP, NSEG * PRE, 3 * PW), F32),
            pltpu.VMEM((NG, GP * PRE, PW), F32),
            pltpu.VMEM((S, 2 * D), BF16),
            pltpu.VMEM((S, D), BF16),
            pltpu.VMEM((S, D), BF16),
            pltpu.VMEM((NSEG, PRE, D), BF16),
            pltpu.VMEM((MEM, D), BF16),
            pltpu.VMEM((3, D // 2, D), U32),
            pltpu.VMEM((D // 2, D), U32),
            pltpu.VMEM((PP, D // 2, 128), U32),
            pltpu.VMEM((NT, SEG, 128), F32),
            pltpu.VMEM((2, NT, A_HALO + SEG, 128), F32),
            pltpu.SemaphoreType.DMA((2, PP, 4)),
            pltpu.SemaphoreType.DMA((5 + NT,)),
            pltpu.SemaphoreType.DMA,
        ],
        compiler_params=pltpu.CompilerParams(vmem_limit_bytes=120 * 1024 * 1024,
                                             disable_bounds_checks=True),
    )(A_x.reshape(S, D), A_wqkv, A_wo, B_x.reshape(S, D), B_x.reshape(NSEG, SEG // PRE, PRE, D),
      B_mem0.reshape(MEM, D), wq_t, wk_t, wv_t, wo)
    return out.reshape(1, S, 2 * D)
```

```python
import functools

import jax
import jax.numpy as jnp
from jax import lax
import jax.experimental.pallas as pl
import jax.experimental.pallas.tpu as pltpu

F32 = jnp.float32
BF16 = jnp.bfloat16
U32 = jnp.uint32

S = 2048
D = 640
NT = D // 128
A_H = 32
A_DH = D // A_H
A_W = 8
A_DIL = 2
A_HALO = 16
B_H = 32
B_DH = 192
MEM = 8
SEG = 32
NSEG = S // SEG
NP = B_H // 2
PW = 2 * B_DH
PRE = 8
FRESH = SEG - PRE
L = MEM + SEG
GP = 4
NG = NP // GP
LOG2E = 1.4426950408889634
NEG = -1000000000.0 * LOG2E
PP = 2
NTRIP = NP // PP - 1
PEEL_CHUNKS = 4
X_ROWS = 288
WO_ROWS = 432
UNR = 2
N_STEPS = NSEG // 2 // UNR

LAT_MM, LAT_SM, LAT_SM_LATE, LAT_T = 190, 650, 330, 600
LATE_FROM = NP - 2
AO_AFTER = (10, 18, 26, 34, 40)
FOLD_T = True
PV_PAD = False
XLU_T_PRE = True
T_F32 = True
XLU_T_MAIN = True


def _segment_order(odd):
    proj = []
    for g in range(NG):
        proj += [("K", GP * g + r) for r in range(GP)]
        for r in range(GP):
            proj += [("V", GP * g + r), ("Q", GP * g + r)]
    dur = {"K": 120, "V": 120, "Q": 120, "S": 24, "PV": 24, "PS": 24, "PPV": 24,
           "W": 180 if odd else 120, "AO": 40, "AP": 200}
    end = {}

    def ready(task):
        k, i = task
        if k == "S":
            deps = [(("Q", i), LAT_MM), (("K", i), LAT_T if XLU_T_MAIN else LAT_MM)]
        elif k == "PV":
            deps = [(("S", i), LAT_SM_LATE if i >= LATE_FROM else LAT_SM), (("V", i), LAT_MM)]
        elif k == "PS":
            deps = [(("K", GP * i + GP - 1), LAT_T if XLU_T_PRE else LAT_MM)]
        elif k == "PPV":
            deps = [(("PS", i), LAT_SM), (("V", GP * i + GP - 1), LAT_MM)]
        else:
            deps = [(("PV", i), LAT_MM)] + ([(("PPV", i // GP), LAT_MM)] if odd else [])
        if any(d not in end for d, _ in deps):
            return None
        return max(end[d] + lat for d, lat in deps)

    pend = ([("W", p) for p in range(NP)] + [("PPV", g) for g in range(NG)]
            + [("PV", p) for p in range(NP)] + [("PS", g) for g in range(NG)]
            + [("S", p) for p in range(NP)])
    fill = [("AP", 0), ("AP", 1)]
    order = []
    now = [0]

    def emit(task):
        order.append(task)
        now[0] += dur[task[0]]
        end[task] = now[0]

    nproj = 0
    while pend:
        cand = [x for x in pend if ready(x) is not None and ready(x) <= now[0]]
        if cand:
            if not proj:
                cand = [x for x in cand if x[0] != "W"] or cand
            pend.remove(cand[0])
            emit(cand[0])
        elif proj:
            emit(proj.pop(0))
            nproj += 1
            if nproj == GP:
                order.append(("LA", 0))
            if nproj in AO_AFTER:
                emit(("AO", AO_AFTER.index(nproj)))
        elif fill:
            emit(fill.pop(0))
        else:
            now[0] = min(ready(x) for x in pend if ready(x) is not None)
    return order + fill + [("AP", 2)]


ORDERS = (
    "K0 K1 K2 K3 V0 LA0 Q1 Q0 V1 S0 V2 PS0 Q2 AO0 S1 V3 Q3 S2 PV0 K4 K5 PPV0 S3 K6 W0 PV1 K7 "
    "PV2 V4 W1 W2 PV3 Q4 AO1 V5 W3 PS1 S4 Q5 V6 Q6 S5 V7 Q7 S6 K8 PPV1 PV4 S7 K9 AO2 K10 W4 PV5 "
    "K11 PV6 V8 W5 W6 PV7 Q8 V9 W7 S8 PS2 Q9 V10 Q10 AO3 S9 V11 PV8 Q11 K12 PPV2 S11 S10 K13 W8 "
    "PV9 K14 K15 W9 PV10 PV11 V12 AO4 Q12 W10 W11 PS3 S12 V13 V15 Q13 Q14 Q15 S13 V14 PV12 S14 "
    "AP0 PPV3 S15 W12 PV13 AP1 PV14 PV15 W13 W14 W15 AP2 ",
    "K0 K1 K2 K3 LA0 V0 Q0 V1 Q1 S0 V2 PS0 Q2 AO0 S1 V3 K4 Q3 S2 PV0 K5 PPV0 S3 K6 PV1 K7 W0 Q4 "
    "W1 PV2 V4 PV3 PS1 AO1 W2 W3 S4 V5 Q5 V6 Q6 S5 V7 Q7 PV4 S6 K8 PPV1 S7 K9 K10 AO2 W4 PV5 "
    "PV6 K11 V8 W5 W6 PV7 Q8 PS2 V9 W7 Q9 S8 V10 Q10 AO3 S9 V11 Q11 PV8 S10 K12 PPV2 S11 K13 "
    "K14 W8 PV9 K15 AO4 PV10 V12 PV11 W10 W9 Q12 PS3 V13 W11 S12 Q13 V14 Q14 S13 V15 Q15 AP0 "
    "S14 PPV3 PV12 S15 AP1 PV13 PV14 W12 PV15 W13 W14 W15 AP2 ",
    "K0 K1 K2 K3 LA0 V0 V1 Q0 Q1 S0 V2 PS0 Q2 AO0 S1 V3 Q3 S2 K4 K5 PPV0 PV0 S3 K6 W0 PV1 K7 "
    "PV2 V4 PV3 W1 W2 Q4 AO1 V5 W3 PS1 S4 Q5 V6 Q6 S5 V7 Q7 S6 K8 S7 PPV1 K9 PV4 AO2 K10 W4 PV5 "
    "PV6 K11 W5 V8 W6 PV7 Q8 W7 V9 PS2 S8 V10 Q9 Q10 AO3 S9 V11 Q11 PV8 S10 K12 PPV2 S11 W8 K13 "
    "PV9 K14 K15 AO4 W9 PV10 PV11 V12 Q12 W10 W11 PS3 S12 Q13 V13 V14 Q14 S13 Q15 PV12 V15 S14 "
    "AP0 PPV3 S15 W12 PV14 PV13 AP1 PV15 W13 W14 W15 AP2 ",
    "K3 K0 K1 K2 LA0 V0 Q0 V1 Q1 S0 V2 PS0 Q2 S1 V3 AO0 S2 K4 PV0 Q3 K5 PPV0 S3 K6 PV1 K7 W0 W1 "
    "PV2 PV3 Q4 V4 W2 W3 AO1 PS1 S4 V5 Q5 V6 Q6 S5 V7 PV4 Q7 S6 K8 S7 K9 AO2 PPV1 K11 K10 W4 "
    "PV5 PV6 V8 W5 PV7 W6 Q8 PS2 V10 V9 W7 S8 Q9 Q10 AO3 S9 V11 Q11 PV8 S10 K12 S11 PPV2 K13 "
    "K14 W8 PV9 K15 AO4 PV10 V12 W9 W10 PV11 Q12 V13 PS3 W11 S12 Q13 V14 S13 V15 Q14 Q15 S14 "
    "AP0 PPV3 PV12 S15 AP1 PV13 PV14 W12 PV15 W13 W14 W15 AP2 ",
)
SKIP_PROLOGUE = False


def _order(u):
    if ORDERS is None or ORDERS[u] is None:
        return _segment_order(u % 2 == 1)
    return [(t.rstrip("0123456789"), int(t.lstrip("ABCDEFGHIJKLMNOPQRSTUVWXYZ")))
            for t in ORDERS[u].split()]


def _nt_dot(a, b):
    return lax.dot_general(a, b, (((1,), (1,)), ((), ())), preferred_element_type=F32)


def _dot(a, b):
    return jnp.dot(a, b, preferred_element_type=F32)


def _pack(x):
    return pltpu.bitcast(x, U32)


def _unpack(x):
    return pltpu.bitcast(x, BF16)


def _recip(x):
    r = pl.reciprocal(x, approx=True)
    return r * (2.0 - x * r)


def _kernel(ax_hbm, awqkv_hbm, awo_hbm, bx_hbm, bx4_hbm, mem0_hbm, wq_hbm, wk_hbm, wv_hbm, wo_hbm,
            out_hbm,
            stage, awo_raw, w_s, wo_s, pre_s, odef_s, out_s,
            xa_s, xb_s, xpre_s, mem0_s, wa_s, awo_s, t1_s, qa_s, kv_s,
            ring_sem, misc_sem, out_sem):
    b_scale = B_DH ** (-0.5) * LOG2E
    a_scale = A_DH ** (-0.5) * LOG2E

    w_hbm = (wq_hbm, wk_hbm, wv_hbm)
    wo32 = wo_hbm.bitcast(U32)
    awo32 = awo_hbm.bitcast(U32)
    hw = PW // 2
    hd = B_H * B_DH

    def w_copy(p, half, q, m):
        rows = pl.ds(pl.multiple_of(p * PW, PW), PW)
        return pltpu.make_async_copy(w_hbm[m].at[rows, :], stage.at[half, q, m],
                                     ring_sem.at[half, q, m])

    def wa_copy(piece, half, q):
        return pltpu.make_async_copy(
            awqkv_hbm.at[pl.ds(pl.multiple_of((piece % NT) * 128, 128), 128),
                         pl.ds(pl.multiple_of((piece // NT) * D, 128), D)],
            stage.at[half, q, 3, :128], ring_sem.at[half, q, 3])

    def trip_copies(g):
        half = g % 2
        src = jnp.minimum(g, NTRIP - 1)
        cps = []
        for q in range(PP):
            cps += [w_copy((src + 1) * PP + q, half, q, m) for m in range(3)]
            cps.append(wa_copy(1 + src * PP + q, half, q))
        return cps

    x0 = S - NTRIP * X_ROWS
    wo0 = hd // 2 - NTRIP * WO_ROWS

    def bulk_copies(xr, wr):
        return [
            pltpu.make_async_copy(ax_hbm.at[xr, :], xa_s.at[xr, :], misc_sem.at[0]),
            pltpu.make_async_copy(bx_hbm.at[xr, :], xb_s.at[xr, :], misc_sem.at[1]),
            pltpu.make_async_copy(wo32.at[wr, :], wo_s.at[wr, :], misc_sem.at[2]),
        ]

    xpre_cp = pltpu.make_async_copy(bx4_hbm.at[:, 0], xpre_s, misc_sem.at[3])
    mem_cp = pltpu.make_async_copy(mem0_hbm, mem0_s, misc_sem.at[4])
    awo_cps = [pltpu.make_async_copy(awo32.at[:, c * 128:(c + 1) * 128], awo_raw.at[c],
                                     misc_sem.at[5 + c]) for c in range(NT)]

    xpre_cp.start()
    for q in range(PP):
        for m in range(3):
            w_copy(q, 1, q, m).start(priority=1)
    wa_copy(0, 1, 0).start(priority=1)
    for cp in trip_copies(0):
        cp.start(priority=1)
    for cp in bulk_copies(pl.ds(0, x0), pl.ds(0, wo0)):
        cp.start(priority=1)
    mem_cp.start(priority=1)
    for cp in awo_cps:
        cp.start(priority=1)
    kv_s[:, :, :A_HALO, :] = jnp.zeros((2, NT, A_HALO, 128), F32)

    def gather_heads(ref):
        rows = []
        for j in range(A_DH // 2):
            u = ref[pl.ds(j, A_H, stride=A_DH // 2), :]
            rows.append(pltpu.bitcast(u << 16, F32))
            rows.append(pltpu.bitcast(u & jnp.uint32(0xFFFF0000), F32))
        return jnp.concatenate(rows, axis=0)

    def pair_prep(p, half, q, m, chunks=1):
        if SKIP_PROLOGUE:
            return
        wt = stage[half, q, m]
        w_s[p, :, m * PW:(m + 1) * PW] = _pack(wt.T)
        n = NSEG // chunks
        for c in range(chunks):
            xp = xpre_s[c * n:(c + 1) * n].reshape(n * PRE, D)
            pre_s[c * n:(c + 1) * n, p, :, m * PW:(m + 1) * PW] = (
                _nt_dot(xp, wt).reshape(n, PRE, PW))

    def wa_prep(piece, half, q):
        t1_s[q] = _pack(stage[half, q, 3, :128].T)
        wa_s[piece // NT, pl.ds(pl.multiple_of((piece % NT) * 64, 64), 64), :] = (
            _pack(gather_heads(t1_s.at[q]).astype(BF16).T))

    xpre_cp.wait()
    w_copy(0, 1, 0, 0).wait()
    pair_prep(0, 1, 0, 0, PEEL_CHUNKS)
    for m in (1, 2):
        w_copy(0, 1, 0, m).wait()
    for m in (1, 2):
        pair_prep(0, 1, 0, m, PEEL_CHUNKS)
    for q in range(1, PP):
        for m in range(3):
            w_copy(q, 1, q, m).wait()
    wa_copy(0, 1, 0).wait()
    for q in range(1, PP):
        for m in range(3):
            pair_prep(q, 1, q, m, PEEL_CHUNKS)
    wa_prep(0, 1, 0)

    def prologue(g, carry):
        half = g % 2
        for cp in bulk_copies(pl.ds(pl.multiple_of(x0 + g * X_ROWS, 16), X_ROWS),
                              pl.ds(pl.multiple_of(wo0 + g * WO_ROWS, 8), WO_ROWS)):
            cp.start()
        for cp in trip_copies(g):
            cp.wait()
        for q in range(PP):
            for m in range(3):
                pair_prep((g + 1) * PP + q, half, q, m)
                if q == 0 and m == 0:
                    for cp in trip_copies(g + 1):
                        cp.start(priority=1)
            wa_prep(1 + g * PP + q, half, q)
        return carry

    lax.fori_loop(0, NTRIP, prologue, 0)

    pltpu.make_async_copy(ax_hbm, xa_s, misc_sem.at[0]).wait()
    pltpu.make_async_copy(bx_hbm, xb_s, misc_sem.at[1]).wait()
    pltpu.make_async_copy(wo32, wo_s, misc_sem.at[2]).wait()
    mem_cp.wait()
    for cp in awo_cps:
        cp.wait()

    def a_store(m, r):
        for j in range(NT):
            t = r[:, j * 128:(j + 1) * 128]
            if m == 0:
                qa_s[j] = t * a_scale
            else:
                kv_s[m - 1, j, A_HALO:, :] = t

    for m in range(3):
        a_store(m, _dot(xa_s[:SEG, :], _unpack(wa_s[m])))
    for c in range(NT):
        awo_s[:, c * 128:(c + 1) * 128] = _pack(gather_heads(awo_raw.at[c]).astype(BF16))

    def segment(s, mem, u):
        odd = u % 2 == 1
        row0 = pl.multiple_of(s * SEG, SEG)
        ninf = jnp.float32(-jnp.inf)

        qi = lax.broadcasted_iota(jnp.int32, (SEG, 2 * L), 0)
        kl = lax.broadcasted_iota(jnp.int32, (SEG, 2 * L), 1)
        is_a = kl < L
        kpos = jnp.where(is_a, kl, kl - L)
        allowed = (qi >= FRESH) | (qi + MEM + PRE >= kpos)
        pi = lax.broadcasted_iota(jnp.int32, (GP * PRE, 128), 0)
        pk = lax.broadcasted_iota(jnp.int32, (GP * PRE, 128), 1)
        p_own = (pk // SEG) == (pi // PRE)
        p_allowed = (pk % (MEM + PRE)) <= (pi % PRE) + MEM
        p_first = (pk % SEG) < MEM + PRE
        p_is_a = p_own & p_first
        p_is_b = p_own & jnp.logical_not(p_first)
        col_a = lax.broadcasted_iota(jnp.int32, (1, PW), 1) < B_DH
        col128_a = lax.broadcasted_iota(jnp.int32, (1, 128), 1) < (B_DH - 128)

        xb = xb_s[pl.ds(row0, SEG), :].astype(F32)
        h = jnp.concatenate([xb[PRE:], mem], axis=0).astype(BF16)

        def proj(p, m):
            return _dot(h, _unpack(w_s[p, :, m * PW:(m + 1) * PW]))

        def pre(p, m):
            return pre_s[s, p, :, m * PW:(m + 1) * PW]

        def block_diag(p, m):
            f = proj(p, m)
            full = jnp.concatenate([f[FRESH:], pre(p, m), f[:FRESH]], axis=0)
            z = jnp.zeros_like(full)
            return jnp.where(col_a, full, z), jnp.where(col_a, z, full)

        def cat(parts):
            return jnp.concatenate(parts, axis=0)

        def qk(q, blocks):
            if not FOLD_T:
                return _dot(q, cat(blocks).T.astype(BF16))
            fold = cat([jnp.concatenate([x[:, :128] if i % 2 == 0 else x[:, 256:], x[:, 128:256]],
                                        axis=1) for i, x in enumerate(blocks)])
            if T_F32:
                t = fold.T
            else:
                t = fold.astype(BF16).T.astype(F32)
            outer = t[:128]
            n = blocks[0].shape[0]
            lane = lax.broadcasted_iota(jnp.int32, outer.shape, 1)
            lane_a = lane < n if len(blocks) == 2 else lane % (2 * n) < n
            z = jnp.zeros_like(outer)
            kt = cat([jnp.where(lane_a, outer, z), t[128:], jnp.where(lane_a, z, outer)])
            return _dot(q, kt.astype(BF16))

        def scores(q, kbd, late_norm):
            sc = qk(q, kbd) * b_scale
            sc = jnp.where(allowed, sc, NEG)
            ma = jnp.max(jnp.where(is_a, sc, ninf), axis=1, keepdims=True)
            mb = jnp.max(jnp.where(is_a, ninf, sc), axis=1, keepdims=True)
            e = jnp.exp2(sc - jnp.where(is_a, ma, mb))
            sa = jnp.sum(jnp.where(is_a, e, 0.0), axis=1, keepdims=True)
            sb = jnp.sum(jnp.where(is_a, 0.0, e), axis=1, keepdims=True)
            def fin(x):
                if PV_PAD:
                    x = jnp.concatenate([x, jnp.zeros((SEG, 128 - 2 * L), F32)], axis=1)
                return x.astype(BF16)
            if late_norm:
                return fin(e), _recip(sa), _recip(sb)
            return fin(e * _recip(jnp.where(is_a, sa, sb))), None, None

        def pv(sm, vbd):
            e, ra, rb = sm
            if PV_PAD:
                vbd = list(vbd) + [jnp.zeros((128 - 2 * L, PW), F32)]
            o = _dot(e, cat(vbd).astype(BF16))
            if ra is not None:
                o = jnp.concatenate([
                    o[:, :128] * ra,
                    o[:, 128:256] * jnp.where(col128_a, ra, rb),
                    o[:, 256:] * rb], axis=1)
            return o

        def pre_scores(g, kbds):
            q = jnp.concatenate([pre(GP * g + r, 0) for r in range(GP)], axis=0).astype(BF16)
            k = [x[:MEM + PRE] for kb in kbds for x in kb]
            sc = qk(q, k) * b_scale
            sc = jnp.where(p_allowed, sc, NEG)
            ma = jnp.max(jnp.where(p_is_a, sc, ninf), axis=1, keepdims=True)
            mb = jnp.max(jnp.where(p_is_b, sc, ninf), axis=1, keepdims=True)
            e = jnp.where(p_own, jnp.exp2(sc - jnp.where(p_first, ma, mb)), 0.0)
            sa = jnp.sum(jnp.where(p_first, e, 0.0), axis=1, keepdims=True)
            sb = jnp.sum(jnp.where(p_first, 0.0, e), axis=1, keepdims=True)
            return (e * _recip(jnp.where(p_first, sa, sb))).astype(BF16)

        def pre_pv(g, pr, vbds):
            v = cat([x[:MEM + PRE] for vb in vbds for x in vb])
            o = _dot(pr, v.astype(BF16))
            if not odd:
                odef_s[g] = o
            return o

        def wout(p, o, opre, acc):
            if odd:
                r = pl.ds((p % GP) * PRE, PRE)
                o = jnp.concatenate(
                    [o, opre[(p % GP) * PRE:(p % GP + 1) * PRE], odef_s[p // GP, r, :]], axis=0)
            contrib = _dot(o.astype(BF16), _unpack(wo_s[p * hw:(p + 1) * hw, :]))
            return contrib if acc is None else acc + contrib

        def window(m, j, w):
            lo = A_HALO - A_DIL * w
            return kv_s[m, j, lo:lo + SEG, :]

        def local_softmax():
            pos = row0 + lax.broadcasted_iota(jnp.int32, (SEG, 128), 0)
            logits = []
            for w in range(A_W):
                t = qa_s[0] * window(0, 0, w)
                for j in range(1, NT):
                    t = t + qa_s[j] * window(0, j, w)
                t = t + pltpu.roll(t, 64, 1)
                t = t + pltpu.roll(t, 32, 1)
                logits.append(t if w == 0 else jnp.where(pos >= A_DIL * w, t, NEG))
            mx = functools.reduce(jnp.maximum, logits)
            es = [jnp.exp2(l - mx) for l in logits]
            inv = _recip(functools.reduce(lambda u, v: u + v, es))
            return es, inv

        def local_out(j, es, inv, acc):
            o = es[0] * window(1, j, 0)
            for w in range(1, A_W):
                o = o + es[w] * window(1, j, w)
            for m in range(2):
                kv_s[m, j, :A_HALO, :] = kv_s[m, j, SEG:, :]
            r = _dot((o * inv).astype(BF16), _unpack(awo_s[j * 64:(j + 1) * 64, :]))
            return r if acc is None else acc + r

        nxt = pl.multiple_of(jnp.minimum(s + 1, NSEG - 1) * SEG, SEG)

        val = {}
        acc = None
        oa = None
        for kind, t in _order(u):
            if kind == "K":
                val[kind, t] = block_diag(t, 1)
            elif kind == "V":
                val[kind, t] = block_diag(t, 2)
            elif kind == "Q":
                val[kind, t] = proj(t, 0).astype(BF16)
            elif kind == "S":
                val[kind, t] = scores(val["Q", t], val["K", t], t >= LATE_FROM)
            elif kind == "PV":
                val[kind, t] = pv(val["S", t], val["V", t])
            elif kind == "PS":
                val[kind, t] = pre_scores(t, [val["K", GP * t + r] for r in range(GP)])
            elif kind == "PPV":
                val[kind, t] = pre_pv(t, val["PS", t], [val["V", GP * t + r] for r in range(GP)])
            elif kind == "W":
                acc = wout(t, val["PV", t], val.get(("PPV", t // GP)), acc)
            elif kind == "LA":
                la = local_softmax()
            elif kind == "AP":
                a_store(t, _dot(xa_s[pl.ds(nxt, SEG), :], _unpack(wa_s[t])))
            elif kind == "AO":
                oa = local_out(t, la[0], la[1], oa)
                if t == NT - 1:
                    out_s[pl.ds(row0, SEG), :D] = oa.astype(BF16)
        return acc

    def out_copy(i):
        r = pl.ds(pl.multiple_of(i * 2 * SEG, 2 * SEG), 2 * SEG)
        return pltpu.make_async_copy(out_s.at[r, :], out_hbm.at[r, :], out_sem)

    def step(i, mem, u):
        acc0 = segment(2 * i, mem, 2 * u)
        acc1 = segment(2 * i + 1, acc0[FRESH:], 2 * u + 1)
        res = jnp.concatenate([acc1[SEG + PRE:], acc0[:FRESH], acc1[SEG:SEG + PRE], acc1[:FRESH]],
                              axis=0)
        out_s[pl.ds(pl.multiple_of(i * 2 * SEG, 2 * SEG), 2 * SEG), D:] = res.astype(BF16)
        out_copy(i).start()
        return acc1[FRESH:SEG]

    def steps(i, mem):
        for u in range(UNR):
            mem = step(i * UNR + u, mem, u)
        return mem

    lax.fori_loop(0, N_STEPS, steps, mem0_s[...].astype(F32))

    for cp in trip_copies(NTRIP):
        cp.wait()

    def wait_out(i, carry):
        out_copy(i).wait()
        return carry

    lax.fori_loop(0, N_STEPS * UNR, wait_out, 0)


@jax.jit
def pallas_concat_heads__sliding_local_dilated__memory_aug_recurrent_mem_tr__prompt_kernel(
    A_x: jax.Array,
    A_wqkv: jax.Array,
    A_wo: jax.Array,
    B_x: jax.Array,
    B_mem0: jax.Array,
    B_Wq: jax.Array,
    B_Wk: jax.Array,
    B_Wv: jax.Array,
    B_Wo: jax.Array,
    B_seg_len,
):
    del B_seg_len
    assert A_x.shape == (1, S, D) and B_x.shape == (1, S, D)
    hd = B_H * B_DH
    wq_t = jnp.transpose(B_Wq, (1, 2, 0)).reshape(hd, D)
    wk_t = jnp.transpose(B_Wk, (1, 2, 0)).reshape(hd, D)
    wv_t = jnp.transpose(B_Wv, (1, 2, 0)).reshape(hd, D)
    wo = B_Wo.reshape(hd, D)

    any_spec = pl.BlockSpec(memory_space=pl.ANY)
    out = pl.pallas_call(
        _kernel,
        out_shape=jax.ShapeDtypeStruct((S, 2 * D), BF16),
        in_specs=[any_spec] * 10,
        out_specs=any_spec,
        scratch_shapes=[
            pltpu.VMEM((2, PP, 4, PW, D), BF16),
            pltpu.VMEM((NT, D // 2, 128), U32),
            pltpu.VMEM((NP, D // 2, 3 * PW), U32),
            pltpu.VMEM((hd // 2, D), U32),
            pltpu.VMEM((NSEG, NP, PRE, 3 * PW), F32),
            pltpu.VMEM((NG, GP * PRE, PW), F32),
            pltpu.VMEM((S, 2 * D), BF16),
            pltpu.VMEM((S, D), BF16),
            pltpu.VMEM((S, D), BF16),
            pltpu.VMEM((NSEG, PRE, D), BF16),
            pltpu.VMEM((MEM, D), BF16),
            pltpu.VMEM((3, D // 2, D), U32),
            pltpu.VMEM((D // 2, D), U32),
            pltpu.VMEM((PP, D // 2, 128), U32),
            pltpu.VMEM((NT, SEG, 128), F32),
            pltpu.VMEM((2, NT, A_HALO + SEG, 128), F32),
            pltpu.SemaphoreType.DMA((2, PP, 4)),
            pltpu.SemaphoreType.DMA((5 + NT,)),
            pltpu.SemaphoreType.DMA,
        ],
        compiler_params=pltpu.CompilerParams(vmem_limit_bytes=120 * 1024 * 1024,
                                             disable_bounds_checks=True),
    )(A_x.reshape(S, D), A_wqkv, A_wo, B_x.reshape(S, D), B_x.reshape(NSEG, SEG // PRE, PRE, D),
      B_mem0.reshape(MEM, D), wq_t, wk_t, wv_t, wo)
    return out.reshape(1, S, 2 * D)
```

```python
import functools

import jax
import jax.numpy as jnp
from jax import lax
import jax.experimental.pallas as pl
import jax.experimental.pallas.tpu as pltpu

F32 = jnp.float32
BF16 = jnp.bfloat16
U32 = jnp.uint32

S = 2048
D = 640
NT = D // 128
A_H = 32
A_DH = D // A_H
A_W = 8
A_DIL = 2
A_HALO = 16
B_H = 32
B_DH = 192
MEM = 8
SEG = 32
NSEG = S // SEG
NP = B_H // 2
PW = 2 * B_DH
PRE = 8
FRESH = SEG - PRE
L = MEM + SEG
GP = 4
NG = NP // GP
LOG2E = 1.4426950408889634
NEG = -1000000000.0 * LOG2E
PP = 2
NTRIP = NP // PP - 1
PEEL_CHUNKS = 4
X_ROWS = 288
WO_ROWS = 432
X_W = 1024
OUT_W = 2048
UNR = 2
N_STEPS = NSEG // 2 // UNR

LAT_MM, LAT_SM, LAT_SM_LATE, LAT_T = 190, 650, 330, 600
LATE_FROM = NP - 2
AO_AFTER = (10, 18, 26, 34, 40)
FOLD_T = True
PV_PAD = False
XLU_T_PRE = True
T_F32 = True
XLU_T_MAIN = True


def _segment_order(odd):
    proj = []
    for g in range(NG):
        proj += [("K", GP * g + r) for r in range(GP)]
        for r in range(GP):
            proj += [("V", GP * g + r), ("Q", GP * g + r)]
    dur = {"K": 120, "V": 120, "Q": 120, "S": 24, "PV": 24, "PS": 24, "PPV": 24,
           "W": 180 if odd else 120, "AO": 40, "AP": 200}
    end = {}

    def ready(task):
        k, i = task
        if k == "S":
            deps = [(("Q", i), LAT_MM), (("K", i), LAT_T if XLU_T_MAIN else LAT_MM)]
        elif k == "PV":
            deps = [(("S", i), LAT_SM_LATE if i >= LATE_FROM else LAT_SM), (("V", i), LAT_MM)]
        elif k == "PS":
            deps = [(("K", GP * i + GP - 1), LAT_T if XLU_T_PRE else LAT_MM)]
        elif k == "PPV":
            deps = [(("PS", i), LAT_SM), (("V", GP * i + GP - 1), LAT_MM)]
        else:
            deps = [(("PV", i), LAT_MM)] + ([(("PPV", i // GP), LAT_MM)] if odd else [])
        if any(d not in end for d, _ in deps):
            return None
        return max(end[d] + lat for d, lat in deps)

    pend = ([("W", p) for p in range(NP)] + [("PPV", g) for g in range(NG)]
            + [("PV", p) for p in range(NP)] + [("PS", g) for g in range(NG)]
            + [("S", p) for p in range(NP)])
    fill = [("AP", 0), ("AP", 1)]
    order = []
    now = [0]

    def emit(task):
        order.append(task)
        now[0] += dur[task[0]]
        end[task] = now[0]

    nproj = 0
    while pend:
        cand = [x for x in pend if ready(x) is not None and ready(x) <= now[0]]
        if cand:
            if not proj:
                cand = [x for x in cand if x[0] != "W"] or cand
            pend.remove(cand[0])
            emit(cand[0])
        elif proj:
            emit(proj.pop(0))
            nproj += 1
            if nproj == GP:
                order.append(("LA", 0))
            if nproj in AO_AFTER:
                emit(("AO", AO_AFTER.index(nproj)))
        elif fill:
            emit(fill.pop(0))
        else:
            now[0] = min(ready(x) for x in pend if ready(x) is not None)
    return order + fill + [("AP", 2)]


ORDERS = (
    "K0 K1 K2 K3 V0 LA0 Q1 Q0 V1 S0 V2 PS0 Q2 AO0 S1 V3 Q3 S2 PV0 K4 K5 PPV0 S3 K6 W0 PV1 K7 "
    "PV2 V4 W1 W2 PV3 Q4 AO1 V5 W3 PS1 S4 Q5 V6 Q6 S5 V7 Q7 S6 K8 PPV1 PV4 S7 K9 AO2 K10 W4 PV5 "
    "K11 PV6 V8 W5 W6 PV7 Q8 V9 W7 S8 PS2 Q9 V10 Q10 AO3 S9 V11 PV8 Q11 K12 PPV2 S11 S10 K13 W8 "
    "PV9 K14 K15 W9 PV10 PV11 V12 AO4 Q12 W10 W11 PS3 S12 V13 V15 Q13 Q14 Q15 S13 V14 PV12 S14 "
    "AP0 PPV3 S15 W12 PV13 AP1 PV14 PV15 W13 W14 W15 AP2 ",
    "K0 K1 K2 K3 LA0 V0 Q0 V1 Q1 S0 V2 PS0 Q2 AO0 S1 V3 K4 Q3 S2 PV0 K5 PPV0 S3 K6 PV1 K7 W0 Q4 "
    "W1 PV2 V4 PV3 PS1 AO1 W2 W3 S4 V5 Q5 V6 Q6 S5 V7 Q7 PV4 S6 K8 PPV1 S7 K9 K10 AO2 W4 PV5 "
    "PV6 K11 V8 W5 W6 PV7 Q8 PS2 V9 W7 Q9 S8 V10 Q10 AO3 S9 V11 Q11 PV8 S10 K12 PPV2 S11 K13 "
    "K14 W8 PV9 K15 AO4 PV10 V12 PV11 W10 W9 Q12 PS3 V13 W11 S12 Q13 V14 Q14 S13 V15 Q15 AP0 "
    "S14 PPV3 PV12 S15 AP1 PV13 PV14 W12 PV15 W13 W14 W15 AP2 ",
    "K0 K1 K2 K3 LA0 V0 V1 Q0 Q1 S0 V2 PS0 Q2 AO0 S1 V3 Q3 S2 K4 K5 PPV0 PV0 S3 K6 W0 PV1 K7 "
    "PV2 V4 PV3 W1 W2 Q4 AO1 V5 W3 PS1 S4 Q5 V6 Q6 S5 V7 Q7 S6 K8 S7 PPV1 K9 PV4 AO2 K10 W4 PV5 "
    "PV6 K11 W5 V8 W6 PV7 Q8 W7 V9 PS2 S8 V10 Q9 Q10 AO3 S9 V11 Q11 PV8 S10 K12 PPV2 S11 W8 K13 "
    "PV9 K14 K15 AO4 W9 PV10 PV11 V12 Q12 W10 W11 PS3 S12 Q13 V13 V14 Q14 S13 Q15 PV12 V15 S14 "
    "AP0 PPV3 S15 W12 PV14 PV13 AP1 PV15 W13 W14 W15 AP2 ",
    "K3 K0 K1 K2 LA0 V0 Q0 V1 Q1 S0 V2 PS0 Q2 S1 V3 AO0 S2 K4 PV0 Q3 K5 PPV0 S3 K6 PV1 K7 W0 W1 "
    "PV2 PV3 Q4 V4 W2 W3 AO1 PS1 S4 V5 Q5 V6 Q6 S5 V7 PV4 Q7 S6 K8 S7 K9 AO2 PPV1 K11 K10 W4 "
    "PV5 PV6 V8 W5 PV7 W6 Q8 PS2 V10 V9 W7 S8 Q9 Q10 AO3 S9 V11 Q11 PV8 S10 K12 S11 PPV2 K13 "
    "K14 W8 PV9 K15 AO4 PV10 V12 W9 W10 PV11 Q12 V13 PS3 W11 S12 Q13 V14 S13 V15 Q14 Q15 S14 "
    "AP0 PPV3 PV12 S15 AP1 PV13 PV14 W12 PV15 W13 W14 W15 AP2 ",
)
SKIP_PROLOGUE = False


def _order(u):
    if ORDERS is None or ORDERS[u] is None:
        return _segment_order(u % 2 == 1)
    return [(t.rstrip("0123456789"), int(t.lstrip("ABCDEFGHIJKLMNOPQRSTUVWXYZ")))
            for t in ORDERS[u].split()]


def _nt_dot(a, b):
    return lax.dot_general(a, b, (((1,), (1,)), ((), ())), preferred_element_type=F32)


def _dot(a, b):
    return jnp.dot(a, b, preferred_element_type=F32)


def _pack(x):
    return pltpu.bitcast(x, U32)


def _unpack(x):
    return pltpu.bitcast(x, BF16)


def _recip(x):
    r = pl.reciprocal(x, approx=True)
    return r * (2.0 - x * r)


def _kernel(ax_hbm, awqkv_hbm, awo_hbm, bx_hbm, bx4_hbm, mem0_hbm, wq_hbm, wk_hbm, wv_hbm, wo_hbm,
            out_hbm,
            stage, awo_raw, w_s, wo_s, pre_s, odef_s, out_s,
            xa_s, xb_s, xpre_s, mem0_s, wa_s, awo_s, t1_s, qa_s, kv_s,
            ring_sem, misc_sem, out_sem):
    b_scale = B_DH ** (-0.5) * LOG2E
    a_scale = A_DH ** (-0.5) * LOG2E

    w_hbm = (wq_hbm, wk_hbm, wv_hbm)
    wo32 = wo_hbm.bitcast(U32)
    awo32 = awo_hbm.bitcast(U32)
    hw = PW // 2
    hd = B_H * B_DH

    def w_copy(p, half, q, m):
        rows = pl.ds(pl.multiple_of(p * PW, PW), PW)
        return pltpu.make_async_copy(w_hbm[m].at[rows, :], stage.at[half, q, m],
                                     ring_sem.at[half, q, m])

    def wa_copy(piece, half, q):
        return pltpu.make_async_copy(
            awqkv_hbm.at[pl.ds(pl.multiple_of((piece % NT) * 128, 128), 128),
                         pl.ds(pl.multiple_of((piece // NT) * D, 128), D)],
            stage.at[half, q, 3, :128], ring_sem.at[half, q, 3])

    def trip_copies(g):
        half = g % 2
        src = jnp.minimum(g, NTRIP - 1)
        cps = []
        for q in range(PP):
            cps += [w_copy((src + 1) * PP + q, half, q, m) for m in range(3)]
            cps.append(wa_copy(1 + src * PP + q, half, q))
        return cps

    x0 = S - NTRIP * X_ROWS
    wo0 = hd // 2 - NTRIP * WO_ROWS

    def bulk_copies(xr, wr):
        return [
            pltpu.make_async_copy(ax_hbm.at[xr, :], xa_s.at[xr, :D], misc_sem.at[0]),
            pltpu.make_async_copy(bx_hbm.at[xr, :], xb_s.at[xr, :D], misc_sem.at[1]),
            pltpu.make_async_copy(wo32.at[wr, :], wo_s.at[wr, :], misc_sem.at[2]),
        ]

    xpre_cp = pltpu.make_async_copy(bx4_hbm.at[:, 0], xpre_s, misc_sem.at[3])
    mem_cp = pltpu.make_async_copy(mem0_hbm, mem0_s, misc_sem.at[4])
    awo_cps = [pltpu.make_async_copy(awo32.at[:, c * 128:(c + 1) * 128], awo_raw.at[c],
                                     misc_sem.at[5 + c]) for c in range(NT)]

    xpre_cp.start()
    for q in range(PP):
        for m in range(3):
            w_copy(q, 1, q, m).start(priority=1)
    wa_copy(0, 1, 0).start(priority=1)
    for cp in trip_copies(0):
        cp.start(priority=1)
    for cp in bulk_copies(pl.ds(0, x0), pl.ds(0, wo0)):
        cp.start(priority=1)
    mem_cp.start(priority=1)
    for cp in awo_cps:
        cp.start(priority=1)
    kv_s[:, :, :A_HALO, :] = jnp.zeros((2, NT, A_HALO, 128), F32)

    def gather_heads(ref):
        rows = []
        for j in range(A_DH // 2):
            u = ref[pl.ds(j, A_H, stride=A_DH // 2), :]
            rows.append(pltpu.bitcast(u << 16, F32))
            rows.append(pltpu.bitcast(u & jnp.uint32(0xFFFF0000), F32))
        return jnp.concatenate(rows, axis=0)

    def pair_prep(p, half, q, m, chunks=1):
        if SKIP_PROLOGUE:
            return
        wt = stage[half, q, m]
        w_s[p, :, m * PW:(m + 1) * PW] = _pack(wt.T)
        n = NSEG // chunks
        for c in range(chunks):
            xp = xpre_s[c * n:(c + 1) * n].reshape(n * PRE, D)
            pre_s[c * n:(c + 1) * n, p, :, m * PW:(m + 1) * PW] = (
                _nt_dot(xp, wt).reshape(n, PRE, PW))

    def wa_prep(piece, half, q):
        t1_s[q] = _pack(stage[half, q, 3, :128].T)
        wa_s[piece // NT, pl.ds(pl.multiple_of((piece % NT) * 64, 64), 64), :] = (
            _pack(gather_heads(t1_s.at[q]).astype(BF16).T))

    xpre_cp.wait()
    w_copy(0, 1, 0, 0).wait()
    pair_prep(0, 1, 0, 0, PEEL_CHUNKS)
    for m in (1, 2):
        w_copy(0, 1, 0, m).wait()
    for m in (1, 2):
        pair_prep(0, 1, 0, m, PEEL_CHUNKS)
    for q in range(1, PP):
        for m in range(3):
            w_copy(q, 1, q, m).wait()
    wa_copy(0, 1, 0).wait()
    for q in range(1, PP):
        for m in range(3):
            pair_prep(q, 1, q, m, PEEL_CHUNKS)
    wa_prep(0, 1, 0)

    def prologue(g, carry):
        half = g % 2
        for cp in bulk_copies(pl.ds(pl.multiple_of(x0 + g * X_ROWS, 16), X_ROWS),
                              pl.ds(pl.multiple_of(wo0 + g * WO_ROWS, 8), WO_ROWS)):
            cp.start()
        for cp in trip_copies(g):
            cp.wait()
        for q in range(PP):
            for m in range(3):
                pair_prep((g + 1) * PP + q, half, q, m)
                if q == 0 and m == 0:
                    for cp in trip_copies(g + 1):
                        cp.start(priority=1)
            wa_prep(1 + g * PP + q, half, q)
        return carry

    lax.fori_loop(0, NTRIP, prologue, 0)

    pltpu.make_async_copy(ax_hbm, xa_s.at[:, :D], misc_sem.at[0]).wait()
    pltpu.make_async_copy(bx_hbm, xb_s.at[:, :D], misc_sem.at[1]).wait()
    pltpu.make_async_copy(wo32, wo_s, misc_sem.at[2]).wait()
    mem_cp.wait()
    for cp in awo_cps:
        cp.wait()

    def a_store(m, r):
        for j in range(NT):
            t = r[:, j * 128:(j + 1) * 128]
            if m == 0:
                qa_s[j] = t * a_scale
            else:
                kv_s[m - 1, j, A_HALO:, :] = t

    for m in range(3):
        a_store(m, _dot(xa_s[:SEG, :D], _unpack(wa_s[m])))
    for c in range(NT):
        awo_s[:, c * 128:(c + 1) * 128] = _pack(gather_heads(awo_raw.at[c]).astype(BF16))

    def segment(s, mem, u):
        odd = u % 2 == 1
        row0 = pl.multiple_of(s * SEG, SEG)
        ninf = jnp.float32(-jnp.inf)

        qi = lax.broadcasted_iota(jnp.int32, (SEG, 2 * L), 0)
        kl = lax.broadcasted_iota(jnp.int32, (SEG, 2 * L), 1)
        is_a = kl < L
        kpos = jnp.where(is_a, kl, kl - L)
        allowed = (qi >= FRESH) | (qi + MEM + PRE >= kpos)
        pi = lax.broadcasted_iota(jnp.int32, (GP * PRE, 128), 0)
        pk = lax.broadcasted_iota(jnp.int32, (GP * PRE, 128), 1)
        p_own = (pk // SEG) == (pi // PRE)
        p_allowed = (pk % (MEM + PRE)) <= (pi % PRE) + MEM
        p_first = (pk % SEG) < MEM + PRE
        p_is_a = p_own & p_first
        p_is_b = p_own & jnp.logical_not(p_first)
        col_a = lax.broadcasted_iota(jnp.int32, (1, PW), 1) < B_DH
        col128_a = lax.broadcasted_iota(jnp.int32, (1, 128), 1) < (B_DH - 128)

        xb = xb_s[pl.ds(row0, SEG), :D].astype(F32)
        h = jnp.concatenate([xb[PRE:], mem], axis=0).astype(BF16)

        def proj(p, m):
            return _dot(h, _unpack(w_s[p, :, m * PW:(m + 1) * PW]))

        def pre(p, m):
            return pre_s[s, p, :, m * PW:(m + 1) * PW]

        def block_diag(p, m):
            f = proj(p, m)
            full = jnp.concatenate([f[FRESH:], pre(p, m), f[:FRESH]], axis=0)
            z = jnp.zeros_like(full)
            return jnp.where(col_a, full, z), jnp.where(col_a, z, full)

        def cat(parts):
            return jnp.concatenate(parts, axis=0)

        def qk(q, blocks):
            if not FOLD_T:
                return _dot(q, cat(blocks).T.astype(BF16))
            fold = cat([jnp.concatenate([x[:, :128] if i % 2 == 0 else x[:, 256:], x[:, 128:256]],
                                        axis=1) for i, x in enumerate(blocks)])
            if T_F32:
                t = fold.T
            else:
                t = fold.astype(BF16).T.astype(F32)
            outer = t[:128]
            n = blocks[0].shape[0]
            lane = lax.broadcasted_iota(jnp.int32, outer.shape, 1)
            lane_a = lane < n if len(blocks) == 2 else lane % (2 * n) < n
            z = jnp.zeros_like(outer)
            kt = cat([jnp.where(lane_a, outer, z), t[128:], jnp.where(lane_a, z, outer)])
            return _dot(q, kt.astype(BF16))

        def scores(q, kbd, late_norm):
            sc = qk(q, kbd) * b_scale
            sc = jnp.where(allowed, sc, NEG)
            ma = jnp.max(jnp.where(is_a, sc, ninf), axis=1, keepdims=True)
            mb = jnp.max(jnp.where(is_a, ninf, sc), axis=1, keepdims=True)
            e = jnp.exp2(sc - jnp.where(is_a, ma, mb))
            sa = jnp.sum(jnp.where(is_a, e, 0.0), axis=1, keepdims=True)
            sb = jnp.sum(jnp.where(is_a, 0.0, e), axis=1, keepdims=True)
            def fin(x):
                if PV_PAD:
                    x = jnp.concatenate([x, jnp.zeros((SEG, 128 - 2 * L), F32)], axis=1)
                return x.astype(BF16)
            if late_norm:
                return fin(e), _recip(sa), _recip(sb)
            return fin(e * _recip(jnp.where(is_a, sa, sb))), None, None

        def pv(sm, vbd):
            e, ra, rb = sm
            if PV_PAD:
                vbd = list(vbd) + [jnp.zeros((128 - 2 * L, PW), F32)]
            o = _dot(e, cat(vbd).astype(BF16))
            if ra is not None:
                o = jnp.concatenate([
                    o[:, :128] * ra,
                    o[:, 128:256] * jnp.where(col128_a, ra, rb),
                    o[:, 256:] * rb], axis=1)
            return o

        def pre_scores(g, kbds):
            q = jnp.concatenate([pre(GP * g + r, 0) for r in range(GP)], axis=0).astype(BF16)
            k = [x[:MEM + PRE] for kb in kbds for x in kb]
            sc = qk(q, k) * b_scale
            sc = jnp.where(p_allowed, sc, NEG)
            ma = jnp.max(jnp.where(p_is_a, sc, ninf), axis=1, keepdims=True)
            mb = jnp.max(jnp.where(p_is_b, sc, ninf), axis=1, keepdims=True)
            e = jnp.where(p_own, jnp.exp2(sc - jnp.where(p_first, ma, mb)), 0.0)
            sa = jnp.sum(jnp.where(p_first, e, 0.0), axis=1, keepdims=True)
            sb = jnp.sum(jnp.where(p_first, 0.0, e), axis=1, keepdims=True)
            return (e * _recip(jnp.where(p_first, sa, sb))).astype(BF16)

        def pre_pv(g, pr, vbds):
            v = cat([x[:MEM + PRE] for vb in vbds for x in vb])
            o = _dot(pr, v.astype(BF16))
            if not odd:
                odef_s[g] = o
            return o

        def wout(p, o, opre, acc):
            if odd:
                r = pl.ds((p % GP) * PRE, PRE)
                o = jnp.concatenate(
                    [o, opre[(p % GP) * PRE:(p % GP + 1) * PRE], odef_s[p // GP, r, :]], axis=0)
            contrib = _dot(o.astype(BF16), _unpack(wo_s[p * hw:(p + 1) * hw, :]))
            return contrib if acc is None else acc + contrib

        def window(m, j, w):
            lo = A_HALO - A_DIL * w
            return kv_s[m, j, lo:lo + SEG, :]

        def local_softmax():
            pos = row0 + lax.broadcasted_iota(jnp.int32, (SEG, 128), 0)
            logits = []
            for w in range(A_W):
                t = qa_s[0] * window(0, 0, w)
                for j in range(1, NT):
                    t = t + qa_s[j] * window(0, j, w)
                t = t + pltpu.roll(t, 64, 1)
                t = t + pltpu.roll(t, 32, 1)
                logits.append(t if w == 0 else jnp.where(pos >= A_DIL * w, t, NEG))
            mx = functools.reduce(jnp.maximum, logits)
            es = [jnp.exp2(l - mx) for l in logits]
            inv = _recip(functools.reduce(lambda u, v: u + v, es))
            return es, inv

        def local_out(j, es, inv, acc):
            o = es[0] * window(1, j, 0)
            for w in range(1, A_W):
                o = o + es[w] * window(1, j, w)
            for m in range(2):
                kv_s[m, j, :A_HALO, :] = kv_s[m, j, SEG:, :]
            r = _dot((o * inv).astype(BF16), _unpack(awo_s[j * 64:(j + 1) * 64, :]))
            return r if acc is None else acc + r

        nxt = pl.multiple_of(jnp.minimum(s + 1, NSEG - 1) * SEG, SEG)

        val = {}
        acc = None
        oa = None
        for kind, t in _order(u):
            if kind == "K":
                val[kind, t] = block_diag(t, 1)
            elif kind == "V":
                val[kind, t] = block_diag(t, 2)
            elif kind == "Q":
                val[kind, t] = proj(t, 0).astype(BF16)
            elif kind == "S":
                val[kind, t] = scores(val["Q", t], val["K", t], t >= LATE_FROM)
            elif kind == "PV":
                val[kind, t] = pv(val["S", t], val["V", t])
            elif kind == "PS":
                val[kind, t] = pre_scores(t, [val["K", GP * t + r] for r in range(GP)])
            elif kind == "PPV":
                val[kind, t] = pre_pv(t, val["PS", t], [val["V", GP * t + r] for r in range(GP)])
            elif kind == "W":
                acc = wout(t, val["PV", t], val.get(("PPV", t // GP)), acc)
            elif kind == "LA":
                la = local_softmax()
            elif kind == "AP":
                a_store(t, _dot(xa_s[pl.ds(nxt, SEG), :D], _unpack(wa_s[t])))
            elif kind == "AO":
                oa = local_out(t, la[0], la[1], oa)
                if t == NT - 1:
                    out_s[pl.ds(row0, SEG), :D] = oa.astype(BF16)
        return acc

    def out_copy(i):
        r = pl.ds(pl.multiple_of(i * 2 * SEG, 2 * SEG), 2 * SEG)
        return pltpu.make_async_copy(out_s.at[r, :2 * D], out_hbm.at[r, :], out_sem)

    def step(i, mem, u):
        acc0 = segment(2 * i, mem, 2 * u)
        acc1 = segment(2 * i + 1, acc0[FRESH:], 2 * u + 1)
        res = jnp.concatenate([acc1[SEG + PRE:], acc0[:FRESH], acc1[SEG:SEG + PRE], acc1[:FRESH]],
                              axis=0)
        out_s[pl.ds(pl.multiple_of(i * 2 * SEG, 2 * SEG), 2 * SEG), D:2 * D] = res.astype(BF16)
        out_copy(i).start()
        return acc1[FRESH:SEG]

    def steps(i, mem):
        for u in range(UNR):
            mem = step(i * UNR + u, mem, u)
        return mem

    lax.fori_loop(0, N_STEPS, steps, mem0_s[...].astype(F32))

    for cp in trip_copies(NTRIP):
        cp.wait()

    def wait_out(i, carry):
        out_copy(i).wait()
        return carry

    lax.fori_loop(0, N_STEPS * UNR, wait_out, 0)


@jax.jit
def pallas_concat_heads__sliding_local_dilated__memory_aug_recurrent_mem_tr__prompt_kernel(
    A_x: jax.Array,
    A_wqkv: jax.Array,
    A_wo: jax.Array,
    B_x: jax.Array,
    B_mem0: jax.Array,
    B_Wq: jax.Array,
    B_Wk: jax.Array,
    B_Wv: jax.Array,
    B_Wo: jax.Array,
    B_seg_len,
):
    del B_seg_len
    assert A_x.shape == (1, S, D) and B_x.shape == (1, S, D)
    hd = B_H * B_DH
    wq_t = jnp.transpose(B_Wq, (1, 2, 0)).reshape(hd, D)
    wk_t = jnp.transpose(B_Wk, (1, 2, 0)).reshape(hd, D)
    wv_t = jnp.transpose(B_Wv, (1, 2, 0)).reshape(hd, D)
    wo = B_Wo.reshape(hd, D)

    any_spec = pl.BlockSpec(memory_space=pl.ANY)
    out = pl.pallas_call(
        _kernel,
        out_shape=jax.ShapeDtypeStruct((S, 2 * D), BF16),
        in_specs=[any_spec] * 10,
        out_specs=any_spec,
        scratch_shapes=[
            pltpu.VMEM((2, PP, 4, PW, D), BF16),
            pltpu.VMEM((NT, D // 2, 128), U32),
            pltpu.VMEM((NP, D // 2, 3 * PW), U32),
            pltpu.VMEM((hd // 2, D), U32),
            pltpu.VMEM((NSEG, NP, PRE, 3 * PW), F32),
            pltpu.VMEM((NG, GP * PRE, PW), F32),
            pltpu.VMEM((S, OUT_W), BF16),
            pltpu.VMEM((S, X_W), BF16),
            pltpu.VMEM((S, X_W), BF16),
            pltpu.VMEM((NSEG, PRE, D), BF16),
            pltpu.VMEM((MEM, D), BF16),
            pltpu.VMEM((3, D // 2, D), U32),
            pltpu.VMEM((D // 2, D), U32),
            pltpu.VMEM((PP, D // 2, 128), U32),
            pltpu.VMEM((NT, SEG, 128), F32),
            pltpu.VMEM((2, NT, A_HALO + SEG, 128), F32),
            pltpu.SemaphoreType.DMA((2, PP, 4)),
            pltpu.SemaphoreType.DMA((5 + NT,)),
            pltpu.SemaphoreType.DMA,
        ],
        compiler_params=pltpu.CompilerParams(vmem_limit_bytes=120 * 1024 * 1024,
                                             disable_bounds_checks=True),
    )(A_x.reshape(S, D), A_wqkv, A_wo, B_x.reshape(S, D), B_x.reshape(NSEG, SEG // PRE, PRE, D),
      B_mem0.reshape(MEM, D), wq_t, wk_t, wv_t, wo)
    return out.reshape(1, S, 2 * D)
```

```python
import functools

import jax
import jax.numpy as jnp
from jax import lax
import jax.experimental.pallas as pl
import jax.experimental.pallas.tpu as pltpu

F32 = jnp.float32
BF16 = jnp.bfloat16
U32 = jnp.uint32

S = 2048
D = 640
NT = D // 128
A_H = 32
A_DH = D // A_H
A_W = 8
A_DIL = 2
A_HALO = 16
B_H = 32
B_DH = 192
MEM = 8
SEG = 32
NSEG = S // SEG
NP = B_H // 2
PW = 2 * B_DH
PRE = 8
FRESH = SEG - PRE
L = MEM + SEG
GP = 4
NG = NP // GP
LOG2E = 1.4426950408889634
NEG = -1000000000.0 * LOG2E
PP = 2
NTRIP = NP // PP - 1
PEEL_CHUNKS = 4
X_ROWS = 288
WO_ROWS = 432
X_W = 1024
OUT_W = 2048
UNR = 2
N_STEPS = NSEG // 2 // UNR

LAT_MM, LAT_SM, LAT_SM_LATE, LAT_T = 190, 650, 330, 600
LATE_FROM = NP - 2
AO_AFTER = (10, 18, 26, 34, 40)
FOLD_T = True
PV_PAD = False
XLU_T_PRE = True
T_F32 = True
XLU_T_MAIN = True


def _segment_order(odd):
    proj = []
    for g in range(NG):
        proj += [("K", GP * g + r) for r in range(GP)]
        for r in range(GP):
            proj += [("V", GP * g + r), ("Q", GP * g + r)]
    dur = {"K": 120, "V": 120, "Q": 120, "S": 24, "PV": 24, "PS": 24, "PPV": 24,
           "W": 180 if odd else 120, "AO": 40, "AP": 200}
    end = {}

    def ready(task):
        k, i = task
        if k == "S":
            deps = [(("Q", i), LAT_MM), (("K", i), LAT_T if XLU_T_MAIN else LAT_MM)]
        elif k == "PV":
            deps = [(("S", i), LAT_SM_LATE if i >= LATE_FROM else LAT_SM), (("V", i), LAT_MM)]
        elif k == "PS":
            deps = [(("K", GP * i + GP - 1), LAT_T if XLU_T_PRE else LAT_MM)]
        elif k == "PPV":
            deps = [(("PS", i), LAT_SM), (("V", GP * i + GP - 1), LAT_MM)]
        else:
            deps = [(("PV", i), LAT_MM)] + ([(("PPV", i // GP), LAT_MM)] if odd else [])
        if any(d not in end for d, _ in deps):
            return None
        return max(end[d] + lat for d, lat in deps)

    pend = ([("W", p) for p in range(NP)] + [("PPV", g) for g in range(NG)]
            + [("PV", p) for p in range(NP)] + [("PS", g) for g in range(NG)]
            + [("S", p) for p in range(NP)])
    fill = [("AP", 0), ("AP", 1)]
    order = []
    now = [0]

    def emit(task):
        order.append(task)
        now[0] += dur[task[0]]
        end[task] = now[0]

    nproj = 0
    while pend:
        cand = [x for x in pend if ready(x) is not None and ready(x) <= now[0]]
        if cand:
            if not proj:
                cand = [x for x in cand if x[0] != "W"] or cand
            pend.remove(cand[0])
            emit(cand[0])
        elif proj:
            emit(proj.pop(0))
            nproj += 1
            if nproj == GP:
                order.append(("LA", 0))
            if nproj in AO_AFTER:
                emit(("AO", AO_AFTER.index(nproj)))
        elif fill:
            emit(fill.pop(0))
        else:
            now[0] = min(ready(x) for x in pend if ready(x) is not None)
    return order + fill + [("AP", 2)]


ORDERS = (
    "K0 K1 K2 K3 V0 LA0 Q1 Q0 V1 S0 V2 PS0 Q2 AO0 S1 V3 Q3 S2 PV0 K4 K5 PPV0 S3 K6 W0 PV1 K7 "
    "PV2 V4 W1 W2 PV3 Q4 AO1 V5 W3 PS1 S4 Q5 V6 Q6 S5 V7 Q7 S6 K8 PPV1 PV4 S7 K9 AO2 K10 W4 PV5 "
    "K11 PV6 V8 W5 W6 PV7 Q8 V9 W7 S8 PS2 Q9 V10 Q10 AO3 S9 V11 PV8 Q11 K12 PPV2 S11 S10 K13 W8 "
    "PV9 K14 K15 W9 PV10 PV11 V12 AO4 Q12 W10 W11 PS3 S12 V13 V15 Q13 Q14 Q15 S13 V14 PV12 S14 "
    "AP0 PPV3 S15 W12 PV13 AP1 PV14 PV15 W13 W14 W15 AP2 ",
    "K0 K1 K2 K3 LA0 V0 Q0 V1 Q1 S0 V2 PS0 Q2 AO0 S1 V3 K4 Q3 S2 PV0 K5 PPV0 S3 K6 PV1 K7 W0 Q4 "
    "W1 PV2 V4 PV3 PS1 AO1 W2 W3 S4 V5 Q5 V6 Q6 S5 V7 Q7 PV4 S6 K8 PPV1 S7 K9 K10 AO2 W4 PV5 "
    "PV6 K11 V8 W5 W6 PV7 Q8 PS2 V9 W7 Q9 S8 V10 Q10 AO3 S9 V11 Q11 PV8 S10 K12 PPV2 S11 K13 "
    "K14 W8 PV9 K15 AO4 PV10 V12 PV11 W10 W9 Q12 PS3 V13 W11 S12 Q13 V14 Q14 S13 V15 Q15 AP0 "
    "S14 PPV3 PV12 S15 AP1 PV13 PV14 W12 PV15 W13 W14 W15 AP2 ",
    "K0 K1 K2 K3 LA0 V0 V1 Q0 Q1 S0 V2 PS0 Q2 AO0 S1 V3 Q3 S2 K4 K5 PPV0 PV0 S3 K6 W0 PV1 K7 "
    "PV2 V4 PV3 W1 W2 Q4 AO1 V5 W3 PS1 S4 Q5 V6 Q6 S5 V7 Q7 S6 K8 S7 PPV1 K9 PV4 AO2 K10 W4 PV5 "
    "PV6 K11 W5 V8 W6 PV7 Q8 W7 V9 PS2 S8 V10 Q9 Q10 AO3 S9 V11 Q11 PV8 S10 K12 PPV2 S11 W8 K13 "
    "PV9 K14 K15 AO4 W9 PV10 PV11 V12 Q12 W10 W11 PS3 S12 Q13 V13 V14 Q14 S13 Q15 PV12 V15 S14 "
    "AP0 PPV3 S15 W12 PV14 PV13 AP1 PV15 W13 W14 W15 AP2 ",
    "K3 K0 K1 K2 LA0 V0 Q0 V1 Q1 S0 V2 PS0 Q2 S1 V3 AO0 S2 K4 PV0 Q3 K5 PPV0 S3 K6 PV1 K7 W0 W1 "
    "PV2 PV3 Q4 V4 W2 W3 AO1 PS1 S4 V5 Q5 V6 Q6 S5 V7 PV4 Q7 S6 K8 S7 K9 AO2 PPV1 K11 K10 W4 "
    "PV5 PV6 V8 W5 PV7 W6 Q8 PS2 V10 V9 W7 S8 Q9 Q10 AO3 S9 V11 Q11 PV8 S10 K12 S11 PPV2 K13 "
    "K14 W8 PV9 K15 AO4 PV10 V12 W9 W10 PV11 Q12 V13 PS3 W11 S12 Q13 V14 S13 V15 Q14 Q15 S14 "
    "AP0 PPV3 PV12 S15 AP1 PV13 PV14 W12 PV15 W13 W14 W15 AP2 ",
)
SKIP_PROLOGUE = False


def _order(u):
    if ORDERS is None or ORDERS[u] is None:
        return _segment_order(u % 2 == 1)
    return [(t.rstrip("0123456789"), int(t.lstrip("ABCDEFGHIJKLMNOPQRSTUVWXYZ")))
            for t in ORDERS[u].split()]


def _nt_dot(a, b):
    return lax.dot_general(a, b, (((1,), (1,)), ((), ())), preferred_element_type=F32)


def _dot(a, b):
    return jnp.dot(a, b, preferred_element_type=F32)


def _pack(x):
    return pltpu.bitcast(x, U32)


def _unpack(x):
    return pltpu.bitcast(x, BF16)


def _recip(x):
    r = pl.reciprocal(x, approx=True)
    return r * (2.0 - x * r)


def _kernel(ax_hbm, awqkv_hbm, awo_hbm, bx_hbm, bx4_hbm, mem0_hbm, wq_hbm, wk_hbm, wv_hbm, wo_hbm,
            out_hbm,
            stage, awo_raw, w_s, wo_s, pre_s, odef_s, out_s,
            xa_s, xb_s, xpre_s, xp_s, mem0_s, wa_s, awo_s, t1_s, qa_s, kv_s,
            sems):
    b_scale = B_DH ** (-0.5) * LOG2E
    a_scale = A_DH ** (-0.5) * LOG2E

    w_hbm = (wq_hbm, wk_hbm, wv_hbm)
    wo32 = wo_hbm.bitcast(U32)
    awo32 = awo_hbm.bitcast(U32)
    hw = PW // 2
    hd = B_H * B_DH

    def w_copy(p, half, q, m, sem):
        rows = pl.ds(pl.multiple_of(p * PW, PW), PW)
        return pltpu.make_async_copy(w_hbm[m].at[rows, :], stage.at[half, q, m], sem)

    def wa_copy(piece, half, q, sem):
        return pltpu.make_async_copy(
            awqkv_hbm.at[pl.ds(pl.multiple_of((piece % NT) * 128, 128), 128),
                         pl.ds(pl.multiple_of((piece // NT) * D, 128), D)],
            stage.at[half, q, 3, :128], sem)

    def start_trip(g):
        half = g % 2
        src = jnp.minimum(g, NTRIP - 1)
        for q in range(PP):
            for m in range(3):
                w_copy((src + 1) * PP + q, half, q, m, sems.at[half]).start(priority=1)
            wa_copy(1 + src * PP + q, half, q, sems.at[half]).start(priority=1)

    def wait_trip(half):
        for view in (stage.at[half, :, :3], stage.at[half, :, 3, :128]):
            pltpu.make_async_copy(view, view, sems.at[half]).wait()

    x0 = S - NTRIP * X_ROWS
    wo0 = hd // 2 - NTRIP * WO_ROWS

    def bulk_copies(xr, wr):
        return [
            pltpu.make_async_copy(ax_hbm.at[xr, :], xa_s.at[xr, :D], sems.at[2]),
            pltpu.make_async_copy(bx_hbm.at[xr, :], xb_s.at[xr, :D], sems.at[2]),
            pltpu.make_async_copy(wo32.at[wr, :], wo_s.at[wr, :], sems.at[2]),
        ]

    xpre_cp = pltpu.make_async_copy(bx4_hbm.at[:, 0], xpre_s, sems.at[3])
    late_cps = [pltpu.make_async_copy(mem0_hbm, mem0_s, sems.at[2])] + [
        pltpu.make_async_copy(awo32.at[:, c * 128:(c + 1) * 128], awo_raw.at[c], sems.at[2])
        for c in range(NT)]
    peel_cps = (
        [w_copy(0, 1, 0, 0, sems.at[4])],
        [w_copy(0, 1, 0, m, sems.at[5]) for m in (1, 2)],
        [w_copy(q, 1, q, m, sems.at[6]) for q in range(1, PP) for m in range(3)]
        + [wa_copy(0, 1, 0, sems.at[6])])

    xpre_cp.start()
    for cps in peel_cps:
        for cp in cps:
            cp.start(priority=1)
    start_trip(0)
    for cp in bulk_copies(pl.ds(0, x0), pl.ds(0, wo0)) + late_cps:
        cp.start(priority=1)
    kv_s[:, :, :A_HALO, :] = jnp.zeros((2, NT, A_HALO, 128), F32)

    def gather_heads(ref):
        rows = []
        for j in range(A_DH // 2):
            u = ref[pl.ds(j, A_H, stride=A_DH // 2), :]
            rows.append(pltpu.bitcast(u << 16, F32))
            rows.append(pltpu.bitcast(u & jnp.uint32(0xFFFF0000), F32))
        return jnp.concatenate(rows, axis=0)

    def pair_prep(p, half, q, m, chunks=1):
        if SKIP_PROLOGUE:
            return
        wt = stage[half, q, m]
        w_s[p, :, m * PW:(m + 1) * PW] = _pack(wt.T)
        n = NSEG // chunks
        for c in range(chunks):
            xp = _unpack(xp_s[c * n * PRE // 2:(c + 1) * n * PRE // 2, :])
            pre_s[c * n:(c + 1) * n, p, :, m * PW:(m + 1) * PW] = (
                _nt_dot(xp, wt).reshape(n, PRE, PW))

    def wa_prep(piece, half, q):
        t1_s[q] = _pack(stage[half, q, 3, :128].T)
        wa_s[piece // NT, pl.ds(pl.multiple_of((piece % NT) * 64, 64), 64), :] = (
            _pack(gather_heads(t1_s.at[q]).astype(BF16).T))

    xpre_cp.wait()
    xp_s[...] = _pack(xpre_s[...].reshape(NSEG * PRE, D))
    for cp in peel_cps[0]:
        cp.wait()
    pair_prep(0, 1, 0, 0, PEEL_CHUNKS)
    for cp in peel_cps[1]:
        cp.wait()
    for m in (1, 2):
        pair_prep(0, 1, 0, m, PEEL_CHUNKS)
    for cp in peel_cps[2]:
        cp.wait()
    for q in range(1, PP):
        for m in range(3):
            pair_prep(q, 1, q, m, PEEL_CHUNKS)
    wa_prep(0, 1, 0)

    def prologue(g, carry):
        half = g % 2
        for cp in bulk_copies(pl.ds(pl.multiple_of(x0 + g * X_ROWS, 16), X_ROWS),
                              pl.ds(pl.multiple_of(wo0 + g * WO_ROWS, 8), WO_ROWS)):
            cp.start()
        wait_trip(half)
        for q in range(PP):
            for m in range(3):
                pair_prep((g + 1) * PP + q, half, q, m)
                if q == 0 and m == 0:
                    start_trip(g + 1)
            wa_prep(1 + g * PP + q, half, q)
        return carry

    lax.fori_loop(0, NTRIP, prologue, 0)

    for cp in bulk_copies(slice(None), slice(None)) + late_cps:
        cp.wait()

    def a_store(m, r):
        for j in range(NT):
            t = r[:, j * 128:(j + 1) * 128]
            if m == 0:
                qa_s[j] = t * a_scale
            else:
                kv_s[m - 1, j, A_HALO:, :] = t

    for m in range(3):
        a_store(m, _dot(xa_s[:SEG, :D], _unpack(wa_s[m])))
    for c in range(NT):
        awo_s[:, c * 128:(c + 1) * 128] = _pack(gather_heads(awo_raw.at[c]).astype(BF16))

    def segment(s, mem, u):
        odd = u % 2 == 1
        row0 = pl.multiple_of(s * SEG, SEG)
        ninf = jnp.float32(-jnp.inf)

        qi = lax.broadcasted_iota(jnp.int32, (SEG, 2 * L), 0)
        kl = lax.broadcasted_iota(jnp.int32, (SEG, 2 * L), 1)
        is_a = kl < L
        kpos = jnp.where(is_a, kl, kl - L)
        allowed = (qi >= FRESH) | (qi + MEM + PRE >= kpos)
        pi = lax.broadcasted_iota(jnp.int32, (GP * PRE, 128), 0)
        pk = lax.broadcasted_iota(jnp.int32, (GP * PRE, 128), 1)
        p_own = (pk // SEG) == (pi // PRE)
        p_allowed = (pk % (MEM + PRE)) <= (pi % PRE) + MEM
        p_first = (pk % SEG) < MEM + PRE
        p_is_a = p_own & p_first
        p_is_b = p_own & jnp.logical_not(p_first)
        col_a = lax.broadcasted_iota(jnp.int32, (1, PW), 1) < B_DH
        col128_a = lax.broadcasted_iota(jnp.int32, (1, 128), 1) < (B_DH - 128)

        xb = xb_s[pl.ds(row0, SEG), :D].astype(F32)
        h = jnp.concatenate([xb[PRE:], mem], axis=0).astype(BF16)

        def proj(p, m):
            return _dot(h, _unpack(w_s[p, :, m * PW:(m + 1) * PW]))

        def pre(p, m):
            return pre_s[s, p, :, m * PW:(m + 1) * PW]

        def block_diag(p, m):
            f = proj(p, m)
            full = jnp.concatenate([f[FRESH:], pre(p, m), f[:FRESH]], axis=0)
            z = jnp.zeros_like(full)
            return jnp.where(col_a, full, z), jnp.where(col_a, z, full)

        def cat(parts):
            return jnp.concatenate(parts, axis=0)

        def qk(q, blocks):
            if not FOLD_T:
                return _dot(q, cat(blocks).T.astype(BF16))
            fold = cat([jnp.concatenate([x[:, :128] if i % 2 == 0 else x[:, 256:], x[:, 128:256]],
                                        axis=1) for i, x in enumerate(blocks)])
            if T_F32:
                t = fold.T
            else:
                t = fold.astype(BF16).T.astype(F32)
            outer = t[:128]
            n = blocks[0].shape[0]
            lane = lax.broadcasted_iota(jnp.int32, outer.shape, 1)
            lane_a = lane < n if len(blocks) == 2 else lane % (2 * n) < n
            z = jnp.zeros_like(outer)
            kt = cat([jnp.where(lane_a, outer, z), t[128:], jnp.where(lane_a, z, outer)])
            return _dot(q, kt.astype(BF16))

        def scores(q, kbd, late_norm):
            sc = qk(q, kbd) * b_scale
            sc = jnp.where(allowed, sc, NEG)
            ma = jnp.max(jnp.where(is_a, sc, ninf), axis=1, keepdims=True)
            mb = jnp.max(jnp.where(is_a, ninf, sc), axis=1, keepdims=True)
            e = jnp.exp2(sc - jnp.where(is_a, ma, mb))
            sa = jnp.sum(jnp.where(is_a, e, 0.0), axis=1, keepdims=True)
            sb = jnp.sum(jnp.where(is_a, 0.0, e), axis=1, keepdims=True)
            def fin(x):
                if PV_PAD:
                    x = jnp.concatenate([x, jnp.zeros((SEG, 128 - 2 * L), F32)], axis=1)
                return x.astype(BF16)
            if late_norm:
                return fin(e), _recip(sa), _recip(sb)
            return fin(e * _recip(jnp.where(is_a, sa, sb))), None, None

        def pv(sm, vbd):
            e, ra, rb = sm
            if PV_PAD:
                vbd = list(vbd) + [jnp.zeros((128 - 2 * L, PW), F32)]
            o = _dot(e, cat(vbd).astype(BF16))
            if ra is not None:
                o = jnp.concatenate([
                    o[:, :128] * ra,
                    o[:, 128:256] * jnp.where(col128_a, ra, rb),
                    o[:, 256:] * rb], axis=1)
            return o

        def pre_scores(g, kbds):
            q = jnp.concatenate([pre(GP * g + r, 0) for r in range(GP)], axis=0).astype(BF16)
            k = [x[:MEM + PRE] for kb in kbds for x in kb]
            sc = qk(q, k) * b_scale
            sc = jnp.where(p_allowed, sc, NEG)
            ma = jnp.max(jnp.where(p_is_a, sc, ninf), axis=1, keepdims=True)
            mb = jnp.max(jnp.where(p_is_b, sc, ninf), axis=1, keepdims=True)
            e = jnp.where(p_own, jnp.exp2(sc - jnp.where(p_first, ma, mb)), 0.0)
            sa = jnp.sum(jnp.where(p_first, e, 0.0), axis=1, keepdims=True)
            sb = jnp.sum(jnp.where(p_first, 0.0, e), axis=1, keepdims=True)
            return (e * _recip(jnp.where(p_first, sa, sb))).astype(BF16)

        def pre_pv(g, pr, vbds):
            v = cat([x[:MEM + PRE] for vb in vbds for x in vb])
            o = _dot(pr, v.astype(BF16))
            if not odd:
                odef_s[g] = o
            return o

        def wout(p, o, opre, acc):
            if odd:
                r = pl.ds((p % GP) * PRE, PRE)
                o = jnp.concatenate(
                    [o, opre[(p % GP) * PRE:(p % GP + 1) * PRE], odef_s[p // GP, r, :]], axis=0)
            contrib = _dot(o.astype(BF16), _unpack(wo_s[p * hw:(p + 1) * hw, :]))
            return contrib if acc is None else acc + contrib

        def window(m, j, w):
            lo = A_HALO - A_DIL * w
            return kv_s[m, j, lo:lo + SEG, :]

        def local_softmax():
            pos = row0 + lax.broadcasted_iota(jnp.int32, (SEG, 128), 0)
            logits = []
            for w in range(A_W):
                t = qa_s[0] * window(0, 0, w)
                for j in range(1, NT):
                    t = t + qa_s[j] * window(0, j, w)
                t = t + pltpu.roll(t, 64, 1)
                t = t + pltpu.roll(t, 32, 1)
                logits.append(t if w == 0 else jnp.where(pos >= A_DIL * w, t, NEG))
            mx = functools.reduce(jnp.maximum, logits)
            es = [jnp.exp2(l - mx) for l in logits]
            inv = _recip(functools.reduce(lambda u, v: u + v, es))
            return es, inv

        def local_out(j, es, inv, acc):
            o = es[0] * window(1, j, 0)
            for w in range(1, A_W):
                o = o + es[w] * window(1, j, w)
            for m in range(2):
                kv_s[m, j, :A_HALO, :] = kv_s[m, j, SEG:, :]
            r = _dot((o * inv).astype(BF16), _unpack(awo_s[j * 64:(j + 1) * 64, :]))
            return r if acc is None else acc + r

        nxt = pl.multiple_of(jnp.minimum(s + 1, NSEG - 1) * SEG, SEG)

        val = {}
        acc = None
        oa = None
        for kind, t in _order(u):
            if kind == "K":
                val[kind, t] = block_diag(t, 1)
            elif kind == "V":
                val[kind, t] = block_diag(t, 2)
            elif kind == "Q":
                val[kind, t] = proj(t, 0).astype(BF16)
            elif kind == "S":
                val[kind, t] = scores(val["Q", t], val["K", t], t >= LATE_FROM)
            elif kind == "PV":
                val[kind, t] = pv(val["S", t], val["V", t])
            elif kind == "PS":
                val[kind, t] = pre_scores(t, [val["K", GP * t + r] for r in range(GP)])
            elif kind == "PPV":
                val[kind, t] = pre_pv(t, val["PS", t], [val["V", GP * t + r] for r in range(GP)])
            elif kind == "W":
                acc = wout(t, val["PV", t], val.get(("PPV", t // GP)), acc)
            elif kind == "LA":
                la = local_softmax()
            elif kind == "AP":
                a_store(t, _dot(xa_s[pl.ds(nxt, SEG), :D], _unpack(wa_s[t])))
            elif kind == "AO":
                oa = local_out(t, la[0], la[1], oa)
                if t == NT - 1:
                    out_s[pl.ds(row0, SEG), :D] = oa.astype(BF16)
        return acc

    def out_copy(i):
        r = pl.ds(pl.multiple_of(i * 2 * SEG, 2 * SEG), 2 * SEG)
        return pltpu.make_async_copy(out_s.at[r, :2 * D], out_hbm.at[r, :], sems.at[7])

    def step(i, mem, u):
        acc0 = segment(2 * i, mem, 2 * u)
        acc1 = segment(2 * i + 1, acc0[FRESH:], 2 * u + 1)
        res = jnp.concatenate([acc1[SEG + PRE:], acc0[:FRESH], acc1[SEG:SEG + PRE], acc1[:FRESH]],
                              axis=0)
        out_s[pl.ds(pl.multiple_of(i * 2 * SEG, 2 * SEG), 2 * SEG), D:2 * D] = res.astype(BF16)
        out_copy(i).start()
        return acc1[FRESH:SEG]

    def steps(i, mem):
        for u in range(UNR):
            mem = step(i * UNR + u, mem, u)
        return mem

    lax.fori_loop(0, N_STEPS, steps, mem0_s[...].astype(F32))

    wait_trip(NTRIP % 2)

    done = N_STEPS * UNR * 2 * SEG
    pltpu.make_async_copy(out_s.at[:done, :2 * D], out_hbm.at[:done, :], sems.at[7]).wait()


@jax.jit
def pallas_concat_heads__sliding_local_dilated__memory_aug_recurrent_mem_tr__prompt_kernel(
    A_x: jax.Array,
    A_wqkv: jax.Array,
    A_wo: jax.Array,
    B_x: jax.Array,
    B_mem0: jax.Array,
    B_Wq: jax.Array,
    B_Wk: jax.Array,
    B_Wv: jax.Array,
    B_Wo: jax.Array,
    B_seg_len,
):
    del B_seg_len
    assert A_x.shape == (1, S, D) and B_x.shape == (1, S, D)
    hd = B_H * B_DH
    wq_t = jnp.transpose(B_Wq, (1, 2, 0)).reshape(hd, D)
    wk_t = jnp.transpose(B_Wk, (1, 2, 0)).reshape(hd, D)
    wv_t = jnp.transpose(B_Wv, (1, 2, 0)).reshape(hd, D)
    wo = B_Wo.reshape(hd, D)

    any_spec = pl.BlockSpec(memory_space=pl.ANY)
    out = pl.pallas_call(
        _kernel,
        out_shape=jax.ShapeDtypeStruct((S, 2 * D), BF16),
        in_specs=[any_spec] * 10,
        out_specs=any_spec,
        scratch_shapes=[
            pltpu.VMEM((2, PP, 4, PW, D), BF16),
            pltpu.VMEM((NT, D // 2, 128), U32),
            pltpu.VMEM((NP, D // 2, 3 * PW), U32),
            pltpu.VMEM((hd // 2, D), U32),
            pltpu.VMEM((NSEG, NP, PRE, 3 * PW), F32),
            pltpu.VMEM((NG, GP * PRE, PW), F32),
            pltpu.VMEM((S, OUT_W), BF16),
            pltpu.VMEM((S, X_W), BF16),
            pltpu.VMEM((S, X_W), BF16),
            pltpu.VMEM((NSEG, PRE, D), BF16),
            pltpu.VMEM((NSEG * PRE // 2, D), U32),
            pltpu.VMEM((MEM, D), BF16),
            pltpu.VMEM((3, D // 2, D), U32),
            pltpu.VMEM((D // 2, D), U32),
            pltpu.VMEM((PP, D // 2, 128), U32),
            pltpu.VMEM((NT, SEG, 128), F32),
            pltpu.VMEM((2, NT, A_HALO + SEG, 128), F32),
            pltpu.SemaphoreType.DMA((8,)),
        ],
        compiler_params=pltpu.CompilerParams(vmem_limit_bytes=120 * 1024 * 1024,
                                             disable_bounds_checks=True),
    )(A_x.reshape(S, D), A_wqkv, A_wo, B_x.reshape(S, D), B_x.reshape(NSEG, SEG // PRE, PRE, D),
      B_mem0.reshape(MEM, D), wq_t, wk_t, wv_t, wo)
    return out.reshape(1, S, 2 * D)
```

```python
import functools

import jax
import jax.numpy as jnp
from jax import lax
import jax.experimental.pallas as pl
import jax.experimental.pallas.tpu as pltpu

F32 = jnp.float32
BF16 = jnp.bfloat16
U32 = jnp.uint32

S = 2048
D = 640
NT = D // 128
A_H = 32
A_DH = D // A_H
A_W = 8
A_DIL = 2
A_HALO = 16
B_H = 32
B_DH = 192
MEM = 8
SEG = 32
NSEG = S // SEG
NP = B_H // 2
PW = 2 * B_DH
PRE = 8
FRESH = SEG - PRE
L = MEM + SEG
GP = 4
NG = NP // GP
LOG2E = 1.4426950408889634
NEG = -1000000000.0 * LOG2E
PP = 2
NTRIP = NP // PP - 1
STRASSEN = True
ST_ROWS = 256
PEEL_CHUNKS = 4
X_ROWS = 288
WO_ROWS = 432
X_W = 1024
OUT_W = 2048
UNR = 2
N_STEPS = NSEG // 2 // UNR

LAT_MM, LAT_SM, LAT_SM_LATE, LAT_T = 190, 650, 330, 600
LATE_FROM = NP - 2
AO_AFTER = (10, 18, 26, 34, 40)
FOLD_T = True
PV_PAD = False
XLU_T_PRE = True
T_F32 = True
XLU_T_MAIN = True


def _segment_order(odd):
    proj = []
    for g in range(NG):
        proj += [("K", GP * g + r) for r in range(GP)]
        for r in range(GP):
            proj += [("V", GP * g + r), ("Q", GP * g + r)]
    dur = {"K": 120, "V": 120, "Q": 120, "S": 24, "PV": 24, "PS": 24, "PPV": 24,
           "W": 180 if odd else 120, "AO": 40, "AP": 200}
    end = {}

    def ready(task):
        k, i = task
        if k == "S":
            deps = [(("Q", i), LAT_MM), (("K", i), LAT_T if XLU_T_MAIN else LAT_MM)]
        elif k == "PV":
            deps = [(("S", i), LAT_SM_LATE if i >= LATE_FROM else LAT_SM), (("V", i), LAT_MM)]
        elif k == "PS":
            deps = [(("K", GP * i + GP - 1), LAT_T if XLU_T_PRE else LAT_MM)]
        elif k == "PPV":
            deps = [(("PS", i), LAT_SM), (("V", GP * i + GP - 1), LAT_MM)]
        else:
            deps = [(("PV", i), LAT_MM)] + ([(("PPV", i // GP), LAT_MM)] if odd else [])
        if any(d not in end for d, _ in deps):
            return None
        return max(end[d] + lat for d, lat in deps)

    pend = ([("W", p) for p in range(NP)] + [("PPV", g) for g in range(NG)]
            + [("PV", p) for p in range(NP)] + [("PS", g) for g in range(NG)]
            + [("S", p) for p in range(NP)])
    fill = [("AP", 0), ("AP", 1)]
    order = []
    now = [0]

    def emit(task):
        order.append(task)
        now[0] += dur[task[0]]
        end[task] = now[0]

    nproj = 0
    while pend:
        cand = [x for x in pend if ready(x) is not None and ready(x) <= now[0]]
        if cand:
            if not proj:
                cand = [x for x in cand if x[0] != "W"] or cand
            pend.remove(cand[0])
            emit(cand[0])
        elif proj:
            emit(proj.pop(0))
            nproj += 1
            if nproj == GP:
                order.append(("LA", 0))
            if nproj in AO_AFTER:
                emit(("AO", AO_AFTER.index(nproj)))
        elif fill:
            emit(fill.pop(0))
        else:
            now[0] = min(ready(x) for x in pend if ready(x) is not None)
    return order + fill + [("AP", 2)]


ORDERS = (
    "K0 K1 K2 K3 V0 LA0 Q1 Q0 V1 S0 V2 PS0 Q2 AO0 S1 V3 Q3 S2 PV0 K4 K5 PPV0 S3 K6 W0 PV1 K7 "
    "PV2 V4 W1 W2 PV3 Q4 AO1 V5 W3 PS1 S4 Q5 V6 Q6 S5 V7 Q7 S6 K8 PPV1 PV4 S7 K9 AO2 K10 W4 PV5 "
    "K11 PV6 V8 W5 W6 PV7 Q8 V9 W7 S8 PS2 Q9 V10 Q10 AO3 S9 V11 PV8 Q11 K12 PPV2 S11 S10 K13 W8 "
    "PV9 K14 K15 W9 PV10 PV11 V12 AO4 Q12 W10 W11 PS3 S12 V13 V15 Q13 Q14 Q15 S13 V14 PV12 S14 "
    "AP0 PPV3 S15 W12 PV13 AP1 PV14 PV15 W13 W14 W15 AP2 ",
    "K0 K1 K2 K3 LA0 V0 Q0 V1 Q1 S0 V2 PS0 Q2 AO0 S1 V3 K4 Q3 S2 PV0 K5 PPV0 S3 K6 PV1 K7 W0 Q4 "
    "W1 PV2 V4 PV3 PS1 AO1 W2 W3 S4 V5 Q5 V6 Q6 S5 V7 Q7 PV4 S6 K8 PPV1 S7 K9 K10 AO2 W4 PV5 "
    "PV6 K11 V8 W5 W6 PV7 Q8 PS2 V9 W7 Q9 S8 V10 Q10 AO3 S9 V11 Q11 PV8 S10 K12 PPV2 S11 K13 "
    "K14 W8 PV9 K15 AO4 PV10 V12 PV11 W10 W9 Q12 PS3 V13 W11 S12 Q13 V14 Q14 S13 V15 Q15 AP0 "
    "S14 PPV3 PV12 S15 AP1 PV13 PV14 W12 PV15 W13 W14 W15 AP2 ",
    "K0 K1 K2 K3 LA0 V0 V1 Q0 Q1 S0 V2 PS0 Q2 AO0 S1 V3 Q3 S2 K4 K5 PPV0 PV0 S3 K6 W0 PV1 K7 "
    "PV2 V4 PV3 W1 W2 Q4 AO1 V5 W3 PS1 S4 Q5 V6 Q6 S5 V7 Q7 S6 K8 S7 PPV1 K9 PV4 AO2 K10 W4 PV5 "
    "PV6 K11 W5 V8 W6 PV7 Q8 W7 V9 PS2 S8 V10 Q9 Q10 AO3 S9 V11 Q11 PV8 S10 K12 PPV2 S11 W8 K13 "
    "PV9 K14 K15 AO4 W9 PV10 PV11 V12 Q12 W10 W11 PS3 S12 Q13 V13 V14 Q14 S13 Q15 PV12 V15 S14 "
    "AP0 PPV3 S15 W12 PV14 PV13 AP1 PV15 W13 W14 W15 AP2 ",
    "K3 K0 K1 K2 LA0 V0 Q0 V1 Q1 S0 V2 PS0 Q2 S1 V3 AO0 S2 K4 PV0 Q3 K5 PPV0 S3 K6 PV1 K7 W0 W1 "
    "PV2 PV3 Q4 V4 W2 W3 AO1 PS1 S4 V5 Q5 V6 Q6 S5 V7 PV4 Q7 S6 K8 S7 K9 AO2 PPV1 K11 K10 W4 "
    "PV5 PV6 V8 W5 PV7 W6 Q8 PS2 V10 V9 W7 S8 Q9 Q10 AO3 S9 V11 Q11 PV8 S10 K12 S11 PPV2 K13 "
    "K14 W8 PV9 K15 AO4 PV10 V12 W9 W10 PV11 Q12 V13 PS3 W11 S12 Q13 V14 S13 V15 Q14 Q15 S14 "
    "AP0 PPV3 PV12 S15 AP1 PV13 PV14 W12 PV15 W13 W14 W15 AP2 ",
)
SKIP_PROLOGUE = False


def _order(u):
    if ORDERS is None or ORDERS[u] is None:
        return _segment_order(u % 2 == 1)
    return [(t.rstrip("0123456789"), int(t.lstrip("ABCDEFGHIJKLMNOPQRSTUVWXYZ")))
            for t in ORDERS[u].split()]


def _nt_dot(a, b):
    return lax.dot_general(a, b, (((1,), (1,)), ((), ())), preferred_element_type=F32)


def _dot(a, b):
    return jnp.dot(a, b, preferred_element_type=F32)


def _pack(x):
    return pltpu.bitcast(x, U32)


def _unpack(x):
    return pltpu.bitcast(x, BF16)


def _recip(x):
    r = pl.reciprocal(x, approx=True)
    return r * (2.0 - x * r)


def _kernel(ax_hbm, awqkv_hbm, awo_hbm, bx_hbm, bx4_hbm, mem0_hbm, wq_hbm, wk_hbm, wv_hbm, wo_hbm,
            out_hbm,
            stage, awo_raw, w_s, wo_s, pre_s, odef_s, out_s,
            xa_s, xb_s, xpre_s, xp_s, xs_s, mem0_s, wa_s, awo_s, t1_s, qa_s, kv_s,
            sems):
    b_scale = B_DH ** (-0.5) * LOG2E
    a_scale = A_DH ** (-0.5) * LOG2E

    w_hbm = (wq_hbm, wk_hbm, wv_hbm)
    wo32 = wo_hbm.bitcast(U32)
    awo32 = awo_hbm.bitcast(U32)
    hw = PW // 2
    hd = B_H * B_DH

    def w_copy(p, half, q, m, sem):
        rows = pl.ds(pl.multiple_of(p * PW, PW), PW)
        return pltpu.make_async_copy(w_hbm[m].at[rows, :], stage.at[half, q, m], sem)

    def wa_copy(piece, half, q, sem):
        return pltpu.make_async_copy(
            awqkv_hbm.at[pl.ds(pl.multiple_of((piece % NT) * 128, 128), 128),
                         pl.ds(pl.multiple_of((piece // NT) * D, 128), D)],
            stage.at[half, q, 3, :128], sem)

    def start_trip(g):
        half = g % 2
        src = jnp.minimum(g, NTRIP - 1)
        for q in range(PP):
            for m in range(3):
                w_copy((src + 1) * PP + q, half, q, m, sems.at[half]).start(priority=1)
            wa_copy(1 + src * PP + q, half, q, sems.at[half]).start(priority=1)

    def wait_trip(half):
        for view in (stage.at[half, :, :3], stage.at[half, :, 3, :128]):
            pltpu.make_async_copy(view, view, sems.at[half]).wait()

    x0 = S - NTRIP * X_ROWS
    wo0 = hd // 2 - NTRIP * WO_ROWS

    def bulk_copies(xr, wr):
        return [
            pltpu.make_async_copy(ax_hbm.at[xr, :], xa_s.at[xr, :D], sems.at[2]),
            pltpu.make_async_copy(bx_hbm.at[xr, :], xb_s.at[xr, :D], sems.at[2]),
            pltpu.make_async_copy(wo32.at[wr, :], wo_s.at[wr, :], sems.at[2]),
        ]

    xpre_cp = pltpu.make_async_copy(bx4_hbm.at[:, 0], xpre_s, sems.at[3])
    late_cps = [pltpu.make_async_copy(mem0_hbm, mem0_s, sems.at[2])] + [
        pltpu.make_async_copy(awo32.at[:, c * 128:(c + 1) * 128], awo_raw.at[c], sems.at[2])
        for c in range(NT)]
    peel_cps = (
        [w_copy(0, 1, 0, 0, sems.at[4])],
        [w_copy(0, 1, 0, m, sems.at[5]) for m in (1, 2)],
        [w_copy(q, 1, q, m, sems.at[6]) for q in range(1, PP) for m in range(3)]
        + [wa_copy(0, 1, 0, sems.at[6])])

    xpre_cp.start()
    for cps in peel_cps:
        for cp in cps:
            cp.start(priority=1)
    start_trip(0)
    for cp in bulk_copies(pl.ds(0, x0), pl.ds(0, wo0)) + late_cps:
        cp.start(priority=1)
    kv_s[:, :, :A_HALO, :] = jnp.zeros((2, NT, A_HALO, 128), F32)

    def gather_heads(ref):
        rows = []
        for j in range(A_DH // 2):
            u = ref[pl.ds(j, A_H, stride=A_DH // 2), :]
            rows.append(pltpu.bitcast(u << 16, F32))
            rows.append(pltpu.bitcast(u & jnp.uint32(0xFFFF0000), F32))
        return jnp.concatenate(rows, axis=0)

    def pair_prep(p, half, q, m, chunks=1):
        if SKIP_PROLOGUE:
            return
        wt = stage[half, q, m]
        w_s[p, :, m * PW:(m + 1) * PW] = _pack(wt.T)
        n = NSEG // chunks
        for c in range(chunks):
            xp = _unpack(xp_s[c * n * PRE // 2:(c + 1) * n * PRE // 2, :])
            pre_s[c * n:(c + 1) * n, p, :, m * PW:(m + 1) * PW] = (
                _nt_dot(xp, wt).reshape(n, PRE, PW))

    KH = 256
    HR = NSEG * PRE // 2

    def xq(i, k):
        return _unpack(xp_s[i * HR // 2:(i + 1) * HR // 2, k * KH:(k + 1) * KH])

    def strassen_lhs():
        f = lambda i, k: xq(i, k).astype(F32)
        sums = (f(0, 0) + f(1, 1), f(1, 0) + f(1, 1), f(0, 0) + f(0, 1),
                f(1, 0) - f(0, 0), f(0, 1) - f(1, 1))
        for n, v in enumerate(sums):
            xs_s[n] = _pack(v.astype(BF16))

    def pair_prep2(p, half, m):
        if SKIP_PROLOGUE:
            return
        for q in range(2):
            w_s[p + q, :, m * PW:(m + 1) * PW] = _pack(stage[half, q, m].T)
        nseg = ST_ROWS // PRE
        for j in range(PW // 128):
            rows = slice(j * 128, (j + 1) * 128)
            b = lambda k, q: stage[half, q, m, rows, k * KH:(k + 1) * KH]
            bf = lambda k, q: b(k, q).astype(F32)
            rhs = ((bf(0, 0) + bf(1, 1)).astype(BF16), b(0, 0),
                   (bf(0, 1) - bf(1, 1)).astype(BF16), (bf(1, 0) - bf(0, 0)).astype(BF16),
                   b(1, 1), (bf(0, 0) + bf(0, 1)).astype(BF16),
                   (bf(1, 0) + bf(1, 1)).astype(BF16))
            tail = [stage[half, q, m, rows, 2 * KH:] for q in range(2)]
            for c in range(HR // ST_ROWS):
                r = slice(c * ST_ROWS // 2, (c + 1) * ST_ROWS // 2)
                sm = lambda n: _unpack(xs_s[n, r, :])
                qd = lambda i, k: _unpack(
                    xp_s[(i * HR + c * ST_ROWS) // 2:(i * HR + (c + 1) * ST_ROWS) // 2,
                         k * KH:(k + 1) * KH])
                rest = lambda i: _unpack(
                    xp_s[(i * HR + c * ST_ROWS) // 2:(i * HR + (c + 1) * ST_ROWS) // 2, 2 * KH:])

                def put(i, q, v):
                    s0 = i * (NSEG // 2) + c * nseg
                    pre_s[s0:s0 + nseg, p + q, :, m * PW + j * 128:m * PW + (j + 1) * 128] = (
                        v.reshape(nseg, PRE, 128))

                m5 = _nt_dot(sm(2), rhs[4])
                m3 = _nt_dot(qd(0, 0), rhs[2])
                put(0, 1, _nt_dot(rest(0), tail[1]) + m3 + m5)
                m1 = _nt_dot(sm(0), rhs[0])
                m4 = _nt_dot(qd(1, 1), rhs[3])
                put(0, 0, _nt_dot(rest(0), tail[0]) + _nt_dot(sm(4), rhs[6]) + (m1 + m4 - m5))
                m2 = _nt_dot(sm(1), rhs[1])
                put(1, 0, _nt_dot(rest(1), tail[0]) + m2 + m4)
                put(1, 1, _nt_dot(rest(1), tail[1]) + _nt_dot(sm(3), rhs[5]) + (m1 - m2 + m3))

    def wa_prep(piece, half, q):
        t1_s[q] = _pack(stage[half, q, 3, :128].T)
        wa_s[piece // NT, pl.ds(pl.multiple_of((piece % NT) * 64, 64), 64), :] = (
            _pack(gather_heads(t1_s.at[q]).astype(BF16).T))

    xpre_cp.wait()
    xp_s[...] = _pack(xpre_s[...].reshape(NSEG * PRE, D))
    if STRASSEN:
        strassen_lhs()
    for cp in peel_cps[0]:
        cp.wait()
    pair_prep(0, 1, 0, 0, PEEL_CHUNKS)
    for cp in peel_cps[1]:
        cp.wait()
    for m in (1, 2):
        pair_prep(0, 1, 0, m, PEEL_CHUNKS)
    for cp in peel_cps[2]:
        cp.wait()
    for q in range(1, PP):
        for m in range(3):
            pair_prep(q, 1, q, m, PEEL_CHUNKS)
    wa_prep(0, 1, 0)

    def prologue(g, carry):
        half = g % 2
        for cp in bulk_copies(pl.ds(pl.multiple_of(x0 + g * X_ROWS, 16), X_ROWS),
                              pl.ds(pl.multiple_of(wo0 + g * WO_ROWS, 8), WO_ROWS)):
            cp.start()
        if STRASSEN:
            start_trip(g + 1)
        wait_trip(half)
        if STRASSEN:
            for m in range(3):
                pair_prep2((g + 1) * PP, half, m)
                if m < PP:
                    wa_prep(1 + g * PP + m, half, m)
            return carry
        for q in range(PP):
            for m in range(3):
                pair_prep((g + 1) * PP + q, half, q, m)
                if q == 0 and m == 0:
                    start_trip(g + 1)
            wa_prep(1 + g * PP + q, half, q)
        return carry

    lax.fori_loop(0, NTRIP, prologue, 0)

    for cp in bulk_copies(slice(None), slice(None)) + late_cps:
        cp.wait()

    def a_store(m, r):
        for j in range(NT):
            t = r[:, j * 128:(j + 1) * 128]
            if m == 0:
                qa_s[j] = t * a_scale
            else:
                kv_s[m - 1, j, A_HALO:, :] = t

    for m in range(3):
        a_store(m, _dot(xa_s[:SEG, :D], _unpack(wa_s[m])))
    for c in range(NT):
        awo_s[:, c * 128:(c + 1) * 128] = _pack(gather_heads(awo_raw.at[c]).astype(BF16))

    def segment(s, mem, u):
        odd = u % 2 == 1
        row0 = pl.multiple_of(s * SEG, SEG)
        ninf = jnp.float32(-jnp.inf)

        qi = lax.broadcasted_iota(jnp.int32, (SEG, 2 * L), 0)
        kl = lax.broadcasted_iota(jnp.int32, (SEG, 2 * L), 1)
        is_a = kl < L
        kpos = jnp.where(is_a, kl, kl - L)
        allowed = (qi >= FRESH) | (qi + MEM + PRE >= kpos)
        pi = lax.broadcasted_iota(jnp.int32, (GP * PRE, 128), 0)
        pk = lax.broadcasted_iota(jnp.int32, (GP * PRE, 128), 1)
        p_own = (pk // SEG) == (pi // PRE)
        p_allowed = (pk % (MEM + PRE)) <= (pi % PRE) + MEM
        p_first = (pk % SEG) < MEM + PRE
        p_is_a = p_own & p_first
        p_is_b = p_own & jnp.logical_not(p_first)
        col_a = lax.broadcasted_iota(jnp.int32, (1, PW), 1) < B_DH
        col128_a = lax.broadcasted_iota(jnp.int32, (1, 128), 1) < (B_DH - 128)

        xb = xb_s[pl.ds(row0, SEG), :D].astype(F32)
        h = jnp.concatenate([xb[PRE:], mem], axis=0).astype(BF16)

        def proj(p, m):
            return _dot(h, _unpack(w_s[p, :, m * PW:(m + 1) * PW]))

        def pre(p, m):
            return pre_s[s, p, :, m * PW:(m + 1) * PW]

        def block_diag(p, m):
            f = proj(p, m)
            full = jnp.concatenate([f[FRESH:], pre(p, m), f[:FRESH]], axis=0)
            z = jnp.zeros_like(full)
            return jnp.where(col_a, full, z), jnp.where(col_a, z, full)

        def cat(parts):
            return jnp.concatenate(parts, axis=0)

        def qk(q, blocks):
            if not FOLD_T:
                return _dot(q, cat(blocks).T.astype(BF16))
            fold = cat([jnp.concatenate([x[:, :128] if i % 2 == 0 else x[:, 256:], x[:, 128:256]],
                                        axis=1) for i, x in enumerate(blocks)])
            if T_F32:
                t = fold.T
            else:
                t = fold.astype(BF16).T.astype(F32)
            outer = t[:128]
            n = blocks[0].shape[0]
            lane = lax.broadcasted_iota(jnp.int32, outer.shape, 1)
            lane_a = lane < n if len(blocks) == 2 else lane % (2 * n) < n
            z = jnp.zeros_like(outer)
            kt = cat([jnp.where(lane_a, outer, z), t[128:], jnp.where(lane_a, z, outer)])
            return _dot(q, kt.astype(BF16))

        def scores(q, kbd, late_norm):
            sc = qk(q, kbd) * b_scale
            sc = jnp.where(allowed, sc, NEG)
            ma = jnp.max(jnp.where(is_a, sc, ninf), axis=1, keepdims=True)
            mb = jnp.max(jnp.where(is_a, ninf, sc), axis=1, keepdims=True)
            e = jnp.exp2(sc - jnp.where(is_a, ma, mb))
            sa = jnp.sum(jnp.where(is_a, e, 0.0), axis=1, keepdims=True)
            sb = jnp.sum(jnp.where(is_a, 0.0, e), axis=1, keepdims=True)
            def fin(x):
                if PV_PAD:
                    x = jnp.concatenate([x, jnp.zeros((SEG, 128 - 2 * L), F32)], axis=1)
                return x.astype(BF16)
            if late_norm:
                return fin(e), _recip(sa), _recip(sb)
            return fin(e * _recip(jnp.where(is_a, sa, sb))), None, None

        def pv(sm, vbd):
            e, ra, rb = sm
            if PV_PAD:
                vbd = list(vbd) + [jnp.zeros((128 - 2 * L, PW), F32)]
            o = _dot(e, cat(vbd).astype(BF16))
            if ra is not None:
                o = jnp.concatenate([
                    o[:, :128] * ra,
                    o[:, 128:256] * jnp.where(col128_a, ra, rb),
                    o[:, 256:] * rb], axis=1)
            return o

        def pre_scores(g, kbds):
            q = jnp.concatenate([pre(GP * g + r, 0) for r in range(GP)], axis=0).astype(BF16)
            k = [x[:MEM + PRE] for kb in kbds for x in kb]
            sc = qk(q, k) * b_scale
            sc = jnp.where(p_allowed, sc, NEG)
            ma = jnp.max(jnp.where(p_is_a, sc, ninf), axis=1, keepdims=True)
            mb = jnp.max(jnp.where(p_is_b, sc, ninf), axis=1, keepdims=True)
            e = jnp.where(p_own, jnp.exp2(sc - jnp.where(p_first, ma, mb)), 0.0)
            sa = jnp.sum(jnp.where(p_first, e, 0.0), axis=1, keepdims=True)
            sb = jnp.sum(jnp.where(p_first, 0.0, e), axis=1, keepdims=True)
            return (e * _recip(jnp.where(p_first, sa, sb))).astype(BF16)

        def pre_pv(g, pr, vbds):
            v = cat([x[:MEM + PRE] for vb in vbds for x in vb])
            o = _dot(pr, v.astype(BF16))
            if not odd:
                odef_s[g] = o
            return o

        def wout(p, o, opre, acc):
            if odd:
                r = pl.ds((p % GP) * PRE, PRE)
                o = jnp.concatenate(
                    [o, opre[(p % GP) * PRE:(p % GP + 1) * PRE], odef_s[p // GP, r, :]], axis=0)
            contrib = _dot(o.astype(BF16), _unpack(wo_s[p * hw:(p + 1) * hw, :]))
            return contrib if acc is None else acc + contrib

        def window(m, j, w):
            lo = A_HALO - A_DIL * w
            return kv_s[m, j, lo:lo + SEG, :]

        def local_softmax():
            pos = row0 + lax.broadcasted_iota(jnp.int32, (SEG, 128), 0)
            logits = []
            for w in range(A_W):
                t = qa_s[0] * window(0, 0, w)
                for j in range(1, NT):
                    t = t + qa_s[j] * window(0, j, w)
                t = t + pltpu.roll(t, 64, 1)
                t = t + pltpu.roll(t, 32, 1)
                logits.append(t if w == 0 else jnp.where(pos >= A_DIL * w, t, NEG))
            mx = functools.reduce(jnp.maximum, logits)
            es = [jnp.exp2(l - mx) for l in logits]
            inv = _recip(functools.reduce(lambda u, v: u + v, es))
            return es, inv

        def local_out(j, es, inv, acc):
            o = es[0] * window(1, j, 0)
            for w in range(1, A_W):
                o = o + es[w] * window(1, j, w)
            for m in range(2):
                kv_s[m, j, :A_HALO, :] = kv_s[m, j, SEG:, :]
            r = _dot((o * inv).astype(BF16), _unpack(awo_s[j * 64:(j + 1) * 64, :]))
            return r if acc is None else acc + r

        nxt = pl.multiple_of(jnp.minimum(s + 1, NSEG - 1) * SEG, SEG)

        val = {}
        acc = None
        oa = None
        for kind, t in _order(u):
            if kind == "K":
                val[kind, t] = block_diag(t, 1)
            elif kind == "V":
                val[kind, t] = block_diag(t, 2)
            elif kind == "Q":
                val[kind, t] = proj(t, 0).astype(BF16)
            elif kind == "S":
                val[kind, t] = scores(val["Q", t], val["K", t], t >= LATE_FROM)
            elif kind == "PV":
                val[kind, t] = pv(val["S", t], val["V", t])
            elif kind == "PS":
                val[kind, t] = pre_scores(t, [val["K", GP * t + r] for r in range(GP)])
            elif kind == "PPV":
                val[kind, t] = pre_pv(t, val["PS", t], [val["V", GP * t + r] for r in range(GP)])
            elif kind == "W":
                acc = wout(t, val["PV", t], val.get(("PPV", t // GP)), acc)
            elif kind == "LA":
                la = local_softmax()
            elif kind == "AP":
                a_store(t, _dot(xa_s[pl.ds(nxt, SEG), :D], _unpack(wa_s[t])))
            elif kind == "AO":
                oa = local_out(t, la[0], la[1], oa)
                if t == NT - 1:
                    out_s[pl.ds(row0, SEG), :D] = oa.astype(BF16)
        return acc

    def out_copy(i):
        r = pl.ds(pl.multiple_of(i * 2 * SEG, 2 * SEG), 2 * SEG)
        return pltpu.make_async_copy(out_s.at[r, :2 * D], out_hbm.at[r, :], sems.at[7])

    def step(i, mem, u):
        acc0 = segment(2 * i, mem, 2 * u)
        acc1 = segment(2 * i + 1, acc0[FRESH:], 2 * u + 1)
        res = jnp.concatenate([acc1[SEG + PRE:], acc0[:FRESH], acc1[SEG:SEG + PRE], acc1[:FRESH]],
                              axis=0)
        out_s[pl.ds(pl.multiple_of(i * 2 * SEG, 2 * SEG), 2 * SEG), D:2 * D] = res.astype(BF16)
        out_copy(i).start()
        return acc1[FRESH:SEG]

    def steps(i, mem):
        for u in range(UNR):
            mem = step(i * UNR + u, mem, u)
        return mem

    lax.fori_loop(0, N_STEPS, steps, mem0_s[...].astype(F32))

    wait_trip(NTRIP % 2)

    done = N_STEPS * UNR * 2 * SEG
    pltpu.make_async_copy(out_s.at[:done, :2 * D], out_hbm.at[:done, :], sems.at[7]).wait()


@jax.jit
def pallas_concat_heads__sliding_local_dilated__memory_aug_recurrent_mem_tr__prompt_kernel(
    A_x: jax.Array,
    A_wqkv: jax.Array,
    A_wo: jax.Array,
    B_x: jax.Array,
    B_mem0: jax.Array,
    B_Wq: jax.Array,
    B_Wk: jax.Array,
    B_Wv: jax.Array,
    B_Wo: jax.Array,
    B_seg_len,
):
    del B_seg_len
    assert A_x.shape == (1, S, D) and B_x.shape == (1, S, D)
    hd = B_H * B_DH
    wq_t = jnp.transpose(B_Wq, (1, 2, 0)).reshape(hd, D)
    wk_t = jnp.transpose(B_Wk, (1, 2, 0)).reshape(hd, D)
    wv_t = jnp.transpose(B_Wv, (1, 2, 0)).reshape(hd, D)
    wo = B_Wo.reshape(hd, D)

    any_spec = pl.BlockSpec(memory_space=pl.ANY)
    out = pl.pallas_call(
        _kernel,
        out_shape=jax.ShapeDtypeStruct((S, 2 * D), BF16),
        in_specs=[any_spec] * 10,
        out_specs=any_spec,
        scratch_shapes=[
            pltpu.VMEM((2, PP, 4, PW, D), BF16),
            pltpu.VMEM((NT, D // 2, 128), U32),
            pltpu.VMEM((NP, D // 2, 3 * PW), U32),
            pltpu.VMEM((hd // 2, D), U32),
            pltpu.VMEM((NSEG, NP, PRE, 3 * PW), F32),
            pltpu.VMEM((NG, GP * PRE, PW), F32),
            pltpu.VMEM((S, OUT_W), BF16),
            pltpu.VMEM((S, X_W), BF16),
            pltpu.VMEM((S, X_W), BF16),
            pltpu.VMEM((NSEG, PRE, D), BF16),
            pltpu.VMEM((NSEG * PRE // 2, D), U32),
            pltpu.VMEM((5, NSEG * PRE // 4, 256), U32),
            pltpu.VMEM((MEM, D), BF16),
            pltpu.VMEM((3, D // 2, D), U32),
            pltpu.VMEM((D // 2, D), U32),
            pltpu.VMEM((PP, D // 2, 128), U32),
            pltpu.VMEM((NT, SEG, 128), F32),
            pltpu.VMEM((2, NT, A_HALO + SEG, 128), F32),
            pltpu.SemaphoreType.DMA((8,)),
        ],
        compiler_params=pltpu.CompilerParams(vmem_limit_bytes=120 * 1024 * 1024,
                                             disable_bounds_checks=True),
    )(A_x.reshape(S, D), A_wqkv, A_wo, B_x.reshape(S, D), B_x.reshape(NSEG, SEG // PRE, PRE, D),
      B_mem0.reshape(MEM, D), wq_t, wk_t, wv_t, wo)
    return out.reshape(1, S, 2 * D)
```

```python
import functools

import jax
import jax.numpy as jnp
from jax import lax
import jax.experimental.pallas as pl
import jax.experimental.pallas.tpu as pltpu

F32 = jnp.float32
BF16 = jnp.bfloat16
U32 = jnp.uint32

S = 2048
D = 640
NT = D // 128
A_H = 32
A_DH = D // A_H
A_W = 8
A_DIL = 2
A_HALO = 16
B_H = 32
B_DH = 192
MEM = 8
SEG = 32
NSEG = S // SEG
NP = B_H // 2
PW = 2 * B_DH
PRE = 8
FRESH = SEG - PRE
L = MEM + SEG
GP = 4
NG = NP // GP
LOG2E = 1.4426950408889634
NEG = -1000000000.0 * LOG2E
PP = 2
NTRIP = NP // PP - 1
STRASSEN = True
ST_ROWS = 256
PEEL_CHUNKS = 4
X_HEAD = 160
WO_ROWS = 432
X_W = 1024
OUT_W = 2048
UNR = 2
N_STEPS = NSEG // 2 // UNR

LAT_MM, LAT_SM, LAT_SM_LATE, LAT_T = 190, 650, 330, 600
LATE_FROM = NP - 2
AO_AFTER = (10, 18, 26, 34, 40)
FOLD_T = True
PV_PAD = False
XLU_T_PRE = True
T_F32 = True
XLU_T_MAIN = True


def _segment_order(odd):
    proj = []
    for g in range(NG):
        proj += [("K", GP * g + r) for r in range(GP)]
        for r in range(GP):
            proj += [("V", GP * g + r), ("Q", GP * g + r)]
    dur = {"K": 120, "V": 120, "Q": 120, "S": 24, "PV": 24, "PS": 24, "PPV": 24,
           "W": 180 if odd else 120, "AO": 40, "AP": 200}
    end = {}

    def ready(task):
        k, i = task
        if k == "S":
            deps = [(("Q", i), LAT_MM), (("K", i), LAT_T if XLU_T_MAIN else LAT_MM)]
        elif k == "PV":
            deps = [(("S", i), LAT_SM_LATE if i >= LATE_FROM else LAT_SM), (("V", i), LAT_MM)]
        elif k == "PS":
            deps = [(("K", GP * i + GP - 1), LAT_T if XLU_T_PRE else LAT_MM)]
        elif k == "PPV":
            deps = [(("PS", i), LAT_SM), (("V", GP * i + GP - 1), LAT_MM)]
        else:
            deps = [(("PV", i), LAT_MM)] + ([(("PPV", i // GP), LAT_MM)] if odd else [])
        if any(d not in end for d, _ in deps):
            return None
        return max(end[d] + lat for d, lat in deps)

    pend = ([("W", p) for p in range(NP)] + [("PPV", g) for g in range(NG)]
            + [("PV", p) for p in range(NP)] + [("PS", g) for g in range(NG)]
            + [("S", p) for p in range(NP)])
    fill = [("AP", 0), ("AP", 1)]
    order = []
    now = [0]

    def emit(task):
        order.append(task)
        now[0] += dur[task[0]]
        end[task] = now[0]

    nproj = 0
    while pend:
        cand = [x for x in pend if ready(x) is not None and ready(x) <= now[0]]
        if cand:
            if not proj:
                cand = [x for x in cand if x[0] != "W"] or cand
            pend.remove(cand[0])
            emit(cand[0])
        elif proj:
            emit(proj.pop(0))
            nproj += 1
            if nproj == GP:
                order.append(("LA", 0))
            if nproj in AO_AFTER:
                emit(("AO", AO_AFTER.index(nproj)))
        elif fill:
            emit(fill.pop(0))
        else:
            now[0] = min(ready(x) for x in pend if ready(x) is not None)
    return order + fill + [("AP", 2)]


ORDERS = (
    "K0 K1 K2 K3 V0 LA0 Q1 Q0 V1 S0 V2 PS0 Q2 AO0 S1 V3 Q3 S2 PV0 K4 K5 PPV0 S3 K6 W0 PV1 K7 "
    "PV2 V4 W1 W2 PV3 Q4 AO1 V5 W3 PS1 S4 Q5 V6 Q6 S5 V7 Q7 S6 K8 PPV1 PV4 S7 K9 AO2 K10 W4 PV5 "
    "K11 PV6 V8 W5 W6 PV7 Q8 V9 W7 S8 PS2 Q9 V10 Q10 AO3 S9 V11 PV8 Q11 K12 PPV2 S11 S10 K13 W8 "
    "PV9 K14 K15 W9 PV10 PV11 V12 AO4 Q12 W10 W11 PS3 S12 V13 V15 Q13 Q14 Q15 S13 V14 PV12 S14 "
    "AP0 PPV3 S15 W12 PV13 AP1 PV14 PV15 W13 W14 W15 AP2 ",
    "K0 K1 K2 K3 LA0 V0 Q0 V1 Q1 S0 V2 PS0 Q2 AO0 S1 V3 K4 Q3 S2 PV0 K5 PPV0 S3 K6 PV1 K7 W0 Q4 "
    "W1 PV2 V4 PV3 PS1 AO1 W2 W3 S4 V5 Q5 V6 Q6 S5 V7 Q7 PV4 S6 K8 PPV1 S7 K9 K10 AO2 W4 PV5 "
    "PV6 K11 V8 W5 W6 PV7 Q8 PS2 V9 W7 Q9 S8 V10 Q10 AO3 S9 V11 Q11 PV8 S10 K12 PPV2 S11 K13 "
    "K14 W8 PV9 K15 AO4 PV10 V12 PV11 W10 W9 Q12 PS3 V13 W11 S12 Q13 V14 Q14 S13 V15 Q15 AP0 "
    "S14 PPV3 PV12 S15 AP1 PV13 PV14 W12 PV15 W13 W14 W15 AP2 ",
    "K0 K1 K2 K3 LA0 V0 V1 Q0 Q1 S0 V2 PS0 Q2 AO0 S1 V3 Q3 S2 K4 K5 PPV0 PV0 S3 K6 W0 PV1 K7 "
    "PV2 V4 PV3 W1 W2 Q4 AO1 V5 W3 PS1 S4 Q5 V6 Q6 S5 V7 Q7 S6 K8 S7 PPV1 K9 PV4 AO2 K10 W4 PV5 "
    "PV6 K11 W5 V8 W6 PV7 Q8 W7 V9 PS2 S8 V10 Q9 Q10 AO3 S9 V11 Q11 PV8 S10 K12 PPV2 S11 W8 K13 "
    "PV9 K14 K15 AO4 W9 PV10 PV11 V12 Q12 W10 W11 PS3 S12 Q13 V13 V14 Q14 S13 Q15 PV12 V15 S14 "
    "AP0 PPV3 S15 W12 PV14 PV13 AP1 PV15 W13 W14 W15 AP2 ",
    "K3 K0 K1 K2 LA0 V0 Q0 V1 Q1 S0 V2 PS0 Q2 S1 V3 AO0 S2 K4 PV0 Q3 K5 PPV0 S3 K6 PV1 K7 W0 W1 "
    "PV2 PV3 Q4 V4 W2 W3 AO1 PS1 S4 V5 Q5 V6 Q6 S5 V7 PV4 Q7 S6 K8 S7 K9 AO2 PPV1 K11 K10 W4 "
    "PV5 PV6 V8 W5 PV7 W6 Q8 PS2 V10 V9 W7 S8 Q9 Q10 AO3 S9 V11 Q11 PV8 S10 K12 S11 PPV2 K13 "
    "K14 W8 PV9 K15 AO4 PV10 V12 W9 W10 PV11 Q12 V13 PS3 W11 S12 Q13 V14 S13 V15 Q14 Q15 S14 "
    "AP0 PPV3 PV12 S15 AP1 PV13 PV14 W12 PV15 W13 W14 W15 AP2 ",
)
SKIP_PROLOGUE = False


def _order(u):
    if ORDERS is None or ORDERS[u] is None:
        return _segment_order(u % 2 == 1)
    return [(t.rstrip("0123456789"), int(t.lstrip("ABCDEFGHIJKLMNOPQRSTUVWXYZ")))
            for t in ORDERS[u].split()]


def _nt_dot(a, b):
    return lax.dot_general(a, b, (((1,), (1,)), ((), ())), preferred_element_type=F32)


def _dot(a, b):
    return jnp.dot(a, b, preferred_element_type=F32)


def _pack(x):
    return pltpu.bitcast(x, U32)


def _unpack(x):
    return pltpu.bitcast(x, BF16)


def _recip(x):
    r = pl.reciprocal(x, approx=True)
    return r * (2.0 - x * r)


def _kernel(ax_hbm, awqkv_hbm, awo_hbm, bx_hbm, bx4_hbm, mem0_hbm, wq_hbm, wk_hbm, wv_hbm, wo_hbm,
            out_hbm,
            stage, awo_raw, w_s, wo_s, pre_s, odef_s, out_s,
            xa_s, xb_s, xpre_s, xp_s, xs_s, mem0_s, wa_s, awo_s, t1_s, qa_s, kv_s,
            sems):
    b_scale = B_DH ** (-0.5) * LOG2E
    a_scale = A_DH ** (-0.5) * LOG2E

    w_hbm = (wq_hbm, wk_hbm, wv_hbm)
    wo32 = wo_hbm.bitcast(U32)
    awo32 = awo_hbm.bitcast(U32)
    hw = PW // 2
    hd = B_H * B_DH

    def w_copy(p, half, q, m, sem):
        rows = pl.ds(pl.multiple_of(p * PW, PW), PW)
        return pltpu.make_async_copy(w_hbm[m].at[rows, :], stage.at[half, q, m], sem)

    def divmod5(n):
        c = (n * 13) >> 6
        return c, n - NT * c

    def wa_copy(piece, half, q, sem):
        c, kt = divmod5(piece)
        return pltpu.make_async_copy(
            awqkv_hbm.at[pl.ds(pl.multiple_of(kt * 128, 128), 128),
                         pl.ds(pl.multiple_of(c * D, 128), D)],
            stage.at[half, q, 3, :128], sem)

    def start_trip(g):
        half = g & 1
        src = jnp.minimum(g, NTRIP - 1)
        for q in range(PP):
            for m in range(3):
                w_copy((src + 1) * PP + q, half, q, m, sems.at[half]).start(priority=1)
            wa_copy(1 + src * PP + q, half, q, sems.at[half]).start(priority=1)

    def wait_trip(half):
        for view in (stage.at[half, :, :3], stage.at[half, :, 3, :128]):
            pltpu.make_async_copy(view, view, sems.at[half]).wait()

    wo0 = hd // 2 - NTRIP * WO_ROWS

    def wo_copy(wr):
        return pltpu.make_async_copy(wo32.at[wr, :], wo_s.at[wr, :], sems.at[2])

    def x_copies(xr, sem):
        return [pltpu.make_async_copy(ax_hbm.at[xr, :], xa_s.at[xr, :D], sem),
                pltpu.make_async_copy(bx_hbm.at[xr, :], xb_s.at[xr, :D], sem)]

    xpre_cp = pltpu.make_async_copy(bx4_hbm.at[:, 0], xpre_s, sems.at[3])
    late_cps = [pltpu.make_async_copy(mem0_hbm, mem0_s, sems.at[2])] + [
        pltpu.make_async_copy(awo32.at[:, c * 128:(c + 1) * 128], awo_raw.at[c], sems.at[2])
        for c in range(NT)] + x_copies(pl.ds(0, X_HEAD), sems.at[2])
    x_rest = x_copies(pl.ds(X_HEAD, S - X_HEAD), sems.at[3])
    peel_cps = (
        [w_copy(0, 1, 0, 0, sems.at[4])],
        [w_copy(0, 1, 0, m, sems.at[5]) for m in (1, 2)],
        [w_copy(q, 1, q, m, sems.at[6]) for q in range(1, PP) for m in range(3)]
        + [wa_copy(0, 1, 0, sems.at[6])])

    xpre_cp.start()
    for cps in peel_cps:
        for cp in cps:
            cp.start(priority=1)
    start_trip(0)
    for cp in [wo_copy(pl.ds(0, wo0))] + late_cps:
        cp.start(priority=1)
    kv_s[:, :, :A_HALO, :] = jnp.zeros((2, NT, A_HALO, 128), F32)

    def gather_heads(ref):
        rows = []
        for j in range(A_DH // 2):
            u = ref[pl.ds(j, A_H, stride=A_DH // 2), :]
            rows.append(pltpu.bitcast(u << 16, F32))
            rows.append(pltpu.bitcast(u & jnp.uint32(0xFFFF0000), F32))
        return jnp.concatenate(rows, axis=0)

    def pair_prep(p, half, q, m, chunks=1):
        if SKIP_PROLOGUE:
            return
        wt = stage[half, q, m]
        w_s[p, :, m * PW:(m + 1) * PW] = _pack(wt.T)
        n = NSEG // chunks
        for c in range(chunks):
            xp = _unpack(xp_s[c * n * PRE // 2:(c + 1) * n * PRE // 2, :])
            pre_s[c * n:(c + 1) * n, p, :, m * PW:(m + 1) * PW] = (
                _nt_dot(xp, wt).reshape(n, PRE, PW))

    KH = 256
    HR = NSEG * PRE // 2

    def xq(i, k):
        return _unpack(xp_s[i * HR // 2:(i + 1) * HR // 2, k * KH:(k + 1) * KH])

    def strassen_lhs():
        f = lambda i, k: xq(i, k).astype(F32)
        sums = (f(0, 0) + f(1, 1), f(1, 0) + f(1, 1), f(0, 0) + f(0, 1),
                f(1, 0) - f(0, 0), f(0, 1) - f(1, 1))
        for n, v in enumerate(sums):
            xs_s[n] = _pack(v.astype(BF16))

    def pair_prep2(p, half, m):
        if SKIP_PROLOGUE:
            return
        for q in range(2):
            w_s[p + q, :, m * PW:(m + 1) * PW] = _pack(stage[half, q, m].T)
        nseg = ST_ROWS // PRE
        for j in range(PW // 128):
            rows = slice(j * 128, (j + 1) * 128)
            b = lambda k, q: stage[half, q, m, rows, k * KH:(k + 1) * KH]
            bf = lambda k, q: b(k, q).astype(F32)
            rhs = ((bf(0, 0) + bf(1, 1)).astype(BF16), b(0, 0),
                   (bf(0, 1) - bf(1, 1)).astype(BF16), (bf(1, 0) - bf(0, 0)).astype(BF16),
                   b(1, 1), (bf(0, 0) + bf(0, 1)).astype(BF16),
                   (bf(1, 0) + bf(1, 1)).astype(BF16))
            tail = [stage[half, q, m, rows, 2 * KH:] for q in range(2)]
            for c in range(HR // ST_ROWS):
                r = slice(c * ST_ROWS // 2, (c + 1) * ST_ROWS // 2)
                sm = lambda n: _unpack(xs_s[n, r, :])
                qd = lambda i, k: _unpack(
                    xp_s[(i * HR + c * ST_ROWS) // 2:(i * HR + (c + 1) * ST_ROWS) // 2,
                         k * KH:(k + 1) * KH])
                rest = lambda i: _unpack(
                    xp_s[(i * HR + c * ST_ROWS) // 2:(i * HR + (c + 1) * ST_ROWS) // 2, 2 * KH:])

                def put(i, q, v):
                    s0 = i * (NSEG // 2) + c * nseg
                    pre_s[s0:s0 + nseg, p + q, :, m * PW + j * 128:m * PW + (j + 1) * 128] = (
                        v.reshape(nseg, PRE, 128))

                m5 = _nt_dot(sm(2), rhs[4])
                m3 = _nt_dot(qd(0, 0), rhs[2])
                put(0, 1, _nt_dot(rest(0), tail[1]) + m3 + m5)
                m1 = _nt_dot(sm(0), rhs[0])
                m4 = _nt_dot(qd(1, 1), rhs[3])
                put(0, 0, _nt_dot(rest(0), tail[0]) + _nt_dot(sm(4), rhs[6]) + (m1 + m4 - m5))
                m2 = _nt_dot(sm(1), rhs[1])
                put(1, 0, _nt_dot(rest(1), tail[0]) + m2 + m4)
                put(1, 1, _nt_dot(rest(1), tail[1]) + _nt_dot(sm(3), rhs[5]) + (m1 - m2 + m3))

    def wa_prep(piece, half, q):
        t1_s[q] = _pack(stage[half, q, 3, :128].T)
        c, kt = divmod5(piece)
        wa_s[c, pl.ds(pl.multiple_of(kt * 64, 64), 64), :] = (
            _pack(gather_heads(t1_s.at[q]).astype(BF16).T))

    xpre_cp.wait()
    xp_s[...] = _pack(xpre_s[...].reshape(NSEG * PRE, D))
    if STRASSEN:
        strassen_lhs()
    for cp in peel_cps[0]:
        cp.wait()
    pair_prep(0, 1, 0, 0, PEEL_CHUNKS)
    for cp in peel_cps[1]:
        cp.wait()
    for m in (1, 2):
        pair_prep(0, 1, 0, m, PEEL_CHUNKS)
    for cp in peel_cps[2]:
        cp.wait()
    for q in range(1, PP):
        for m in range(3):
            pair_prep(q, 1, q, m, PEEL_CHUNKS)
    wa_prep(0, 1, 0)

    def prologue(g, carry):
        half = g & 1
        wo_copy(pl.ds(pl.multiple_of(wo0 + g * WO_ROWS, 8), WO_ROWS)).start()
        if STRASSEN:
            start_trip(g + 1)
        wait_trip(half)
        if STRASSEN:
            for m in range(3):
                pair_prep2((g + 1) * PP, half, m)
                if m < PP:
                    wa_prep(1 + g * PP + m, half, m)
            return carry
        for q in range(PP):
            for m in range(3):
                pair_prep((g + 1) * PP + q, half, q, m)
                if q == 0 and m == 0:
                    start_trip(g + 1)
            wa_prep(1 + g * PP + q, half, q)
        return carry

    lax.fori_loop(0, NTRIP, prologue, 0)

    for cp in [wo_copy(slice(None))] + late_cps:
        cp.wait()
    for cp in x_rest:
        cp.start()

    def a_store(m, r):
        for j in range(NT):
            t = r[:, j * 128:(j + 1) * 128]
            if m == 0:
                qa_s[j] = t * a_scale
            else:
                kv_s[m - 1, j, A_HALO:, :] = t

    for m in range(3):
        a_store(m, _dot(xa_s[:SEG, :D], _unpack(wa_s[m])))
    for c in range(NT):
        awo_s[:, c * 128:(c + 1) * 128] = _pack(gather_heads(awo_raw.at[c]).astype(BF16))

    def segment(s, mem, u):
        odd = u % 2 == 1
        row0 = pl.multiple_of(s * SEG, SEG)
        ninf = jnp.float32(-jnp.inf)

        qi = lax.broadcasted_iota(jnp.int32, (SEG, 2 * L), 0)
        kl = lax.broadcasted_iota(jnp.int32, (SEG, 2 * L), 1)
        is_a = kl < L
        kpos = jnp.where(is_a, kl, kl - L)
        allowed = (qi >= FRESH) | (qi + MEM + PRE >= kpos)
        pi = lax.broadcasted_iota(jnp.int32, (GP * PRE, 128), 0)
        pk = lax.broadcasted_iota(jnp.int32, (GP * PRE, 128), 1)
        p_own = (pk // SEG) == (pi // PRE)
        p_allowed = (pk % (MEM + PRE)) <= (pi % PRE) + MEM
        p_first = (pk % SEG) < MEM + PRE
        p_is_a = p_own & p_first
        p_is_b = p_own & jnp.logical_not(p_first)
        col_a = lax.broadcasted_iota(jnp.int32, (1, PW), 1) < B_DH
        col128_a = lax.broadcasted_iota(jnp.int32, (1, 128), 1) < (B_DH - 128)

        xb = xb_s[pl.ds(row0, SEG), :D].astype(F32)
        h = jnp.concatenate([xb[PRE:], mem], axis=0).astype(BF16)

        def proj(p, m):
            return _dot(h, _unpack(w_s[p, :, m * PW:(m + 1) * PW]))

        def pre(p, m):
            return pre_s[s, p, :, m * PW:(m + 1) * PW]

        def block_diag(p, m):
            f = proj(p, m)
            full = jnp.concatenate([f[FRESH:], pre(p, m), f[:FRESH]], axis=0)
            z = jnp.zeros_like(full)
            return jnp.where(col_a, full, z), jnp.where(col_a, z, full)

        def cat(parts):
            return jnp.concatenate(parts, axis=0)

        def qk(q, blocks):
            if not FOLD_T:
                return _dot(q, cat(blocks).T.astype(BF16))
            fold = cat([jnp.concatenate([x[:, :128] if i % 2 == 0 else x[:, 256:], x[:, 128:256]],
                                        axis=1) for i, x in enumerate(blocks)])
            if T_F32:
                t = fold.T
            else:
                t = fold.astype(BF16).T.astype(F32)
            outer = t[:128]
            n = blocks[0].shape[0]
            lane = lax.broadcasted_iota(jnp.int32, outer.shape, 1)
            lane_a = lane < n if len(blocks) == 2 else lane % (2 * n) < n
            z = jnp.zeros_like(outer)
            kt = cat([jnp.where(lane_a, outer, z), t[128:], jnp.where(lane_a, z, outer)])
            return _dot(q, kt.astype(BF16))

        def scores(q, kbd, late_norm):
            sc = qk(q, kbd) * b_scale
            sc = jnp.where(allowed, sc, NEG)
            ma = jnp.max(jnp.where(is_a, sc, ninf), axis=1, keepdims=True)
            mb = jnp.max(jnp.where(is_a, ninf, sc), axis=1, keepdims=True)
            e = jnp.exp2(sc - jnp.where(is_a, ma, mb))
            sa = jnp.sum(jnp.where(is_a, e, 0.0), axis=1, keepdims=True)
            sb = jnp.sum(jnp.where(is_a, 0.0, e), axis=1, keepdims=True)
            def fin(x):
                if PV_PAD:
                    x = jnp.concatenate([x, jnp.zeros((SEG, 128 - 2 * L), F32)], axis=1)
                return x.astype(BF16)
            if late_norm:
                return fin(e), _recip(sa), _recip(sb)
            return fin(e * _recip(jnp.where(is_a, sa, sb))), None, None

        def pv(sm, vbd):
            e, ra, rb = sm
            if PV_PAD:
                vbd = list(vbd) + [jnp.zeros((128 - 2 * L, PW), F32)]
            o = _dot(e, cat(vbd).astype(BF16))
            if ra is not None:
                o = jnp.concatenate([
                    o[:, :128] * ra,
                    o[:, 128:256] * jnp.where(col128_a, ra, rb),
                    o[:, 256:] * rb], axis=1)
            return o

        def pre_scores(g, kbds):
            q = jnp.concatenate([pre(GP * g + r, 0) for r in range(GP)], axis=0).astype(BF16)
            k = [x[:MEM + PRE] for kb in kbds for x in kb]
            sc = qk(q, k) * b_scale
            sc = jnp.where(p_allowed, sc, NEG)
            ma = jnp.max(jnp.where(p_is_a, sc, ninf), axis=1, keepdims=True)
            mb = jnp.max(jnp.where(p_is_b, sc, ninf), axis=1, keepdims=True)
            e = jnp.where(p_own, jnp.exp2(sc - jnp.where(p_first, ma, mb)), 0.0)
            sa = jnp.sum(jnp.where(p_first, e, 0.0), axis=1, keepdims=True)
            sb = jnp.sum(jnp.where(p_first, 0.0, e), axis=1, keepdims=True)
            return (e * _recip(jnp.where(p_first, sa, sb))).astype(BF16)

        def pre_pv(g, pr, vbds):
            v = cat([x[:MEM + PRE] for vb in vbds for x in vb])
            o = _dot(pr, v.astype(BF16))
            if not odd:
                odef_s[g] = o
            return o

        def wout(p, o, opre, acc):
            if odd:
                r = pl.ds((p % GP) * PRE, PRE)
                o = jnp.concatenate(
                    [o, opre[(p % GP) * PRE:(p % GP + 1) * PRE], odef_s[p // GP, r, :]], axis=0)
            contrib = _dot(o.astype(BF16), _unpack(wo_s[p * hw:(p + 1) * hw, :]))
            return contrib if acc is None else acc + contrib

        def window(m, j, w):
            lo = A_HALO - A_DIL * w
            return kv_s[m, j, lo:lo + SEG, :]

        def local_softmax():
            pos = row0 + lax.broadcasted_iota(jnp.int32, (SEG, 128), 0)
            logits = []
            for w in range(A_W):
                t = qa_s[0] * window(0, 0, w)
                for j in range(1, NT):
                    t = t + qa_s[j] * window(0, j, w)
                t = t + pltpu.roll(t, 64, 1)
                t = t + pltpu.roll(t, 32, 1)
                logits.append(t if w == 0 else jnp.where(pos >= A_DIL * w, t, NEG))
            mx = functools.reduce(jnp.maximum, logits)
            es = [jnp.exp2(l - mx) for l in logits]
            inv = _recip(functools.reduce(lambda u, v: u + v, es))
            return es, inv

        def local_out(j, es, inv, acc):
            o = es[0] * window(1, j, 0)
            for w in range(1, A_W):
                o = o + es[w] * window(1, j, w)
            for m in range(2):
                kv_s[m, j, :A_HALO, :] = kv_s[m, j, SEG:, :]
            r = _dot((o * inv).astype(BF16), _unpack(awo_s[j * 64:(j + 1) * 64, :]))
            return r if acc is None else acc + r

        nxt = pl.multiple_of(jnp.minimum(s + 1, NSEG - 1) * SEG, SEG)

        val = {}
        acc = None
        oa = None
        for kind, t in _order(u):
            if kind == "K":
                val[kind, t] = block_diag(t, 1)
            elif kind == "V":
                val[kind, t] = block_diag(t, 2)
            elif kind == "Q":
                val[kind, t] = proj(t, 0).astype(BF16)
            elif kind == "S":
                val[kind, t] = scores(val["Q", t], val["K", t], t >= LATE_FROM)
            elif kind == "PV":
                val[kind, t] = pv(val["S", t], val["V", t])
            elif kind == "PS":
                val[kind, t] = pre_scores(t, [val["K", GP * t + r] for r in range(GP)])
            elif kind == "PPV":
                val[kind, t] = pre_pv(t, val["PS", t], [val["V", GP * t + r] for r in range(GP)])
            elif kind == "W":
                acc = wout(t, val["PV", t], val.get(("PPV", t // GP)), acc)
            elif kind == "LA":
                la = local_softmax()
            elif kind == "AP":
                a_store(t, _dot(xa_s[pl.ds(nxt, SEG), :D], _unpack(wa_s[t])))
            elif kind == "AO":
                oa = local_out(t, la[0], la[1], oa)
                if t == NT - 1:
                    out_s[pl.ds(row0, SEG), :D] = oa.astype(BF16)
        return acc

    def out_copy(i):
        r = pl.ds(pl.multiple_of(i * 2 * SEG, 2 * SEG), 2 * SEG)
        return pltpu.make_async_copy(out_s.at[r, :2 * D], out_hbm.at[r, :], sems.at[7])

    def step(i, mem, u):
        acc0 = segment(2 * i, mem, 2 * u)
        acc1 = segment(2 * i + 1, acc0[FRESH:], 2 * u + 1)
        res = jnp.concatenate([acc1[SEG + PRE:], acc0[:FRESH], acc1[SEG:SEG + PRE], acc1[:FRESH]],
                              axis=0)
        out_s[pl.ds(pl.multiple_of(i * 2 * SEG, 2 * SEG), 2 * SEG), D:2 * D] = res.astype(BF16)
        out_copy(i).start()
        return acc1[FRESH:SEG]

    def steps(i, mem):
        @pl.when(i == 1)
        def _():
            for cp in x_rest:
                cp.wait()

        for u in range(UNR):
            mem = step(i * UNR + u, mem, u)
        return mem

    lax.fori_loop(0, N_STEPS, steps, mem0_s[...].astype(F32))

    wait_trip(NTRIP % 2)

    done = N_STEPS * UNR * 2 * SEG
    pltpu.make_async_copy(out_s.at[:done, :2 * D], out_hbm.at[:done, :], sems.at[7]).wait()


@jax.jit
def pallas_concat_heads__sliding_local_dilated__memory_aug_recurrent_mem_tr__prompt_kernel(
    A_x: jax.Array,
    A_wqkv: jax.Array,
    A_wo: jax.Array,
    B_x: jax.Array,
    B_mem0: jax.Array,
    B_Wq: jax.Array,
    B_Wk: jax.Array,
    B_Wv: jax.Array,
    B_Wo: jax.Array,
    B_seg_len,
):
    del B_seg_len
    assert A_x.shape == (1, S, D) and B_x.shape == (1, S, D)
    hd = B_H * B_DH
    wq_t = jnp.transpose(B_Wq, (1, 2, 0)).reshape(hd, D)
    wk_t = jnp.transpose(B_Wk, (1, 2, 0)).reshape(hd, D)
    wv_t = jnp.transpose(B_Wv, (1, 2, 0)).reshape(hd, D)
    wo = B_Wo.reshape(hd, D)

    any_spec = pl.BlockSpec(memory_space=pl.ANY)
    out = pl.pallas_call(
        _kernel,
        out_shape=jax.ShapeDtypeStruct((S, 2 * D), BF16),
        in_specs=[any_spec] * 10,
        out_specs=any_spec,
        scratch_shapes=[
            pltpu.VMEM((2, PP, 4, PW, D), BF16),
            pltpu.VMEM((NT, D // 2, 128), U32),
            pltpu.VMEM((NP, D // 2, 3 * PW), U32),
            pltpu.VMEM((hd // 2, D), U32),
            pltpu.VMEM((NSEG, NP, PRE, 3 * PW), F32),
            pltpu.VMEM((NG, GP * PRE, PW), F32),
            pltpu.VMEM((S, OUT_W), BF16),
            pltpu.VMEM((S, X_W), BF16),
            pltpu.VMEM((S, X_W), BF16),
            pltpu.VMEM((NSEG, PRE, D), BF16),
            pltpu.VMEM((NSEG * PRE // 2, D), U32),
            pltpu.VMEM((5, NSEG * PRE // 4, 256), U32),
            pltpu.VMEM((MEM, D), BF16),
            pltpu.VMEM((3, D // 2, D), U32),
            pltpu.VMEM((D // 2, D), U32),
            pltpu.VMEM((PP, D // 2, 128), U32),
            pltpu.VMEM((NT, SEG, 128), F32),
            pltpu.VMEM((2, NT, A_HALO + SEG, 128), F32),
            pltpu.SemaphoreType.DMA((8,)),
        ],
        compiler_params=pltpu.CompilerParams(vmem_limit_bytes=120 * 1024 * 1024,
                                             disable_bounds_checks=True),
    )(A_x.reshape(S, D), A_wqkv, A_wo, B_x.reshape(S, D), B_x.reshape(NSEG, SEG // PRE, PRE, D),
      B_mem0.reshape(MEM, D), wq_t, wk_t, wv_t, wo)
    return out.reshape(1, S, 2 * D)
```

```python
import functools

import jax
import jax.numpy as jnp
from jax import lax
import jax.experimental.pallas as pl
import jax.experimental.pallas.tpu as pltpu

F32 = jnp.float32
BF16 = jnp.bfloat16
U32 = jnp.uint32

S = 2048
D = 640
NT = D // 128
A_H = 32
A_DH = D // A_H
A_W = 8
A_DIL = 2
A_HALO = 16
B_H = 32
B_DH = 192
MEM = 8
SEG = 32
NSEG = S // SEG
NP = B_H // 2
PW = 2 * B_DH
PRE = 8
FRESH = SEG - PRE
L = MEM + SEG
GP = 4
NG = NP // GP
LOG2E = 1.4426950408889634
NEG = -1000000000.0 * LOG2E
PP = 2
NTRIP = NP // PP - 1
ST_ROWS = 256
X_HEAD = 160
WO_ROWS = 432
X_W = 1024
OUT_W = 2048
UNR = 2
N_STEPS = NSEG // 2 // UNR

LAT_MM, LAT_SM, LAT_SM_LATE, LAT_T = 190, 650, 330, 600
LATE_FROM = NP - 2
AO_AFTER = (10, 18, 26, 34, 40)
FOLD_T = True
PV_PAD = False
XLU_T_PRE = True
T_F32 = True
XLU_T_MAIN = True


def _segment_order(odd):
    proj = []
    for g in range(NG):
        proj += [("K", GP * g + r) for r in range(GP)]
        for r in range(GP):
            proj += [("V", GP * g + r), ("Q", GP * g + r)]
    dur = {"K": 120, "V": 120, "Q": 120, "S": 24, "PV": 24, "PS": 24, "PPV": 24,
           "W": 180 if odd else 120, "AO": 40, "AP": 200}
    end = {}

    def ready(task):
        k, i = task
        if k == "S":
            deps = [(("Q", i), LAT_MM), (("K", i), LAT_T if XLU_T_MAIN else LAT_MM)]
        elif k == "PV":
            deps = [(("S", i), LAT_SM_LATE if i >= LATE_FROM else LAT_SM), (("V", i), LAT_MM)]
        elif k == "PS":
            deps = [(("K", GP * i + GP - 1), LAT_T if XLU_T_PRE else LAT_MM)]
        elif k == "PPV":
            deps = [(("PS", i), LAT_SM), (("V", GP * i + GP - 1), LAT_MM)]
        else:
            deps = [(("PV", i), LAT_MM)] + ([(("PPV", i // GP), LAT_MM)] if odd else [])
        if any(d not in end for d, _ in deps):
            return None
        return max(end[d] + lat for d, lat in deps)

    pend = ([("W", p) for p in range(NP)] + [("PPV", g) for g in range(NG)]
            + [("PV", p) for p in range(NP)] + [("PS", g) for g in range(NG)]
            + [("S", p) for p in range(NP)])
    fill = [("AP", 0), ("AP", 1)]
    order = []
    now = [0]

    def emit(task):
        order.append(task)
        now[0] += dur[task[0]]
        end[task] = now[0]

    nproj = 0
    while pend:
        cand = [x for x in pend if ready(x) is not None and ready(x) <= now[0]]
        if cand:
            if not proj:
                cand = [x for x in cand if x[0] != "W"] or cand
            pend.remove(cand[0])
            emit(cand[0])
        elif proj:
            emit(proj.pop(0))
            nproj += 1
            if nproj == GP:
                order.append(("LA", 0))
            if nproj in AO_AFTER:
                emit(("AO", AO_AFTER.index(nproj)))
        elif fill:
            emit(fill.pop(0))
        else:
            now[0] = min(ready(x) for x in pend if ready(x) is not None)
    return order + fill + [("AP", 2)]


ORDERS = (
    "K0 K1 K2 K3 V0 LA0 Q1 Q0 V1 S0 V2 PS0 Q2 AO0 S1 V3 Q3 S2 PV0 K4 K5 PPV0 S3 K6 W0 PV1 K7 "
    "PV2 V4 W1 W2 PV3 Q4 AO1 V5 W3 PS1 S4 Q5 V6 Q6 S5 V7 Q7 S6 K8 PPV1 PV4 S7 K9 AO2 K10 W4 PV5 "
    "K11 PV6 V8 W5 W6 PV7 Q8 V9 W7 S8 PS2 Q9 V10 Q10 AO3 S9 V11 PV8 Q11 K12 PPV2 S11 S10 K13 W8 "
    "PV9 K14 K15 W9 PV10 PV11 V12 AO4 Q12 W10 W11 PS3 S12 V13 V15 Q13 Q14 Q15 S13 V14 PV12 S14 "
    "AP0 PPV3 S15 W12 PV13 AP1 PV14 PV15 W13 W14 W15 AP2 ",
    "K0 K1 K2 K3 LA0 V0 Q0 V1 Q1 S0 V2 PS0 Q2 AO0 S1 V3 K4 Q3 S2 PV0 K5 PPV0 S3 K6 PV1 K7 W0 Q4 "
    "W1 PV2 V4 PV3 PS1 AO1 W2 W3 S4 V5 Q5 V6 Q6 S5 V7 Q7 PV4 S6 K8 PPV1 S7 K9 K10 AO2 W4 PV5 "
    "PV6 K11 V8 W5 W6 PV7 Q8 PS2 V9 W7 Q9 S8 V10 Q10 AO3 S9 V11 Q11 PV8 S10 K12 PPV2 S11 K13 "
    "K14 W8 PV9 K15 AO4 PV10 V12 PV11 W10 W9 Q12 PS3 V13 W11 S12 Q13 V14 Q14 S13 V15 Q15 AP0 "
    "S14 PPV3 PV12 S15 AP1 PV13 PV14 W12 PV15 W13 W14 W15 AP2 ",
    "K0 K1 K2 K3 LA0 V0 V1 Q0 Q1 S0 V2 PS0 Q2 AO0 S1 V3 Q3 S2 K4 K5 PPV0 PV0 S3 K6 W0 PV1 K7 "
    "PV2 V4 PV3 W1 W2 Q4 AO1 V5 W3 PS1 S4 Q5 V6 Q6 S5 V7 Q7 S6 K8 S7 PPV1 K9 PV4 AO2 K10 W4 PV5 "
    "PV6 K11 W5 V8 W6 PV7 Q8 W7 V9 PS2 S8 V10 Q9 Q10 AO3 S9 V11 Q11 PV8 S10 K12 PPV2 S11 W8 K13 "
    "PV9 K14 K15 AO4 W9 PV10 PV11 V12 Q12 W10 W11 PS3 S12 Q13 V13 V14 Q14 S13 Q15 PV12 V15 S14 "
    "AP0 PPV3 S15 W12 PV14 PV13 AP1 PV15 W13 W14 W15 AP2 ",
    "K3 K0 K1 K2 LA0 V0 Q0 V1 Q1 S0 V2 PS0 Q2 S1 V3 AO0 S2 K4 PV0 Q3 K5 PPV0 S3 K6 PV1 K7 W0 W1 "
    "PV2 PV3 Q4 V4 W2 W3 AO1 PS1 S4 V5 Q5 V6 Q6 S5 V7 PV4 Q7 S6 K8 S7 K9 AO2 PPV1 K11 K10 W4 "
    "PV5 PV6 V8 W5 PV7 W6 Q8 PS2 V10 V9 W7 S8 Q9 Q10 AO3 S9 V11 Q11 PV8 S10 K12 S11 PPV2 K13 "
    "K14 W8 PV9 K15 AO4 PV10 V12 W9 W10 PV11 Q12 V13 PS3 W11 S12 Q13 V14 S13 V15 Q14 Q15 S14 "
    "AP0 PPV3 PV12 S15 AP1 PV13 PV14 W12 PV15 W13 W14 W15 AP2 ",
)
SKIP_PROLOGUE = False


def _order(u):
    if ORDERS is None or ORDERS[u] is None:
        return _segment_order(u % 2 == 1)
    return [(t.rstrip("0123456789"), int(t.lstrip("ABCDEFGHIJKLMNOPQRSTUVWXYZ")))
            for t in ORDERS[u].split()]


def _nt_dot(a, b):
    return lax.dot_general(a, b, (((1,), (1,)), ((), ())), preferred_element_type=F32)


def _dot(a, b):
    return jnp.dot(a, b, preferred_element_type=F32)


def _pack(x):
    return pltpu.bitcast(x, U32)


def _unpack(x):
    return pltpu.bitcast(x, BF16)


def _recip(x):
    r = pl.reciprocal(x, approx=True)
    return r * (2.0 - x * r)


def _kernel(ax_hbm, awqkv_hbm, awo_hbm, bx_hbm, bx4_hbm, mem0_hbm, wq_hbm, wk_hbm, wv_hbm, wo_hbm,
            out_hbm,
            stage, awo_raw, w_s, wo_s, pre_s, odef_s, out_s,
            xa_s, xb_s, xpre_s, xp_s, xs_s, mem0_s, wa_s, awo_s, t1_s, qa_s, kv_s,
            sems):
    b_scale = B_DH ** (-0.5) * LOG2E
    a_scale = A_DH ** (-0.5) * LOG2E

    w_hbm = (wq_hbm, wk_hbm, wv_hbm)
    wo32 = wo_hbm.bitcast(U32)
    awo32 = awo_hbm.bitcast(U32)
    hw = PW // 2
    hd = B_H * B_DH

    def w_copy(p, half, q, m, sem):
        rows = pl.ds(pl.multiple_of(p * PW, PW), PW)
        return pltpu.make_async_copy(w_hbm[m].at[rows, :], stage.at[half, q, m], sem)

    def divmod5(n):
        c = (n * 13) >> 6
        return c, n - NT * c

    def wa_copy(piece, half, q, sem):
        c, kt = divmod5(piece)
        return pltpu.make_async_copy(
            awqkv_hbm.at[pl.ds(pl.multiple_of(kt * 128, 128), 128),
                         pl.ds(pl.multiple_of(c * D, 128), D)],
            stage.at[half, q, 3, :128], sem)

    def start_trip(g):
        half = g & 1
        src = jnp.minimum(g, NTRIP - 1)
        for q in range(PP):
            for m in range(3):
                w_copy((src + 1) * PP + q, half, q, m, sems.at[half]).start(priority=1)
            wa_copy(1 + src * PP + q, half, q, sems.at[half]).start(priority=1)

    def wait_trip(half):
        for view in (stage.at[half, :, :3], stage.at[half, :, 3, :128]):
            pltpu.make_async_copy(view, view, sems.at[half]).wait()

    wo0 = hd // 2 - NTRIP * WO_ROWS

    def wo_copy(wr):
        return pltpu.make_async_copy(wo32.at[wr, :], wo_s.at[wr, :], sems.at[2])

    def x_copies(xr, sem):
        return [pltpu.make_async_copy(ax_hbm.at[xr, :], xa_s.at[xr, :D], sem),
                pltpu.make_async_copy(bx_hbm.at[xr, :], xb_s.at[xr, :D], sem)]

    xpre_cp = pltpu.make_async_copy(bx4_hbm.at[:, 0], xpre_s, sems.at[3])
    late_cps = [pltpu.make_async_copy(mem0_hbm, mem0_s, sems.at[2])] + [
        pltpu.make_async_copy(awo32.at[:, c * 128:(c + 1) * 128], awo_raw.at[c], sems.at[2])
        for c in range(NT)] + x_copies(pl.ds(0, X_HEAD), sems.at[2])
    x_rest = x_copies(pl.ds(X_HEAD, S - X_HEAD), sems.at[3])
    peel_cps = [[w_copy(q, 1, q, m, sems.at[4 + m]) for q in range(PP)] for m in range(3)]
    peel_cps[2].append(wa_copy(0, 1, 0, sems.at[6]))

    xpre_cp.start()
    for cps in peel_cps:
        for cp in cps:
            cp.start(priority=1)
    start_trip(0)
    for cp in [wo_copy(pl.ds(0, wo0))] + late_cps:
        cp.start(priority=1)
    kv_s[:, :, :A_HALO, :] = jnp.zeros((2, NT, A_HALO, 128), F32)

    def gather_heads(ref):
        rows = []
        for j in range(A_DH // 2):
            u = ref[pl.ds(j, A_H, stride=A_DH // 2), :]
            rows.append(pltpu.bitcast(u << 16, F32))
            rows.append(pltpu.bitcast(u & jnp.uint32(0xFFFF0000), F32))
        return jnp.concatenate(rows, axis=0)

    KH = 256
    HR = NSEG * PRE // 2

    def xq(i, k):
        return _unpack(xp_s[i * HR // 2:(i + 1) * HR // 2, k * KH:(k + 1) * KH])

    def strassen_lhs():
        f = lambda i, k: xq(i, k).astype(F32)
        sums = (f(0, 0) + f(1, 1), f(1, 0) + f(1, 1), f(0, 0) + f(0, 1),
                f(1, 0) - f(0, 0), f(0, 1) - f(1, 1))
        for n, v in enumerate(sums):
            xs_s[n] = _pack(v.astype(BF16))

    def pair_prep2(p, half, m):
        if SKIP_PROLOGUE:
            return
        for q in range(2):
            w_s[p + q, :, m * PW:(m + 1) * PW] = _pack(stage[half, q, m].T)
        nseg = ST_ROWS // PRE
        for j in range(PW // 128):
            rows = slice(j * 128, (j + 1) * 128)
            b = lambda k, q: stage[half, q, m, rows, k * KH:(k + 1) * KH]
            bf = lambda k, q: b(k, q).astype(F32)
            rhs = ((bf(0, 0) + bf(1, 1)).astype(BF16), b(0, 0),
                   (bf(0, 1) - bf(1, 1)).astype(BF16), (bf(1, 0) - bf(0, 0)).astype(BF16),
                   b(1, 1), (bf(0, 0) + bf(0, 1)).astype(BF16),
                   (bf(1, 0) + bf(1, 1)).astype(BF16))
            tail = [stage[half, q, m, rows, 2 * KH:] for q in range(2)]
            for c in range(HR // ST_ROWS):
                r = slice(c * ST_ROWS // 2, (c + 1) * ST_ROWS // 2)
                sm = lambda n: _unpack(xs_s[n, r, :])
                qd = lambda i, k: _unpack(
                    xp_s[(i * HR + c * ST_ROWS) // 2:(i * HR + (c + 1) * ST_ROWS) // 2,
                         k * KH:(k + 1) * KH])
                rest = lambda i: _unpack(
                    xp_s[(i * HR + c * ST_ROWS) // 2:(i * HR + (c + 1) * ST_ROWS) // 2, 2 * KH:])

                def put(i, q, v):
                    s0 = i * (NSEG // 2) + c * nseg
                    pre_s[s0:s0 + nseg, p + q, :, m * PW + j * 128:m * PW + (j + 1) * 128] = (
                        v.reshape(nseg, PRE, 128))

                m5 = _nt_dot(sm(2), rhs[4])
                m3 = _nt_dot(qd(0, 0), rhs[2])
                put(0, 1, _nt_dot(rest(0), tail[1]) + m3 + m5)
                m1 = _nt_dot(sm(0), rhs[0])
                m4 = _nt_dot(qd(1, 1), rhs[3])
                put(0, 0, _nt_dot(rest(0), tail[0]) + _nt_dot(sm(4), rhs[6]) + (m1 + m4 - m5))
                m2 = _nt_dot(sm(1), rhs[1])
                put(1, 0, _nt_dot(rest(1), tail[0]) + m2 + m4)
                put(1, 1, _nt_dot(rest(1), tail[1]) + _nt_dot(sm(3), rhs[5]) + (m1 - m2 + m3))

    def wa_prep(piece, half, q):
        t1_s[q] = _pack(stage[half, q, 3, :128].T)
        c, kt = divmod5(piece)
        wa_s[c, pl.ds(pl.multiple_of(kt * 64, 64), 64), :] = (
            _pack(gather_heads(t1_s.at[q]).astype(BF16).T))

    xpre_cp.wait()
    xp_s[...] = _pack(xpre_s[...].reshape(NSEG * PRE, D))
    strassen_lhs()
    for m in range(3):
        for cp in peel_cps[m]:
            cp.wait()
        pair_prep2(0, 1, m)
    wa_prep(0, 1, 0)

    def prologue(g, carry):
        half = g & 1
        wo_copy(pl.ds(pl.multiple_of(wo0 + g * WO_ROWS, 8), WO_ROWS)).start()
        start_trip(g + 1)
        wait_trip(half)
        for m in range(3):
            pair_prep2((g + 1) * PP, half, m)
            if m < PP:
                wa_prep(1 + g * PP + m, half, m)
        return carry

    lax.fori_loop(0, NTRIP, prologue, 0)

    for cp in [wo_copy(slice(None))] + late_cps:
        cp.wait()
    for cp in x_rest:
        cp.start()

    def a_store(m, r):
        for j in range(NT):
            t = r[:, j * 128:(j + 1) * 128]
            if m == 0:
                qa_s[j] = t * a_scale
            else:
                kv_s[m - 1, j, A_HALO:, :] = t

    for m in range(3):
        a_store(m, _dot(xa_s[:SEG, :D], _unpack(wa_s[m])))
    for c in range(NT):
        awo_s[:, c * 128:(c + 1) * 128] = _pack(gather_heads(awo_raw.at[c]).astype(BF16))

    def segment(s, mem, u):
        odd = u % 2 == 1
        row0 = pl.multiple_of(s * SEG, SEG)
        ninf = jnp.float32(-jnp.inf)

        qi = lax.broadcasted_iota(jnp.int32, (SEG, 2 * L), 0)
        kl = lax.broadcasted_iota(jnp.int32, (SEG, 2 * L), 1)
        is_a = kl < L
        kpos = jnp.where(is_a, kl, kl - L)
        allowed = (qi >= FRESH) | (qi + MEM + PRE >= kpos)
        pi = lax.broadcasted_iota(jnp.int32, (GP * PRE, 128), 0)
        pk = lax.broadcasted_iota(jnp.int32, (GP * PRE, 128), 1)
        p_own = (pk // SEG) == (pi // PRE)
        p_allowed = (pk % (MEM + PRE)) <= (pi % PRE) + MEM
        p_first = (pk % SEG) < MEM + PRE
        p_is_a = p_own & p_first
        p_is_b = p_own & jnp.logical_not(p_first)
        col_a = lax.broadcasted_iota(jnp.int32, (1, PW), 1) < B_DH
        col128_a = lax.broadcasted_iota(jnp.int32, (1, 128), 1) < (B_DH - 128)

        xb = xb_s[pl.ds(row0, SEG), :D].astype(F32)
        h = jnp.concatenate([xb[PRE:], mem], axis=0).astype(BF16)

        def proj(p, m):
            return _dot(h, _unpack(w_s[p, :, m * PW:(m + 1) * PW]))

        def pre(p, m):
            return pre_s[s, p, :, m * PW:(m + 1) * PW]

        def block_diag(p, m):
            f = proj(p, m)
            full = jnp.concatenate([f[FRESH:], pre(p, m), f[:FRESH]], axis=0)
            z = jnp.zeros_like(full)
            return jnp.where(col_a, full, z), jnp.where(col_a, z, full)

        def cat(parts):
            return jnp.concatenate(parts, axis=0)

        def qk(q, blocks):
            if not FOLD_T:
                return _dot(q, cat(blocks).T.astype(BF16))
            fold = cat([jnp.concatenate([x[:, :128] if i % 2 == 0 else x[:, 256:], x[:, 128:256]],
                                        axis=1) for i, x in enumerate(blocks)])
            if T_F32:
                t = fold.T
            else:
                t = fold.astype(BF16).T.astype(F32)
            outer = t[:128]
            n = blocks[0].shape[0]
            lane = lax.broadcasted_iota(jnp.int32, outer.shape, 1)
            lane_a = lane < n if len(blocks) == 2 else lane % (2 * n) < n
            z = jnp.zeros_like(outer)
            kt = cat([jnp.where(lane_a, outer, z), t[128:], jnp.where(lane_a, z, outer)])
            return _dot(q, kt.astype(BF16))

        def scores(q, kbd, late_norm):
            sc = qk(q, kbd) * b_scale
            sc = jnp.where(allowed, sc, NEG)
            ma = jnp.max(jnp.where(is_a, sc, ninf), axis=1, keepdims=True)
            mb = jnp.max(jnp.where(is_a, ninf, sc), axis=1, keepdims=True)
            e = jnp.exp2(sc - jnp.where(is_a, ma, mb))
            sa = jnp.sum(jnp.where(is_a, e, 0.0), axis=1, keepdims=True)
            sb = jnp.sum(jnp.where(is_a, 0.0, e), axis=1, keepdims=True)
            def fin(x):
                if PV_PAD:
                    x = jnp.concatenate([x, jnp.zeros((SEG, 128 - 2 * L), F32)], axis=1)
                return x.astype(BF16)
            if late_norm:
                return fin(e), _recip(sa), _recip(sb)
            return fin(e * _recip(jnp.where(is_a, sa, sb))), None, None

        def pv(sm, vbd):
            e, ra, rb = sm
            if PV_PAD:
                vbd = list(vbd) + [jnp.zeros((128 - 2 * L, PW), F32)]
            o = _dot(e, cat(vbd).astype(BF16))
            if ra is not None:
                o = jnp.concatenate([
                    o[:, :128] * ra,
                    o[:, 128:256] * jnp.where(col128_a, ra, rb),
                    o[:, 256:] * rb], axis=1)
            return o

        def pre_scores(g, kbds):
            q = jnp.concatenate([pre(GP * g + r, 0) for r in range(GP)], axis=0).astype(BF16)
            k = [x[:MEM + PRE] for kb in kbds for x in kb]
            sc = qk(q, k) * b_scale
            sc = jnp.where(p_allowed, sc, NEG)
            ma = jnp.max(jnp.where(p_is_a, sc, ninf), axis=1, keepdims=True)
            mb = jnp.max(jnp.where(p_is_b, sc, ninf), axis=1, keepdims=True)
            e = jnp.where(p_own, jnp.exp2(sc - jnp.where(p_first, ma, mb)), 0.0)
            sa = jnp.sum(jnp.where(p_first, e, 0.0), axis=1, keepdims=True)
            sb = jnp.sum(jnp.where(p_first, 0.0, e), axis=1, keepdims=True)
            return (e * _recip(jnp.where(p_first, sa, sb))).astype(BF16)

        def pre_pv(g, pr, vbds):
            v = cat([x[:MEM + PRE] for vb in vbds for x in vb])
            o = _dot(pr, v.astype(BF16))
            if not odd:
                odef_s[g] = o
            return o

        def wout(p, o, opre, acc):
            if odd:
                r = pl.ds((p % GP) * PRE, PRE)
                o = jnp.concatenate(
                    [o, opre[(p % GP) * PRE:(p % GP + 1) * PRE], odef_s[p // GP, r, :]], axis=0)
            contrib = _dot(o.astype(BF16), _unpack(wo_s[p * hw:(p + 1) * hw, :]))
            return contrib if acc is None else acc + contrib

        def window(m, j, w):
            lo = A_HALO - A_DIL * w
            return kv_s[m, j, lo:lo + SEG, :]

        def local_softmax():
            pos = row0 + lax.broadcasted_iota(jnp.int32, (SEG, 128), 0)
            logits = []
            for w in range(A_W):
                t = qa_s[0] * window(0, 0, w)
                for j in range(1, NT):
                    t = t + qa_s[j] * window(0, j, w)
                t = t + pltpu.roll(t, 64, 1)
                t = t + pltpu.roll(t, 32, 1)
                logits.append(t if w == 0 else jnp.where(pos >= A_DIL * w, t, NEG))
            mx = functools.reduce(jnp.maximum, logits)
            es = [jnp.exp2(l - mx) for l in logits]
            inv = _recip(functools.reduce(lambda u, v: u + v, es))
            return es, inv

        def local_out(j, es, inv, acc):
            o = es[0] * window(1, j, 0)
            for w in range(1, A_W):
                o = o + es[w] * window(1, j, w)
            for m in range(2):
                kv_s[m, j, :A_HALO, :] = kv_s[m, j, SEG:, :]
            r = _dot((o * inv).astype(BF16), _unpack(awo_s[j * 64:(j + 1) * 64, :]))
            return r if acc is None else acc + r

        nxt = pl.multiple_of(jnp.minimum(s + 1, NSEG - 1) * SEG, SEG)

        val = {}
        acc = None
        oa = None
        for kind, t in _order(u):
            if kind == "K":
                val[kind, t] = block_diag(t, 1)
            elif kind == "V":
                val[kind, t] = block_diag(t, 2)
            elif kind == "Q":
                val[kind, t] = proj(t, 0).astype(BF16)
            elif kind == "S":
                val[kind, t] = scores(val["Q", t], val["K", t], t >= LATE_FROM)
            elif kind == "PV":
                val[kind, t] = pv(val["S", t], val["V", t])
            elif kind == "PS":
                val[kind, t] = pre_scores(t, [val["K", GP * t + r] for r in range(GP)])
            elif kind == "PPV":
                val[kind, t] = pre_pv(t, val["PS", t], [val["V", GP * t + r] for r in range(GP)])
            elif kind == "W":
                acc = wout(t, val["PV", t], val.get(("PPV", t // GP)), acc)
            elif kind == "LA":
                la = local_softmax()
            elif kind == "AP":
                a_store(t, _dot(xa_s[pl.ds(nxt, SEG), :D], _unpack(wa_s[t])))
            elif kind == "AO":
                oa = local_out(t, la[0], la[1], oa)
                if t == NT - 1:
                    out_s[pl.ds(row0, SEG), :D] = oa.astype(BF16)
        return acc

    def out_copy(i):
        r = pl.ds(pl.multiple_of(i * 2 * SEG, 2 * SEG), 2 * SEG)
        return pltpu.make_async_copy(out_s.at[r, :2 * D], out_hbm.at[r, :], sems.at[7])

    def step(i, mem, u):
        acc0 = segment(2 * i, mem, 2 * u)
        acc1 = segment(2 * i + 1, acc0[FRESH:], 2 * u + 1)
        res = jnp.concatenate([acc1[SEG + PRE:], acc0[:FRESH], acc1[SEG:SEG + PRE], acc1[:FRESH]],
                              axis=0)
        out_s[pl.ds(pl.multiple_of(i * 2 * SEG, 2 * SEG), 2 * SEG), D:2 * D] = res.astype(BF16)
        out_copy(i).start()
        return acc1[FRESH:SEG]

    def steps(i, mem):
        @pl.when(i == 1)
        def _():
            for cp in x_rest:
                cp.wait()

        for u in range(UNR):
            mem = step(i * UNR + u, mem, u)
        return mem

    lax.fori_loop(0, N_STEPS, steps, mem0_s[...].astype(F32))

    wait_trip(NTRIP % 2)

    done = N_STEPS * UNR * 2 * SEG
    pltpu.make_async_copy(out_s.at[:done, :2 * D], out_hbm.at[:done, :], sems.at[7]).wait()


@jax.jit
def pallas_concat_heads__sliding_local_dilated__memory_aug_recurrent_mem_tr__prompt_kernel(
    A_x: jax.Array,
    A_wqkv: jax.Array,
    A_wo: jax.Array,
    B_x: jax.Array,
    B_mem0: jax.Array,
    B_Wq: jax.Array,
    B_Wk: jax.Array,
    B_Wv: jax.Array,
    B_Wo: jax.Array,
    B_seg_len,
):
    del B_seg_len
    assert A_x.shape == (1, S, D) and B_x.shape == (1, S, D)
    hd = B_H * B_DH
    wq_t = jnp.transpose(B_Wq, (1, 2, 0)).reshape(hd, D)
    wk_t = jnp.transpose(B_Wk, (1, 2, 0)).reshape(hd, D)
    wv_t = jnp.transpose(B_Wv, (1, 2, 0)).reshape(hd, D)
    wo = B_Wo.reshape(hd, D)

    any_spec = pl.BlockSpec(memory_space=pl.ANY)
    out = pl.pallas_call(
        _kernel,
        out_shape=jax.ShapeDtypeStruct((S, 2 * D), BF16),
        in_specs=[any_spec] * 10,
        out_specs=any_spec,
        scratch_shapes=[
            pltpu.VMEM((2, PP, 4, PW, D), BF16),
            pltpu.VMEM((NT, D // 2, 128), U32),
            pltpu.VMEM((NP, D // 2, 3 * PW), U32),
            pltpu.VMEM((hd // 2, D), U32),
            pltpu.VMEM((NSEG, NP, PRE, 3 * PW), F32),
            pltpu.VMEM((NG, GP * PRE, PW), F32),
            pltpu.VMEM((S, OUT_W), BF16),
            pltpu.VMEM((S, X_W), BF16),
            pltpu.VMEM((S, X_W), BF16),
            pltpu.VMEM((NSEG, PRE, D), BF16),
            pltpu.VMEM((NSEG * PRE // 2, D), U32),
            pltpu.VMEM((5, NSEG * PRE // 4, 256), U32),
            pltpu.VMEM((MEM, D), BF16),
            pltpu.VMEM((3, D // 2, D), U32),
            pltpu.VMEM((D // 2, D), U32),
            pltpu.VMEM((PP, D // 2, 128), U32),
            pltpu.VMEM((NT, SEG, 128), F32),
            pltpu.VMEM((2, NT, A_HALO + SEG, 128), F32),
            pltpu.SemaphoreType.DMA((8,)),
        ],
        compiler_params=pltpu.CompilerParams(vmem_limit_bytes=120 * 1024 * 1024,
                                             disable_bounds_checks=True),
    )(A_x.reshape(S, D), A_wqkv, A_wo, B_x.reshape(S, D), B_x.reshape(NSEG, SEG // PRE, PRE, D),
      B_mem0.reshape(MEM, D), wq_t, wk_t, wv_t, wo)
    return out.reshape(1, S, 2 * D)
```

```python
import functools

import jax
import jax.numpy as jnp
from jax import lax
import jax.experimental.pallas as pl
import jax.experimental.pallas.tpu as pltpu

F32 = jnp.float32
BF16 = jnp.bfloat16
U32 = jnp.uint32

S = 2048
D = 640
NT = D // 128
A_H = 32
A_DH = D // A_H
A_W = 8
A_DIL = 2
A_HALO = 16
B_H = 32
B_DH = 192
MEM = 8
SEG = 32
NSEG = S // SEG
NP = B_H // 2
PW = 2 * B_DH
PRE = 8
FRESH = SEG - PRE
L = MEM + SEG
GP = 4
NG = NP // GP
LOG2E = 1.4426950408889634
NEG = -1000000000.0 * LOG2E
PP = 2
NTRIP = NP // PP - 1
ST_ROWS = 256
X_HEAD = 128
WO_ROWS = 432
KV_ROWS = 80
X_W = 1024
OUT_W = 2048
UNR = 2
N_STEPS = NSEG // 2 // UNR

LAT_MM, LAT_SM, LAT_SM_LATE, LAT_T = 190, 650, 420, 600
LATE_FROM = NP - 2
AP_AFTER = (5, 14, 23, 32)
AO_AFTER = (30, 40)
TAIL_FILL = (2, 2)
HOLD_W = (0, 2)
PV_PAD = False


def _segment_order(odd):
    proj = []
    for g in range(NG):
        proj += [("K", GP * g + r) for r in range(GP)]
        for r in range(GP):
            proj += [("V", GP * g + r), ("Q", GP * g + r)]
    dur = {"K": 120, "V": 120, "Q": 120, "S": 24, "PV": 24, "PS": 24, "PPV": 24,
           "W": 180 if odd else 120, "AO": 80, "AP": 125}
    end = {}

    def ready(task):
        k, i = task
        if k == "S":
            deps = [(("Q", i), LAT_MM), (("K", i), LAT_T)]
        elif k == "PV":
            deps = [(("S", i), LAT_SM_LATE if i >= LATE_FROM else LAT_SM), (("V", i), LAT_MM)]
        elif k == "PS":
            deps = [(("K", GP * i + GP - 1), LAT_T)]
        elif k == "PPV":
            deps = [(("PS", i), LAT_SM), (("V", GP * i + GP - 1), LAT_MM)]
        else:
            deps = [(("PV", i), LAT_MM)] + ([(("PPV", i // GP), LAT_MM)] if odd else [])
        if any(d not in end for d, _ in deps):
            return None
        return max(end[d] + lat for d, lat in deps)

    pend = ([("W", p) for p in range(NP)] + [("PPV", g) for g in range(NG)]
            + [("PV", p) for p in range(NP)] + [("PS", g) for g in range(NG)]
            + [("S", p) for p in range(NP)])
    fill = [("AO", j) for j in range(NT)] if odd else [("AP", j) for j in range(9)]
    order = []
    now = [0]

    def emit(task):
        order.append(task)
        now[0] += dur[task[0]]
        end[task] = now[0]

    nproj = 0
    while pend:
        cand = [x for x in pend if ready(x) is not None and ready(x) <= now[0]]
        if proj:
            cand = [x for x in cand if not (x[0] == "W" and x[1] >= NP - GP - HOLD_W[odd])]
        if cand:
            if not proj:
                cand = [x for x in cand if x[0] != "W"] or cand
            pend.remove(cand[0])
            emit(cand[0])
        elif proj:
            emit(proj.pop(0))
            nproj += 1
            if odd and nproj == GP:
                order += [("LA", 0), ("LA", 1)]
            if nproj in (AO_AFTER if odd else AP_AFTER):
                emit(fill.pop(0))
        elif len(fill) > TAIL_FILL[odd]:
            emit(fill.pop(0))
        else:
            now[0] = min(ready(x) for x in pend if ready(x) is not None)
    return order + fill


ORDERS = None
SKIP_PROLOGUE = False


def _order(u):
    if ORDERS is None or ORDERS[u] is None:
        return _segment_order(u % 2 == 1)
    return [(t.rstrip("0123456789"), int(t.lstrip("ABCDEFGHIJKLMNOPQRSTUVWXYZ")))
            for t in ORDERS[u].split()]


def _nt_dot(a, b):
    return lax.dot_general(a, b, (((1,), (1,)), ((), ())), preferred_element_type=F32)


def _dot(a, b):
    return jnp.dot(a, b, preferred_element_type=F32)


def _pack(x):
    return pltpu.bitcast(x, U32)


def _unpack(x):
    return pltpu.bitcast(x, BF16)


def cat(parts):
    return jnp.concatenate(parts, axis=0)


def _recip(x):
    r = pl.reciprocal(x, approx=True)
    return r * (2.0 - x * r)


def _kernel(ax_hbm, awqkv_hbm, awo_hbm, bx_hbm, bx4_hbm, mem0_hbm, wq_hbm, wk_hbm, wv_hbm, wo_hbm,
            out_hbm,
            stage, awo_raw, w_s, wo_s, pre_s, odef_s, out_s,
            xa_s, xb_s, xpre_s, xp_s, xs_s, mem0_s, wa_s, wc_s, awo_s, t1_s, qa_s, kv_s,
            sems):
    b_scale = B_DH ** (-0.5) * LOG2E
    a_scale = A_DH ** (-0.5) * LOG2E

    w_hbm = (wq_hbm, wk_hbm, wv_hbm)
    wo32 = wo_hbm.bitcast(U32)
    awo32 = awo_hbm.bitcast(U32)
    hw = PW // 2
    hd = B_H * B_DH

    def w_copy(p, half, q, m, sem):
        rows = pl.ds(pl.multiple_of(p * PW, PW), PW)
        return pltpu.make_async_copy(w_hbm[m].at[rows, :], stage.at[half, q, m], sem)

    def wa_piece(g, q):
        last = g >= 2 * 3
        return jnp.where(last, 1 + q, g >> 1), jnp.where(last, NT - 1, (g & 1) + 2 * q)

    def wa_copy(c, kt, half, q, sem):
        return pltpu.make_async_copy(
            awqkv_hbm.at[pl.ds(pl.multiple_of(kt * 128, 128), 128),
                         pl.ds(pl.multiple_of(c * D, 128), D)],
            stage.at[half, q, 3, :128], sem)

    def start_trip(g):
        half = g & 1
        src = jnp.minimum(g, NTRIP - 1)
        for q in range(PP):
            for m in range(3):
                w_copy((src + 1) * PP + q, half, q, m, sems.at[half]).start(priority=1)
            wa_copy(*wa_piece(src, q), half, q, sems.at[half]).start(priority=1)

    def wait_trip(half):
        for view in (stage.at[half, :, :3], stage.at[half, :, 3, :128]):
            pltpu.make_async_copy(view, view, sems.at[half]).wait()

    wo0 = hd // 2 - NTRIP * WO_ROWS

    def wo_copy(wr):
        return pltpu.make_async_copy(wo32.at[wr, :], wo_s.at[wr, :], sems.at[2])

    def x_copies(xr, sem):
        return [pltpu.make_async_copy(ax_hbm.at[xr, :], xa_s.at[xr, :D], sem),
                pltpu.make_async_copy(bx_hbm.at[xr, :], xb_s.at[xr, :D], sem)]

    xpre_cp = pltpu.make_async_copy(bx4_hbm.at[:, 0], xpre_s, sems.at[3])
    late_cps = [pltpu.make_async_copy(mem0_hbm, mem0_s, sems.at[2])] + [
        pltpu.make_async_copy(awo32.at[:, c * 128:(c + 1) * 128], awo_raw.at[c], sems.at[2])
        for c in range(NT)] + x_copies(pl.ds(0, X_HEAD), sems.at[2])
    x_rest = x_copies(pl.ds(X_HEAD, S - X_HEAD), sems.at[3])
    peel_cps = [[w_copy(q, 1, q, m, sems.at[4 + m]) for q in range(PP)] for m in range(3)]
    peel_cps[2].append(wa_copy(0, NT - 1, 1, 0, sems.at[6]))

    xpre_cp.start()
    for cps in peel_cps:
        for cp in cps:
            cp.start(priority=1)
    start_trip(0)
    for cp in [wo_copy(pl.ds(0, wo0))] + late_cps:
        cp.start(priority=1)
    kv_s[:, :, :A_HALO, :] = jnp.zeros((2, NT, A_HALO, 128), F32)

    def gather_heads(ref):
        rows = []
        for j in range(A_DH // 2):
            u = ref[pl.ds(j, A_H, stride=A_DH // 2), :]
            rows.append(pltpu.bitcast(u << 16, F32))
            rows.append(pltpu.bitcast(u & jnp.uint32(0xFFFF0000), F32))
        return jnp.concatenate(rows, axis=0)

    KH = 256
    HR = NSEG * PRE // 2

    def xq(i, k):
        return _unpack(xp_s[i * HR // 2:(i + 1) * HR // 2, k * KH:(k + 1) * KH])

    def strassen_lhs():
        f = lambda i, k: xq(i, k).astype(F32)
        sums = (f(0, 0) + f(1, 1), f(1, 0) + f(1, 1), f(0, 0) + f(0, 1),
                f(1, 0) - f(0, 0), f(0, 1) - f(1, 1))
        for n, v in enumerate(sums):
            xs_s[n] = _pack(v.astype(BF16))

    def pair_prep2(p, half, m):
        if SKIP_PROLOGUE:
            return
        for q in range(2):
            w_s[p + q, :, m * PW:(m + 1) * PW] = _pack(stage[half, q, m].T)
        nseg = ST_ROWS // PRE
        for j in range(PW // 128):
            rows = slice(j * 128, (j + 1) * 128)
            b = lambda k, q: stage[half, q, m, rows, k * KH:(k + 1) * KH]
            bf = lambda k, q: b(k, q).astype(F32)
            rhs = ((bf(0, 0) + bf(1, 1)).astype(BF16), b(0, 0),
                   (bf(0, 1) - bf(1, 1)).astype(BF16), (bf(1, 0) - bf(0, 0)).astype(BF16),
                   b(1, 1), (bf(0, 0) + bf(0, 1)).astype(BF16),
                   (bf(1, 0) + bf(1, 1)).astype(BF16))
            tail = [stage[half, q, m, rows, 2 * KH:] for q in range(2)]
            for c in range(HR // ST_ROWS):
                r = slice(c * ST_ROWS // 2, (c + 1) * ST_ROWS // 2)
                sm = lambda n: _unpack(xs_s[n, r, :])
                qd = lambda i, k: _unpack(
                    xp_s[(i * HR + c * ST_ROWS) // 2:(i * HR + (c + 1) * ST_ROWS) // 2,
                         k * KH:(k + 1) * KH])
                rest = lambda i: _unpack(
                    xp_s[(i * HR + c * ST_ROWS) // 2:(i * HR + (c + 1) * ST_ROWS) // 2, 2 * KH:])

                def put(i, q, v):
                    s0 = i * (NSEG // 2) + c * nseg
                    pre_s[s0:s0 + nseg, p + q, :, m * PW + j * 128:m * PW + (j + 1) * 128] = (
                        v.reshape(nseg, PRE, 128))

                m5 = _nt_dot(sm(2), rhs[4])
                m3 = _nt_dot(qd(0, 0), rhs[2])
                put(0, 1, _nt_dot(rest(0), tail[1]) + m3 + m5)
                m1 = _nt_dot(sm(0), rhs[0])
                m4 = _nt_dot(qd(1, 1), rhs[3])
                put(0, 0, _nt_dot(rest(0), tail[0]) + _nt_dot(sm(4), rhs[6]) + (m1 + m4 - m5))
                m2 = _nt_dot(sm(1), rhs[1])
                put(1, 0, _nt_dot(rest(1), tail[0]) + m2 + m4)
                put(1, 1, _nt_dot(rest(1), tail[1]) + _nt_dot(sm(3), rhs[5]) + (m1 - m2 + m3))

    def wa_prep(c, kt, half, q):
        t1_s[q] = _pack(stage[half, q, 3, :128].T)
        g = gather_heads(t1_s.at[q])
        wa_s[c, pl.ds(pl.multiple_of(kt * 64, 64), 64), :] = _pack(g.astype(BF16).T)
        return g

    def wa_trip(g, half):
        lo, hi = [wa_prep(*wa_piece(g, q), half, q) for q in range(2)]
        for t in range(2):
            b11, b12 = lo[2 * t * 128:(2 * t + 1) * 128], lo[(2 * t + 1) * 128:(2 * t + 2) * 128]
            b21, b22 = hi[2 * t * 128:(2 * t + 1) * 128], hi[(2 * t + 1) * 128:(2 * t + 2) * 128]
            sums = cat([b11 + b22, b12 - b22, b21 - b11, b11 + b12, b21 + b22])
            wc_s[g, t] = _pack(sums.astype(BF16).T)

    xpre_cp.wait()
    xp_s[...] = _pack(xpre_s[...].reshape(NSEG * PRE, D))
    strassen_lhs()
    for m in range(3):
        for cp in peel_cps[m]:
            cp.wait()
        pair_prep2(0, 1, m)
    wa_prep(0, NT - 1, 1, 0)

    def prologue(g, carry):
        half = g & 1
        wo_copy(pl.ds(pl.multiple_of(wo0 + g * WO_ROWS, 8), WO_ROWS)).start()
        start_trip(g + 1)
        wait_trip(half)
        for m in range(3):
            pair_prep2((g + 1) * PP, half, m)
            if m == 0:
                wa_trip(g, half)
        return carry

    lax.fori_loop(0, NTRIP, prologue, 0)

    for cp in [wo_copy(slice(None))] + late_cps:
        cp.wait()
    for cp in x_rest:
        cp.start()

    for c in range(NT):
        awo_s[:, c * 128:(c + 1) * 128] = _pack(gather_heads(awo_raw.at[c]).astype(BF16))

    def segment(s, mem, u):
        odd = u % 2 == 1
        row0 = pl.multiple_of(s * SEG, SEG)
        ninf = jnp.float32(-jnp.inf)

        qi = lax.broadcasted_iota(jnp.int32, (SEG, 2 * L), 0)
        kl = lax.broadcasted_iota(jnp.int32, (SEG, 2 * L), 1)
        is_a = kl < L
        kpos = jnp.where(is_a, kl, kl - L)
        allowed = (qi >= FRESH) | (qi + MEM + PRE >= kpos)
        pi = lax.broadcasted_iota(jnp.int32, (GP * PRE, 128), 0)
        pk = lax.broadcasted_iota(jnp.int32, (GP * PRE, 128), 1)
        p_own = (pk // SEG) == (pi // PRE)
        p_allowed = (pk % (MEM + PRE)) <= (pi % PRE) + MEM
        p_first = (pk % SEG) < MEM + PRE
        p_is_a = p_own & p_first
        p_is_b = p_own & jnp.logical_not(p_first)
        col_a = lax.broadcasted_iota(jnp.int32, (1, PW), 1) < B_DH
        col128_a = lax.broadcasted_iota(jnp.int32, (1, 128), 1) < (B_DH - 128)

        xb = xb_s[pl.ds(row0, SEG), :D].astype(F32)
        h = jnp.concatenate([xb[PRE:], mem], axis=0).astype(BF16)

        def proj(p, m):
            return _dot(h, _unpack(w_s[p, :, m * PW:(m + 1) * PW]))

        def pre(p, m):
            return pre_s[s, p, :, m * PW:(m + 1) * PW]

        def block_diag(p, m):
            f = proj(p, m)
            full = jnp.concatenate([f[FRESH:], pre(p, m), f[:FRESH]], axis=0)
            z = jnp.zeros_like(full)
            return jnp.where(col_a, full, z), jnp.where(col_a, z, full)

        def qk(q, blocks):
            fold = cat([jnp.concatenate([x[:, :128] if i % 2 == 0 else x[:, 256:], x[:, 128:256]],
                                        axis=1) for i, x in enumerate(blocks)])
            t = fold.T
            outer = t[:128]
            n = blocks[0].shape[0]
            lane = lax.broadcasted_iota(jnp.int32, outer.shape, 1)
            lane_a = lane < n if len(blocks) == 2 else lane % (2 * n) < n
            z = jnp.zeros_like(outer)
            kt = cat([jnp.where(lane_a, outer, z), t[128:], jnp.where(lane_a, z, outer)])
            return _dot(q, kt.astype(BF16))

        def scores(q, kbd, late_norm):
            sc = qk(q, kbd) * b_scale
            sc = jnp.where(allowed, sc, NEG)
            ma = jnp.max(jnp.where(is_a, sc, ninf), axis=1, keepdims=True)
            mb = jnp.max(jnp.where(is_a, ninf, sc), axis=1, keepdims=True)
            e = jnp.exp2(sc - jnp.where(is_a, ma, mb))
            sa = jnp.sum(jnp.where(is_a, e, 0.0), axis=1, keepdims=True)
            sb = jnp.sum(jnp.where(is_a, 0.0, e), axis=1, keepdims=True)
            def fin(x):
                if PV_PAD:
                    x = jnp.concatenate([x, jnp.zeros((SEG, 128 - 2 * L), F32)], axis=1)
                return x.astype(BF16)
            if late_norm:
                return fin(e), _recip(sa), _recip(sb)
            return fin(e * _recip(jnp.where(is_a, sa, sb))), None, None

        def pv(sm, vbd):
            e, ra, rb = sm
            if PV_PAD:
                vbd = list(vbd) + [jnp.zeros((128 - 2 * L, PW), F32)]
            o = _dot(e, cat(vbd).astype(BF16))
            if ra is not None:
                o = jnp.concatenate([
                    o[:, :128] * ra,
                    o[:, 128:256] * jnp.where(col128_a, ra, rb),
                    o[:, 256:] * rb], axis=1)
            return o

        def pre_scores(g, kbds):
            q = jnp.concatenate([pre(GP * g + r, 0) for r in range(GP)], axis=0).astype(BF16)
            k = [x[:MEM + PRE] for kb in kbds for x in kb]
            sc = qk(q, k) * b_scale
            sc = jnp.where(p_allowed, sc, NEG)
            ma = jnp.max(jnp.where(p_is_a, sc, ninf), axis=1, keepdims=True)
            mb = jnp.max(jnp.where(p_is_b, sc, ninf), axis=1, keepdims=True)
            e = jnp.where(p_own, jnp.exp2(sc - jnp.where(p_first, ma, mb)), 0.0)
            sa = jnp.sum(jnp.where(p_first, e, 0.0), axis=1, keepdims=True)
            sb = jnp.sum(jnp.where(p_first, 0.0, e), axis=1, keepdims=True)
            return (e * _recip(jnp.where(p_first, sa, sb))).astype(BF16)

        def pre_pv(g, pr, vbds):
            v = cat([x[:MEM + PRE] for vb in vbds for x in vb])
            o = _dot(pr, v.astype(BF16))
            if not odd:
                odef_s[g] = o
            return o

        def wout(p, o, opre, acc):
            if odd:
                r = pl.ds((p % GP) * PRE, PRE)
                o = jnp.concatenate(
                    [o, opre[(p % GP) * PRE:(p % GP + 1) * PRE], odef_s[p // GP, r, :]], axis=0)
            contrib = _dot(o.astype(BF16), _unpack(wo_s[p * hw:(p + 1) * hw, :]))
            return contrib if acc is None else acc + contrib

        arow0 = pl.multiple_of((s - u % 2) * SEG, 2 * SEG)

        def a_put(m, j, r):
            if m == 0:
                qa_s[j] = r * a_scale
            else:
                kv_s[m - 1, j, A_HALO:A_HALO + 2 * SEG, :] = r

        def a_proj(idx):
            m, t = divmod(idx, 3)
            if "xa" not in val:
                xa = xa_s[pl.ds(arow0, 2 * SEG), :D]
                xf = xa.astype(F32)
                f = lambda i, k: xf[i * SEG:(i + 1) * SEG, k * KH:(k + 1) * KH]
                val["xa"] = xa
                val["xs"] = [v.astype(BF16) for v in (
                    f(0, 0) + f(1, 1), f(1, 0) + f(1, 1), f(0, 0), f(1, 1), f(0, 0) + f(0, 1),
                    f(1, 0) - f(0, 0), f(0, 1) - f(1, 1))]
                val["xr"] = xf[:, 2 * KH:].astype(BF16)
            if t == 2:
                a_put(m, NT - 1, _dot(val["xa"], _unpack(wa_s[m, :, (NT - 1) * 128:])))
                return
            sm = lambda n: _unpack(cat([wc_s[2 * m + k, t, :, n * 128:(n + 1) * 128]
                                        for k in range(2)]))
            blk = lambda k, j: _unpack(wa_s[m, k * KH // 2:(k + 1) * KH // 2,
                                            (2 * t + j) * 128:(2 * t + j + 1) * 128])
            rhs = (sm(0), blk(0, 0), sm(1), sm(2), blk(1, 1), sm(3), sm(4))
            mm = lambda n: _dot(val["xs"][n], rhs[n])
            tail = [_dot(val["xr"], _unpack(wa_s[m, KH:, (2 * t + j) * 128:(2 * t + j + 1) * 128]))
                    for j in range(2)]
            m1, m2, m3, m4, m5 = [mm(n) for n in range(5)]
            a_put(m, 2 * t, tail[0] + cat([mm(6) + (m1 + m4 - m5), m2 + m4]))
            a_put(m, 2 * t + 1, tail[1] + cat([m3 + m5, mm(5) + (m1 - m2 + m3)]))

        def window(m, j, w, hf):
            lo = A_HALO + hf * SEG - A_DIL * w
            return kv_s[m, j, lo:lo + SEG, :]

        def local_softmax(hf):
            pos = arow0 + hf * SEG + lax.broadcasted_iota(jnp.int32, (SEG, 128), 0)
            rows = slice(hf * SEG, (hf + 1) * SEG)
            logits = []
            for w in range(A_W):
                t = qa_s[0, rows, :] * window(0, 0, w, hf)
                for j in range(1, NT):
                    t = t + qa_s[j, rows, :] * window(0, j, w, hf)
                t = t + pltpu.roll(t, 64, 1)
                t = t + pltpu.roll(t, 32, 1)
                if w > 0 and hf == 0:
                    t = jnp.where(pos >= A_DIL * w, t, NEG)
                logits.append(t)
            mx = functools.reduce(jnp.maximum, logits)
            es = [jnp.exp2(l - mx) for l in logits]
            inv = _recip(functools.reduce(lambda x, y: x + y, es))
            return es, inv

        def local_pv(j, hf):
            es, inv = val["LA", hf]
            o = es[0] * window(1, j, 0, hf)
            for w in range(1, A_W):
                o = o + es[w] * window(1, j, w, hf)
            return o * inv

        def local_out(j, acc):
            wj = _unpack(awo_s[j * 64:(j + 1) * 64, :])
            if ("AX", j) in val:
                r = cat([val["AX", j], _dot(local_pv(j, 1).astype(BF16), wj)])
            else:
                r = _dot(cat([local_pv(j, 0), local_pv(j, 1)]).astype(BF16), wj)
            for m in range(2):
                kv_s[m, j, :A_HALO, :] = kv_s[m, j, 2 * SEG:2 * SEG + A_HALO, :]
            return r if acc is None else acc + r

        val = {}
        acc = None
        oa = None
        for kind, t in _order(u):
            if kind == "K":
                val[kind, t] = block_diag(t, 1)
            elif kind == "V":
                val[kind, t] = block_diag(t, 2)
            elif kind == "Q":
                val[kind, t] = proj(t, 0).astype(BF16)
            elif kind == "S":
                val[kind, t] = scores(val["Q", t], val["K", t], t >= LATE_FROM)
            elif kind == "PV":
                val[kind, t] = pv(val["S", t], val["V", t])
            elif kind == "PS":
                val[kind, t] = pre_scores(t, [val["K", GP * t + r] for r in range(GP)])
            elif kind == "PPV":
                val[kind, t] = pre_pv(t, val["PS", t], [val["V", GP * t + r] for r in range(GP)])
            elif kind == "W":
                acc = wout(t, val["PV", t], val.get(("PPV", t // GP)), acc)
            elif kind == "LA":
                val[kind, t] = local_softmax(t)
            elif kind == "AP":
                a_proj(t)
            elif kind == "AX":
                val[kind, t] = _dot(local_pv(t, 0).astype(BF16),
                                    _unpack(awo_s[t * 64:(t + 1) * 64, :]))
            elif kind == "AO":
                oa = local_out(t, oa)
                if t == NT - 1:
                    out_s[pl.ds(arow0, 2 * SEG), :D] = oa.astype(BF16)
        return acc

    def out_copy(i):
        r = pl.ds(pl.multiple_of(i * 2 * SEG, 2 * SEG), 2 * SEG)
        return pltpu.make_async_copy(out_s.at[r, :2 * D], out_hbm.at[r, :], sems.at[7])

    def step(i, mem, u):
        acc0 = segment(2 * i, mem, 2 * u)
        acc1 = segment(2 * i + 1, acc0[FRESH:], 2 * u + 1)
        res = jnp.concatenate([acc1[SEG + PRE:], acc0[:FRESH], acc1[SEG:SEG + PRE], acc1[:FRESH]],
                              axis=0)
        out_s[pl.ds(pl.multiple_of(i * 2 * SEG, 2 * SEG), 2 * SEG), D:2 * D] = res.astype(BF16)
        out_copy(i).start()
        return acc1[FRESH:SEG]

    def steps(i, mem):
        @pl.when(i == 1)
        def _():
            for cp in x_rest:
                cp.wait()

        for u in range(UNR):
            mem = step(i * UNR + u, mem, u)
        return mem

    lax.fori_loop(0, N_STEPS, steps, mem0_s[...].astype(F32))

    wait_trip(NTRIP % 2)

    done = N_STEPS * UNR * 2 * SEG
    pltpu.make_async_copy(out_s.at[:done, :2 * D], out_hbm.at[:done, :], sems.at[7]).wait()


@jax.jit
def pallas_concat_heads__sliding_local_dilated__memory_aug_recurrent_mem_tr__prompt_kernel(
    A_x: jax.Array,
    A_wqkv: jax.Array,
    A_wo: jax.Array,
    B_x: jax.Array,
    B_mem0: jax.Array,
    B_Wq: jax.Array,
    B_Wk: jax.Array,
    B_Wv: jax.Array,
    B_Wo: jax.Array,
    B_seg_len,
):
    del B_seg_len
    assert A_x.shape == (1, S, D) and B_x.shape == (1, S, D)
    hd = B_H * B_DH
    wq_t = jnp.transpose(B_Wq, (1, 2, 0)).reshape(hd, D)
    wk_t = jnp.transpose(B_Wk, (1, 2, 0)).reshape(hd, D)
    wv_t = jnp.transpose(B_Wv, (1, 2, 0)).reshape(hd, D)
    wo = B_Wo.reshape(hd, D)

    any_spec = pl.BlockSpec(memory_space=pl.ANY)
    out = pl.pallas_call(
        _kernel,
        out_shape=jax.ShapeDtypeStruct((S, 2 * D), BF16),
        in_specs=[any_spec] * 10,
        out_specs=any_spec,
        scratch_shapes=[
            pltpu.VMEM((2, PP, 4, PW, D), BF16),
            pltpu.VMEM((NT, D // 2, 128), U32),
            pltpu.VMEM((NP, D // 2, 3 * PW), U32),
            pltpu.VMEM((hd // 2, D), U32),
            pltpu.VMEM((NSEG, NP, PRE, 3 * PW), F32),
            pltpu.VMEM((NG, GP * PRE, PW), F32),
            pltpu.VMEM((S, OUT_W), BF16),
            pltpu.VMEM((S, X_W), BF16),
            pltpu.VMEM((S, X_W), BF16),
            pltpu.VMEM((NSEG, PRE, D), BF16),
            pltpu.VMEM((NSEG * PRE // 2, D), U32),
            pltpu.VMEM((5, NSEG * PRE // 4, 256), U32),
            pltpu.VMEM((MEM, D), BF16),
            pltpu.VMEM((3, D // 2, D), U32),
            pltpu.VMEM((NTRIP, 2, 64, D), U32),
            pltpu.VMEM((D // 2, D), U32),
            pltpu.VMEM((PP, D // 2, 128), U32),
            pltpu.VMEM((NT, 2 * SEG, 128), F32),
            pltpu.VMEM((2, NT, KV_ROWS, 128), F32),
            pltpu.SemaphoreType.DMA((8,)),
        ],
        compiler_params=pltpu.CompilerParams(vmem_limit_bytes=120 * 1024 * 1024,
                                             disable_bounds_checks=True),
    )(A_x.reshape(S, D), A_wqkv, A_wo, B_x.reshape(S, D), B_x.reshape(NSEG, SEG // PRE, PRE, D),
      B_mem0.reshape(MEM, D), wq_t, wk_t, wv_t, wo)
    return out.reshape(1, S, 2 * D)
```

```python
import functools

import jax
import jax.numpy as jnp
from jax import lax
import jax.experimental.pallas as pl
import jax.experimental.pallas.tpu as pltpu

F32 = jnp.float32
BF16 = jnp.bfloat16
U32 = jnp.uint32

S = 2048
D = 640
NT = D // 128
A_H = 32
A_DH = D // A_H
A_W = 8
A_DIL = 2
A_HALO = 16
B_H = 32
B_DH = 192
MEM = 8
SEG = 32
NSEG = S // SEG
NP = B_H // 2
PW = 2 * B_DH
PRE = 8
FRESH = SEG - PRE
L = MEM + SEG
GP = 4
NG = NP // GP
LOG2E = 1.4426950408889634
NEG = -1000000000.0 * LOG2E
PP = 2
NTRIP = NP // PP - 1
ST_ROWS = 256
X_HEAD = 128
WO_ROWS = 432
KV_ROWS = 80
X_W = 1024
OUT_W = 2048
UNR = 2
N_STEPS = NSEG // 2 // UNR

LAT_MM, LAT_X, LAT_T, LAT_N, LAT_N_LATE = 190, 190, 380, 230, 100
LATE_FROM = NP - 2
AP_AFTER = (6, 16, 26)
AO_AFTER = (30, 40)
TAIL_FILL = (2, 2)
HOLD_W = (0, 2)


def _segment_order(odd):
    proj = []
    for g in range(NG):
        proj += [("K", GP * g + r) for r in range(GP)]
        for r in range(GP):
            proj += [("V", GP * g + r), ("Q", GP * g + r)]
    dur = {"K": 120, "V": 120, "Q": 120, "S": 24, "PV": 24, "PS": 24, "PPV": 24,
           "W": 180 if odd else 120, "AO": 80, "AP": 125,
           "T": 0, "M": 0, "E": 0, "TG": 0, "MG": 0, "EG": 0}
    end = {}

    def ready(task):
        k, i = task
        if k == "T":
            deps = [(("K", i), LAT_MM)]
        elif k == "S":
            deps = [(("Q", i), LAT_MM), (("T", i), LAT_T)]
        elif k == "M":
            deps = [(("S", i), LAT_MM - 40)]
        elif k == "E":
            deps = [(("M", i), LAT_X)]
        elif k == "PV":
            deps = [(("E", i), LAT_N_LATE if i >= LATE_FROM else LAT_N), (("V", i), LAT_MM)]
        elif k == "TG":
            deps = [(("K", GP * i + r), LAT_MM) for r in range(GP)]
        elif k == "PS":
            deps = [(("TG", i), LAT_T)]
        elif k == "MG":
            deps = [(("PS", i), LAT_MM - 40)]
        elif k == "EG":
            deps = [(("MG", i), LAT_X)]
        elif k == "PPV":
            deps = [(("EG", i), LAT_N), (("V", GP * i + GP - 1), LAT_MM)]
        else:
            deps = [(("PV", i), LAT_MM)] + ([(("PPV", i // GP), LAT_MM)] if odd else [])
        if any(d not in end for d, _ in deps):
            return None
        return max(end[d] + lat for d, lat in deps)

    pend = ([(k, p) for k in ("E", "M", "T") for p in range(NP)]
            + [(k, g) for k in ("EG", "MG", "TG") for g in range(NG)]
            + [("W", p) for p in range(NP)] + [("PPV", g) for g in range(NG)]
            + [("PV", p) for p in range(NP)] + [("PS", g) for g in range(NG)]
            + [("S", p) for p in range(NP)])
    fill = [("AO", j) for j in range(NT)] if odd else [("AP", j) for j in range(9)]
    order = []
    now = [0]

    def emit(task):
        order.append(task)
        now[0] += dur[task[0]]
        end[task] = now[0]

    nproj = 0
    while pend:
        cand = [x for x in pend if ready(x) is not None and ready(x) <= now[0]]
        if proj:
            cand = [x for x in cand if not (x[0] == "W" and x[1] >= NP - GP - HOLD_W[odd])]
        if cand:
            if not proj:
                cand = [x for x in cand if x[0] != "W"] or cand
            pend.remove(cand[0])
            emit(cand[0])
        elif proj:
            emit(proj.pop(0))
            nproj += 1
            if odd and nproj == GP:
                order += [("LA", 0), ("LA", 1)]
            if nproj in (AO_AFTER if odd else AP_AFTER):
                emit(fill.pop(0))
        elif len(fill) > TAIL_FILL[odd]:
            emit(fill.pop(0))
        else:
            now[0] = min(ready(x) for x in pend if ready(x) is not None)
    return order + fill


ORDERS = None
SKIP_PROLOGUE = False


def _order(u):
    if ORDERS is None or ORDERS[u] is None:
        return _segment_order(u % 2 == 1)
    return [(t.rstrip("0123456789"), int(t.lstrip("ABCDEFGHIJKLMNOPQRSTUVWXYZ")))
            for t in ORDERS[u].split()]


def _nt_dot(a, b):
    return lax.dot_general(a, b, (((1,), (1,)), ((), ())), preferred_element_type=F32)


def _dot(a, b):
    return jnp.dot(a, b, preferred_element_type=F32)


def _pack(x):
    return pltpu.bitcast(x, U32)


def _unpack(x):
    return pltpu.bitcast(x, BF16)


def cat(parts):
    return jnp.concatenate(parts, axis=0)


def _recip(x):
    r = pl.reciprocal(x, approx=True)
    return r * (2.0 - x * r)


def _kernel(ax_hbm, awqkv_hbm, awo_hbm, bx_hbm, bx4_hbm, mem0_hbm, wq_hbm, wk_hbm, wv_hbm, wo_hbm,
            out_hbm,
            stage, awo_raw, w_s, wo_s, pre_s, odef_s, out_s,
            xa_s, xb_s, xpre_s, xp_s, xs_s, mem0_s, wa_s, wc_s, awo_s, t1_s, qa_s, kv_s,
            sems):
    b_scale = B_DH ** (-0.5) * LOG2E
    a_scale = A_DH ** (-0.5) * LOG2E

    w_hbm = (wq_hbm, wk_hbm, wv_hbm)
    wo32 = wo_hbm.bitcast(U32)
    awo32 = awo_hbm.bitcast(U32)
    hw = PW // 2
    hd = B_H * B_DH

    def w_copy(p, half, q, m, sem):
        rows = pl.ds(pl.multiple_of(p * PW, PW), PW)
        return pltpu.make_async_copy(w_hbm[m].at[rows, :], stage.at[half, q, m], sem)

    def wa_piece(g, q):
        last = g >= 2 * 3
        return jnp.where(last, 1 + q, g >> 1), jnp.where(last, NT - 1, (g & 1) + 2 * q)

    def wa_copy(c, kt, half, q, sem):
        return pltpu.make_async_copy(
            awqkv_hbm.at[pl.ds(pl.multiple_of(kt * 128, 128), 128),
                         pl.ds(pl.multiple_of(c * D, 128), D)],
            stage.at[half, q, 3, :128], sem)

    def start_trip(g):
        half = g & 1
        src = jnp.minimum(g, NTRIP - 1)
        for q in range(PP):
            for m in range(3):
                w_copy((src + 1) * PP + q, half, q, m, sems.at[half]).start(priority=1)
            wa_copy(*wa_piece(src, q), half, q, sems.at[half]).start(priority=1)

    def wait_trip(half):
        for view in (stage.at[half, :, :3], stage.at[half, :, 3, :128]):
            pltpu.make_async_copy(view, view, sems.at[half]).wait()

    wo0 = hd // 2 - NTRIP * WO_ROWS

    def wo_copy(wr):
        return pltpu.make_async_copy(wo32.at[wr, :], wo_s.at[wr, :], sems.at[2])

    def x_copies(xr, sem):
        return [pltpu.make_async_copy(ax_hbm.at[xr, :], xa_s.at[xr, :D], sem),
                pltpu.make_async_copy(bx_hbm.at[xr, :], xb_s.at[xr, :D], sem)]

    xpre_cp = pltpu.make_async_copy(bx4_hbm.at[:, 0], xpre_s, sems.at[3])
    late_cps = [pltpu.make_async_copy(mem0_hbm, mem0_s, sems.at[2])] + [
        pltpu.make_async_copy(awo32.at[:, c * 128:(c + 1) * 128], awo_raw.at[c], sems.at[2])
        for c in range(NT)] + x_copies(pl.ds(0, X_HEAD), sems.at[2])
    x_rest = x_copies(pl.ds(X_HEAD, S - X_HEAD), sems.at[3])
    peel_cps = [[w_copy(q, 1, q, m, sems.at[4 + m]) for q in range(PP)] for m in range(3)]
    peel_cps[2].append(wa_copy(0, NT - 1, 1, 0, sems.at[6]))

    xpre_cp.start()
    for cps in peel_cps:
        for cp in cps:
            cp.start(priority=1)
    start_trip(0)
    for cp in [wo_copy(pl.ds(0, wo0))] + late_cps:
        cp.start(priority=1)
    kv_s[:, :, :A_HALO, :] = jnp.zeros((2, NT, A_HALO, 128), F32)

    def gather_heads(ref):
        rows = []
        for j in range(A_DH // 2):
            u = ref[pl.ds(j, A_H, stride=A_DH // 2), :]
            rows.append(pltpu.bitcast(u << 16, F32))
            rows.append(pltpu.bitcast(u & jnp.uint32(0xFFFF0000), F32))
        return jnp.concatenate(rows, axis=0)

    KH = 256
    HR = NSEG * PRE // 2

    def xq(i, k):
        return _unpack(xp_s[i * HR // 2:(i + 1) * HR // 2, k * KH:(k + 1) * KH])

    def strassen_lhs():
        f = lambda i, k: xq(i, k).astype(F32)
        sums = (f(0, 0) + f(1, 1), f(1, 0) + f(1, 1), f(0, 0) + f(0, 1),
                f(1, 0) - f(0, 0), f(0, 1) - f(1, 1))
        for n, v in enumerate(sums):
            xs_s[n] = _pack(v.astype(BF16))

    def pair_prep2(p, half, m):
        if SKIP_PROLOGUE:
            return
        for q in range(2):
            w_s[p + q, :, m * PW:(m + 1) * PW] = _pack(stage[half, q, m].T)
        nseg = ST_ROWS // PRE
        for j in range(PW // 128):
            rows = slice(j * 128, (j + 1) * 128)
            b = lambda k, q: stage[half, q, m, rows, k * KH:(k + 1) * KH]
            bf = lambda k, q: b(k, q).astype(F32)
            rhs = ((bf(0, 0) + bf(1, 1)).astype(BF16), b(0, 0),
                   (bf(0, 1) - bf(1, 1)).astype(BF16), (bf(1, 0) - bf(0, 0)).astype(BF16),
                   b(1, 1), (bf(0, 0) + bf(0, 1)).astype(BF16),
                   (bf(1, 0) + bf(1, 1)).astype(BF16))
            tail = [stage[half, q, m, rows, 2 * KH:] for q in range(2)]
            for c in range(HR // ST_ROWS):
                r = slice(c * ST_ROWS // 2, (c + 1) * ST_ROWS // 2)
                sm = lambda n: _unpack(xs_s[n, r, :])
                qd = lambda i, k: _unpack(
                    xp_s[(i * HR + c * ST_ROWS) // 2:(i * HR + (c + 1) * ST_ROWS) // 2,
                         k * KH:(k + 1) * KH])
                rest = lambda i: _unpack(
                    xp_s[(i * HR + c * ST_ROWS) // 2:(i * HR + (c + 1) * ST_ROWS) // 2, 2 * KH:])

                def put(i, q, v):
                    s0 = i * (NSEG // 2) + c * nseg
                    pre_s[s0:s0 + nseg, p + q, :, m * PW + j * 128:m * PW + (j + 1) * 128] = (
                        v.reshape(nseg, PRE, 128))

                m5 = _nt_dot(sm(2), rhs[4])
                m3 = _nt_dot(qd(0, 0), rhs[2])
                put(0, 1, _nt_dot(rest(0), tail[1]) + m3 + m5)
                m1 = _nt_dot(sm(0), rhs[0])
                m4 = _nt_dot(qd(1, 1), rhs[3])
                put(0, 0, _nt_dot(rest(0), tail[0]) + _nt_dot(sm(4), rhs[6]) + (m1 + m4 - m5))
                m2 = _nt_dot(sm(1), rhs[1])
                put(1, 0, _nt_dot(rest(1), tail[0]) + m2 + m4)
                put(1, 1, _nt_dot(rest(1), tail[1]) + _nt_dot(sm(3), rhs[5]) + (m1 - m2 + m3))

    def wa_prep(c, kt, half, q):
        t1_s[q] = _pack(stage[half, q, 3, :128].T)
        g = gather_heads(t1_s.at[q])
        wa_s[c, pl.ds(pl.multiple_of(kt * 64, 64), 64), :] = _pack(g.astype(BF16).T)
        return g

    def wa_trip(g, half):
        lo, hi = [wa_prep(*wa_piece(g, q), half, q) for q in range(2)]
        for t in range(2):
            b11, b12 = lo[2 * t * 128:(2 * t + 1) * 128], lo[(2 * t + 1) * 128:(2 * t + 2) * 128]
            b21, b22 = hi[2 * t * 128:(2 * t + 1) * 128], hi[(2 * t + 1) * 128:(2 * t + 2) * 128]
            sums = cat([b11 + b22, b12 - b22, b21 - b11, b11 + b12, b21 + b22])
            wc_s[g, t] = _pack(sums.astype(BF16).T)

    xpre_cp.wait()
    xp_s[...] = _pack(xpre_s[...].reshape(NSEG * PRE, D))
    strassen_lhs()
    for m in range(3):
        for cp in peel_cps[m]:
            cp.wait()
        pair_prep2(0, 1, m)
    wa_prep(0, NT - 1, 1, 0)

    def prologue(g, carry):
        half = g & 1
        wo_copy(pl.ds(pl.multiple_of(wo0 + g * WO_ROWS, 8), WO_ROWS)).start()
        start_trip(g + 1)
        wait_trip(half)
        for m in range(3):
            pair_prep2((g + 1) * PP, half, m)
            if m == 0:
                wa_trip(g, half)
        return carry

    lax.fori_loop(0, NTRIP, prologue, 0)

    for cp in [wo_copy(slice(None))] + late_cps:
        cp.wait()
    for cp in x_rest:
        cp.start()

    for c in range(NT):
        awo_s[:, c * 128:(c + 1) * 128] = _pack(gather_heads(awo_raw.at[c]).astype(BF16))

    def segment(s, mem, u):
        odd = u % 2 == 1
        row0 = pl.multiple_of(s * SEG, SEG)
        ninf = jnp.float32(-jnp.inf)

        qi = lax.broadcasted_iota(jnp.int32, (SEG, 2 * L), 0)
        kl = lax.broadcasted_iota(jnp.int32, (SEG, 2 * L), 1)
        is_a = kl < L
        is_b = kl >= L
        kpos = jnp.where(is_a, kl, kl - L)
        allowed = (qi >= FRESH) | (qi + MEM + PRE >= kpos)
        pi = lax.broadcasted_iota(jnp.int32, (GP * PRE, 128), 0)
        pk = lax.broadcasted_iota(jnp.int32, (GP * PRE, 128), 1)
        p_own = (pk // SEG) == (pi // PRE)
        p_allowed = (pk % (MEM + PRE)) <= (pi % PRE) + MEM
        p_first = (pk % SEG) < MEM + PRE
        p_is_a = p_own & p_first
        p_is_b = p_own & jnp.logical_not(p_first)
        col_a = lax.broadcasted_iota(jnp.int32, (1, PW), 1) < B_DH
        col128_a = lax.broadcasted_iota(jnp.int32, (1, 128), 1) < (B_DH - 128)

        xb = xb_s[pl.ds(row0, SEG), :D].astype(F32)
        h = jnp.concatenate([xb[PRE:], mem], axis=0).astype(BF16)

        def proj(p, m):
            return _dot(h, _unpack(w_s[p, :, m * PW:(m + 1) * PW]))

        def pre(p, m):
            return pre_s[s, p, :, m * PW:(m + 1) * PW]

        def block_diag(p, m):
            f = proj(p, m)
            full = jnp.concatenate([f[FRESH:], pre(p, m), f[:FRESH]], axis=0)
            z = jnp.zeros_like(full)
            return jnp.where(col_a, full, z), jnp.where(col_a, z, full)

        def keys_t(blocks):
            fold = cat([jnp.concatenate([x[:, :128] if i % 2 == 0 else x[:, 256:], x[:, 128:256]],
                                        axis=1) for i, x in enumerate(blocks)])
            t = fold.T
            outer = t[:128]
            n = blocks[0].shape[0]
            lane = lax.broadcasted_iota(jnp.int32, outer.shape, 1)
            lane_a = lane < n if len(blocks) == 2 else lane % (2 * n) < n
            z = jnp.zeros_like(outer)
            kt = cat([jnp.where(lane_a, outer, z), t[128:], jnp.where(lane_a, z, outer)])
            return kt.astype(BF16)

        def row_max(raw, ok, in_a, in_b):
            sc = jnp.where(ok, raw * b_scale, NEG)
            ma = jnp.max(jnp.where(in_a, sc, ninf), axis=1, keepdims=True)
            mb = jnp.max(jnp.where(in_b, sc, ninf), axis=1, keepdims=True)
            return sc, ma, mb

        def probs(mx, first, own, late_norm):
            sc, ma, mb = mx
            e = jnp.exp2(sc - jnp.where(first, ma, mb))
            if own is not None:
                e = jnp.where(own, e, 0.0)
            sa = jnp.sum(jnp.where(first, e, 0.0), axis=1, keepdims=True)
            sb = jnp.sum(jnp.where(first, 0.0, e), axis=1, keepdims=True)
            if late_norm:
                return e.astype(BF16), _recip(sa), _recip(sb)
            return (e * _recip(jnp.where(first, sa, sb))).astype(BF16), None, None

        def pv(sm, vbd):
            e, ra, rb = sm
            o = _dot(e, cat(vbd).astype(BF16))
            if ra is not None:
                o = jnp.concatenate([
                    o[:, :128] * ra,
                    o[:, 128:256] * jnp.where(col128_a, ra, rb),
                    o[:, 256:] * rb], axis=1)
            return o

        def pre_pv(g, pr, vbds):
            v = cat([x[:MEM + PRE] for vb in vbds for x in vb])
            o = _dot(pr, v.astype(BF16))
            if not odd:
                odef_s[g] = o
            return o

        def wout(p, o, opre, acc):
            if odd:
                r = pl.ds((p % GP) * PRE, PRE)
                o = jnp.concatenate(
                    [o, opre[(p % GP) * PRE:(p % GP + 1) * PRE], odef_s[p // GP, r, :]], axis=0)
            contrib = _dot(o.astype(BF16), _unpack(wo_s[p * hw:(p + 1) * hw, :]))
            return contrib if acc is None else acc + contrib

        arow0 = pl.multiple_of((s - u % 2) * SEG, 2 * SEG)

        def a_put(m, j, r):
            if m == 0:
                qa_s[j] = r * a_scale
            else:
                kv_s[m - 1, j, A_HALO:A_HALO + 2 * SEG, :] = r

        def a_proj(idx):
            m, t = divmod(idx, 3)
            if "xa" not in val:
                xa = xa_s[pl.ds(arow0, 2 * SEG), :D]
                xf = xa.astype(F32)
                f = lambda i, k: xf[i * SEG:(i + 1) * SEG, k * KH:(k + 1) * KH]
                val["xa"] = xa
                val["xs"] = [v.astype(BF16) for v in (
                    f(0, 0) + f(1, 1), f(1, 0) + f(1, 1), f(0, 0), f(1, 1), f(0, 0) + f(0, 1),
                    f(1, 0) - f(0, 0), f(0, 1) - f(1, 1))]
                val["xr"] = xf[:, 2 * KH:].astype(BF16)
            if t == 2:
                a_put(m, NT - 1, _dot(val["xa"], _unpack(wa_s[m, :, (NT - 1) * 128:])))
                return
            sm = lambda n: _unpack(cat([wc_s[2 * m + k, t, :, n * 128:(n + 1) * 128]
                                        for k in range(2)]))
            blk = lambda k, j: _unpack(wa_s[m, k * KH // 2:(k + 1) * KH // 2,
                                            (2 * t + j) * 128:(2 * t + j + 1) * 128])
            rhs = (sm(0), blk(0, 0), sm(1), sm(2), blk(1, 1), sm(3), sm(4))
            mm = lambda n: _dot(val["xs"][n], rhs[n])
            tail = [_dot(val["xr"], _unpack(wa_s[m, KH:, (2 * t + j) * 128:(2 * t + j + 1) * 128]))
                    for j in range(2)]
            m1, m2, m3, m4, m5 = [mm(n) for n in range(5)]
            a_put(m, 2 * t, tail[0] + cat([mm(6) + (m1 + m4 - m5), m2 + m4]))
            a_put(m, 2 * t + 1, tail[1] + cat([m3 + m5, mm(5) + (m1 - m2 + m3)]))

        def window(m, j, w, hf):
            lo = A_HALO + hf * SEG - A_DIL * w
            return kv_s[m, j, lo:lo + SEG, :]

        def local_softmax(hf):
            pos = arow0 + hf * SEG + lax.broadcasted_iota(jnp.int32, (SEG, 128), 0)
            rows = slice(hf * SEG, (hf + 1) * SEG)
            logits = []
            for w in range(A_W):
                t = qa_s[0, rows, :] * window(0, 0, w, hf)
                for j in range(1, NT):
                    t = t + qa_s[j, rows, :] * window(0, j, w, hf)
                t = t + pltpu.roll(t, 64, 1)
                t = t + pltpu.roll(t, 32, 1)
                if w > 0 and hf == 0:
                    t = jnp.where(pos >= A_DIL * w, t, NEG)
                logits.append(t)
            mx = functools.reduce(jnp.maximum, logits)
            es = [jnp.exp2(l - mx) for l in logits]
            inv = _recip(functools.reduce(lambda x, y: x + y, es))
            return es, inv

        def local_pv(j, hf):
            es, inv = val["LA", hf]
            o = es[0] * window(1, j, 0, hf)
            for w in range(1, A_W):
                o = o + es[w] * window(1, j, w, hf)
            return o * inv

        def local_out(j, acc):
            wj = _unpack(awo_s[j * 64:(j + 1) * 64, :])
            if ("AX", j) in val:
                r = cat([val["AX", j], _dot(local_pv(j, 1).astype(BF16), wj)])
            else:
                r = _dot(cat([local_pv(j, 0), local_pv(j, 1)]).astype(BF16), wj)
            for m in range(2):
                kv_s[m, j, :A_HALO, :] = kv_s[m, j, 2 * SEG:2 * SEG + A_HALO, :]
            return r if acc is None else acc + r

        val = {}
        acc = None
        oa = None
        for kind, t in _order(u):
            if kind == "K":
                val[kind, t] = block_diag(t, 1)
            elif kind == "V":
                val[kind, t] = block_diag(t, 2)
            elif kind == "Q":
                val[kind, t] = proj(t, 0).astype(BF16)
            elif kind == "T":
                val[kind, t] = keys_t(val["K", t])
            elif kind == "S":
                val[kind, t] = _dot(val["Q", t], val["T", t])
            elif kind == "M":
                val[kind, t] = row_max(val["S", t], allowed, is_a, is_b)
            elif kind == "E":
                val[kind, t] = probs(val["M", t], is_a, None, t >= LATE_FROM)
            elif kind == "PV":
                val[kind, t] = pv(val["E", t], val["V", t])
            elif kind == "TG":
                val[kind, t] = keys_t([x[:MEM + PRE] for r in range(GP)
                                       for x in val["K", GP * t + r]])
            elif kind == "PS":
                q = cat([pre(GP * t + r, 0) for r in range(GP)]).astype(BF16)
                val[kind, t] = _dot(q, val["TG", t])
            elif kind == "MG":
                val[kind, t] = row_max(val["PS", t], p_allowed, p_is_a, p_is_b)
            elif kind == "EG":
                val[kind, t] = probs(val["MG", t], p_first, p_own, False)[0]
            elif kind == "PPV":
                val[kind, t] = pre_pv(t, val["EG", t], [val["V", GP * t + r] for r in range(GP)])
            elif kind == "W":
                acc = wout(t, val["PV", t], val.get(("PPV", t // GP)), acc)
            elif kind == "LA":
                val[kind, t] = local_softmax(t)
            elif kind == "AP":
                a_proj(t)
            elif kind == "AX":
                val[kind, t] = _dot(local_pv(t, 0).astype(BF16),
                                    _unpack(awo_s[t * 64:(t + 1) * 64, :]))
            elif kind == "AO":
                oa = local_out(t, oa)
                if t == NT - 1:
                    out_s[pl.ds(arow0, 2 * SEG), :D] = oa.astype(BF16)
        return acc

    def out_copy(i):
        r = pl.ds(pl.multiple_of(i * 2 * SEG, 2 * SEG), 2 * SEG)
        return pltpu.make_async_copy(out_s.at[r, :2 * D], out_hbm.at[r, :], sems.at[7])

    def step(i, mem, u):
        acc0 = segment(2 * i, mem, 2 * u)
        acc1 = segment(2 * i + 1, acc0[FRESH:], 2 * u + 1)
        res = jnp.concatenate([acc1[SEG + PRE:], acc0[:FRESH], acc1[SEG:SEG + PRE], acc1[:FRESH]],
                              axis=0)
        out_s[pl.ds(pl.multiple_of(i * 2 * SEG, 2 * SEG), 2 * SEG), D:2 * D] = res.astype(BF16)
        out_copy(i).start()
        return acc1[FRESH:SEG]

    def steps(i, mem):
        @pl.when(i == 1)
        def _():
            for cp in x_rest:
                cp.wait()

        for u in range(UNR):
            mem = step(i * UNR + u, mem, u)
        return mem

    lax.fori_loop(0, N_STEPS, steps, mem0_s[...].astype(F32))

    wait_trip(NTRIP % 2)

    done = N_STEPS * UNR * 2 * SEG
    pltpu.make_async_copy(out_s.at[:done, :2 * D], out_hbm.at[:done, :], sems.at[7]).wait()


@jax.jit
def pallas_concat_heads__sliding_local_dilated__memory_aug_recurrent_mem_tr__prompt_kernel(
    A_x: jax.Array,
    A_wqkv: jax.Array,
    A_wo: jax.Array,
    B_x: jax.Array,
    B_mem0: jax.Array,
    B_Wq: jax.Array,
    B_Wk: jax.Array,
    B_Wv: jax.Array,
    B_Wo: jax.Array,
    B_seg_len,
):
    del B_seg_len
    assert A_x.shape == (1, S, D) and B_x.shape == (1, S, D)
    hd = B_H * B_DH
    wq_t = jnp.transpose(B_Wq, (1, 2, 0)).reshape(hd, D)
    wk_t = jnp.transpose(B_Wk, (1, 2, 0)).reshape(hd, D)
    wv_t = jnp.transpose(B_Wv, (1, 2, 0)).reshape(hd, D)
    wo = B_Wo.reshape(hd, D)

    any_spec = pl.BlockSpec(memory_space=pl.ANY)
    out = pl.pallas_call(
        _kernel,
        out_shape=jax.ShapeDtypeStruct((S, 2 * D), BF16),
        in_specs=[any_spec] * 10,
        out_specs=any_spec,
        scratch_shapes=[
            pltpu.VMEM((2, PP, 4, PW, D), BF16),
            pltpu.VMEM((NT, D // 2, 128), U32),
            pltpu.VMEM((NP, D // 2, 3 * PW), U32),
            pltpu.VMEM((hd // 2, D), U32),
            pltpu.VMEM((NSEG, NP, PRE, 3 * PW), F32),
            pltpu.VMEM((NG, GP * PRE, PW), F32),
            pltpu.VMEM((S, OUT_W), BF16),
            pltpu.VMEM((S, X_W), BF16),
            pltpu.VMEM((S, X_W), BF16),
            pltpu.VMEM((NSEG, PRE, D), BF16),
            pltpu.VMEM((NSEG * PRE // 2, D), U32),
            pltpu.VMEM((5, NSEG * PRE // 4, 256), U32),
            pltpu.VMEM((MEM, D), BF16),
            pltpu.VMEM((3, D // 2, D), U32),
            pltpu.VMEM((NTRIP, 2, 64, D), U32),
            pltpu.VMEM((D // 2, D), U32),
            pltpu.VMEM((PP, D // 2, 128), U32),
            pltpu.VMEM((NT, 2 * SEG, 128), F32),
            pltpu.VMEM((2, NT, KV_ROWS, 128), F32),
            pltpu.SemaphoreType.DMA((8,)),
        ],
        compiler_params=pltpu.CompilerParams(vmem_limit_bytes=120 * 1024 * 1024,
                                             disable_bounds_checks=True),
    )(A_x.reshape(S, D), A_wqkv, A_wo, B_x.reshape(S, D), B_x.reshape(NSEG, SEG // PRE, PRE, D),
      B_mem0.reshape(MEM, D), wq_t, wk_t, wv_t, wo)
    return out.reshape(1, S, 2 * D)
```

```python
import functools

import jax
import jax.numpy as jnp
from jax import lax
import jax.experimental.pallas as pl
import jax.experimental.pallas.tpu as pltpu

F32 = jnp.float32
BF16 = jnp.bfloat16
U32 = jnp.uint32

S = 2048
D = 640
NT = D // 128
A_H = 32
A_DH = D // A_H
A_W = 8
A_DIL = 2
A_HALO = 16
B_H = 32
B_DH = 192
MEM = 8
SEG = 32
NSEG = S // SEG
NP = B_H // 2
PW = 2 * B_DH
PRE = 8
FRESH = SEG - PRE
L = MEM + SEG
GP = 4
NG = NP // GP
LOG2E = 1.4426950408889634
NEG = -1000000000.0 * LOG2E
PP = 2
NTRIP = NP // PP - 1
PEEL = (2, 3, 4)
ST_ROWS = 256
X_HEAD = 128
WO_ROWS = 432
KV_ROWS = 80
X_W = 1024
OUT_W = 2048
UNR = 2
N_STEPS = NSEG // 2 // UNR

LAT_MM, LAT_X, LAT_T, LAT_N, LAT_N_LATE = 190, 190, 380, 230, 100
LATE_FROM = NP - 2
AP_AFTER = (6, 16, 26)
AO_AFTER = (30, 40)
TAIL_FILL = (2, 2)
HOLD_W = (0, 2)


def _segment_order(odd):
    proj = []
    for g in range(NG):
        proj += [("K", GP * g + r) for r in range(GP)]
        for r in range(GP):
            proj += [("V", GP * g + r), ("Q", GP * g + r)]
    dur = {"K": 120, "V": 120, "Q": 120, "S": 24, "PV": 24, "PS": 24, "PPV": 24,
           "W": 180 if odd else 120, "AO": 80, "AP": 125,
           "T": 0, "M": 0, "E": 0, "TG": 0, "MG": 0, "EG": 0}
    end = {}

    def ready(task):
        k, i = task
        if k == "T":
            deps = [(("K", i), LAT_MM)]
        elif k == "S":
            deps = [(("Q", i), LAT_MM), (("T", i), LAT_T)]
        elif k == "M":
            deps = [(("S", i), LAT_MM - 40)]
        elif k == "E":
            deps = [(("M", i), LAT_X)]
        elif k == "PV":
            deps = [(("E", i), LAT_N_LATE if i >= LATE_FROM else LAT_N), (("V", i), LAT_MM)]
        elif k == "TG":
            deps = [(("K", GP * i + r), LAT_MM) for r in range(GP)]
        elif k == "PS":
            deps = [(("TG", i), LAT_T)]
        elif k == "MG":
            deps = [(("PS", i), LAT_MM - 40)]
        elif k == "EG":
            deps = [(("MG", i), LAT_X)]
        elif k == "PPV":
            deps = [(("EG", i), LAT_N), (("V", GP * i + GP - 1), LAT_MM)]
        else:
            deps = [(("PV", i), LAT_MM)] + ([(("PPV", i // GP), LAT_MM)] if odd else [])
        if any(d not in end for d, _ in deps):
            return None
        return max(end[d] + lat for d, lat in deps)

    pend = ([(k, p) for k in ("E", "M", "T") for p in range(NP)]
            + [(k, g) for k in ("EG", "MG", "TG") for g in range(NG)]
            + [("W", p) for p in range(NP)] + [("PPV", g) for g in range(NG)]
            + [("PV", p) for p in range(NP)] + [("PS", g) for g in range(NG)]
            + [("S", p) for p in range(NP)])
    fill = [("AO", j) for j in range(NT)] if odd else [("AP", j) for j in (3, 4, 5, 0, 1, 2, 6, 7, 8)]
    order = []
    now = [0]

    def emit(task):
        order.append(task)
        now[0] += dur[task[0]]
        end[task] = now[0]

    nproj = 0
    while pend:
        cand = [x for x in pend if ready(x) is not None and ready(x) <= now[0]]
        if proj:
            cand = [x for x in cand if not (x[0] == "W" and x[1] >= NP - GP - HOLD_W[odd])]
        if cand:
            if not proj:
                cand = [x for x in cand if x[0] != "W"] or cand
            pend.remove(cand[0])
            emit(cand[0])
        elif proj:
            emit(proj.pop(0))
            nproj += 1
            if odd and nproj == GP:
                order += [("LA", 0), ("LA", 1)]
            if nproj in (AO_AFTER if odd else AP_AFTER):
                emit(fill.pop(0))
        elif len(fill) > TAIL_FILL[odd]:
            emit(fill.pop(0))
        else:
            now[0] = min(ready(x) for x in pend if ready(x) is not None)
    return order + fill


ORDERS = None
SKIP_PROLOGUE = False


def _order(u):
    if ORDERS is None or ORDERS[u] is None:
        return _segment_order(u % 2 == 1)
    return [(t.rstrip("0123456789"), int(t.lstrip("ABCDEFGHIJKLMNOPQRSTUVWXYZ")))
            for t in ORDERS[u].split()]


def _nt_dot(a, b):
    return lax.dot_general(a, b, (((1,), (1,)), ((), ())), preferred_element_type=F32)


def _dot(a, b):
    return jnp.dot(a, b, preferred_element_type=F32)


def _pack(x):
    return pltpu.bitcast(x, U32)


def _unpack(x):
    return pltpu.bitcast(x, BF16)


def cat(parts):
    return jnp.concatenate(parts, axis=0)


def _recip(x):
    r = pl.reciprocal(x, approx=True)
    return r * (2.0 - x * r)


def _kernel(ax_hbm, awqkv_hbm, awo_hbm, bx_hbm, bx4_hbm, mem0_hbm, wq_hbm, wk_hbm, wv_hbm, wo_hbm,
            out_hbm,
            stage, awo_raw, w_s, wo_s, pre_s, odef_s, out_s,
            xa_s, xb_s, xpre_s, xp_s, xs_s, mem0_s, wa_s, wc_s, awo_s, t1_s, qa_s, kv_s,
            sems):
    b_scale = B_DH ** (-0.5) * LOG2E
    a_scale = A_DH ** (-0.5) * LOG2E

    w_hbm = (wq_hbm, wk_hbm, wv_hbm)
    wo32 = wo_hbm.bitcast(U32)
    awo32 = awo_hbm.bitcast(U32)
    hw = PW // 2
    hd = B_H * B_DH

    def w_copy(p, half, q, m, sem):
        rows = pl.ds(pl.multiple_of(p * PW, PW), PW)
        return pltpu.make_async_copy(w_hbm[m].at[rows, :], stage.at[half, q, m], sem)

    def wa_piece(g, q):
        last = g >= 2 * 3
        return jnp.where(last, 1 + q, g >> 1), jnp.where(last, NT - 1, (g & 1) + 2 * q)

    def wa_copy(c, kt, half, q, sem):
        return pltpu.make_async_copy(
            awqkv_hbm.at[pl.ds(pl.multiple_of(kt * 128, 128), 128),
                         pl.ds(pl.multiple_of(c * D, 128), D)],
            stage.at[half, q, 3, :128], sem)

    def start_trip(g):
        half = g & 1
        src = jnp.minimum(g, NTRIP - 1)
        for q in range(PP):
            for m in range(3):
                w_copy((src + 1) * PP + q, half, q, m, sems.at[half]).start(priority=1)
            wa_copy(*wa_piece(src, q), half, q, sems.at[half]).start(priority=1)

    def wait_trip(half):
        for view in (stage.at[half, :, :3], stage.at[half, :, 3, :128]):
            pltpu.make_async_copy(view, view, sems.at[half]).wait()

    wo0 = hd // 2 - NTRIP * WO_ROWS

    def wo_copy(wr):
        return pltpu.make_async_copy(wo32.at[wr, :], wo_s.at[wr, :], sems.at[2])

    def x_copies(xr, sem):
        return [pltpu.make_async_copy(ax_hbm.at[xr, :], xa_s.at[xr, :D], sem),
                pltpu.make_async_copy(bx_hbm.at[xr, :], xb_s.at[xr, :D], sem)]

    xpre_cp = pltpu.make_async_copy(bx4_hbm.at[:, 0], xpre_s, sems.at[3])
    late_cps = [pltpu.make_async_copy(mem0_hbm, mem0_s, sems.at[2])] + [
        pltpu.make_async_copy(awo32.at[:, c * 128:(c + 1) * 128], awo_raw.at[c], sems.at[2])
        for c in range(NT)] + x_copies(pl.ds(0, X_HEAD), sems.at[2])
    x_rest = x_copies(pl.ds(X_HEAD, S - X_HEAD), sems.at[3])
    tiles = [(m, j) for m in range(3) for j in range(PW // 128)]
    peel = [tiles[sum(PEEL[:n]):sum(PEEL[:n + 1])] for n in range(len(PEEL))]
    peel_cps = [[pltpu.make_async_copy(w_hbm[m].at[pl.ds(q * PW + j * 128, 128), :],
                                       stage.at[1, q, m, pl.ds(j * 128, 128), :], sems.at[4 + n])
                 for m, j in blk for q in range(PP)] for n, blk in enumerate(peel)]
    peel_cps[-1].append(wa_copy(0, NT - 1, 1, 0, sems.at[3 + len(PEEL)]))

    xpre_cp.start()
    for cps in peel_cps:
        for cp in cps:
            cp.start(priority=1)
    start_trip(0)
    for cp in [wo_copy(pl.ds(0, wo0))] + late_cps:
        cp.start(priority=1)
    kv_s[:, :, :A_HALO, :] = jnp.zeros((2, NT, A_HALO, 128), F32)

    def gather_heads(ref):
        rows = []
        for j in range(A_DH // 2):
            u = ref[pl.ds(j, A_H, stride=A_DH // 2), :]
            rows.append(pltpu.bitcast(u << 16, F32))
            rows.append(pltpu.bitcast(u & jnp.uint32(0xFFFF0000), F32))
        return jnp.concatenate(rows, axis=0)

    KH = 256
    HR = NSEG * PRE // 2

    def xq(i, k):
        return _unpack(xp_s[i * HR // 2:(i + 1) * HR // 2, k * KH:(k + 1) * KH])

    def strassen_lhs():
        f = lambda i, k: xq(i, k).astype(F32)
        sums = (f(0, 0) + f(1, 1), f(1, 0) + f(1, 1), f(0, 0) + f(0, 1),
                f(1, 0) - f(0, 0), f(0, 1) - f(1, 1))
        for n, v in enumerate(sums):
            xs_s[n] = _pack(v.astype(BF16))

    def pair_prep2(p, half, m, js=(0, 1, 2)):
        if SKIP_PROLOGUE:
            return
        for q in range(2):
            lo, hi = js[0] * 128, (js[-1] + 1) * 128
            w_s[p + q, :, m * PW + lo:m * PW + hi] = _pack(stage[half, q, m, lo:hi, :].T)
        nseg = ST_ROWS // PRE
        for j in js:
            rows = slice(j * 128, (j + 1) * 128)
            b = lambda k, q: stage[half, q, m, rows, k * KH:(k + 1) * KH]
            bf = lambda k, q: b(k, q).astype(F32)
            rhs = ((bf(0, 0) + bf(1, 1)).astype(BF16), b(0, 0),
                   (bf(0, 1) - bf(1, 1)).astype(BF16), (bf(1, 0) - bf(0, 0)).astype(BF16),
                   b(1, 1), (bf(0, 0) + bf(0, 1)).astype(BF16),
                   (bf(1, 0) + bf(1, 1)).astype(BF16))
            tail = [stage[half, q, m, rows, 2 * KH:] for q in range(2)]
            for c in range(HR // ST_ROWS):
                r = slice(c * ST_ROWS // 2, (c + 1) * ST_ROWS // 2)
                sm = lambda n: _unpack(xs_s[n, r, :])
                qd = lambda i, k: _unpack(
                    xp_s[(i * HR + c * ST_ROWS) // 2:(i * HR + (c + 1) * ST_ROWS) // 2,
                         k * KH:(k + 1) * KH])
                rest = lambda i: _unpack(
                    xp_s[(i * HR + c * ST_ROWS) // 2:(i * HR + (c + 1) * ST_ROWS) // 2, 2 * KH:])

                def put(i, q, v):
                    s0 = i * (NSEG // 2) + c * nseg
                    pre_s[s0:s0 + nseg, p + q, :, m * PW + j * 128:m * PW + (j + 1) * 128] = (
                        v.reshape(nseg, PRE, 128))

                m5 = _nt_dot(sm(2), rhs[4])
                m3 = _nt_dot(qd(0, 0), rhs[2])
                put(0, 1, _nt_dot(rest(0), tail[1]) + m3 + m5)
                m1 = _nt_dot(sm(0), rhs[0])
                m4 = _nt_dot(qd(1, 1), rhs[3])
                put(0, 0, _nt_dot(rest(0), tail[0]) + _nt_dot(sm(4), rhs[6]) + (m1 + m4 - m5))
                m2 = _nt_dot(sm(1), rhs[1])
                put(1, 0, _nt_dot(rest(1), tail[0]) + m2 + m4)
                put(1, 1, _nt_dot(rest(1), tail[1]) + _nt_dot(sm(3), rhs[5]) + (m1 - m2 + m3))

    def wa_prep(c, kt, half, q):
        t1_s[q] = _pack(stage[half, q, 3, :128].T)
        g = gather_heads(t1_s.at[q])
        wa_s[c, pl.ds(pl.multiple_of(kt * 64, 64), 64), :] = _pack(g.astype(BF16).T)
        return g

    def wa_trip(g, half):
        lo, hi = [wa_prep(*wa_piece(g, q), half, q) for q in range(2)]
        for t in range(2):
            b11, b12 = lo[2 * t * 128:(2 * t + 1) * 128], lo[(2 * t + 1) * 128:(2 * t + 2) * 128]
            b21, b22 = hi[2 * t * 128:(2 * t + 1) * 128], hi[(2 * t + 1) * 128:(2 * t + 2) * 128]
            sums = cat([b11 + b22, b12 - b22, b21 - b11, b11 + b12, b21 + b22])
            wc_s[g, t] = _pack(sums.astype(BF16).T)

    xpre_cp.wait()
    xp_s[...] = _pack(xpre_s[...].reshape(NSEG * PRE, D))
    strassen_lhs()
    for blk, cps in zip(peel, peel_cps):
        for cp in cps:
            cp.wait()
        for m in range(3):
            js = tuple(j for mm, j in blk if mm == m)
            if js:
                pair_prep2(0, 1, m, js)
    wa_prep(0, NT - 1, 1, 0)

    def prologue(g, carry):
        half = g & 1
        wo_copy(pl.ds(pl.multiple_of(wo0 + g * WO_ROWS, 8), WO_ROWS)).start()
        start_trip(g + 1)
        wait_trip(half)
        for m in range(3):
            pair_prep2((g + 1) * PP, half, m)
            if m == 0:
                wa_trip(g, half)
        return carry

    lax.fori_loop(0, NTRIP, prologue, 0)

    for cp in [wo_copy(slice(None))] + late_cps:
        cp.wait()
    for cp in x_rest:
        cp.start()

    for c in range(NT):
        awo_s[:, c * 128:(c + 1) * 128] = _pack(gather_heads(awo_raw.at[c]).astype(BF16))

    def segment(s, mem, u):
        odd = u % 2 == 1
        row0 = pl.multiple_of(s * SEG, SEG)
        ninf = jnp.float32(-jnp.inf)

        qi = lax.broadcasted_iota(jnp.int32, (SEG, 2 * L), 0)
        kl = lax.broadcasted_iota(jnp.int32, (SEG, 2 * L), 1)
        is_a = kl < L
        is_b = kl >= L
        kpos = jnp.where(is_a, kl, kl - L)
        allowed = (qi >= FRESH) | (qi + MEM + PRE >= kpos)
        pi = lax.broadcasted_iota(jnp.int32, (GP * PRE, 128), 0)
        pk = lax.broadcasted_iota(jnp.int32, (GP * PRE, 128), 1)
        p_own = (pk // SEG) == (pi // PRE)
        p_allowed = (pk % (MEM + PRE)) <= (pi % PRE) + MEM
        p_first = (pk % SEG) < MEM + PRE
        p_is_a = p_own & p_first
        p_is_b = p_own & jnp.logical_not(p_first)
        col_a = lax.broadcasted_iota(jnp.int32, (1, PW), 1) < B_DH
        col128_a = lax.broadcasted_iota(jnp.int32, (1, 128), 1) < (B_DH - 128)

        xb = xb_s[pl.ds(row0, SEG), :D].astype(F32)
        h = jnp.concatenate([xb[PRE:], mem], axis=0).astype(BF16)

        def proj(p, m):
            return _dot(h, _unpack(w_s[p, :, m * PW:(m + 1) * PW]))

        def pre(p, m):
            return pre_s[s, p, :, m * PW:(m + 1) * PW]

        def block_diag(p, m):
            f = proj(p, m)
            full = jnp.concatenate([f[FRESH:], pre(p, m), f[:FRESH]], axis=0)
            z = jnp.zeros_like(full)
            return jnp.where(col_a, full, z), jnp.where(col_a, z, full)

        def keys_t(blocks):
            fold = cat([jnp.concatenate([x[:, :128] if i % 2 == 0 else x[:, 256:], x[:, 128:256]],
                                        axis=1) for i, x in enumerate(blocks)])
            t = fold.T
            outer = t[:128]
            n = blocks[0].shape[0]
            lane = lax.broadcasted_iota(jnp.int32, outer.shape, 1)
            lane_a = lane < n if len(blocks) == 2 else lane % (2 * n) < n
            z = jnp.zeros_like(outer)
            kt = cat([jnp.where(lane_a, outer, z), t[128:], jnp.where(lane_a, z, outer)])
            return kt.astype(BF16)

        def row_max(raw, ok, in_a, in_b):
            sc = jnp.where(ok, raw * b_scale, NEG)
            ma = jnp.max(jnp.where(in_a, sc, ninf), axis=1, keepdims=True)
            mb = jnp.max(jnp.where(in_b, sc, ninf), axis=1, keepdims=True)
            return sc, ma, mb

        def probs(mx, first, own, late_norm):
            sc, ma, mb = mx
            e = jnp.exp2(sc - jnp.where(first, ma, mb))
            if own is not None:
                e = jnp.where(own, e, 0.0)
            sa = jnp.sum(jnp.where(first, e, 0.0), axis=1, keepdims=True)
            sb = jnp.sum(jnp.where(first, 0.0, e), axis=1, keepdims=True)
            if late_norm:
                return e.astype(BF16), _recip(sa), _recip(sb)
            return (e * _recip(jnp.where(first, sa, sb))).astype(BF16), None, None

        def pv(sm, vbd):
            e, ra, rb = sm
            o = _dot(e, cat(vbd).astype(BF16))
            if ra is not None:
                o = jnp.concatenate([
                    o[:, :128] * ra,
                    o[:, 128:256] * jnp.where(col128_a, ra, rb),
                    o[:, 256:] * rb], axis=1)
            return o

        def pre_pv(g, pr, vbds):
            v = cat([x[:MEM + PRE] for vb in vbds for x in vb])
            o = _dot(pr, v.astype(BF16))
            if not odd:
                odef_s[g] = o
            return o

        def wout(p, o, opre, acc):
            if odd:
                r = pl.ds((p % GP) * PRE, PRE)
                o = jnp.concatenate(
                    [o, opre[(p % GP) * PRE:(p % GP + 1) * PRE], odef_s[p // GP, r, :]], axis=0)
            contrib = _dot(o.astype(BF16), _unpack(wo_s[p * hw:(p + 1) * hw, :]))
            return contrib if acc is None else acc + contrib

        arow0 = pl.multiple_of((s - u % 2) * SEG, 2 * SEG)

        def a_put(m, j, r):
            if m == 0:
                qa_s[j] = r * a_scale
            else:
                kv_s[m - 1, j, A_HALO:A_HALO + 2 * SEG, :] = r

        def a_proj(idx):
            m, t = divmod(idx, 3)
            if "xa" not in val:
                xa = xa_s[pl.ds(arow0, 2 * SEG), :D]
                xf = xa.astype(F32)
                f = lambda i, k: xf[i * SEG:(i + 1) * SEG, k * KH:(k + 1) * KH]
                val["xa"] = xa
                val["xs"] = [v.astype(BF16) for v in (
                    f(0, 0) + f(1, 1), f(1, 0) + f(1, 1), f(0, 0), f(1, 1), f(0, 0) + f(0, 1),
                    f(1, 0) - f(0, 0), f(0, 1) - f(1, 1))]
                val["xr"] = xf[:, 2 * KH:].astype(BF16)
            if t == 2:
                a_put(m, NT - 1, _dot(val["xa"], _unpack(wa_s[m, :, (NT - 1) * 128:])))
                return
            sm = lambda n: _unpack(cat([wc_s[2 * m + k, t, :, n * 128:(n + 1) * 128]
                                        for k in range(2)]))
            blk = lambda k, j: _unpack(wa_s[m, k * KH // 2:(k + 1) * KH // 2,
                                            (2 * t + j) * 128:(2 * t + j + 1) * 128])
            rhs = (sm(0), blk(0, 0), sm(1), sm(2), blk(1, 1), sm(3), sm(4))
            mm = lambda n: _dot(val["xs"][n], rhs[n])
            tail = [_dot(val["xr"], _unpack(wa_s[m, KH:, (2 * t + j) * 128:(2 * t + j + 1) * 128]))
                    for j in range(2)]
            m1, m2, m3, m4, m5 = [mm(n) for n in range(5)]
            a_put(m, 2 * t, tail[0] + cat([mm(6) + (m1 + m4 - m5), m2 + m4]))
            a_put(m, 2 * t + 1, tail[1] + cat([m3 + m5, mm(5) + (m1 - m2 + m3)]))

        def window(m, j, w, hf):
            lo = A_HALO + hf * SEG - A_DIL * w
            return kv_s[m, j, lo:lo + SEG, :]

        def local_softmax(hf):
            pos = arow0 + hf * SEG + lax.broadcasted_iota(jnp.int32, (SEG, 128), 0)
            rows = slice(hf * SEG, (hf + 1) * SEG)
            logits = []
            for w in range(A_W):
                t = qa_s[0, rows, :] * window(0, 0, w, hf)
                for j in range(1, NT):
                    t = t + qa_s[j, rows, :] * window(0, j, w, hf)
                t = t + pltpu.roll(t, 64, 1)
                t = t + pltpu.roll(t, 32, 1)
                if w > 0 and hf == 0:
                    t = jnp.where(pos >= A_DIL * w, t, NEG)
                logits.append(t)
            mx = functools.reduce(jnp.maximum, logits)
            es = [jnp.exp2(l - mx) for l in logits]
            inv = _recip(functools.reduce(lambda x, y: x + y, es))
            return es, inv

        def local_pv(j, hf):
            es, inv = val["LA", hf]
            o = es[0] * window(1, j, 0, hf)
            for w in range(1, A_W):
                o = o + es[w] * window(1, j, w, hf)
            return o * inv

        def local_out(j, acc):
            wj = _unpack(awo_s[j * 64:(j + 1) * 64, :])
            if ("AX", j) in val:
                r = cat([val["AX", j], _dot(local_pv(j, 1).astype(BF16), wj)])
            else:
                r = _dot(cat([local_pv(j, 0), local_pv(j, 1)]).astype(BF16), wj)
            for m in range(2):
                kv_s[m, j, :A_HALO, :] = kv_s[m, j, 2 * SEG:2 * SEG + A_HALO, :]
            return r if acc is None else acc + r

        val = {}
        acc = None
        oa = None
        for kind, t in _order(u):
            if kind == "K":
                val[kind, t] = block_diag(t, 1)
            elif kind == "V":
                val[kind, t] = block_diag(t, 2)
            elif kind == "Q":
                val[kind, t] = proj(t, 0).astype(BF16)
            elif kind == "T":
                val[kind, t] = keys_t(val["K", t])
            elif kind == "S":
                val[kind, t] = _dot(val["Q", t], val["T", t])
            elif kind == "M":
                val[kind, t] = row_max(val["S", t], allowed, is_a, is_b)
            elif kind == "E":
                val[kind, t] = probs(val["M", t], is_a, None, t >= LATE_FROM)
            elif kind == "PV":
                val[kind, t] = pv(val["E", t], val["V", t])
            elif kind == "TG":
                val[kind, t] = keys_t([x[:MEM + PRE] for r in range(GP)
                                       for x in val["K", GP * t + r]])
            elif kind == "PS":
                q = cat([pre(GP * t + r, 0) for r in range(GP)]).astype(BF16)
                val[kind, t] = _dot(q, val["TG", t])
            elif kind == "MG":
                val[kind, t] = row_max(val["PS", t], p_allowed, p_is_a, p_is_b)
            elif kind == "EG":
                val[kind, t] = probs(val["MG", t], p_first, p_own, False)[0]
            elif kind == "PPV":
                val[kind, t] = pre_pv(t, val["EG", t], [val["V", GP * t + r] for r in range(GP)])
            elif kind == "W":
                acc = wout(t, val["PV", t], val.get(("PPV", t // GP)), acc)
            elif kind == "LA":
                val[kind, t] = local_softmax(t)
            elif kind == "AP":
                a_proj(t)
            elif kind == "AX":
                val[kind, t] = _dot(local_pv(t, 0).astype(BF16),
                                    _unpack(awo_s[t * 64:(t + 1) * 64, :]))
            elif kind == "AO":
                oa = local_out(t, oa)
                if t == NT - 1:
                    out_s[pl.ds(arow0, 2 * SEG), :D] = oa.astype(BF16)
        return acc

    def out_copy(i):
        r = pl.ds(pl.multiple_of(i * 2 * SEG, 2 * SEG), 2 * SEG)
        return pltpu.make_async_copy(out_s.at[r, :2 * D], out_hbm.at[r, :], sems.at[7])

    def step(i, mem, u):
        acc0 = segment(2 * i, mem, 2 * u)
        acc1 = segment(2 * i + 1, acc0[FRESH:], 2 * u + 1)
        res = jnp.concatenate([acc1[SEG + PRE:], acc0[:FRESH], acc1[SEG:SEG + PRE], acc1[:FRESH]],
                              axis=0)
        out_s[pl.ds(pl.multiple_of(i * 2 * SEG, 2 * SEG), 2 * SEG), D:2 * D] = res.astype(BF16)
        out_copy(i).start()
        return acc1[FRESH:SEG]

    def steps(i, mem):
        @pl.when(i == 1)
        def _():
            for cp in x_rest:
                cp.wait()

        for u in range(UNR):
            mem = step(i * UNR + u, mem, u)
        return mem

    lax.fori_loop(0, N_STEPS, steps, mem0_s[...].astype(F32))

    wait_trip(NTRIP % 2)

    done = N_STEPS * UNR * 2 * SEG
    pltpu.make_async_copy(out_s.at[:done, :2 * D], out_hbm.at[:done, :], sems.at[7]).wait()


@jax.jit
def pallas_concat_heads__sliding_local_dilated__memory_aug_recurrent_mem_tr__prompt_kernel(
    A_x: jax.Array,
    A_wqkv: jax.Array,
    A_wo: jax.Array,
    B_x: jax.Array,
    B_mem0: jax.Array,
    B_Wq: jax.Array,
    B_Wk: jax.Array,
    B_Wv: jax.Array,
    B_Wo: jax.Array,
    B_seg_len,
):
    del B_seg_len
    assert A_x.shape == (1, S, D) and B_x.shape == (1, S, D)
    hd = B_H * B_DH
    wq_t = jnp.transpose(B_Wq, (1, 2, 0)).reshape(hd, D)
    wk_t = jnp.transpose(B_Wk, (1, 2, 0)).reshape(hd, D)
    wv_t = jnp.transpose(B_Wv, (1, 2, 0)).reshape(hd, D)
    wo = B_Wo.reshape(hd, D)

    any_spec = pl.BlockSpec(memory_space=pl.ANY)
    out = pl.pallas_call(
        _kernel,
        out_shape=jax.ShapeDtypeStruct((S, 2 * D), BF16),
        in_specs=[any_spec] * 10,
        out_specs=any_spec,
        scratch_shapes=[
            pltpu.VMEM((2, PP, 4, PW, D), BF16),
            pltpu.VMEM((NT, D // 2, 128), U32),
            pltpu.VMEM((NP, D // 2, 3 * PW), U32),
            pltpu.VMEM((hd // 2, D), U32),
            pltpu.VMEM((NSEG, NP, PRE, 3 * PW), F32),
            pltpu.VMEM((NG, GP * PRE, PW), F32),
            pltpu.VMEM((S, OUT_W), BF16),
            pltpu.VMEM((S, X_W), BF16),
            pltpu.VMEM((S, X_W), BF16),
            pltpu.VMEM((NSEG, PRE, D), BF16),
            pltpu.VMEM((NSEG * PRE // 2, D), U32),
            pltpu.VMEM((5, NSEG * PRE // 4, 256), U32),
            pltpu.VMEM((MEM, D), BF16),
            pltpu.VMEM((3, D // 2, D), U32),
            pltpu.VMEM((NTRIP, 2, 64, D), U32),
            pltpu.VMEM((D // 2, D), U32),
            pltpu.VMEM((PP, D // 2, 128), U32),
            pltpu.VMEM((NT, 2 * SEG, 128), F32),
            pltpu.VMEM((2, NT, KV_ROWS, 128), F32),
            pltpu.SemaphoreType.DMA((8,)),
        ],
        compiler_params=pltpu.CompilerParams(vmem_limit_bytes=120 * 1024 * 1024,
                                             disable_bounds_checks=True),
    )(A_x.reshape(S, D), A_wqkv, A_wo, B_x.reshape(S, D), B_x.reshape(NSEG, SEG // PRE, PRE, D),
      B_mem0.reshape(MEM, D), wq_t, wk_t, wv_t, wo)
    return out.reshape(1, S, 2 * D)
```

```python
import functools

import jax
import jax.numpy as jnp
from jax import lax
import jax.experimental.pallas as pl
import jax.experimental.pallas.tpu as pltpu

F32 = jnp.float32
BF16 = jnp.bfloat16
U32 = jnp.uint32

S = 2048
D = 640
NT = D // 128
A_H = 32
A_DH = D // A_H
A_W = 8
A_DIL = 2
A_HALO = 16
B_H = 32
B_DH = 192
MEM = 8
SEG = 32
NSEG = S // SEG
NP = B_H // 2
PW = 2 * B_DH
PRE = 8
FRESH = SEG - PRE
L = MEM + SEG
GP = 4
NG = NP // GP
LOG2E = 1.4426950408889634
NEG = -1000000000.0 * LOG2E
PP = 2
NTRIP = NP // PP - 1
PEEL = (2, 3, 4)
KH = 256
WO_HEAD = 384
WO_ROWS = 448
WX_TAIL = 3
WX_ROWS = 8
WX_SKIP = 1
ST_ROWS = 256
X_HEAD = 128
KV_ROWS = 80
X_W = 1024
OUT_W = 2048
SPT = 4
N_STEPS = NSEG // SPT
NQ = NP // 2

LAT_MM, LAT_X, LAT_T, LAT_N, LAT_N_LATE = 190, 190, 380, 230, 100
LATE_FROM = NP - 2
AP_AFTER = (6, 16, 26)
AO_AFTER = (30, 40)
TAIL_FILL = (2, 2, 2, 0)
HOLD_W = (0, 3, 0, 0)


def _segment_order(u):
    odd, last = u % 2 == 1, u == SPT - 1
    proj = []
    for g in range(NG):
        proj += [("K", GP * g + r) for r in range(GP)]
        for r in range(GP):
            proj += [("V", GP * g + r), ("Q", GP * g + r)]
    dur = {"K": 120, "V": 120, "Q": 120, "S": 24, "PV": 24, "PS": 24, "PPV": 24,
           "W": 120, "XA": 96, "XB": 192, "XC": 48, "Y": 96, "AO": 80, "AP": 125,
           "T": 0, "M": 0, "E": 0, "TG": 0, "MG": 0, "EG": 0}
    end = {}

    def ready(task):
        k, i = task
        if k == "T":
            deps = [(("K", i), LAT_MM)]
        elif k == "S":
            deps = [(("Q", i), LAT_MM), (("T", i), LAT_T)]
        elif k == "M":
            deps = [(("S", i), LAT_MM - 40)]
        elif k == "E":
            deps = [(("M", i), LAT_X)]
        elif k == "PV":
            deps = [(("E", i), LAT_N_LATE if i >= LATE_FROM else LAT_N), (("V", i), LAT_MM)]
        elif k == "TG":
            deps = [(("K", GP * i + r), LAT_MM) for r in range(GP)]
        elif k == "PS":
            deps = [(("TG", i), LAT_T)]
        elif k == "MG":
            deps = [(("PS", i), LAT_MM - 40)]
        elif k == "EG":
            deps = [(("MG", i), LAT_X)]
        elif k == "PPV":
            deps = [(("EG", i), LAT_N), (("V", GP * i + GP - 1), LAT_MM)]
        elif k == "W":
            deps = [(("PV", i), LAT_MM)]
        else:
            deps = [(("PV", 2 * i), LAT_MM), (("PPV", 2 * i // GP), LAT_MM)]
            if k != "XA":
                deps.append((("PV", 2 * i + 1), LAT_MM))
        if any(d not in end for d, _ in deps):
            return None
        return max(end[d] + lat for d, lat in deps)

    pend = ([(k, p) for k in ("E", "M", "T") for p in range(NP)]
            + [(k, g) for k in ("EG", "MG", "TG") for g in range(NG)]
            + ([(k, q) for q in range(NQ) for k in ("XA", "XB", "Y", "XC")] if last
               else [("W", p) for p in range(NP)])
            + [("PPV", g) for g in range(NG)]
            + [("PV", p) for p in range(NP)] + [("PS", g) for g in range(NG)]
            + [("S", p) for p in range(NP)])
    fill = [("AO", j) for j in range(NT)] if odd else [("AP", j) for j in (3, 4, 5, 0, 1, 2, 6, 7, 8)]
    order = []
    now = [0]

    def emit(task):
        order.append(task)
        now[0] += dur[task[0]]
        end[task] = now[0]

    nproj = 0
    while pend:
        cand = [x for x in pend if ready(x) is not None and ready(x) <= now[0]]
        if proj:
            cand = [x for x in cand if not (x[0] == "W" and x[1] >= NP - GP - HOLD_W[u])]
        if cand:
            if not proj:
                cand = [x for x in cand if x[0] not in ("W", "XA", "XB", "XC", "Y")] or cand
            pend.remove(cand[0])
            emit(cand[0])
        elif proj:
            emit(proj.pop(0))
            nproj += 1
            if odd and nproj == GP:
                order += [("LA", 0), ("LA", 1)]
            if nproj in (AO_AFTER if odd else AP_AFTER):
                emit(fill.pop(0))
        elif len(fill) > TAIL_FILL[u]:
            emit(fill.pop(0))
        else:
            now[0] = min(ready(x) for x in pend if ready(x) is not None)
    return order + fill


ORDERS = (
    "K0 K1 K2 T0 K3 T1 V0 T2 Q0 AP3 T3 TG0 V1 S0 Q1 M0 PS0 Q2 V2 V3 E0 MG0 S1 Q3 M1 S2 K4 EG0 PV0 "
    "K5 E1 M2 S3 K6 T4 W0 E2 M3 T5 PPV0 PV1 K7 AP4 E3 T6 W1 T7 TG1 PV2 PV3 Q4 W2 V4 W3 PS1 S4 V5 "
    "Q5 M4 MG1 V6 Q7 Q6 E4 EG1 S5 V7 M5 PV4 S6 K8 PPV1 E5 S7 M6 W4 K9 AP5 E6 M7 T8 PV5 K10 T9 K11 "
    "E7 W5 T10 PV6 V8 T11 TG2 PV7 Q8 W6 W7 PS2 S8 V10 V9 Q9 M8 MG2 Q10 E8 EG2 S9 V11 Q11 M9 PV8 "
    "S10 K12 PPV2 E9 S11 M10 W8 K13 E10 M11 T12 PV9 K14 K15 E11 T13 W9 PV10 V12 T14 T15 TG3 PV11 "
    "Q12 W10 W11 PS3 S12 Q13 V13 M12 MG3 V15 V14 E12 Q14 EG3 S13 Q15 M13 PV12 S14 AP0 PPV3 E13 "
    "S15 M14 W12 AP1 E14 PV13 M15 AP2 PV14 AP6 E15 W13 PV15 W14 W15 AP8 AP7 ",
    "K0 K1 K2 T0 K3 LA0 LA1 T1 V0 T2 Q0 T3 TG0 V1 Q1 S0 V2 PS0 Q2 M0 S1 V3 MG0 Q3 E0 M1 S2 K4 EG0 "
    "K5 E1 M2 PV0 S3 K6 T4 PPV0 E2 T5 K7 M3 W0 T6 PV1 PV2 V4 E3 T7 TG1 Q4 W1 W2 PV3 PS1 S4 V5 Q5 "
    "AO0 M4 MG1 W3 S5 V6 E4 EG1 Q6 M5 V7 PV4 Q7 E5 S6 K8 W4 M6 PPV1 PV5 S7 T8 K9 E6 K10 M7 W5 T9 "
    "PV6 K11 E7 T10 V8 W6 T11 TG2 PV7 Q8 AO1 W7 S8 V9 PS2 Q9 M8 V10 MG2 Q10 E8 S9 V11 EG2 Q11 M9 "
    "PV8 S10 K12 PPV2 E9 S11 M10 W8 K13 E10 M11 T12 PV9 K14 K15 AO2 E11 T13 T14 PV10 V12 T15 TG3 "
    "Q12 PV11 V13 Q13 PS3 S12 V14 Q14 M12 MG3 S13 V15 Q15 E12 M13 EG3 S14 W9 E13 M14 PPV3 W10 "
    "PV12 S15 W11 E14 M15 PV13 W12 PV14 E15 W13 PV15 W14 W15 AO3 AO4 ",
    "K0 K1 K2 T0 K3 T1 V0 Q0 AP3 TG0 T3 T2 V1 S0 Q1 V2 M0 PS0 Q2 S1 V3 E0 MG0 Q3 M1 S2 K4 EG0 PV0 "
    "K5 E1 M2 S3 K6 T4 W0 E2 M3 T5 PPV0 PV1 K7 AP4 E3 W1 T6 T7 TG1 PV2 V4 PV3 Q4 W2 W3 PS1 S4 V5 "
    "M4 Q5 MG1 V6 Q6 E4 EG1 S5 V7 Q7 M5 PV4 S6 K8 PPV1 E5 S7 M6 W4 K9 AP5 E6 M7 T8 PV5 K10 T9 K11 "
    "E7 W5 T10 PV6 V8 T11 TG2 PV7 Q8 W6 W7 S8 PS2 V9 Q9 M8 MG2 V10 Q10 E8 EG2 S9 V11 Q11 M9 PV8 "
    "S10 K12 PPV2 E9 S11 M10 W8 K13 E10 M11 T12 PV9 K14 K15 E11 T13 W9 PV11 T14 PV10 V12 T15 TG3 "
    "Q12 W10 W11 PS3 S12 MG3 V13 Q13 M12 V14 Q14 E12 EG3 S13 V15 Q15 M13 PV12 S14 AP0 PPV3 E13 "
    "S15 M14 W12 AP1 E14 M15 AP2 PV13 PV14 AP6 E15 W13 PV15 W14 W15 AP7 AP8 ",
    "K1 K0 K2 T0 K3 LA0 LA1 T1 V0 T2 Q0 T3 TG0 V1 Q1 S0 V2 PS0 Q2 M0 S1 V3 MG0 Q3 E0 M1 S2 K4 EG0 "
    "K5 E1 M2 T4 PV0 AO0 PPV0 S3 K6 E2 T5 K7 M3 XA0 T6 PV1 PV2 V4 E3 T7 TG1 Q4 XB0 Y0 XC0 XA1 PV3 "
    "PS1 S4 V5 Q5 M4 MG1 XB1 E4 EG1 Y1 XC1 S5 V6 PV4 Q6 M5 V7 S6 Q7 AO1 E5 PPV1 K8 S7 K9 M6 XA2 "
    "M7 T8 PV5 K10 E6 T9 K11 E7 XB2 T10 T11 TG2 Y2 XC2 PV6 PV7 V8 Q8 XA3 XB3 Y3 XC3 PS2 S8 V9 Q9 "
    "M8 MG2 V10 Q10 AO2 E8 EG2 S9 V11 S10 Q11 M9 PV8 K12 M10 PPV2 K13 E9 S11 K14 E10 T12 XA4 M11 "
    "T13 PV9 K15 T14 PV10 V12 E11 XB4 T15 TG3 Y4 XC4 XA5 PV11 Q12 AO3 XB5 Y5 PS3 XC5 S12 V13 Q13 "
    "M12 MG3 V14 Q14 E12 EG3 S13 V15 Q15 M13 PV12 S14 AO4 PPV3 E13 S15 M14 XA6 E14 M15 PV13 PV14 "
    "E15 XB6 PV15 Y6 XC6 XA7 XB7 Y7 XC7 ",
)
SKIP_PROLOGUE = False


def _order(u):
    if ORDERS is None or ORDERS[u] is None:
        return _segment_order(u)
    return [(t.rstrip("0123456789"), int(t.lstrip("ABCDEFGHIJKLMNOPQRSTUVWXYZ")))
            for t in ORDERS[u].split()]


def _nt_dot(a, b):
    return lax.dot_general(a, b, (((1,), (1,)), ((), ())), preferred_element_type=F32)


def _dot(a, b):
    return jnp.dot(a, b, preferred_element_type=F32)


def _pack(x):
    return pltpu.bitcast(x, U32)


def _unpack(x):
    return pltpu.bitcast(x, BF16)


def cat(parts):
    return jnp.concatenate(parts, axis=0)


def _recip(x):
    r = pl.reciprocal(x, approx=True)
    return r * (2.0 - x * r)


def _kernel(ax_hbm, awqkv_hbm, awo_hbm, bx_hbm, bx4_hbm, mem0_hbm, wq_hbm, wk_hbm, wv_hbm, wo_hbm,
            out_hbm,
            stage, awo_raw, w_s, wo_s, wx_s, pre_s, odef_s, out_s,
            xa_s, xb_s, xpre_s, xp_s, xs_s, mem0_s, wa_s, wc_s, awo_s, t1_s, qa_s, kv_s,
            sems):
    b_scale = B_DH ** (-0.5) * LOG2E
    a_scale = A_DH ** (-0.5) * LOG2E

    w_hbm = (wq_hbm, wk_hbm, wv_hbm)
    wo32 = wo_hbm.bitcast(U32)
    awo32 = awo_hbm.bitcast(U32)
    hw = PW // 2
    hd = B_H * B_DH

    def w_copy(p, half, q, m, sem):
        rows = pl.ds(pl.multiple_of(p * PW, PW), PW)
        return pltpu.make_async_copy(w_hbm[m].at[rows, :], stage.at[half, q, m], sem)

    def wa_piece(g, q):
        last = g >= 2 * 3
        return jnp.where(last, 1 + q, g >> 1), jnp.where(last, NT - 1, (g & 1) + 2 * q)

    def wa_copy(c, kt, half, q, sem):
        return pltpu.make_async_copy(
            awqkv_hbm.at[pl.ds(pl.multiple_of(kt * 128, 128), 128),
                         pl.ds(pl.multiple_of(c * D, 128), D)],
            stage.at[half, q, 3, :128], sem)

    def start_trip(g):
        half = g & 1
        src = jnp.minimum(g, NTRIP - 1)
        for q in range(PP):
            for m in range(3):
                w_copy((src + 1) * PP + q, half, q, m, sems.at[half]).start(priority=1)
            wa_copy(*wa_piece(src, q), half, q, sems.at[half]).start(priority=1)

    def wait_trip(half):
        for view in (stage.at[half, :, :3], stage.at[half, :, 3, :128]):
            pltpu.make_async_copy(view, view, sems.at[half]).wait()

    qr = 2 * hw

    def wo_copy(start, n, sem):
        wr = pl.ds(pl.multiple_of(start, 8), n)
        return pltpu.make_async_copy(wo32.at[wr, :], wo_s.at[wr, :], sem)

    def wo_sums(q, piece, anchor=None, never=None):
        def blk(k, n):
            w = wo_s[pl.ds(pl.multiple_of(q * qr + k * hw + piece * WX_ROWS, 8), WX_ROWS),
                     n * KH:(n + 1) * KH]
            if anchor is not None:
                w = jnp.where(never, anchor, w)
            return _unpack(w).astype(F32)

        b11, b12, b21, b22 = blk(0, 0), blk(0, 1), blk(1, 0), blk(1, 1)
        for n, v in enumerate((b11 + b22, b12 - b22, b21 - b11, b11 + b12, b21 + b22)):
            wx_s[q, n, pl.ds(pl.multiple_of(piece * WX_ROWS, 8), WX_ROWS), :] = (
                _pack(v.astype(BF16)))

    def x_copies(xr, sem):
        return [pltpu.make_async_copy(ax_hbm.at[xr, :], xa_s.at[xr, :D], sem),
                pltpu.make_async_copy(bx_hbm.at[xr, :], xb_s.at[xr, :D], sem)]

    xpre_cp = pltpu.make_async_copy(bx4_hbm.at[:, 0], xpre_s, sems.at[3])
    late_cps = [pltpu.make_async_copy(mem0_hbm, mem0_s, sems.at[2])] + [
        pltpu.make_async_copy(awo32.at[:, c * 128:(c + 1) * 128], awo_raw.at[c], sems.at[2])
        for c in range(NT)] + x_copies(pl.ds(0, X_HEAD), sems.at[2])
    wo_head = wo_copy(0, WO_HEAD, sems.at[9])
    x_rest = x_copies(pl.ds(X_HEAD, S - X_HEAD), sems.at[3])
    tiles = [(m, j) for m in range(3) for j in range(PW // 128)]
    peel = [tiles[sum(PEEL[:n]):sum(PEEL[:n + 1])] for n in range(len(PEEL))]
    peel_cps = [[pltpu.make_async_copy(w_hbm[m].at[pl.ds(q * PW + j * 128, 128), :],
                                       stage.at[1, q, m, pl.ds(j * 128, 128), :], sems.at[4 + n])
                 for m, j in blk for q in range(PP)] for n, blk in enumerate(peel)]
    peel_cps[-1].append(wa_copy(0, NT - 1, 1, 0, sems.at[3 + len(PEEL)]))

    xpre_cp.start()
    for cps in peel_cps:
        for cp in cps:
            cp.start(priority=1)
    start_trip(0)
    for cp in [wo_head] + late_cps:
        cp.start(priority=1)
    kv_s[:, :, :A_HALO, :] = jnp.zeros((2, NT, A_HALO, 128), F32)
    wo_s[NQ * qr:, :] = jnp.zeros((qr, D), U32)

    def gather_heads(ref):
        rows = []
        for j in range(A_DH // 2):
            u = ref[pl.ds(j, A_H, stride=A_DH // 2), :]
            rows.append(pltpu.bitcast(u << 16, F32))
            rows.append(pltpu.bitcast(u & jnp.uint32(0xFFFF0000), F32))
        return jnp.concatenate(rows, axis=0)

    HR = NSEG * PRE // 2

    def xq(i, k):
        return _unpack(xp_s[i * HR // 2:(i + 1) * HR // 2, k * KH:(k + 1) * KH])

    def strassen_lhs():
        f = lambda i, k: xq(i, k).astype(F32)
        sums = (f(0, 0) + f(1, 1), f(1, 0) + f(1, 1), f(0, 0) + f(0, 1),
                f(1, 0) - f(0, 0), f(0, 1) - f(1, 1))
        for n, v in enumerate(sums):
            xs_s[n] = _pack(v.astype(BF16))

    def pair_prep2(p, half, m, js=(0, 1, 2), hook=None):
        if SKIP_PROLOGUE:
            return
        for q in range(2):
            lo, hi = js[0] * 128, (js[-1] + 1) * 128
            w_s[p + q, :, m * PW + lo:m * PW + hi] = _pack(stage[half, q, m, lo:hi, :].T)
        nseg = ST_ROWS // PRE
        for j in js:
            rows = slice(j * 128, (j + 1) * 128)
            b = lambda k, q: stage[half, q, m, rows, k * KH:(k + 1) * KH]
            bf = lambda k, q: b(k, q).astype(F32)
            rhs = ((bf(0, 0) + bf(1, 1)).astype(BF16), b(0, 0),
                   (bf(0, 1) - bf(1, 1)).astype(BF16), (bf(1, 0) - bf(0, 0)).astype(BF16),
                   b(1, 1), (bf(0, 0) + bf(0, 1)).astype(BF16),
                   (bf(1, 0) + bf(1, 1)).astype(BF16))
            tail = [stage[half, q, m, rows, 2 * KH:] for q in range(2)]
            for c in range(HR // ST_ROWS):
                r = slice(c * ST_ROWS // 2, (c + 1) * ST_ROWS // 2)
                sm = lambda n: _unpack(xs_s[n, r, :])
                qd = lambda i, k: _unpack(
                    xp_s[(i * HR + c * ST_ROWS) // 2:(i * HR + (c + 1) * ST_ROWS) // 2,
                         k * KH:(k + 1) * KH])
                rest = lambda i: _unpack(
                    xp_s[(i * HR + c * ST_ROWS) // 2:(i * HR + (c + 1) * ST_ROWS) // 2, 2 * KH:])

                def put(i, q, v):
                    s0 = i * (NSEG // 2) + c * nseg
                    pre_s[s0:s0 + nseg, p + q, :, m * PW + j * 128:m * PW + (j + 1) * 128] = (
                        v.reshape(nseg, PRE, 128))
                    if hook is not None:
                        hook(v)

                m5 = _nt_dot(sm(2), rhs[4])
                m3 = _nt_dot(qd(0, 0), rhs[2])
                put(0, 1, _nt_dot(rest(0), tail[1]) + m3 + m5)
                m1 = _nt_dot(sm(0), rhs[0])
                m4 = _nt_dot(qd(1, 1), rhs[3])
                put(0, 0, _nt_dot(rest(0), tail[0]) + _nt_dot(sm(4), rhs[6]) + (m1 + m4 - m5))
                m2 = _nt_dot(sm(1), rhs[1])
                put(1, 0, _nt_dot(rest(1), tail[0]) + m2 + m4)
                put(1, 1, _nt_dot(rest(1), tail[1]) + _nt_dot(sm(3), rhs[5]) + (m1 - m2 + m3))

    def wa_prep(c, kt, half, q):
        t1_s[q] = _pack(stage[half, q, 3, :128].T)
        g = gather_heads(t1_s.at[q])
        wa_s[c, pl.ds(pl.multiple_of(kt * 64, 64), 64), :] = _pack(g.astype(BF16).T)
        return g

    def wa_trip(g, half):
        lo, hi = [wa_prep(*wa_piece(g, q), half, q) for q in range(2)]
        for t in range(2):
            b11, b12 = lo[2 * t * 128:(2 * t + 1) * 128], lo[(2 * t + 1) * 128:(2 * t + 2) * 128]
            b21, b22 = hi[2 * t * 128:(2 * t + 1) * 128], hi[(2 * t + 1) * 128:(2 * t + 2) * 128]
            sums = cat([b11 + b22, b12 - b22, b21 - b11, b11 + b12, b21 + b22])
            wc_s[g, t] = _pack(sums.astype(BF16).T)

    xpre_cp.wait()
    xp_s[...] = _pack(xpre_s[...].reshape(NSEG * PRE, D))
    strassen_lhs()
    for blk, cps in zip(peel, peel_cps):
        for cp in cps:
            cp.wait()
        for m in range(3):
            js = tuple(j for mm, j in blk if mm == m)
            if js:
                pair_prep2(0, 1, m, js)
    wa_prep(0, NT - 1, 1, 0)

    def prologue(g, carry):
        half = g & 1

        @pl.when(g > 0)
        def _():
            wo_copy(WO_HEAD + (g - 1) * WO_ROWS, WO_ROWS, sems.at[8]).wait()

        @pl.when(g == 1)
        def _():
            wo_head.wait()

        @pl.when(g < NTRIP - 1)
        def _():
            wo_copy(WO_HEAD + g * WO_ROWS, WO_ROWS, sems.at[8]).start()

        start_trip(g + 1)
        wait_trip(half)
        calls = [0]
        per = hw // WX_ROWS
        todo = list(range(NQ * per // (NTRIP - 1)))
        total = len(todo)

        def hook(v):
            calls[0] += 1
            want = (calls[0] - WX_SKIP) * total // (36 - WX_SKIP - WX_TAIL)
            t = 0
            while todo and todo[0] < want:
                k = jnp.where(g > 0, (g - 1) * total, NQ * per) + todo.pop(0)
                q = jnp.minimum(k // per, NQ)
                anchor = jnp.concatenate(
                    [v[(2 * t + c) * WX_ROWS:(2 * t + c + 1) * WX_ROWS] for c in range(2)], axis=1)
                wo_sums(q, k % per, pltpu.bitcast(anchor, U32), g > NSEG)
                t += 1

        for m in range(3):
            pair_prep2((g + 1) * PP, half, m, hook=hook)
            if m == 0:
                wa_trip(g, half)
        return carry

    lax.fori_loop(0, NTRIP, prologue, 0)

    for cp in late_cps:
        cp.wait()
    for cp in x_rest:
        cp.start()

    for c in range(NT):
        awo_s[:, c * 128:(c + 1) * 128] = _pack(gather_heads(awo_raw.at[c]).astype(BF16))

    def out_copy(row, n, half):
        r = pl.ds(row, n)
        c = slice(half * D, (half + 1) * D)
        return pltpu.make_async_copy(out_s.at[r, c], out_hbm.at[r, c], sems.at[7])

    def segment(s, mem, u):
        last = u == SPT - 1
        row0 = pl.multiple_of(s * SEG, SEG)
        ninf = jnp.float32(-jnp.inf)

        qi = lax.broadcasted_iota(jnp.int32, (SEG, 2 * L), 0)
        kl = lax.broadcasted_iota(jnp.int32, (SEG, 2 * L), 1)
        is_a = kl < L
        is_b = kl >= L
        kpos = jnp.where(is_a, kl, kl - L)
        allowed = (qi >= FRESH) | (qi + MEM + PRE >= kpos)
        pi = lax.broadcasted_iota(jnp.int32, (GP * PRE, 128), 0)
        pk = lax.broadcasted_iota(jnp.int32, (GP * PRE, 128), 1)
        p_own = (pk // SEG) == (pi // PRE)
        p_allowed = (pk % (MEM + PRE)) <= (pi % PRE) + MEM
        p_first = (pk % SEG) < MEM + PRE
        p_is_a = p_own & p_first
        p_is_b = p_own & jnp.logical_not(p_first)
        col_a = lax.broadcasted_iota(jnp.int32, (1, PW), 1) < B_DH
        col128_a = lax.broadcasted_iota(jnp.int32, (1, 128), 1) < (B_DH - 128)

        xb = xb_s[pl.ds(row0, SEG), :D].astype(F32)
        h = jnp.concatenate([xb[PRE:], mem], axis=0).astype(BF16)

        def proj(p, m):
            return _dot(h, _unpack(w_s[p, :, m * PW:(m + 1) * PW]))

        def pre(p, m):
            return pre_s[s, p, :, m * PW:(m + 1) * PW]

        def block_diag(p, m):
            f = proj(p, m)
            full = jnp.concatenate([f[FRESH:], pre(p, m), f[:FRESH]], axis=0)
            z = jnp.zeros_like(full)
            return jnp.where(col_a, full, z), jnp.where(col_a, z, full)

        def keys_t(blocks):
            fold = cat([jnp.concatenate([x[:, :128] if i % 2 == 0 else x[:, 256:], x[:, 128:256]],
                                        axis=1) for i, x in enumerate(blocks)])
            t = fold.T
            outer = t[:128]
            n = blocks[0].shape[0]
            lane = lax.broadcasted_iota(jnp.int32, outer.shape, 1)
            lane_a = lane < n if len(blocks) == 2 else lane % (2 * n) < n
            z = jnp.zeros_like(outer)
            kt = cat([jnp.where(lane_a, outer, z), t[128:], jnp.where(lane_a, z, outer)])
            return kt.astype(BF16)

        def row_max(raw, ok, in_a, in_b):
            sc = jnp.where(ok, raw * b_scale, NEG)
            ma = jnp.max(jnp.where(in_a, sc, ninf), axis=1, keepdims=True)
            mb = jnp.max(jnp.where(in_b, sc, ninf), axis=1, keepdims=True)
            return sc, ma, mb

        def probs(mx, first, own, late_norm):
            sc, ma, mb = mx
            e = jnp.exp2(sc - jnp.where(first, ma, mb))
            if own is not None:
                e = jnp.where(own, e, 0.0)
            sa = jnp.sum(jnp.where(first, e, 0.0), axis=1, keepdims=True)
            sb = jnp.sum(jnp.where(first, 0.0, e), axis=1, keepdims=True)
            if late_norm:
                return e.astype(BF16), _recip(sa), _recip(sb)
            return (e * _recip(jnp.where(first, sa, sb))).astype(BF16), None, None

        def pv(sm, vbd):
            e, ra, rb = sm
            o = _dot(e, cat(vbd).astype(BF16))
            if ra is not None:
                o = jnp.concatenate([
                    o[:, :128] * ra,
                    o[:, 128:256] * jnp.where(col128_a, ra, rb),
                    o[:, 256:] * rb], axis=1)
            return o

        def pre_pv(g, pr, vbds):
            v = cat([x[:MEM + PRE] for vb in vbds for x in vb])
            o = _dot(pr, v.astype(BF16))
            if not last:
                odef_s[u, g] = o
            return o

        def wout(p, o, acc):
            contrib = _dot(o.astype(BF16), _unpack(wo_s[p * hw:(p + 1) * hw, :]))
            return contrib if acc is None else acc + contrib

        def deferred(p):
            r = slice((p % GP) * PRE, (p % GP + 1) * PRE)
            return cat([odef_s[v, p // GP, r, :] for v in range(SPT - 1)]
                       + [val["PPV", p // GP][r]])

        def wout_strassen(kind, q):
            a11, a21 = val["PV", 2 * q], deferred(2 * q)
            if kind != "XA":
                a12, a22 = val["PV", 2 * q + 1], deferred(2 * q + 1)
            blk = lambda k, n: _unpack(
                wo_s[q * qr + k * hw:q * qr + (k + 1) * hw, n * KH:(n + 1) * KH])
            sm = lambda n: _unpack(wx_s[q, n])
            if kind == "XA":
                terms = {3: (a11, sm(1)), 6: (a21 - a11, sm(3))}
            elif kind == "XB":
                terms = {1: (a11 + a22, sm(0)), 4: (a22, sm(2)), 5: (a11 + a12, blk(1, 1)),
                         7: (a12 - a22, sm(4))}
            elif kind == "XC":
                terms = {2: (a21 + a22, blk(0, 0))}
            else:
                lhs = jnp.concatenate([cat([a11, a21]), cat([a12, a22])], axis=1)
                terms = {0: (lhs, _unpack(wo_s[q * qr:(q + 1) * qr, 2 * KH:]))}
            for n, (x, w) in terms.items():
                r = _dot(x.astype(BF16), w)
                val["acc", n] = val["acc", n] + r if ("acc", n) in val else r

        arow0 = pl.multiple_of((s - u % 2) * SEG, 2 * SEG)

        def a_put(m, j, r):
            if m == 0:
                qa_s[j] = r * a_scale
            else:
                kv_s[m - 1, j, A_HALO:A_HALO + 2 * SEG, :] = r

        def a_proj(idx):
            m, t = divmod(idx, 3)
            if "xa" not in val:
                xa = xa_s[pl.ds(arow0, 2 * SEG), :D]
                xf = xa.astype(F32)
                f = lambda i, k: xf[i * SEG:(i + 1) * SEG, k * KH:(k + 1) * KH]
                val["xa"] = xa
                val["xs"] = [v.astype(BF16) for v in (
                    f(0, 0) + f(1, 1), f(1, 0) + f(1, 1), f(0, 0), f(1, 1), f(0, 0) + f(0, 1),
                    f(1, 0) - f(0, 0), f(0, 1) - f(1, 1))]
                val["xr"] = xf[:, 2 * KH:].astype(BF16)
            if t == 2:
                a_put(m, NT - 1, _dot(val["xa"], _unpack(wa_s[m, :, (NT - 1) * 128:])))
                return
            sm = lambda n: _unpack(cat([wc_s[2 * m + k, t, :, n * 128:(n + 1) * 128]
                                        for k in range(2)]))
            blk = lambda k, j: _unpack(wa_s[m, k * KH // 2:(k + 1) * KH // 2,
                                            (2 * t + j) * 128:(2 * t + j + 1) * 128])
            rhs = (sm(0), blk(0, 0), sm(1), sm(2), blk(1, 1), sm(3), sm(4))
            mm = lambda n: _dot(val["xs"][n], rhs[n])
            tail = [_dot(val["xr"], _unpack(wa_s[m, KH:, (2 * t + j) * 128:(2 * t + j + 1) * 128]))
                    for j in range(2)]
            m1, m2, m3, m4, m5 = [mm(n) for n in range(5)]
            a_put(m, 2 * t, tail[0] + cat([mm(6) + (m1 + m4 - m5), m2 + m4]))
            a_put(m, 2 * t + 1, tail[1] + cat([m3 + m5, mm(5) + (m1 - m2 + m3)]))

        def window(m, j, w, hf):
            lo = A_HALO + hf * SEG - A_DIL * w
            return kv_s[m, j, lo:lo + SEG, :]

        def local_softmax(hf):
            pos = arow0 + hf * SEG + lax.broadcasted_iota(jnp.int32, (SEG, 128), 0)
            rows = slice(hf * SEG, (hf + 1) * SEG)
            logits = []
            for w in range(A_W):
                t = qa_s[0, rows, :] * window(0, 0, w, hf)
                for j in range(1, NT):
                    t = t + qa_s[j, rows, :] * window(0, j, w, hf)
                t = t + pltpu.roll(t, 64, 1)
                t = t + pltpu.roll(t, 32, 1)
                if w > 0 and hf == 0:
                    t = jnp.where(pos >= A_DIL * w, t, NEG)
                logits.append(t)
            mx = functools.reduce(jnp.maximum, logits)
            es = [jnp.exp2(l - mx) for l in logits]
            inv = _recip(functools.reduce(lambda x, y: x + y, es))
            return es, inv

        def local_pv(j, hf):
            es, inv = val["LA", hf]
            o = es[0] * window(1, j, 0, hf)
            for w in range(1, A_W):
                o = o + es[w] * window(1, j, w, hf)
            return o * inv

        def local_out(j, acc):
            wj = _unpack(awo_s[j * 64:(j + 1) * 64, :])
            if ("AX", j) in val:
                r = cat([val["AX", j], _dot(local_pv(j, 1).astype(BF16), wj)])
            else:
                r = _dot(cat([local_pv(j, 0), local_pv(j, 1)]).astype(BF16), wj)
            for m in range(2):
                kv_s[m, j, :A_HALO, :] = kv_s[m, j, 2 * SEG:2 * SEG + A_HALO, :]
            return r if acc is None else acc + r

        val = {}
        acc = None
        oa = None
        for kind, t in _order(u):
            if kind == "K":
                val[kind, t] = block_diag(t, 1)
            elif kind == "V":
                val[kind, t] = block_diag(t, 2)
            elif kind == "Q":
                val[kind, t] = proj(t, 0).astype(BF16)
            elif kind == "T":
                val[kind, t] = keys_t(val["K", t])
            elif kind == "S":
                val[kind, t] = _dot(val["Q", t], val["T", t])
            elif kind == "M":
                val[kind, t] = row_max(val["S", t], allowed, is_a, is_b)
            elif kind == "E":
                val[kind, t] = probs(val["M", t], is_a, None, t >= LATE_FROM)
            elif kind == "PV":
                val[kind, t] = pv(val["E", t], val["V", t])
            elif kind == "TG":
                val[kind, t] = keys_t([x[:MEM + PRE] for r in range(GP)
                                       for x in val["K", GP * t + r]])
            elif kind == "PS":
                q = cat([pre(GP * t + r, 0) for r in range(GP)]).astype(BF16)
                val[kind, t] = _dot(q, val["TG", t])
            elif kind == "MG":
                val[kind, t] = row_max(val["PS", t], p_allowed, p_is_a, p_is_b)
            elif kind == "EG":
                val[kind, t] = probs(val["MG", t], p_first, p_own, False)[0]
            elif kind == "PPV":
                val[kind, t] = pre_pv(t, val["EG", t], [val["V", GP * t + r] for r in range(GP)])
            elif kind == "W":
                acc = wout(t, val["PV", t], acc)
            elif kind in ("XA", "XB", "XC", "Y"):
                wout_strassen(kind, t)
            elif kind == "LA":
                val[kind, t] = local_softmax(t)
            elif kind == "AP":
                a_proj(t)
            elif kind == "AX":
                val[kind, t] = _dot(local_pv(t, 0).astype(BF16),
                                    _unpack(awo_s[t * 64:(t + 1) * 64, :]))
            elif kind == "AO":
                oa = local_out(t, oa)
                if t == NT - 1:
                    out_s[pl.ds(arow0, 2 * SEG), :D] = oa.astype(BF16)
                    out_copy(arow0, 2 * SEG, 0).start()
        if last:
            m = lambda n: val["acc", n]
            acc = jnp.concatenate([
                cat([m(1) + m(4) - m(5) + m(7), m(2) + m(4)]),
                cat([m(3) + m(5), m(1) - m(2) + m(3) + m(6)]), m(0)], axis=1)
        return acc

    def steps(i, mem):
        @pl.when(i == 1)
        def _():
            for cp in x_rest:
                cp.wait()

        accs = []
        for u in range(SPT):
            accs.append(segment(i * SPT + u, mem, u))
            mem = accs[-1][FRESH:SEG]
        res = cat([x for u in range(SPT) for x in (
            accs[-1][SEG + u * PRE:SEG + (u + 1) * PRE], accs[u][:FRESH])])
        row = pl.multiple_of(i * SPT * SEG, SPT * SEG)
        out_s[pl.ds(row, SPT * SEG), D:2 * D] = res.astype(BF16)
        out_copy(row, SPT * SEG, 1).start()
        return mem

    lax.fori_loop(0, N_STEPS, steps, mem0_s[...].astype(F32))

    wait_trip(NTRIP % 2)

    done = N_STEPS * SPT * SEG
    pltpu.make_async_copy(out_s.at[:done, :2 * D], out_hbm.at[:done, :], sems.at[7]).wait()


@jax.jit
def pallas_concat_heads__sliding_local_dilated__memory_aug_recurrent_mem_tr__prompt_kernel(
    A_x: jax.Array,
    A_wqkv: jax.Array,
    A_wo: jax.Array,
    B_x: jax.Array,
    B_mem0: jax.Array,
    B_Wq: jax.Array,
    B_Wk: jax.Array,
    B_Wv: jax.Array,
    B_Wo: jax.Array,
    B_seg_len,
):
    del B_seg_len
    assert A_x.shape == (1, S, D) and B_x.shape == (1, S, D)
    hd = B_H * B_DH
    wq_t = jnp.transpose(B_Wq, (1, 2, 0)).reshape(hd, D)
    wk_t = jnp.transpose(B_Wk, (1, 2, 0)).reshape(hd, D)
    wv_t = jnp.transpose(B_Wv, (1, 2, 0)).reshape(hd, D)
    wo = B_Wo.reshape(hd, D)

    any_spec = pl.BlockSpec(memory_space=pl.ANY)
    out = pl.pallas_call(
        _kernel,
        out_shape=jax.ShapeDtypeStruct((S, 2 * D), BF16),
        in_specs=[any_spec] * 10,
        out_specs=any_spec,
        scratch_shapes=[
            pltpu.VMEM((2, PP, 4, PW, D), BF16),
            pltpu.VMEM((NT, D // 2, 128), U32),
            pltpu.VMEM((NP, D // 2, 3 * PW), U32),
            pltpu.VMEM((hd // 2 + PW, D), U32),
            pltpu.VMEM((NQ + 1, 5, PW // 2, KH), U32),
            pltpu.VMEM((NSEG, NP, PRE, 3 * PW), F32),
            pltpu.VMEM((SPT - 1, NG, GP * PRE, PW), F32),
            pltpu.VMEM((S, OUT_W), BF16),
            pltpu.VMEM((S, X_W), BF16),
            pltpu.VMEM((S, X_W), BF16),
            pltpu.VMEM((NSEG, PRE, D), BF16),
            pltpu.VMEM((NSEG * PRE // 2, D), U32),
            pltpu.VMEM((5, NSEG * PRE // 4, 256), U32),
            pltpu.VMEM((MEM, D), BF16),
            pltpu.VMEM((3, D // 2, D), U32),
            pltpu.VMEM((NTRIP, 2, 64, D), U32),
            pltpu.VMEM((D // 2, D), U32),
            pltpu.VMEM((PP, D // 2, 128), U32),
            pltpu.VMEM((NT, 2 * SEG, 128), F32),
            pltpu.VMEM((2, NT, KV_ROWS, 128), F32),
            pltpu.SemaphoreType.DMA((10,)),
        ],
        compiler_params=pltpu.CompilerParams(vmem_limit_bytes=120 * 1024 * 1024,
                                             disable_bounds_checks=True),
    )(A_x.reshape(S, D), A_wqkv, A_wo, B_x.reshape(S, D), B_x.reshape(NSEG, SEG // PRE, PRE, D),
      B_mem0.reshape(MEM, D), wq_t, wk_t, wv_t, wo)
    return out.reshape(1, S, 2 * D)
```

```python
import functools

import jax
import jax.numpy as jnp
from jax import lax
import jax.experimental.pallas as pl
import jax.experimental.pallas.tpu as pltpu

F32 = jnp.float32
BF16 = jnp.bfloat16
U32 = jnp.uint32

S = 2048
D = 640
NT = D // 128
A_H = 32
A_DH = D // A_H
A_W = 8
A_DIL = 2
A_HALO = 16
B_H = 32
B_DH = 192
MEM = 8
SEG = 32
NSEG = S // SEG
NP = B_H // 2
PW = 2 * B_DH
PRE = 8
FRESH = SEG - PRE
L = MEM + SEG
GP = 4
NG = NP // GP
LOG2E = 1.4426950408889634
NEG = -1000000000.0 * LOG2E
PP = 2
NTRIP = NP // PP - 1
PEEL = (2, 2, 5)
KH = 256
WO_ROWS = 512
WX_DONE = (0, 24, 56, 96, 120, 152, 192)
WX_TAIL = 2
WX_ROWS = 8
WX_SKIP = 0
ST_ROWS = 256
X_HEAD = 128
KV_ROWS = 80
X_W = 1024
OUT_W = 2048
SPT = 4
N_STEPS = NSEG // SPT
NQ = NP // 2

LAT_MM, LAT_X, LAT_T, LAT_N, LAT_N_LATE = 190, 190, 380, 230, 100
LATE_FROM = NP - 2
AP_AFTER = (6, 16, 26)
AO_AFTER = (30, 40)
TAIL_FILL = (2, 2, 2, 0)
HOLD_W = (0, 3, 0, 0)


def _segment_order(u):
    odd, last = u % 2 == 1, u == SPT - 1
    proj = []
    for g in range(NG):
        proj += [("K", GP * g + r) for r in range(GP)]
        for r in range(GP):
            proj += [("V", GP * g + r), ("Q", GP * g + r)]
    dur = {"K": 120, "V": 120, "Q": 120, "S": 24, "PV": 24, "PS": 24, "PPV": 24,
           "W": 120, "XA": 96, "XB": 192, "XC": 48, "Y": 96, "AO": 80, "AP": 125,
           "T": 0, "M": 0, "E": 0, "TG": 0, "MG": 0, "EG": 0}
    end = {}

    def ready(task):
        k, i = task
        if k == "T":
            deps = [(("K", i), LAT_MM)]
        elif k == "S":
            deps = [(("Q", i), LAT_MM), (("T", i), LAT_T)]
        elif k == "M":
            deps = [(("S", i), LAT_MM - 40)]
        elif k == "E":
            deps = [(("M", i), LAT_X)]
        elif k == "PV":
            deps = [(("E", i), LAT_N_LATE if i >= LATE_FROM else LAT_N), (("V", i), LAT_MM)]
        elif k == "TG":
            deps = [(("K", GP * i + r), LAT_MM) for r in range(GP)]
        elif k == "PS":
            deps = [(("TG", i), LAT_T)]
        elif k == "MG":
            deps = [(("PS", i), LAT_MM - 40)]
        elif k == "EG":
            deps = [(("MG", i), LAT_X)]
        elif k == "PPV":
            deps = [(("EG", i), LAT_N), (("V", GP * i + GP - 1), LAT_MM)]
        elif k == "W":
            deps = [(("PV", i), LAT_MM)]
        else:
            deps = [(("PV", 2 * i), LAT_MM), (("PPV", 2 * i // GP), LAT_MM)]
            if k != "XA":
                deps.append((("PV", 2 * i + 1), LAT_MM))
        if any(d not in end for d, _ in deps):
            return None
        return max(end[d] + lat for d, lat in deps)

    pend = ([(k, p) for k in ("E", "M", "T") for p in range(NP)]
            + [(k, g) for k in ("EG", "MG", "TG") for g in range(NG)]
            + ([(k, q) for q in range(NQ) for k in ("XA", "XB", "Y", "XC")] if last
               else [("W", p) for p in range(NP)])
            + [("PPV", g) for g in range(NG)]
            + [("PV", p) for p in range(NP)] + [("PS", g) for g in range(NG)]
            + [("S", p) for p in range(NP)])
    fill = [("AO", j) for j in range(NT)] if odd else [("AP", j) for j in (3, 4, 5, 0, 1, 2, 6, 7, 8)]
    order = []
    now = [0]

    def emit(task):
        order.append(task)
        now[0] += dur[task[0]]
        end[task] = now[0]

    nproj = 0
    while pend:
        cand = [x for x in pend if ready(x) is not None and ready(x) <= now[0]]
        if proj:
            cand = [x for x in cand if not (x[0] == "W" and x[1] >= NP - GP - HOLD_W[u])]
        if cand:
            if not proj:
                cand = [x for x in cand if x[0] not in ("W", "XA", "XB", "XC", "Y")] or cand
            pend.remove(cand[0])
            emit(cand[0])
        elif proj:
            emit(proj.pop(0))
            nproj += 1
            if odd and nproj == GP:
                order += [("LA", 0), ("LA", 1)]
            if nproj in (AO_AFTER if odd else AP_AFTER):
                emit(fill.pop(0))
        elif len(fill) > TAIL_FILL[u]:
            emit(fill.pop(0))
        else:
            now[0] = min(ready(x) for x in pend if ready(x) is not None)
    return order + fill


ORDERS = (
    "K0 K1 K2 T0 K3 T1 V0 T2 Q0 AP3 T3 TG0 V1 S0 Q1 M0 PS0 Q2 V2 V3 E0 MG0 S1 S2 Q3 M1 K4 EG0 PV0 "
    "K5 E1 M2 S3 K6 T4 W0 E2 M3 T5 PPV0 PV1 K7 AP4 E3 T6 W1 T7 TG1 PV2 PV3 Q4 W2 V4 W3 PS1 S4 V5 "
    "Q5 M4 MG1 V6 Q7 Q6 E4 EG1 S5 V7 M5 PV4 S6 K8 PPV1 E5 S7 M6 W4 K9 AP5 E6 M7 T8 K10 PV5 T9 K11 "
    "E7 W5 T10 PV6 V8 T11 TG2 PV7 Q8 W6 W7 PS2 S8 V10 V9 Q9 M8 MG2 Q10 E8 EG2 V11 S9 Q11 M9 PV8 "
    "S10 K12 PPV2 E9 S11 M10 W8 K13 E10 M11 T12 PV9 K14 K15 E11 T13 W9 PV10 V12 T14 T15 TG3 PV11 "
    "Q12 W10 W11 PS3 S12 Q13 V13 M12 MG3 V15 V14 E12 Q14 EG3 Q15 S13 M13 PV12 S14 AP0 PPV3 E13 "
    "S15 M14 W12 AP1 E14 PV13 M15 AP2 PV14 AP6 E15 W13 PV15 W14 W15 AP8 AP7 ",
    "K0 K1 K2 T0 K3 LA0 LA1 T1 V0 T2 Q0 T3 TG0 V1 Q1 S0 V2 PS0 Q2 M0 S1 V3 MG0 Q3 E0 M1 S2 K4 EG0 "
    "K5 E1 M2 PV0 S3 K6 T4 PPV0 E2 T5 K7 M3 W0 T6 PV1 PV2 V4 E3 T7 TG1 Q4 W1 W2 PV3 PS1 S4 V5 Q5 "
    "AO0 M4 MG1 W3 S5 V6 E4 EG1 Q6 M5 V7 PV4 Q7 E5 S6 K8 W4 M6 PPV1 PV5 S7 T8 K9 E6 K10 M7 W5 T9 "
    "PV6 K11 E7 T10 V8 W6 T11 TG2 PV7 Q8 AO1 W7 S8 V9 PS2 Q9 M8 V10 MG2 Q10 E8 S9 V11 EG2 Q11 M9 "
    "PV8 S10 K12 PPV2 E9 S11 M10 W8 K13 E10 M11 T12 PV9 K14 K15 E11 T13 T14 PV10 AO2 V12 T15 TG3 "
    "Q12 PV11 V13 Q13 PS3 S12 V14 Q14 M12 MG3 S13 V15 Q15 E12 M13 EG3 S14 W9 E13 M14 PPV3 W10 "
    "PV12 S15 W11 E14 M15 PV13 W12 PV14 E15 W13 PV15 W14 W15 AO3 AO4 ",
    "K0 K1 K2 T0 K3 T1 V0 Q0 AP3 TG0 T3 T2 V1 S0 Q1 Q2 V2 M0 PS0 S1 V3 E0 MG0 Q3 M1 S2 K4 EG0 PV0 "
    "K5 E1 M2 S3 K6 T4 W0 E2 M3 T5 PPV0 PV1 K7 AP4 E3 W1 T6 T7 TG1 PV2 V4 PV3 Q4 W2 W3 PS1 S4 V5 "
    "M4 Q5 MG1 V6 Q6 EG1 S5 E4 V7 Q7 M5 PV4 S6 K8 PPV1 E5 S7 M6 W4 K9 AP5 E6 M7 T8 PV5 K10 T9 K11 "
    "E7 W5 T10 PV6 V8 T11 TG2 PV7 Q8 W6 W7 S8 PS2 V9 Q9 M8 MG2 V10 Q10 E8 EG2 S9 V11 Q11 M9 PV8 "
    "S10 K12 PPV2 E9 S11 M10 W8 K13 E10 M11 T12 PV9 K14 K15 E11 T13 W9 PV11 T14 PV10 V12 T15 TG3 "
    "Q12 W10 W11 PS3 S12 MG3 V13 Q13 M12 V14 Q14 E12 EG3 S13 V15 Q15 M13 PV12 S14 AP0 PPV3 E13 "
    "S15 M14 W12 AP1 E14 M15 AP2 PV13 PV14 AP6 E15 W13 PV15 W14 W15 AP7 AP8 ",
    "K1 K0 K2 T0 K3 LA0 LA1 T1 V0 T2 Q0 T3 TG0 V1 Q1 S0 V2 PS0 Q2 M0 V3 MG0 Q3 S1 E0 M1 S2 K4 EG0 "
    "K5 E1 M2 T4 PV0 AO0 PPV0 S3 K6 E2 T5 K7 M3 XA0 T6 PV1 PV2 V4 E3 T7 TG1 XB0 Y0 Q4 XC0 XA1 PV3 "
    "PS1 S4 V5 Q5 M4 MG1 XB1 E4 EG1 Y1 XC1 S5 V6 PV4 Q6 M5 V7 S6 Q7 AO1 E5 PPV1 K8 S7 K9 M6 XA2 "
    "M7 T8 PV5 K10 E6 T9 XB2 K11 E7 T10 T11 TG2 Y2 XC2 PV6 PV7 V8 Q8 XA3 XB3 Y3 XC3 PS2 S8 V9 Q9 "
    "M8 MG2 V10 Q10 AO2 E8 EG2 S9 V11 S10 Q11 M9 PV8 K12 M10 PPV2 K13 E9 S11 K14 E10 T12 XA4 M11 "
    "T13 PV9 K15 T14 PV10 V12 E11 XB4 T15 TG3 Y4 XC4 XA5 PV11 Q12 AO3 XB5 Y5 PS3 XC5 S12 V13 Q13 "
    "M12 MG3 V14 Q14 E12 EG3 S13 V15 Q15 M13 PV12 S14 AO4 PPV3 E13 S15 M14 E14 XA6 M15 PV13 PV14 "
    "E15 XB6 PV15 Y6 XC6 XA7 XB7 Y7 XC7 ",
)
SKIP_PROLOGUE = False


def _order(u):
    if ORDERS is None or ORDERS[u] is None:
        return _segment_order(u)
    return [(t.rstrip("0123456789"), int(t.lstrip("ABCDEFGHIJKLMNOPQRSTUVWXYZ")))
            for t in ORDERS[u].split()]


def _nt_dot(a, b):
    return lax.dot_general(a, b, (((1,), (1,)), ((), ())), preferred_element_type=F32)


def _dot(a, b):
    return jnp.dot(a, b, preferred_element_type=F32)


def _pack(x):
    return pltpu.bitcast(x, U32)


def _unpack(x):
    return pltpu.bitcast(x, BF16)


def cat(parts):
    return jnp.concatenate(parts, axis=0)


def _recip(x):
    r = pl.reciprocal(x, approx=True)
    return r * (2.0 - x * r)


def _kernel(ax_hbm, awqkv_hbm, awo_hbm, bx_hbm, bx4_hbm, mem0_hbm, wq_hbm, wk_hbm, wv_hbm, wo_hbm,
            out_hbm,
            stage, awo_raw, w_s, wo_s, wx_s, pre_s, odef_s, out_s,
            xa_s, xb_s, xpre_s, xp_s, xs_s, mem0_s, wa_s, wc_s, awo_s, t1_s, qa_s, kv_s,
            sems):
    b_scale = B_DH ** (-0.5) * LOG2E
    a_scale = A_DH ** (-0.5) * LOG2E

    w_hbm = (wq_hbm, wk_hbm, wv_hbm)
    wo32 = wo_hbm.bitcast(U32)
    awo32 = awo_hbm.bitcast(U32)
    hw = PW // 2
    hd = B_H * B_DH

    def w_copy(p, half, q, m, sem):
        rows = pl.ds(pl.multiple_of(p * PW, PW), PW)
        return pltpu.make_async_copy(w_hbm[m].at[rows, :], stage.at[half, q, m], sem)

    def wa_piece(g, q):
        last = g >= 2 * 3
        return jnp.where(last, 1 + q, g >> 1), jnp.where(last, NT - 1, (g & 1) + 2 * q)

    def wa_copy(c, kt, half, q, sem):
        return pltpu.make_async_copy(
            awqkv_hbm.at[pl.ds(pl.multiple_of(kt * 128, 128), 128),
                         pl.ds(pl.multiple_of(c * D, 128), D)],
            stage.at[half, q, 3, :128], sem)

    def start_trip(g):
        half = g & 1
        src = jnp.minimum(g, NTRIP - 1)
        for q in range(PP):
            for m in range(3):
                w_copy((src + 1) * PP + q, half, q, m, sems.at[half]).start(priority=1)
            wa_copy(*wa_piece(src, q), half, q, sems.at[half]).start(priority=1)

    def wait_trip(half):
        for view in (stage.at[half, :, :3], stage.at[half, :, 3, :128]):
            pltpu.make_async_copy(view, view, sems.at[half]).wait()

    qr = 2 * hw

    def wo_copy(start, n, sem):
        wr = pl.ds(pl.multiple_of(start, 8), n)
        return pltpu.make_async_copy(wo32.at[wr, :], wo_s.at[wr, :], sem)

    def wo_sums(q, piece, anchor=None, never=None):
        def blk(k, n):
            w = wo_s[pl.ds(pl.multiple_of(q * qr + k * hw + piece * WX_ROWS, 8), WX_ROWS),
                     n * KH:(n + 1) * KH]
            if anchor is not None:
                w = jnp.where(never, anchor, w)
            return _unpack(w).astype(F32)

        b11, b12, b21, b22 = blk(0, 0), blk(0, 1), blk(1, 0), blk(1, 1)
        for n, v in enumerate((b11 + b22, b12 - b22, b21 - b11, b11 + b12, b21 + b22)):
            wx_s[q, n, pl.ds(pl.multiple_of(piece * WX_ROWS, 8), WX_ROWS), :] = (
                _pack(v.astype(BF16)))

    def x_copies(xr, sem):
        return [pltpu.make_async_copy(ax_hbm.at[xr, :], xa_s.at[xr, :D], sem),
                pltpu.make_async_copy(bx_hbm.at[xr, :], xb_s.at[xr, :D], sem)]

    xpre_cp = pltpu.make_async_copy(bx4_hbm.at[:, 0], xpre_s, sems.at[3])
    late_cps = ([pltpu.make_async_copy(mem0_hbm, mem0_s, sems.at[2])]
                + x_copies(pl.ds(0, X_HEAD), sems.at[2]))
    awo_cps = [
        pltpu.make_async_copy(awo32.at[:, c * 128:(c + 1) * 128], awo_raw.at[c], sems.at[2])
        for c in range(NT)]
    x_rest = x_copies(pl.ds(X_HEAD, S - X_HEAD), sems.at[3])
    tiles = [(m, j) for m in range(3) for j in range(PW // 128)]
    peel = [tiles[sum(PEEL[:n]):sum(PEEL[:n + 1])] for n in range(len(PEEL))]
    peel_cps = [[pltpu.make_async_copy(w_hbm[m].at[pl.ds(q * PW + j * 128, 128), :],
                                       stage.at[1, q, m, pl.ds(j * 128, 128), :], sems.at[4 + n])
                 for m, j in blk for q in range(PP)] for n, blk in enumerate(peel)]
    peel_cps[-1].append(wa_copy(0, NT - 1, 1, 0, sems.at[3 + len(PEEL)]))

    xpre_cp.start()
    for cps in peel_cps:
        for cp in cps:
            cp.start(priority=1)
    start_trip(0)
    for cp in late_cps:
        cp.start(priority=1)
    kv_s[:, :, :A_HALO, :] = jnp.zeros((2, NT, A_HALO, 128), F32)
    wo_s[NQ * qr:, :] = jnp.zeros((qr, D), U32)

    def gather_heads(ref):
        rows = []
        for j in range(A_DH // 2):
            u = ref[pl.ds(j, A_H, stride=A_DH // 2), :]
            rows.append(pltpu.bitcast(u << 16, F32))
            rows.append(pltpu.bitcast(u & jnp.uint32(0xFFFF0000), F32))
        return jnp.concatenate(rows, axis=0)

    HR = NSEG * PRE // 2

    def xq(i, k):
        return _unpack(xp_s[i * HR // 2:(i + 1) * HR // 2, k * KH:(k + 1) * KH])

    def strassen_lhs():
        f = lambda i, k: xq(i, k).astype(F32)
        sums = (f(0, 0) + f(1, 1), f(1, 0) + f(1, 1), f(0, 0) + f(0, 1),
                f(1, 0) - f(0, 0), f(0, 1) - f(1, 1))
        for n, v in enumerate(sums):
            xs_s[n] = _pack(v.astype(BF16))

    def pair_prep2(p, half, m, js=(0, 1, 2), hook=None):
        if SKIP_PROLOGUE:
            return
        for q in range(2):
            lo, hi = js[0] * 128, (js[-1] + 1) * 128
            w_s[p + q, :, m * PW + lo:m * PW + hi] = _pack(stage[half, q, m, lo:hi, :].T)
        nseg = ST_ROWS // PRE
        for j in js:
            rows = slice(j * 128, (j + 1) * 128)
            b = lambda k, q: stage[half, q, m, rows, k * KH:(k + 1) * KH]
            bf = lambda k, q: b(k, q).astype(F32)
            rhs = ((bf(0, 0) + bf(1, 1)).astype(BF16), b(0, 0),
                   (bf(0, 1) - bf(1, 1)).astype(BF16), (bf(1, 0) - bf(0, 0)).astype(BF16),
                   b(1, 1), (bf(0, 0) + bf(0, 1)).astype(BF16),
                   (bf(1, 0) + bf(1, 1)).astype(BF16))
            tail = [stage[half, q, m, rows, 2 * KH:] for q in range(2)]
            for c in range(HR // ST_ROWS):
                r = slice(c * ST_ROWS // 2, (c + 1) * ST_ROWS // 2)
                sm = lambda n: _unpack(xs_s[n, r, :])
                qd = lambda i, k: _unpack(
                    xp_s[(i * HR + c * ST_ROWS) // 2:(i * HR + (c + 1) * ST_ROWS) // 2,
                         k * KH:(k + 1) * KH])
                rest = lambda i: _unpack(
                    xp_s[(i * HR + c * ST_ROWS) // 2:(i * HR + (c + 1) * ST_ROWS) // 2, 2 * KH:])

                def put(i, q, v):
                    s0 = i * (NSEG // 2) + c * nseg
                    pre_s[s0:s0 + nseg, p + q, :, m * PW + j * 128:m * PW + (j + 1) * 128] = (
                        v.reshape(nseg, PRE, 128))
                    if hook is not None:
                        hook(v)

                m5 = _nt_dot(sm(2), rhs[4])
                m3 = _nt_dot(qd(0, 0), rhs[2])
                put(0, 1, _nt_dot(rest(0), tail[1]) + m3 + m5)
                m1 = _nt_dot(sm(0), rhs[0])
                m4 = _nt_dot(qd(1, 1), rhs[3])
                put(0, 0, _nt_dot(rest(0), tail[0]) + _nt_dot(sm(4), rhs[6]) + (m1 + m4 - m5))
                m2 = _nt_dot(sm(1), rhs[1])
                put(1, 0, _nt_dot(rest(1), tail[0]) + m2 + m4)
                put(1, 1, _nt_dot(rest(1), tail[1]) + _nt_dot(sm(3), rhs[5]) + (m1 - m2 + m3))

    def wa_prep(c, kt, half, q):
        t1_s[q] = _pack(stage[half, q, 3, :128].T)
        g = gather_heads(t1_s.at[q])
        wa_s[c, pl.ds(pl.multiple_of(kt * 64, 64), 64), :] = _pack(g.astype(BF16).T)
        return g

    def wa_trip(g, half):
        lo, hi = [wa_prep(*wa_piece(g, q), half, q) for q in range(2)]
        for t in range(2):
            b11, b12 = lo[2 * t * 128:(2 * t + 1) * 128], lo[(2 * t + 1) * 128:(2 * t + 2) * 128]
            b21, b22 = hi[2 * t * 128:(2 * t + 1) * 128], hi[(2 * t + 1) * 128:(2 * t + 2) * 128]
            sums = cat([b11 + b22, b12 - b22, b21 - b11, b11 + b12, b21 + b22])
            wc_s[g, t] = _pack(sums.astype(BF16).T)

    xpre_cp.wait()
    xp_s[...] = _pack(xpre_s[...].reshape(NSEG * PRE, D))
    strassen_lhs()
    for blk, cps in zip(peel, peel_cps):
        for cp in cps:
            cp.wait()
        for m in range(3):
            js = tuple(j for mm, j in blk if mm == m)
            if js:
                pair_prep2(0, 1, m, js)
    wa_prep(0, NT - 1, 1, 0)

    def prologue(g, carry):
        half = g & 1

        @pl.when(g > 0)
        def _():
            wo_copy((g - 1) * WO_ROWS, WO_ROWS, sems.at[8]).wait()

        @pl.when(g == NTRIP - 1)
        def _():
            for cp in awo_cps:
                cp.start(priority=1)

        @pl.when(g < NTRIP - 1)
        def _():
            wo_copy(g * WO_ROWS, WO_ROWS, sems.at[8]).start()

        start_trip(g + 1)
        wait_trip(half)
        calls = [0]
        per = hw // WX_ROWS
        total = max(b - a for a, b in zip(WX_DONE, WX_DONE[1:]))
        todo = list(range(total))
        first, stop = NQ * per, (NQ + 1) * per
        for trip in range(1, NTRIP):
            first = jnp.where(g == trip, WX_DONE[trip - 1], first)
            stop = jnp.where(g == trip, WX_DONE[trip], stop)

        def hook(v):
            calls[0] += 1
            want = (calls[0] - WX_SKIP) * total // (36 - WX_SKIP - WX_TAIL)
            t = 0
            while todo and todo[0] < want:
                k = jnp.minimum(first + todo.pop(0), stop - 1)
                q = k // per
                anchor = jnp.concatenate(
                    [v[(2 * t + c) * WX_ROWS:(2 * t + c + 1) * WX_ROWS] for c in range(2)], axis=1)
                wo_sums(q, k % per, pltpu.bitcast(anchor, U32), g > NSEG)
                t += 1

        for m in range(3):
            pair_prep2((g + 1) * PP, half, m, hook=hook)
            if m == 0:
                wa_trip(g, half)
        return carry

    lax.fori_loop(0, NTRIP, prologue, 0)

    for cp in late_cps + awo_cps:
        cp.wait()
    for cp in x_rest:
        cp.start()

    for c in range(NT):
        awo_s[:, c * 128:(c + 1) * 128] = _pack(gather_heads(awo_raw.at[c]).astype(BF16))

    def out_copy(row, n, half):
        r = pl.ds(row, n)
        c = slice(half * D, (half + 1) * D)
        return pltpu.make_async_copy(out_s.at[r, c], out_hbm.at[r, c], sems.at[7])

    def segment(s, mem, u):
        last = u == SPT - 1
        row0 = pl.multiple_of(s * SEG, SEG)
        ninf = jnp.float32(-jnp.inf)

        qi = lax.broadcasted_iota(jnp.int32, (SEG, 2 * L), 0)
        kl = lax.broadcasted_iota(jnp.int32, (SEG, 2 * L), 1)
        is_a = kl < L
        is_b = kl >= L
        kpos = jnp.where(is_a, kl, kl - L)
        allowed = (qi >= FRESH) | (qi + MEM + PRE >= kpos)
        pi = lax.broadcasted_iota(jnp.int32, (GP * PRE, 128), 0)
        pk = lax.broadcasted_iota(jnp.int32, (GP * PRE, 128), 1)
        p_own = (pk // SEG) == (pi // PRE)
        p_allowed = (pk % (MEM + PRE)) <= (pi % PRE) + MEM
        p_first = (pk % SEG) < MEM + PRE
        p_is_a = p_own & p_first
        p_is_b = p_own & jnp.logical_not(p_first)
        col_a = lax.broadcasted_iota(jnp.int32, (1, PW), 1) < B_DH
        col128_a = lax.broadcasted_iota(jnp.int32, (1, 128), 1) < (B_DH - 128)

        xb = xb_s[pl.ds(row0, SEG), :D].astype(F32)
        h = jnp.concatenate([xb[PRE:], mem], axis=0).astype(BF16)

        def proj(p, m):
            return _dot(h, _unpack(w_s[p, :, m * PW:(m + 1) * PW]))

        def pre(p, m):
            return pre_s[s, p, :, m * PW:(m + 1) * PW]

        def block_diag(p, m):
            f = proj(p, m)
            full = jnp.concatenate([f[FRESH:], pre(p, m), f[:FRESH]], axis=0)
            z = jnp.zeros_like(full)
            return jnp.where(col_a, full, z), jnp.where(col_a, z, full)

        def keys_t(blocks):
            fold = cat([jnp.concatenate([x[:, :128] if i % 2 == 0 else x[:, 256:], x[:, 128:256]],
                                        axis=1) for i, x in enumerate(blocks)])
            t = fold.T
            outer = t[:128]
            n = blocks[0].shape[0]
            lane = lax.broadcasted_iota(jnp.int32, outer.shape, 1)
            lane_a = lane < n if len(blocks) == 2 else lane % (2 * n) < n
            z = jnp.zeros_like(outer)
            kt = cat([jnp.where(lane_a, outer, z), t[128:], jnp.where(lane_a, z, outer)])
            return kt.astype(BF16)

        def row_max(raw, ok, in_a, in_b):
            sc = jnp.where(ok, raw * b_scale, NEG)
            ma = jnp.max(jnp.where(in_a, sc, ninf), axis=1, keepdims=True)
            mb = jnp.max(jnp.where(in_b, sc, ninf), axis=1, keepdims=True)
            return sc, ma, mb

        def probs(mx, first, own, late_norm):
            sc, ma, mb = mx
            e = jnp.exp2(sc - jnp.where(first, ma, mb))
            if own is not None:
                e = jnp.where(own, e, 0.0)
            sa = jnp.sum(jnp.where(first, e, 0.0), axis=1, keepdims=True)
            sb = jnp.sum(jnp.where(first, 0.0, e), axis=1, keepdims=True)
            if late_norm:
                return e.astype(BF16), _recip(sa), _recip(sb)
            return (e * _recip(jnp.where(first, sa, sb))).astype(BF16), None, None

        def pv(sm, vbd):
            e, ra, rb = sm
            o = _dot(e, cat(vbd).astype(BF16))
            if ra is not None:
                o = jnp.concatenate([
                    o[:, :128] * ra,
                    o[:, 128:256] * jnp.where(col128_a, ra, rb),
                    o[:, 256:] * rb], axis=1)
            return o

        def pre_pv(g, pr, vbds):
            v = cat([x[:MEM + PRE] for vb in vbds for x in vb])
            o = _dot(pr, v.astype(BF16))
            if not last:
                odef_s[u, g] = o
            return o

        def wout(p, o, acc):
            contrib = _dot(o.astype(BF16), _unpack(wo_s[p * hw:(p + 1) * hw, :]))
            return contrib if acc is None else acc + contrib

        def deferred(p):
            r = slice((p % GP) * PRE, (p % GP + 1) * PRE)
            return cat([odef_s[v, p // GP, r, :] for v in range(SPT - 1)]
                       + [val["PPV", p // GP][r]])

        def wout_strassen(kind, q):
            a11, a21 = val["PV", 2 * q], deferred(2 * q)
            if kind != "XA":
                a12, a22 = val["PV", 2 * q + 1], deferred(2 * q + 1)
            blk = lambda k, n: _unpack(
                wo_s[q * qr + k * hw:q * qr + (k + 1) * hw, n * KH:(n + 1) * KH])
            sm = lambda n: _unpack(wx_s[q, n])
            if kind == "XA":
                terms = {3: (a11, sm(1)), 6: (a21 - a11, sm(3))}
            elif kind == "XB":
                terms = {1: (a11 + a22, sm(0)), 4: (a22, sm(2)), 5: (a11 + a12, blk(1, 1)),
                         7: (a12 - a22, sm(4))}
            elif kind == "XC":
                terms = {2: (a21 + a22, blk(0, 0))}
            else:
                lhs = jnp.concatenate([cat([a11, a21]), cat([a12, a22])], axis=1)
                terms = {0: (lhs, _unpack(wo_s[q * qr:(q + 1) * qr, 2 * KH:]))}
            for n, (x, w) in terms.items():
                r = _dot(x.astype(BF16), w)
                val["acc", n] = val["acc", n] + r if ("acc", n) in val else r

        arow0 = pl.multiple_of((s - u % 2) * SEG, 2 * SEG)

        def a_put(m, j, r):
            if m == 0:
                qa_s[j] = r * a_scale
            else:
                kv_s[m - 1, j, A_HALO:A_HALO + 2 * SEG, :] = r

        def a_proj(idx):
            m, t = divmod(idx, 3)
            if "xa" not in val:
                xa = xa_s[pl.ds(arow0, 2 * SEG), :D]
                xf = xa.astype(F32)
                f = lambda i, k: xf[i * SEG:(i + 1) * SEG, k * KH:(k + 1) * KH]
                val["xa"] = xa
                val["xs"] = [v.astype(BF16) for v in (
                    f(0, 0) + f(1, 1), f(1, 0) + f(1, 1), f(0, 0), f(1, 1), f(0, 0) + f(0, 1),
                    f(1, 0) - f(0, 0), f(0, 1) - f(1, 1))]
                val["xr"] = xf[:, 2 * KH:].astype(BF16)
            if t == 2:
                a_put(m, NT - 1, _dot(val["xa"], _unpack(wa_s[m, :, (NT - 1) * 128:])))
                return
            sm = lambda n: _unpack(cat([wc_s[2 * m + k, t, :, n * 128:(n + 1) * 128]
                                        for k in range(2)]))
            blk = lambda k, j: _unpack(wa_s[m, k * KH // 2:(k + 1) * KH // 2,
                                            (2 * t + j) * 128:(2 * t + j + 1) * 128])
            rhs = (sm(0), blk(0, 0), sm(1), sm(2), blk(1, 1), sm(3), sm(4))
            mm = lambda n: _dot(val["xs"][n], rhs[n])
            tail = [_dot(val["xr"], _unpack(wa_s[m, KH:, (2 * t + j) * 128:(2 * t + j + 1) * 128]))
                    for j in range(2)]
            m1, m2, m3, m4, m5 = [mm(n) for n in range(5)]
            a_put(m, 2 * t, tail[0] + cat([mm(6) + (m1 + m4 - m5), m2 + m4]))
            a_put(m, 2 * t + 1, tail[1] + cat([m3 + m5, mm(5) + (m1 - m2 + m3)]))

        def window(m, j, w, hf):
            lo = A_HALO + hf * SEG - A_DIL * w
            return kv_s[m, j, lo:lo + SEG, :]

        def local_softmax(hf):
            pos = arow0 + hf * SEG + lax.broadcasted_iota(jnp.int32, (SEG, 128), 0)
            rows = slice(hf * SEG, (hf + 1) * SEG)
            logits = []
            for w in range(A_W):
                t = qa_s[0, rows, :] * window(0, 0, w, hf)
                for j in range(1, NT):
                    t = t + qa_s[j, rows, :] * window(0, j, w, hf)
                t = t + pltpu.roll(t, 64, 1)
                t = t + pltpu.roll(t, 32, 1)
                if w > 0 and hf == 0:
                    t = jnp.where(pos >= A_DIL * w, t, NEG)
                logits.append(t)
            mx = functools.reduce(jnp.maximum, logits)
            es = [jnp.exp2(l - mx) for l in logits]
            inv = _recip(functools.reduce(lambda x, y: x + y, es))
            return es, inv

        def local_pv(j, hf):
            es, inv = val["LA", hf]
            o = es[0] * window(1, j, 0, hf)
            for w in range(1, A_W):
                o = o + es[w] * window(1, j, w, hf)
            return o * inv

        def local_out(j, acc):
            wj = _unpack(awo_s[j * 64:(j + 1) * 64, :])
            if ("AX", j) in val:
                r = cat([val["AX", j], _dot(local_pv(j, 1).astype(BF16), wj)])
            else:
                r = _dot(cat([local_pv(j, 0), local_pv(j, 1)]).astype(BF16), wj)
            for m in range(2):
                kv_s[m, j, :A_HALO, :] = kv_s[m, j, 2 * SEG:2 * SEG + A_HALO, :]
            return r if acc is None else acc + r

        val = {}
        acc = None
        oa = None
        for kind, t in _order(u):
            if kind == "K":
                val[kind, t] = block_diag(t, 1)
            elif kind == "V":
                val[kind, t] = block_diag(t, 2)
            elif kind == "Q":
                val[kind, t] = proj(t, 0).astype(BF16)
            elif kind == "T":
                val[kind, t] = keys_t(val["K", t])
            elif kind == "S":
                val[kind, t] = _dot(val["Q", t], val["T", t])
            elif kind == "M":
                val[kind, t] = row_max(val["S", t], allowed, is_a, is_b)
            elif kind == "E":
                val[kind, t] = probs(val["M", t], is_a, None, t >= LATE_FROM)
            elif kind == "PV":
                val[kind, t] = pv(val["E", t], val["V", t])
            elif kind == "TG":
                val[kind, t] = keys_t([x[:MEM + PRE] for r in range(GP)
                                       for x in val["K", GP * t + r]])
            elif kind == "PS":
                q = cat([pre(GP * t + r, 0) for r in range(GP)]).astype(BF16)
                val[kind, t] = _dot(q, val["TG", t])
            elif kind == "MG":
                val[kind, t] = row_max(val["PS", t], p_allowed, p_is_a, p_is_b)
            elif kind == "EG":
                val[kind, t] = probs(val["MG", t], p_first, p_own, False)[0]
            elif kind == "PPV":
                val[kind, t] = pre_pv(t, val["EG", t], [val["V", GP * t + r] for r in range(GP)])
            elif kind == "W":
                acc = wout(t, val["PV", t], acc)
            elif kind in ("XA", "XB", "XC", "Y"):
                wout_strassen(kind, t)
            elif kind == "LA":
                val[kind, t] = local_softmax(t)
            elif kind == "AP":
                a_proj(t)
            elif kind == "AX":
                val[kind, t] = _dot(local_pv(t, 0).astype(BF16),
                                    _unpack(awo_s[t * 64:(t + 1) * 64, :]))
            elif kind == "AO":
                oa = local_out(t, oa)
                if t == NT - 1:
                    out_s[pl.ds(arow0, 2 * SEG), :D] = oa.astype(BF16)
                    out_copy(arow0, 2 * SEG, 0).start()
        if last:
            m = lambda n: val["acc", n]
            acc = jnp.concatenate([
                cat([m(1) + m(4) - m(5) + m(7), m(2) + m(4)]),
                cat([m(3) + m(5), m(1) - m(2) + m(3) + m(6)]), m(0)], axis=1)
        return acc

    def steps(i, mem):
        @pl.when(i == 1)
        def _():
            for cp in x_rest:
                cp.wait()

        accs = []
        for u in range(SPT):
            accs.append(segment(i * SPT + u, mem, u))
            mem = accs[-1][FRESH:SEG]
        res = cat([x for u in range(SPT) for x in (
            accs[-1][SEG + u * PRE:SEG + (u + 1) * PRE], accs[u][:FRESH])])
        row = pl.multiple_of(i * SPT * SEG, SPT * SEG)
        out_s[pl.ds(row, SPT * SEG), D:2 * D] = res.astype(BF16)
        out_copy(row, SPT * SEG, 1).start()
        return mem

    lax.fori_loop(0, N_STEPS, steps, mem0_s[...].astype(F32))

    wait_trip(NTRIP % 2)

    done = N_STEPS * SPT * SEG
    pltpu.make_async_copy(out_s.at[:done, :2 * D], out_hbm.at[:done, :], sems.at[7]).wait()


@jax.jit
def pallas_concat_heads__sliding_local_dilated__memory_aug_recurrent_mem_tr__prompt_kernel(
    A_x: jax.Array,
    A_wqkv: jax.Array,
    A_wo: jax.Array,
    B_x: jax.Array,
    B_mem0: jax.Array,
    B_Wq: jax.Array,
    B_Wk: jax.Array,
    B_Wv: jax.Array,
    B_Wo: jax.Array,
    B_seg_len,
):
    del B_seg_len
    assert A_x.shape == (1, S, D) and B_x.shape == (1, S, D)
    hd = B_H * B_DH
    wq_t = jnp.transpose(B_Wq, (1, 2, 0)).reshape(hd, D)
    wk_t = jnp.transpose(B_Wk, (1, 2, 0)).reshape(hd, D)
    wv_t = jnp.transpose(B_Wv, (1, 2, 0)).reshape(hd, D)
    wo = B_Wo.reshape(hd, D)

    any_spec = pl.BlockSpec(memory_space=pl.ANY)
    out = pl.pallas_call(
        _kernel,
        out_shape=jax.ShapeDtypeStruct((S, 2 * D), BF16),
        in_specs=[any_spec] * 10,
        out_specs=any_spec,
        scratch_shapes=[
            pltpu.VMEM((2, PP, 4, PW, D), BF16),
            pltpu.VMEM((NT, D // 2, 128), U32),
            pltpu.VMEM((NP, D // 2, 3 * PW), U32),
            pltpu.VMEM((hd // 2 + PW, D), U32),
            pltpu.VMEM((NQ + 1, 5, PW // 2, KH), U32),
            pltpu.VMEM((NSEG, NP, PRE, 3 * PW), F32),
            pltpu.VMEM((SPT - 1, NG, GP * PRE, PW), F32),
            pltpu.VMEM((S, OUT_W), BF16),
            pltpu.VMEM((S, X_W), BF16),
            pltpu.VMEM((S, X_W), BF16),
            pltpu.VMEM((NSEG, PRE, D), BF16),
            pltpu.VMEM((NSEG * PRE // 2, D), U32),
            pltpu.VMEM((5, NSEG * PRE // 4, 256), U32),
            pltpu.VMEM((MEM, D), BF16),
            pltpu.VMEM((3, D // 2, D), U32),
            pltpu.VMEM((NTRIP, 2, 64, D), U32),
            pltpu.VMEM((D // 2, D), U32),
            pltpu.VMEM((PP, D // 2, 128), U32),
            pltpu.VMEM((NT, 2 * SEG, 128), F32),
            pltpu.VMEM((2, NT, KV_ROWS, 128), F32),
            pltpu.SemaphoreType.DMA((9,)),
        ],
        compiler_params=pltpu.CompilerParams(vmem_limit_bytes=120 * 1024 * 1024,
                                             disable_bounds_checks=True),
    )(A_x.reshape(S, D), A_wqkv, A_wo, B_x.reshape(S, D), B_x.reshape(NSEG, SEG // PRE, PRE, D),
      B_mem0.reshape(MEM, D), wq_t, wk_t, wv_t, wo)
    return out.reshape(1, S, 2 * D)
```

```python
import functools

import jax
import jax.numpy as jnp
from jax import lax
import jax.experimental.pallas as pl
import jax.experimental.pallas.tpu as pltpu

F32 = jnp.float32
BF16 = jnp.bfloat16
U32 = jnp.uint32

S = 2048
D = 640
NT = D // 128
A_H = 32
A_DH = D // A_H
A_W = 8
A_DIL = 2
A_HALO = 16
B_H = 32
B_DH = 192
MEM = 8
SEG = 32
NSEG = S // SEG
NP = B_H // 2
PW = 2 * B_DH
PRE = 8
FRESH = SEG - PRE
L = MEM + SEG
GP = 4
NG = NP // GP
LOG2E = 1.4426950408889634
NEG = -1000000000.0 * LOG2E
PP = 2
NTRIP = NP // PP - 1
PEEL = (2, 2, 5)
KH = 256
WO_ROWS = 512
WX_DONE = (0, 24, 56, 96, 120, 152, 192)
WX_TAIL = 2
WX_ROWS = 8
WX_SKIP = 0
ST_ROWS = 256
X_HEAD = 128
KV_ROWS = 80
X_W = 1024
OUT_W = 2048
SPT = 4
N_STEPS = NSEG // SPT
NQ = NP // 2

LAT_MM, LAT_X, LAT_T, LAT_N, LAT_N_LATE = 190, 190, 380, 230, 100
LATE_FROM = NP - 2
AP_AFTER = (6, 16, 26)
AO_AFTER = (30, 40)
TAIL_FILL = (2, 2, 2, 0)
HOLD_W = (0, 3, 0, 0)


def _segment_order(u):
    odd, last = u % 2 == 1, u == SPT - 1
    proj = []
    for g in range(NG):
        proj += [("K", GP * g + r) for r in range(GP)]
        for r in range(GP):
            proj += [("V", GP * g + r), ("Q", GP * g + r)]
    dur = {"K": 120, "V": 120, "Q": 120, "S": 24, "PV": 24, "PS": 24, "PPV": 24,
           "W": 120, "XA": 96, "XB": 192, "XC": 48, "Y": 96, "AO": 80, "AP": 125,
           "T": 0, "M": 0, "E": 0, "TG": 0, "MG": 0, "EG": 0}
    end = {}

    def ready(task):
        k, i = task
        if k == "T":
            deps = [(("K", i), LAT_MM)]
        elif k == "S":
            deps = [(("Q", i), LAT_MM), (("T", i), LAT_T)]
        elif k == "M":
            deps = [(("S", i), LAT_MM - 40)]
        elif k == "E":
            deps = [(("M", i), LAT_X)]
        elif k == "PV":
            deps = [(("E", i), LAT_N_LATE if i >= LATE_FROM else LAT_N), (("V", i), LAT_MM)]
        elif k == "TG":
            deps = [(("K", GP * i + r), LAT_MM) for r in range(GP)]
        elif k == "PS":
            deps = [(("TG", i), LAT_T)]
        elif k == "MG":
            deps = [(("PS", i), LAT_MM - 40)]
        elif k == "EG":
            deps = [(("MG", i), LAT_X)]
        elif k == "PPV":
            deps = [(("EG", i), LAT_N), (("V", GP * i + GP - 1), LAT_MM)]
        elif k == "W":
            deps = [(("PV", i), LAT_MM)]
        else:
            deps = [(("PV", 2 * i), LAT_MM), (("PPV", 2 * i // GP), LAT_MM)]
            if k != "XA":
                deps.append((("PV", 2 * i + 1), LAT_MM))
        if any(d not in end for d, _ in deps):
            return None
        return max(end[d] + lat for d, lat in deps)

    pend = ([(k, p) for k in ("E", "M", "T") for p in range(NP)]
            + [(k, g) for k in ("EG", "MG", "TG") for g in range(NG)]
            + ([(k, q) for q in range(NQ) for k in ("XA", "XB", "Y", "XC")] if last
               else [("W", p) for p in range(NP)])
            + [("PPV", g) for g in range(NG)]
            + [("PV", p) for p in range(NP)] + [("PS", g) for g in range(NG)]
            + [("S", p) for p in range(NP)])
    fill = [("AO", j) for j in range(NT)] if odd else [("AP", j) for j in (3, 4, 5, 0, 1, 2, 6, 7, 8)]
    order = []
    now = [0]

    def emit(task):
        order.append(task)
        now[0] += dur[task[0]]
        end[task] = now[0]

    nproj = 0
    while pend:
        cand = [x for x in pend if ready(x) is not None and ready(x) <= now[0]]
        if proj:
            cand = [x for x in cand if not (x[0] == "W" and x[1] >= NP - GP - HOLD_W[u])]
        if cand:
            if not proj:
                cand = [x for x in cand if x[0] not in ("W", "XA", "XB", "XC", "Y")] or cand
            pend.remove(cand[0])
            emit(cand[0])
        elif proj:
            emit(proj.pop(0))
            nproj += 1
            if odd and nproj == GP:
                order += [("LA", 0), ("LA", 1)]
            if nproj in (AO_AFTER if odd else AP_AFTER):
                emit(fill.pop(0))
        elif len(fill) > TAIL_FILL[u]:
            emit(fill.pop(0))
        else:
            now[0] = min(ready(x) for x in pend if ready(x) is not None)
    return order + fill


ORDERS = (
    "K0 K1 K2 T0 K3 T1 V0 T2 Q0 AP3 T3 TG0 S0 M0 PS0 V1 Q1 Q2 V2 V3 E0 MG0 S1 S2 Q3 M1 K4 EG0 PV0 "
    "K5 E1 M2 S3 K6 T4 W0 E2 M3 T5 PPV0 PV1 K7 AP4 E3 T6 W1 T7 TG1 PV2 PV3 Q4 W2 V4 W3 PS1 S4 V5 "
    "Q5 M4 MG1 V6 Q7 Q6 E4 S5 EG1 V7 M5 PV4 S6 K8 PPV1 E5 S7 M6 K9 W4 AP5 E6 M7 T8 K10 PV5 T9 K11 "
    "E7 W5 T10 PV6 V8 T11 TG2 PV7 Q8 W6 W7 S8 PS2 V10 V9 Q9 M8 MG2 Q10 E8 EG2 V11 S9 Q11 M9 PV8 "
    "S10 K12 PPV2 E9 S11 M10 W8 K13 E10 M11 T12 PV9 K14 K15 E11 T13 W9 PV10 V12 T14 T15 TG3 PV11 "
    "Q12 W10 W11 PS3 S12 Q13 V13 M12 MG3 V15 V14 E12 Q14 EG3 Q15 S13 M13 PV12 S14 AP0 PPV3 E13 "
    "S15 M14 W12 AP1 E14 PV13 M15 AP2 PV14 AP6 E15 W13 PV15 W14 W15 AP8 AP7 ",
    "K0 K1 K2 T0 K3 LA0 LA1 T1 V0 T2 Q0 T3 TG0 V1 Q1 S0 V2 PS0 Q2 M0 S1 V3 MG0 Q3 E0 M1 S2 K4 EG0 "
    "K5 E1 M2 PV0 S3 K6 T4 PPV0 E2 T5 K7 M3 W0 T6 PV1 PV2 V4 E3 T7 TG1 Q4 W1 W2 PV3 PS1 S4 V5 Q5 "
    "AO0 M4 MG1 W3 S5 V6 E4 EG1 Q6 M5 V7 PV4 Q7 E5 S6 K8 W4 M6 PPV1 PV5 S7 T8 K9 E6 K10 M7 W5 T9 "
    "PV6 K11 E7 T10 V8 W6 T11 TG2 PV7 Q8 AO1 W7 S8 V9 PS2 Q9 M8 V10 MG2 Q10 E8 S9 V11 EG2 Q11 PV8 "
    "M9 S10 K12 PPV2 E9 S11 M10 W8 K13 E10 M11 T12 PV9 K14 K15 E11 T13 T14 PV10 AO2 V12 T15 TG3 "
    "Q12 PV11 V13 Q13 PS3 S12 V14 Q14 M12 MG3 S13 V15 Q15 E12 M13 EG3 S14 W9 E13 M14 PPV3 W10 "
    "PV12 S15 W11 E14 M15 PV13 W12 PV14 E15 W13 PV15 W14 W15 AO3 AO4 ",
    "K0 K1 K2 T0 K3 T1 V0 Q0 AP3 TG0 T3 T2 V1 S0 Q1 Q2 V2 M0 PS0 S1 V3 E0 MG0 Q3 M1 S2 K4 EG0 PV0 "
    "K5 E1 M2 S3 K6 T4 W0 E2 M3 T5 PPV0 PV1 K7 AP4 E3 W1 T6 T7 TG1 PV2 V4 PV3 Q4 W2 W3 PS1 S4 V5 "
    "M4 Q5 MG1 V6 Q6 EG1 S5 E4 V7 Q7 M5 PV4 S6 K8 PPV1 E5 S7 M6 W4 K9 AP5 E6 M7 T8 PV5 K10 T9 K11 "
    "E7 W5 T10 PV6 V8 T11 TG2 PV7 Q8 W6 W7 S8 PS2 V9 Q9 M8 MG2 V10 Q10 E8 EG2 S9 V11 Q11 M9 PV8 "
    "S10 K12 PPV2 E9 S11 M10 W8 K13 E10 M11 T12 PV9 K14 K15 E11 T13 W9 PV11 T14 PV10 V12 T15 TG3 "
    "Q12 W10 W11 PS3 S12 MG3 V13 Q13 M12 V14 Q14 E12 EG3 S13 V15 Q15 M13 PV12 S14 AP0 PPV3 E13 "
    "S15 M14 W12 AP1 E14 M15 AP2 PV13 PV14 AP6 E15 W13 PV15 W14 W15 AP7 AP8 ",
    "K1 K0 K2 T0 K3 LA0 LA1 T1 V0 T2 Q0 T3 TG0 V1 Q1 S0 V2 PS0 Q2 M0 V3 MG0 Q3 S1 E0 M1 S2 K4 EG0 "
    "K5 E1 M2 T4 PV0 AO0 PPV0 S3 K6 E2 T5 K7 M3 XA0 T6 PV1 PV2 V4 E3 T7 TG1 Y0 XB0 Q4 XC0 XA1 PV3 "
    "PS1 S4 V5 Q5 M4 MG1 XB1 E4 EG1 Y1 XC1 S5 V6 PV4 Q6 M5 V7 S6 Q7 AO1 E5 PPV1 K8 S7 K9 M6 XA2 "
    "M7 T8 PV5 K10 E6 T9 XB2 K11 E7 T10 T11 TG2 Y2 XC2 PV6 PV7 V8 Q8 XA3 XB3 Y3 XC3 PS2 S8 V9 Q9 "
    "M8 MG2 V10 Q10 AO2 E8 EG2 S9 V11 S10 Q11 M9 PV8 K12 M10 PPV2 K13 E9 S11 K14 E10 T12 XA4 M11 "
    "T13 PV9 K15 T14 PV10 V12 E11 XB4 T15 TG3 Y4 XC4 XA5 PV11 Q12 AO3 XB5 Y5 PS3 XC5 S12 V13 Q13 "
    "M12 MG3 V14 Q14 E12 EG3 S13 V15 Q15 M13 PV12 S14 AO4 PPV3 E13 S15 M14 E14 XA6 M15 PV13 PV14 "
    "E15 XB6 PV15 Y6 XC6 XA7 XB7 Y7 XC7 ",
)
SKIP_PROLOGUE = False


def _order(u):
    if ORDERS is None or ORDERS[u] is None:
        return _segment_order(u)
    return [(t.rstrip("0123456789"), int(t.lstrip("ABCDEFGHIJKLMNOPQRSTUVWXYZ")))
            for t in ORDERS[u].split()]


def _nt_dot(a, b):
    return lax.dot_general(a, b, (((1,), (1,)), ((), ())), preferred_element_type=F32)


def _dot(a, b):
    return jnp.dot(a, b, preferred_element_type=F32)


def _pack(x):
    return pltpu.bitcast(x, U32)


def _unpack(x):
    return pltpu.bitcast(x, BF16)


def cat(parts):
    return jnp.concatenate(parts, axis=0)


def _recip(x):
    r = pl.reciprocal(x, approx=True)
    return r * (2.0 - x * r)


def _kernel(ax_hbm, awqkv_hbm, awo_hbm, bx_hbm, bx4_hbm, mem0_hbm, wq_hbm, wk_hbm, wv_hbm, wo_hbm,
            out_hbm,
            stage, awo_raw, w_s, wo_s, wx_s, pre_s, odef_s, out_s,
            xa_s, xb_s, xpre_s, xp_s, xs_s, mem0_s, wa_s, wc_s, awo_s, t1_s, qa_s, kv_s,
            sems):
    b_scale = B_DH ** (-0.5) * LOG2E
    a_scale = A_DH ** (-0.5) * LOG2E

    w_hbm = (wq_hbm, wk_hbm, wv_hbm)
    wo32 = wo_hbm.bitcast(U32)
    awo32 = awo_hbm.bitcast(U32)
    hw = PW // 2
    hd = B_H * B_DH

    def w_copy(p, half, q, m, sem):
        rows = pl.ds(pl.multiple_of(p * PW, PW), PW)
        return pltpu.make_async_copy(w_hbm[m].at[rows, :], stage.at[half, q, m], sem)

    def wa_piece(g, q):
        last = g >= 2 * 3
        return jnp.where(last, 1 + q, g >> 1), jnp.where(last, NT - 1, (g & 1) + 2 * q)

    def wa_copy(c, kt, half, q, sem):
        return pltpu.make_async_copy(
            awqkv_hbm.at[pl.ds(pl.multiple_of(kt * 128, 128), 128),
                         pl.ds(pl.multiple_of(c * D, 128), D)],
            stage.at[half, q, 3, :128], sem)

    def start_trip(g):
        half = g & 1
        src = jnp.minimum(g, NTRIP - 1)
        for q in range(PP):
            for m in range(3):
                w_copy((src + 1) * PP + q, half, q, m, sems.at[half]).start(priority=1)
            wa_copy(*wa_piece(src, q), half, q, sems.at[half]).start(priority=1)

    def wait_trip(half):
        for view in (stage.at[half, :, :3], stage.at[half, :, 3, :128]):
            pltpu.make_async_copy(view, view, sems.at[half]).wait()

    qr = 2 * hw

    def wo_copy(start, n, sem):
        wr = pl.ds(pl.multiple_of(start, 8), n)
        return pltpu.make_async_copy(wo32.at[wr, :], wo_s.at[wr, :], sem)

    def wo_sums(q, piece, anchor=None, never=None):
        def blk(k, n):
            w = wo_s[pl.ds(pl.multiple_of(q * qr + k * hw + piece * WX_ROWS, 8), WX_ROWS),
                     n * KH:(n + 1) * KH]
            if anchor is not None:
                w = jnp.where(never, anchor, w)
            return _unpack(w).astype(F32)

        b11, b12, b21, b22 = blk(0, 0), blk(0, 1), blk(1, 0), blk(1, 1)
        for n, v in enumerate((b11 + b22, b12 - b22, b21 - b11, b11 + b12, b21 + b22)):
            wx_s[q, n, pl.ds(pl.multiple_of(piece * WX_ROWS, 8), WX_ROWS), :] = (
                _pack(v.astype(BF16)))

    def x_copies(xr, sem):
        return [pltpu.make_async_copy(ax_hbm.at[xr, :], xa_s.at[xr, :D], sem),
                pltpu.make_async_copy(bx_hbm.at[xr, :], xb_s.at[xr, :D], sem)]

    xpre_cp = pltpu.make_async_copy(bx4_hbm.at[:, 0], xpre_s, sems.at[3])
    late_cps = ([pltpu.make_async_copy(mem0_hbm, mem0_s, sems.at[2])]
                + x_copies(pl.ds(0, X_HEAD), sems.at[2]))
    awo_cps = [
        pltpu.make_async_copy(awo32.at[:, c * 128:(c + 1) * 128], awo_raw.at[c], sems.at[2])
        for c in range(NT)]
    x_rest = x_copies(pl.ds(X_HEAD, S - X_HEAD), sems.at[3])
    tiles = [(m, j) for m in range(3) for j in range(PW // 128)]
    peel = [tiles[sum(PEEL[:n]):sum(PEEL[:n + 1])] for n in range(len(PEEL))]
    peel_cps = [[pltpu.make_async_copy(w_hbm[m].at[pl.ds(q * PW + j * 128, 128), :],
                                       stage.at[1, q, m, pl.ds(j * 128, 128), :], sems.at[4 + n])
                 for m, j in blk for q in range(PP)] for n, blk in enumerate(peel)]
    peel_cps[-1].append(wa_copy(0, NT - 1, 1, 0, sems.at[3 + len(PEEL)]))

    xpre_cp.start()
    for cps in peel_cps:
        for cp in cps:
            cp.start(priority=1)
    start_trip(0)
    for cp in late_cps:
        cp.start(priority=1)
    kv_s[:, :, :A_HALO, :] = jnp.zeros((2, NT, A_HALO, 128), F32)
    wo_s[NQ * qr:, :] = jnp.zeros((qr, D), U32)

    def gather_heads(ref):
        rows = []
        for j in range(A_DH // 2):
            u = ref[pl.ds(j, A_H, stride=A_DH // 2), :]
            rows.append(pltpu.bitcast(u << 16, F32))
            rows.append(pltpu.bitcast(u & jnp.uint32(0xFFFF0000), F32))
        return jnp.concatenate(rows, axis=0)

    HR = NSEG * PRE // 2

    def xq(i, k):
        return _unpack(xp_s[i * HR // 2:(i + 1) * HR // 2, k * KH:(k + 1) * KH])

    def strassen_lhs():
        f = lambda i, k: xq(i, k).astype(F32)
        sums = (f(0, 0) + f(1, 1), f(1, 0) + f(1, 1), f(0, 0) + f(0, 1),
                f(1, 0) - f(0, 0), f(0, 1) - f(1, 1))
        for n, v in enumerate(sums):
            xs_s[n] = _pack(v.astype(BF16))

    def pair_prep2(p, half, m, js=(0, 1, 2), hook=None):
        if SKIP_PROLOGUE:
            return
        for q in range(2):
            lo, hi = js[0] * 128, (js[-1] + 1) * 128
            w_s[p + q, :, m * PW + lo:m * PW + hi] = _pack(stage[half, q, m, lo:hi, :].T)
        nseg = ST_ROWS // PRE
        for j in js:
            rows = slice(j * 128, (j + 1) * 128)
            b = lambda k, q: stage[half, q, m, rows, k * KH:(k + 1) * KH]
            bf = lambda k, q: b(k, q).astype(F32)
            rhs = ((bf(0, 0) + bf(1, 1)).astype(BF16), b(0, 0),
                   (bf(0, 1) - bf(1, 1)).astype(BF16), (bf(1, 0) - bf(0, 0)).astype(BF16),
                   b(1, 1), (bf(0, 0) + bf(0, 1)).astype(BF16),
                   (bf(1, 0) + bf(1, 1)).astype(BF16))
            tail = [stage[half, q, m, rows, 2 * KH:] for q in range(2)]
            for c in range(HR // ST_ROWS):
                r = slice(c * ST_ROWS // 2, (c + 1) * ST_ROWS // 2)
                sm = lambda n: _unpack(xs_s[n, r, :])
                qd = lambda i, k: _unpack(
                    xp_s[(i * HR + c * ST_ROWS) // 2:(i * HR + (c + 1) * ST_ROWS) // 2,
                         k * KH:(k + 1) * KH])
                rest = lambda i: _unpack(
                    xp_s[(i * HR + c * ST_ROWS) // 2:(i * HR + (c + 1) * ST_ROWS) // 2, 2 * KH:])

                def put(i, q, v):
                    s0 = i * (NSEG // 2) + c * nseg
                    pre_s[s0:s0 + nseg, p + q, :, m * PW + j * 128:m * PW + (j + 1) * 128] = (
                        v.reshape(nseg, PRE, 128))
                    if hook is not None:
                        hook(v)

                m5 = _nt_dot(sm(2), rhs[4])
                m3 = _nt_dot(qd(0, 0), rhs[2])
                put(0, 1, _nt_dot(rest(0), tail[1]) + m3 + m5)
                m1 = _nt_dot(sm(0), rhs[0])
                m4 = _nt_dot(qd(1, 1), rhs[3])
                put(0, 0, _nt_dot(rest(0), tail[0]) + _nt_dot(sm(4), rhs[6]) + (m1 + m4 - m5))
                m2 = _nt_dot(sm(1), rhs[1])
                put(1, 0, _nt_dot(rest(1), tail[0]) + m2 + m4)
                put(1, 1, _nt_dot(rest(1), tail[1]) + _nt_dot(sm(3), rhs[5]) + (m1 - m2 + m3))

    def wa_prep(c, kt, half, q):
        t1_s[q] = _pack(stage[half, q, 3, :128].T)
        g = gather_heads(t1_s.at[q])
        wa_s[c, pl.ds(pl.multiple_of(kt * 64, 64), 64), :] = _pack(g.astype(BF16).T)
        return g

    def wa_trip(g, half):
        lo, hi = [wa_prep(*wa_piece(g, q), half, q) for q in range(2)]
        for t in range(2):
            b11, b12 = lo[2 * t * 128:(2 * t + 1) * 128], lo[(2 * t + 1) * 128:(2 * t + 2) * 128]
            b21, b22 = hi[2 * t * 128:(2 * t + 1) * 128], hi[(2 * t + 1) * 128:(2 * t + 2) * 128]
            sums = cat([b11 + b22, b12 - b22, b21 - b11, b11 + b12, b21 + b22])
            wc_s[g, t] = _pack(sums.astype(BF16).T)

    xpre_cp.wait()
    xp_s[...] = _pack(xpre_s[...].reshape(NSEG * PRE, D))
    strassen_lhs()
    for blk, cps in zip(peel, peel_cps):
        for cp in cps:
            cp.wait()
        for m in range(3):
            js = tuple(j for mm, j in blk if mm == m)
            if js:
                pair_prep2(0, 1, m, js)
    wa_prep(0, NT - 1, 1, 0)

    def prologue(g, carry):
        half = g & 1

        @pl.when(g > 0)
        def _():
            wo_copy((g - 1) * WO_ROWS, WO_ROWS, sems.at[8]).wait()

        @pl.when(g == NTRIP - 1)
        def _():
            for cp in awo_cps:
                cp.start(priority=1)

        @pl.when(g < NTRIP - 1)
        def _():
            wo_copy(g * WO_ROWS, WO_ROWS, sems.at[8]).start()

        start_trip(g + 1)
        wait_trip(half)
        calls = [0]
        per = hw // WX_ROWS
        total = max(b - a for a, b in zip(WX_DONE, WX_DONE[1:]))
        todo = list(range(total))
        first, stop = NQ * per, (NQ + 1) * per
        for trip in range(1, NTRIP):
            first = jnp.where(g == trip, WX_DONE[trip - 1], first)
            stop = jnp.where(g == trip, WX_DONE[trip], stop)

        def hook(v):
            calls[0] += 1
            want = (calls[0] - WX_SKIP) * total // (36 - WX_SKIP - WX_TAIL)
            t = 0
            while todo and todo[0] < want:
                k = jnp.minimum(first + todo.pop(0), stop - 1)
                q = k // per
                anchor = jnp.concatenate(
                    [v[(2 * t + c) * WX_ROWS:(2 * t + c + 1) * WX_ROWS] for c in range(2)], axis=1)
                wo_sums(q, k % per, pltpu.bitcast(anchor, U32), g > NSEG)
                t += 1

        for m in range(3):
            pair_prep2((g + 1) * PP, half, m, hook=hook)
            if m == 0:
                wa_trip(g, half)
        return carry

    lax.fori_loop(0, NTRIP, prologue, 0)

    for cp in late_cps + awo_cps:
        cp.wait()
    for cp in x_rest:
        cp.start()

    for c in range(NT):
        awo_s[:, c * 128:(c + 1) * 128] = _pack(gather_heads(awo_raw.at[c]).astype(BF16))

    def out_copy(row, n, half):
        r = pl.ds(row, n)
        c = slice(half * D, (half + 1) * D)
        return pltpu.make_async_copy(out_s.at[r, c], out_hbm.at[r, c], sems.at[7])

    def segment(s, mem, u):
        last = u == SPT - 1
        row0 = pl.multiple_of(s * SEG, SEG)
        ninf = jnp.float32(-jnp.inf)

        qi = lax.broadcasted_iota(jnp.int32, (SEG, 2 * L), 0)
        kl = lax.broadcasted_iota(jnp.int32, (SEG, 2 * L), 1)
        is_a = kl < L
        is_b = kl >= L
        kpos = jnp.where(is_a, kl, kl - L)
        allowed = (qi >= FRESH) | (qi + MEM + PRE >= kpos)
        pi = lax.broadcasted_iota(jnp.int32, (GP * PRE, 128), 0)
        pk = lax.broadcasted_iota(jnp.int32, (GP * PRE, 128), 1)
        p_own = (pk // SEG) == (pi // PRE)
        p_allowed = (pk % (MEM + PRE)) <= (pi % PRE) + MEM
        p_first = (pk % SEG) < MEM + PRE
        p_is_a = p_own & p_first
        p_is_b = p_own & jnp.logical_not(p_first)
        col_a = lax.broadcasted_iota(jnp.int32, (1, PW), 1) < B_DH
        col128_a = lax.broadcasted_iota(jnp.int32, (1, 128), 1) < (B_DH - 128)

        xb = xb_s[pl.ds(row0, SEG), :D].astype(F32)
        h = jnp.concatenate([xb[PRE:], mem], axis=0).astype(BF16)

        def proj(p, m):
            return _dot(h, _unpack(w_s[p, :, m * PW:(m + 1) * PW]))

        def pre(p, m):
            return pre_s[s, p, :, m * PW:(m + 1) * PW]

        def block_diag(p, m):
            f = proj(p, m)
            full = jnp.concatenate([f[FRESH:], pre(p, m), f[:FRESH]], axis=0)
            z = jnp.zeros_like(full)
            return jnp.where(col_a, full, z), jnp.where(col_a, z, full)

        def keys_t(blocks):
            fold = cat([jnp.concatenate([x[:, :128] if i % 2 == 0 else x[:, 256:], x[:, 128:256]],
                                        axis=1) for i, x in enumerate(blocks)])
            t = fold.T
            outer = t[:128]
            n = blocks[0].shape[0]
            lane = lax.broadcasted_iota(jnp.int32, outer.shape, 1)
            lane_a = lane < n if len(blocks) == 2 else lane % (2 * n) < n
            z = jnp.zeros_like(outer)
            kt = cat([jnp.where(lane_a, outer, z), t[128:], jnp.where(lane_a, z, outer)])
            return kt.astype(BF16)

        def row_max(raw, ok, in_a, in_b):
            sc = jnp.where(ok, raw * b_scale, NEG)
            ma = jnp.max(jnp.where(in_a, sc, ninf), axis=1, keepdims=True)
            mb = jnp.max(jnp.where(in_b, sc, ninf), axis=1, keepdims=True)
            return sc, ma, mb

        def probs(mx, first, own, late_norm):
            sc, ma, mb = mx
            e = jnp.exp2(sc - jnp.where(first, ma, mb))
            if own is not None:
                e = jnp.where(own, e, 0.0)
            sa = jnp.sum(jnp.where(first, e, 0.0), axis=1, keepdims=True)
            sb = jnp.sum(jnp.where(first, 0.0, e), axis=1, keepdims=True)
            if late_norm:
                return e.astype(BF16), _recip(sa), _recip(sb)
            return (e * _recip(jnp.where(first, sa, sb))).astype(BF16), None, None

        def pv(sm, vbd):
            e, ra, rb = sm
            o = _dot(e, cat(vbd).astype(BF16))
            if ra is not None:
                o = jnp.concatenate([
                    o[:, :128] * ra,
                    o[:, 128:256] * jnp.where(col128_a, ra, rb),
                    o[:, 256:] * rb], axis=1)
            return o

        def pre_pv(g, pr, vbds):
            v = cat([x[:MEM + PRE] for vb in vbds for x in vb])
            o = _dot(pr, v.astype(BF16))
            if not last:
                odef_s[u, g] = o
            return o

        def wout(p, o, acc):
            contrib = _dot(o.astype(BF16), _unpack(wo_s[p * hw:(p + 1) * hw, :]))
            return contrib if acc is None else acc + contrib

        def deferred(p):
            r = slice((p % GP) * PRE, (p % GP + 1) * PRE)
            return cat([odef_s[v, p // GP, r, :] for v in range(SPT - 1)]
                       + [val["PPV", p // GP][r]])

        def wout_strassen(kind, q):
            a11, a21 = val["PV", 2 * q], deferred(2 * q)
            if kind != "XA":
                a12, a22 = val["PV", 2 * q + 1], deferred(2 * q + 1)
            blk = lambda k, n: _unpack(
                wo_s[q * qr + k * hw:q * qr + (k + 1) * hw, n * KH:(n + 1) * KH])
            sm = lambda n: _unpack(wx_s[q, n])
            if kind == "XA":
                terms = {3: (a11, sm(1)), 6: (a21 - a11, sm(3))}
            elif kind == "XB":
                terms = {1: (a11 + a22, sm(0)), 4: (a22, sm(2)), 5: (a11 + a12, blk(1, 1)),
                         7: (a12 - a22, sm(4))}
            elif kind == "XC":
                terms = {2: (a21 + a22, blk(0, 0))}
            else:
                lhs = jnp.concatenate([cat([a11, a21]), cat([a12, a22])], axis=1)
                terms = {0: (lhs, _unpack(wo_s[q * qr:(q + 1) * qr, 2 * KH:]))}
            for n, (x, w) in terms.items():
                r = _dot(x.astype(BF16), w)
                val["acc", n] = val["acc", n] + r if ("acc", n) in val else r

        arow0 = pl.multiple_of((s - u % 2) * SEG, 2 * SEG)

        def a_put(m, j, r):
            if m == 0:
                qa_s[j] = r * a_scale
            else:
                kv_s[m - 1, j, A_HALO:A_HALO + 2 * SEG, :] = r

        def a_proj(idx):
            m, t = divmod(idx, 3)
            if "xa" not in val:
                xa = xa_s[pl.ds(arow0, 2 * SEG), :D]
                xf = xa.astype(F32)
                f = lambda i, k: xf[i * SEG:(i + 1) * SEG, k * KH:(k + 1) * KH]
                val["xa"] = xa
                val["xs"] = [v.astype(BF16) for v in (
                    f(0, 0) + f(1, 1), f(1, 0) + f(1, 1), f(0, 0), f(1, 1), f(0, 0) + f(0, 1),
                    f(1, 0) - f(0, 0), f(0, 1) - f(1, 1))]
                val["xr"] = xf[:, 2 * KH:].astype(BF16)
            if t == 2:
                a_put(m, NT - 1, _dot(val["xa"], _unpack(wa_s[m, :, (NT - 1) * 128:])))
                return
            sm = lambda n: _unpack(cat([wc_s[2 * m + k, t, :, n * 128:(n + 1) * 128]
                                        for k in range(2)]))
            blk = lambda k, j: _unpack(wa_s[m, k * KH // 2:(k + 1) * KH // 2,
                                            (2 * t + j) * 128:(2 * t + j + 1) * 128])
            rhs = (sm(0), blk(0, 0), sm(1), sm(2), blk(1, 1), sm(3), sm(4))
            mm = lambda n: _dot(val["xs"][n], rhs[n])
            tail = [_dot(val["xr"], _unpack(wa_s[m, KH:, (2 * t + j) * 128:(2 * t + j + 1) * 128]))
                    for j in range(2)]
            m1, m2, m3, m4, m5 = [mm(n) for n in range(5)]
            a_put(m, 2 * t, tail[0] + cat([mm(6) + (m1 + m4 - m5), m2 + m4]))
            a_put(m, 2 * t + 1, tail[1] + cat([m3 + m5, mm(5) + (m1 - m2 + m3)]))

        def window(m, j, w, hf):
            lo = A_HALO + hf * SEG - A_DIL * w
            return kv_s[m, j, lo:lo + SEG, :]

        def local_softmax(hf):
            pos = arow0 + hf * SEG + lax.broadcasted_iota(jnp.int32, (SEG, 128), 0)
            rows = slice(hf * SEG, (hf + 1) * SEG)
            logits = []
            for w in range(A_W):
                t = qa_s[0, rows, :] * window(0, 0, w, hf)
                for j in range(1, NT):
                    t = t + qa_s[j, rows, :] * window(0, j, w, hf)
                t = t + pltpu.roll(t, 64, 1)
                t = t + pltpu.roll(t, 32, 1)
                if w > 0 and hf == 0:
                    t = jnp.where(pos >= A_DIL * w, t, NEG)
                logits.append(t)
            mx = functools.reduce(jnp.maximum, logits)
            es = [jnp.exp2(l - mx) for l in logits]
            inv = _recip(functools.reduce(lambda x, y: x + y, es))
            return es, inv

        def local_pv(j, hf):
            es, inv = val["LA", hf]
            o = es[0] * window(1, j, 0, hf)
            for w in range(1, A_W):
                o = o + es[w] * window(1, j, w, hf)
            return o * inv

        def local_out(j, acc):
            wj = _unpack(awo_s[j * 64:(j + 1) * 64, :])
            if ("AX", j) in val:
                r = cat([val["AX", j], _dot(local_pv(j, 1).astype(BF16), wj)])
            else:
                r = _dot(cat([local_pv(j, 0), local_pv(j, 1)]).astype(BF16), wj)
            for m in range(2):
                kv_s[m, j, :A_HALO, :] = kv_s[m, j, 2 * SEG:2 * SEG + A_HALO, :]
            return r if acc is None else acc + r

        val = {}
        acc = None
        oa = None
        for kind, t in _order(u):
            if kind == "K":
                val[kind, t] = block_diag(t, 1)
            elif kind == "V":
                val[kind, t] = block_diag(t, 2)
            elif kind == "Q":
                val[kind, t] = proj(t, 0).astype(BF16)
            elif kind == "T":
                val[kind, t] = keys_t(val["K", t])
            elif kind == "S":
                val[kind, t] = _dot(val["Q", t], val["T", t])
            elif kind == "M":
                val[kind, t] = row_max(val["S", t], allowed, is_a, is_b)
            elif kind == "E":
                val[kind, t] = probs(val["M", t], is_a, None, t >= LATE_FROM)
            elif kind == "PV":
                val[kind, t] = pv(val["E", t], val["V", t])
            elif kind == "TG":
                val[kind, t] = keys_t([x[:MEM + PRE] for r in range(GP)
                                       for x in val["K", GP * t + r]])
            elif kind == "PS":
                q = cat([pre(GP * t + r, 0) for r in range(GP)]).astype(BF16)
                val[kind, t] = _dot(q, val["TG", t])
            elif kind == "MG":
                val[kind, t] = row_max(val["PS", t], p_allowed, p_is_a, p_is_b)
            elif kind == "EG":
                val[kind, t] = probs(val["MG", t], p_first, p_own, False)[0]
            elif kind == "PPV":
                val[kind, t] = pre_pv(t, val["EG", t], [val["V", GP * t + r] for r in range(GP)])
            elif kind == "W":
                acc = wout(t, val["PV", t], acc)
            elif kind in ("XA", "XB", "XC", "Y"):
                wout_strassen(kind, t)
            elif kind == "LA":
                val[kind, t] = local_softmax(t)
            elif kind == "AP":
                a_proj(t)
            elif kind == "AX":
                val[kind, t] = _dot(local_pv(t, 0).astype(BF16),
                                    _unpack(awo_s[t * 64:(t + 1) * 64, :]))
            elif kind == "AO":
                oa = local_out(t, oa)
                if t == NT - 1:
                    out_s[pl.ds(arow0, 2 * SEG), :D] = oa.astype(BF16)
                    out_copy(arow0, 2 * SEG, 0).start()
        if last:
            m = lambda n: val["acc", n]
            acc = jnp.concatenate([
                cat([m(1) + m(4) - m(5) + m(7), m(2) + m(4)]),
                cat([m(3) + m(5), m(1) - m(2) + m(3) + m(6)]), m(0)], axis=1)
        return acc

    def steps(i, mem):
        @pl.when(i == 1)
        def _():
            for cp in x_rest:
                cp.wait()

        accs = []
        for u in range(SPT):
            accs.append(segment(i * SPT + u, mem, u))
            mem = accs[-1][FRESH:SEG]
        res = cat([x for u in range(SPT) for x in (
            accs[-1][SEG + u * PRE:SEG + (u + 1) * PRE], accs[u][:FRESH])])
        row = pl.multiple_of(i * SPT * SEG, SPT * SEG)
        out_s[pl.ds(row, SPT * SEG), D:2 * D] = res.astype(BF16)
        out_copy(row, SPT * SEG, 1).start()
        return mem

    lax.fori_loop(0, N_STEPS, steps, mem0_s[...].astype(F32))

    wait_trip(NTRIP % 2)

    done = N_STEPS * SPT * SEG
    pltpu.make_async_copy(out_s.at[:done, :2 * D], out_hbm.at[:done, :], sems.at[7]).wait()


@jax.jit
def pallas_concat_heads__sliding_local_dilated__memory_aug_recurrent_mem_tr__prompt_kernel(
    A_x: jax.Array,
    A_wqkv: jax.Array,
    A_wo: jax.Array,
    B_x: jax.Array,
    B_mem0: jax.Array,
    B_Wq: jax.Array,
    B_Wk: jax.Array,
    B_Wv: jax.Array,
    B_Wo: jax.Array,
    B_seg_len,
):
    del B_seg_len
    assert A_x.shape == (1, S, D) and B_x.shape == (1, S, D)
    hd = B_H * B_DH
    wq_t = jnp.transpose(B_Wq, (1, 2, 0)).reshape(hd, D)
    wk_t = jnp.transpose(B_Wk, (1, 2, 0)).reshape(hd, D)
    wv_t = jnp.transpose(B_Wv, (1, 2, 0)).reshape(hd, D)
    wo = B_Wo.reshape(hd, D)

    any_spec = pl.BlockSpec(memory_space=pl.ANY)
    out = pl.pallas_call(
        _kernel,
        out_shape=jax.ShapeDtypeStruct((S, 2 * D), BF16),
        in_specs=[any_spec] * 10,
        out_specs=any_spec,
        scratch_shapes=[
            pltpu.VMEM((2, PP, 4, PW, D), BF16),
            pltpu.VMEM((NT, D // 2, 128), U32),
            pltpu.VMEM((NP, D // 2, 3 * PW), U32),
            pltpu.VMEM((hd // 2 + PW, D), U32),
            pltpu.VMEM((NQ + 1, 5, PW // 2, KH), U32),
            pltpu.VMEM((NSEG, NP, PRE, 3 * PW), F32),
            pltpu.VMEM((SPT - 1, NG, GP * PRE, PW), F32),
            pltpu.VMEM((S, OUT_W), BF16),
            pltpu.VMEM((S, X_W), BF16),
            pltpu.VMEM((S, X_W), BF16),
            pltpu.VMEM((NSEG, PRE, D), BF16),
            pltpu.VMEM((NSEG * PRE // 2, D), U32),
            pltpu.VMEM((5, NSEG * PRE // 4, 256), U32),
            pltpu.VMEM((MEM, D), BF16),
            pltpu.VMEM((3, D // 2, D), U32),
            pltpu.VMEM((NTRIP, 2, 64, D), U32),
            pltpu.VMEM((D // 2, D), U32),
            pltpu.VMEM((PP, D // 2, 128), U32),
            pltpu.VMEM((NT, 2 * SEG, 128), F32),
            pltpu.VMEM((2, NT, KV_ROWS, 128), F32),
            pltpu.SemaphoreType.DMA((9,)),
        ],
        compiler_params=pltpu.CompilerParams(vmem_limit_bytes=120 * 1024 * 1024,
                                             disable_bounds_checks=True),
    )(A_x.reshape(S, D), A_wqkv, A_wo, B_x.reshape(S, D), B_x.reshape(NSEG, SEG // PRE, PRE, D),
      B_mem0.reshape(MEM, D), wq_t, wk_t, wv_t, wo)
    return out.reshape(1, S, 2 * D)
```

```python
import functools

import jax
import jax.numpy as jnp
from jax import lax
import jax.experimental.pallas as pl
import jax.experimental.pallas.tpu as pltpu

F32 = jnp.float32
BF16 = jnp.bfloat16
U32 = jnp.uint32

S = 2048
D = 640
NT = D // 128
A_H = 32
A_DH = D // A_H
A_W = 8
A_DIL = 2
A_HALO = 16
B_H = 32
B_DH = 192
MEM = 8
SEG = 32
NSEG = S // SEG
NP = B_H // 2
PW = 2 * B_DH
PRE = 8
FRESH = SEG - PRE
L = MEM + SEG
GP = 4
NG = NP // GP
LOG2E = 1.4426950408889634
NEG = -1000000000.0 * LOG2E
PP = 2
NTRIP = NP // PP - 1
PEEL = (2, 2, 5)
KH = 256
WO_ROWS = 512
WX_DONE = (0, 24, 56, 96, 120, 152, 192)
WX_TAIL = 2
WX_ROWS = 8
WX_SKIP = 0
ST_ROWS = 256
X_HEAD = 128
KV_ROWS = 80
X_W = 1024
OUT_W = 2048
SPT = 4
N_STEPS = NSEG // SPT
NQ = NP // 2

LAT_MM, LAT_X, LAT_T, LAT_N, LAT_N_LATE = 190, 190, 380, 230, 100
LATE_FROM = NP - 2
AP_AFTER = (6, 16, 26)
AO_AFTER = (30, 40)
TAIL_FILL = (2, 2, 2, 0)
HOLD_W = (0, 3, 0, 0)


def _segment_order(u):
    odd, last = u % 2 == 1, u == SPT - 1
    proj = []
    for g in range(NG):
        proj += [("K", GP * g + r) for r in range(GP)]
        for r in range(GP):
            proj += [("V", GP * g + r), ("Q", GP * g + r)]
    dur = {"K": 120, "V": 120, "Q": 120, "S": 24, "PV": 24, "PS": 24, "PPV": 24,
           "W": 120, "XA": 96, "XB": 192, "XC": 48, "Y": 96, "AO": 80, "AP": 125,
           "T": 0, "M": 0, "E": 0, "TG": 0, "MG": 0, "EG": 0}
    end = {}

    def ready(task):
        k, i = task
        if k == "T":
            deps = [(("K", i), LAT_MM)]
        elif k == "S":
            deps = [(("Q", i), LAT_MM), (("T", i), LAT_T)]
        elif k == "M":
            deps = [(("S", i), LAT_MM - 40)]
        elif k == "E":
            deps = [(("M", i), LAT_X)]
        elif k == "PV":
            deps = [(("E", i), LAT_N_LATE if i >= LATE_FROM else LAT_N), (("V", i), LAT_MM)]
        elif k == "TG":
            deps = [(("K", GP * i + r), LAT_MM) for r in range(GP)]
        elif k == "PS":
            deps = [(("TG", i), LAT_T)]
        elif k == "MG":
            deps = [(("PS", i), LAT_MM - 40)]
        elif k == "EG":
            deps = [(("MG", i), LAT_X)]
        elif k == "PPV":
            deps = [(("EG", i), LAT_N), (("V", GP * i + GP - 1), LAT_MM)]
        elif k == "W":
            deps = [(("PV", i), LAT_MM)]
        else:
            deps = [(("PV", 2 * i), LAT_MM), (("PPV", 2 * i // GP), LAT_MM)]
            if k != "XA":
                deps.append((("PV", 2 * i + 1), LAT_MM))
        if any(d not in end for d, _ in deps):
            return None
        return max(end[d] + lat for d, lat in deps)

    pend = ([(k, p) for k in ("E", "M", "T") for p in range(NP)]
            + [(k, g) for k in ("EG", "MG", "TG") for g in range(NG)]
            + ([(k, q) for q in range(NQ) for k in ("XA", "XB", "Y", "XC")] if last
               else [("W", p) for p in range(NP)])
            + [("PPV", g) for g in range(NG)]
            + [("PV", p) for p in range(NP)] + [("PS", g) for g in range(NG)]
            + [("S", p) for p in range(NP)])
    fill = [("AO", j) for j in range(NT)] if odd else [("AP", j) for j in (3, 4, 5, 0, 1, 2, 6, 7, 8)]
    order = []
    now = [0]

    def emit(task):
        order.append(task)
        now[0] += dur[task[0]]
        end[task] = now[0]

    nproj = 0
    while pend:
        cand = [x for x in pend if ready(x) is not None and ready(x) <= now[0]]
        if proj:
            cand = [x for x in cand if not (x[0] == "W" and x[1] >= NP - GP - HOLD_W[u])]
        if cand:
            if not proj:
                cand = [x for x in cand if x[0] not in ("W", "XA", "XB", "XC", "Y")] or cand
            pend.remove(cand[0])
            emit(cand[0])
        elif proj:
            emit(proj.pop(0))
            nproj += 1
            if odd and nproj == GP:
                order += [("LA", 0), ("LA", 1)]
            if nproj in (AO_AFTER if odd else AP_AFTER):
                emit(fill.pop(0))
        elif len(fill) > TAIL_FILL[u]:
            emit(fill.pop(0))
        else:
            now[0] = min(ready(x) for x in pend if ready(x) is not None)
    return order + fill


ORDERS = (
    "K0 K1 K2 T0 K3 T1 V0 T2 Q0 AP3 T3 TG0 S0 M0 PS0 V1 Q1 Q2 V2 V3 E0 MG0 S1 S2 Q3 M1 K4 EG0 PV0 "
    "K5 E1 M2 S3 K6 T4 W0 E2 M3 T5 PPV0 PV1 K7 AP4 E3 T6 W1 T7 TG1 PV2 PV3 Q4 W2 V4 W3 PS1 S4 V5 "
    "Q5 M4 MG1 V6 Q7 Q6 E4 S5 EG1 V7 M5 PV4 S6 K8 PPV1 E5 S7 M6 K9 W4 AP5 E6 M7 T8 K10 PV5 T9 K11 "
    "E7 W5 T10 PV6 V8 T11 TG2 PV7 Q8 W6 W7 S8 PS2 V10 V9 Q9 M8 MG2 Q10 E8 EG2 V11 S9 Q11 M9 PV8 "
    "S10 K12 PPV2 E9 S11 M10 W8 K13 E10 M11 T12 PV9 K14 K15 E11 T13 W9 PV10 V12 T14 T15 TG3 PV11 "
    "Q12 W10 W11 PS3 S12 Q13 V13 M12 MG3 V15 V14 E12 Q14 EG3 Q15 S13 M13 PV12 S14 AP0 PPV3 E13 "
    "S15 M14 W12 AP1 E14 PV13 M15 AP2 PV14 AP6 E15 W13 PV15 W14 W15 AP8 AP7 ",
    "K0 K1 K2 T0 K3 LA0 LA1 T1 V0 T2 Q0 T3 TG0 V1 Q1 S0 V2 PS0 Q2 M0 S1 V3 MG0 Q3 E0 M1 S2 K4 EG0 "
    "K5 E1 M2 PV0 S3 K6 T4 PPV0 E2 T5 K7 M3 W0 T6 PV1 PV2 V4 E3 T7 TG1 Q4 W1 W2 PV3 PS1 S4 V5 Q5 "
    "AO0 M4 MG1 W3 S5 V6 E4 EG1 Q6 M5 V7 PV4 Q7 E5 S6 K8 W4 M6 PPV1 PV5 S7 T8 K9 E6 K10 M7 W5 T9 "
    "PV6 K11 E7 T10 V8 W6 T11 TG2 PV7 Q8 AO1 W7 S8 V9 PS2 Q9 M8 V10 MG2 Q10 E8 S9 V11 EG2 Q11 PV8 "
    "M9 S10 K12 PPV2 E9 S11 M10 W8 K13 E10 M11 T12 PV9 K14 K15 E11 T13 T14 PV10 AO2 V12 T15 TG3 "
    "Q12 PV11 V13 Q13 PS3 S12 V14 Q14 M12 MG3 S13 V15 Q15 E12 M13 EG3 S14 W9 E13 M14 PPV3 W10 "
    "PV12 S15 W11 E14 M15 PV13 W12 PV14 E15 W13 PV15 W14 W15 AO3 AO4 ",
    "K0 K1 K2 T0 K3 T1 V0 Q0 AP3 TG0 T3 T2 V1 S0 Q1 Q2 V2 M0 PS0 S1 V3 E0 MG0 Q3 M1 S2 K4 EG0 PV0 "
    "K5 E1 M2 S3 K6 T4 W0 E2 M3 T5 PPV0 PV1 K7 AP4 E3 W1 T6 T7 TG1 PV2 V4 PV3 Q4 W2 W3 PS1 S4 V5 "
    "M4 Q5 MG1 V6 Q6 EG1 S5 E4 V7 Q7 M5 PV4 S6 K8 PPV1 E5 S7 M6 W4 K9 AP5 E6 M7 T8 PV5 K10 T9 K11 "
    "E7 W5 T10 PV6 V8 T11 TG2 PV7 Q8 W6 W7 S8 PS2 V9 Q9 M8 MG2 V10 Q10 E8 EG2 S9 V11 Q11 M9 PV8 "
    "S10 K12 PPV2 E9 S11 M10 W8 K13 E10 M11 T12 PV9 K14 K15 E11 T13 W9 PV11 T14 PV10 V12 T15 TG3 "
    "Q12 W10 W11 PS3 S12 MG3 V13 Q13 M12 V14 Q14 E12 EG3 S13 V15 Q15 M13 PV12 S14 AP0 PPV3 E13 "
    "S15 M14 W12 AP1 E14 M15 AP2 PV13 PV14 AP6 E15 W13 PV15 W14 W15 AP7 AP8 ",
    "K1 K0 K2 T0 K3 LA0 LA1 T1 V0 T2 Q0 T3 TG0 V1 Q1 S0 V2 PS0 Q2 M0 V3 MG0 Q3 S1 E0 M1 S2 K4 EG0 "
    "K5 E1 M2 T4 PV0 AO0 PPV0 S3 K6 E2 T5 K7 M3 XA0 T6 PV1 PV2 V4 E3 T7 TG1 Y0 XB0 Q4 XC0 XA1 PV3 "
    "PS1 S4 V5 Q5 M4 MG1 XB1 E4 EG1 Y1 XC1 S5 V6 PV4 Q6 M5 V7 S6 Q7 AO1 E5 PPV1 K8 S7 K9 M6 XA2 "
    "M7 T8 PV5 K10 E6 T9 XB2 K11 E7 T10 T11 TG2 Y2 XC2 PV6 PV7 V8 Q8 XA3 XB3 Y3 XC3 PS2 S8 V9 Q9 "
    "M8 MG2 V10 Q10 AO2 E8 EG2 S9 V11 S10 Q11 M9 PV8 K12 M10 PPV2 K13 E9 S11 K14 E10 T12 XA4 M11 "
    "T13 PV9 K15 T14 PV10 V12 E11 XB4 T15 TG3 Y4 XC4 XA5 PV11 Q12 AO3 XB5 Y5 PS3 XC5 S12 V13 Q13 "
    "M12 MG3 V14 Q14 E12 EG3 S13 V15 Q15 M13 PV12 S14 AO4 PPV3 E13 S15 M14 E14 XA6 M15 PV13 PV14 "
    "E15 XB6 PV15 Y6 XC6 XA7 XB7 Y7 XC7 ",
)
SKIP_PROLOGUE = False


def _order(u):
    if ORDERS is None or ORDERS[u] is None:
        return _segment_order(u)
    return [(t.rstrip("0123456789"), int(t.lstrip("ABCDEFGHIJKLMNOPQRSTUVWXYZ")))
            for t in ORDERS[u].split()]


def _nt_dot(a, b):
    return lax.dot_general(a, b, (((1,), (1,)), ((), ())), preferred_element_type=F32)


def _dot(a, b):
    return jnp.dot(a, b, preferred_element_type=F32)


def _pack(x):
    return pltpu.bitcast(x, U32)


def _unpack(x):
    return pltpu.bitcast(x, BF16)


def cat(parts):
    return jnp.concatenate(parts, axis=0)


def _recip(x):
    r = pl.reciprocal(x, approx=True)
    return r * (2.0 - x * r)


def _kernel(ax_hbm, awqkv_hbm, awo_hbm, bx_hbm, bx4_hbm, mem0_hbm, wq_hbm, wk_hbm, wv_hbm, wo_hbm,
            out_hbm,
            stage, awo_raw, w_s, wo_s, wx_s, pre_s, odef_s, out_s,
            xa_s, xb_s, xpre_s, xp_s, xs_s, mem0_s, wa_s, wc_s, awo_s, t1_s, qa_s, kv_s,
            sems):
    b_scale = B_DH ** (-0.5) * LOG2E
    a_scale = A_DH ** (-0.5) * LOG2E

    w_hbm = (wq_hbm, wk_hbm, wv_hbm)
    wo32 = wo_hbm.bitcast(U32)
    awo32 = awo_hbm.bitcast(U32)
    hw = PW // 2
    hd = B_H * B_DH

    def w_copy(p, half, q, m, sem):
        rows = pl.ds(pl.multiple_of(p * PW, PW), PW)
        return pltpu.make_async_copy(w_hbm[m].at[rows, :], stage.at[half, q, m], sem)

    def wa_piece(g, q):
        last = g >= 2 * 3
        return jnp.where(last, 1 + q, g >> 1), jnp.where(last, NT - 1, (g & 1) + 2 * q)

    def wa_copy(c, kt, half, q, sem):
        return pltpu.make_async_copy(
            awqkv_hbm.at[pl.ds(pl.multiple_of(kt * 128, 128), 128),
                         pl.ds(pl.multiple_of(c * D, 128), D)],
            stage.at[half, q, 3, :128], sem)

    def start_trip(g):
        half = g & 1
        src = jnp.minimum(g, NTRIP - 1)
        for q in range(PP):
            for m in range(3):
                w_copy((src + 1) * PP + q, half, q, m, sems.at[half]).start(priority=1)
            wa_copy(*wa_piece(src, q), half, q, sems.at[half]).start(priority=1)

    def wait_trip(half):
        for view in (stage.at[half, :, :3], stage.at[half, :, 3, :128]):
            pltpu.make_async_copy(view, view, sems.at[half]).wait()

    qr = 2 * hw

    def wo_copy(start, n, sem):
        wr = pl.ds(pl.multiple_of(start, 8), n)
        return pltpu.make_async_copy(wo32.at[wr, :], wo_s.at[wr, :], sem)

    def wo_sums(q, piece, anchor=None, never=None):
        def blk(k, n):
            w = wo_s[pl.ds(pl.multiple_of(q * qr + k * hw + piece * WX_ROWS, 8), WX_ROWS),
                     n * KH:(n + 1) * KH]
            if anchor is not None:
                w = jnp.where(never, anchor, w)
            return _unpack(w).astype(F32)

        b11, b12, b21, b22 = blk(0, 0), blk(0, 1), blk(1, 0), blk(1, 1)
        for n, v in enumerate((b11 + b22, b12 - b22, b21 - b11, b11 + b12, b21 + b22)):
            wx_s[q, n, pl.ds(pl.multiple_of(piece * WX_ROWS, 8), WX_ROWS), :] = (
                _pack(v.astype(BF16)))

    def x_copies(xr, sem):
        return [pltpu.make_async_copy(ax_hbm.at[xr, :], xa_s.at[xr, :D], sem),
                pltpu.make_async_copy(bx_hbm.at[xr, :], xb_s.at[xr, :D], sem)]

    xpre_cp = pltpu.make_async_copy(bx4_hbm.at[:, 0], xpre_s, sems.at[3])
    late_cps = ([pltpu.make_async_copy(mem0_hbm, mem0_s, sems.at[2])]
                + x_copies(pl.ds(0, X_HEAD), sems.at[2]))
    awo_cps = [
        pltpu.make_async_copy(awo32.at[:, c * 128:(c + 1) * 128], awo_raw.at[c], sems.at[2])
        for c in range(NT)]
    x_rest = x_copies(pl.ds(X_HEAD, S - X_HEAD), sems.at[3])
    tiles = [(m, j) for m in range(3) for j in range(PW // 128)]
    peel = [tiles[sum(PEEL[:n]):sum(PEEL[:n + 1])] for n in range(len(PEEL))]
    peel_cps = [[pltpu.make_async_copy(w_hbm[m].at[pl.ds(q * PW + j * 128, 128), :],
                                       stage.at[1, q, m, pl.ds(j * 128, 128), :], sems.at[4 + n])
                 for m, j in blk for q in range(PP)] for n, blk in enumerate(peel)]
    peel_cps[-1].append(wa_copy(0, NT - 1, 1, 0, sems.at[3 + len(PEEL)]))

    xpre_cp.start()
    for cps in peel_cps:
        for cp in cps:
            cp.start(priority=1)
    start_trip(0)
    for cp in late_cps:
        cp.start(priority=1)
    kv_s[:, :, :A_HALO, :] = jnp.zeros((2, NT, A_HALO, 128), F32)
    wo_s[NQ * qr:, :] = jnp.zeros((qr, D), U32)

    def gather_heads(ref):
        rows = []
        for j in range(A_DH // 2):
            u = ref[pl.ds(j, A_H, stride=A_DH // 2), :]
            rows.append(pltpu.bitcast(u << 16, F32))
            rows.append(pltpu.bitcast(u & jnp.uint32(0xFFFF0000), F32))
        return jnp.concatenate(rows, axis=0)

    HR = NSEG * PRE // 2

    def xq(i, k):
        return _unpack(xp_s[i * HR // 2:(i + 1) * HR // 2, k * KH:(k + 1) * KH])

    def strassen_lhs():
        f = lambda i, k: xq(i, k).astype(F32)
        sums = (f(0, 0) + f(1, 1), f(1, 0) + f(1, 1), f(0, 0) + f(0, 1),
                f(1, 0) - f(0, 0), f(0, 1) - f(1, 1))
        for n, v in enumerate(sums):
            xs_s[n] = _pack(v.astype(BF16))

    def pair_prep2(p, half, m, js=(0, 1, 2), hook=None):
        if SKIP_PROLOGUE:
            return
        for q in range(2):
            lo, hi = js[0] * 128, (js[-1] + 1) * 128
            w_s[p + q, :, m * PW + lo:m * PW + hi] = _pack(stage[half, q, m, lo:hi, :].T)
        nseg = ST_ROWS // PRE
        for j in js:
            rows = slice(j * 128, (j + 1) * 128)
            b = lambda k, q: stage[half, q, m, rows, k * KH:(k + 1) * KH]
            bf = lambda k, q: b(k, q).astype(F32)
            rhs = ((bf(0, 0) + bf(1, 1)).astype(BF16), b(0, 0),
                   (bf(0, 1) - bf(1, 1)).astype(BF16), (bf(1, 0) - bf(0, 0)).astype(BF16),
                   b(1, 1), (bf(0, 0) + bf(0, 1)).astype(BF16),
                   (bf(1, 0) + bf(1, 1)).astype(BF16))
            tail = [stage[half, q, m, rows, 2 * KH:] for q in range(2)]
            for c in range(HR // ST_ROWS):
                r = slice(c * ST_ROWS // 2, (c + 1) * ST_ROWS // 2)
                sm = lambda n: _unpack(xs_s[n, r, :])
                qd = lambda i, k: _unpack(
                    xp_s[(i * HR + c * ST_ROWS) // 2:(i * HR + (c + 1) * ST_ROWS) // 2,
                         k * KH:(k + 1) * KH])
                rest = lambda i: _unpack(
                    xp_s[(i * HR + c * ST_ROWS) // 2:(i * HR + (c + 1) * ST_ROWS) // 2, 2 * KH:])

                def put(i, q, v):
                    s0 = i * (NSEG // 2) + c * nseg
                    pre_s[s0:s0 + nseg, p + q, :, m * PW + j * 128:m * PW + (j + 1) * 128] = (
                        v.reshape(nseg, PRE, 128))
                    if hook is not None:
                        hook(v)

                m5 = _nt_dot(sm(2), rhs[4])
                m3 = _nt_dot(qd(0, 0), rhs[2])
                put(0, 1, _nt_dot(rest(0), tail[1]) + m3 + m5)
                m1 = _nt_dot(sm(0), rhs[0])
                m4 = _nt_dot(qd(1, 1), rhs[3])
                put(0, 0, _nt_dot(rest(0), tail[0]) + _nt_dot(sm(4), rhs[6]) + (m1 + m4 - m5))
                m2 = _nt_dot(sm(1), rhs[1])
                put(1, 0, _nt_dot(rest(1), tail[0]) + m2 + m4)
                put(1, 1, _nt_dot(rest(1), tail[1]) + _nt_dot(sm(3), rhs[5]) + (m1 - m2 + m3))

    def wa_prep(c, kt, half, q):
        t1_s[q] = _pack(stage[half, q, 3, :128].T)
        g = gather_heads(t1_s.at[q])
        wa_s[c, pl.ds(pl.multiple_of(kt * 64, 64), 64), :] = _pack(g.astype(BF16).T)
        return g

    def wa_trip(g, half):
        lo, hi = [wa_prep(*wa_piece(g, q), half, q) for q in range(2)]
        for t in range(2):
            b11, b12 = lo[2 * t * 128:(2 * t + 1) * 128], lo[(2 * t + 1) * 128:(2 * t + 2) * 128]
            b21, b22 = hi[2 * t * 128:(2 * t + 1) * 128], hi[(2 * t + 1) * 128:(2 * t + 2) * 128]
            sums = cat([b11 + b22, b12 - b22, b21 - b11, b11 + b12, b21 + b22])
            wc_s[g, t] = _pack(sums.astype(BF16).T)

    xpre_cp.wait()
    xp_s[...] = _pack(xpre_s[...].reshape(NSEG * PRE, D))
    strassen_lhs()
    for blk, cps in zip(peel, peel_cps):
        for cp in cps:
            cp.wait()
        for m in range(3):
            js = tuple(j for mm, j in blk if mm == m)
            if js:
                pair_prep2(0, 1, m, js)
    wa_prep(0, NT - 1, 1, 0)

    def prologue(g, carry):
        half = g & 1

        @pl.when(g > 0)
        def _():
            wo_copy((g - 1) * WO_ROWS, WO_ROWS, sems.at[8]).wait()

        @pl.when(g == NTRIP - 1)
        def _():
            for cp in awo_cps:
                cp.start(priority=1)

        @pl.when(g < NTRIP - 1)
        def _():
            wo_copy(g * WO_ROWS, WO_ROWS, sems.at[8]).start()

        start_trip(g + 1)
        wait_trip(half)
        calls = [0]
        per = hw // WX_ROWS
        total = max(b - a for a, b in zip(WX_DONE, WX_DONE[1:]))
        todo = list(range(total))
        first, stop = NQ * per, (NQ + 1) * per
        for trip in range(1, NTRIP):
            first = jnp.where(g == trip, WX_DONE[trip - 1], first)
            stop = jnp.where(g == trip, WX_DONE[trip], stop)

        def hook(v):
            calls[0] += 1
            want = (calls[0] - WX_SKIP) * total // (36 - WX_SKIP - WX_TAIL)
            t = 0
            while todo and todo[0] < want:
                k = jnp.minimum(first + todo.pop(0), stop - 1)
                q = k // per
                anchor = jnp.concatenate(
                    [v[(2 * t + c) * WX_ROWS:(2 * t + c + 1) * WX_ROWS] for c in range(2)], axis=1)
                wo_sums(q, k % per, pltpu.bitcast(anchor, U32), g > NSEG)
                t += 1

        for m in range(3):
            pair_prep2((g + 1) * PP, half, m, hook=hook)
            if m == 0:
                wa_trip(g, half)
        return carry

    lax.fori_loop(0, NTRIP, prologue, 0)

    for cp in late_cps + awo_cps:
        cp.wait()
    for cp in x_rest:
        cp.start()

    for c in range(NT):
        awo_s[:, c * 128:(c + 1) * 128] = _pack(gather_heads(awo_raw.at[c]).astype(BF16))

    def out_copy(row, n, half):
        r = pl.ds(row, n)
        c = slice(half * D, (half + 1) * D)
        return pltpu.make_async_copy(out_s.at[r, c], out_hbm.at[r, c], sems.at[7])

    def segment(s, mem, u):
        last = u == SPT - 1
        row0 = pl.multiple_of(s * SEG, SEG)
        ninf = jnp.float32(-jnp.inf)

        qi = lax.broadcasted_iota(jnp.int32, (SEG, 128), 0)
        kl = lax.broadcasted_iota(jnp.int32, (SEG, 128), 1)
        is_a = kl < L
        real = kl < 2 * L
        kpos = jnp.where(is_a, kl, kl - L)
        allowed = ((qi >= FRESH) | (qi + MEM + PRE >= kpos)) & real
        fill = jnp.where(real, NEG, ninf)
        pi = lax.broadcasted_iota(jnp.int32, (GP * PRE, 128), 0)
        pk = lax.broadcasted_iota(jnp.int32, (GP * PRE, 128), 1)
        p_own = (pk // SEG) == (pi // PRE)
        p_allowed = (pk % (MEM + PRE)) <= (pi % PRE) + MEM
        p_first = (pk % SEG) < MEM + PRE
        p_allowed = p_allowed & p_own
        p_fill = jnp.where(p_own, NEG, ninf)
        col_a = lax.broadcasted_iota(jnp.int32, (1, PW), 1) < B_DH
        col128_a = lax.broadcasted_iota(jnp.int32, (1, 128), 1) < (B_DH - 128)

        xb = xb_s[pl.ds(row0, SEG), :D].astype(F32)
        h = jnp.concatenate([xb[PRE:], mem], axis=0).astype(BF16)

        def proj(p, m):
            return _dot(h, _unpack(w_s[p, :, m * PW:(m + 1) * PW]))

        def pre(p, m):
            return pre_s[s, p, :, m * PW:(m + 1) * PW]

        def block_diag(p, m):
            f = proj(p, m)
            full = jnp.concatenate([f[FRESH:], pre(p, m), f[:FRESH]], axis=0)
            z = jnp.zeros_like(full)
            return jnp.where(col_a, full, z), jnp.where(col_a, z, full)

        def keys_t(blocks):
            fold = cat([jnp.concatenate([x[:, :128] if i % 2 == 0 else x[:, 256:], x[:, 128:256]],
                                        axis=1) for i, x in enumerate(blocks)])
            t = fold.T
            if t.shape[1] < 128:
                t = jnp.concatenate([t, jnp.zeros((256, 128 - t.shape[1]), F32)], axis=1)
            outer = t[:128]
            n = blocks[0].shape[0]
            lane = lax.broadcasted_iota(jnp.int32, outer.shape, 1)
            lane_a = lane < n if len(blocks) == 2 else lane % (2 * n) < n
            z = jnp.zeros_like(outer)
            kt = cat([jnp.where(lane_a, outer, z), t[128:], jnp.where(lane_a, z, outer)])
            return kt.astype(BF16)

        def row_max(raw, ok, other, first):
            sc = jnp.where(ok, raw * b_scale, other)
            ma = jnp.max(jnp.where(first, sc, ninf), axis=1, keepdims=True)
            mb = jnp.max(jnp.where(first, ninf, sc), axis=1, keepdims=True)
            return sc, ma, mb

        def probs(mx, first, late_norm):
            sc, ma, mb = mx
            e = jnp.exp2(sc - jnp.where(first, ma, mb))
            sa = jnp.sum(jnp.where(first, e, 0.0), axis=1, keepdims=True)
            sb = jnp.sum(jnp.where(first, 0.0, e), axis=1, keepdims=True)
            if late_norm:
                return e.astype(BF16), _recip(sa), _recip(sb)
            return (e * _recip(jnp.where(first, sa, sb))).astype(BF16), None, None

        def pv(sm, vbd):
            e, ra, rb = sm
            o = _dot(e, cat(list(vbd) + [jnp.zeros((128 - 2 * L, PW), F32)]).astype(BF16))
            if ra is not None:
                o = jnp.concatenate([
                    o[:, :128] * ra,
                    o[:, 128:256] * jnp.where(col128_a, ra, rb),
                    o[:, 256:] * rb], axis=1)
            return o

        def pre_pv(g, pr, vbds):
            v = cat([x[:MEM + PRE] for vb in vbds for x in vb])
            o = _dot(pr, v.astype(BF16))
            if not last:
                odef_s[u, g] = o
            return o

        def wout(p, o, acc):
            contrib = _dot(o.astype(BF16), _unpack(wo_s[p * hw:(p + 1) * hw, :]))
            return contrib if acc is None else acc + contrib

        def deferred(p):
            r = slice((p % GP) * PRE, (p % GP + 1) * PRE)
            return cat([odef_s[v, p // GP, r, :] for v in range(SPT - 1)]
                       + [val["PPV", p // GP][r]])

        def wout_strassen(kind, q):
            a11, a21 = val["PV", 2 * q], deferred(2 * q)
            if kind != "XA":
                a12, a22 = val["PV", 2 * q + 1], deferred(2 * q + 1)
            blk = lambda k, n: _unpack(
                wo_s[q * qr + k * hw:q * qr + (k + 1) * hw, n * KH:(n + 1) * KH])
            sm = lambda n: _unpack(wx_s[q, n])
            if kind == "XA":
                terms = {3: (a11, sm(1)), 6: (a21 - a11, sm(3))}
            elif kind == "XB":
                terms = {1: (a11 + a22, sm(0)), 4: (a22, sm(2)), 5: (a11 + a12, blk(1, 1)),
                         7: (a12 - a22, sm(4))}
            elif kind == "XC":
                terms = {2: (a21 + a22, blk(0, 0))}
            else:
                lhs = jnp.concatenate([cat([a11, a21]), cat([a12, a22])], axis=1)
                terms = {0: (lhs, _unpack(wo_s[q * qr:(q + 1) * qr, 2 * KH:]))}
            for n, (x, w) in terms.items():
                r = _dot(x.astype(BF16), w)
                val["acc", n] = val["acc", n] + r if ("acc", n) in val else r

        arow0 = pl.multiple_of((s - u % 2) * SEG, 2 * SEG)

        def a_put(m, j, r):
            if m == 0:
                qa_s[j] = r * a_scale
            else:
                kv_s[m - 1, j, A_HALO:A_HALO + 2 * SEG, :] = r

        def a_proj(idx):
            m, t = divmod(idx, 3)
            if "xa" not in val:
                xa = xa_s[pl.ds(arow0, 2 * SEG), :D]
                xf = xa.astype(F32)
                f = lambda i, k: xf[i * SEG:(i + 1) * SEG, k * KH:(k + 1) * KH]
                val["xa"] = xa
                val["xs"] = [v.astype(BF16) for v in (
                    f(0, 0) + f(1, 1), f(1, 0) + f(1, 1), f(0, 0), f(1, 1), f(0, 0) + f(0, 1),
                    f(1, 0) - f(0, 0), f(0, 1) - f(1, 1))]
                val["xr"] = xf[:, 2 * KH:].astype(BF16)
            if t == 2:
                a_put(m, NT - 1, _dot(val["xa"], _unpack(wa_s[m, :, (NT - 1) * 128:])))
                return
            sm = lambda n: _unpack(cat([wc_s[2 * m + k, t, :, n * 128:(n + 1) * 128]
                                        for k in range(2)]))
            blk = lambda k, j: _unpack(wa_s[m, k * KH // 2:(k + 1) * KH // 2,
                                            (2 * t + j) * 128:(2 * t + j + 1) * 128])
            rhs = (sm(0), blk(0, 0), sm(1), sm(2), blk(1, 1), sm(3), sm(4))
            mm = lambda n: _dot(val["xs"][n], rhs[n])
            tail = [_dot(val["xr"], _unpack(wa_s[m, KH:, (2 * t + j) * 128:(2 * t + j + 1) * 128]))
                    for j in range(2)]
            m1, m2, m3, m4, m5 = [mm(n) for n in range(5)]
            a_put(m, 2 * t, tail[0] + cat([mm(6) + (m1 + m4 - m5), m2 + m4]))
            a_put(m, 2 * t + 1, tail[1] + cat([m3 + m5, mm(5) + (m1 - m2 + m3)]))

        def window(m, j, w, hf):
            lo = A_HALO + hf * SEG - A_DIL * w
            return kv_s[m, j, lo:lo + SEG, :]

        def local_softmax(hf):
            pos = arow0 + hf * SEG + lax.broadcasted_iota(jnp.int32, (SEG, 128), 0)
            rows = slice(hf * SEG, (hf + 1) * SEG)
            logits = []
            for w in range(A_W):
                t = qa_s[0, rows, :] * window(0, 0, w, hf)
                for j in range(1, NT):
                    t = t + qa_s[j, rows, :] * window(0, j, w, hf)
                t = t + pltpu.roll(t, 64, 1)
                t = t + pltpu.roll(t, 32, 1)
                if w > 0 and hf == 0:
                    t = jnp.where(pos >= A_DIL * w, t, NEG)
                logits.append(t)
            mx = functools.reduce(jnp.maximum, logits)
            es = [jnp.exp2(l - mx) for l in logits]
            inv = _recip(functools.reduce(lambda x, y: x + y, es))
            return es, inv

        def local_pv(j, hf):
            es, inv = val["LA", hf]
            o = es[0] * window(1, j, 0, hf)
            for w in range(1, A_W):
                o = o + es[w] * window(1, j, w, hf)
            return o * inv

        def local_out(j, acc):
            wj = _unpack(awo_s[j * 64:(j + 1) * 64, :])
            if ("AX", j) in val:
                r = cat([val["AX", j], _dot(local_pv(j, 1).astype(BF16), wj)])
            else:
                r = _dot(cat([local_pv(j, 0), local_pv(j, 1)]).astype(BF16), wj)
            for m in range(2):
                kv_s[m, j, :A_HALO, :] = kv_s[m, j, 2 * SEG:2 * SEG + A_HALO, :]
            return r if acc is None else acc + r

        val = {}
        acc = None
        oa = None
        for kind, t in _order(u):
            if kind == "K":
                val[kind, t] = block_diag(t, 1)
            elif kind == "V":
                val[kind, t] = block_diag(t, 2)
            elif kind == "Q":
                val[kind, t] = proj(t, 0).astype(BF16)
            elif kind == "T":
                val[kind, t] = keys_t(val["K", t])
            elif kind == "S":
                val[kind, t] = _dot(val["Q", t], val["T", t])
            elif kind == "M":
                val[kind, t] = row_max(val["S", t], allowed, fill, is_a)
            elif kind == "E":
                val[kind, t] = probs(val["M", t], is_a, t >= LATE_FROM)
            elif kind == "PV":
                val[kind, t] = pv(val["E", t], val["V", t])
            elif kind == "TG":
                val[kind, t] = keys_t([x[:MEM + PRE] for r in range(GP)
                                       for x in val["K", GP * t + r]])
            elif kind == "PS":
                q = cat([pre(GP * t + r, 0) for r in range(GP)]).astype(BF16)
                val[kind, t] = _dot(q, val["TG", t])
            elif kind == "MG":
                val[kind, t] = row_max(val["PS", t], p_allowed, p_fill, p_first)
            elif kind == "EG":
                val[kind, t] = probs(val["MG", t], p_first, False)[0]
            elif kind == "PPV":
                val[kind, t] = pre_pv(t, val["EG", t], [val["V", GP * t + r] for r in range(GP)])
            elif kind == "W":
                acc = wout(t, val["PV", t], acc)
            elif kind in ("XA", "XB", "XC", "Y"):
                wout_strassen(kind, t)
            elif kind == "LA":
                val[kind, t] = local_softmax(t)
            elif kind == "AP":
                a_proj(t)
            elif kind == "AX":
                val[kind, t] = _dot(local_pv(t, 0).astype(BF16),
                                    _unpack(awo_s[t * 64:(t + 1) * 64, :]))
            elif kind == "AO":
                oa = local_out(t, oa)
                if t == NT - 1:
                    out_s[pl.ds(arow0, 2 * SEG), :D] = oa.astype(BF16)
                    out_copy(arow0, 2 * SEG, 0).start()
        if last:
            m = lambda n: val["acc", n]
            acc = jnp.concatenate([
                cat([m(1) + m(4) - m(5) + m(7), m(2) + m(4)]),
                cat([m(3) + m(5), m(1) - m(2) + m(3) + m(6)]), m(0)], axis=1)
        return acc

    def steps(i, mem):
        @pl.when(i == 1)
        def _():
            for cp in x_rest:
                cp.wait()

        accs = []
        for u in range(SPT):
            accs.append(segment(i * SPT + u, mem, u))
            mem = accs[-1][FRESH:SEG]
        res = cat([x for u in range(SPT) for x in (
            accs[-1][SEG + u * PRE:SEG + (u + 1) * PRE], accs[u][:FRESH])])
        row = pl.multiple_of(i * SPT * SEG, SPT * SEG)
        out_s[pl.ds(row, SPT * SEG), D:2 * D] = res.astype(BF16)
        out_copy(row, SPT * SEG, 1).start()
        return mem

    lax.fori_loop(0, N_STEPS, steps, mem0_s[...].astype(F32))

    wait_trip(NTRIP % 2)

    done = N_STEPS * SPT * SEG
    pltpu.make_async_copy(out_s.at[:done, :2 * D], out_hbm.at[:done, :], sems.at[7]).wait()


@jax.jit
def pallas_concat_heads__sliding_local_dilated__memory_aug_recurrent_mem_tr__prompt_kernel(
    A_x: jax.Array,
    A_wqkv: jax.Array,
    A_wo: jax.Array,
    B_x: jax.Array,
    B_mem0: jax.Array,
    B_Wq: jax.Array,
    B_Wk: jax.Array,
    B_Wv: jax.Array,
    B_Wo: jax.Array,
    B_seg_len,
):
    del B_seg_len
    assert A_x.shape == (1, S, D) and B_x.shape == (1, S, D)
    hd = B_H * B_DH
    wq_t = jnp.transpose(B_Wq, (1, 2, 0)).reshape(hd, D)
    wk_t = jnp.transpose(B_Wk, (1, 2, 0)).reshape(hd, D)
    wv_t = jnp.transpose(B_Wv, (1, 2, 0)).reshape(hd, D)
    wo = B_Wo.reshape(hd, D)

    any_spec = pl.BlockSpec(memory_space=pl.ANY)
    out = pl.pallas_call(
        _kernel,
        out_shape=jax.ShapeDtypeStruct((S, 2 * D), BF16),
        in_specs=[any_spec] * 10,
        out_specs=any_spec,
        scratch_shapes=[
            pltpu.VMEM((2, PP, 4, PW, D), BF16),
            pltpu.VMEM((NT, D // 2, 128), U32),
            pltpu.VMEM((NP, D // 2, 3 * PW), U32),
            pltpu.VMEM((hd // 2 + PW, D), U32),
            pltpu.VMEM((NQ + 1, 5, PW // 2, KH), U32),
            pltpu.VMEM((NSEG, NP, PRE, 3 * PW), F32),
            pltpu.VMEM((SPT - 1, NG, GP * PRE, PW), F32),
            pltpu.VMEM((S, OUT_W), BF16),
            pltpu.VMEM((S, X_W), BF16),
            pltpu.VMEM((S, X_W), BF16),
            pltpu.VMEM((NSEG, PRE, D), BF16),
            pltpu.VMEM((NSEG * PRE // 2, D), U32),
            pltpu.VMEM((5, NSEG * PRE // 4, 256), U32),
            pltpu.VMEM((MEM, D), BF16),
            pltpu.VMEM((3, D // 2, D), U32),
            pltpu.VMEM((NTRIP, 2, 64, D), U32),
            pltpu.VMEM((D // 2, D), U32),
            pltpu.VMEM((PP, D // 2, 128), U32),
            pltpu.VMEM((NT, 2 * SEG, 128), F32),
            pltpu.VMEM((2, NT, KV_ROWS, 128), F32),
            pltpu.SemaphoreType.DMA((9,)),
        ],
        compiler_params=pltpu.CompilerParams(vmem_limit_bytes=120 * 1024 * 1024,
                                             disable_bounds_checks=True),
    )(A_x.reshape(S, D), A_wqkv, A_wo, B_x.reshape(S, D), B_x.reshape(NSEG, SEG // PRE, PRE, D),
      B_mem0.reshape(MEM, D), wq_t, wk_t, wv_t, wo)
    return out.reshape(1, S, 2 * D)
```

```python
import functools

import jax
import jax.numpy as jnp
from jax import lax
import jax.experimental.pallas as pl
import jax.experimental.pallas.tpu as pltpu

F32 = jnp.float32
BF16 = jnp.bfloat16
U32 = jnp.uint32

S = 2048
D = 640
NT = D // 128
A_H = 32
A_DH = D // A_H
A_W = 8
A_DIL = 2
A_HALO = 16
B_H = 32
B_DH = 192
MEM = 8
SEG = 32
NSEG = S // SEG
NP = B_H // 2
PW = 2 * B_DH
PRE = 8
FRESH = SEG - PRE
L = MEM + SEG
GP = 4
NG = NP // GP
LOG2E = 1.4426950408889634
NEG = -1000000000.0 * LOG2E
PP = 2
NTRIP = NP // PP - 1
PEEL = (2, 2, 5)
KH = 256
WO_ROWS = 512
WX_DONE = (0, 24, 56, 96, 120, 152, 192)
WX_TAIL = 2
WX_ROWS = 8
WX_SKIP = 0
ST_ROWS = 256
X_HEAD = 128
KV_ROWS = 80
X_W = 1024
OUT_W = 2048
SPT = 4
N_STEPS = NSEG // SPT
NQ = NP // 2

LAT_MM, LAT_X, LAT_T, LAT_N, LAT_N_LATE = 190, 190, 380, 230, 100
LATE_FROM = NP - 2
AP_AFTER = (6, 16, 26)
AO_AFTER = (30, 40)
TAIL_FILL = (2, 2, 2, 0)
HOLD_W = (0, 3, 0, 0)


def _segment_order(u):
    odd, last = u % 2 == 1, u == SPT - 1
    proj = []
    for g in range(NG):
        proj += [("K", GP * g + r) for r in range(GP)]
        for r in range(GP):
            proj += [("V", GP * g + r), ("Q", GP * g + r)]
    dur = {"K": 120, "V": 120, "Q": 120, "S": 24, "PV": 24, "PS": 24, "PPV": 24,
           "W": 120, "XA": 96, "XB": 192, "XC": 48, "Y": 96, "AO": 80, "AP": 125,
           "T": 0, "M": 0, "E": 0, "TG": 0, "MG": 0, "EG": 0}
    end = {}

    def ready(task):
        k, i = task
        if k == "T":
            deps = [(("K", i), LAT_MM)]
        elif k == "S":
            deps = [(("Q", i), LAT_MM), (("T", i), LAT_T)]
        elif k == "M":
            deps = [(("S", i), LAT_MM - 40)]
        elif k == "E":
            deps = [(("M", i), LAT_X)]
        elif k == "PV":
            deps = [(("E", i), LAT_N_LATE if i >= LATE_FROM else LAT_N), (("V", i), LAT_MM)]
        elif k == "TG":
            deps = [(("K", GP * i + r), LAT_MM) for r in range(GP)]
        elif k == "PS":
            deps = [(("TG", i), LAT_T)]
        elif k == "MG":
            deps = [(("PS", i), LAT_MM - 40)]
        elif k == "EG":
            deps = [(("MG", i), LAT_X)]
        elif k == "PPV":
            deps = [(("EG", i), LAT_N), (("V", GP * i + GP - 1), LAT_MM)]
        elif k == "W":
            deps = [(("PV", i), LAT_MM)]
        else:
            deps = [(("PV", 2 * i), LAT_MM), (("PPV", 2 * i // GP), LAT_MM)]
            if k != "XA":
                deps.append((("PV", 2 * i + 1), LAT_MM))
        if any(d not in end for d, _ in deps):
            return None
        return max(end[d] + lat for d, lat in deps)

    pend = ([(k, p) for k in ("E", "M", "T") for p in range(NP)]
            + [(k, g) for k in ("EG", "MG", "TG") for g in range(NG)]
            + ([(k, q) for q in range(NQ) for k in ("XA", "XB", "Y", "XC")] if last
               else [("W", p) for p in range(NP)])
            + [("PPV", g) for g in range(NG)]
            + [("PV", p) for p in range(NP)] + [("PS", g) for g in range(NG)]
            + [("S", p) for p in range(NP)])
    fill = [("AO", j) for j in range(NT)] if odd else [("AP", j) for j in (3, 4, 5, 0, 1, 2, 6, 7, 8)]
    order = []
    now = [0]

    def emit(task):
        order.append(task)
        now[0] += dur[task[0]]
        end[task] = now[0]

    nproj = 0
    while pend:
        cand = [x for x in pend if ready(x) is not None and ready(x) <= now[0]]
        if proj:
            cand = [x for x in cand if not (x[0] == "W" and x[1] >= NP - GP - HOLD_W[u])]
        if cand:
            if not proj:
                cand = [x for x in cand if x[0] not in ("W", "XA", "XB", "XC", "Y")] or cand
            pend.remove(cand[0])
            emit(cand[0])
        elif proj:
            emit(proj.pop(0))
            nproj += 1
            if odd and nproj == GP:
                order += [("LA", 0), ("LA", 1)]
            if nproj in (AO_AFTER if odd else AP_AFTER):
                emit(fill.pop(0))
        elif len(fill) > TAIL_FILL[u]:
            emit(fill.pop(0))
        else:
            now[0] = min(ready(x) for x in pend if ready(x) is not None)
    return order + fill


ORDERS = (
    "K0 T0 K1 K2 K3 V0 T1 T2 Q1 T3 Q0 AP3 S0 TG0 M0 PS0 V1 Q2 V2 V3 E0 MG0 S1 S2 M1 K4 Q3 EG0 PV0 "
    "K5 E1 M2 S3 K6 T4 W0 E2 M3 T5 PPV0 PV1 K7 AP4 E3 T6 W1 T7 TG1 PV2 PV3 Q4 W2 V4 W3 PS1 S4 Q5 "
    "V5 M4 MG1 V6 Q7 Q6 E4 S5 EG1 V7 M5 PV4 S6 K8 PPV1 E5 S7 M6 W4 K9 E6 M7 T8 K10 PV5 AP5 T9 K11 "
    "E7 W5 T10 PV6 TG2 V8 T11 PV7 Q8 W7 W6 S8 PS2 V10 V9 Q9 M8 MG2 Q10 E8 EG2 V11 S9 Q11 M9 PV8 "
    "S10 K12 T12 PPV2 E9 S11 M10 W8 E10 M11 PV9 K14 K13 K15 E11 T13 W9 PV10 V12 T14 T15 TG3 PV11 "
    "Q12 W10 W11 PS3 S12 Q13 V13 M12 MG3 V15 V14 E12 Q14 EG3 Q15 S13 M13 PV12 S14 AP0 PPV3 E13 "
    "S15 M14 W12 AP1 E14 PV13 M15 AP2 AP6 PV14 W13 E15 PV15 W14 W15 AP8 AP7 ",
    "K0 K1 K2 T0 K3 LA0 LA1 Q0 V1 T1 V0 T2 T3 TG0 Q1 S0 V2 PS0 Q2 M0 S1 V3 MG0 Q3 M1 S2 K4 EG0 K5 "
    "E0 E1 M2 PV0 S3 K6 T4 PPV0 E2 T5 K7 M3 W0 T6 PV1 PV2 V4 E3 T7 TG1 Q4 W1 W2 PV3 PS1 S4 V5 Q5 "
    "M4 MG1 W3 AO0 S5 V6 E4 EG1 Q6 M5 V7 PV4 Q7 E5 S6 K8 W4 M6 PPV1 PV5 S7 T8 K9 E6 K10 M7 W5 T9 "
    "PV6 K11 E7 T10 V8 W6 T11 TG2 PV7 Q8 AO1 W7 S8 V9 PS2 Q9 M8 V10 MG2 Q10 E8 S9 V11 EG2 Q11 PV8 "
    "M9 S10 K12 PPV2 E9 S11 M10 K13 W8 E10 M11 T12 PV9 K14 K15 E11 T13 T14 PV10 AO2 V12 T15 TG3 "
    "Q12 PV11 V13 Q13 PS3 S12 V14 Q14 M12 S13 MG3 V15 Q15 E12 M13 EG3 S14 W9 E13 M14 PPV3 W10 "
    "PV12 S15 W11 E14 M15 PV13 W12 PV14 E15 W13 PV15 W14 W15 AO3 AO4 ",
    "K0 K2 K1 T0 K3 T1 AP3 V0 Q0 TG0 T3 T2 V1 S0 Q1 PS0 Q2 V2 M0 S1 V3 E0 MG0 Q3 M1 K4 S2 EG0 PV0 "
    "K5 E1 M2 PPV0 S3 K6 T4 W0 E2 M3 T5 AP4 PV1 K7 E3 W1 T6 T7 TG1 PV2 V4 PV3 Q4 W2 W3 PS1 S4 V5 "
    "M4 Q5 MG1 V6 S5 Q6 EG1 E4 V7 Q7 M5 PV4 S6 K8 PPV1 E5 S7 M6 W4 AP5 K9 E6 M7 T8 PV5 K10 T9 K11 "
    "E7 W5 T10 PV6 V8 T11 TG2 PV7 Q8 W6 W7 S8 PS2 V9 Q9 M8 MG2 V10 Q10 E8 EG2 S9 V11 Q11 M9 PV8 "
    "S10 K12 PPV2 E9 W8 S11 M10 K13 E10 M11 T12 PV9 K14 K15 E11 T13 W9 PV11 T14 PV10 V12 T15 TG3 "
    "Q12 W10 V13 W11 PS3 S12 MG3 Q13 M12 V14 Q14 E12 EG3 S13 V15 Q15 M13 PV12 S14 E13 AP0 PPV3 "
    "S15 M14 AP1 W12 M15 AP2 E14 PV13 PV14 AP6 E15 W13 PV15 W14 W15 AP7 AP8 ",
    "K1 K0 K2 T0 K3 LA0 LA1 T1 V0 T2 Q0 T3 TG0 V1 Q1 S0 PS0 V2 Q2 M0 V3 MG0 Q3 S1 E0 M1 S2 EG0 K4 "
    "K5 M2 T4 PV0 E1 AO0 PPV0 S3 K6 E2 T5 K7 M3 XA0 T6 PV1 PV2 V4 E3 T7 TG1 Y0 Q4 XB0 XC0 XA1 PV3 "
    "PS1 S4 V5 Q5 M4 MG1 XB1 E4 Y1 XC1 EG1 S5 Q6 V6 M5 V7 S6 PV4 AO1 Q7 E5 PPV1 K8 S7 M6 XA2 K9 "
    "M7 T8 PV5 K10 E6 T9 XB2 E7 T10 Y2 K11 TG2 T11 XC2 PV6 PV7 V8 Q8 XA3 XB3 Y3 PS2 S8 V9 Q9 M8 "
    "MG2 V10 Q10 AO2 E8 EG2 S9 V11 S10 M9 PV8 K12 Q11 M10 PPV2 K13 E9 K14 S11 E10 T12 M11 T13 K15 "
    "PV9 XA4 T14 PV10 V12 E11 XB4 T15 TG3 XA5 Y4 Q12 AO3 PV11 XB5 PS3 S12 V13 Q13 MG3 V14 M12 Q14 "
    "EG3 S13 V15 E12 M13 PV12 Q15 S14 AO4 PPV3 E13 S15 M14 E14 XA6 M15 XC3 XC4 XC5 PV13 E15 Y5 "
    "PV14 XB6 PV15 XC6 Y6 XA7 XB7 Y7 XC7 ",
)
SKIP_PROLOGUE = False
PVFOLD = False


def _order(u):
    if ORDERS is None or ORDERS[u] is None:
        return _segment_order(u)
    return [(t.rstrip("0123456789"), int(t.lstrip("ABCDEFGHIJKLMNOPQRSTUVWXYZ")))
            for t in ORDERS[u].split()]


def _nt_dot(a, b):
    return lax.dot_general(a, b, (((1,), (1,)), ((), ())), preferred_element_type=F32)


def _dot(a, b):
    return jnp.dot(a, b, preferred_element_type=F32)


def _pack(x):
    return pltpu.bitcast(x, U32)


def _unpack(x):
    return pltpu.bitcast(x, BF16)


def cat(parts):
    return jnp.concatenate(parts, axis=0)


def _recip(x):
    r = pl.reciprocal(x, approx=True)
    return r * (2.0 - x * r)


def _kernel(ax_hbm, awqkv_hbm, awo_hbm, bx_hbm, bx4_hbm, mem0_hbm, wq_hbm, wk_hbm, wv_hbm, wo_hbm,
            out_hbm,
            stage, awo_raw, w_s, wo_s, wx_s, pre_s, odef_s, out_s,
            xa_s, xb_s, xpre_s, xp_s, xs_s, mem0_s, wa_s, wc_s, awo_s, t1_s, qa_s, kv_s,
            sems):
    b_scale = B_DH ** (-0.5) * LOG2E
    a_scale = A_DH ** (-0.5) * LOG2E

    w_hbm = (wq_hbm, wk_hbm, wv_hbm)
    wo32 = wo_hbm.bitcast(U32)
    awo32 = awo_hbm.bitcast(U32)
    hw = PW // 2
    hd = B_H * B_DH

    def w_copy(p, half, q, m, sem):
        rows = pl.ds(pl.multiple_of(p * PW, PW), PW)
        return pltpu.make_async_copy(w_hbm[m].at[rows, :], stage.at[half, q, m], sem)

    def wa_piece(g, q):
        last = g >= 2 * 3
        return jnp.where(last, 1 + q, g >> 1), jnp.where(last, NT - 1, (g & 1) + 2 * q)

    def wa_copy(c, kt, half, q, sem):
        return pltpu.make_async_copy(
            awqkv_hbm.at[pl.ds(pl.multiple_of(kt * 128, 128), 128),
                         pl.ds(pl.multiple_of(c * D, 128), D)],
            stage.at[half, q, 3, :128], sem)

    def start_trip(g):
        half = g & 1
        src = jnp.minimum(g, NTRIP - 1)
        for q in range(PP):
            for m in range(3):
                w_copy((src + 1) * PP + q, half, q, m, sems.at[half]).start(priority=1)
            wa_copy(*wa_piece(src, q), half, q, sems.at[half]).start(priority=1)

    def wait_trip(half):
        for view in (stage.at[half, :, :3], stage.at[half, :, 3, :128]):
            pltpu.make_async_copy(view, view, sems.at[half]).wait()

    qr = 2 * hw

    def wo_copy(start, n, sem):
        wr = pl.ds(pl.multiple_of(start, 8), n)
        return pltpu.make_async_copy(wo32.at[wr, :], wo_s.at[wr, :], sem)

    def wo_sums(q, piece, anchor=None, never=None):
        def blk(k, n):
            w = wo_s[pl.ds(pl.multiple_of(q * qr + k * hw + piece * WX_ROWS, 8), WX_ROWS),
                     n * KH:(n + 1) * KH]
            if anchor is not None:
                w = jnp.where(never, anchor, w)
            return _unpack(w).astype(F32)

        b11, b12, b21, b22 = blk(0, 0), blk(0, 1), blk(1, 0), blk(1, 1)
        for n, v in enumerate((b11 + b22, b12 - b22, b21 - b11, b11 + b12, b21 + b22)):
            wx_s[q, n, pl.ds(pl.multiple_of(piece * WX_ROWS, 8), WX_ROWS), :] = (
                _pack(v.astype(BF16)))

    def x_copies(xr, sem):
        return [pltpu.make_async_copy(ax_hbm.at[xr, :], xa_s.at[xr, :D], sem),
                pltpu.make_async_copy(bx_hbm.at[xr, :], xb_s.at[xr, :D], sem)]

    xpre_cp = pltpu.make_async_copy(bx4_hbm.at[:, 0], xpre_s, sems.at[3])
    late_cps = ([pltpu.make_async_copy(mem0_hbm, mem0_s, sems.at[2])]
                + x_copies(pl.ds(0, X_HEAD), sems.at[2]))
    awo_cps = [
        pltpu.make_async_copy(awo32.at[:, c * 128:(c + 1) * 128], awo_raw.at[c], sems.at[2])
        for c in range(NT)]
    x_rest = x_copies(pl.ds(X_HEAD, S - X_HEAD), sems.at[3])
    tiles = [(m, j) for m in range(3) for j in range(PW // 128)]
    peel = [tiles[sum(PEEL[:n]):sum(PEEL[:n + 1])] for n in range(len(PEEL))]
    peel_cps = [[pltpu.make_async_copy(w_hbm[m].at[pl.ds(q * PW + j * 128, 128), :],
                                       stage.at[1, q, m, pl.ds(j * 128, 128), :], sems.at[4 + n])
                 for m, j in blk for q in range(PP)] for n, blk in enumerate(peel)]
    peel_cps[-1].append(wa_copy(0, NT - 1, 1, 0, sems.at[3 + len(PEEL)]))

    xpre_cp.start()
    for cps in peel_cps:
        for cp in cps:
            cp.start(priority=1)
    start_trip(0)
    for cp in late_cps:
        cp.start(priority=1)
    kv_s[:, :, :A_HALO, :] = jnp.zeros((2, NT, A_HALO, 128), F32)
    wo_s[NQ * qr:, :] = jnp.zeros((qr, D), U32)

    def gather_heads(ref):
        rows = []
        for j in range(A_DH // 2):
            u = ref[pl.ds(j, A_H, stride=A_DH // 2), :]
            rows.append(pltpu.bitcast(u << 16, F32))
            rows.append(pltpu.bitcast(u & jnp.uint32(0xFFFF0000), F32))
        return jnp.concatenate(rows, axis=0)

    HR = NSEG * PRE // 2

    def xq(i, k):
        return _unpack(xp_s[i * HR // 2:(i + 1) * HR // 2, k * KH:(k + 1) * KH])

    def strassen_lhs():
        f = lambda i, k: xq(i, k).astype(F32)
        sums = (f(0, 0) + f(1, 1), f(1, 0) + f(1, 1), f(0, 0) + f(0, 1),
                f(1, 0) - f(0, 0), f(0, 1) - f(1, 1))
        for n, v in enumerate(sums):
            xs_s[n] = _pack(v.astype(BF16))

    def pair_prep2(p, half, m, js=(0, 1, 2), hook=None):
        if SKIP_PROLOGUE:
            return
        for q in range(2):
            lo, hi = js[0] * 128, (js[-1] + 1) * 128
            w_s[p + q, :, m * PW + lo:m * PW + hi] = _pack(stage[half, q, m, lo:hi, :].T)
        nseg = ST_ROWS // PRE
        for j in js:
            rows = slice(j * 128, (j + 1) * 128)
            b = lambda k, q: stage[half, q, m, rows, k * KH:(k + 1) * KH]
            bf = lambda k, q: b(k, q).astype(F32)
            rhs = ((bf(0, 0) + bf(1, 1)).astype(BF16), b(0, 0),
                   (bf(0, 1) - bf(1, 1)).astype(BF16), (bf(1, 0) - bf(0, 0)).astype(BF16),
                   b(1, 1), (bf(0, 0) + bf(0, 1)).astype(BF16),
                   (bf(1, 0) + bf(1, 1)).astype(BF16))
            tail = [stage[half, q, m, rows, 2 * KH:] for q in range(2)]
            for c in range(HR // ST_ROWS):
                r = slice(c * ST_ROWS // 2, (c + 1) * ST_ROWS // 2)
                sm = lambda n: _unpack(xs_s[n, r, :])
                qd = lambda i, k: _unpack(
                    xp_s[(i * HR + c * ST_ROWS) // 2:(i * HR + (c + 1) * ST_ROWS) // 2,
                         k * KH:(k + 1) * KH])
                rest = lambda i: _unpack(
                    xp_s[(i * HR + c * ST_ROWS) // 2:(i * HR + (c + 1) * ST_ROWS) // 2, 2 * KH:])

                def put(i, q, v):
                    s0 = i * (NSEG // 2) + c * nseg
                    pre_s[s0:s0 + nseg, p + q, :, m * PW + j * 128:m * PW + (j + 1) * 128] = (
                        v.reshape(nseg, PRE, 128))
                    if hook is not None:
                        hook(v)

                m5 = _nt_dot(sm(2), rhs[4])
                m3 = _nt_dot(qd(0, 0), rhs[2])
                put(0, 1, _nt_dot(rest(0), tail[1]) + m3 + m5)
                m1 = _nt_dot(sm(0), rhs[0])
                m4 = _nt_dot(qd(1, 1), rhs[3])
                put(0, 0, _nt_dot(rest(0), tail[0]) + _nt_dot(sm(4), rhs[6]) + (m1 + m4 - m5))
                m2 = _nt_dot(sm(1), rhs[1])
                put(1, 0, _nt_dot(rest(1), tail[0]) + m2 + m4)
                put(1, 1, _nt_dot(rest(1), tail[1]) + _nt_dot(sm(3), rhs[5]) + (m1 - m2 + m3))

    def wa_prep(c, kt, half, q):
        t1_s[q] = _pack(stage[half, q, 3, :128].T)
        g = gather_heads(t1_s.at[q])
        wa_s[c, pl.ds(pl.multiple_of(kt * 64, 64), 64), :] = _pack(g.astype(BF16).T)
        return g

    def wa_trip(g, half):
        lo, hi = [wa_prep(*wa_piece(g, q), half, q) for q in range(2)]
        for t in range(2):
            b11, b12 = lo[2 * t * 128:(2 * t + 1) * 128], lo[(2 * t + 1) * 128:(2 * t + 2) * 128]
            b21, b22 = hi[2 * t * 128:(2 * t + 1) * 128], hi[(2 * t + 1) * 128:(2 * t + 2) * 128]
            sums = cat([b11 + b22, b12 - b22, b21 - b11, b11 + b12, b21 + b22])
            wc_s[g, t] = _pack(sums.astype(BF16).T)

    xpre_cp.wait()
    xp_s[...] = _pack(xpre_s[...].reshape(NSEG * PRE, D))
    strassen_lhs()
    for blk, cps in zip(peel, peel_cps):
        for cp in cps:
            cp.wait()
        for m in range(3):
            js = tuple(j for mm, j in blk if mm == m)
            if js:
                pair_prep2(0, 1, m, js)
    wa_prep(0, NT - 1, 1, 0)

    def prologue(g, carry):
        half = g & 1

        @pl.when(g > 0)
        def _():
            wo_copy((g - 1) * WO_ROWS, WO_ROWS, sems.at[8]).wait()

        @pl.when(g == NTRIP - 1)
        def _():
            for cp in awo_cps:
                cp.start(priority=1)

        @pl.when(g < NTRIP - 1)
        def _():
            wo_copy(g * WO_ROWS, WO_ROWS, sems.at[8]).start()

        start_trip(g + 1)
        wait_trip(half)
        calls = [0]
        per = hw // WX_ROWS
        total = max(b - a for a, b in zip(WX_DONE, WX_DONE[1:]))
        todo = list(range(total))
        first, stop = NQ * per, (NQ + 1) * per
        for trip in range(1, NTRIP):
            first = jnp.where(g == trip, WX_DONE[trip - 1], first)
            stop = jnp.where(g == trip, WX_DONE[trip], stop)

        def hook(v):
            calls[0] += 1
            want = (calls[0] - WX_SKIP) * total // (36 - WX_SKIP - WX_TAIL)
            t = 0
            while todo and todo[0] < want:
                k = jnp.minimum(first + todo.pop(0), stop - 1)
                q = k // per
                anchor = jnp.concatenate(
                    [v[(2 * t + c) * WX_ROWS:(2 * t + c + 1) * WX_ROWS] for c in range(2)], axis=1)
                wo_sums(q, k % per, pltpu.bitcast(anchor, U32), g > NSEG)
                t += 1

        for m in range(3):
            pair_prep2((g + 1) * PP, half, m, hook=hook)
            if m == 0:
                wa_trip(g, half)
        return carry

    lax.fori_loop(0, NTRIP, prologue, 0)

    for cp in late_cps + awo_cps:
        cp.wait()
    for cp in x_rest:
        cp.start()

    for c in range(NT):
        awo_s[:, c * 128:(c + 1) * 128] = _pack(gather_heads(awo_raw.at[c]).astype(BF16))

    def out_copy(row, n, half):
        r = pl.ds(row, n)
        c = slice(half * D, (half + 1) * D)
        return pltpu.make_async_copy(out_s.at[r, c], out_hbm.at[r, c], sems.at[7])

    def segment(s, mem, u):
        last = u == SPT - 1
        row0 = pl.multiple_of(s * SEG, SEG)
        ninf = jnp.float32(-jnp.inf)

        qi = lax.broadcasted_iota(jnp.int32, (SEG, 128), 0)
        kl = lax.broadcasted_iota(jnp.int32, (SEG, 128), 1)
        is_a = kl < L
        a80 = lax.broadcasted_iota(jnp.int32, (SEG, 2 * L), 1) < L
        real = kl < 2 * L
        kpos = jnp.where(is_a, kl, kl - L)
        allowed = ((qi >= FRESH) | (qi + MEM + PRE >= kpos)) & real
        fill = jnp.where(real, NEG, ninf)
        pi = lax.broadcasted_iota(jnp.int32, (GP * PRE, 128), 0)
        pk = lax.broadcasted_iota(jnp.int32, (GP * PRE, 128), 1)
        p_own = (pk // SEG) == (pi // PRE)
        p_allowed = (pk % (MEM + PRE)) <= (pi % PRE) + MEM
        p_first = (pk % SEG) < MEM + PRE
        p_allowed = p_allowed & p_own
        p_fill = jnp.where(p_own, NEG, ninf)
        col_a = lax.broadcasted_iota(jnp.int32, (1, PW), 1) < B_DH
        col128_a = lax.broadcasted_iota(jnp.int32, (1, 128), 1) < (B_DH - 128)

        xb = xb_s[pl.ds(row0, SEG), :D].astype(F32)
        h = jnp.concatenate([xb[PRE:], mem], axis=0).astype(BF16)

        def proj(p, m):
            return _dot(h, _unpack(w_s[p, :, m * PW:(m + 1) * PW]))

        def pre(p, m):
            return pre_s[s, p, :, m * PW:(m + 1) * PW]

        def block_diag(p, m):
            f = proj(p, m)
            full = jnp.concatenate([f[FRESH:], pre(p, m), f[:FRESH]], axis=0)
            z = jnp.zeros_like(full)
            return jnp.where(col_a, full, z), jnp.where(col_a, z, full)

        def keys_t(blocks):
            fold = cat([jnp.concatenate([x[:, :128] if i % 2 == 0 else x[:, 256:], x[:, 128:256]],
                                        axis=1) for i, x in enumerate(blocks)])
            t = fold.T
            return t[:128].astype(BF16), t[128:].astype(BF16)

        def qk(q, kt, lane_a):
            outer = _dot(cat([q[:, :128], q[:, 256:]]).astype(BF16), kt[0])
            sc = (jnp.where(lane_a, outer[:SEG], outer[SEG:])
                  + _dot(q[:, 128:256].astype(BF16), kt[1]))
            if sc.shape[1] < 128:
                sc = jnp.concatenate([sc, jnp.zeros((SEG, 128 - sc.shape[1]), F32)], axis=1)
            return sc

        def row_max(raw, ok, other, first):
            sc = jnp.where(ok, raw * b_scale, other)
            ma = jnp.max(jnp.where(first, sc, ninf), axis=1, keepdims=True)
            mb = jnp.max(jnp.where(first, ninf, sc), axis=1, keepdims=True)
            return sc, ma, mb

        def probs(mx, first, late_norm):
            sc, ma, mb = mx
            e = jnp.exp2(sc - jnp.where(first, ma, mb))
            ea, eb = jnp.where(first, e, 0.0), jnp.where(first, 0.0, e)
            sa = jnp.sum(ea, axis=1, keepdims=True)
            sb = jnp.sum(eb, axis=1, keepdims=True)
            if PVFOLD:
                if late_norm:
                    return (e, ea, eb), _recip(sa), _recip(sb)
                pr = e * _recip(jnp.where(first, sa, sb))
                return (pr, jnp.where(first, pr, 0.0), jnp.where(first, 0.0, pr)), None, None
            if late_norm:
                return e.astype(BF16), _recip(sa), _recip(sb)
            return (e * _recip(jnp.where(first, sa, sb))).astype(BF16), None, None

        def apply_v(e, blocks):
            pad = 128 - sum(x.shape[0] for x in blocks)
            if not PVFOLD:
                return _dot(e, cat(list(blocks) + ([jnp.zeros((pad, PW), F32)] if pad else [])
                                   ).astype(BF16))
            z = [jnp.zeros((pad, 128), F32)] if pad else []
            outer = cat([x[:, :128] if i % 2 == 0 else x[:, 256:]
                         for i, x in enumerate(blocks)] + z)
            mid = cat([x[:, 128:256] for x in blocks] + z)
            oo = _dot(cat([e[1], e[2]]).astype(BF16), outer.astype(BF16))
            om = _dot(e[0].astype(BF16), mid.astype(BF16))
            return jnp.concatenate([oo[:SEG], om, oo[SEG:]], axis=1)

        def pv(sm, vbd):
            e, ra, rb = sm
            o = apply_v(e, vbd)
            if ra is not None:
                o = jnp.concatenate([
                    o[:, :128] * ra,
                    o[:, 128:256] * jnp.where(col128_a, ra, rb),
                    o[:, 256:] * rb], axis=1)
            return o

        def pre_pv(g, pr, vbds):
            o = apply_v(pr, [x[:MEM + PRE] for vb in vbds for x in vb])
            if not last:
                odef_s[u, g] = o
            return o

        def wout(p, o, acc):
            contrib = _dot(o.astype(BF16), _unpack(wo_s[p * hw:(p + 1) * hw, :]))
            return contrib if acc is None else acc + contrib

        def deferred(p):
            r = slice((p % GP) * PRE, (p % GP + 1) * PRE)
            return cat([odef_s[v, p // GP, r, :] for v in range(SPT - 1)]
                       + [val["PPV", p // GP][r]])

        def wout_strassen(kind, q):
            a11, a21 = val["PV", 2 * q], deferred(2 * q)
            if kind != "XA":
                a12, a22 = val["PV", 2 * q + 1], deferred(2 * q + 1)
            blk = lambda k, n: _unpack(
                wo_s[q * qr + k * hw:q * qr + (k + 1) * hw, n * KH:(n + 1) * KH])
            sm = lambda n: _unpack(wx_s[q, n])
            if kind == "XA":
                terms = {3: (a11, sm(1)), 6: (a21 - a11, sm(3))}
            elif kind == "XB":
                terms = {1: (a11 + a22, sm(0)), 4: (a22, sm(2)), 5: (a11 + a12, blk(1, 1)),
                         7: (a12 - a22, sm(4))}
            elif kind == "XC":
                terms = {2: (a21 + a22, blk(0, 0))}
            else:
                lhs = jnp.concatenate([cat([a11, a21]), cat([a12, a22])], axis=1)
                terms = {0: (lhs, _unpack(wo_s[q * qr:(q + 1) * qr, 2 * KH:]))}
            for n, (x, w) in terms.items():
                r = _dot(x.astype(BF16), w)
                val["acc", n] = val["acc", n] + r if ("acc", n) in val else r

        arow0 = pl.multiple_of((s - u % 2) * SEG, 2 * SEG)

        def a_put(m, j, r):
            if m == 0:
                qa_s[j] = r * a_scale
            else:
                kv_s[m - 1, j, A_HALO:A_HALO + 2 * SEG, :] = r

        def a_proj(idx):
            m, t = divmod(idx, 3)
            if "xa" not in val:
                xa = xa_s[pl.ds(arow0, 2 * SEG), :D]
                xf = xa.astype(F32)
                f = lambda i, k: xf[i * SEG:(i + 1) * SEG, k * KH:(k + 1) * KH]
                val["xa"] = xa
                val["xs"] = [v.astype(BF16) for v in (
                    f(0, 0) + f(1, 1), f(1, 0) + f(1, 1), f(0, 0), f(1, 1), f(0, 0) + f(0, 1),
                    f(1, 0) - f(0, 0), f(0, 1) - f(1, 1))]
                val["xr"] = xf[:, 2 * KH:].astype(BF16)
            if t == 2:
                a_put(m, NT - 1, _dot(val["xa"], _unpack(wa_s[m, :, (NT - 1) * 128:])))
                return
            sm = lambda n: _unpack(cat([wc_s[2 * m + k, t, :, n * 128:(n + 1) * 128]
                                        for k in range(2)]))
            blk = lambda k, j: _unpack(wa_s[m, k * KH // 2:(k + 1) * KH // 2,
                                            (2 * t + j) * 128:(2 * t + j + 1) * 128])
            rhs = (sm(0), blk(0, 0), sm(1), sm(2), blk(1, 1), sm(3), sm(4))
            mm = lambda n: _dot(val["xs"][n], rhs[n])
            tail = [_dot(val["xr"], _unpack(wa_s[m, KH:, (2 * t + j) * 128:(2 * t + j + 1) * 128]))
                    for j in range(2)]
            m1, m2, m3, m4, m5 = [mm(n) for n in range(5)]
            a_put(m, 2 * t, tail[0] + cat([mm(6) + (m1 + m4 - m5), m2 + m4]))
            a_put(m, 2 * t + 1, tail[1] + cat([m3 + m5, mm(5) + (m1 - m2 + m3)]))

        def window(m, j, w, hf):
            lo = A_HALO + hf * SEG - A_DIL * w
            return kv_s[m, j, lo:lo + SEG, :]

        def local_softmax(hf):
            pos = arow0 + hf * SEG + lax.broadcasted_iota(jnp.int32, (SEG, 128), 0)
            rows = slice(hf * SEG, (hf + 1) * SEG)
            logits = []
            for w in range(A_W):
                t = qa_s[0, rows, :] * window(0, 0, w, hf)
                for j in range(1, NT):
                    t = t + qa_s[j, rows, :] * window(0, j, w, hf)
                t = t + pltpu.roll(t, 64, 1)
                t = t + pltpu.roll(t, 32, 1)
                if w > 0 and hf == 0:
                    t = jnp.where(pos >= A_DIL * w, t, NEG)
                logits.append(t)
            mx = functools.reduce(jnp.maximum, logits)
            es = [jnp.exp2(l - mx) for l in logits]
            inv = _recip(functools.reduce(lambda x, y: x + y, es))
            return es, inv

        def local_pv(j, hf):
            es, inv = val["LA", hf]
            o = es[0] * window(1, j, 0, hf)
            for w in range(1, A_W):
                o = o + es[w] * window(1, j, w, hf)
            return o * inv

        def local_out(j, acc):
            wj = _unpack(awo_s[j * 64:(j + 1) * 64, :])
            if ("AX", j) in val:
                r = cat([val["AX", j], _dot(local_pv(j, 1).astype(BF16), wj)])
            else:
                r = _dot(cat([local_pv(j, 0), local_pv(j, 1)]).astype(BF16), wj)
            for m in range(2):
                kv_s[m, j, :A_HALO, :] = kv_s[m, j, 2 * SEG:2 * SEG + A_HALO, :]
            return r if acc is None else acc + r

        val = {}
        acc = None
        oa = None
        for kind, t in _order(u):
            if kind == "K":
                val[kind, t] = block_diag(t, 1)
            elif kind == "V":
                val[kind, t] = block_diag(t, 2)
            elif kind == "Q":
                val[kind, t] = proj(t, 0)
            elif kind == "T":
                val[kind, t] = keys_t(val["K", t])
            elif kind == "S":
                val[kind, t] = qk(val["Q", t], val["T", t], a80)
            elif kind == "M":
                val[kind, t] = row_max(val["S", t], allowed, fill, is_a)
            elif kind == "E":
                val[kind, t] = probs(val["M", t], is_a, t >= LATE_FROM)
            elif kind == "PV":
                val[kind, t] = pv(val["E", t], val["V", t])
            elif kind == "TG":
                val[kind, t] = keys_t([x[:MEM + PRE] for r in range(GP)
                                       for x in val["K", GP * t + r]])
            elif kind == "PS":
                q = cat([pre(GP * t + r, 0) for r in range(GP)])
                val[kind, t] = qk(q, val["TG", t], p_first)
            elif kind == "MG":
                val[kind, t] = row_max(val["PS", t], p_allowed, p_fill, p_first)
            elif kind == "EG":
                val[kind, t] = probs(val["MG", t], p_first, False)[0]
            elif kind == "PPV":
                val[kind, t] = pre_pv(t, val["EG", t], [val["V", GP * t + r] for r in range(GP)])
            elif kind == "W":
                acc = wout(t, val["PV", t], acc)
            elif kind in ("XA", "XB", "XC", "Y"):
                wout_strassen(kind, t)
            elif kind == "LA":
                val[kind, t] = local_softmax(t)
            elif kind == "AP":
                a_proj(t)
            elif kind == "AX":
                val[kind, t] = _dot(local_pv(t, 0).astype(BF16),
                                    _unpack(awo_s[t * 64:(t + 1) * 64, :]))
            elif kind == "AO":
                oa = local_out(t, oa)
                if t == NT - 1:
                    out_s[pl.ds(arow0, 2 * SEG), :D] = oa.astype(BF16)
                    out_copy(arow0, 2 * SEG, 0).start()
        if last:
            m = lambda n: val["acc", n]
            acc = jnp.concatenate([
                cat([m(1) + m(4) - m(5) + m(7), m(2) + m(4)]),
                cat([m(3) + m(5), m(1) - m(2) + m(3) + m(6)]), m(0)], axis=1)
        return acc

    def steps(i, mem):
        @pl.when(i == 1)
        def _():
            for cp in x_rest:
                cp.wait()

        accs = []
        for u in range(SPT):
            accs.append(segment(i * SPT + u, mem, u))
            mem = accs[-1][FRESH:SEG]
        res = cat([x for u in range(SPT) for x in (
            accs[-1][SEG + u * PRE:SEG + (u + 1) * PRE], accs[u][:FRESH])])
        row = pl.multiple_of(i * SPT * SEG, SPT * SEG)
        out_s[pl.ds(row, SPT * SEG), D:2 * D] = res.astype(BF16)
        out_copy(row, SPT * SEG, 1).start()
        return mem

    lax.fori_loop(0, N_STEPS, steps, mem0_s[...].astype(F32))

    wait_trip(NTRIP % 2)

    done = N_STEPS * SPT * SEG
    pltpu.make_async_copy(out_s.at[:done, :2 * D], out_hbm.at[:done, :], sems.at[7]).wait()


@jax.jit
def pallas_concat_heads__sliding_local_dilated__memory_aug_recurrent_mem_tr__prompt_kernel(
    A_x: jax.Array,
    A_wqkv: jax.Array,
    A_wo: jax.Array,
    B_x: jax.Array,
    B_mem0: jax.Array,
    B_Wq: jax.Array,
    B_Wk: jax.Array,
    B_Wv: jax.Array,
    B_Wo: jax.Array,
    B_seg_len,
):
    del B_seg_len
    assert A_x.shape == (1, S, D) and B_x.shape == (1, S, D)
    hd = B_H * B_DH
    wq_t = jnp.transpose(B_Wq, (1, 2, 0)).reshape(hd, D)
    wk_t = jnp.transpose(B_Wk, (1, 2, 0)).reshape(hd, D)
    wv_t = jnp.transpose(B_Wv, (1, 2, 0)).reshape(hd, D)
    wo = B_Wo.reshape(hd, D)

    any_spec = pl.BlockSpec(memory_space=pl.ANY)
    out = pl.pallas_call(
        _kernel,
        out_shape=jax.ShapeDtypeStruct((S, 2 * D), BF16),
        in_specs=[any_spec] * 10,
        out_specs=any_spec,
        scratch_shapes=[
            pltpu.VMEM((2, PP, 4, PW, D), BF16),
            pltpu.VMEM((NT, D // 2, 128), U32),
            pltpu.VMEM((NP, D // 2, 3 * PW), U32),
            pltpu.VMEM((hd // 2 + PW, D), U32),
            pltpu.VMEM((NQ + 1, 5, PW // 2, KH), U32),
            pltpu.VMEM((NSEG, NP, PRE, 3 * PW), F32),
            pltpu.VMEM((SPT - 1, NG, GP * PRE, PW), F32),
            pltpu.VMEM((S, OUT_W), BF16),
            pltpu.VMEM((S, X_W), BF16),
            pltpu.VMEM((S, X_W), BF16),
            pltpu.VMEM((NSEG, PRE, D), BF16),
            pltpu.VMEM((NSEG * PRE // 2, D), U32),
            pltpu.VMEM((5, NSEG * PRE // 4, 256), U32),
            pltpu.VMEM((MEM, D), BF16),
            pltpu.VMEM((3, D // 2, D), U32),
            pltpu.VMEM((NTRIP, 2, 64, D), U32),
            pltpu.VMEM((D // 2, D), U32),
            pltpu.VMEM((PP, D // 2, 128), U32),
            pltpu.VMEM((NT, 2 * SEG, 128), F32),
            pltpu.VMEM((2, NT, KV_ROWS, 128), F32),
            pltpu.SemaphoreType.DMA((9,)),
        ],
        compiler_params=pltpu.CompilerParams(vmem_limit_bytes=120 * 1024 * 1024,
                                             disable_bounds_checks=True),
    )(A_x.reshape(S, D), A_wqkv, A_wo, B_x.reshape(S, D), B_x.reshape(NSEG, SEG // PRE, PRE, D),
      B_mem0.reshape(MEM, D), wq_t, wk_t, wv_t, wo)
    return out.reshape(1, S, 2 * D)
```

```python
import functools

import jax
import jax.numpy as jnp
from jax import lax
import jax.experimental.pallas as pl
import jax.experimental.pallas.tpu as pltpu

F32 = jnp.float32
BF16 = jnp.bfloat16
U32 = jnp.uint32

S = 2048
D = 640
NT = D // 128
A_H = 32
A_DH = D // A_H
A_W = 8
A_DIL = 2
A_HALO = 16
B_H = 32
B_DH = 192
MEM = 8
SEG = 32
NSEG = S // SEG
NP = B_H // 2
PW = 2 * B_DH
PRE = 8
FRESH = SEG - PRE
L = MEM + SEG
GP = 4
NG = NP // GP
LOG2E = 1.4426950408889634
NEG = -1000000000.0 * LOG2E
PP = 2
NTRIP = NP // PP - 1
PEEL = (2, 2, 5)
KH = 256
WO_ROWS = 512
WX_DONE = (0, 24, 56, 96, 120, 152, 192)
WX_TAIL = 2
WX_ROWS = 8
WX_SKIP = 0
ST_ROWS = 256
X_HEAD = 128
KV_ROWS = 80
X_W = 1024
OUT_W = 2048
SPT = 4
N_STEPS = NSEG // SPT
NQ = NP // 2

LAT_MM, LAT_X, LAT_T, LAT_N, LAT_N_LATE = 190, 190, 380, 230, 100
LATE_FROM = NP - 2
AP_AFTER = (6, 16, 26)
AO_AFTER = (30, 40)
TAIL_FILL = (2, 2, 2, 0)
HOLD_W = (0, 3, 0, 0)


def _segment_order(u):
    odd, last = u % 2 == 1, u == SPT - 1
    proj = []
    for g in range(NG):
        proj += [("K", GP * g + r) for r in range(GP)]
        for r in range(GP):
            proj += [("V", GP * g + r), ("Q", GP * g + r)]
    dur = {"K": 120, "V": 120, "Q": 120, "S": 24, "PV": 24, "PS": 24, "PPV": 24,
           "W": 120, "XA": 96, "XB": 192, "XC": 48, "Y": 96, "AO": 80, "AP": 125,
           "T": 0, "M": 0, "E": 0, "TG": 0, "MG": 0, "EG": 0}
    end = {}

    def ready(task):
        k, i = task
        if k == "T":
            deps = [(("K", i), LAT_MM)]
        elif k == "S":
            deps = [(("Q", i), LAT_MM), (("T", i), LAT_T)]
        elif k == "M":
            deps = [(("S", i), LAT_MM - 40)]
        elif k == "E":
            deps = [(("M", i), LAT_X)]
        elif k == "PV":
            deps = [(("E", i), LAT_N_LATE if i >= LATE_FROM else LAT_N), (("V", i), LAT_MM)]
        elif k == "TG":
            deps = [(("K", GP * i + r), LAT_MM) for r in range(GP)]
        elif k == "PS":
            deps = [(("TG", i), LAT_T)]
        elif k == "MG":
            deps = [(("PS", i), LAT_MM - 40)]
        elif k == "EG":
            deps = [(("MG", i), LAT_X)]
        elif k == "PPV":
            deps = [(("EG", i), LAT_N), (("V", GP * i + GP - 1), LAT_MM)]
        elif k == "W":
            deps = [(("PV", i), LAT_MM)]
        else:
            deps = [(("PV", 2 * i), LAT_MM), (("PPV", 2 * i // GP), LAT_MM)]
            if k != "XA":
                deps.append((("PV", 2 * i + 1), LAT_MM))
        if any(d not in end for d, _ in deps):
            return None
        return max(end[d] + lat for d, lat in deps)

    pend = ([(k, p) for k in ("E", "M", "T") for p in range(NP)]
            + [(k, g) for k in ("EG", "MG", "TG") for g in range(NG)]
            + ([(k, q) for q in range(NQ) for k in ("XA", "XB", "Y", "XC")] if last
               else [("W", p) for p in range(NP)])
            + [("PPV", g) for g in range(NG)]
            + [("PV", p) for p in range(NP)] + [("PS", g) for g in range(NG)]
            + [("S", p) for p in range(NP)])
    fill = [("AO", j) for j in range(NT)] if odd else [("AP", j) for j in (3, 4, 5, 0, 1, 2, 6, 7, 8)]
    order = []
    now = [0]

    def emit(task):
        order.append(task)
        now[0] += dur[task[0]]
        end[task] = now[0]

    nproj = 0
    while pend:
        cand = [x for x in pend if ready(x) is not None and ready(x) <= now[0]]
        if proj:
            cand = [x for x in cand if not (x[0] == "W" and x[1] >= NP - GP - HOLD_W[u])]
        if cand:
            if not proj:
                cand = [x for x in cand if x[0] not in ("W", "XA", "XB", "XC", "Y")] or cand
            pend.remove(cand[0])
            emit(cand[0])
        elif proj:
            emit(proj.pop(0))
            nproj += 1
            if odd and nproj == GP:
                order += [("LA", 0), ("LA", 1)]
            if nproj in (AO_AFTER if odd else AP_AFTER):
                emit(fill.pop(0))
        elif len(fill) > TAIL_FILL[u]:
            emit(fill.pop(0))
        else:
            now[0] = min(ready(x) for x in pend if ready(x) is not None)
    return order + fill


ORDERS = (
    "K0 T0 K1 K2 K3 V0 T1 T2 Q1 T3 Q0 AP3 S0 TG0 M0 PS0 V1 Q2 V2 V3 E0 MG0 S1 S2 M1 K4 Q3 EG0 PV0 "
    "K5 E1 M2 S3 K6 T4 W0 E2 M3 T5 PPV0 PV1 K7 AP4 E3 T6 W1 T7 TG1 PV2 PV3 Q4 W2 V4 W3 PS1 S4 Q5 "
    "V5 M4 MG1 V6 Q7 Q6 E4 S5 EG1 V7 M5 PV4 S6 K8 PPV1 E5 S7 M6 W4 K9 E6 M7 T8 K10 PV5 AP5 T9 K11 "
    "E7 W5 T10 PV6 TG2 V8 T11 PV7 Q8 W7 W6 S8 PS2 V10 V9 Q9 M8 MG2 Q10 E8 EG2 V11 S9 Q11 M9 PV8 "
    "S10 K12 T12 PPV2 E9 S11 M10 W8 E10 M11 PV9 K14 K13 K15 E11 T13 W9 PV10 V12 T14 T15 TG3 PV11 "
    "Q12 W10 W11 PS3 S12 Q13 V13 M12 MG3 V15 V14 E12 Q14 EG3 Q15 S13 M13 PV12 S14 AP0 PPV3 E13 "
    "S15 M14 W12 AP1 E14 PV13 M15 AP2 AP6 PV14 W13 E15 PV15 W14 W15 AP8 AP7 ",
    "K0 K1 K2 T0 K3 LA0 LA1 Q0 V1 T1 V0 T2 T3 TG0 Q1 S0 V2 PS0 Q2 M0 S1 V3 MG0 Q3 M1 S2 K4 EG0 K5 "
    "E0 E1 M2 PV0 S3 K6 T4 PPV0 E2 T5 K7 M3 W0 T6 PV1 PV2 V4 E3 T7 TG1 Q4 W1 W2 PV3 PS1 S4 V5 Q5 "
    "M4 MG1 W3 AO0 S5 V6 E4 EG1 Q6 M5 V7 PV4 Q7 E5 S6 K8 W4 M6 PPV1 PV5 S7 T8 K9 E6 K10 M7 W5 T9 "
    "PV6 K11 E7 T10 V8 W6 T11 TG2 PV7 Q8 AO1 W7 S8 V9 PS2 Q9 M8 V10 MG2 Q10 E8 S9 V11 EG2 Q11 PV8 "
    "M9 S10 K12 PPV2 E9 S11 M10 K13 W8 E10 M11 T12 PV9 K14 K15 E11 T13 T14 PV10 AO2 V12 T15 TG3 "
    "Q12 PV11 V13 Q13 PS3 S12 V14 Q14 M12 S13 MG3 V15 Q15 E12 M13 EG3 S14 W9 E13 M14 PPV3 W10 "
    "PV12 S15 W11 E14 M15 PV13 W12 PV14 E15 W13 PV15 W14 W15 AO3 AO4 ",
    "K0 K2 K1 T0 K3 T1 AP3 V0 Q0 TG0 T3 T2 V1 S0 Q1 PS0 Q2 V2 M0 S1 V3 E0 MG0 Q3 M1 K4 S2 EG0 PV0 "
    "K5 E1 M2 PPV0 S3 K6 T4 W0 E2 M3 T5 AP4 PV1 K7 E3 W1 T6 T7 TG1 PV2 V4 PV3 Q4 W2 W3 PS1 S4 V5 "
    "M4 Q5 MG1 V6 S5 Q6 EG1 E4 V7 Q7 M5 PV4 S6 K8 PPV1 E5 S7 M6 W4 AP5 K9 E6 M7 T8 PV5 K10 T9 K11 "
    "E7 W5 T10 PV6 V8 T11 TG2 PV7 Q8 W6 W7 S8 PS2 V9 Q9 M8 MG2 V10 Q10 E8 EG2 S9 V11 Q11 M9 PV8 "
    "S10 K12 PPV2 E9 W8 S11 M10 K13 E10 M11 T12 PV9 K14 K15 E11 T13 W9 PV11 T14 PV10 V12 T15 TG3 "
    "Q12 W10 V13 W11 PS3 S12 MG3 Q13 M12 V14 Q14 E12 EG3 S13 V15 Q15 M13 PV12 S14 E13 AP0 PPV3 "
    "S15 M14 AP1 W12 M15 AP2 E14 PV13 PV14 AP6 E15 W13 PV15 W14 W15 AP7 AP8 ",
    "K1 K0 K2 T0 K3 LA0 LA1 T1 V0 T2 Q0 T3 TG0 V1 Q1 S0 PS0 V2 Q2 M0 V3 MG0 Q3 S1 E0 M1 S2 EG0 K4 "
    "K5 M2 T4 PV0 E1 AO0 PPV0 S3 K6 E2 T5 K7 M3 XA0 T6 PV1 PV2 V4 E3 T7 TG1 Y0 Q4 XB0 XC0 XA1 PV3 "
    "PS1 S4 V5 Q5 M4 MG1 XB1 E4 Y1 XC1 EG1 S5 Q6 V6 M5 V7 S6 PV4 AO1 Q7 E5 PPV1 K8 S7 M6 XA2 K9 "
    "M7 T8 PV5 K10 E6 T9 XB2 E7 T10 Y2 K11 TG2 T11 XC2 PV6 PV7 V8 Q8 XA3 XB3 Y3 PS2 S8 V9 Q9 M8 "
    "MG2 V10 Q10 AO2 E8 EG2 S9 V11 S10 M9 PV8 K12 Q11 M10 PPV2 K13 E9 K14 S11 E10 T12 M11 T13 K15 "
    "PV9 XA4 T14 PV10 V12 E11 XB4 T15 TG3 XA5 Y4 Q12 AO3 PV11 XB5 PS3 S12 V13 Q13 MG3 V14 M12 Q14 "
    "EG3 S13 V15 E12 M13 PV12 Q15 S14 AO4 PPV3 E13 S15 M14 E14 XA6 M15 XC3 XC4 XC5 PV13 E15 Y5 "
    "PV14 XB6 PV15 XC6 Y6 XA7 XB7 Y7 XC7 ",
)
SKIP_PROLOGUE = False
PVFOLD = False


def _order(u):
    if ORDERS is None or ORDERS[u] is None:
        return _segment_order(u)
    return [(t.rstrip("0123456789"), int(t.lstrip("ABCDEFGHIJKLMNOPQRSTUVWXYZ")))
            for t in ORDERS[u].split()]


def _nt_dot(a, b):
    return lax.dot_general(a, b, (((1,), (1,)), ((), ())), preferred_element_type=F32)


def _dot(a, b):
    return jnp.dot(a, b, preferred_element_type=F32)


def _pack(x):
    return pltpu.bitcast(x, U32)


def _unpack(x):
    return pltpu.bitcast(x, BF16)


def cat(parts):
    return jnp.concatenate(parts, axis=0)


def _recip(x):
    r = pl.reciprocal(x, approx=True)
    return r * (2.0 - x * r)


def _kernel(ax_hbm, awqkv_hbm, awo_hbm, bx_hbm, bx4_hbm, mem0_hbm, wq_hbm, wk_hbm, wv_hbm, wo_hbm,
            out_hbm,
            stage, awo_raw, w_s, wo_s, wx_s, pre_s, odef_s, out_s,
            xa_s, xb_s, xpre_s, xp_s, xs_s, mem0_s, wa_s, wc_s, awo_s, t1_s, qa_s, kv_s,
            sems):
    b_scale = B_DH ** (-0.5) * LOG2E
    a_scale = A_DH ** (-0.5) * LOG2E

    w_hbm = (wq_hbm, wk_hbm, wv_hbm)
    wo32 = wo_hbm.bitcast(U32)
    awo32 = awo_hbm.bitcast(U32)
    hw = PW // 2
    hd = B_H * B_DH

    def w_copy(p, half, q, m, sem):
        rows = pl.ds(pl.multiple_of(p * PW, PW), PW)
        return pltpu.make_async_copy(w_hbm[m].at[rows, :], stage.at[half, q, m], sem)

    def wa_piece(g, q):
        last = g >= 2 * 3
        return jnp.where(last, 1 + q, g >> 1), jnp.where(last, NT - 1, (g & 1) + 2 * q)

    def wa_copy(c, kt, half, q, sem):
        return pltpu.make_async_copy(
            awqkv_hbm.at[pl.ds(pl.multiple_of(kt * 128, 128), 128),
                         pl.ds(pl.multiple_of(c * D, 128), D)],
            stage.at[half, q, 3, :128], sem)

    def start_trip(g):
        half = g & 1
        src = jnp.minimum(g, NTRIP - 1)
        for q in range(PP):
            for m in range(3):
                w_copy((src + 1) * PP + q, half, q, m, sems.at[half]).start(priority=1)
            wa_copy(*wa_piece(src, q), half, q, sems.at[half]).start(priority=1)

    def wait_trip(half):
        for view in (stage.at[half, :, :3], stage.at[half, :, 3, :128]):
            pltpu.make_async_copy(view, view, sems.at[half]).wait()

    qr = 2 * hw

    def wo_copy(start, n, sem):
        wr = pl.ds(pl.multiple_of(start, 8), n)
        return pltpu.make_async_copy(wo32.at[wr, :], wo_s.at[wr, :], sem)

    def wo_sums(q, piece, anchor=None, never=None):
        def blk(k, n):
            w = wo_s[pl.ds(pl.multiple_of(q * qr + k * hw + piece * WX_ROWS, 8), WX_ROWS),
                     n * KH:(n + 1) * KH]
            if anchor is not None:
                w = jnp.where(never, anchor, w)
            return _unpack(w).astype(F32)

        b11, b12, b21, b22 = blk(0, 0), blk(0, 1), blk(1, 0), blk(1, 1)
        for n, v in enumerate((b11 + b22, b12 - b22, b21 - b11, b11 + b12, b21 + b22)):
            wx_s[q, n, pl.ds(pl.multiple_of(piece * WX_ROWS, 8), WX_ROWS), :] = (
                _pack(v.astype(BF16)))

    def x_copies(xr, sem):
        return [pltpu.make_async_copy(ax_hbm.at[xr, :], xa_s.at[xr, :D], sem),
                pltpu.make_async_copy(bx_hbm.at[xr, :], xb_s.at[xr, :D], sem)]

    xpre_cp = pltpu.make_async_copy(bx4_hbm.at[:, 0], xpre_s, sems.at[3])
    late_cps = ([pltpu.make_async_copy(mem0_hbm, mem0_s, sems.at[2])]
                + x_copies(pl.ds(0, X_HEAD), sems.at[2]))
    awo_cps = [
        pltpu.make_async_copy(awo32.at[:, c * 128:(c + 1) * 128], awo_raw.at[c], sems.at[2])
        for c in range(NT)]
    x_rest = x_copies(pl.ds(X_HEAD, S - X_HEAD), sems.at[3])
    tiles = [(m, j) for m in range(3) for j in range(PW // 128)]
    peel = [tiles[sum(PEEL[:n]):sum(PEEL[:n + 1])] for n in range(len(PEEL))]
    peel_cps = [[pltpu.make_async_copy(w_hbm[m].at[pl.ds(q * PW + j * 128, 128), :],
                                       stage.at[1, q, m, pl.ds(j * 128, 128), :], sems.at[4 + n])
                 for m, j in blk for q in range(PP)] for n, blk in enumerate(peel)]
    peel_cps[-1].append(wa_copy(0, NT - 1, 1, 0, sems.at[3 + len(PEEL)]))

    xpre_cp.start()
    for cps in peel_cps:
        for cp in cps:
            cp.start(priority=1)
    start_trip(0)
    for cp in late_cps:
        cp.start(priority=1)
    kv_s[:, :, :A_HALO, :] = jnp.zeros((2, NT, A_HALO, 128), F32)
    wo_s[NQ * qr:, :] = jnp.zeros((qr, D), U32)

    def gather_heads(ref):
        rows = []
        for j in range(A_DH // 2):
            u = ref[pl.ds(j, A_H, stride=A_DH // 2), :]
            rows.append(pltpu.bitcast(u << 16, F32))
            rows.append(pltpu.bitcast(u & jnp.uint32(0xFFFF0000), F32))
        return jnp.concatenate(rows, axis=0)

    HR = NSEG * PRE // 2

    def xq(i, k):
        return _unpack(xp_s[i * HR // 2:(i + 1) * HR // 2, k * KH:(k + 1) * KH])

    def strassen_lhs():
        f = lambda i, k: xq(i, k).astype(F32)
        sums = (f(0, 0) + f(1, 1), f(1, 0) + f(1, 1), f(0, 0) + f(0, 1),
                f(1, 0) - f(0, 0), f(0, 1) - f(1, 1))
        for n, v in enumerate(sums):
            xs_s[n] = _pack(v.astype(BF16))

    def pair_prep2(p, half, m, js=(0, 1, 2), hook=None):
        if SKIP_PROLOGUE:
            return
        for q in range(2):
            lo, hi = js[0] * 128, (js[-1] + 1) * 128
            w_s[p + q, :, m * PW + lo:m * PW + hi] = _pack(stage[half, q, m, lo:hi, :].T)
        nseg = ST_ROWS // PRE
        for j in js:
            rows = slice(j * 128, (j + 1) * 128)
            b = lambda k, q: stage[half, q, m, rows, k * KH:(k + 1) * KH]
            bf = lambda k, q: b(k, q).astype(F32)
            rhs = ((bf(0, 0) + bf(1, 1)).astype(BF16), b(0, 0),
                   (bf(0, 1) - bf(1, 1)).astype(BF16), (bf(1, 0) - bf(0, 0)).astype(BF16),
                   b(1, 1), (bf(0, 0) + bf(0, 1)).astype(BF16),
                   (bf(1, 0) + bf(1, 1)).astype(BF16))
            tail = [stage[half, q, m, rows, 2 * KH:] for q in range(2)]
            for c in range(HR // ST_ROWS):
                r = slice(c * ST_ROWS // 2, (c + 1) * ST_ROWS // 2)
                sm = lambda n: _unpack(xs_s[n, r, :])
                qd = lambda i, k: _unpack(
                    xp_s[(i * HR + c * ST_ROWS) // 2:(i * HR + (c + 1) * ST_ROWS) // 2,
                         k * KH:(k + 1) * KH])
                rest = lambda i: _unpack(
                    xp_s[(i * HR + c * ST_ROWS) // 2:(i * HR + (c + 1) * ST_ROWS) // 2, 2 * KH:])

                def put(i, q, v):
                    s0 = i * (NSEG // 2) + c * nseg
                    pre_s[s0:s0 + nseg, p + q, :, m * PW + j * 128:m * PW + (j + 1) * 128] = (
                        v.reshape(nseg, PRE, 128))
                    if hook is not None:
                        hook(v)

                m5 = _nt_dot(sm(2), rhs[4])
                m3 = _nt_dot(qd(0, 0), rhs[2])
                put(0, 1, _nt_dot(rest(0), tail[1]) + m3 + m5)
                m1 = _nt_dot(sm(0), rhs[0])
                m4 = _nt_dot(qd(1, 1), rhs[3])
                put(0, 0, _nt_dot(rest(0), tail[0]) + _nt_dot(sm(4), rhs[6]) + (m1 + m4 - m5))
                m2 = _nt_dot(sm(1), rhs[1])
                put(1, 0, _nt_dot(rest(1), tail[0]) + m2 + m4)
                put(1, 1, _nt_dot(rest(1), tail[1]) + _nt_dot(sm(3), rhs[5]) + (m1 - m2 + m3))

    def wa_prep(c, kt, half, q):
        t1_s[q] = _pack(stage[half, q, 3, :128].T)
        g = gather_heads(t1_s.at[q])
        wa_s[c, pl.ds(pl.multiple_of(kt * 64, 64), 64), :] = _pack(g.astype(BF16).T)
        return g

    def wa_trip(g, half):
        lo, hi = [wa_prep(*wa_piece(g, q), half, q) for q in range(2)]
        for t in range(2):
            b11, b12 = lo[2 * t * 128:(2 * t + 1) * 128], lo[(2 * t + 1) * 128:(2 * t + 2) * 128]
            b21, b22 = hi[2 * t * 128:(2 * t + 1) * 128], hi[(2 * t + 1) * 128:(2 * t + 2) * 128]
            sums = cat([b11 + b22, b12 - b22, b21 - b11, b11 + b12, b21 + b22])
            wc_s[g, t] = _pack(sums.astype(BF16).T)

    xpre_cp.wait()
    xp_s[...] = _pack(xpre_s[...].reshape(NSEG * PRE, D))
    strassen_lhs()
    for blk, cps in zip(peel, peel_cps):
        for cp in cps:
            cp.wait()
        for m in range(3):
            js = tuple(j for mm, j in blk if mm == m)
            if js:
                pair_prep2(0, 1, m, js)
    wa_prep(0, NT - 1, 1, 0)
    start_trip(1)

    def prologue(g, carry):
        half = g & 1

        @pl.when(g > 0)
        def _():
            wo_copy((g - 1) * WO_ROWS, WO_ROWS, sems.at[8]).wait()

        @pl.when(g == NTRIP - 1)
        def _():
            for cp in awo_cps:
                cp.start(priority=1)

        @pl.when(g < NTRIP - 1)
        def _():
            wo_copy(g * WO_ROWS, WO_ROWS, sems.at[8]).start()

        wait_trip(half)
        calls = [0]
        per = hw // WX_ROWS
        total = max(b - a for a, b in zip(WX_DONE, WX_DONE[1:]))
        todo = list(range(total))
        first, stop = NQ * per, (NQ + 1) * per
        for trip in range(1, NTRIP):
            first = jnp.where(g == trip, WX_DONE[trip - 1], first)
            stop = jnp.where(g == trip, WX_DONE[trip], stop)

        def hook(v):
            calls[0] += 1
            want = (calls[0] - WX_SKIP) * total // (36 - WX_SKIP - WX_TAIL)
            t = 0
            while todo and todo[0] < want:
                k = jnp.minimum(first + todo.pop(0), stop - 1)
                q = k // per
                anchor = jnp.concatenate(
                    [v[(2 * t + c) * WX_ROWS:(2 * t + c + 1) * WX_ROWS] for c in range(2)], axis=1)
                wo_sums(q, k % per, pltpu.bitcast(anchor, U32), g > NSEG)
                t += 1

        for m in range(3):
            pair_prep2((g + 1) * PP, half, m, hook=hook)
            if m == 0:
                wa_trip(g, half)
        start_trip(g + 2)
        return carry

    lax.fori_loop(0, NTRIP, prologue, 0)

    for cp in late_cps + awo_cps:
        cp.wait()
    for cp in x_rest:
        cp.start()

    for c in range(NT):
        awo_s[:, c * 128:(c + 1) * 128] = _pack(gather_heads(awo_raw.at[c]).astype(BF16))

    def out_copy(row, n, half):
        r = pl.ds(row, n)
        c = slice(half * D, (half + 1) * D)
        return pltpu.make_async_copy(out_s.at[r, c], out_hbm.at[r, c], sems.at[7])

    def segment(s, mem, u):
        last = u == SPT - 1
        row0 = pl.multiple_of(s * SEG, SEG)
        ninf = jnp.float32(-jnp.inf)

        qi = lax.broadcasted_iota(jnp.int32, (SEG, 128), 0)
        kl = lax.broadcasted_iota(jnp.int32, (SEG, 128), 1)
        is_a = kl < L
        a80 = lax.broadcasted_iota(jnp.int32, (SEG, 2 * L), 1) < L
        real = kl < 2 * L
        kpos = jnp.where(is_a, kl, kl - L)
        allowed = ((qi >= FRESH) | (qi + MEM + PRE >= kpos)) & real
        fill = jnp.where(real, NEG, ninf)
        pi = lax.broadcasted_iota(jnp.int32, (GP * PRE, 128), 0)
        pk = lax.broadcasted_iota(jnp.int32, (GP * PRE, 128), 1)
        p_own = (pk // SEG) == (pi // PRE)
        p_allowed = (pk % (MEM + PRE)) <= (pi % PRE) + MEM
        p_first = (pk % SEG) < MEM + PRE
        p_allowed = p_allowed & p_own
        p_fill = jnp.where(p_own, NEG, ninf)
        col_a = lax.broadcasted_iota(jnp.int32, (1, PW), 1) < B_DH
        col128_a = lax.broadcasted_iota(jnp.int32, (1, 128), 1) < (B_DH - 128)

        xb = xb_s[pl.ds(row0, SEG), :D].astype(F32)
        h = jnp.concatenate([xb[PRE:], mem], axis=0).astype(BF16)

        def proj(p, m):
            return _dot(h, _unpack(w_s[p, :, m * PW:(m + 1) * PW]))

        def pre(p, m):
            return pre_s[s, p, :, m * PW:(m + 1) * PW]

        def block_diag(p, m):
            f = proj(p, m)
            full = jnp.concatenate([f[FRESH:], pre(p, m), f[:FRESH]], axis=0)
            z = jnp.zeros_like(full)
            return jnp.where(col_a, full, z), jnp.where(col_a, z, full)

        def keys_t(blocks):
            fold = cat([jnp.concatenate([x[:, :128] if i % 2 == 0 else x[:, 256:], x[:, 128:256]],
                                        axis=1) for i, x in enumerate(blocks)])
            t = fold.T
            return t[:128].astype(BF16), t[128:].astype(BF16)

        def qk(q, kt, lane_a):
            outer = _dot(cat([q[:, :128], q[:, 256:]]).astype(BF16), kt[0])
            sc = (jnp.where(lane_a, outer[:SEG], outer[SEG:])
                  + _dot(q[:, 128:256].astype(BF16), kt[1]))
            if sc.shape[1] < 128:
                sc = jnp.concatenate([sc, jnp.zeros((SEG, 128 - sc.shape[1]), F32)], axis=1)
            return sc

        def row_max(raw, ok, other, first):
            sc = jnp.where(ok, raw * b_scale, other)
            ma = jnp.max(jnp.where(first, sc, ninf), axis=1, keepdims=True)
            mb = jnp.max(jnp.where(first, ninf, sc), axis=1, keepdims=True)
            return sc, ma, mb

        def probs(mx, first, late_norm):
            sc, ma, mb = mx
            e = jnp.exp2(sc - jnp.where(first, ma, mb))
            ea, eb = jnp.where(first, e, 0.0), jnp.where(first, 0.0, e)
            sa = jnp.sum(ea, axis=1, keepdims=True)
            sb = jnp.sum(eb, axis=1, keepdims=True)
            if PVFOLD:
                if late_norm:
                    return (e, ea, eb), _recip(sa), _recip(sb)
                pr = e * _recip(jnp.where(first, sa, sb))
                return (pr, jnp.where(first, pr, 0.0), jnp.where(first, 0.0, pr)), None, None
            if late_norm:
                return e.astype(BF16), _recip(sa), _recip(sb)
            return (e * _recip(jnp.where(first, sa, sb))).astype(BF16), None, None

        def apply_v(e, blocks):
            pad = 128 - sum(x.shape[0] for x in blocks)
            if not PVFOLD:
                return _dot(e, cat(list(blocks) + ([jnp.zeros((pad, PW), F32)] if pad else [])
                                   ).astype(BF16))
            z = [jnp.zeros((pad, 128), F32)] if pad else []
            outer = cat([x[:, :128] if i % 2 == 0 else x[:, 256:]
                         for i, x in enumerate(blocks)] + z)
            mid = cat([x[:, 128:256] for x in blocks] + z)
            oo = _dot(cat([e[1], e[2]]).astype(BF16), outer.astype(BF16))
            om = _dot(e[0].astype(BF16), mid.astype(BF16))
            return jnp.concatenate([oo[:SEG], om, oo[SEG:]], axis=1)

        def pv(sm, vbd):
            e, ra, rb = sm
            o = apply_v(e, vbd)
            if ra is not None:
                o = jnp.concatenate([
                    o[:, :128] * ra,
                    o[:, 128:256] * jnp.where(col128_a, ra, rb),
                    o[:, 256:] * rb], axis=1)
            return o

        def pre_pv(g, pr, vbds):
            o = apply_v(pr, [x[:MEM + PRE] for vb in vbds for x in vb])
            if not last:
                odef_s[u, g] = o
            return o

        def wout(p, o, acc):
            contrib = _dot(o.astype(BF16), _unpack(wo_s[p * hw:(p + 1) * hw, :]))
            return contrib if acc is None else acc + contrib

        def deferred(p):
            r = slice((p % GP) * PRE, (p % GP + 1) * PRE)
            return cat([odef_s[v, p // GP, r, :] for v in range(SPT - 1)]
                       + [val["PPV", p // GP][r]])

        def wout_strassen(kind, q):
            a11, a21 = val["PV", 2 * q], deferred(2 * q)
            if kind != "XA":
                a12, a22 = val["PV", 2 * q + 1], deferred(2 * q + 1)
            blk = lambda k, n: _unpack(
                wo_s[q * qr + k * hw:q * qr + (k + 1) * hw, n * KH:(n + 1) * KH])
            sm = lambda n: _unpack(wx_s[q, n])
            if kind == "XA":
                terms = {3: (a11, sm(1)), 6: (a21 - a11, sm(3))}
            elif kind == "XB":
                terms = {1: (a11 + a22, sm(0)), 4: (a22, sm(2)), 5: (a11 + a12, blk(1, 1)),
                         7: (a12 - a22, sm(4))}
            elif kind == "XC":
                terms = {2: (a21 + a22, blk(0, 0))}
            else:
                lhs = jnp.concatenate([cat([a11, a21]), cat([a12, a22])], axis=1)
                terms = {0: (lhs, _unpack(wo_s[q * qr:(q + 1) * qr, 2 * KH:]))}
            for n, (x, w) in terms.items():
                r = _dot(x.astype(BF16), w)
                val["acc", n] = val["acc", n] + r if ("acc", n) in val else r

        arow0 = pl.multiple_of((s - u % 2) * SEG, 2 * SEG)

        def a_put(m, j, r):
            if m == 0:
                qa_s[j] = r * a_scale
            else:
                kv_s[m - 1, j, A_HALO:A_HALO + 2 * SEG, :] = r

        def a_proj(idx):
            m, t = divmod(idx, 3)
            if "xa" not in val:
                xa = xa_s[pl.ds(arow0, 2 * SEG), :D]
                xf = xa.astype(F32)
                f = lambda i, k: xf[i * SEG:(i + 1) * SEG, k * KH:(k + 1) * KH]
                val["xa"] = xa
                val["xs"] = [v.astype(BF16) for v in (
                    f(0, 0) + f(1, 1), f(1, 0) + f(1, 1), f(0, 0), f(1, 1), f(0, 0) + f(0, 1),
                    f(1, 0) - f(0, 0), f(0, 1) - f(1, 1))]
                val["xr"] = xf[:, 2 * KH:].astype(BF16)
            if t == 2:
                a_put(m, NT - 1, _dot(val["xa"], _unpack(wa_s[m, :, (NT - 1) * 128:])))
                return
            sm = lambda n: _unpack(cat([wc_s[2 * m + k, t, :, n * 128:(n + 1) * 128]
                                        for k in range(2)]))
            blk = lambda k, j: _unpack(wa_s[m, k * KH // 2:(k + 1) * KH // 2,
                                            (2 * t + j) * 128:(2 * t + j + 1) * 128])
            rhs = (sm(0), blk(0, 0), sm(1), sm(2), blk(1, 1), sm(3), sm(4))
            mm = lambda n: _dot(val["xs"][n], rhs[n])
            tail = [_dot(val["xr"], _unpack(wa_s[m, KH:, (2 * t + j) * 128:(2 * t + j + 1) * 128]))
                    for j in range(2)]
            m1, m2, m3, m4, m5 = [mm(n) for n in range(5)]
            a_put(m, 2 * t, tail[0] + cat([mm(6) + (m1 + m4 - m5), m2 + m4]))
            a_put(m, 2 * t + 1, tail[1] + cat([m3 + m5, mm(5) + (m1 - m2 + m3)]))

        def window(m, j, w, hf):
            lo = A_HALO + hf * SEG - A_DIL * w
            return kv_s[m, j, lo:lo + SEG, :]

        def local_softmax(hf):
            pos = arow0 + hf * SEG + lax.broadcasted_iota(jnp.int32, (SEG, 128), 0)
            rows = slice(hf * SEG, (hf + 1) * SEG)
            logits = []
            for w in range(A_W):
                t = qa_s[0, rows, :] * window(0, 0, w, hf)
                for j in range(1, NT):
                    t = t + qa_s[j, rows, :] * window(0, j, w, hf)
                t = t + pltpu.roll(t, 64, 1)
                t = t + pltpu.roll(t, 32, 1)
                if w > 0 and hf == 0:
                    t = jnp.where(pos >= A_DIL * w, t, NEG)
                logits.append(t)
            mx = functools.reduce(jnp.maximum, logits)
            es = [jnp.exp2(l - mx) for l in logits]
            inv = _recip(functools.reduce(lambda x, y: x + y, es))
            return es, inv

        def local_pv(j, hf):
            es, inv = val["LA", hf]
            o = es[0] * window(1, j, 0, hf)
            for w in range(1, A_W):
                o = o + es[w] * window(1, j, w, hf)
            return o * inv

        def local_out(j, acc):
            wj = _unpack(awo_s[j * 64:(j + 1) * 64, :])
            if ("AX", j) in val:
                r = cat([val["AX", j], _dot(local_pv(j, 1).astype(BF16), wj)])
            else:
                r = _dot(cat([local_pv(j, 0), local_pv(j, 1)]).astype(BF16), wj)
            for m in range(2):
                kv_s[m, j, :A_HALO, :] = kv_s[m, j, 2 * SEG:2 * SEG + A_HALO, :]
            return r if acc is None else acc + r

        val = {}
        acc = None
        oa = None
        for kind, t in _order(u):
            if kind == "K":
                val[kind, t] = block_diag(t, 1)
            elif kind == "V":
                val[kind, t] = block_diag(t, 2)
            elif kind == "Q":
                val[kind, t] = proj(t, 0)
            elif kind == "T":
                val[kind, t] = keys_t(val["K", t])
            elif kind == "S":
                val[kind, t] = qk(val["Q", t], val["T", t], a80)
            elif kind == "M":
                val[kind, t] = row_max(val["S", t], allowed, fill, is_a)
            elif kind == "E":
                val[kind, t] = probs(val["M", t], is_a, t >= LATE_FROM)
            elif kind == "PV":
                val[kind, t] = pv(val["E", t], val["V", t])
            elif kind == "TG":
                val[kind, t] = keys_t([x[:MEM + PRE] for r in range(GP)
                                       for x in val["K", GP * t + r]])
            elif kind == "PS":
                q = cat([pre(GP * t + r, 0) for r in range(GP)])
                val[kind, t] = qk(q, val["TG", t], p_first)
            elif kind == "MG":
                val[kind, t] = row_max(val["PS", t], p_allowed, p_fill, p_first)
            elif kind == "EG":
                val[kind, t] = probs(val["MG", t], p_first, False)[0]
            elif kind == "PPV":
                val[kind, t] = pre_pv(t, val["EG", t], [val["V", GP * t + r] for r in range(GP)])
            elif kind == "W":
                acc = wout(t, val["PV", t], acc)
            elif kind in ("XA", "XB", "XC", "Y"):
                wout_strassen(kind, t)
            elif kind == "LA":
                val[kind, t] = local_softmax(t)
            elif kind == "AP":
                a_proj(t)
            elif kind == "AX":
                val[kind, t] = _dot(local_pv(t, 0).astype(BF16),
                                    _unpack(awo_s[t * 64:(t + 1) * 64, :]))
            elif kind == "AO":
                oa = local_out(t, oa)
                if t == NT - 1:
                    out_s[pl.ds(arow0, 2 * SEG), :D] = oa.astype(BF16)
                    out_copy(arow0, 2 * SEG, 0).start()
        if last:
            m = lambda n: val["acc", n]
            acc = jnp.concatenate([
                cat([m(1) + m(4) - m(5) + m(7), m(2) + m(4)]),
                cat([m(3) + m(5), m(1) - m(2) + m(3) + m(6)]), m(0)], axis=1)
        return acc

    def steps(i, mem):
        @pl.when(i == 1)
        def _():
            for cp in x_rest:
                cp.wait()

        accs = []
        for u in range(SPT):
            accs.append(segment(i * SPT + u, mem, u))
            mem = accs[-1][FRESH:SEG]
        res = cat([x for u in range(SPT) for x in (
            accs[-1][SEG + u * PRE:SEG + (u + 1) * PRE], accs[u][:FRESH])])
        row = pl.multiple_of(i * SPT * SEG, SPT * SEG)
        out_s[pl.ds(row, SPT * SEG), D:2 * D] = res.astype(BF16)
        out_copy(row, SPT * SEG, 1).start()
        return mem

    lax.fori_loop(0, N_STEPS, steps, mem0_s[...].astype(F32))

    wait_trip(0)
    wait_trip(1)

    done = N_STEPS * SPT * SEG
    pltpu.make_async_copy(out_s.at[:done, :2 * D], out_hbm.at[:done, :], sems.at[7]).wait()


@jax.jit
def pallas_concat_heads__sliding_local_dilated__memory_aug_recurrent_mem_tr__prompt_kernel(
    A_x: jax.Array,
    A_wqkv: jax.Array,
    A_wo: jax.Array,
    B_x: jax.Array,
    B_mem0: jax.Array,
    B_Wq: jax.Array,
    B_Wk: jax.Array,
    B_Wv: jax.Array,
    B_Wo: jax.Array,
    B_seg_len,
):
    del B_seg_len
    assert A_x.shape == (1, S, D) and B_x.shape == (1, S, D)
    hd = B_H * B_DH
    wq_t = jnp.transpose(B_Wq, (1, 2, 0)).reshape(hd, D)
    wk_t = jnp.transpose(B_Wk, (1, 2, 0)).reshape(hd, D)
    wv_t = jnp.transpose(B_Wv, (1, 2, 0)).reshape(hd, D)
    wo = B_Wo.reshape(hd, D)

    any_spec = pl.BlockSpec(memory_space=pl.ANY)
    out = pl.pallas_call(
        _kernel,
        out_shape=jax.ShapeDtypeStruct((S, 2 * D), BF16),
        in_specs=[any_spec] * 10,
        out_specs=any_spec,
        scratch_shapes=[
            pltpu.VMEM((2, PP, 4, PW, D), BF16),
            pltpu.VMEM((NT, D // 2, 128), U32),
            pltpu.VMEM((NP, D // 2, 3 * PW), U32),
            pltpu.VMEM((hd // 2 + PW, D), U32),
            pltpu.VMEM((NQ + 1, 5, PW // 2, KH), U32),
            pltpu.VMEM((NSEG, NP, PRE, 3 * PW), F32),
            pltpu.VMEM((SPT - 1, NG, GP * PRE, PW), F32),
            pltpu.VMEM((S, OUT_W), BF16),
            pltpu.VMEM((S, X_W), BF16),
            pltpu.VMEM((S, X_W), BF16),
            pltpu.VMEM((NSEG, PRE, D), BF16),
            pltpu.VMEM((NSEG * PRE // 2, D), U32),
            pltpu.VMEM((5, NSEG * PRE // 4, 256), U32),
            pltpu.VMEM((MEM, D), BF16),
            pltpu.VMEM((3, D // 2, D), U32),
            pltpu.VMEM((NTRIP, 2, 64, D), U32),
            pltpu.VMEM((D // 2, D), U32),
            pltpu.VMEM((PP, D // 2, 128), U32),
            pltpu.VMEM((NT, 2 * SEG, 128), F32),
            pltpu.VMEM((2, NT, KV_ROWS, 128), F32),
            pltpu.SemaphoreType.DMA((9,)),
        ],
        compiler_params=pltpu.CompilerParams(vmem_limit_bytes=120 * 1024 * 1024,
                                             disable_bounds_checks=True),
    )(A_x.reshape(S, D), A_wqkv, A_wo, B_x.reshape(S, D), B_x.reshape(NSEG, SEG // PRE, PRE, D),
      B_mem0.reshape(MEM, D), wq_t, wk_t, wv_t, wo)
    return out.reshape(1, S, 2 * D)
```

```python
import functools

import jax
import jax.numpy as jnp
from jax import lax
import jax.experimental.pallas as pl
import jax.experimental.pallas.tpu as pltpu

F32 = jnp.float32
BF16 = jnp.bfloat16
U32 = jnp.uint32

S = 2048
D = 640
NT = D // 128
A_H = 32
A_DH = D // A_H
A_W = 8
A_DIL = 2
A_HALO = 16
B_H = 32
B_DH = 192
MEM = 8
SEG = 32
NSEG = S // SEG
NP = B_H // 2
PW = 2 * B_DH
PRE = 8
FRESH = SEG - PRE
L = MEM + SEG
GP = 4
NG = NP // GP
LOG2E = 1.4426950408889634
NEG = -1000000000.0 * LOG2E
PP = 2
NTRIP = NP // PP - 1
PEEL = (2, 2, 5)
KH = 256
WO_ROWS = 512
WX_DONE = (0, 24, 56, 96, 120, 152, 192)
WX_TAIL = 2
WX_ROWS = 8
WX_SKIP = 0
ST_ROWS = 256
X_HEAD = 128
KV_ROWS = 80
X_W = 1024
OUT_W = 2048
SPT = 4
N_STEPS = NSEG // SPT
NQ = NP // 2

LAT_MM, LAT_X, LAT_T, LAT_N, LAT_N_LATE = 190, 190, 380, 230, 100
LATE_FROM = NP - 2
AP_AFTER = (6, 16, 26)
AO_AFTER = (30, 40)
TAIL_FILL = (2, 2, 2, 0)
HOLD_W = (0, 3, 0, 0)


def _segment_order(u):
    odd, last = u % 2 == 1, u == SPT - 1
    proj = []
    for g in range(NG):
        proj += [("K", GP * g + r) for r in range(GP)]
        for r in range(GP):
            proj += [("V", GP * g + r), ("Q", GP * g + r)]
    dur = {"K": 120, "V": 120, "Q": 120, "S": 24, "PV": 24, "PS": 24, "PPV": 24,
           "W": 120, "XA": 96, "XB": 192, "XC": 48, "Y": 96, "AO": 80, "AP": 125,
           "T": 0, "M": 0, "E": 0, "TG": 0, "MG": 0, "EG": 0}
    end = {}

    def ready(task):
        k, i = task
        if k == "T":
            deps = [(("K", i), LAT_MM)]
        elif k == "S":
            deps = [(("Q", i), LAT_MM), (("T", i), LAT_T)]
        elif k == "M":
            deps = [(("S", i), LAT_MM - 40)]
        elif k == "E":
            deps = [(("M", i), LAT_X)]
        elif k == "PV":
            deps = [(("E", i), LAT_N_LATE if i >= LATE_FROM else LAT_N), (("V", i), LAT_MM)]
        elif k == "TG":
            deps = [(("K", GP * i + r), LAT_MM) for r in range(GP)]
        elif k == "PS":
            deps = [(("TG", i), LAT_T)]
        elif k == "MG":
            deps = [(("PS", i), LAT_MM - 40)]
        elif k == "EG":
            deps = [(("MG", i), LAT_X)]
        elif k == "PPV":
            deps = [(("EG", i), LAT_N), (("V", GP * i + GP - 1), LAT_MM)]
        elif k == "W":
            deps = [(("PV", i), LAT_MM)]
        else:
            deps = [(("PV", 2 * i), LAT_MM), (("PPV", 2 * i // GP), LAT_MM)]
            if k != "XA":
                deps.append((("PV", 2 * i + 1), LAT_MM))
        if any(d not in end for d, _ in deps):
            return None
        return max(end[d] + lat for d, lat in deps)

    pend = ([(k, p) for k in ("E", "M", "T") for p in range(NP)]
            + [(k, g) for k in ("EG", "MG", "TG") for g in range(NG)]
            + ([(k, q) for q in range(NQ) for k in ("XA", "XB", "Y", "XC")] if last
               else [("W", p) for p in range(NP)])
            + [("PPV", g) for g in range(NG)]
            + [("PV", p) for p in range(NP)] + [("PS", g) for g in range(NG)]
            + [("S", p) for p in range(NP)])
    fill = [("AO", j) for j in range(NT)] if odd else [("AP", j) for j in (3, 4, 5, 0, 1, 2, 6, 7, 8)]
    order = []
    now = [0]

    def emit(task):
        order.append(task)
        now[0] += dur[task[0]]
        end[task] = now[0]

    nproj = 0
    while pend:
        cand = [x for x in pend if ready(x) is not None and ready(x) <= now[0]]
        if proj:
            cand = [x for x in cand if not (x[0] == "W" and x[1] >= NP - GP - HOLD_W[u])]
        if cand:
            if not proj:
                cand = [x for x in cand if x[0] not in ("W", "XA", "XB", "XC", "Y")] or cand
            pend.remove(cand[0])
            emit(cand[0])
        elif proj:
            emit(proj.pop(0))
            nproj += 1
            if odd and nproj == GP:
                order += [("LA", 0), ("LA", 1)]
            if nproj in (AO_AFTER if odd else AP_AFTER):
                emit(fill.pop(0))
        elif len(fill) > TAIL_FILL[u]:
            emit(fill.pop(0))
        else:
            now[0] = min(ready(x) for x in pend if ready(x) is not None)
    return order + fill


ORDERS = (
    "K0 T0 K1 K2 K3 V0 T1 T2 Q1 T3 Q0 AP3 S0 TG0 M0 PS0 V1 Q2 V2 V3 E0 MG0 S1 S2 M1 K4 Q3 EG0 PV0 "
    "K5 E1 M2 S3 K6 T4 W0 E2 M3 T5 PPV0 PV1 K7 AP4 E3 T6 W1 T7 TG1 PV2 PV3 Q4 W2 V4 W3 PS1 S4 Q5 "
    "V5 M4 MG1 V6 Q7 Q6 E4 S5 EG1 V7 M5 PV4 S6 K8 PPV1 E5 S7 M6 W4 K9 E6 M7 T8 K10 PV5 AP5 T9 K11 "
    "E7 W5 T10 PV6 TG2 V8 T11 PV7 Q8 W7 W6 S8 PS2 V10 V9 Q9 M8 MG2 Q10 E8 EG2 V11 S9 Q11 M9 PV8 "
    "S10 K12 T12 PPV2 E9 S11 M10 W8 E10 M11 PV9 K14 K13 K15 E11 T13 W9 PV10 V12 T14 T15 TG3 PV11 "
    "Q12 W10 W11 PS3 S12 Q13 V13 M12 MG3 V15 V14 E12 Q14 EG3 Q15 S13 M13 PV12 S14 AP0 PPV3 E13 "
    "S15 M14 W12 AP1 E14 PV13 M15 AP2 AP6 PV14 W13 E15 PV15 W14 W15 AP8 AP7 ",
    "K0 K1 K2 T0 K3 LA0 LA1 Q0 V1 T1 V0 T2 T3 TG0 Q1 S0 V2 PS0 Q2 M0 S1 V3 MG0 Q3 M1 S2 K4 EG0 K5 "
    "E0 E1 M2 PV0 S3 K6 T4 PPV0 E2 T5 K7 M3 W0 T6 PV1 PV2 V4 E3 T7 TG1 Q4 W1 W2 PV3 PS1 S4 V5 Q5 "
    "M4 MG1 W3 AO0 S5 V6 E4 EG1 Q6 M5 V7 PV4 Q7 E5 S6 K8 W4 M6 PPV1 PV5 S7 T8 K9 E6 K10 M7 W5 T9 "
    "PV6 K11 E7 T10 V8 W6 T11 TG2 PV7 Q8 AO1 W7 S8 V9 PS2 Q9 M8 V10 MG2 Q10 E8 S9 V11 EG2 Q11 PV8 "
    "M9 S10 K12 PPV2 E9 S11 M10 K13 W8 E10 M11 T12 PV9 K14 K15 E11 T13 T14 PV10 AO2 V12 T15 TG3 "
    "Q12 PV11 V13 Q13 PS3 S12 V14 Q14 M12 S13 MG3 V15 Q15 E12 M13 EG3 S14 W9 E13 M14 PPV3 W10 "
    "PV12 S15 W11 E14 M15 PV13 W12 PV14 E15 W13 PV15 W14 W15 AO3 AO4 ",
    "K0 K2 K1 T0 K3 T1 AP3 V0 Q0 TG0 T3 T2 V1 S0 Q1 PS0 Q2 V2 M0 S1 V3 E0 MG0 Q3 M1 K4 S2 EG0 PV0 "
    "K5 E1 M2 PPV0 S3 K6 T4 W0 E2 M3 T5 AP4 PV1 K7 E3 W1 T6 T7 TG1 PV2 V4 PV3 Q4 W2 W3 PS1 S4 V5 "
    "M4 Q5 MG1 V6 S5 Q6 EG1 E4 V7 Q7 M5 PV4 S6 K8 PPV1 E5 S7 M6 W4 AP5 K9 E6 M7 T8 PV5 K10 T9 K11 "
    "E7 W5 T10 PV6 V8 T11 TG2 PV7 Q8 W6 W7 S8 PS2 V9 Q9 M8 MG2 V10 Q10 E8 EG2 S9 V11 Q11 M9 PV8 "
    "S10 K12 PPV2 E9 W8 S11 M10 K13 E10 M11 T12 PV9 K14 K15 E11 T13 W9 PV11 T14 PV10 V12 T15 TG3 "
    "Q12 W10 V13 W11 PS3 S12 MG3 Q13 M12 V14 Q14 E12 EG3 S13 V15 Q15 M13 PV12 S14 E13 AP0 PPV3 "
    "S15 M14 AP1 W12 M15 AP2 E14 PV13 PV14 AP6 E15 W13 PV15 W14 W15 AP7 AP8 ",
    "K1 K0 K2 T0 K3 LA0 LA1 T1 V0 T2 Q0 T3 TG0 V1 Q1 S0 PS0 V2 Q2 M0 V3 MG0 Q3 S1 E0 M1 S2 EG0 K4 "
    "K5 M2 T4 PV0 E1 AO0 PPV0 S3 K6 E2 T5 K7 M3 XA0 T6 PV1 PV2 V4 E3 T7 TG1 Y0 Q4 XB0 XC0 XA1 PV3 "
    "PS1 S4 V5 Q5 M4 MG1 XB1 E4 Y1 XC1 EG1 S5 Q6 V6 M5 V7 S6 PV4 AO1 Q7 E5 PPV1 K8 S7 M6 XA2 K9 "
    "M7 T8 PV5 K10 E6 T9 XB2 E7 T10 Y2 K11 TG2 T11 XC2 PV6 PV7 V8 Q8 XA3 XB3 Y3 PS2 S8 V9 Q9 M8 "
    "MG2 V10 Q10 AO2 E8 EG2 S9 V11 S10 M9 PV8 K12 Q11 M10 PPV2 K13 E9 K14 S11 E10 T12 M11 T13 K15 "
    "PV9 XA4 T14 PV10 V12 E11 XB4 T15 TG3 XA5 Y4 Q12 AO3 PV11 XB5 PS3 S12 V13 Q13 MG3 V14 M12 Q14 "
    "EG3 S13 V15 E12 M13 PV12 Q15 S14 AO4 PPV3 E13 S15 M14 E14 XA6 M15 XC3 XC4 XC5 PV13 E15 Y5 "
    "PV14 XB6 PV15 XC6 Y6 XA7 XB7 Y7 XC7 ",
)
SKIP_PROLOGUE = False


def _order(u):
    if ORDERS is None or ORDERS[u] is None:
        return _segment_order(u)
    return [(t.rstrip("0123456789"), int(t.lstrip("ABCDEFGHIJKLMNOPQRSTUVWXYZ")))
            for t in ORDERS[u].split()]


def _nt_dot(a, b):
    return lax.dot_general(a, b, (((1,), (1,)), ((), ())), preferred_element_type=F32)


def _dot(a, b):
    return jnp.dot(a, b, preferred_element_type=F32)


def _pack(x):
    return pltpu.bitcast(x, U32)


def _unpack(x):
    return pltpu.bitcast(x, BF16)


def cat(parts):
    return jnp.concatenate(parts, axis=0)


def _recip(x):
    r = pl.reciprocal(x, approx=True)
    return r * (2.0 - x * r)


def _kernel(ax_hbm, awqkv_hbm, awo_hbm, bx_hbm, bx4_hbm, mem0_hbm, wq_hbm, wk_hbm, wv_hbm, wo_hbm,
            out_hbm,
            stage, awo_raw, w_s, wo_s, wx_s, pre_s, odef_s, out_s,
            xa_s, xb_s, xpre_s, xp_s, xs_s, mem0_s, wa_s, wc_s, awo_s, t1_s, qa_s, kv_s,
            sems):
    b_scale = B_DH ** (-0.5) * LOG2E
    a_scale = A_DH ** (-0.5) * LOG2E

    w_hbm = (wq_hbm, wk_hbm, wv_hbm)
    wo32 = wo_hbm.bitcast(U32)
    awo32 = awo_hbm.bitcast(U32)
    hw = PW // 2
    hd = B_H * B_DH

    def w_copy(p, half, q, m, sem):
        rows = pl.ds(pl.multiple_of(p * PW, PW), PW)
        return pltpu.make_async_copy(w_hbm[m].at[rows, :], stage.at[half, q, m], sem)

    def wa_piece(g, q):
        last = g >= 2 * 3
        return jnp.where(last, 1 + q, g >> 1), jnp.where(last, NT - 1, (g & 1) + 2 * q)

    def wa_copy(c, kt, half, q, sem):
        return pltpu.make_async_copy(
            awqkv_hbm.at[pl.ds(pl.multiple_of(kt * 128, 128), 128),
                         pl.ds(pl.multiple_of(c * D, 128), D)],
            stage.at[half, q, 3, :128], sem)

    def start_trip(g):
        half = g & 1
        src = jnp.minimum(g, NTRIP - 1)
        for q in range(PP):
            for m in range(3):
                w_copy((src + 1) * PP + q, half, q, m, sems.at[half]).start(priority=1)
            wa_copy(*wa_piece(src, q), half, q, sems.at[half]).start(priority=1)

    def wait_trip(half):
        for view in (stage.at[half, :, :3], stage.at[half, :, 3, :128]):
            pltpu.make_async_copy(view, view, sems.at[half]).wait()

    qr = 2 * hw

    def wo_copy(start, n, sem):
        wr = pl.ds(pl.multiple_of(start, 8), n)
        return pltpu.make_async_copy(wo32.at[wr, :], wo_s.at[wr, :], sem)

    def wo_sums(q, piece, anchor=None, never=None):
        def blk(k, n):
            w = wo_s[pl.ds(pl.multiple_of(q * qr + k * hw + piece * WX_ROWS, 8), WX_ROWS),
                     n * KH:(n + 1) * KH]
            if anchor is not None:
                w = jnp.where(never, anchor, w)
            return _unpack(w).astype(F32)

        b11, b12, b21, b22 = blk(0, 0), blk(0, 1), blk(1, 0), blk(1, 1)
        for n, v in enumerate((b11 + b22, b12 - b22, b21 - b11, b11 + b12, b21 + b22)):
            wx_s[q, n, pl.ds(pl.multiple_of(piece * WX_ROWS, 8), WX_ROWS), :] = (
                _pack(v.astype(BF16)))

    def x_copies(xr, sem):
        return [pltpu.make_async_copy(ax_hbm.at[xr, :], xa_s.at[xr, :D], sem),
                pltpu.make_async_copy(bx_hbm.at[xr, :], xb_s.at[xr, :D], sem)]

    xpre_cp = pltpu.make_async_copy(bx4_hbm.at[:, 0], xpre_s, sems.at[3])
    late_cps = ([pltpu.make_async_copy(mem0_hbm, mem0_s, sems.at[2])]
                + x_copies(pl.ds(0, X_HEAD), sems.at[2]))
    awo_cps = [
        pltpu.make_async_copy(awo32.at[:, c * 128:(c + 1) * 128], awo_raw.at[c], sems.at[2])
        for c in range(NT)]
    x_rest = x_copies(pl.ds(X_HEAD, S - X_HEAD), sems.at[3])
    tiles = [(m, j) for m in range(3) for j in range(PW // 128)]
    peel = [tiles[sum(PEEL[:n]):sum(PEEL[:n + 1])] for n in range(len(PEEL))]
    peel_cps = [[pltpu.make_async_copy(w_hbm[m].at[pl.ds(q * PW + j * 128, 128), :],
                                       stage.at[1, q, m, pl.ds(j * 128, 128), :], sems.at[4 + n])
                 for m, j in blk for q in range(PP)] for n, blk in enumerate(peel)]
    peel_cps[-1].append(wa_copy(0, NT - 1, 1, 0, sems.at[3 + len(PEEL)]))

    xpre_cp.start()
    for cps in peel_cps:
        for cp in cps:
            cp.start(priority=1)
    start_trip(0)
    for cp in late_cps:
        cp.start(priority=1)
    kv_s[:, :, :A_HALO, :] = jnp.zeros((2, NT, A_HALO, 128), F32)
    wo_s[NQ * qr:, :] = jnp.zeros((qr, D), U32)

    def gather_heads(ref):
        rows = []
        for j in range(A_DH // 2):
            u = ref[pl.ds(j, A_H, stride=A_DH // 2), :]
            rows.append(pltpu.bitcast(u << 16, F32))
            rows.append(pltpu.bitcast(u & jnp.uint32(0xFFFF0000), F32))
        return jnp.concatenate(rows, axis=0)

    HR = NSEG * PRE // 2

    def xq(i, k):
        return _unpack(xp_s[i * HR // 2:(i + 1) * HR // 2, k * KH:(k + 1) * KH])

    def strassen_lhs():
        f = lambda i, k: xq(i, k).astype(F32)
        sums = (f(0, 0) + f(1, 1), f(1, 0) + f(1, 1), f(0, 0) + f(0, 1),
                f(1, 0) - f(0, 0), f(0, 1) - f(1, 1))
        for n, v in enumerate(sums):
            xs_s[n] = _pack(v.astype(BF16))

    def pair_prep2(p, half, m, js=(0, 1, 2), hook=None):
        if SKIP_PROLOGUE:
            return
        for q in range(2):
            lo, hi = js[0] * 128, (js[-1] + 1) * 128
            w_s[p + q, :, m * PW + lo:m * PW + hi] = _pack(stage[half, q, m, lo:hi, :].T)
        nseg = ST_ROWS // PRE
        for j in js:
            rows = slice(j * 128, (j + 1) * 128)
            b = lambda k, q: stage[half, q, m, rows, k * KH:(k + 1) * KH]
            bf = lambda k, q: b(k, q).astype(F32)
            rhs = ((bf(0, 0) + bf(1, 1)).astype(BF16), b(0, 0),
                   (bf(0, 1) - bf(1, 1)).astype(BF16), (bf(1, 0) - bf(0, 0)).astype(BF16),
                   b(1, 1), (bf(0, 0) + bf(0, 1)).astype(BF16),
                   (bf(1, 0) + bf(1, 1)).astype(BF16))
            tail = [stage[half, q, m, rows, 2 * KH:] for q in range(2)]
            for c in range(HR // ST_ROWS):
                r = slice(c * ST_ROWS // 2, (c + 1) * ST_ROWS // 2)
                sm = lambda n: _unpack(xs_s[n, r, :])
                qd = lambda i, k: _unpack(
                    xp_s[(i * HR + c * ST_ROWS) // 2:(i * HR + (c + 1) * ST_ROWS) // 2,
                         k * KH:(k + 1) * KH])
                rest = lambda i: _unpack(
                    xp_s[(i * HR + c * ST_ROWS) // 2:(i * HR + (c + 1) * ST_ROWS) // 2, 2 * KH:])

                def put(i, q, v):
                    s0 = i * (NSEG // 2) + c * nseg
                    pre_s[s0:s0 + nseg, p + q, :, m * PW + j * 128:m * PW + (j + 1) * 128] = (
                        v.reshape(nseg, PRE, 128))
                    if hook is not None:
                        hook(v)

                m5 = _nt_dot(sm(2), rhs[4])
                m3 = _nt_dot(qd(0, 0), rhs[2])
                put(0, 1, _nt_dot(rest(0), tail[1]) + m3 + m5)
                m1 = _nt_dot(sm(0), rhs[0])
                m4 = _nt_dot(qd(1, 1), rhs[3])
                put(0, 0, _nt_dot(rest(0), tail[0]) + _nt_dot(sm(4), rhs[6]) + (m1 + m4 - m5))
                m2 = _nt_dot(sm(1), rhs[1])
                put(1, 0, _nt_dot(rest(1), tail[0]) + m2 + m4)
                put(1, 1, _nt_dot(rest(1), tail[1]) + _nt_dot(sm(3), rhs[5]) + (m1 - m2 + m3))

    def wa_prep(c, kt, half, q):
        t1_s[q] = _pack(stage[half, q, 3, :128].T)
        g = gather_heads(t1_s.at[q])
        wa_s[c, pl.ds(pl.multiple_of(kt * 64, 64), 64), :] = _pack(g.astype(BF16).T)
        return g

    def wa_trip(g, half):
        lo, hi = [wa_prep(*wa_piece(g, q), half, q) for q in range(2)]
        for t in range(2):
            b11, b12 = lo[2 * t * 128:(2 * t + 1) * 128], lo[(2 * t + 1) * 128:(2 * t + 2) * 128]
            b21, b22 = hi[2 * t * 128:(2 * t + 1) * 128], hi[(2 * t + 1) * 128:(2 * t + 2) * 128]
            sums = cat([b11 + b22, b12 - b22, b21 - b11, b11 + b12, b21 + b22])
            wc_s[g, t] = _pack(sums.astype(BF16).T)

    xpre_cp.wait()
    xp_s[...] = _pack(xpre_s[...].reshape(NSEG * PRE, D))
    strassen_lhs()
    for blk, cps in zip(peel, peel_cps):
        for cp in cps:
            cp.wait()
        for m in range(3):
            js = tuple(j for mm, j in blk if mm == m)
            if js:
                pair_prep2(0, 1, m, js)
    wa_prep(0, NT - 1, 1, 0)
    start_trip(1)

    def prologue(g, carry):
        half = g & 1

        @pl.when(g > 0)
        def _():
            wo_copy((g - 1) * WO_ROWS, WO_ROWS, sems.at[8]).wait()

        @pl.when(g == NTRIP - 1)
        def _():
            for cp in awo_cps:
                cp.start(priority=1)

        @pl.when(g < NTRIP - 1)
        def _():
            wo_copy(g * WO_ROWS, WO_ROWS, sems.at[8]).start()

        wait_trip(half)
        calls = [0]
        per = hw // WX_ROWS
        total = max(b - a for a, b in zip(WX_DONE, WX_DONE[1:]))
        todo = list(range(total))
        first, stop = NQ * per, (NQ + 1) * per
        for trip in range(1, NTRIP):
            first = jnp.where(g == trip, WX_DONE[trip - 1], first)
            stop = jnp.where(g == trip, WX_DONE[trip], stop)

        def hook(v):
            calls[0] += 1
            want = (calls[0] - WX_SKIP) * total // (36 - WX_SKIP - WX_TAIL)
            t = 0
            while todo and todo[0] < want:
                k = jnp.minimum(first + todo.pop(0), stop - 1)
                q = k // per
                anchor = jnp.concatenate(
                    [v[(2 * t + c) * WX_ROWS:(2 * t + c + 1) * WX_ROWS] for c in range(2)], axis=1)
                wo_sums(q, k % per, pltpu.bitcast(anchor, U32), g > NSEG)
                t += 1

        for m in range(3):
            pair_prep2((g + 1) * PP, half, m, hook=hook)
            if m == 0:
                wa_trip(g, half)
        start_trip(g + 2)
        return carry

    lax.fori_loop(0, NTRIP, prologue, 0)

    for cp in late_cps + awo_cps:
        cp.wait()
    for cp in x_rest:
        cp.start()

    for c in range(NT):
        awo_s[:, c * 128:(c + 1) * 128] = _pack(gather_heads(awo_raw.at[c]).astype(BF16))

    def out_copy(row, n, half):
        r = pl.ds(row, n)
        c = slice(half * D, (half + 1) * D)
        return pltpu.make_async_copy(out_s.at[r, c], out_hbm.at[r, c], sems.at[7])

    def segment(s, mem, u):
        last = u == SPT - 1
        row0 = pl.multiple_of(s * SEG, SEG)
        ninf = jnp.float32(-jnp.inf)

        qi = lax.broadcasted_iota(jnp.int32, (SEG, 128), 0)
        kl = lax.broadcasted_iota(jnp.int32, (SEG, 128), 1)
        is_a = kl < L
        a80 = lax.broadcasted_iota(jnp.int32, (SEG, 2 * L), 1) < L
        real = kl < 2 * L
        kpos = jnp.where(is_a, kl, kl - L)
        allowed = ((qi >= FRESH) | (qi + MEM + PRE >= kpos)) & real
        fill = jnp.where(real, NEG, ninf)
        pi = lax.broadcasted_iota(jnp.int32, (GP * PRE, 128), 0)
        pk = lax.broadcasted_iota(jnp.int32, (GP * PRE, 128), 1)
        p_own = (pk // SEG) == (pi // PRE)
        p_allowed = (pk % (MEM + PRE)) <= (pi % PRE) + MEM
        p_first = (pk % SEG) < MEM + PRE
        p_allowed = p_allowed & p_own
        p_fill = jnp.where(p_own, NEG, ninf)
        col_a = lax.broadcasted_iota(jnp.int32, (1, PW), 1) < B_DH
        col128_a = lax.broadcasted_iota(jnp.int32, (1, 128), 1) < (B_DH - 128)

        xb = xb_s[pl.ds(row0, SEG), :D].astype(F32)
        h = jnp.concatenate([xb[PRE:], mem], axis=0).astype(BF16)

        def proj(p, m):
            return _dot(h, _unpack(w_s[p, :, m * PW:(m + 1) * PW]))

        def pre(p, m):
            return pre_s[s, p, :, m * PW:(m + 1) * PW]

        def block_diag(p, m):
            f = proj(p, m)
            full = jnp.concatenate([f[FRESH:], pre(p, m), f[:FRESH]], axis=0)
            z = jnp.zeros_like(full)
            return jnp.where(col_a, full, z), jnp.where(col_a, z, full)

        def keys_t(blocks):
            fold = cat([jnp.concatenate([x[:, :128] if i % 2 == 0 else x[:, 256:], x[:, 128:256]],
                                        axis=1) for i, x in enumerate(blocks)])
            t = fold.T
            return t[:128].astype(BF16), t[128:].astype(BF16)

        def qk(q, kt, lane_a):
            outer = _dot(cat([q[:, :128], q[:, 256:]]).astype(BF16), kt[0])
            sc = (jnp.where(lane_a, outer[:SEG], outer[SEG:])
                  + _dot(q[:, 128:256].astype(BF16), kt[1]))
            if sc.shape[1] < 128:
                sc = jnp.concatenate([sc, jnp.zeros((SEG, 128 - sc.shape[1]), F32)], axis=1)
            return sc

        def row_max(raw, ok, other, first):
            sc = jnp.where(ok, raw * b_scale, other)
            ma = jnp.max(jnp.where(first, sc, ninf), axis=1, keepdims=True)
            mb = jnp.max(jnp.where(first, ninf, sc), axis=1, keepdims=True)
            return sc, ma, mb

        def probs(mx, first, late_norm):
            sc, ma, mb = mx
            e = jnp.exp2(sc - jnp.where(first, ma, mb))
            ea, eb = jnp.where(first, e, 0.0), jnp.where(first, 0.0, e)
            sa = jnp.sum(ea, axis=1, keepdims=True)
            sb = jnp.sum(eb, axis=1, keepdims=True)
            if late_norm:
                return e.astype(BF16), _recip(sa), _recip(sb)
            return (e * _recip(jnp.where(first, sa, sb))).astype(BF16), None, None

        def apply_v(e, blocks):
            pad = 128 - sum(x.shape[0] for x in blocks)
            rows = list(blocks) + ([jnp.zeros((pad, PW), F32)] if pad else [])
            return _dot(e, cat(rows).astype(BF16))

        def pv(sm, vbd):
            e, ra, rb = sm
            o = apply_v(e, vbd)
            if ra is not None:
                o = jnp.concatenate([
                    o[:, :128] * ra,
                    o[:, 128:256] * jnp.where(col128_a, ra, rb),
                    o[:, 256:] * rb], axis=1)
            return o

        def pre_pv(g, pr, vbds):
            o = apply_v(pr, [x[:MEM + PRE] for vb in vbds for x in vb])
            if not last:
                odef_s[u, g] = o
            return o

        def wout(p, o, acc):
            contrib = _dot(o.astype(BF16), _unpack(wo_s[p * hw:(p + 1) * hw, :]))
            return contrib if acc is None else acc + contrib

        def deferred(p):
            r = slice((p % GP) * PRE, (p % GP + 1) * PRE)
            return cat([odef_s[v, p // GP, r, :] for v in range(SPT - 1)]
                       + [val["PPV", p // GP][r]])

        def wout_strassen(kind, q):
            a11, a21 = val["PV", 2 * q], deferred(2 * q)
            if kind != "XA":
                a12, a22 = val["PV", 2 * q + 1], deferred(2 * q + 1)
            blk = lambda k, n: _unpack(
                wo_s[q * qr + k * hw:q * qr + (k + 1) * hw, n * KH:(n + 1) * KH])
            sm = lambda n: _unpack(wx_s[q, n])
            if kind == "XA":
                terms = {3: (a11, sm(1)), 6: (a21 - a11, sm(3))}
            elif kind == "XB":
                terms = {1: (a11 + a22, sm(0)), 4: (a22, sm(2)), 5: (a11 + a12, blk(1, 1)),
                         7: (a12 - a22, sm(4))}
            elif kind == "XC":
                terms = {2: (a21 + a22, blk(0, 0))}
            else:
                lhs = jnp.concatenate([cat([a11, a21]), cat([a12, a22])], axis=1)
                terms = {0: (lhs, _unpack(wo_s[q * qr:(q + 1) * qr, 2 * KH:]))}
            for n, (x, w) in terms.items():
                r = _dot(x.astype(BF16), w)
                val["acc", n] = val["acc", n] + r if ("acc", n) in val else r

        arow0 = pl.multiple_of((s - u % 2) * SEG, 2 * SEG)

        def a_put(m, j, r):
            if m == 0:
                qa_s[j] = r * a_scale
            else:
                kv_s[m - 1, j, A_HALO:A_HALO + 2 * SEG, :] = r

        def a_proj(idx):
            m, t = divmod(idx, 3)
            if "xa" not in val:
                xa = xa_s[pl.ds(arow0, 2 * SEG), :D]
                xf = xa.astype(F32)
                f = lambda i, k: xf[i * SEG:(i + 1) * SEG, k * KH:(k + 1) * KH]
                val["xa"] = xa
                val["xs"] = [v.astype(BF16) for v in (
                    f(0, 0) + f(1, 1), f(1, 0) + f(1, 1), f(0, 0), f(1, 1), f(0, 0) + f(0, 1),
                    f(1, 0) - f(0, 0), f(0, 1) - f(1, 1))]
                val["xr"] = xf[:, 2 * KH:].astype(BF16)
            if t == 2:
                a_put(m, NT - 1, _dot(val["xa"], _unpack(wa_s[m, :, (NT - 1) * 128:])))
                return
            sm = lambda n: _unpack(cat([wc_s[2 * m + k, t, :, n * 128:(n + 1) * 128]
                                        for k in range(2)]))
            blk = lambda k, j: _unpack(wa_s[m, k * KH // 2:(k + 1) * KH // 2,
                                            (2 * t + j) * 128:(2 * t + j + 1) * 128])
            rhs = (sm(0), blk(0, 0), sm(1), sm(2), blk(1, 1), sm(3), sm(4))
            mm = lambda n: _dot(val["xs"][n], rhs[n])
            tail = [_dot(val["xr"], _unpack(wa_s[m, KH:, (2 * t + j) * 128:(2 * t + j + 1) * 128]))
                    for j in range(2)]
            m1, m2, m3, m4, m5 = [mm(n) for n in range(5)]
            a_put(m, 2 * t, tail[0] + cat([mm(6) + (m1 + m4 - m5), m2 + m4]))
            a_put(m, 2 * t + 1, tail[1] + cat([m3 + m5, mm(5) + (m1 - m2 + m3)]))

        def window(m, j, w, hf):
            lo = A_HALO + hf * SEG - A_DIL * w
            return kv_s[m, j, lo:lo + SEG, :]

        def local_softmax(hf):
            pos = arow0 + hf * SEG + lax.broadcasted_iota(jnp.int32, (SEG, 128), 0)
            rows = slice(hf * SEG, (hf + 1) * SEG)
            logits = []
            for w in range(A_W):
                t = qa_s[0, rows, :] * window(0, 0, w, hf)
                for j in range(1, NT):
                    t = t + qa_s[j, rows, :] * window(0, j, w, hf)
                t = t + pltpu.roll(t, 64, 1)
                t = t + pltpu.roll(t, 32, 1)
                if w > 0 and hf == 0:
                    t = jnp.where(pos >= A_DIL * w, t, NEG)
                logits.append(t)
            mx = functools.reduce(jnp.maximum, logits)
            es = [jnp.exp2(l - mx) for l in logits]
            inv = _recip(functools.reduce(lambda x, y: x + y, es))
            return es, inv

        def local_pv(j, hf):
            es, inv = val["LA", hf]
            o = es[0] * window(1, j, 0, hf)
            for w in range(1, A_W):
                o = o + es[w] * window(1, j, w, hf)
            return o * inv

        def local_out(j, acc):
            wj = _unpack(awo_s[j * 64:(j + 1) * 64, :])
            r = _dot(cat([local_pv(j, 0), local_pv(j, 1)]).astype(BF16), wj)
            for m in range(2):
                kv_s[m, j, :A_HALO, :] = kv_s[m, j, 2 * SEG:2 * SEG + A_HALO, :]
            return r if acc is None else acc + r

        val = {}
        acc = None
        oa = None
        for kind, t in _order(u):
            if kind == "K":
                val[kind, t] = block_diag(t, 1)
            elif kind == "V":
                val[kind, t] = block_diag(t, 2)
            elif kind == "Q":
                val[kind, t] = proj(t, 0)
            elif kind == "T":
                val[kind, t] = keys_t(val["K", t])
            elif kind == "S":
                val[kind, t] = qk(val["Q", t], val["T", t], a80)
            elif kind == "M":
                val[kind, t] = row_max(val["S", t], allowed, fill, is_a)
            elif kind == "E":
                val[kind, t] = probs(val["M", t], is_a, t >= LATE_FROM)
            elif kind == "PV":
                val[kind, t] = pv(val["E", t], val["V", t])
            elif kind == "TG":
                val[kind, t] = keys_t([x[:MEM + PRE] for r in range(GP)
                                       for x in val["K", GP * t + r]])
            elif kind == "PS":
                q = cat([pre(GP * t + r, 0) for r in range(GP)])
                val[kind, t] = qk(q, val["TG", t], p_first)
            elif kind == "MG":
                val[kind, t] = row_max(val["PS", t], p_allowed, p_fill, p_first)
            elif kind == "EG":
                val[kind, t] = probs(val["MG", t], p_first, False)[0]
            elif kind == "PPV":
                val[kind, t] = pre_pv(t, val["EG", t], [val["V", GP * t + r] for r in range(GP)])
            elif kind == "W":
                acc = wout(t, val["PV", t], acc)
            elif kind in ("XA", "XB", "XC", "Y"):
                wout_strassen(kind, t)
            elif kind == "LA":
                val[kind, t] = local_softmax(t)
            elif kind == "AP":
                a_proj(t)
            elif kind == "AO":
                oa = local_out(t, oa)
                if t == NT - 1:
                    out_s[pl.ds(arow0, 2 * SEG), :D] = oa.astype(BF16)
                    out_copy(arow0, 2 * SEG, 0).start()
        if last:
            m = lambda n: val["acc", n]
            acc = jnp.concatenate([
                cat([m(1) + m(4) - m(5) + m(7), m(2) + m(4)]),
                cat([m(3) + m(5), m(1) - m(2) + m(3) + m(6)]), m(0)], axis=1)
        return acc

    def steps(i, mem):
        @pl.when(i == 1)
        def _():
            for cp in x_rest:
                cp.wait()

        accs = []
        for u in range(SPT):
            accs.append(segment(i * SPT + u, mem, u))
            mem = accs[-1][FRESH:SEG]
        res = cat([x for u in range(SPT) for x in (
            accs[-1][SEG + u * PRE:SEG + (u + 1) * PRE], accs[u][:FRESH])])
        row = pl.multiple_of(i * SPT * SEG, SPT * SEG)
        out_s[pl.ds(row, SPT * SEG), D:2 * D] = res.astype(BF16)
        out_copy(row, SPT * SEG, 1).start()
        return mem

    lax.fori_loop(0, N_STEPS, steps, mem0_s[...].astype(F32))

    wait_trip(0)
    wait_trip(1)

    done = N_STEPS * SPT * SEG
    pltpu.make_async_copy(out_s.at[:done, :2 * D], out_hbm.at[:done, :], sems.at[7]).wait()


@jax.jit
def pallas_concat_heads__sliding_local_dilated__memory_aug_recurrent_mem_tr__prompt_kernel(
    A_x: jax.Array,
    A_wqkv: jax.Array,
    A_wo: jax.Array,
    B_x: jax.Array,
    B_mem0: jax.Array,
    B_Wq: jax.Array,
    B_Wk: jax.Array,
    B_Wv: jax.Array,
    B_Wo: jax.Array,
    B_seg_len,
):
    del B_seg_len
    assert A_x.shape == (1, S, D) and B_x.shape == (1, S, D)
    hd = B_H * B_DH
    wq_t = jnp.transpose(B_Wq, (1, 2, 0)).reshape(hd, D)
    wk_t = jnp.transpose(B_Wk, (1, 2, 0)).reshape(hd, D)
    wv_t = jnp.transpose(B_Wv, (1, 2, 0)).reshape(hd, D)
    wo = B_Wo.reshape(hd, D)

    any_spec = pl.BlockSpec(memory_space=pl.ANY)
    out = pl.pallas_call(
        _kernel,
        out_shape=jax.ShapeDtypeStruct((S, 2 * D), BF16),
        in_specs=[any_spec] * 10,
        out_specs=any_spec,
        scratch_shapes=[
            pltpu.VMEM((2, PP, 4, PW, D), BF16),
            pltpu.VMEM((NT, D // 2, 128), U32),
            pltpu.VMEM((NP, D // 2, 3 * PW), U32),
            pltpu.VMEM((hd // 2 + PW, D), U32),
            pltpu.VMEM((NQ + 1, 5, PW // 2, KH), U32),
            pltpu.VMEM((NSEG, NP, PRE, 3 * PW), F32),
            pltpu.VMEM((SPT - 1, NG, GP * PRE, PW), F32),
            pltpu.VMEM((S, OUT_W), BF16),
            pltpu.VMEM((S, X_W), BF16),
            pltpu.VMEM((S, X_W), BF16),
            pltpu.VMEM((NSEG, PRE, D), BF16),
            pltpu.VMEM((NSEG * PRE // 2, D), U32),
            pltpu.VMEM((5, NSEG * PRE // 4, 256), U32),
            pltpu.VMEM((MEM, D), BF16),
            pltpu.VMEM((3, D // 2, D), U32),
            pltpu.VMEM((NTRIP, 2, 64, D), U32),
            pltpu.VMEM((D // 2, D), U32),
            pltpu.VMEM((PP, D // 2, 128), U32),
            pltpu.VMEM((NT, 2 * SEG, 128), F32),
            pltpu.VMEM((2, NT, KV_ROWS, 128), F32),
            pltpu.SemaphoreType.DMA((9,)),
        ],
        compiler_params=pltpu.CompilerParams(vmem_limit_bytes=120 * 1024 * 1024,
                                             disable_bounds_checks=True),
    )(A_x.reshape(S, D), A_wqkv, A_wo, B_x.reshape(S, D), B_x.reshape(NSEG, SEG // PRE, PRE, D),
      B_mem0.reshape(MEM, D), wq_t, wk_t, wv_t, wo)
    return out.reshape(1, S, 2 * D)
```

```python
import functools

import jax
import jax.numpy as jnp
from jax import lax
import jax.experimental.pallas as pl
import jax.experimental.pallas.tpu as pltpu

F32 = jnp.float32
BF16 = jnp.bfloat16
U32 = jnp.uint32

S = 2048
D = 640
NT = D // 128
A_H = 32
A_DH = D // A_H
A_W = 8
A_DIL = 2
A_HALO = 16
B_H = 32
B_DH = 192
MEM = 8
SEG = 32
NSEG = S // SEG
NP = B_H // 2
PW = 2 * B_DH
PRE = 8
FRESH = SEG - PRE
L = MEM + SEG
GP = 4
NG = NP // GP
LOG2E = 1.4426950408889634
NEG = -1000000000.0 * LOG2E
PP = 2
NTRIP = NP // PP - 1
PEEL = (2, 2, 5)
KH = 256
WO_ROWS = 512
WX_DONE = (0, 24, 56, 96, 120, 152, 192)
WX_TAIL = 2
WX_ROWS = 8
WX_SKIP = 0
ST_ROWS = 256
X_HEAD = 128
KV_ROWS = 80
X_W = 1024
OUT_W = 2048
SPT = 4
N_STEPS = NSEG // SPT
NQ = NP // 2

LAT_MM, LAT_X, LAT_T, LAT_N, LAT_N_LATE = 190, 190, 380, 230, 100
LATE_FROM = NP - 2
AP_AFTER = (6, 12, 18, 24, 30)
AO_AFTER = (30, 40)
TAIL_FILL = (2, 2, 2, 0)
HOLD_W = (0, 3, 0, 0)


def _segment_order(u):
    odd, last = u % 2 == 1, u == SPT - 1
    proj = []
    for g in range(NG):
        proj += [("K", GP * g + r) for r in range(GP)]
        for r in range(GP):
            proj += [("V", GP * g + r), ("Q", GP * g + r)]
    dur = {"K": 120, "V": 120, "Q": 120, "S": 24, "PV": 24, "PS": 24, "PPV": 24,
           "W": 120, "XA": 96, "XB": 192, "XC": 48, "Y": 96, "AO": 80, "AP": 90,
           "T": 0, "M": 0, "E": 0, "TG": 0, "MG": 0, "EG": 0}
    end = {}

    def ready(task):
        k, i = task
        if k == "T":
            deps = [(("K", i), LAT_MM)]
        elif k == "S":
            deps = [(("Q", i), LAT_MM), (("T", i), LAT_T)]
        elif k == "M":
            deps = [(("S", i), LAT_MM - 40)]
        elif k == "E":
            deps = [(("M", i), LAT_X)]
        elif k == "PV":
            deps = [(("E", i), LAT_N_LATE if i >= LATE_FROM else LAT_N), (("V", i), LAT_MM)]
        elif k == "TG":
            deps = [(("K", GP * i + r), LAT_MM) for r in range(GP)]
        elif k == "PS":
            deps = [(("TG", i), LAT_T)]
        elif k == "MG":
            deps = [(("PS", i), LAT_MM - 40)]
        elif k == "EG":
            deps = [(("MG", i), LAT_X)]
        elif k == "PPV":
            deps = [(("EG", i), LAT_N), (("V", GP * i + GP - 1), LAT_MM)]
        elif k == "W":
            deps = [(("PV", i), LAT_MM)]
        else:
            deps = [(("PV", 2 * i), LAT_MM), (("PPV", 2 * i // GP), LAT_MM)]
            if k != "XA":
                deps.append((("PV", 2 * i + 1), LAT_MM))
        if any(d not in end for d, _ in deps):
            return None
        return max(end[d] + lat for d, lat in deps)

    pend = ([(k, p) for k in ("E", "M", "T") for p in range(NP)]
            + [(k, g) for k in ("EG", "MG", "TG") for g in range(NG)]
            + ([(k, q) for q in range(NQ) for k in ("XA", "XB", "Y", "XC")] if last
               else [("W", p) for p in range(NP)])
            + [("PPV", g) for g in range(NG)]
            + [("PV", p) for p in range(NP)] + [("PS", g) for g in range(NG)]
            + [("S", p) for p in range(NP)])
    fill = [("AO", j) for j in range(NT)] if odd else [("AP", j) for j in (5, 6, 7, 8, 9, 0, 1, 2, 3, 4, 10, 12, 14)]
    order = []
    now = [0]

    def emit(task):
        order.append(task)
        now[0] += dur[task[0]]
        end[task] = now[0]

    nproj = 0
    while pend:
        cand = [x for x in pend if ready(x) is not None and ready(x) <= now[0]]
        if proj:
            cand = [x for x in cand if not (x[0] == "W" and x[1] >= NP - GP - HOLD_W[u])]
        if cand:
            if not proj:
                cand = [x for x in cand if x[0] not in ("W", "XA", "XB", "XC", "Y")] or cand
            pend.remove(cand[0])
            emit(cand[0])
        elif proj:
            emit(proj.pop(0))
            nproj += 1
            if odd and nproj == GP:
                order += [("LA", 0), ("LA", 1)]
            if nproj in (AO_AFTER if odd else AP_AFTER):
                emit(fill.pop(0))
        elif len(fill) > TAIL_FILL[u]:
            emit(fill.pop(0))
        else:
            now[0] = min(ready(x) for x in pend if ready(x) is not None)
    return order + fill


ORDERS = (
    "K0 T0 K1 K2 K3 V0 T1 T2 Q1 T3 Q0 AP5 AP6 S0 TG0 M0 PS0 V1 Q2 V2 V3 E0 MG0 S1 S2 M1 K4 Q3 EG0 "
    "PV0 K5 E1 M2 S3 K6 T4 W0 E2 M3 T5 PPV0 PV1 K7 AP7 AP8 E3 T6 W1 T7 TG1 PV2 PV3 Q4 W2 V4 W3 "
    "PS1 S4 Q5 V5 M4 MG1 V6 Q7 Q6 E4 S5 EG1 V7 M5 PV4 S6 K8 PPV1 E5 S7 M6 W4 K9 E6 M7 T8 K10 PV5 "
    "AP9 T9 K11 E7 W5 T10 PV6 TG2 V8 T11 PV7 Q8 W7 W6 S8 PS2 V10 V9 Q9 M8 MG2 Q10 E8 EG2 V11 S9 "
    "Q11 M9 PV8 S10 K12 T12 PPV2 E9 S11 M10 W8 E10 M11 PV9 K14 K13 K15 E11 T13 W9 PV10 V12 T14 "
    "T15 TG3 PV11 Q12 W10 W11 PS3 S12 Q13 V13 M12 MG3 V15 V14 E12 Q14 EG3 Q15 S13 M13 PV12 S14 "
    "AP0 AP1 PPV3 E13 S15 M14 W12 AP2 AP3 E14 PV13 M15 AP4 AP10 PV14 W13 E15 PV15 W14 W15 AP14 "
    "AP12 ",
    "K0 K1 K2 T0 K3 LA0 LA1 Q0 V1 T1 V0 T2 T3 TG0 Q1 S0 V2 PS0 Q2 M0 S1 V3 MG0 Q3 M1 S2 K4 EG0 K5 "
    "E0 E1 M2 PV0 S3 K6 T4 PPV0 E2 T5 K7 M3 W0 T6 PV1 PV2 V4 E3 T7 TG1 Q4 W1 W2 PV3 PS1 S4 V5 Q5 "
    "M4 MG1 W3 AO0 S5 V6 E4 EG1 Q6 M5 V7 PV4 Q7 E5 S6 K8 W4 M6 PPV1 PV5 S7 T8 K9 E6 K10 M7 W5 T9 "
    "PV6 K11 E7 T10 V8 W6 T11 TG2 PV7 Q8 AO1 W7 S8 V9 PS2 Q9 M8 V10 MG2 Q10 E8 S9 V11 EG2 Q11 PV8 "
    "M9 S10 K12 PPV2 E9 S11 M10 K13 W8 E10 M11 T12 PV9 K14 K15 E11 T13 T14 PV10 AO2 V12 T15 TG3 "
    "Q12 PV11 V13 Q13 PS3 S12 V14 Q14 M12 S13 MG3 V15 Q15 E12 M13 EG3 S14 W9 E13 M14 PPV3 W10 "
    "PV12 S15 W11 E14 M15 PV13 W12 PV14 E15 W13 PV15 W14 W15 AO3 AO4 ",
    "K0 K2 K1 T0 K3 T1 AP5 AP6 V0 Q0 TG0 T3 T2 V1 S0 Q1 PS0 Q2 V2 M0 S1 V3 E0 MG0 Q3 M1 K4 S2 EG0 "
    "PV0 K5 E1 M2 PPV0 S3 K6 T4 W0 E2 M3 T5 AP7 AP8 PV1 K7 E3 W1 T6 T7 TG1 PV2 V4 PV3 Q4 W2 W3 "
    "PS1 S4 V5 M4 Q5 MG1 V6 S5 Q6 EG1 E4 V7 Q7 M5 PV4 S6 K8 PPV1 E5 S7 M6 W4 AP9 K9 E6 M7 T8 PV5 "
    "K10 T9 K11 E7 W5 T10 PV6 V8 T11 TG2 PV7 Q8 W6 W7 S8 PS2 V9 Q9 M8 MG2 V10 Q10 E8 EG2 S9 V11 "
    "Q11 M9 PV8 S10 K12 PPV2 E9 W8 S11 M10 K13 E10 M11 T12 PV9 K14 K15 E11 T13 W9 PV11 T14 PV10 "
    "V12 T15 TG3 Q12 W10 V13 W11 PS3 S12 MG3 Q13 M12 V14 Q14 E12 EG3 S13 V15 Q15 M13 PV12 S14 E13 "
    "AP0 AP1 PPV3 S15 M14 AP2 AP3 W12 M15 AP4 E14 PV13 PV14 AP10 E15 W13 PV15 W14 W15 AP12 AP14 ",
    "K1 K0 K2 T0 K3 LA0 LA1 T1 V0 T2 Q0 T3 TG0 V1 Q1 S0 PS0 V2 Q2 M0 V3 MG0 Q3 S1 E0 M1 S2 EG0 K4 "
    "K5 M2 T4 PV0 E1 AO0 PPV0 S3 K6 E2 T5 K7 M3 XA0 T6 PV1 PV2 V4 E3 T7 TG1 Y0 Q4 XB0 XC0 XA1 PV3 "
    "PS1 S4 V5 Q5 M4 MG1 XB1 E4 Y1 XC1 EG1 S5 Q6 V6 M5 V7 S6 PV4 AO1 Q7 E5 PPV1 K8 S7 M6 XA2 K9 "
    "M7 T8 PV5 K10 E6 T9 XB2 E7 T10 Y2 K11 TG2 T11 XC2 PV6 PV7 V8 Q8 XA3 XB3 Y3 PS2 S8 V9 Q9 M8 "
    "MG2 V10 Q10 AO2 E8 EG2 S9 V11 S10 M9 PV8 K12 Q11 M10 PPV2 K13 E9 K14 S11 E10 T12 M11 T13 K15 "
    "PV9 XA4 T14 PV10 V12 E11 XB4 T15 TG3 XA5 Y4 Q12 AO3 PV11 XB5 PS3 S12 V13 Q13 MG3 V14 M12 Q14 "
    "EG3 S13 V15 E12 M13 PV12 Q15 S14 AO4 PPV3 E13 S15 M14 E14 XA6 M15 XC3 XC4 XC5 PV13 E15 Y5 "
    "PV14 XB6 PV15 XC6 Y6 XA7 XB7 Y7 XC7 ",
)
SKIP_PROLOGUE = False


def _order(u):
    if ORDERS is None or ORDERS[u] is None:
        return _segment_order(u)
    return [(t.rstrip("0123456789"), int(t.lstrip("ABCDEFGHIJKLMNOPQRSTUVWXYZ")))
            for t in ORDERS[u].split()]


def _nt_dot(a, b):
    return lax.dot_general(a, b, (((1,), (1,)), ((), ())), preferred_element_type=F32)


def _dot(a, b):
    return jnp.dot(a, b, preferred_element_type=F32)


def _pack(x):
    return pltpu.bitcast(x, U32)


def _unpack(x):
    return pltpu.bitcast(x, BF16)


def cat(parts):
    return jnp.concatenate(parts, axis=0)


def _round(x):
    return x.astype(BF16).astype(F32)


def _recip(x):
    r = pl.reciprocal(x, approx=True)
    return r * (2.0 - x * r)


def _kernel(ax_hbm, awqkv_hbm, awo_hbm, bx_hbm, bx4_hbm, mem0_hbm, wq_hbm, wk_hbm, wv_hbm, wo_hbm,
            out_hbm,
            stage, awo_raw, w_s, wo_s, wx_s, pre_s, odef_s, out_s,
            xa_s, xb_s, xpre_s, xp_s, xs_s, mem0_s, wa_s, wc_s, awo_s, t1_s, qa_s, kv_s,
            sems):
    b_scale = 0.072265625 * LOG2E
    a_scale = 0.2236328125

    w_hbm = (wq_hbm, wk_hbm, wv_hbm)
    wo32 = wo_hbm.bitcast(U32)
    awo32 = awo_hbm.bitcast(U32)
    hw = PW // 2
    hd = B_H * B_DH

    def w_copy(p, half, q, m, sem):
        rows = pl.ds(pl.multiple_of(p * PW, PW), PW)
        return pltpu.make_async_copy(w_hbm[m].at[rows, :], stage.at[half, q, m], sem)

    def wa_piece(g, q):
        last = g >= 2 * 3
        return jnp.where(last, 1 + q, g >> 1), jnp.where(last, NT - 1, (g & 1) + 2 * q)

    def wa_copy(c, kt, half, q, sem):
        return pltpu.make_async_copy(
            awqkv_hbm.at[pl.ds(pl.multiple_of(kt * 128, 128), 128),
                         pl.ds(pl.multiple_of(c * D, 128), D)],
            stage.at[half, q, 3, :128], sem)

    def start_trip(g):
        half = g & 1
        src = jnp.minimum(g, NTRIP - 1)
        for q in range(PP):
            for m in range(3):
                w_copy((src + 1) * PP + q, half, q, m, sems.at[half]).start(priority=1)
            wa_copy(*wa_piece(src, q), half, q, sems.at[half]).start(priority=1)

    def wait_trip(half):
        for view in (stage.at[half, :, :3], stage.at[half, :, 3, :128]):
            pltpu.make_async_copy(view, view, sems.at[half]).wait()

    qr = 2 * hw

    def wo_copy(start, n, sem):
        wr = pl.ds(pl.multiple_of(start, 8), n)
        return pltpu.make_async_copy(wo32.at[wr, :], wo_s.at[wr, :], sem)

    def wo_sums(q, piece, anchor=None, never=None):
        def blk(k, n):
            w = wo_s[pl.ds(pl.multiple_of(q * qr + k * hw + piece * WX_ROWS, 8), WX_ROWS),
                     n * KH:(n + 1) * KH]
            if anchor is not None:
                w = jnp.where(never, anchor, w)
            return _unpack(w).astype(F32)

        b11, b12, b21, b22 = blk(0, 0), blk(0, 1), blk(1, 0), blk(1, 1)
        for n, v in enumerate((b11 + b22, b12 - b22, b21 - b11, b11 + b12, b21 + b22)):
            wx_s[q, n, pl.ds(pl.multiple_of(piece * WX_ROWS, 8), WX_ROWS), :] = (
                _pack(v.astype(BF16)))

    def x_copies(xr, sem):
        return [pltpu.make_async_copy(ax_hbm.at[xr, :], xa_s.at[xr, :D], sem),
                pltpu.make_async_copy(bx_hbm.at[xr, :], xb_s.at[xr, :D], sem)]

    xpre_cp = pltpu.make_async_copy(bx4_hbm.at[:, 0], xpre_s, sems.at[3])
    late_cps = ([pltpu.make_async_copy(mem0_hbm, mem0_s, sems.at[2])]
                + x_copies(pl.ds(0, X_HEAD), sems.at[2]))
    awo_cps = [
        pltpu.make_async_copy(awo32.at[:, c * 128:(c + 1) * 128], awo_raw.at[c], sems.at[2])
        for c in range(NT)]
    x_rest = x_copies(pl.ds(X_HEAD, S - X_HEAD), sems.at[3])
    tiles = [(m, j) for m in range(3) for j in range(PW // 128)]
    peel = [tiles[sum(PEEL[:n]):sum(PEEL[:n + 1])] for n in range(len(PEEL))]
    peel_cps = [[pltpu.make_async_copy(w_hbm[m].at[pl.ds(q * PW + j * 128, 128), :],
                                       stage.at[1, q, m, pl.ds(j * 128, 128), :], sems.at[4 + n])
                 for m, j in blk for q in range(PP)] for n, blk in enumerate(peel)]
    peel_cps[-1].append(wa_copy(0, NT - 1, 1, 0, sems.at[3 + len(PEEL)]))

    xpre_cp.start()
    for cps in peel_cps:
        for cp in cps:
            cp.start(priority=1)
    start_trip(0)
    for cp in late_cps:
        cp.start(priority=1)
    kv_s[:, :, :A_HALO, :] = jnp.zeros((2, NT, A_HALO, 128), F32)
    wo_s[NQ * qr:, :] = jnp.zeros((qr, D), U32)

    def gather_heads(ref):
        rows = []
        for j in range(A_DH // 2):
            u = ref[pl.ds(j, A_H, stride=A_DH // 2), :]
            rows.append(pltpu.bitcast(u << 16, F32))
            rows.append(pltpu.bitcast(u & jnp.uint32(0xFFFF0000), F32))
        return jnp.concatenate(rows, axis=0)

    HR = NSEG * PRE // 2

    def xq(i, k):
        return _unpack(xp_s[i * HR // 2:(i + 1) * HR // 2, k * KH:(k + 1) * KH])

    def strassen_lhs():
        f = lambda i, k: xq(i, k).astype(F32)
        sums = (f(0, 0) + f(1, 1), f(1, 0) + f(1, 1), f(0, 0) + f(0, 1),
                f(1, 0) - f(0, 0), f(0, 1) - f(1, 1))
        for n, v in enumerate(sums):
            xs_s[n] = _pack(v.astype(BF16))

    def pair_prep2(p, half, m, js=(0, 1, 2), hook=None):
        if SKIP_PROLOGUE:
            return
        for q in range(2):
            lo, hi = js[0] * 128, (js[-1] + 1) * 128
            w_s[p + q, :, m * PW + lo:m * PW + hi] = _pack(stage[half, q, m, lo:hi, :].T)
        nseg = ST_ROWS // PRE
        for j in js:
            rows = slice(j * 128, (j + 1) * 128)
            b = lambda k, q: stage[half, q, m, rows, k * KH:(k + 1) * KH]
            bf = lambda k, q: b(k, q).astype(F32)
            rhs = ((bf(0, 0) + bf(1, 1)).astype(BF16), b(0, 0),
                   (bf(0, 1) - bf(1, 1)).astype(BF16), (bf(1, 0) - bf(0, 0)).astype(BF16),
                   b(1, 1), (bf(0, 0) + bf(0, 1)).astype(BF16),
                   (bf(1, 0) + bf(1, 1)).astype(BF16))
            tail = [stage[half, q, m, rows, 2 * KH:] for q in range(2)]
            for c in range(HR // ST_ROWS):
                r = slice(c * ST_ROWS // 2, (c + 1) * ST_ROWS // 2)
                sm = lambda n: _unpack(xs_s[n, r, :])
                qd = lambda i, k: _unpack(
                    xp_s[(i * HR + c * ST_ROWS) // 2:(i * HR + (c + 1) * ST_ROWS) // 2,
                         k * KH:(k + 1) * KH])
                rest = lambda i: _unpack(
                    xp_s[(i * HR + c * ST_ROWS) // 2:(i * HR + (c + 1) * ST_ROWS) // 2, 2 * KH:])

                def put(i, q, v):
                    s0 = i * (NSEG // 2) + c * nseg
                    pre_s[s0:s0 + nseg, p + q, :, m * PW + j * 128:m * PW + (j + 1) * 128] = (
                        v.reshape(nseg, PRE, 128))
                    if hook is not None:
                        hook(v)

                m5 = _nt_dot(sm(2), rhs[4])
                m3 = _nt_dot(qd(0, 0), rhs[2])
                put(0, 1, _nt_dot(rest(0), tail[1]) + m3 + m5)
                m1 = _nt_dot(sm(0), rhs[0])
                m4 = _nt_dot(qd(1, 1), rhs[3])
                put(0, 0, _nt_dot(rest(0), tail[0]) + _nt_dot(sm(4), rhs[6]) + (m1 + m4 - m5))
                m2 = _nt_dot(sm(1), rhs[1])
                put(1, 0, _nt_dot(rest(1), tail[0]) + m2 + m4)
                put(1, 1, _nt_dot(rest(1), tail[1]) + _nt_dot(sm(3), rhs[5]) + (m1 - m2 + m3))

    def wa_prep(c, kt, half, q):
        t1_s[q] = _pack(stage[half, q, 3, :128].T)
        g = gather_heads(t1_s.at[q])
        wa_s[c, pl.ds(pl.multiple_of(kt * 64, 64), 64), :] = _pack(g.astype(BF16).T)
        return g

    def wa_trip(g, half):
        lo, hi = [wa_prep(*wa_piece(g, q), half, q) for q in range(2)]
        for t in range(2):
            b11, b12 = lo[2 * t * 128:(2 * t + 1) * 128], lo[(2 * t + 1) * 128:(2 * t + 2) * 128]
            b21, b22 = hi[2 * t * 128:(2 * t + 1) * 128], hi[(2 * t + 1) * 128:(2 * t + 2) * 128]
            sums = cat([b11 + b22, b12 - b22, b21 - b11, b11 + b12, b21 + b22])
            wc_s[g, t] = _pack(sums.astype(BF16).T)

    xpre_cp.wait()
    xp_s[...] = _pack(xpre_s[...].reshape(NSEG * PRE, D))
    strassen_lhs()
    for blk, cps in zip(peel, peel_cps):
        for cp in cps:
            cp.wait()
        for m in range(3):
            js = tuple(j for mm, j in blk if mm == m)
            if js:
                pair_prep2(0, 1, m, js)
    wa_prep(0, NT - 1, 1, 0)
    start_trip(1)

    def prologue(g, carry):
        half = g & 1

        @pl.when(g > 0)
        def _():
            wo_copy((g - 1) * WO_ROWS, WO_ROWS, sems.at[8]).wait()

        @pl.when(g == NTRIP - 1)
        def _():
            for cp in awo_cps:
                cp.start(priority=1)

        @pl.when(g < NTRIP - 1)
        def _():
            wo_copy(g * WO_ROWS, WO_ROWS, sems.at[8]).start()

        wait_trip(half)
        calls = [0]
        per = hw // WX_ROWS
        total = max(b - a for a, b in zip(WX_DONE, WX_DONE[1:]))
        todo = list(range(total))
        first, stop = NQ * per, (NQ + 1) * per
        for trip in range(1, NTRIP):
            first = jnp.where(g == trip, WX_DONE[trip - 1], first)
            stop = jnp.where(g == trip, WX_DONE[trip], stop)

        def hook(v):
            calls[0] += 1
            want = (calls[0] - WX_SKIP) * total // (36 - WX_SKIP - WX_TAIL)
            t = 0
            while todo and todo[0] < want:
                k = jnp.minimum(first + todo.pop(0), stop - 1)
                q = k // per
                anchor = jnp.concatenate(
                    [v[(2 * t + c) * WX_ROWS:(2 * t + c + 1) * WX_ROWS] for c in range(2)], axis=1)
                wo_sums(q, k % per, pltpu.bitcast(anchor, U32), g > NSEG)
                t += 1

        for m in range(3):
            pair_prep2((g + 1) * PP, half, m, hook=hook)
            if m == 0:
                wa_trip(g, half)
        start_trip(g + 2)
        return carry

    lax.fori_loop(0, NTRIP, prologue, 0)

    for cp in late_cps + awo_cps:
        cp.wait()
    for cp in x_rest:
        cp.start()

    for c in range(NT):
        awo_s[:, c * 128:(c + 1) * 128] = _pack(gather_heads(awo_raw.at[c]).astype(BF16))

    def out_copy(row, n, half):
        r = pl.ds(row, n)
        c = slice(half * D, (half + 1) * D)
        return pltpu.make_async_copy(out_s.at[r, c], out_hbm.at[r, c], sems.at[7])

    def segment(s, mem, u):
        last = u == SPT - 1
        row0 = pl.multiple_of(s * SEG, SEG)
        ninf = jnp.float32(-jnp.inf)

        qi = lax.broadcasted_iota(jnp.int32, (SEG, 128), 0)
        kl = lax.broadcasted_iota(jnp.int32, (SEG, 128), 1)
        is_a = kl < L
        a80 = lax.broadcasted_iota(jnp.int32, (SEG, 2 * L), 1) < L
        real = kl < 2 * L
        kpos = jnp.where(is_a, kl, kl - L)
        allowed = ((qi >= FRESH) | (qi + MEM + PRE >= kpos)) & real
        fill = jnp.where(real, NEG, ninf)
        pi = lax.broadcasted_iota(jnp.int32, (GP * PRE, 128), 0)
        pk = lax.broadcasted_iota(jnp.int32, (GP * PRE, 128), 1)
        p_own = (pk // SEG) == (pi // PRE)
        p_allowed = (pk % (MEM + PRE)) <= (pi % PRE) + MEM
        p_first = (pk % SEG) < MEM + PRE
        p_allowed = p_allowed & p_own
        p_fill = jnp.where(p_own, NEG, ninf)
        col_a = lax.broadcasted_iota(jnp.int32, (1, PW), 1) < B_DH
        col128_a = lax.broadcasted_iota(jnp.int32, (1, 128), 1) < (B_DH - 128)

        xb = xb_s[pl.ds(row0, SEG), :D].astype(F32)
        h = jnp.concatenate([xb[PRE:], mem], axis=0).astype(BF16)

        def proj(p, m):
            return _dot(h, _unpack(w_s[p, :, m * PW:(m + 1) * PW]))

        def pre(p, m):
            return pre_s[s, p, :, m * PW:(m + 1) * PW]

        def block_diag(p, m):
            f = proj(p, m)
            full = jnp.concatenate([f[FRESH:], pre(p, m), f[:FRESH]], axis=0)
            z = jnp.zeros_like(full)
            return jnp.where(col_a, full, z), jnp.where(col_a, z, full)

        def keys_t(blocks):
            fold = cat([jnp.concatenate([x[:, :128] if i % 2 == 0 else x[:, 256:], x[:, 128:256]],
                                        axis=1) for i, x in enumerate(blocks)])
            t = fold.T
            return t[:128].astype(BF16), t[128:].astype(BF16)

        def qk(q, kt, lane_a):
            outer = _dot(cat([q[:, :128], q[:, 256:]]).astype(BF16), kt[0])
            sc = (jnp.where(lane_a, outer[:SEG], outer[SEG:])
                  + _dot(q[:, 128:256].astype(BF16), kt[1]))
            if sc.shape[1] < 128:
                sc = jnp.concatenate([sc, jnp.zeros((SEG, 128 - sc.shape[1]), F32)], axis=1)
            return sc

        def row_max(raw, ok, other, first):
            sc = jnp.where(ok, raw * b_scale, other)
            ma = jnp.max(jnp.where(first, sc, ninf), axis=1, keepdims=True)
            mb = jnp.max(jnp.where(first, ninf, sc), axis=1, keepdims=True)
            return sc, ma, mb

        def probs(mx, first, late_norm):
            sc, ma, mb = mx
            e = jnp.exp2(sc - jnp.where(first, ma, mb))
            ea, eb = jnp.where(first, e, 0.0), jnp.where(first, 0.0, e)
            sa = jnp.sum(ea, axis=1, keepdims=True)
            sb = jnp.sum(eb, axis=1, keepdims=True)
            if late_norm:
                return e.astype(BF16), _recip(sa), _recip(sb)
            return (e * _recip(jnp.where(first, sa, sb))).astype(BF16), None, None

        def apply_v(e, blocks):
            pad = 128 - sum(x.shape[0] for x in blocks)
            rows = list(blocks) + ([jnp.zeros((pad, PW), F32)] if pad else [])
            return _dot(e, cat(rows).astype(BF16))

        def pv(sm, vbd):
            e, ra, rb = sm
            o = apply_v(e, vbd)
            if ra is not None:
                o = jnp.concatenate([
                    o[:, :128] * ra,
                    o[:, 128:256] * jnp.where(col128_a, ra, rb),
                    o[:, 256:] * rb], axis=1)
            return o

        def pre_pv(g, pr, vbds):
            o = apply_v(pr, [x[:MEM + PRE] for vb in vbds for x in vb])
            if not last:
                odef_s[u, g] = o
            return o

        def wout(p, o, acc):
            contrib = _dot(o.astype(BF16), _unpack(wo_s[p * hw:(p + 1) * hw, :]))
            return contrib if acc is None else acc + contrib

        def deferred(p):
            r = slice((p % GP) * PRE, (p % GP + 1) * PRE)
            return cat([odef_s[v, p // GP, r, :] for v in range(SPT - 1)]
                       + [val["PPV", p // GP][r]])

        def wout_strassen(kind, q):
            a11, a21 = val["PV", 2 * q], deferred(2 * q)
            if kind != "XA":
                a12, a22 = val["PV", 2 * q + 1], deferred(2 * q + 1)
            blk = lambda k, n: _unpack(
                wo_s[q * qr + k * hw:q * qr + (k + 1) * hw, n * KH:(n + 1) * KH])
            sm = lambda n: _unpack(wx_s[q, n])
            if kind == "XA":
                terms = {3: (a11, sm(1)), 6: (a21 - a11, sm(3))}
            elif kind == "XB":
                terms = {1: (a11 + a22, sm(0)), 4: (a22, sm(2)), 5: (a11 + a12, blk(1, 1)),
                         7: (a12 - a22, sm(4))}
            elif kind == "XC":
                terms = {2: (a21 + a22, blk(0, 0))}
            else:
                lhs = jnp.concatenate([cat([a11, a21]), cat([a12, a22])], axis=1)
                terms = {0: (lhs, _unpack(wo_s[q * qr:(q + 1) * qr, 2 * KH:]))}
            for n, (x, w) in terms.items():
                r = _dot(x.astype(BF16), w)
                val["acc", n] = val["acc", n] + r if ("acc", n) in val else r

        arow0 = pl.multiple_of((s - u % 2) * SEG, 2 * SEG)

        def a_put(m, j, r):
            if m == 0:
                qa_s[j] = _round(r)
            else:
                kv_s[m - 1, j, A_HALO:A_HALO + 2 * SEG, :] = _round(r) if m == 1 else r

        def a_proj(idx):
            m, j = divmod(idx, NT)
            if "xa" not in val:
                val["xa"] = xa_s[pl.ds(arow0, 2 * SEG), :D]
            if m < 2 or j == NT - 1:
                a_put(m, j, _dot(val["xa"], _unpack(wa_s[m, :, j * 128:(j + 1) * 128])))
                return
            t = j // 2
            if "xs" not in val:
                xf = val["xa"].astype(F32)
                f = lambda i, k: xf[i * SEG:(i + 1) * SEG, k * KH:(k + 1) * KH]
                val["xs"] = [v.astype(BF16) for v in (
                    f(0, 0) + f(1, 1), f(1, 0) + f(1, 1), f(0, 0), f(1, 1), f(0, 0) + f(0, 1),
                    f(1, 0) - f(0, 0), f(0, 1) - f(1, 1))]
                val["xr"] = xf[:, 2 * KH:].astype(BF16)
            sm = lambda n: _unpack(cat([wc_s[2 * m + k, t, :, n * 128:(n + 1) * 128]
                                        for k in range(2)]))
            blk = lambda k, j: _unpack(wa_s[m, k * KH // 2:(k + 1) * KH // 2,
                                            (2 * t + j) * 128:(2 * t + j + 1) * 128])
            rhs = (sm(0), blk(0, 0), sm(1), sm(2), blk(1, 1), sm(3), sm(4))
            mm = lambda n: _dot(val["xs"][n], rhs[n])
            tail = [_dot(val["xr"], _unpack(wa_s[m, KH:, (2 * t + j) * 128:(2 * t + j + 1) * 128]))
                    for j in range(2)]
            m1, m2, m3, m4, m5 = [mm(n) for n in range(5)]
            a_put(m, 2 * t, tail[0] + cat([mm(6) + (m1 + m4 - m5), m2 + m4]))
            a_put(m, 2 * t + 1, tail[1] + cat([m3 + m5, mm(5) + (m1 - m2 + m3)]))

        def window(m, j, w, hf):
            lo = A_HALO + hf * SEG - A_DIL * w
            return kv_s[m, j, lo:lo + SEG, :]

        def local_softmax(hf):
            pos = arow0 + hf * SEG + lax.broadcasted_iota(jnp.int32, (SEG, 128), 0)
            rows = slice(hf * SEG, (hf + 1) * SEG)
            logits = []
            for w in range(A_W):
                t = qa_s[0, rows, :] * window(0, 0, w, hf)
                for j in range(1, NT):
                    t = t + qa_s[j, rows, :] * window(0, j, w, hf)
                t = t + pltpu.roll(t, 64, 1)
                t = t + pltpu.roll(t, 32, 1)
                t = _round(_round(t) * a_scale)
                if w > 0 and hf == 0:
                    t = jnp.where(pos >= A_DIL * w, t, -1000000000.0)
                logits.append(t)
            mx = functools.reduce(jnp.maximum, logits)
            es = [jnp.exp(l - mx) for l in logits]
            inv = _recip(functools.reduce(lambda x, y: x + y, es))
            return es, inv

        def local_pv(j, hf):
            es, inv = val["LA", hf]
            o = es[0] * window(1, j, 0, hf)
            for w in range(1, A_W):
                o = o + es[w] * window(1, j, w, hf)
            return o * inv

        def local_out(j, acc):
            wj = _unpack(awo_s[j * 64:(j + 1) * 64, :])
            r = _dot(cat([local_pv(j, 0), local_pv(j, 1)]).astype(BF16), wj)
            for m in range(2):
                kv_s[m, j, :A_HALO, :] = kv_s[m, j, 2 * SEG:2 * SEG + A_HALO, :]
            return r if acc is None else acc + r

        val = {}
        acc = None
        oa = None
        for kind, t in _order(u):
            if kind == "K":
                val[kind, t] = block_diag(t, 1)
            elif kind == "V":
                val[kind, t] = block_diag(t, 2)
            elif kind == "Q":
                val[kind, t] = proj(t, 0)
            elif kind == "T":
                val[kind, t] = keys_t(val["K", t])
            elif kind == "S":
                val[kind, t] = qk(val["Q", t], val["T", t], a80)
            elif kind == "M":
                val[kind, t] = row_max(val["S", t], allowed, fill, is_a)
            elif kind == "E":
                val[kind, t] = probs(val["M", t], is_a, t >= LATE_FROM)
            elif kind == "PV":
                val[kind, t] = pv(val["E", t], val["V", t])
            elif kind == "TG":
                val[kind, t] = keys_t([x[:MEM + PRE] for r in range(GP)
                                       for x in val["K", GP * t + r]])
            elif kind == "PS":
                q = cat([pre(GP * t + r, 0) for r in range(GP)])
                val[kind, t] = qk(q, val["TG", t], p_first)
            elif kind == "MG":
                val[kind, t] = row_max(val["PS", t], p_allowed, p_fill, p_first)
            elif kind == "EG":
                val[kind, t] = probs(val["MG", t], p_first, False)[0]
            elif kind == "PPV":
                val[kind, t] = pre_pv(t, val["EG", t], [val["V", GP * t + r] for r in range(GP)])
            elif kind == "W":
                acc = wout(t, val["PV", t], acc)
            elif kind in ("XA", "XB", "XC", "Y"):
                wout_strassen(kind, t)
            elif kind == "LA":
                val[kind, t] = local_softmax(t)
            elif kind == "AP":
                a_proj(t)
            elif kind == "AO":
                oa = local_out(t, oa)
                if t == NT - 1:
                    out_s[pl.ds(arow0, 2 * SEG), :D] = oa.astype(BF16)
                    out_copy(arow0, 2 * SEG, 0).start()
        if last:
            m = lambda n: val["acc", n]
            acc = jnp.concatenate([
                cat([m(1) + m(4) - m(5) + m(7), m(2) + m(4)]),
                cat([m(3) + m(5), m(1) - m(2) + m(3) + m(6)]), m(0)], axis=1)
        return acc

    def steps(i, mem):
        @pl.when(i == 1)
        def _():
            for cp in x_rest:
                cp.wait()

        accs = []
        for u in range(SPT):
            accs.append(segment(i * SPT + u, mem, u))
            mem = accs[-1][FRESH:SEG]
        res = cat([x for u in range(SPT) for x in (
            accs[-1][SEG + u * PRE:SEG + (u + 1) * PRE], accs[u][:FRESH])])
        row = pl.multiple_of(i * SPT * SEG, SPT * SEG)
        out_s[pl.ds(row, SPT * SEG), D:2 * D] = res.astype(BF16)
        out_copy(row, SPT * SEG, 1).start()
        return mem

    lax.fori_loop(0, N_STEPS, steps, mem0_s[...].astype(F32))

    wait_trip(0)
    wait_trip(1)

    done = N_STEPS * SPT * SEG
    pltpu.make_async_copy(out_s.at[:done, :2 * D], out_hbm.at[:done, :], sems.at[7]).wait()


@jax.jit
def pallas_concat_heads__sliding_local_dilated__memory_aug_recurrent_mem_tr__prompt_kernel(
    A_x: jax.Array,
    A_wqkv: jax.Array,
    A_wo: jax.Array,
    B_x: jax.Array,
    B_mem0: jax.Array,
    B_Wq: jax.Array,
    B_Wk: jax.Array,
    B_Wv: jax.Array,
    B_Wo: jax.Array,
    B_seg_len,
):
    del B_seg_len
    assert A_x.shape == (1, S, D) and B_x.shape == (1, S, D)
    hd = B_H * B_DH
    wq_t = jnp.transpose(B_Wq, (1, 2, 0)).reshape(hd, D)
    wk_t = jnp.transpose(B_Wk, (1, 2, 0)).reshape(hd, D)
    wv_t = jnp.transpose(B_Wv, (1, 2, 0)).reshape(hd, D)
    wo = B_Wo.reshape(hd, D)

    any_spec = pl.BlockSpec(memory_space=pl.ANY)
    out = pl.pallas_call(
        _kernel,
        out_shape=jax.ShapeDtypeStruct((S, 2 * D), BF16),
        in_specs=[any_spec] * 10,
        out_specs=any_spec,
        scratch_shapes=[
            pltpu.VMEM((2, PP, 4, PW, D), BF16),
            pltpu.VMEM((NT, D // 2, 128), U32),
            pltpu.VMEM((NP, D // 2, 3 * PW), U32),
            pltpu.VMEM((hd // 2 + PW, D), U32),
            pltpu.VMEM((NQ + 1, 5, PW // 2, KH), U32),
            pltpu.VMEM((NSEG, NP, PRE, 3 * PW), F32),
            pltpu.VMEM((SPT - 1, NG, GP * PRE, PW), F32),
            pltpu.VMEM((S, OUT_W), BF16),
            pltpu.VMEM((S, X_W), BF16),
            pltpu.VMEM((S, X_W), BF16),
            pltpu.VMEM((NSEG, PRE, D), BF16),
            pltpu.VMEM((NSEG * PRE // 2, D), U32),
            pltpu.VMEM((5, NSEG * PRE // 4, 256), U32),
            pltpu.VMEM((MEM, D), BF16),
            pltpu.VMEM((3, D // 2, D), U32),
            pltpu.VMEM((NTRIP, 2, 64, D), U32),
            pltpu.VMEM((D // 2, D), U32),
            pltpu.VMEM((PP, D // 2, 128), U32),
            pltpu.VMEM((NT, 2 * SEG, 128), F32),
            pltpu.VMEM((2, NT, KV_ROWS, 128), F32),
            pltpu.SemaphoreType.DMA((9,)),
        ],
        compiler_params=pltpu.CompilerParams(vmem_limit_bytes=120 * 1024 * 1024,
                                             disable_bounds_checks=True),
    )(A_x.reshape(S, D), A_wqkv, A_wo, B_x.reshape(S, D), B_x.reshape(NSEG, SEG // PRE, PRE, D),
      B_mem0.reshape(MEM, D), wq_t, wk_t, wv_t, wo)
    return out.reshape(1, S, 2 * D)
```

```python
import functools

import jax
import jax.numpy as jnp
from jax import lax
import jax.experimental.pallas as pl
import jax.experimental.pallas.tpu as pltpu

F32 = jnp.float32
BF16 = jnp.bfloat16
U32 = jnp.uint32

S = 2048
D = 640
NT = D // 128
A_H = 32
A_DH = D // A_H
A_W = 8
A_DIL = 2
A_HALO = 16
B_H = 32
B_DH = 192
MEM = 8
SEG = 32
NSEG = S // SEG
NP = B_H // 2
PW = 2 * B_DH
PRE = 8
FRESH = SEG - PRE
L = MEM + SEG
GP = 4
NG = NP // GP
LOG2E = 1.4426950408889634
NEG = -1000000000.0 * LOG2E
PP = 2
NTRIP = NP // PP - 1
PEEL = (2, 2, 5)
KH = 256
WO_ROWS = 512
WX_DONE = (0, 24, 56, 96, 120, 152, 192)
WX_TAIL = 2
WX_ROWS = 8
WX_SKIP = 0
ST_ROWS = 256
X_HEAD = 128
KV_ROWS = 80
X_W = 1024
OUT_W = 2048
SPT = 4
N_STEPS = NSEG // SPT
NQ = NP // 2

LAT_MM, LAT_X, LAT_T, LAT_N, LAT_N_LATE = 190, 190, 380, 230, 100
LATE_FROM = NP - 2
AP_AFTER = (6, 12, 18, 24, 30)
AO_AFTER = (30, 40)
TAIL_FILL = (2, 2, 2, 0)
HOLD_W = (0, 3, 0, 0)


def _segment_order(u):
    odd, last = u % 2 == 1, u == SPT - 1
    proj = []
    for g in range(NG):
        proj += [("K", GP * g + r) for r in range(GP)]
        for r in range(GP):
            proj += [("V", GP * g + r), ("Q", GP * g + r)]
    dur = {"K": 120, "V": 120, "Q": 120, "S": 24, "PV": 24, "PS": 24, "PPV": 24,
           "W": 120, "XA": 96, "XB": 192, "XC": 48, "Y": 96, "AO": 80, "AP": 90,
           "T": 0, "M": 0, "E": 0, "TG": 0, "MG": 0, "EG": 0}
    end = {}

    def ready(task):
        k, i = task
        if k == "T":
            deps = [(("K", i), LAT_MM)]
        elif k == "S":
            deps = [(("Q", i), LAT_MM), (("T", i), LAT_T)]
        elif k == "M":
            deps = [(("S", i), LAT_MM - 40)]
        elif k == "E":
            deps = [(("M", i), LAT_X)]
        elif k == "PV":
            deps = [(("E", i), LAT_N_LATE if i >= LATE_FROM else LAT_N), (("V", i), LAT_MM)]
        elif k == "TG":
            deps = [(("K", GP * i + r), LAT_MM) for r in range(GP)]
        elif k == "PS":
            deps = [(("TG", i), LAT_T)]
        elif k == "MG":
            deps = [(("PS", i), LAT_MM - 40)]
        elif k == "EG":
            deps = [(("MG", i), LAT_X)]
        elif k == "PPV":
            deps = [(("EG", i), LAT_N), (("V", GP * i + GP - 1), LAT_MM)]
        elif k == "W":
            deps = [(("PV", i), LAT_MM)]
        else:
            deps = [(("PV", 2 * i), LAT_MM), (("PPV", 2 * i // GP), LAT_MM)]
            if k != "XA":
                deps.append((("PV", 2 * i + 1), LAT_MM))
        if any(d not in end for d, _ in deps):
            return None
        return max(end[d] + lat for d, lat in deps)

    pend = ([(k, p) for k in ("E", "M", "T") for p in range(NP)]
            + [(k, g) for k in ("EG", "MG", "TG") for g in range(NG)]
            + ([(k, q) for q in range(NQ) for k in ("XA", "XB", "Y", "XC")] if last
               else [("W", p) for p in range(NP)])
            + [("PPV", g) for g in range(NG)]
            + [("PV", p) for p in range(NP)] + [("PS", g) for g in range(NG)]
            + [("S", p) for p in range(NP)])
    fill = [("AO", j) for j in range(NT)] if odd else [("AP", j) for j in (5, 6, 7, 8, 9, 0, 1, 2, 3, 4, 10, 12, 14)]
    order = []
    now = [0]

    def emit(task):
        order.append(task)
        now[0] += dur[task[0]]
        end[task] = now[0]

    nproj = 0
    while pend:
        cand = [x for x in pend if ready(x) is not None and ready(x) <= now[0]]
        if proj:
            cand = [x for x in cand if not (x[0] == "W" and x[1] >= NP - GP - HOLD_W[u])]
        if cand:
            if not proj:
                cand = [x for x in cand if x[0] not in ("W", "XA", "XB", "XC", "Y")] or cand
            pend.remove(cand[0])
            emit(cand[0])
        elif proj:
            emit(proj.pop(0))
            nproj += 1
            if odd and nproj == GP:
                order += [("LA", 0), ("LA", 1)]
            if nproj in (AO_AFTER if odd else AP_AFTER):
                emit(fill.pop(0))
        elif len(fill) > TAIL_FILL[u]:
            emit(fill.pop(0))
        else:
            now[0] = min(ready(x) for x in pend if ready(x) is not None)
    return order + fill


ORDERS = (
    "K0 T0 K1 K3 K2 V0 T1 T2 Q1 T3 Q0 AP5 Q2 AP6 S0 TG0 M0 PS0 V1 V2 V3 E0 MG0 S1 S2 M1 Q3 EG0 "
    "PV0 K4 K5 E1 M2 S3 K6 T4 W0 E2 M3 T5 PPV0 PV1 K7 AP7 AP8 E3 T6 W1 T7 TG1 PV2 PV3 Q4 W2 V4 W3 "
    "PS1 Q5 S4 V5 M4 MG1 V6 Q7 Q6 E4 S5 EG1 V7 M5 PV4 S6 K8 PPV1 E5 S7 M6 W4 K9 E6 M7 T8 K10 PV5 "
    "AP9 T9 K11 E7 W5 T10 TG2 PV6 V8 T11 PV7 Q8 W7 W6 S8 PS2 V10 V9 Q9 M8 MG2 Q10 E8 EG2 V11 S9 "
    "Q11 M9 PV8 S10 K12 T12 PPV2 E9 S11 M10 W8 E10 M11 PV9 K14 K13 K15 E11 T13 W9 PV10 V12 T14 "
    "T15 TG3 PV11 Q12 W10 W11 PS3 S12 Q13 V13 M12 MG3 V15 V14 E12 Q14 EG3 Q15 S13 M13 PV12 S14 "
    "AP0 AP1 PPV3 E13 W12 S15 M14 AP2 AP3 E14 PV13 M15 AP4 AP10 PV14 W13 E15 PV15 W14 W15 AP14 "
    "AP12 ",
    "K0 K2 K1 T0 K3 LA0 LA1 Q0 V1 T1 V0 T2 T3 TG0 Q1 S0 V2 PS0 Q2 M0 S1 V3 MG0 Q3 M1 S2 K4 EG0 K5 "
    "E0 E1 M2 PV0 S3 K6 T4 PPV0 E2 T5 K7 M3 W0 T6 PV1 PV2 V4 E3 T7 TG1 Q4 W1 W2 PV3 PS1 S4 V5 Q5 "
    "M4 MG1 W3 AO0 S5 V6 E4 EG1 Q6 M5 V7 PV4 Q7 E5 S6 K8 W4 M6 PPV1 PV5 S7 K9 T8 E6 K10 M7 W5 T9 "
    "PV6 K11 E7 T10 V8 W6 T11 TG2 PV7 Q8 AO1 W7 S8 V9 PS2 Q9 M8 V10 MG2 Q10 E8 S9 V11 EG2 Q11 PV8 "
    "M9 S10 K12 PPV2 E9 S11 M10 K13 W8 E10 M11 T12 PV9 K14 K15 E11 T13 T14 PV10 AO2 V12 T15 TG3 "
    "Q12 PV11 V13 Q13 PS3 S12 V14 Q14 M12 S13 MG3 V15 Q15 E12 M13 EG3 S14 W9 E13 M14 PPV3 W10 "
    "PV12 S15 W11 E14 M15 PV13 W12 PV14 E15 W13 PV15 W14 W15 AO3 AO4 ",
    "K0 K1 T0 K3 T1 AP5 K2 AP6 V0 Q0 TG0 T3 T2 V1 S0 Q1 PS0 Q2 V2 M0 S1 V3 E0 MG0 Q3 M1 K4 S2 EG0 "
    "PV0 K5 E1 M2 PPV0 S3 K6 T4 W0 E2 M3 T5 AP7 AP8 PV1 K7 E3 W1 T6 T7 TG1 PV2 V4 PV3 Q4 W2 W3 "
    "PS1 S4 V5 M4 Q5 MG1 V6 S5 Q6 EG1 E4 V7 Q7 M5 PV4 S6 K8 PPV1 E5 S7 M6 W4 AP9 K9 E6 M7 T8 PV5 "
    "K10 T9 K11 E7 W5 T10 PV6 V8 T11 TG2 Q8 PV7 W6 W7 S8 PS2 Q9 M8 MG2 V10 V9 Q10 E8 EG2 S9 V11 "
    "Q11 M9 PV8 S10 K12 PPV2 E9 W8 S11 M10 K13 E10 M11 T12 PV9 K14 K15 E11 T13 W9 PV11 T14 PV10 "
    "V12 T15 TG3 Q12 W10 V13 W11 PS3 S12 Q13 MG3 M12 V14 Q14 E12 EG3 S13 V15 Q15 M13 PV12 S14 E13 "
    "AP0 AP1 PPV3 S15 M14 W12 AP2 AP3 M15 AP4 E14 PV13 PV14 AP10 E15 W13 PV15 W14 W15 AP12 AP14 ",
    "K1 K0 K2 T0 K3 LA0 LA1 T1 V0 T2 Q0 T3 TG0 V1 Q1 S0 PS0 V2 Q2 M0 V3 MG0 Q3 S1 E0 M1 S2 EG0 K4 "
    "K5 M2 T4 PV0 E1 AO0 PPV0 S3 K6 E2 T5 K7 M3 XA0 T6 PV1 PV2 V4 E3 T7 TG1 Y0 Q4 XB0 XC0 XA1 PV3 "
    "PS1 S4 V5 Q5 M4 MG1 XB1 E4 Y1 XC1 EG1 S5 Q6 V6 M5 V7 S6 PV4 AO1 Q7 E5 PPV1 K8 S7 M6 XA2 K9 "
    "M7 T8 PV5 K10 E6 T9 XB2 E7 T10 Y2 K11 TG2 T11 XC2 PV6 PV7 V8 Q8 XA3 XB3 Y3 PS2 S8 V9 Q9 M8 "
    "MG2 V10 Q10 AO2 E8 EG2 S9 V11 S10 M9 PV8 K12 Q11 M10 PPV2 K13 E9 K14 S11 E10 T12 M11 T13 K15 "
    "PV10 PV9 XA4 T14 V12 E11 XB4 T15 TG3 XA5 Y4 Q12 AO3 PV11 XB5 PS3 S12 V13 Q13 MG3 V14 M12 Q14 "
    "EG3 S13 V15 E12 M13 PV12 Q15 S14 AO4 PPV3 E13 S15 M14 E14 XA6 M15 XC3 XC4 XC5 PV13 E15 Y5 "
    "PV14 XB6 PV15 Y6 XA7 XB7 XC6 Y7 XC7 ",
)
SKIP_PROLOGUE = False


def _order(u):
    if ORDERS is None or ORDERS[u] is None:
        return _segment_order(u)
    return [(t.rstrip("0123456789"), int(t.lstrip("ABCDEFGHIJKLMNOPQRSTUVWXYZ")))
            for t in ORDERS[u].split()]


def _nt_dot(a, b):
    return lax.dot_general(a, b, (((1,), (1,)), ((), ())), preferred_element_type=F32)


def _dot(a, b):
    return jnp.dot(a, b, preferred_element_type=F32)


def _pack(x):
    return pltpu.bitcast(x, U32)


def _unpack(x):
    return pltpu.bitcast(x, BF16)


def cat(parts):
    return jnp.concatenate(parts, axis=0)


def _round(x):
    return x.astype(BF16).astype(F32)


def _recip(x):
    r = pl.reciprocal(x, approx=True)
    return r * (2.0 - x * r)


def _kernel(ax_hbm, awqkv_hbm, awo_hbm, bx_hbm, bx4_hbm, mem0_hbm, wq_hbm, wk_hbm, wv_hbm, wo_hbm,
            out_hbm,
            stage, awo_raw, w_s, wo_s, wx_s, pre_s, odef_s, out_s,
            xa_s, xb_s, xpre_s, xp_s, xs_s, mem0_s, wa_s, wc_s, awo_s, t1_s, qa_s, kv_s,
            sems):
    b_scale = 0.072265625 * LOG2E
    a_scale = 0.2236328125

    w_hbm = (wq_hbm, wk_hbm, wv_hbm)
    wo32 = wo_hbm.bitcast(U32)
    awo32 = awo_hbm.bitcast(U32)
    hw = PW // 2
    hd = B_H * B_DH

    def w_copy(p, half, q, m, sem):
        rows = pl.ds(pl.multiple_of(p * PW, PW), PW)
        return pltpu.make_async_copy(w_hbm[m].at[rows, :], stage.at[half, q, m], sem)

    def wa_piece(g, q):
        last = g >= 2 * 3
        return jnp.where(last, 1 + q, g >> 1), jnp.where(last, NT - 1, (g & 1) + 2 * q)

    def wa_copy(c, kt, half, q, sem):
        return pltpu.make_async_copy(
            awqkv_hbm.at[pl.ds(pl.multiple_of(kt * 128, 128), 128),
                         pl.ds(pl.multiple_of(c * D, 128), D)],
            stage.at[half, q, 3, :128], sem)

    def start_trip(g):
        half = g & 1
        src = jnp.minimum(g, NTRIP - 1)
        for q in range(PP):
            for m in range(3):
                w_copy((src + 1) * PP + q, half, q, m, sems.at[half]).start(priority=1)
            wa_copy(*wa_piece(src, q), half, q, sems.at[half]).start(priority=1)

    def wait_trip(half):
        for view in (stage.at[half, :, :3], stage.at[half, :, 3, :128]):
            pltpu.make_async_copy(view, view, sems.at[half]).wait()

    qr = 2 * hw

    def wo_copy(start, n, sem):
        wr = pl.ds(pl.multiple_of(start, 8), n)
        return pltpu.make_async_copy(wo32.at[wr, :], wo_s.at[wr, :], sem)

    def wo_sums(q, piece, anchor=None, never=None):
        def blk(k, n):
            w = wo_s[pl.ds(pl.multiple_of(q * qr + k * hw + piece * WX_ROWS, 8), WX_ROWS),
                     n * KH:(n + 1) * KH]
            if anchor is not None:
                w = jnp.where(never, anchor, w)
            return _unpack(w).astype(F32)

        b11, b12, b21, b22 = blk(0, 0), blk(0, 1), blk(1, 0), blk(1, 1)
        for n, v in enumerate((b11 + b22, b12 - b22, b21 - b11, b11 + b12, b21 + b22)):
            wx_s[q, n, pl.ds(pl.multiple_of(piece * WX_ROWS, 8), WX_ROWS), :] = (
                _pack(v.astype(BF16)))

    def x_copies(xr, sem):
        return [pltpu.make_async_copy(ax_hbm.at[xr, :], xa_s.at[xr, :D], sem),
                pltpu.make_async_copy(bx_hbm.at[xr, :], xb_s.at[xr, :D], sem)]

    xpre_cp = pltpu.make_async_copy(bx4_hbm.at[:, 0], xpre_s, sems.at[3])
    late_cps = ([pltpu.make_async_copy(mem0_hbm, mem0_s, sems.at[2])]
                + x_copies(pl.ds(0, X_HEAD), sems.at[2]))
    awo_cps = [
        pltpu.make_async_copy(awo32.at[:, c * 128:(c + 1) * 128], awo_raw.at[c], sems.at[2])
        for c in range(NT)]
    x_rest = x_copies(pl.ds(X_HEAD, S - X_HEAD), sems.at[3])
    tiles = [(m, j) for m in range(3) for j in range(PW // 128)]
    peel = [tiles[sum(PEEL[:n]):sum(PEEL[:n + 1])] for n in range(len(PEEL))]
    peel_cps = [[pltpu.make_async_copy(w_hbm[m].at[pl.ds(q * PW + j * 128, 128), :],
                                       stage.at[1, q, m, pl.ds(j * 128, 128), :], sems.at[4 + n])
                 for m, j in blk for q in range(PP)] for n, blk in enumerate(peel)]
    peel_cps[-1].append(wa_copy(0, NT - 1, 1, 0, sems.at[3 + len(PEEL)]))

    xpre_cp.start()
    for cps in peel_cps:
        for cp in cps:
            cp.start(priority=1)
    start_trip(0)
    for cp in late_cps:
        cp.start(priority=1)
    kv_s[:, :, :A_HALO, :] = jnp.zeros((2, NT, A_HALO, 128), F32)
    wo_s[NQ * qr:, :] = jnp.zeros((qr, D), U32)

    def gather_heads(ref):
        rows = []
        for j in range(A_DH // 2):
            u = ref[pl.ds(j, A_H, stride=A_DH // 2), :]
            rows.append(pltpu.bitcast(u << 16, F32))
            rows.append(pltpu.bitcast(u & jnp.uint32(0xFFFF0000), F32))
        return jnp.concatenate(rows, axis=0)

    HR = NSEG * PRE // 2

    def xq(i, k):
        return _unpack(xp_s[i * HR // 2:(i + 1) * HR // 2, k * KH:(k + 1) * KH])

    def strassen_lhs():
        f = lambda i, k: xq(i, k).astype(F32)
        sums = (f(0, 0) + f(1, 1), f(1, 0) + f(1, 1), f(0, 0) + f(0, 1),
                f(1, 0) - f(0, 0), f(0, 1) - f(1, 1))
        for n, v in enumerate(sums):
            xs_s[n] = _pack(v.astype(BF16))

    def pair_prep2(p, half, m, js=(0, 1, 2), hook=None):
        if SKIP_PROLOGUE:
            return
        for q in range(2):
            lo, hi = js[0] * 128, (js[-1] + 1) * 128
            w_s[p + q, :, m * PW + lo:m * PW + hi] = _pack(stage[half, q, m, lo:hi, :].T)
        nseg = ST_ROWS // PRE
        for j in js:
            rows = slice(j * 128, (j + 1) * 128)
            b = lambda k, q: stage[half, q, m, rows, k * KH:(k + 1) * KH]
            bf = lambda k, q: b(k, q).astype(F32)
            rhs = ((bf(0, 0) + bf(1, 1)).astype(BF16), b(0, 0),
                   (bf(0, 1) - bf(1, 1)).astype(BF16), (bf(1, 0) - bf(0, 0)).astype(BF16),
                   b(1, 1), (bf(0, 0) + bf(0, 1)).astype(BF16),
                   (bf(1, 0) + bf(1, 1)).astype(BF16))
            tail = [stage[half, q, m, rows, 2 * KH:] for q in range(2)]
            for c in range(HR // ST_ROWS):
                r = slice(c * ST_ROWS // 2, (c + 1) * ST_ROWS // 2)
                sm = lambda n: _unpack(xs_s[n, r, :])
                qd = lambda i, k: _unpack(
                    xp_s[(i * HR + c * ST_ROWS) // 2:(i * HR + (c + 1) * ST_ROWS) // 2,
                         k * KH:(k + 1) * KH])
                rest = lambda i: _unpack(
                    xp_s[(i * HR + c * ST_ROWS) // 2:(i * HR + (c + 1) * ST_ROWS) // 2, 2 * KH:])

                def put(i, q, v):
                    s0 = i * (NSEG // 2) + c * nseg
                    pre_s[s0:s0 + nseg, p + q, :, m * PW + j * 128:m * PW + (j + 1) * 128] = (
                        v.reshape(nseg, PRE, 128))
                    if hook is not None:
                        hook(v)

                m5 = _nt_dot(sm(2), rhs[4])
                m3 = _nt_dot(qd(0, 0), rhs[2])
                put(0, 1, _nt_dot(rest(0), tail[1]) + m3 + m5)
                m1 = _nt_dot(sm(0), rhs[0])
                m4 = _nt_dot(qd(1, 1), rhs[3])
                put(0, 0, _nt_dot(rest(0), tail[0]) + _nt_dot(sm(4), rhs[6]) + (m1 + m4 - m5))
                m2 = _nt_dot(sm(1), rhs[1])
                put(1, 0, _nt_dot(rest(1), tail[0]) + m2 + m4)
                put(1, 1, _nt_dot(rest(1), tail[1]) + _nt_dot(sm(3), rhs[5]) + (m1 - m2 + m3))

    def wa_prep(c, kt, half, q):
        t1_s[q] = _pack(stage[half, q, 3, :128].T)
        g = gather_heads(t1_s.at[q])
        wa_s[c, pl.ds(pl.multiple_of(kt * 64, 64), 64), :] = _pack(g.astype(BF16).T)
        return g

    def wa_trip(g, half):
        lo, hi = [wa_prep(*wa_piece(g, q), half, q) for q in range(2)]
        for t in range(2):
            b11, b12 = lo[2 * t * 128:(2 * t + 1) * 128], lo[(2 * t + 1) * 128:(2 * t + 2) * 128]
            b21, b22 = hi[2 * t * 128:(2 * t + 1) * 128], hi[(2 * t + 1) * 128:(2 * t + 2) * 128]
            sums = cat([b11 + b22, b12 - b22, b21 - b11, b11 + b12, b21 + b22])
            wc_s[g, t] = _pack(sums.astype(BF16).T)

    xpre_cp.wait()
    xp_s[...] = _pack(xpre_s[...].reshape(NSEG * PRE, D))
    strassen_lhs()
    for blk, cps in zip(peel, peel_cps):
        for cp in cps:
            cp.wait()
        for m in range(3):
            js = tuple(j for mm, j in blk if mm == m)
            if js:
                pair_prep2(0, 1, m, js)
    wa_prep(0, NT - 1, 1, 0)
    start_trip(1)

    def prologue(g, carry):
        half = g & 1

        @pl.when(g > 0)
        def _():
            wo_copy((g - 1) * WO_ROWS, WO_ROWS, sems.at[8]).wait()

        @pl.when(g == NTRIP - 1)
        def _():
            for cp in awo_cps:
                cp.start(priority=1)

        @pl.when(g < NTRIP - 1)
        def _():
            wo_copy(g * WO_ROWS, WO_ROWS, sems.at[8]).start()

        wait_trip(half)
        calls = [0]
        per = hw // WX_ROWS
        total = max(b - a for a, b in zip(WX_DONE, WX_DONE[1:]))
        todo = list(range(total))
        first, stop = NQ * per, (NQ + 1) * per
        for trip in range(1, NTRIP):
            first = jnp.where(g == trip, WX_DONE[trip - 1], first)
            stop = jnp.where(g == trip, WX_DONE[trip], stop)

        def hook(v):
            calls[0] += 1
            want = (calls[0] - WX_SKIP) * total // (36 - WX_SKIP - WX_TAIL)
            t = 0
            while todo and todo[0] < want:
                k = jnp.minimum(first + todo.pop(0), stop - 1)
                q = k // per
                anchor = jnp.concatenate(
                    [v[(2 * t + c) * WX_ROWS:(2 * t + c + 1) * WX_ROWS] for c in range(2)], axis=1)
                wo_sums(q, k % per, pltpu.bitcast(anchor, U32), g > NSEG)
                t += 1

        for m in range(3):
            pair_prep2((g + 1) * PP, half, m, hook=hook)
            if m == 0:
                wa_trip(g, half)
        start_trip(g + 2)
        return carry

    lax.fori_loop(0, NTRIP, prologue, 0)

    for cp in late_cps + awo_cps:
        cp.wait()
    for cp in x_rest:
        cp.start()

    for c in range(NT):
        awo_s[:, c * 128:(c + 1) * 128] = _pack(gather_heads(awo_raw.at[c]).astype(BF16))

    def out_copy(row, n, half):
        r = pl.ds(row, n)
        c = slice(half * D, (half + 1) * D)
        return pltpu.make_async_copy(out_s.at[r, c], out_hbm.at[r, c], sems.at[7])

    def segment(s, mem, u):
        last = u == SPT - 1
        row0 = pl.multiple_of(s * SEG, SEG)
        ninf = jnp.float32(-jnp.inf)

        qi = lax.broadcasted_iota(jnp.int32, (SEG, 128), 0)
        kl = lax.broadcasted_iota(jnp.int32, (SEG, 128), 1)
        is_a = kl < L
        a80 = lax.broadcasted_iota(jnp.int32, (SEG, 2 * L), 1) < L
        real = kl < 2 * L
        kpos = jnp.where(is_a, kl, kl - L)
        allowed = ((qi >= FRESH) | (qi + MEM + PRE >= kpos)) & real
        fill = jnp.where(real, NEG, ninf)
        pi = lax.broadcasted_iota(jnp.int32, (GP * PRE, 128), 0)
        pk = lax.broadcasted_iota(jnp.int32, (GP * PRE, 128), 1)
        p_own = (pk // SEG) == (pi // PRE)
        p_allowed = (pk % (MEM + PRE)) <= (pi % PRE) + MEM
        p_first = (pk % SEG) < MEM + PRE
        p_allowed = p_allowed & p_own
        p_fill = jnp.where(p_own, NEG, ninf)
        col_a = lax.broadcasted_iota(jnp.int32, (1, PW), 1) < B_DH
        col128_a = lax.broadcasted_iota(jnp.int32, (1, 128), 1) < (B_DH - 128)

        xb = xb_s[pl.ds(row0, SEG), :D].astype(F32)
        h = jnp.concatenate([xb[PRE:], mem], axis=0).astype(BF16)

        def proj(p, m):
            return _dot(h, _unpack(w_s[p, :, m * PW:(m + 1) * PW]))

        def pre(p, m):
            return pre_s[s, p, :, m * PW:(m + 1) * PW]

        def block_diag(p, m):
            f = proj(p, m)
            full = jnp.concatenate([f[FRESH:], pre(p, m), f[:FRESH]], axis=0)
            z = jnp.zeros_like(full)
            return jnp.where(col_a, full, z), jnp.where(col_a, z, full)

        def keys_t(blocks):
            fold = cat([jnp.concatenate([x[:, :128] if i % 2 == 0 else x[:, 256:], x[:, 128:256]],
                                        axis=1) for i, x in enumerate(blocks)])
            t = fold.T
            return t[:128].astype(BF16), t[128:].astype(BF16)

        def qk(q, kt, lane_a):
            outer = _dot(cat([q[:, :128], q[:, 256:]]).astype(BF16), kt[0])
            sc = (jnp.where(lane_a, outer[:SEG], outer[SEG:])
                  + _dot(q[:, 128:256].astype(BF16), kt[1]))
            if sc.shape[1] < 128:
                sc = jnp.concatenate([sc, jnp.zeros((SEG, 128 - sc.shape[1]), F32)], axis=1)
            return sc

        def row_max(raw, ok, other, first):
            sc = jnp.where(ok, raw * b_scale, other)
            ma = jnp.max(jnp.where(first, sc, ninf), axis=1, keepdims=True)
            mb = jnp.max(jnp.where(first, ninf, sc), axis=1, keepdims=True)
            return sc, ma, mb

        def probs(mx, first, late_norm):
            sc, ma, mb = mx
            e = jnp.exp2(sc - jnp.where(first, ma, mb))
            ea, eb = jnp.where(first, e, 0.0), jnp.where(first, 0.0, e)
            sa = jnp.sum(ea, axis=1, keepdims=True)
            sb = jnp.sum(eb, axis=1, keepdims=True)
            if late_norm:
                return e.astype(BF16), _recip(sa), _recip(sb)
            return (e * _recip(jnp.where(first, sa, sb))).astype(BF16), None, None

        def apply_v(e, blocks):
            pad = 128 - sum(x.shape[0] for x in blocks)
            rows = list(blocks) + ([jnp.zeros((pad, PW), F32)] if pad else [])
            return _dot(e, cat(rows).astype(BF16))

        def pv(sm, vbd):
            e, ra, rb = sm
            o = apply_v(e, vbd)
            if ra is not None:
                o = jnp.concatenate([
                    o[:, :128] * ra,
                    o[:, 128:256] * jnp.where(col128_a, ra, rb),
                    o[:, 256:] * rb], axis=1)
            return o

        def pre_pv(g, pr, vbds):
            o = apply_v(pr, [x[:MEM + PRE] for vb in vbds for x in vb])
            if not last:
                odef_s[u, g] = o
            return o

        def wout(p, o, acc):
            contrib = _dot(o.astype(BF16), _unpack(wo_s[p * hw:(p + 1) * hw, :]))
            return contrib if acc is None else acc + contrib

        def deferred(p):
            r = slice((p % GP) * PRE, (p % GP + 1) * PRE)
            return cat([odef_s[v, p // GP, r, :] for v in range(SPT - 1)]
                       + [val["PPV", p // GP][r]])

        def wout_strassen(kind, q):
            a11, a21 = val["PV", 2 * q], deferred(2 * q)
            if kind != "XA":
                a12, a22 = val["PV", 2 * q + 1], deferred(2 * q + 1)
            blk = lambda k, n: _unpack(
                wo_s[q * qr + k * hw:q * qr + (k + 1) * hw, n * KH:(n + 1) * KH])
            sm = lambda n: _unpack(wx_s[q, n])
            if kind == "XA":
                terms = {3: (a11, sm(1)), 6: (a21 - a11, sm(3))}
            elif kind == "XB":
                terms = {1: (a11 + a22, sm(0)), 4: (a22, sm(2)), 5: (a11 + a12, blk(1, 1)),
                         7: (a12 - a22, sm(4))}
            elif kind == "XC":
                terms = {2: (a21 + a22, blk(0, 0))}
            else:
                lhs = jnp.concatenate([cat([a11, a21]), cat([a12, a22])], axis=1)
                terms = {0: (lhs, _unpack(wo_s[q * qr:(q + 1) * qr, 2 * KH:]))}
            for n, (x, w) in terms.items():
                r = _dot(x.astype(BF16), w)
                val["acc", n] = val["acc", n] + r if ("acc", n) in val else r

        arow0 = pl.multiple_of((s - u % 2) * SEG, 2 * SEG)

        def a_put(m, j, r):
            if m == 0:
                qa_s[j] = _round(r)
            else:
                kv_s[m - 1, j, A_HALO:A_HALO + 2 * SEG, :] = _round(r) if m == 1 else r

        def a_proj(idx):
            m, j = divmod(idx, NT)
            if "xa" not in val:
                val["xa"] = xa_s[pl.ds(arow0, 2 * SEG), :D]
            if m < 2 or j == NT - 1:
                a_put(m, j, _dot(val["xa"], _unpack(wa_s[m, :, j * 128:(j + 1) * 128])))
                return
            t = j // 2
            if "xs" not in val:
                xf = val["xa"].astype(F32)
                f = lambda i, k: xf[i * SEG:(i + 1) * SEG, k * KH:(k + 1) * KH]
                val["xs"] = [v.astype(BF16) for v in (
                    f(0, 0) + f(1, 1), f(1, 0) + f(1, 1), f(0, 0), f(1, 1), f(0, 0) + f(0, 1),
                    f(1, 0) - f(0, 0), f(0, 1) - f(1, 1))]
                val["xr"] = xf[:, 2 * KH:].astype(BF16)
            sm = lambda n: _unpack(cat([wc_s[2 * m + k, t, :, n * 128:(n + 1) * 128]
                                        for k in range(2)]))
            blk = lambda k, j: _unpack(wa_s[m, k * KH // 2:(k + 1) * KH // 2,
                                            (2 * t + j) * 128:(2 * t + j + 1) * 128])
            rhs = (sm(0), blk(0, 0), sm(1), sm(2), blk(1, 1), sm(3), sm(4))
            mm = lambda n: _dot(val["xs"][n], rhs[n])
            tail = [_dot(val["xr"], _unpack(wa_s[m, KH:, (2 * t + j) * 128:(2 * t + j + 1) * 128]))
                    for j in range(2)]
            m1, m2, m3, m4, m5 = [mm(n) for n in range(5)]
            a_put(m, 2 * t, tail[0] + cat([mm(6) + (m1 + m4 - m5), m2 + m4]))
            a_put(m, 2 * t + 1, tail[1] + cat([m3 + m5, mm(5) + (m1 - m2 + m3)]))

        def window(m, j, w, hf):
            lo = A_HALO + hf * SEG - A_DIL * w
            return kv_s[m, j, lo:lo + SEG, :]

        def local_softmax(hf):
            pos = arow0 + hf * SEG + lax.broadcasted_iota(jnp.int32, (SEG, 128), 0)
            rows = slice(hf * SEG, (hf + 1) * SEG)
            logits = []
            for w in range(A_W):
                t = qa_s[0, rows, :] * window(0, 0, w, hf)
                for j in range(1, NT):
                    t = t + qa_s[j, rows, :] * window(0, j, w, hf)
                t = t + pltpu.roll(t, 64, 1)
                t = t + pltpu.roll(t, 32, 1)
                t = _round(_round(t) * a_scale)
                if w > 0 and hf == 0:
                    t = jnp.where(pos >= A_DIL * w, t, -1000000000.0)
                logits.append(t)
            mx = functools.reduce(jnp.maximum, logits)
            es = [jnp.exp(l - mx) for l in logits]
            inv = _recip(functools.reduce(lambda x, y: x + y, es))
            return es, inv

        def local_pv(j, hf):
            es, inv = val["LA", hf]
            o = es[0] * window(1, j, 0, hf)
            for w in range(1, A_W):
                o = o + es[w] * window(1, j, w, hf)
            return o * inv

        def local_out(j, acc):
            wj = _unpack(awo_s[j * 64:(j + 1) * 64, :])
            r = _dot(cat([local_pv(j, 0), local_pv(j, 1)]).astype(BF16), wj)
            for m in range(2):
                kv_s[m, j, :A_HALO, :] = kv_s[m, j, 2 * SEG:2 * SEG + A_HALO, :]
            return r if acc is None else acc + r

        val = {}
        acc = None
        oa = None
        for kind, t in _order(u):
            if kind == "K":
                val[kind, t] = block_diag(t, 1)
            elif kind == "V":
                val[kind, t] = block_diag(t, 2)
            elif kind == "Q":
                val[kind, t] = proj(t, 0)
            elif kind == "T":
                val[kind, t] = keys_t(val["K", t])
            elif kind == "S":
                val[kind, t] = qk(val["Q", t], val["T", t], a80)
            elif kind == "M":
                val[kind, t] = row_max(val["S", t], allowed, fill, is_a)
            elif kind == "E":
                val[kind, t] = probs(val["M", t], is_a, t >= LATE_FROM)
            elif kind == "PV":
                val[kind, t] = pv(val["E", t], val["V", t])
            elif kind == "TG":
                val[kind, t] = keys_t([x[:MEM + PRE] for r in range(GP)
                                       for x in val["K", GP * t + r]])
            elif kind == "PS":
                q = cat([pre(GP * t + r, 0) for r in range(GP)])
                val[kind, t] = qk(q, val["TG", t], p_first)
            elif kind == "MG":
                val[kind, t] = row_max(val["PS", t], p_allowed, p_fill, p_first)
            elif kind == "EG":
                val[kind, t] = probs(val["MG", t], p_first, False)[0]
            elif kind == "PPV":
                val[kind, t] = pre_pv(t, val["EG", t], [val["V", GP * t + r] for r in range(GP)])
            elif kind == "W":
                acc = wout(t, val["PV", t], acc)
            elif kind in ("XA", "XB", "XC", "Y"):
                wout_strassen(kind, t)
            elif kind == "LA":
                val[kind, t] = local_softmax(t)
            elif kind == "AP":
                a_proj(t)
            elif kind == "AO":
                oa = local_out(t, oa)
                if t == NT - 1:
                    out_s[pl.ds(arow0, 2 * SEG), :D] = oa.astype(BF16)
                    out_copy(arow0, 2 * SEG, 0).start()
        if last:
            m = lambda n: val["acc", n]
            acc = jnp.concatenate([
                cat([m(1) + m(4) - m(5) + m(7), m(2) + m(4)]),
                cat([m(3) + m(5), m(1) - m(2) + m(3) + m(6)]), m(0)], axis=1)
        return acc

    def steps(i, mem):
        @pl.when(i == 1)
        def _():
            for cp in x_rest:
                cp.wait()

        accs = []
        for u in range(SPT):
            accs.append(segment(i * SPT + u, mem, u))
            mem = accs[-1][FRESH:SEG]
        res = cat([x for u in range(SPT) for x in (
            accs[-1][SEG + u * PRE:SEG + (u + 1) * PRE], accs[u][:FRESH])])
        row = pl.multiple_of(i * SPT * SEG, SPT * SEG)
        out_s[pl.ds(row, SPT * SEG), D:2 * D] = res.astype(BF16)
        out_copy(row, SPT * SEG, 1).start()
        return mem

    lax.fori_loop(0, N_STEPS, steps, mem0_s[...].astype(F32))

    wait_trip(0)
    wait_trip(1)

    done = N_STEPS * SPT * SEG
    pltpu.make_async_copy(out_s.at[:done, :2 * D], out_hbm.at[:done, :], sems.at[7]).wait()


@jax.jit
def pallas_concat_heads__sliding_local_dilated__memory_aug_recurrent_mem_tr__prompt_kernel(
    A_x: jax.Array,
    A_wqkv: jax.Array,
    A_wo: jax.Array,
    B_x: jax.Array,
    B_mem0: jax.Array,
    B_Wq: jax.Array,
    B_Wk: jax.Array,
    B_Wv: jax.Array,
    B_Wo: jax.Array,
    B_seg_len,
):
    del B_seg_len
    assert A_x.shape == (1, S, D) and B_x.shape == (1, S, D)
    hd = B_H * B_DH
    wq_t = jnp.transpose(B_Wq, (1, 2, 0)).reshape(hd, D)
    wk_t = jnp.transpose(B_Wk, (1, 2, 0)).reshape(hd, D)
    wv_t = jnp.transpose(B_Wv, (1, 2, 0)).reshape(hd, D)
    wo = B_Wo.reshape(hd, D)

    any_spec = pl.BlockSpec(memory_space=pl.ANY)
    out = pl.pallas_call(
        _kernel,
        out_shape=jax.ShapeDtypeStruct((S, 2 * D), BF16),
        in_specs=[any_spec] * 10,
        out_specs=any_spec,
        scratch_shapes=[
            pltpu.VMEM((2, PP, 4, PW, D), BF16),
            pltpu.VMEM((NT, D // 2, 128), U32),
            pltpu.VMEM((NP, D // 2, 3 * PW), U32),
            pltpu.VMEM((hd // 2 + PW, D), U32),
            pltpu.VMEM((NQ + 1, 5, PW // 2, KH), U32),
            pltpu.VMEM((NSEG, NP, PRE, 3 * PW), F32),
            pltpu.VMEM((SPT - 1, NG, GP * PRE, PW), F32),
            pltpu.VMEM((S, OUT_W), BF16),
            pltpu.VMEM((S, X_W), BF16),
            pltpu.VMEM((S, X_W), BF16),
            pltpu.VMEM((NSEG, PRE, D), BF16),
            pltpu.VMEM((NSEG * PRE // 2, D), U32),
            pltpu.VMEM((5, NSEG * PRE // 4, 256), U32),
            pltpu.VMEM((MEM, D), BF16),
            pltpu.VMEM((3, D // 2, D), U32),
            pltpu.VMEM((NTRIP, 2, 64, D), U32),
            pltpu.VMEM((D // 2, D), U32),
            pltpu.VMEM((PP, D // 2, 128), U32),
            pltpu.VMEM((NT, 2 * SEG, 128), F32),
            pltpu.VMEM((2, NT, KV_ROWS, 128), F32),
            pltpu.SemaphoreType.DMA((9,)),
        ],
        compiler_params=pltpu.CompilerParams(vmem_limit_bytes=120 * 1024 * 1024,
                                             disable_bounds_checks=True),
    )(A_x.reshape(S, D), A_wqkv, A_wo, B_x.reshape(S, D), B_x.reshape(NSEG, SEG // PRE, PRE, D),
      B_mem0.reshape(MEM, D), wq_t, wk_t, wv_t, wo)
    return out.reshape(1, S, 2 * D)
```

```python
import functools

import jax
import jax.numpy as jnp
from jax import lax
import jax.experimental.pallas as pl
import jax.experimental.pallas.tpu as pltpu

F32 = jnp.float32
BF16 = jnp.bfloat16
U32 = jnp.uint32

S = 2048
D = 640
NT = D // 128
A_H = 32
A_DH = D // A_H
A_W = 8
A_DIL = 2
A_HALO = 16
B_H = 32
B_DH = 192
MEM = 8
SEG = 32
NSEG = S // SEG
NP = B_H // 2
PW = 2 * B_DH
PRE = 8
FRESH = SEG - PRE
L = MEM + SEG
GP = 4
NG = NP // GP
LOG2E = 1.4426950408889634
NEG = -1000000000.0 * LOG2E
PP = 2
NTRIP = NP // PP - 1
PEEL = (2, 2, 5)
KH = 256
WO_ROWS = 512
WX_DONE = (0, 24, 56, 96, 120, 152, 192)
WX_ROWS = 8
WX_SKIP, WX_TAIL = 0, 2
ST_ROWS = 256
X_HEAD = 128
X_W = 1024
OUT_W = 2048
SPT = 4
N_STEPS = NSEG // SPT
NQ = NP // 2

LAT_MM, LAT_X, LAT_T, LAT_N, LAT_N_LATE = 190, 190, 380, 230, 100
LATE_FROM = NP - 2
AP_AFTER = (6, 12, 18, 24, 30)
AO_AFTER = (30, 40)
TAIL_FILL = (2, 2, 2, 0)
HOLD_W = (0, 3, 0, 0)


def _segment_order(u):
    odd, last = u % 2 == 1, u == SPT - 1
    proj = []
    for g in range(NG):
        proj += [("K", GP * g + r) for r in range(GP)]
        for r in range(GP):
            proj += [("V", GP * g + r), ("Q", GP * g + r)]
    dur = {"K": 120, "V": 120, "Q": 120, "S": 24, "PV": 24, "PS": 24, "PPV": 24,
           "W": 120, "XA": 96, "XB": 192, "XC": 48, "Y": 96, "AO": 80, "AP": 90,
           "T": 0, "M": 0, "E": 0, "TG": 0, "MG": 0, "EG": 0}
    end = {}

    def ready(task):
        k, i = task
        if k == "T":
            deps = [(("K", i), LAT_MM)]
        elif k == "S":
            deps = [(("Q", i), LAT_MM), (("T", i), LAT_T)]
        elif k == "M":
            deps = [(("S", i), LAT_MM - 40)]
        elif k == "E":
            deps = [(("M", i), LAT_X)]
        elif k == "PV":
            deps = [(("E", i), LAT_N_LATE if i >= LATE_FROM else LAT_N), (("V", i), LAT_MM)]
        elif k == "TG":
            deps = [(("K", GP * i + r), LAT_MM) for r in range(GP)]
        elif k == "PS":
            deps = [(("TG", i), LAT_T)]
        elif k == "MG":
            deps = [(("PS", i), LAT_MM - 40)]
        elif k == "EG":
            deps = [(("MG", i), LAT_X)]
        elif k == "PPV":
            deps = [(("EG", i), LAT_N), (("V", GP * i + GP - 1), LAT_MM)]
        elif k == "W":
            deps = [(("PV", i), LAT_MM)]
        else:
            deps = [(("PV", 2 * i), LAT_MM), (("PPV", 2 * i // GP), LAT_MM)]
            if k != "XA":
                deps.append((("PV", 2 * i + 1), LAT_MM))
        if any(d not in end for d, _ in deps):
            return None
        return max(end[d] + lat for d, lat in deps)

    pend = ([(k, p) for k in ("E", "M", "T") for p in range(NP)]
            + [(k, g) for k in ("EG", "MG", "TG") for g in range(NG)]
            + ([(k, q) for q in range(NQ) for k in ("XA", "XB", "Y", "XC")] if last
               else [("W", p) for p in range(NP)])
            + [("PPV", g) for g in range(NG)]
            + [("PV", p) for p in range(NP)] + [("PS", g) for g in range(NG)]
            + [("S", p) for p in range(NP)])
    fill = [("AO", j) for j in range(NT)] if odd else [("AP", j) for j in (5, 6, 7, 8, 9, 0, 1, 2, 3, 4, 10, 12, 14)]
    order = []
    now = [0]

    def emit(task):
        order.append(task)
        now[0] += dur[task[0]]
        end[task] = now[0]

    nproj = 0
    while pend:
        cand = [x for x in pend if ready(x) is not None and ready(x) <= now[0]]
        if proj:
            cand = [x for x in cand if not (x[0] == "W" and x[1] >= NP - GP - HOLD_W[u])]
        if cand:
            if not proj:
                cand = [x for x in cand if x[0] not in ("W", "XA", "XB", "XC", "Y")] or cand
            pend.remove(cand[0])
            emit(cand[0])
        elif proj:
            emit(proj.pop(0))
            nproj += 1
            if odd and nproj == GP:
                order += [("LA", 0), ("LA", 1)]
            if nproj in (AO_AFTER if odd else AP_AFTER):
                emit(fill.pop(0))
        elif len(fill) > TAIL_FILL[u]:
            emit(fill.pop(0))
        else:
            now[0] = min(ready(x) for x in pend if ready(x) is not None)
    return order + fill


ORDERS = (
    "K0 T0 K1 K3 K2 V0 T1 T2 Q1 T3 Q0 AP5 Q2 AP6 S0 TG0 M0 PS0 V1 V2 V3 E0 MG0 S1 S2 M1 Q3 EG0 "
    "PV0 K4 K5 E1 M2 S3 K6 T4 W0 E2 M3 T5 PPV0 PV1 K7 AP7 AP8 E3 T6 W1 T7 TG1 PV2 PV3 Q4 W2 V4 W3 "
    "PS1 Q5 S4 V5 M4 MG1 V6 Q7 Q6 E4 S5 EG1 V7 M5 PV4 S6 K8 PPV1 E5 S7 M6 W4 K9 E6 M7 T8 K10 PV5 "
    "AP9 T9 K11 E7 W5 T10 TG2 PV6 V8 T11 PV7 Q8 W7 S8 W6 PS2 V10 V9 Q9 M8 MG2 Q10 E8 EG2 V11 S9 "
    "Q11 M9 PV8 S10 K12 T12 PPV2 E9 S11 M10 W8 E10 M11 PV9 K14 K13 K15 E11 T13 W9 PV10 V12 T14 "
    "T15 TG3 PV11 Q12 W10 W11 PS3 S12 Q13 V13 M12 MG3 V15 V14 E12 Q14 EG3 Q15 S13 M13 PV12 S14 "
    "AP0 AP1 PPV3 E13 W12 S15 M14 AP2 AP3 E14 PV13 M15 AP4 AP10 PV14 W13 E15 PV15 W14 W15 AP14 "
    "AP12 ",
    "K0 K2 K1 T0 K3 LA0 LA1 Q0 V1 T1 V0 T2 T3 TG0 Q1 S0 V2 PS0 Q2 M0 S1 V3 MG0 Q3 M1 S2 K4 EG0 K5 "
    "E0 E1 M2 PV0 S3 K6 T4 K7 PPV0 E2 T5 M3 W0 T6 PV1 PV2 V4 E3 T7 TG1 Q4 W1 W2 PV3 PS1 S4 V5 Q5 "
    "M4 MG1 W3 AO0 S5 V6 E4 EG1 Q6 M5 V7 PV4 Q7 E5 S6 K8 W4 M6 PPV1 PV5 S7 K9 T8 E6 W5 K10 M7 PV6 "
    "T9 K11 E7 T10 V8 W6 T11 TG2 PV7 Q8 AO1 W7 S8 V9 PS2 Q9 M8 V10 MG2 Q10 E8 S9 V11 EG2 Q11 PV8 "
    "M9 S10 K12 PPV2 E9 S11 M10 K13 W8 E10 M11 T12 PV9 K14 K15 E11 T13 T14 PV10 AO2 V12 T15 TG3 "
    "Q12 PV11 V13 Q13 PS3 S12 V14 Q14 M12 S13 MG3 V15 Q15 E12 M13 EG3 S14 W9 E13 M14 PPV3 W10 "
    "PV12 S15 W11 E14 M15 PV13 W12 PV14 E15 W13 PV15 W14 W15 AO3 AO4 ",
    "K0 K1 T0 K3 T1 AP5 K2 AP6 V0 Q0 TG0 T3 T2 V1 S0 Q1 PS0 Q2 V2 M0 S1 V3 E0 MG0 Q3 M1 K4 S2 EG0 "
    "PV0 K5 E1 M2 PPV0 S3 K6 T4 W0 E2 M3 T5 AP7 AP8 PV1 K7 E3 W1 T6 T7 TG1 PV2 V4 PV3 Q4 W2 W3 "
    "PS1 S4 V5 M4 Q5 MG1 V6 S5 Q6 EG1 E4 V7 Q7 M5 PV4 S6 K8 PPV1 E5 S7 M6 W4 AP9 K9 E6 M7 T8 PV5 "
    "K10 T9 K11 E7 W5 T10 PV6 V8 T11 TG2 Q8 PV7 W6 W7 S8 PS2 Q9 M8 MG2 V10 V9 Q10 E8 EG2 S9 V11 "
    "Q11 M9 PV8 S10 K12 PPV2 E9 W8 S11 M10 K13 E10 M11 T12 PV9 K14 K15 E11 T13 W9 PV11 T14 PV10 "
    "V12 T15 TG3 Q12 W10 V13 W11 PS3 S12 Q13 MG3 M12 V14 Q14 E12 EG3 S13 V15 Q15 M13 PV12 S14 E13 "
    "AP0 AP1 PPV3 S15 M14 W12 AP2 AP3 M15 AP4 E14 PV14 PV13 AP10 E15 W13 PV15 W14 W15 AP12 AP14 ",
    "K1 K0 K2 T0 K3 LA0 LA1 T1 V0 T2 Q0 T3 TG0 V1 Q1 S0 PS0 M0 V2 Q2 V3 MG0 Q3 S1 E0 M1 S2 EG0 K4 "
    "K5 M2 T4 PV0 E1 AO0 PPV0 S3 K6 E2 T5 K7 M3 XA0 T6 PV1 PV2 Y0 V4 E3 T7 TG1 Q4 XB0 XC0 XA1 PV3 "
    "PS1 S4 V5 Q5 M4 MG1 XB1 E4 Y1 XC1 EG1 S5 Q6 V6 M5 V7 S6 PV4 AO1 Q7 E5 PPV1 K8 S7 M6 XA2 K9 "
    "M7 T8 PV5 K10 E6 T9 XB2 E7 T10 Y2 K11 TG2 T11 XC2 PV6 PV7 V8 Y3 Q8 XA3 XB3 PS2 S8 V9 Q9 M8 "
    "MG2 V10 Q10 AO2 E8 EG2 S9 V11 S10 M9 PV8 K12 Q11 M10 PPV2 K13 E9 K14 S11 E10 T12 M11 T13 K15 "
    "PV10 PV9 XA4 T14 V12 E11 XB4 T15 TG3 XA5 Y4 Q12 AO3 PV11 XB5 PS3 S12 V13 Q13 MG3 V14 M12 Q14 "
    "EG3 S13 V15 E12 M13 PV12 Q15 S14 AO4 PPV3 E13 S15 M14 E14 XA6 M15 XC3 XC4 XC5 PV13 E15 Y5 "
    "PV14 XB6 PV15 Y6 XA7 XB7 XC6 Y7 XC7 ",
)
SKIP_PROLOGUE = False


def _order(u):
    if ORDERS is None or ORDERS[u] is None:
        return _segment_order(u)
    return [(t.rstrip("0123456789"), int(t.lstrip("ABCDEFGHIJKLMNOPQRSTUVWXYZ")))
            for t in ORDERS[u].split()]


def _nt_dot(a, b):
    return lax.dot_general(a, b, (((1,), (1,)), ((), ())), preferred_element_type=F32)


def _dot(a, b):
    return jnp.dot(a, b, preferred_element_type=F32)


def _pack(x):
    return pltpu.bitcast(x, U32)


def _unpack(x):
    return pltpu.bitcast(x, BF16)


def cat(parts):
    return jnp.concatenate(parts, axis=0)


def _round(x):
    return x.astype(BF16).astype(F32)


def _recip(x):
    r = pl.reciprocal(x, approx=True)
    return r * (2.0 - x * r)


def _kernel(ax_hbm, awqkv_hbm, awo_hbm, bx_hbm, bx4_hbm, mem0_hbm, wq_hbm, wk_hbm, wv_hbm, wo_hbm,
            out_hbm,
            stage, awo_raw, w_s, wo_s, wx_s, pre_s, odef_s, out_s,
            xa_s, xb_s, xpre_s, xp_s, xs_s, mem0_s, wa_s, wc_s, awo_s, t1_s, qa_s, kv_s,
            sems):
    b_scale = 0.072265625 * LOG2E
    a_scale = 0.2236328125

    w_hbm = (wq_hbm, wk_hbm, wv_hbm)
    wo32 = wo_hbm.bitcast(U32)
    awo32 = awo_hbm.bitcast(U32)
    hw = PW // 2
    hd = B_H * B_DH

    def w_copy(p, half, q, m, sem):
        rows = pl.ds(pl.multiple_of(p * PW, PW), PW)
        return pltpu.make_async_copy(w_hbm[m].at[rows, :], stage.at[half, q, m], sem)

    def wa_piece(g, q):
        last = g >= 2 * 3
        return jnp.where(last, 1 + q, g >> 1), jnp.where(last, NT - 1, (g & 1) + 2 * q)

    def wa_copy(c, kt, half, q, sem):
        return pltpu.make_async_copy(
            awqkv_hbm.at[pl.ds(pl.multiple_of(kt * 128, 128), 128),
                         pl.ds(pl.multiple_of(c * D, 128), D)],
            stage.at[half, q, 3, :128], sem)

    def trip_copies(g):
        half = g & 1
        src = jnp.minimum(g, NTRIP - 1)
        cps = []
        for q in range(PP):
            cps += [w_copy((src + 1) * PP + q, half, q, m, sems.at[half]) for m in range(3)]
            cps.append(wa_copy(*wa_piece(src, q), half, q, sems.at[half]))
        return cps

    def start_trip(g):
        for cp in trip_copies(g):
            cp.start(priority=1)

    def wait_trip(g):
        for cp in trip_copies(g):
            cp.wait()

    qr = 2 * hw

    def wo_copy(start, n, sem):
        wr = pl.ds(pl.multiple_of(start, 8), n)
        return pltpu.make_async_copy(wo32.at[wr, :], wo_s.at[wr, :], sem)

    def wo_sums(q, piece, anchor=None, never=None):
        def blk(k, n):
            w = wo_s[pl.ds(pl.multiple_of(q * qr + k * hw + piece * WX_ROWS, 8), WX_ROWS),
                     n * KH:(n + 1) * KH]
            if anchor is not None:
                w = jnp.where(never, anchor, w)
            return _unpack(w).astype(F32)

        b11, b12, b21, b22 = blk(0, 0), blk(0, 1), blk(1, 0), blk(1, 1)
        for n, v in enumerate((b11 + b22, b12 - b22, b21 - b11, b11 + b12, b21 + b22)):
            wx_s[q, n, pl.ds(pl.multiple_of(piece * WX_ROWS, 8), WX_ROWS), :] = (
                _pack(v.astype(BF16)))

    def x_copies(xr, sem):
        return [pltpu.make_async_copy(ax_hbm.at[xr, :], xa_s.at[xr, :D], sem),
                pltpu.make_async_copy(bx_hbm.at[xr, :], xb_s.at[xr, :D], sem)]

    xpre_cp = pltpu.make_async_copy(bx4_hbm.at[:, 0], xpre_s, sems.at[3])
    late_cps = ([pltpu.make_async_copy(mem0_hbm, mem0_s, sems.at[2])]
                + x_copies(pl.ds(0, X_HEAD), sems.at[2]))
    awo_cps = [
        pltpu.make_async_copy(awo32.at[:, c * 128:(c + 1) * 128], awo_raw.at[c], sems.at[2])
        for c in range(NT)]
    x_rest = x_copies(pl.ds(X_HEAD, S - X_HEAD), sems.at[3])
    tiles = [(m, j) for m in range(3) for j in range(PW // 128)]
    peel = [tiles[sum(PEEL[:n]):sum(PEEL[:n + 1])] for n in range(len(PEEL))]
    peel_cps = [[pltpu.make_async_copy(w_hbm[m].at[pl.ds(q * PW + j * 128, 128), :],
                                       stage.at[1, q, m, pl.ds(j * 128, 128), :], sems.at[4 + n])
                 for m, j in blk for q in range(PP)] for n, blk in enumerate(peel)]
    peel_cps[-1].append(wa_copy(0, NT - 1, 1, 0, sems.at[3 + len(PEEL)]))

    xpre_cp.start()
    for cps in peel_cps:
        for cp in cps:
            cp.start(priority=1)
    start_trip(0)
    for cp in late_cps:
        cp.start(priority=1)
    kv_s[:, :, :A_HALO, :] = jnp.zeros((2, NT, A_HALO, 128), F32)
    wo_s[NQ * qr:, :] = jnp.zeros((qr, D), U32)

    def gather_heads(ref):
        rows = []
        for j in range(A_DH // 2):
            u = ref[pl.ds(j, A_H, stride=A_DH // 2), :]
            rows.append(pltpu.bitcast(u << 16, F32))
            rows.append(pltpu.bitcast(u & jnp.uint32(0xFFFF0000), F32))
        return jnp.concatenate(rows, axis=0)

    HR = NSEG * PRE // 2

    def xq(i, k):
        return _unpack(xp_s[i * HR // 2:(i + 1) * HR // 2, k * KH:(k + 1) * KH])

    def strassen_lhs():
        f = lambda i, k: xq(i, k).astype(F32)
        sums = (f(0, 0) + f(1, 1), f(1, 0) + f(1, 1), f(0, 0) + f(0, 1),
                f(1, 0) - f(0, 0), f(0, 1) - f(1, 1))
        for n, v in enumerate(sums):
            xs_s[n] = _pack(v.astype(BF16))

    def pair_prep2(p, half, m, js=(0, 1, 2), hook=None):
        if SKIP_PROLOGUE:
            return
        for q in range(2):
            lo, hi = js[0] * 128, (js[-1] + 1) * 128
            w_s[p + q, :, m * PW + lo:m * PW + hi] = _pack(stage[half, q, m, lo:hi, :].T)
        nseg = ST_ROWS // PRE
        for j in js:
            rows = slice(j * 128, (j + 1) * 128)
            b = lambda k, q: stage[half, q, m, rows, k * KH:(k + 1) * KH]
            bf = lambda k, q: b(k, q).astype(F32)
            rhs = ((bf(0, 0) + bf(1, 1)).astype(BF16), b(0, 0),
                   (bf(0, 1) - bf(1, 1)).astype(BF16), (bf(1, 0) - bf(0, 0)).astype(BF16),
                   b(1, 1), (bf(0, 0) + bf(0, 1)).astype(BF16),
                   (bf(1, 0) + bf(1, 1)).astype(BF16))
            tail = [stage[half, q, m, rows, 2 * KH:] for q in range(2)]
            for c in range(HR // ST_ROWS):
                r = slice(c * ST_ROWS // 2, (c + 1) * ST_ROWS // 2)
                sm = lambda n: _unpack(xs_s[n, r, :])
                qd = lambda i, k: _unpack(
                    xp_s[(i * HR + c * ST_ROWS) // 2:(i * HR + (c + 1) * ST_ROWS) // 2,
                         k * KH:(k + 1) * KH])
                rest = lambda i: _unpack(
                    xp_s[(i * HR + c * ST_ROWS) // 2:(i * HR + (c + 1) * ST_ROWS) // 2, 2 * KH:])

                def put(i, q, v):
                    s0 = i * (NSEG // 2) + c * nseg
                    pre_s[s0:s0 + nseg, p + q, :, m * PW + j * 128:m * PW + (j + 1) * 128] = (
                        v.reshape(nseg, PRE, 128))
                    if hook is not None:
                        hook(v)

                m5 = _nt_dot(sm(2), rhs[4])
                m3 = _nt_dot(qd(0, 0), rhs[2])
                put(0, 1, _nt_dot(rest(0), tail[1]) + m3 + m5)
                m1 = _nt_dot(sm(0), rhs[0])
                m4 = _nt_dot(qd(1, 1), rhs[3])
                put(0, 0, _nt_dot(rest(0), tail[0]) + _nt_dot(sm(4), rhs[6]) + (m1 + m4 - m5))
                m2 = _nt_dot(sm(1), rhs[1])
                put(1, 0, _nt_dot(rest(1), tail[0]) + m2 + m4)
                put(1, 1, _nt_dot(rest(1), tail[1]) + _nt_dot(sm(3), rhs[5]) + (m1 - m2 + m3))

    def wa_prep(c, kt, half, q):
        t1_s[q] = _pack(stage[half, q, 3, :128].T)
        g = gather_heads(t1_s.at[q])
        wa_s[c, pl.ds(pl.multiple_of(kt * 64, 64), 64), :] = _pack(g.astype(BF16).T)
        return g

    def wa_trip(g, half):
        lo, hi = [wa_prep(*wa_piece(g, q), half, q) for q in range(2)]
        for t in range(2):
            b11, b12 = lo[2 * t * 128:(2 * t + 1) * 128], lo[(2 * t + 1) * 128:(2 * t + 2) * 128]
            b21, b22 = hi[2 * t * 128:(2 * t + 1) * 128], hi[(2 * t + 1) * 128:(2 * t + 2) * 128]
            sums = cat([b11 + b22, b12 - b22, b21 - b11, b11 + b12, b21 + b22])
            wc_s[g, t] = _pack(sums.astype(BF16).T)

    xpre_cp.wait()
    xp_s[...] = _pack(xpre_s[...].reshape(NSEG * PRE, D))
    strassen_lhs()
    for blk, cps in zip(peel, peel_cps):
        for cp in cps:
            cp.wait()
        for m in range(3):
            js = tuple(j for mm, j in blk if mm == m)
            if js:
                pair_prep2(0, 1, m, js)
    wa_prep(0, NT - 1, 1, 0)
    start_trip(1)

    def prologue(g, carry):
        half = g & 1

        @pl.when(g > 0)
        def _():
            wo_copy((g - 1) * WO_ROWS, WO_ROWS, sems.at[8]).wait()

        @pl.when(g == NTRIP - 1)
        def _():
            for cp in awo_cps:
                cp.start(priority=1)

        @pl.when(g < NTRIP - 1)
        def _():
            wo_copy(g * WO_ROWS, WO_ROWS, sems.at[8]).start()

        wait_trip(g)
        calls = [0]
        per = hw // WX_ROWS
        total = max(b - a for a, b in zip(WX_DONE, WX_DONE[1:]))
        todo = list(range(total))
        first, stop = NQ * per, (NQ + 1) * per
        for trip in range(1, NTRIP):
            first = jnp.where(g == trip, WX_DONE[trip - 1], first)
            stop = jnp.where(g == trip, WX_DONE[trip], stop)

        def hook(v):
            calls[0] += 1
            want = (calls[0] - WX_SKIP) * total // (36 - WX_SKIP - WX_TAIL)
            t = 0
            while todo and todo[0] < want:
                k = jnp.minimum(first + todo.pop(0), stop - 1)
                q = k // per
                anchor = jnp.concatenate(
                    [v[(2 * t + c) * WX_ROWS:(2 * t + c + 1) * WX_ROWS] for c in range(2)], axis=1)
                wo_sums(q, k % per, pltpu.bitcast(anchor, U32), g > NSEG)
                t += 1

        for m in range(3):
            pair_prep2((g + 1) * PP, half, m, hook=hook)
            if m == 0:
                wa_trip(g, half)
        start_trip(g + 2)
        return carry

    lax.fori_loop(0, NTRIP, prologue, 0)

    for cp in late_cps + awo_cps:
        cp.wait()
    for cp in x_rest:
        cp.start()

    for c in range(NT):
        awo_s[:, c * 128:(c + 1) * 128] = _pack(gather_heads(awo_raw.at[c]).astype(BF16))

    def out_copy(row, n, half):
        r = pl.ds(row, n)
        c = slice(half * D, (half + 1) * D)
        return pltpu.make_async_copy(out_s.at[r, c], out_hbm.at[r, c], sems.at[7])

    def segment(s, mem, u):
        last = u == SPT - 1
        row0 = pl.multiple_of(s * SEG, SEG)
        ninf = jnp.float32(-jnp.inf)

        qi = lax.broadcasted_iota(jnp.int32, (SEG, 128), 0)
        kl = lax.broadcasted_iota(jnp.int32, (SEG, 128), 1)
        is_a = kl < L
        a80 = lax.broadcasted_iota(jnp.int32, (SEG, 2 * L), 1) < L
        real = kl < 2 * L
        kpos = jnp.where(is_a, kl, kl - L)
        allowed = ((qi >= FRESH) | (qi + MEM + PRE >= kpos)) & real
        fill = jnp.where(real, NEG, ninf)
        pi = lax.broadcasted_iota(jnp.int32, (GP * PRE, 128), 0)
        pk = lax.broadcasted_iota(jnp.int32, (GP * PRE, 128), 1)
        p_own = (pk // SEG) == (pi // PRE)
        p_allowed = (pk % (MEM + PRE)) <= (pi % PRE) + MEM
        p_first = (pk % SEG) < MEM + PRE
        p_allowed = p_allowed & p_own
        p_fill = jnp.where(p_own, NEG, ninf)
        col_a = lax.broadcasted_iota(jnp.int32, (1, PW), 1) < B_DH
        col128_a = lax.broadcasted_iota(jnp.int32, (1, 128), 1) < (B_DH - 128)

        xb = xb_s[pl.ds(row0, SEG), :D].astype(F32)
        h = jnp.concatenate([xb[PRE:], mem], axis=0).astype(BF16)

        def proj(p, m):
            return _dot(h, _unpack(w_s[p, :, m * PW:(m + 1) * PW]))

        def pre(p, m):
            return pre_s[s, p, :, m * PW:(m + 1) * PW]

        def block_diag(p, m):
            f = proj(p, m)
            full = jnp.concatenate([f[FRESH:], pre(p, m), f[:FRESH]], axis=0)
            z = jnp.zeros_like(full)
            return jnp.where(col_a, full, z), jnp.where(col_a, z, full)

        def keys_t(blocks):
            fold = cat([jnp.concatenate([x[:, :128] if i % 2 == 0 else x[:, 256:], x[:, 128:256]],
                                        axis=1) for i, x in enumerate(blocks)])
            t = fold.T
            return t[:128].astype(BF16), t[128:].astype(BF16)

        def qk(q, kt, lane_a):
            outer = _dot(cat([q[:, :128], q[:, 256:]]).astype(BF16), kt[0])
            sc = (jnp.where(lane_a, outer[:SEG], outer[SEG:])
                  + _dot(q[:, 128:256].astype(BF16), kt[1]))
            if sc.shape[1] < 128:
                sc = jnp.concatenate([sc, jnp.zeros((SEG, 128 - sc.shape[1]), F32)], axis=1)
            return sc

        def row_max(raw, ok, other, first):
            sc = jnp.where(ok, raw * b_scale, other)
            ma = jnp.max(jnp.where(first, sc, ninf), axis=1, keepdims=True)
            mb = jnp.max(jnp.where(first, ninf, sc), axis=1, keepdims=True)
            return sc, ma, mb

        def probs(mx, first, late_norm):
            sc, ma, mb = mx
            e = jnp.exp2(sc - jnp.where(first, ma, mb))
            ea, eb = jnp.where(first, e, 0.0), jnp.where(first, 0.0, e)
            sa = jnp.sum(ea, axis=1, keepdims=True)
            sb = jnp.sum(eb, axis=1, keepdims=True)
            if late_norm:
                return e.astype(BF16), _recip(sa), _recip(sb)
            return (e * _recip(jnp.where(first, sa, sb))).astype(BF16), None, None

        def apply_v(e, blocks):
            pad = 128 - sum(x.shape[0] for x in blocks)
            rows = list(blocks) + ([jnp.zeros((pad, PW), F32)] if pad else [])
            return _dot(e, cat(rows).astype(BF16))

        def pv(sm, vbd):
            e, ra, rb = sm
            o = apply_v(e, vbd)
            if ra is not None:
                o = jnp.concatenate([
                    o[:, :128] * ra,
                    o[:, 128:256] * jnp.where(col128_a, ra, rb),
                    o[:, 256:] * rb], axis=1)
            return o

        def pre_pv(g, pr, vbds):
            o = apply_v(pr, [x[:MEM + PRE] for vb in vbds for x in vb])
            if not last:
                odef_s[u, g] = o
            return o

        def wout(p, o, acc):
            contrib = _dot(o.astype(BF16), _unpack(wo_s[p * hw:(p + 1) * hw, :]))
            return contrib if acc is None else acc + contrib

        def deferred(p):
            r = slice((p % GP) * PRE, (p % GP + 1) * PRE)
            return cat([odef_s[v, p // GP, r, :] for v in range(SPT - 1)]
                       + [val["PPV", p // GP][r]])

        def wout_strassen(kind, q):
            a11, a21 = val["PV", 2 * q], deferred(2 * q)
            if kind != "XA":
                a12, a22 = val["PV", 2 * q + 1], deferred(2 * q + 1)
            blk = lambda k, n: _unpack(
                wo_s[q * qr + k * hw:q * qr + (k + 1) * hw, n * KH:(n + 1) * KH])
            sm = lambda n: _unpack(wx_s[q, n])
            if kind == "XA":
                terms = {3: (a11, sm(1)), 6: (a21 - a11, sm(3))}
            elif kind == "XB":
                terms = {1: (a11 + a22, sm(0)), 4: (a22, sm(2)), 5: (a11 + a12, blk(1, 1)),
                         7: (a12 - a22, sm(4))}
            elif kind == "XC":
                terms = {2: (a21 + a22, blk(0, 0))}
            else:
                lhs = jnp.concatenate([cat([a11, a21]), cat([a12, a22])], axis=1)
                terms = {0: (lhs, _unpack(wo_s[q * qr:(q + 1) * qr, 2 * KH:]))}
            for n, (x, w) in terms.items():
                r = _dot(x.astype(BF16), w)
                val["acc", n] = val["acc", n] + r if ("acc", n) in val else r

        arow0 = pl.multiple_of((s - u % 2) * SEG, 2 * SEG)

        def a_put(m, j, r):
            if m == 0:
                qa_s[j] = _round(r)
            else:
                kv_s[m - 1, j, A_HALO:A_HALO + 2 * SEG, :] = _round(r) if m == 1 else r

        def a_proj(idx):
            m, j = divmod(idx, NT)
            if "xa" not in val:
                val["xa"] = xa_s[pl.ds(arow0, 2 * SEG), :D]
            if m < 2 or j == NT - 1:
                a_put(m, j, _dot(val["xa"], _unpack(wa_s[m, :, j * 128:(j + 1) * 128])))
                return
            t = j // 2
            if "xs" not in val:
                xf = val["xa"].astype(F32)
                f = lambda i, k: xf[i * SEG:(i + 1) * SEG, k * KH:(k + 1) * KH]
                val["xs"] = [v.astype(BF16) for v in (
                    f(0, 0) + f(1, 1), f(1, 0) + f(1, 1), f(0, 0), f(1, 1), f(0, 0) + f(0, 1),
                    f(1, 0) - f(0, 0), f(0, 1) - f(1, 1))]
                val["xr"] = xf[:, 2 * KH:].astype(BF16)
            sm = lambda n: _unpack(cat([wc_s[2 * m + k, t, :, n * 128:(n + 1) * 128]
                                        for k in range(2)]))
            blk = lambda k, j: _unpack(wa_s[m, k * KH // 2:(k + 1) * KH // 2,
                                            (2 * t + j) * 128:(2 * t + j + 1) * 128])
            rhs = (sm(0), blk(0, 0), sm(1), sm(2), blk(1, 1), sm(3), sm(4))
            mm = lambda n: _dot(val["xs"][n], rhs[n])
            tail = [_dot(val["xr"], _unpack(wa_s[m, KH:, (2 * t + j) * 128:(2 * t + j + 1) * 128]))
                    for j in range(2)]
            m1, m2, m3, m4, m5 = [mm(n) for n in range(5)]
            a_put(m, 2 * t, tail[0] + cat([mm(6) + (m1 + m4 - m5), m2 + m4]))
            a_put(m, 2 * t + 1, tail[1] + cat([m3 + m5, mm(5) + (m1 - m2 + m3)]))

        def window(m, j, w, hf):
            lo = A_HALO + hf * SEG - A_DIL * w
            return kv_s[m, j, lo:lo + SEG, :]

        def local_softmax(hf):
            pos = arow0 + hf * SEG + lax.broadcasted_iota(jnp.int32, (SEG, 128), 0)
            rows = slice(hf * SEG, (hf + 1) * SEG)
            logits = []
            for w in range(A_W):
                t = qa_s[0, rows, :] * window(0, 0, w, hf)
                for j in range(1, NT):
                    t = t + qa_s[j, rows, :] * window(0, j, w, hf)
                t = t + pltpu.roll(t, 64, 1)
                t = t + pltpu.roll(t, 32, 1)
                t = _round(_round(t) * a_scale)
                if w > 0 and hf == 0:
                    t = jnp.where(pos >= A_DIL * w, t, -1000000000.0)
                logits.append(t)
            mx = functools.reduce(jnp.maximum, logits)
            es = [jnp.exp(l - mx) for l in logits]
            inv = _recip(functools.reduce(lambda x, y: x + y, es))
            return es, inv

        def local_pv(j, hf):
            es, inv = val["LA", hf]
            o = es[0] * window(1, j, 0, hf)
            for w in range(1, A_W):
                o = o + es[w] * window(1, j, w, hf)
            return o * inv

        def local_out(j, acc):
            wj = _unpack(awo_s[j * 64:(j + 1) * 64, :])
            r = _dot(cat([local_pv(j, 0), local_pv(j, 1)]).astype(BF16), wj)
            for m in range(2):
                kv_s[m, j, :A_HALO, :] = kv_s[m, j, 2 * SEG:2 * SEG + A_HALO, :]
            return r if acc is None else acc + r

        val = {}
        acc = None
        oa = None
        for kind, t in _order(u):
            if kind == "K":
                val[kind, t] = block_diag(t, 1)
            elif kind == "V":
                val[kind, t] = block_diag(t, 2)
            elif kind == "Q":
                val[kind, t] = proj(t, 0)
            elif kind == "T":
                val[kind, t] = keys_t(val["K", t])
            elif kind == "S":
                val[kind, t] = qk(val["Q", t], val["T", t], a80)
            elif kind == "M":
                val[kind, t] = row_max(val["S", t], allowed, fill, is_a)
            elif kind == "E":
                val[kind, t] = probs(val["M", t], is_a, t >= LATE_FROM)
            elif kind == "PV":
                val[kind, t] = pv(val["E", t], val["V", t])
            elif kind == "TG":
                val[kind, t] = keys_t([x[:MEM + PRE] for r in range(GP)
                                       for x in val["K", GP * t + r]])
            elif kind == "PS":
                q = cat([pre(GP * t + r, 0) for r in range(GP)])
                val[kind, t] = qk(q, val["TG", t], p_first)
            elif kind == "MG":
                val[kind, t] = row_max(val["PS", t], p_allowed, p_fill, p_first)
            elif kind == "EG":
                val[kind, t] = probs(val["MG", t], p_first, False)[0]
            elif kind == "PPV":
                val[kind, t] = pre_pv(t, val["EG", t], [val["V", GP * t + r] for r in range(GP)])
            elif kind == "W":
                acc = wout(t, val["PV", t], acc)
            elif kind in ("XA", "XB", "XC", "Y"):
                wout_strassen(kind, t)
            elif kind == "LA":
                val[kind, t] = local_softmax(t)
            elif kind == "AP":
                a_proj(t)
            elif kind == "AO":
                oa = local_out(t, oa)
                if t == NT - 1:
                    out_s[pl.ds(arow0, 2 * SEG), :D] = oa.astype(BF16)
                    out_copy(arow0, 2 * SEG, 0).start()
        if last:
            m = lambda n: val["acc", n]
            acc = jnp.concatenate([
                cat([m(1) + m(4) - m(5) + m(7), m(2) + m(4)]),
                cat([m(3) + m(5), m(1) - m(2) + m(3) + m(6)]), m(0)], axis=1)
        return acc

    def steps(i, mem):
        @pl.when(i == 1)
        def _():
            for cp in x_rest:
                cp.wait()

        accs = []
        for u in range(SPT):
            accs.append(segment(i * SPT + u, mem, u))
            mem = accs[-1][FRESH:SEG]
        res = cat([x for u in range(SPT) for x in (
            accs[-1][SEG + u * PRE:SEG + (u + 1) * PRE], accs[u][:FRESH])])
        row = pl.multiple_of(i * SPT * SEG, SPT * SEG)
        out_s[pl.ds(row, SPT * SEG), D:2 * D] = res.astype(BF16)
        out_copy(row, SPT * SEG, 1).start()
        return mem

    lax.fori_loop(0, N_STEPS, steps, mem0_s[...].astype(F32))

    wait_trip(NTRIP)
    wait_trip(NTRIP + 1)

    done = N_STEPS * SPT * SEG
    pltpu.make_async_copy(out_s.at[:done, :2 * D], out_hbm.at[:done, :], sems.at[7]).wait()


@jax.jit
def pallas_concat_heads__sliding_local_dilated__memory_aug_recurrent_mem_tr__prompt_kernel(
    A_x: jax.Array,
    A_wqkv: jax.Array,
    A_wo: jax.Array,
    B_x: jax.Array,
    B_mem0: jax.Array,
    B_Wq: jax.Array,
    B_Wk: jax.Array,
    B_Wv: jax.Array,
    B_Wo: jax.Array,
    B_seg_len,
):
    del B_seg_len
    assert A_x.shape == (1, S, D) and B_x.shape == (1, S, D)
    hd = B_H * B_DH
    wq_t = jnp.transpose(B_Wq, (1, 2, 0)).reshape(hd, D)
    wk_t = jnp.transpose(B_Wk, (1, 2, 0)).reshape(hd, D)
    wv_t = jnp.transpose(B_Wv, (1, 2, 0)).reshape(hd, D)
    wo = B_Wo.reshape(hd, D)

    any_spec = pl.BlockSpec(memory_space=pl.ANY)
    out = pl.pallas_call(
        _kernel,
        out_shape=jax.ShapeDtypeStruct((S, 2 * D), BF16),
        in_specs=[any_spec] * 10,
        out_specs=any_spec,
        scratch_shapes=[
            pltpu.VMEM((2, PP, 4, PW, D), BF16),
            pltpu.VMEM((NT, D // 2, 128), U32),
            pltpu.VMEM((NP, D // 2, 3 * PW), U32),
            pltpu.VMEM((hd // 2 + PW, D), U32),
            pltpu.VMEM((NQ + 1, 5, PW // 2, KH), U32),
            pltpu.VMEM((NSEG, NP, PRE, 3 * PW), F32),
            pltpu.VMEM((SPT - 1, NG, GP * PRE, PW), F32),
            pltpu.VMEM((S, OUT_W), BF16),
            pltpu.VMEM((S, X_W), BF16),
            pltpu.VMEM((S, X_W), BF16),
            pltpu.VMEM((NSEG, PRE, D), BF16),
            pltpu.VMEM((NSEG * PRE // 2, D), U32),
            pltpu.VMEM((5, NSEG * PRE // 4, 256), U32),
            pltpu.VMEM((MEM, D), BF16),
            pltpu.VMEM((3, D // 2, D), U32),
            pltpu.VMEM((NTRIP, 2, 64, D), U32),
            pltpu.VMEM((D // 2, D), U32),
            pltpu.VMEM((PP, D // 2, 128), U32),
            pltpu.VMEM((NT, 2 * SEG, 128), F32),
            pltpu.VMEM((2, NT, A_HALO + 2 * SEG, 128), F32),
            pltpu.SemaphoreType.DMA((9,)),
        ],
        compiler_params=pltpu.CompilerParams(vmem_limit_bytes=120 * 1024 * 1024,
                                             disable_bounds_checks=True),
    )(A_x.reshape(S, D), A_wqkv, A_wo, B_x.reshape(S, D), B_x.reshape(NSEG, SEG // PRE, PRE, D),
      B_mem0.reshape(MEM, D), wq_t, wk_t, wv_t, wo)
    return out.reshape(1, S, 2 * D)
```

```python
import functools

import jax
import jax.numpy as jnp
from jax import lax
import jax.experimental.pallas as pl
import jax.experimental.pallas.tpu as pltpu

F32 = jnp.float32
BF16 = jnp.bfloat16
U32 = jnp.uint32

S = 2048
D = 640
NT = D // 128
A_H = 32
A_DH = D // A_H
A_W = 8
A_DIL = 2
A_HALO = 16
B_H = 32
B_DH = 192
MEM = 8
SEG = 32
NSEG = S // SEG
NP = B_H // 2
PW = 2 * B_DH
PRE = 8
FRESH = SEG - PRE
L = MEM + SEG
GP = 4
NG = NP // GP
LOG2E = 1.4426950408889634
NEG = -1000000000.0 * LOG2E
PP = 2
NTRIP = NP // PP - 1
PEEL = (2, 2, 5)
KH = 256
WO_ROWS = 512
WX_DONE = (0, 24, 56, 96, 120, 152, 192)
WX_ROWS = 8
WX_SKIP, WX_TAIL = 2, 2
ST_ROWS = 256
X_HEAD = 128
X_W = 1024
OUT_W = 2048
SPT = 4
N_STEPS = NSEG // SPT
NQ = NP // 2

LAT_MM, LAT_X, LAT_T, LAT_N, LAT_N_LATE = 190, 190, 380, 230, 100
LATE_FROM = NP - 2
AP_AFTER = (6, 12, 18, 24, 30)
AO_AFTER = (30, 40)
TAIL_FILL = (2, 2, 2, 0)
HOLD_W = (0, 3, 0, 0)


def _segment_order(u):
    odd, last = u % 2 == 1, u == SPT - 1
    proj = []
    for g in range(NG):
        proj += [("K", GP * g + r) for r in range(GP)]
        for r in range(GP):
            proj += [("V", GP * g + r), ("Q", GP * g + r)]
    dur = {"K": 120, "V": 120, "Q": 120, "S": 24, "PV": 24, "PS": 24, "PPV": 24,
           "W": 120, "XA": 96, "XB": 192, "XC": 48, "Y": 96, "AO": 80, "AP": 90,
           "T": 0, "M": 0, "E": 0, "TG": 0, "MG": 0, "EG": 0}
    end = {}

    def ready(task):
        k, i = task
        if k == "T":
            deps = [(("K", i), LAT_MM)]
        elif k == "S":
            deps = [(("Q", i), LAT_MM), (("T", i), LAT_T)]
        elif k == "M":
            deps = [(("S", i), LAT_MM - 40)]
        elif k == "E":
            deps = [(("M", i), LAT_X)]
        elif k == "PV":
            deps = [(("E", i), LAT_N_LATE if i >= LATE_FROM else LAT_N), (("V", i), LAT_MM)]
        elif k == "TG":
            deps = [(("K", GP * i + r), LAT_MM) for r in range(GP)]
        elif k == "PS":
            deps = [(("TG", i), LAT_T)]
        elif k == "MG":
            deps = [(("PS", i), LAT_MM - 40)]
        elif k == "EG":
            deps = [(("MG", i), LAT_X)]
        elif k == "PPV":
            deps = [(("EG", i), LAT_N), (("V", GP * i + GP - 1), LAT_MM)]
        elif k == "W":
            deps = [(("PV", i), LAT_MM)]
        else:
            deps = [(("PV", 2 * i), LAT_MM), (("PPV", 2 * i // GP), LAT_MM)]
            if k != "XA":
                deps.append((("PV", 2 * i + 1), LAT_MM))
        if any(d not in end for d, _ in deps):
            return None
        return max(end[d] + lat for d, lat in deps)

    pend = ([(k, p) for k in ("E", "M", "T") for p in range(NP)]
            + [(k, g) for k in ("EG", "MG", "TG") for g in range(NG)]
            + ([(k, q) for q in range(NQ) for k in ("XA", "XB", "Y", "XC")] if last
               else [("W", p) for p in range(NP)])
            + [("PPV", g) for g in range(NG)]
            + [("PV", p) for p in range(NP)] + [("PS", g) for g in range(NG)]
            + [("S", p) for p in range(NP)])
    fill = [("AO", j) for j in range(NT)] if odd else [("AP", j) for j in (5, 6, 7, 8, 9, 0, 1, 2, 3, 4, 10, 12, 14)]
    order = []
    now = [0]

    def emit(task):
        order.append(task)
        now[0] += dur[task[0]]
        end[task] = now[0]

    nproj = 0
    while pend:
        cand = [x for x in pend if ready(x) is not None and ready(x) <= now[0]]
        if proj:
            cand = [x for x in cand if not (x[0] == "W" and x[1] >= NP - GP - HOLD_W[u])]
        if cand:
            if not proj:
                cand = [x for x in cand if x[0] not in ("W", "XA", "XB", "XC", "Y")] or cand
            pend.remove(cand[0])
            emit(cand[0])
        elif proj:
            emit(proj.pop(0))
            nproj += 1
            if odd and nproj == GP:
                order += [("LA", 0), ("LA", 1)]
            if nproj in (AO_AFTER if odd else AP_AFTER):
                emit(fill.pop(0))
        elif len(fill) > TAIL_FILL[u]:
            emit(fill.pop(0))
        else:
            now[0] = min(ready(x) for x in pend if ready(x) is not None)
    return order + fill


ORDERS = (
    "K0 T0 K1 K3 K2 V0 T1 T2 Q1 T3 Q0 AP5 Q2 AP6 S0 TG0 M0 PS0 V1 V2 V3 E0 MG0 S1 S2 M1 Q3 EG0 "
    "PV0 K4 K5 E1 M2 S3 K6 T4 W0 E2 M3 T5 PPV0 PV1 K7 AP7 AP8 E3 T6 W1 T7 TG1 PV2 PV3 Q4 W2 V4 W3 "
    "PS1 Q5 S4 V5 M4 MG1 V6 Q7 Q6 E4 S5 EG1 V7 M5 PV4 S6 K8 PPV1 E5 S7 M6 W4 K9 E6 M7 T8 K10 PV5 "
    "AP9 T9 K11 E7 W5 T10 TG2 PV6 V8 T11 PV7 Q8 W7 S8 W6 PS2 V10 V9 Q9 M8 MG2 Q10 E8 EG2 V11 S9 "
    "Q11 M9 PV8 S10 K12 T12 PPV2 E9 S11 M10 W8 E10 M11 PV9 K14 K13 K15 E11 T13 W9 PV10 V12 T14 "
    "T15 TG3 PV11 Q12 W10 W11 PS3 S12 Q13 V13 M12 MG3 V15 V14 E12 Q14 EG3 Q15 S13 M13 PV12 S14 "
    "AP0 AP1 PPV3 E13 W12 S15 M14 AP2 AP3 E14 PV13 M15 AP4 AP10 PV14 W13 E15 PV15 W14 W15 AP14 "
    "AP12 ",
    "K0 K2 K1 T0 K3 LA0 LA1 Q0 V1 T1 V0 T2 T3 TG0 Q1 S0 V2 PS0 Q2 M0 S1 V3 MG0 Q3 M1 S2 K4 EG0 K5 "
    "E0 E1 M2 PV0 S3 K6 T4 K7 PPV0 E2 T5 M3 W0 T6 PV1 PV2 V4 E3 T7 TG1 Q4 W1 W2 PV3 PS1 S4 V5 Q5 "
    "M4 MG1 W3 AO0 S5 V6 E4 EG1 Q6 M5 V7 PV4 Q7 E5 S6 K8 W4 M6 PPV1 PV5 S7 K9 T8 E6 W5 K10 M7 PV6 "
    "T9 K11 E7 T10 V8 W6 T11 TG2 PV7 Q8 AO1 W7 S8 V9 PS2 Q9 M8 V10 MG2 Q10 E8 S9 V11 EG2 Q11 PV8 "
    "M9 S10 K12 PPV2 E9 S11 M10 K13 W8 E10 M11 T12 PV9 K14 K15 E11 T13 T14 PV10 AO2 V12 T15 TG3 "
    "Q12 PV11 V13 Q13 PS3 S12 V14 Q14 M12 S13 MG3 V15 Q15 E12 M13 EG3 S14 W9 E13 M14 PPV3 W10 "
    "PV12 S15 W11 E14 M15 PV13 W12 PV14 E15 W13 PV15 W14 W15 AO3 AO4 ",
    "K0 K1 T0 K3 T1 AP5 K2 AP6 V0 Q0 TG0 T3 T2 V1 S0 Q1 PS0 Q2 V2 M0 S1 V3 E0 MG0 Q3 M1 K4 S2 EG0 "
    "PV0 K5 E1 M2 PPV0 S3 K6 T4 W0 E2 M3 T5 AP7 AP8 PV1 K7 E3 W1 T6 T7 TG1 PV2 V4 PV3 Q4 W2 W3 "
    "PS1 S4 V5 M4 Q5 MG1 V6 S5 Q6 EG1 E4 V7 Q7 M5 PV4 S6 K8 PPV1 E5 S7 M6 W4 AP9 K9 E6 M7 T8 PV5 "
    "K10 T9 K11 E7 W5 T10 PV6 V8 T11 TG2 Q8 PV7 W6 W7 S8 PS2 Q9 M8 MG2 V10 V9 Q10 E8 EG2 S9 V11 "
    "Q11 M9 PV8 S10 K12 PPV2 E9 W8 S11 M10 K13 E10 M11 T12 PV9 K14 K15 E11 T13 W9 PV11 T14 PV10 "
    "V12 T15 TG3 Q12 W10 V13 W11 PS3 S12 Q13 MG3 M12 V14 Q14 E12 EG3 S13 V15 Q15 M13 PV12 S14 E13 "
    "AP0 AP1 PPV3 S15 M14 W12 AP2 AP3 M15 AP4 E14 PV14 PV13 AP10 E15 W13 PV15 W14 W15 AP12 AP14 ",
    "K1 K0 K2 T0 K3 LA0 LA1 T1 V0 T2 Q0 T3 TG0 V1 Q1 S0 PS0 M0 V2 Q2 V3 MG0 Q3 S1 E0 M1 S2 EG0 K4 "
    "K5 M2 T4 PV0 E1 AO0 PPV0 S3 K6 E2 T5 K7 M3 XA0 T6 PV1 PV2 Y0 V4 E3 T7 TG1 Q4 XB0 XC0 XA1 PV3 "
    "PS1 S4 V5 Q5 M4 MG1 XB1 E4 Y1 XC1 EG1 S5 Q6 V6 M5 V7 S6 PV4 AO1 Q7 E5 PPV1 K8 S7 M6 XA2 K9 "
    "M7 T8 PV5 K10 E6 T9 XB2 E7 T10 Y2 K11 TG2 T11 XC2 PV6 PV7 V8 Y3 Q8 XA3 XB3 PS2 S8 V9 Q9 M8 "
    "MG2 V10 Q10 AO2 E8 EG2 S9 V11 S10 M9 PV8 K12 Q11 M10 PPV2 K13 E9 K14 S11 E10 T12 M11 T13 K15 "
    "PV10 PV9 XA4 T14 V12 E11 XB4 T15 TG3 XA5 Y4 Q12 AO3 PV11 XB5 PS3 S12 V13 Q13 MG3 V14 M12 Q14 "
    "EG3 S13 V15 E12 M13 PV12 Q15 S14 AO4 PPV3 E13 S15 M14 E14 XA6 M15 XC3 XC4 XC5 PV13 E15 Y5 "
    "PV14 XB6 PV15 Y6 XA7 XB7 XC6 Y7 XC7 ",
)
SKIP_PROLOGUE = False


def _order(u):
    if ORDERS is None or ORDERS[u] is None:
        return _segment_order(u)
    return [(t.rstrip("0123456789"), int(t.lstrip("ABCDEFGHIJKLMNOPQRSTUVWXYZ")))
            for t in ORDERS[u].split()]


def _nt_dot(a, b):
    return lax.dot_general(a, b, (((1,), (1,)), ((), ())), preferred_element_type=F32)


def _dot(a, b):
    return jnp.dot(a, b, preferred_element_type=F32)


def _pack(x):
    return pltpu.bitcast(x, U32)


def _unpack(x):
    return pltpu.bitcast(x, BF16)


def cat(parts):
    return jnp.concatenate(parts, axis=0)


def _round(x):
    return x.astype(BF16).astype(F32)


def _recip(x):
    r = pl.reciprocal(x, approx=True)
    return r * (2.0 - x * r)


def _kernel(ax_hbm, awqkv_hbm, awo_hbm, bx_hbm, bx4_hbm, mem0_hbm, wq_hbm, wk_hbm, wv_hbm, wo_hbm,
            out_hbm,
            stage, awo_raw, wo_raw, w_s, wo_s, wx_s, pre_s, odef_s, out_s,
            xa_s, xb_s, xpre_s, xp_s, xs_s, mem0_s, wa_s, wc_s, awo_s, t1_s, qa_s, kv_s,
            sems):
    b_scale = 0.072265625 * LOG2E
    a_scale = 0.2236328125

    w_hbm = (wq_hbm, wk_hbm, wv_hbm)
    hw = PW // 2
    hd = B_H * B_DH

    def w_copy(p, half, q, m, sem):
        rows = pl.ds(pl.multiple_of(p * PW, PW), PW)
        return pltpu.make_async_copy(w_hbm[m].at[rows, :], stage.at[half, q, m], sem)

    def wa_piece(g, q):
        last = g >= 2 * 3
        return jnp.where(last, 1 + q, g >> 1), jnp.where(last, NT - 1, (g & 1) + 2 * q)

    def wa_copy(c, kt, half, q, sem):
        return pltpu.make_async_copy(
            awqkv_hbm.at[pl.ds(pl.multiple_of(kt * 128, 128), 128),
                         pl.ds(pl.multiple_of(c * D, 128), D)],
            stage.at[half, q, 3, :128], sem)

    def trip_copies(g):
        half = g & 1
        src = jnp.minimum(g, NTRIP - 1)
        cps = []
        for q in range(PP):
            cps += [w_copy((src + 1) * PP + q, half, q, m, sems.at[half]) for m in range(3)]
            cps.append(wa_copy(*wa_piece(src, q), half, q, sems.at[half]))
        return cps

    def start_trip(g):
        for cp in trip_copies(g):
            cp.start(priority=1)

    def wait_trip(g):
        for cp in trip_copies(g):
            cp.wait()

    qr = 2 * hw

    def wo_copy(c):
        src = jnp.minimum(c, hd // (2 * WO_ROWS) - 1)
        rows = pl.ds(pl.multiple_of(src * 2 * WO_ROWS, 2 * WO_ROWS), 2 * WO_ROWS)
        return pltpu.make_async_copy(wo_hbm.at[rows, :], wo_raw.at[lax.rem(c, 3)],
                                     sems.at[8 + (c & 1)])

    def wo_piece(q, piece, spare, anchor, never):
        half = []
        for k in range(2):
            r = q * qr + k * hw + piece * WX_ROWS
            c = r // WO_ROWS
            slot = jnp.where(spare, 3, lax.rem(c, 3))
            off = jnp.where(spare, 0, 2 * (r - c * WO_ROWS))
            rows = pl.ds(pl.multiple_of(off, 16), 2 * WX_ROWS)
            w = jnp.where(never, anchor, _pack(wo_raw[slot, rows, :]))
            wo_s[pl.ds(pl.multiple_of(r, 8), WX_ROWS), :] = w
            half.append(_unpack(w[:, :2 * KH]).astype(F32))
        b11, b12, b21, b22 = [half[k][:, n * KH:(n + 1) * KH] for k in range(2) for n in range(2)]
        for n, v in enumerate((b11 + b22, b12 - b22, b21 - b11, b11 + b12, b21 + b22)):
            wx_s[q, n, pl.ds(pl.multiple_of(piece * WX_ROWS, 8), WX_ROWS), :] = (
                _pack(v.astype(BF16)))

    def x_copies(xr, sem):
        return [pltpu.make_async_copy(ax_hbm.at[xr, :], xa_s.at[xr, :D], sem),
                pltpu.make_async_copy(bx_hbm.at[xr, :], xb_s.at[xr, :D], sem)]

    xpre_cp = pltpu.make_async_copy(bx4_hbm.at[:, 0], xpre_s, sems.at[3])
    late_cps = ([pltpu.make_async_copy(mem0_hbm, mem0_s, sems.at[2])]
                + x_copies(pl.ds(0, X_HEAD), sems.at[2]))
    awo_cps = [
        pltpu.make_async_copy(awo_hbm.at[:, c * 128:(c + 1) * 128], awo_raw.at[c], sems.at[2])
        for c in range(NT)]
    x_rest = x_copies(pl.ds(X_HEAD, S - X_HEAD), sems.at[3])
    tiles = [(m, j) for m in range(3) for j in range(PW // 128)]
    peel = [tiles[sum(PEEL[:n]):sum(PEEL[:n + 1])] for n in range(len(PEEL))]
    peel_cps = [[pltpu.make_async_copy(w_hbm[m].at[pl.ds(q * PW + j * 128, 128), :],
                                       stage.at[1, q, m, pl.ds(j * 128, 128), :], sems.at[4 + n])
                 for m, j in blk for q in range(PP)] for n, blk in enumerate(peel)]
    peel_cps[-1].append(wa_copy(0, NT - 1, 1, 0, sems.at[3 + len(PEEL)]))

    xpre_cp.start()
    for cps in peel_cps:
        for cp in cps:
            cp.start(priority=1)
    start_trip(0)
    for cp in late_cps:
        cp.start(priority=1)
    kv_s[:, :, :A_HALO, :] = jnp.zeros((2, NT, A_HALO, 128), F32)
    wo_raw[3, :2 * WX_ROWS, :] = jnp.zeros((2 * WX_ROWS, D), BF16)

    def gather_heads(ref):
        rows = []
        for j in range(A_DH // 2):
            u = ref[pl.ds(j, A_H, stride=A_DH // 2), :]
            rows.append(pltpu.bitcast(u << 16, F32))
            rows.append(pltpu.bitcast(u & jnp.uint32(0xFFFF0000), F32))
        return jnp.concatenate(rows, axis=0)

    HR = NSEG * PRE // 2

    def xq(i, k):
        return _unpack(xp_s[i * HR // 2:(i + 1) * HR // 2, k * KH:(k + 1) * KH])

    def strassen_lhs():
        f = lambda i, k: xq(i, k).astype(F32)
        sums = (f(0, 0) + f(1, 1), f(1, 0) + f(1, 1), f(0, 0) + f(0, 1),
                f(1, 0) - f(0, 0), f(0, 1) - f(1, 1))
        for n, v in enumerate(sums):
            xs_s[n] = _pack(v.astype(BF16))

    def pair_prep2(p, half, m, js=(0, 1, 2), hook=None):
        if SKIP_PROLOGUE:
            return
        for q in range(2):
            lo, hi = js[0] * 128, (js[-1] + 1) * 128
            w_s[p + q, :, m * PW + lo:m * PW + hi] = _pack(stage[half, q, m, lo:hi, :].T)
        nseg = ST_ROWS // PRE
        for j in js:
            rows = slice(j * 128, (j + 1) * 128)
            b = lambda k, q: stage[half, q, m, rows, k * KH:(k + 1) * KH]
            bf = lambda k, q: b(k, q).astype(F32)
            rhs = ((bf(0, 0) + bf(1, 1)).astype(BF16), b(0, 0),
                   (bf(0, 1) - bf(1, 1)).astype(BF16), (bf(1, 0) - bf(0, 0)).astype(BF16),
                   b(1, 1), (bf(0, 0) + bf(0, 1)).astype(BF16),
                   (bf(1, 0) + bf(1, 1)).astype(BF16))
            tail = [stage[half, q, m, rows, 2 * KH:] for q in range(2)]
            for c in range(HR // ST_ROWS):
                r = slice(c * ST_ROWS // 2, (c + 1) * ST_ROWS // 2)
                sm = lambda n: _unpack(xs_s[n, r, :])
                qd = lambda i, k: _unpack(
                    xp_s[(i * HR + c * ST_ROWS) // 2:(i * HR + (c + 1) * ST_ROWS) // 2,
                         k * KH:(k + 1) * KH])
                rest = lambda i: _unpack(
                    xp_s[(i * HR + c * ST_ROWS) // 2:(i * HR + (c + 1) * ST_ROWS) // 2, 2 * KH:])

                def put(i, q, v):
                    s0 = i * (NSEG // 2) + c * nseg
                    pre_s[s0:s0 + nseg, p + q, :, m * PW + j * 128:m * PW + (j + 1) * 128] = (
                        v.reshape(nseg, PRE, 128))
                    if hook is not None:
                        hook(v)

                m5 = _nt_dot(sm(2), rhs[4])
                m3 = _nt_dot(qd(0, 0), rhs[2])
                put(0, 1, _nt_dot(rest(0), tail[1]) + m3 + m5)
                m1 = _nt_dot(sm(0), rhs[0])
                m4 = _nt_dot(qd(1, 1), rhs[3])
                put(0, 0, _nt_dot(rest(0), tail[0]) + _nt_dot(sm(4), rhs[6]) + (m1 + m4 - m5))
                m2 = _nt_dot(sm(1), rhs[1])
                put(1, 0, _nt_dot(rest(1), tail[0]) + m2 + m4)
                put(1, 1, _nt_dot(rest(1), tail[1]) + _nt_dot(sm(3), rhs[5]) + (m1 - m2 + m3))

    def wa_prep(c, kt, half, q):
        t1_s[q] = _pack(stage[half, q, 3, :128].T)
        g = gather_heads(t1_s.at[q])
        wa_s[c, pl.ds(pl.multiple_of(kt * 64, 64), 64), :] = _pack(g.astype(BF16).T)
        return g

    def wa_trip(g, half):
        lo, hi = [wa_prep(*wa_piece(g, q), half, q) for q in range(2)]
        for t in range(2):
            b11, b12 = lo[2 * t * 128:(2 * t + 1) * 128], lo[(2 * t + 1) * 128:(2 * t + 2) * 128]
            b21, b22 = hi[2 * t * 128:(2 * t + 1) * 128], hi[(2 * t + 1) * 128:(2 * t + 2) * 128]
            sums = cat([b11 + b22, b12 - b22, b21 - b11, b11 + b12, b21 + b22])
            wc_s[g, t] = _pack(sums.astype(BF16).T)

    xpre_cp.wait()
    xp_s[...] = _pack(xpre_s[...].reshape(NSEG * PRE, D))
    strassen_lhs()
    for blk, cps in zip(peel, peel_cps):
        for cp in cps:
            cp.wait()
        for m in range(3):
            js = tuple(j for mm, j in blk if mm == m)
            if js:
                pair_prep2(0, 1, m, js)
    wa_prep(0, NT - 1, 1, 0)
    wo_copy(0).start(priority=1)
    start_trip(1)

    def prologue(g, carry):
        half = g & 1

        @pl.when(g > 0)
        def _():
            wo_copy(g - 1).wait()

        @pl.when(g == NTRIP - 1)
        def _():
            for cp in awo_cps:
                cp.start()

        wait_trip(g)
        calls = [0]
        per = hw // WX_ROWS
        total = max(b - a for a, b in zip(WX_DONE, WX_DONE[1:]))
        todo = list(range(total))
        first, stop = NQ * per, (NQ + 1) * per
        for trip in range(1, NTRIP):
            first = jnp.where(g == trip, WX_DONE[trip - 1], first)
            stop = jnp.where(g == trip, WX_DONE[trip], stop)

        def hook(v):
            calls[0] += 1
            want = (calls[0] - WX_SKIP) * total // (36 - WX_SKIP - WX_TAIL)
            t = 0
            while todo and todo[0] < want:
                k = jnp.minimum(first + todo.pop(0), stop - 1)
                q = k // per
                anchor = jnp.concatenate(
                    [v[(NT * t + c) * WX_ROWS:(NT * t + c + 1) * WX_ROWS] for c in range(NT)],
                    axis=1)
                wo_piece(q, k % per, g == 0, pltpu.bitcast(anchor, U32), g > NSEG)
                t += 1

        for m in range(3):
            pair_prep2((g + 1) * PP, half, m, hook=hook)
            if m == 0:
                wa_trip(g, half)
        wo_copy(g + 1).start(priority=1)
        start_trip(g + 2)
        return carry

    lax.fori_loop(0, NTRIP, prologue, 0)

    for cp in late_cps + awo_cps:
        cp.wait()
    for cp in x_rest:
        cp.start()

    for c in range(NT):
        t1_s[c % PP] = _pack(awo_raw[c])
        awo_s[:, c * 128:(c + 1) * 128] = _pack(gather_heads(t1_s.at[c % PP]).astype(BF16))

    def out_copy(row, n, half):
        r = pl.ds(row, n)
        c = slice(half * D, (half + 1) * D)
        return pltpu.make_async_copy(out_s.at[r, c], out_hbm.at[r, c], sems.at[7])

    def segment(s, mem, u):
        last = u == SPT - 1
        row0 = pl.multiple_of(s * SEG, SEG)
        ninf = jnp.float32(-jnp.inf)

        qi = lax.broadcasted_iota(jnp.int32, (SEG, 128), 0)
        kl = lax.broadcasted_iota(jnp.int32, (SEG, 128), 1)
        is_a = kl < L
        a80 = lax.broadcasted_iota(jnp.int32, (SEG, 2 * L), 1) < L
        real = kl < 2 * L
        kpos = jnp.where(is_a, kl, kl - L)
        allowed = ((qi >= FRESH) | (qi + MEM + PRE >= kpos)) & real
        fill = jnp.where(real, NEG, ninf)
        pi = lax.broadcasted_iota(jnp.int32, (GP * PRE, 128), 0)
        pk = lax.broadcasted_iota(jnp.int32, (GP * PRE, 128), 1)
        p_own = (pk // SEG) == (pi // PRE)
        p_allowed = (pk % (MEM + PRE)) <= (pi % PRE) + MEM
        p_first = (pk % SEG) < MEM + PRE
        p_allowed = p_allowed & p_own
        p_fill = jnp.where(p_own, NEG, ninf)
        col_a = lax.broadcasted_iota(jnp.int32, (1, PW), 1) < B_DH
        col128_a = lax.broadcasted_iota(jnp.int32, (1, 128), 1) < (B_DH - 128)

        xb = xb_s[pl.ds(row0, SEG), :D].astype(F32)
        h = jnp.concatenate([xb[PRE:], mem], axis=0).astype(BF16)

        def proj(p, m):
            return _dot(h, _unpack(w_s[p, :, m * PW:(m + 1) * PW]))

        def pre(p, m):
            return pre_s[s, p, :, m * PW:(m + 1) * PW]

        def block_diag(p, m):
            f = proj(p, m)
            full = jnp.concatenate([f[FRESH:], pre(p, m), f[:FRESH]], axis=0)
            z = jnp.zeros_like(full)
            return jnp.where(col_a, full, z), jnp.where(col_a, z, full)

        def keys_t(blocks):
            fold = cat([jnp.concatenate([x[:, :128] if i % 2 == 0 else x[:, 256:], x[:, 128:256]],
                                        axis=1) for i, x in enumerate(blocks)])
            t = fold.T
            return t[:128].astype(BF16), t[128:].astype(BF16)

        def qk(q, kt, lane_a):
            outer = _dot(cat([q[:, :128], q[:, 256:]]).astype(BF16), kt[0])
            sc = (jnp.where(lane_a, outer[:SEG], outer[SEG:])
                  + _dot(q[:, 128:256].astype(BF16), kt[1]))
            if sc.shape[1] < 128:
                sc = jnp.concatenate([sc, jnp.zeros((SEG, 128 - sc.shape[1]), F32)], axis=1)
            return sc

        def row_max(raw, ok, other, first):
            sc = jnp.where(ok, raw * b_scale, other)
            ma = jnp.max(jnp.where(first, sc, ninf), axis=1, keepdims=True)
            mb = jnp.max(jnp.where(first, ninf, sc), axis=1, keepdims=True)
            return sc, ma, mb

        def probs(mx, first, late_norm):
            sc, ma, mb = mx
            e = jnp.exp2(sc - jnp.where(first, ma, mb))
            ea, eb = jnp.where(first, e, 0.0), jnp.where(first, 0.0, e)
            sa = jnp.sum(ea, axis=1, keepdims=True)
            sb = jnp.sum(eb, axis=1, keepdims=True)
            if late_norm:
                return e.astype(BF16), _recip(sa), _recip(sb)
            return (e * _recip(jnp.where(first, sa, sb))).astype(BF16), None, None

        def apply_v(e, blocks):
            pad = 128 - sum(x.shape[0] for x in blocks)
            rows = list(blocks) + ([jnp.zeros((pad, PW), F32)] if pad else [])
            return _dot(e, cat(rows).astype(BF16))

        def pv(sm, vbd):
            e, ra, rb = sm
            o = apply_v(e, vbd)
            if ra is not None:
                o = jnp.concatenate([
                    o[:, :128] * ra,
                    o[:, 128:256] * jnp.where(col128_a, ra, rb),
                    o[:, 256:] * rb], axis=1)
            return o

        def pre_pv(g, pr, vbds):
            o = apply_v(pr, [x[:MEM + PRE] for vb in vbds for x in vb])
            if not last:
                odef_s[u, g] = o
            return o

        def wout(p, o, acc):
            contrib = _dot(o.astype(BF16), _unpack(wo_s[p * hw:(p + 1) * hw, :]))
            return contrib if acc is None else acc + contrib

        def deferred(p):
            r = slice((p % GP) * PRE, (p % GP + 1) * PRE)
            return cat([odef_s[v, p // GP, r, :] for v in range(SPT - 1)]
                       + [val["PPV", p // GP][r]])

        def wout_strassen(kind, q):
            a11, a21 = val["PV", 2 * q], deferred(2 * q)
            if kind != "XA":
                a12, a22 = val["PV", 2 * q + 1], deferred(2 * q + 1)
            blk = lambda k, n: _unpack(
                wo_s[q * qr + k * hw:q * qr + (k + 1) * hw, n * KH:(n + 1) * KH])
            sm = lambda n: _unpack(wx_s[q, n])
            if kind == "XA":
                terms = {3: (a11, sm(1)), 6: (a21 - a11, sm(3))}
            elif kind == "XB":
                terms = {1: (a11 + a22, sm(0)), 4: (a22, sm(2)), 5: (a11 + a12, blk(1, 1)),
                         7: (a12 - a22, sm(4))}
            elif kind == "XC":
                terms = {2: (a21 + a22, blk(0, 0))}
            else:
                lhs = jnp.concatenate([cat([a11, a21]), cat([a12, a22])], axis=1)
                terms = {0: (lhs, _unpack(wo_s[q * qr:(q + 1) * qr, 2 * KH:]))}
            for n, (x, w) in terms.items():
                r = _dot(x.astype(BF16), w)
                val["acc", n] = val["acc", n] + r if ("acc", n) in val else r

        arow0 = pl.multiple_of((s - u % 2) * SEG, 2 * SEG)

        def a_put(m, j, r):
            if m == 0:
                qa_s[j] = _round(r)
            else:
                kv_s[m - 1, j, A_HALO:A_HALO + 2 * SEG, :] = _round(r) if m == 1 else r

        def a_proj(idx):
            m, j = divmod(idx, NT)
            if "xa" not in val:
                val["xa"] = xa_s[pl.ds(arow0, 2 * SEG), :D]
            if m < 2 or j == NT - 1:
                a_put(m, j, _dot(val["xa"], _unpack(wa_s[m, :, j * 128:(j + 1) * 128])))
                return
            t = j // 2
            if "xs" not in val:
                xf = val["xa"].astype(F32)
                f = lambda i, k: xf[i * SEG:(i + 1) * SEG, k * KH:(k + 1) * KH]
                val["xs"] = [v.astype(BF16) for v in (
                    f(0, 0) + f(1, 1), f(1, 0) + f(1, 1), f(0, 0), f(1, 1), f(0, 0) + f(0, 1),
                    f(1, 0) - f(0, 0), f(0, 1) - f(1, 1))]
                val["xr"] = xf[:, 2 * KH:].astype(BF16)
            sm = lambda n: _unpack(cat([wc_s[2 * m + k, t, :, n * 128:(n + 1) * 128]
                                        for k in range(2)]))
            blk = lambda k, j: _unpack(wa_s[m, k * KH // 2:(k + 1) * KH // 2,
                                            (2 * t + j) * 128:(2 * t + j + 1) * 128])
            rhs = (sm(0), blk(0, 0), sm(1), sm(2), blk(1, 1), sm(3), sm(4))
            mm = lambda n: _dot(val["xs"][n], rhs[n])
            tail = [_dot(val["xr"], _unpack(wa_s[m, KH:, (2 * t + j) * 128:(2 * t + j + 1) * 128]))
                    for j in range(2)]
            m1, m2, m3, m4, m5 = [mm(n) for n in range(5)]
            a_put(m, 2 * t, tail[0] + cat([mm(6) + (m1 + m4 - m5), m2 + m4]))
            a_put(m, 2 * t + 1, tail[1] + cat([m3 + m5, mm(5) + (m1 - m2 + m3)]))

        def window(m, j, w, hf):
            lo = A_HALO + hf * SEG - A_DIL * w
            return kv_s[m, j, lo:lo + SEG, :]

        def local_softmax(hf):
            pos = arow0 + hf * SEG + lax.broadcasted_iota(jnp.int32, (SEG, 128), 0)
            rows = slice(hf * SEG, (hf + 1) * SEG)
            logits = []
            for w in range(A_W):
                t = qa_s[0, rows, :] * window(0, 0, w, hf)
                for j in range(1, NT):
                    t = t + qa_s[j, rows, :] * window(0, j, w, hf)
                t = t + pltpu.roll(t, 64, 1)
                t = t + pltpu.roll(t, 32, 1)
                t = _round(_round(t) * a_scale)
                if w > 0 and hf == 0:
                    t = jnp.where(pos >= A_DIL * w, t, -1000000000.0)
                logits.append(t)
            mx = functools.reduce(jnp.maximum, logits)
            es = [jnp.exp(l - mx) for l in logits]
            inv = _recip(functools.reduce(lambda x, y: x + y, es))
            return es, inv

        def local_pv(j, hf):
            es, inv = val["LA", hf]
            o = es[0] * window(1, j, 0, hf)
            for w in range(1, A_W):
                o = o + es[w] * window(1, j, w, hf)
            return o * inv

        def local_out(j, acc):
            wj = _unpack(awo_s[j * 64:(j + 1) * 64, :])
            r = _dot(cat([local_pv(j, 0), local_pv(j, 1)]).astype(BF16), wj)
            for m in range(2):
                kv_s[m, j, :A_HALO, :] = kv_s[m, j, 2 * SEG:2 * SEG + A_HALO, :]
            return r if acc is None else acc + r

        val = {}
        acc = None
        oa = None
        for kind, t in _order(u):
            if kind == "K":
                val[kind, t] = block_diag(t, 1)
            elif kind == "V":
                val[kind, t] = block_diag(t, 2)
            elif kind == "Q":
                val[kind, t] = proj(t, 0)
            elif kind == "T":
                val[kind, t] = keys_t(val["K", t])
            elif kind == "S":
                val[kind, t] = qk(val["Q", t], val["T", t], a80)
            elif kind == "M":
                val[kind, t] = row_max(val["S", t], allowed, fill, is_a)
            elif kind == "E":
                val[kind, t] = probs(val["M", t], is_a, t >= LATE_FROM)
            elif kind == "PV":
                val[kind, t] = pv(val["E", t], val["V", t])
            elif kind == "TG":
                val[kind, t] = keys_t([x[:MEM + PRE] for r in range(GP)
                                       for x in val["K", GP * t + r]])
            elif kind == "PS":
                q = cat([pre(GP * t + r, 0) for r in range(GP)])
                val[kind, t] = qk(q, val["TG", t], p_first)
            elif kind == "MG":
                val[kind, t] = row_max(val["PS", t], p_allowed, p_fill, p_first)
            elif kind == "EG":
                val[kind, t] = probs(val["MG", t], p_first, False)[0]
            elif kind == "PPV":
                val[kind, t] = pre_pv(t, val["EG", t], [val["V", GP * t + r] for r in range(GP)])
            elif kind == "W":
                acc = wout(t, val["PV", t], acc)
            elif kind in ("XA", "XB", "XC", "Y"):
                wout_strassen(kind, t)
            elif kind == "LA":
                val[kind, t] = local_softmax(t)
            elif kind == "AP":
                a_proj(t)
            elif kind == "AO":
                oa = local_out(t, oa)
                if t == NT - 1:
                    out_s[pl.ds(arow0, 2 * SEG), :D] = oa.astype(BF16)
                    out_copy(arow0, 2 * SEG, 0).start()
        if last:
            m = lambda n: val["acc", n]
            acc = jnp.concatenate([
                cat([m(1) + m(4) - m(5) + m(7), m(2) + m(4)]),
                cat([m(3) + m(5), m(1) - m(2) + m(3) + m(6)]), m(0)], axis=1)
        return acc

    def steps(i, mem):
        @pl.when(i == 1)
        def _():
            for cp in x_rest:
                cp.wait()

        accs = []
        for u in range(SPT):
            accs.append(segment(i * SPT + u, mem, u))
            mem = accs[-1][FRESH:SEG]
        res = cat([x for u in range(SPT) for x in (
            accs[-1][SEG + u * PRE:SEG + (u + 1) * PRE], accs[u][:FRESH])])
        row = pl.multiple_of(i * SPT * SEG, SPT * SEG)
        out_s[pl.ds(row, SPT * SEG), D:2 * D] = res.astype(BF16)
        out_copy(row, SPT * SEG, 1).start()
        return mem

    lax.fori_loop(0, N_STEPS, steps, mem0_s[...].astype(F32))

    wo_copy(NTRIP - 1).wait()
    wo_copy(NTRIP).wait()
    wait_trip(NTRIP)
    wait_trip(NTRIP + 1)

    done = N_STEPS * SPT * SEG
    pltpu.make_async_copy(out_s.at[:done, :2 * D], out_hbm.at[:done, :], sems.at[7]).wait()


@jax.jit
def pallas_concat_heads__sliding_local_dilated__memory_aug_recurrent_mem_tr__prompt_kernel(
    A_x: jax.Array,
    A_wqkv: jax.Array,
    A_wo: jax.Array,
    B_x: jax.Array,
    B_mem0: jax.Array,
    B_Wq: jax.Array,
    B_Wk: jax.Array,
    B_Wv: jax.Array,
    B_Wo: jax.Array,
    B_seg_len,
):
    del B_seg_len
    assert A_x.shape == (1, S, D) and B_x.shape == (1, S, D)
    hd = B_H * B_DH
    wq_t = jnp.transpose(B_Wq, (1, 2, 0)).reshape(hd, D)
    wk_t = jnp.transpose(B_Wk, (1, 2, 0)).reshape(hd, D)
    wv_t = jnp.transpose(B_Wv, (1, 2, 0)).reshape(hd, D)
    wo = B_Wo.reshape(hd, D)

    any_spec = pl.BlockSpec(memory_space=pl.ANY)
    out = pl.pallas_call(
        _kernel,
        out_shape=jax.ShapeDtypeStruct((S, 2 * D), BF16),
        in_specs=[any_spec] * 10,
        out_specs=any_spec,
        scratch_shapes=[
            pltpu.VMEM((2, PP, 4, PW, D), BF16),
            pltpu.VMEM((NT, D, 128), BF16),
            pltpu.VMEM((4, 2 * WO_ROWS, D), BF16),
            pltpu.VMEM((NP, D // 2, 3 * PW), U32),
            pltpu.VMEM((hd // 2 + PW, D), U32),
            pltpu.VMEM((NQ + 1, 5, PW // 2, KH), U32),
            pltpu.VMEM((NSEG, NP, PRE, 3 * PW), F32),
            pltpu.VMEM((SPT - 1, NG, GP * PRE, PW), F32),
            pltpu.VMEM((S, OUT_W), BF16),
            pltpu.VMEM((S, X_W), BF16),
            pltpu.VMEM((S, X_W), BF16),
            pltpu.VMEM((NSEG, PRE, D), BF16),
            pltpu.VMEM((NSEG * PRE // 2, D), U32),
            pltpu.VMEM((5, NSEG * PRE // 4, 256), U32),
            pltpu.VMEM((MEM, D), BF16),
            pltpu.VMEM((3, D // 2, D), U32),
            pltpu.VMEM((NTRIP, 2, 64, D), U32),
            pltpu.VMEM((D // 2, D), U32),
            pltpu.VMEM((PP, D // 2, 128), U32),
            pltpu.VMEM((NT, 2 * SEG, 128), F32),
            pltpu.VMEM((2, NT, A_HALO + 2 * SEG, 128), F32),
            pltpu.SemaphoreType.DMA((10,)),
        ],
        compiler_params=pltpu.CompilerParams(vmem_limit_bytes=120 * 1024 * 1024,
                                             disable_bounds_checks=True),
    )(A_x.reshape(S, D), A_wqkv, A_wo, B_x.reshape(S, D), B_x.reshape(NSEG, SEG // PRE, PRE, D),
      B_mem0.reshape(MEM, D), wq_t, wk_t, wv_t, wo)
    return out.reshape(1, S, 2 * D)
```

```python
import functools

import jax
import jax.numpy as jnp
from jax import lax
import jax.experimental.pallas as pl
import jax.experimental.pallas.tpu as pltpu

F32 = jnp.float32
BF16 = jnp.bfloat16
U32 = jnp.uint32

S = 2048
D = 640
NT = D // 128
A_H = 32
A_DH = D // A_H
A_W = 8
A_DIL = 2
A_HALO = 16
B_H = 32
B_DH = 192
MEM = 8
SEG = 32
NSEG = S // SEG
NP = B_H // 2
PW = 2 * B_DH
PRE = 8
FRESH = SEG - PRE
L = MEM + SEG
GP = 4
NG = NP // GP
LOG2E = 1.4426950408889634
NEG = -1000000000.0 * LOG2E
PP = 2
NTRIP = NP // PP - 1
PEEL = (2, 2, 5)
KH = 256
WO_ROWS = 512
WX_DONE = (0, 192, 448, 768, 960, 1216, 1536)
WX_ROWS = 16
WX_SKIP, WX_TAIL = 2, 2
ST_ROWS = 256
X_HEAD = 128
X_W = 768
WO_W = 768
PRE_W = 2560
SPT = 4
N_STEPS = NSEG // SPT
NQ = NP // 2

LAT_MM, LAT_X, LAT_T, LAT_N, LAT_N_LATE = 190, 190, 380, 230, 100
LATE_FROM = NP - 2
AP_AFTER = (6, 12, 18, 24, 30)
AO_AFTER = (30, 40)
TAIL_FILL = (2, 2, 2, 0)
HOLD_W = (0, 3, 0, 0)


def _segment_order(u):
    odd, last = u % 2 == 1, u == SPT - 1
    proj = []
    for g in range(NG):
        proj += [("K", GP * g + r) for r in range(GP)]
        for r in range(GP):
            proj += [("V", GP * g + r), ("Q", GP * g + r)]
    dur = {"K": 120, "V": 120, "Q": 120, "S": 24, "PV": 24, "PS": 24, "PPV": 24,
           "W": 120, "XA": 96, "XB": 192, "XC": 48, "Y": 96, "AO": 80, "AP": 90,
           "T": 0, "M": 0, "E": 0, "TG": 0, "MG": 0, "EG": 0}
    end = {}

    def ready(task):
        k, i = task
        if k == "T":
            deps = [(("K", i), LAT_MM)]
        elif k == "S":
            deps = [(("Q", i), LAT_MM), (("T", i), LAT_T)]
        elif k == "M":
            deps = [(("S", i), LAT_MM - 40)]
        elif k == "E":
            deps = [(("M", i), LAT_X)]
        elif k == "PV":
            deps = [(("E", i), LAT_N_LATE if i >= LATE_FROM else LAT_N), (("V", i), LAT_MM)]
        elif k == "TG":
            deps = [(("K", GP * i + r), LAT_MM) for r in range(GP)]
        elif k == "PS":
            deps = [(("TG", i), LAT_T)]
        elif k == "MG":
            deps = [(("PS", i), LAT_MM - 40)]
        elif k == "EG":
            deps = [(("MG", i), LAT_X)]
        elif k == "PPV":
            deps = [(("EG", i), LAT_N), (("V", GP * i + GP - 1), LAT_MM)]
        elif k == "W":
            deps = [(("PV", i), LAT_MM)]
        else:
            deps = [(("PV", 2 * i), LAT_MM), (("PPV", 2 * i // GP), LAT_MM)]
            if k != "XA":
                deps.append((("PV", 2 * i + 1), LAT_MM))
        if any(d not in end for d, _ in deps):
            return None
        return max(end[d] + lat for d, lat in deps)

    pend = ([(k, p) for k in ("E", "M", "T") for p in range(NP)]
            + [(k, g) for k in ("EG", "MG", "TG") for g in range(NG)]
            + ([(k, q) for q in range(NQ) for k in ("XA", "XB", "Y", "XC")] if last
               else [("W", p) for p in range(NP)])
            + [("PPV", g) for g in range(NG)]
            + [("PV", p) for p in range(NP)] + [("PS", g) for g in range(NG)]
            + [("S", p) for p in range(NP)])
    fill = [("AO", j) for j in range(NT)] if odd else [("AP", j) for j in (5, 6, 7, 8, 9, 0, 1, 2, 3, 4, 10, 12, 14)]
    order = []
    now = [0]

    def emit(task):
        order.append(task)
        now[0] += dur[task[0]]
        end[task] = now[0]

    nproj = 0
    while pend:
        cand = [x for x in pend if ready(x) is not None and ready(x) <= now[0]]
        if proj:
            cand = [x for x in cand if not (x[0] == "W" and x[1] >= NP - GP - HOLD_W[u])]
        if cand:
            if not proj:
                cand = [x for x in cand if x[0] not in ("W", "XA", "XB", "XC", "Y")] or cand
            pend.remove(cand[0])
            emit(cand[0])
        elif proj:
            emit(proj.pop(0))
            nproj += 1
            if odd and nproj == GP:
                order += [("LA", 0), ("LA", 1)]
            if nproj in (AO_AFTER if odd else AP_AFTER):
                emit(fill.pop(0))
        elif len(fill) > TAIL_FILL[u]:
            emit(fill.pop(0))
        else:
            now[0] = min(ready(x) for x in pend if ready(x) is not None)
    return order + fill


ORDERS = (
    "K0 T0 K1 K3 K2 V0 T1 T2 Q1 T3 Q0 AP5 Q2 AP6 S0 TG0 M0 PS0 V1 V2 V3 E0 MG0 S1 S2 M1 Q3 EG0 "
    "PV0 K4 K5 E1 M2 S3 K6 T4 W0 E2 M3 T5 PPV0 PV1 K7 AP7 AP8 E3 T6 W1 T7 TG1 PV2 PV3 Q4 W2 V4 W3 "
    "PS1 Q5 S4 V5 M4 MG1 V6 Q7 Q6 E4 S5 EG1 V7 M5 PV4 S6 K8 PPV1 E5 S7 M6 W4 K9 E6 M7 T8 K10 PV5 "
    "AP9 T9 K11 E7 W5 T10 TG2 PV6 V8 T11 PV7 Q8 W7 S8 W6 PS2 V10 V9 Q9 M8 MG2 Q10 E8 EG2 V11 S9 "
    "Q11 M9 PV8 S10 K12 T12 PPV2 E9 S11 M10 W8 E10 M11 PV9 K14 K13 K15 E11 T13 W9 PV10 V12 T14 "
    "T15 TG3 PV11 Q12 W10 W11 PS3 S12 Q13 V13 M12 MG3 V15 V14 E12 Q14 EG3 Q15 S13 M13 PV12 S14 "
    "AP0 AP1 PPV3 E13 W12 S15 M14 AP2 AP3 E14 PV13 M15 AP4 AP10 PV14 W13 E15 PV15 W14 W15 AP14 "
    "AP12 ",
    "K0 K2 K1 T0 K3 LA0 LA1 Q0 V1 T1 V0 T2 T3 TG0 Q1 S0 V2 PS0 Q2 M0 S1 V3 MG0 Q3 M1 S2 K4 EG0 K5 "
    "E0 E1 M2 PV0 S3 K6 T4 K7 PPV0 E2 T5 M3 W0 T6 PV1 PV2 V4 E3 T7 TG1 Q4 W1 W2 PV3 PS1 S4 V5 Q5 "
    "M4 MG1 W3 AO0 S5 V6 E4 EG1 Q6 M5 V7 PV4 Q7 E5 S6 K8 W4 M6 PPV1 PV5 S7 K9 T8 E6 W5 K10 M7 PV6 "
    "T9 K11 E7 T10 V8 W6 T11 TG2 PV7 Q8 AO1 W7 S8 V9 PS2 Q9 M8 V10 MG2 Q10 E8 S9 V11 EG2 Q11 PV8 "
    "M9 S10 K12 PPV2 E9 S11 M10 K13 W8 E10 M11 T12 PV9 K14 K15 E11 T13 T14 PV10 AO2 V12 T15 TG3 "
    "Q12 PV11 V13 Q13 PS3 S12 V14 Q14 M12 S13 MG3 V15 Q15 E12 M13 EG3 S14 W9 E13 M14 PPV3 W10 "
    "PV12 S15 W11 E14 M15 PV13 W12 PV14 E15 W13 PV15 W14 W15 AO3 AO4 ",
    "K0 K1 T0 K3 T1 AP5 K2 AP6 V0 Q0 TG0 T3 T2 V1 S0 Q1 PS0 Q2 V2 M0 S1 V3 E0 MG0 Q3 M1 K4 S2 EG0 "
    "PV0 K5 E1 M2 PPV0 S3 K6 T4 W0 E2 M3 T5 AP7 AP8 PV1 K7 E3 W1 T6 T7 TG1 PV2 V4 PV3 Q4 W2 W3 "
    "PS1 S4 V5 M4 Q5 MG1 V6 S5 Q6 EG1 E4 V7 Q7 M5 PV4 S6 K8 PPV1 E5 S7 M6 W4 AP9 K9 E6 M7 T8 PV5 "
    "K10 T9 K11 E7 W5 T10 PV6 V8 T11 TG2 Q8 PV7 W6 W7 S8 PS2 Q9 M8 MG2 V10 V9 Q10 E8 EG2 S9 V11 "
    "Q11 M9 PV8 S10 K12 PPV2 E9 W8 S11 M10 K13 E10 M11 T12 PV9 K14 K15 E11 T13 W9 PV11 T14 PV10 "
    "V12 T15 TG3 Q12 W10 V13 W11 PS3 S12 Q13 MG3 M12 V14 Q14 E12 EG3 S13 V15 Q15 M13 PV12 S14 E13 "
    "AP0 AP1 PPV3 S15 M14 W12 AP2 AP3 M15 AP4 E14 PV14 PV13 AP10 E15 W13 PV15 W14 W15 AP12 AP14 ",
    "K1 K0 K2 T0 K3 LA0 LA1 T1 V0 T2 Q0 T3 TG0 V1 Q1 S0 PS0 M0 V2 Q2 V3 MG0 Q3 S1 E0 M1 S2 EG0 K4 "
    "K5 M2 T4 PV0 E1 AO0 PPV0 S3 K6 E2 T5 K7 M3 XA0 T6 PV1 PV2 Y0 V4 E3 T7 TG1 Q4 XB0 XC0 XA1 PV3 "
    "PS1 S4 V5 Q5 M4 MG1 XB1 E4 Y1 XC1 EG1 S5 Q6 V6 M5 V7 S6 PV4 AO1 Q7 E5 PPV1 K8 S7 M6 XA2 K9 "
    "M7 T8 PV5 K10 E6 T9 XB2 E7 T10 Y2 K11 TG2 T11 XC2 PV6 PV7 V8 Y3 Q8 XA3 XB3 PS2 S8 V9 Q9 M8 "
    "MG2 V10 Q10 AO2 E8 EG2 S9 V11 S10 M9 PV8 K12 Q11 M10 PPV2 K13 E9 K14 S11 E10 T12 M11 T13 K15 "
    "PV10 PV9 XA4 T14 V12 E11 XB4 T15 TG3 XA5 Y4 Q12 AO3 PV11 XB5 PS3 S12 V13 Q13 MG3 V14 M12 Q14 "
    "EG3 S13 V15 E12 M13 PV12 Q15 S14 AO4 PPV3 E13 S15 M14 E14 XA6 M15 XC3 XC4 XC5 PV13 E15 Y5 "
    "PV14 XB6 PV15 Y6 XA7 XB7 XC6 Y7 XC7 ",
)
SKIP_PROLOGUE = False


def _order(u):
    if ORDERS is None or ORDERS[u] is None:
        return _segment_order(u)
    return [(t.rstrip("0123456789"), int(t.lstrip("ABCDEFGHIJKLMNOPQRSTUVWXYZ")))
            for t in ORDERS[u].split()]


def _nt_dot(a, b):
    return lax.dot_general(a, b, (((1,), (1,)), ((), ())), preferred_element_type=F32)


def _dot(a, b):
    return jnp.dot(a, b, preferred_element_type=F32)


def _pack(x):
    return pltpu.bitcast(x, U32)


def _unpack(x):
    return pltpu.bitcast(x, BF16)


def cat(parts):
    return jnp.concatenate(parts, axis=0)


def _round(x):
    return x.astype(BF16).astype(F32)


def _recip(x):
    r = pl.reciprocal(x, approx=True)
    return r * (2.0 - x * r)


def _kernel(ax_hbm, awqkv_hbm, awo_hbm, bx_hbm, bx4_hbm, mem0_hbm, wq_hbm, wk_hbm, wv_hbm, wo_hbm,
            out_hbm,
            stage, awo_raw, wo_raw, w_s, wo_s, wx_s, pre_s, odef_s, out_s,
            xa_s, xb_s, xpre_s, xp_s, xs_s, mem0_s, wa_s, wc_s, awo_s, t1_s, qa_s, kv_s,
            sems):
    b_scale = 0.072265625 * LOG2E
    a_scale = 0.2236328125

    w_hbm = (wq_hbm, wk_hbm, wv_hbm)
    hw = PW // 2
    hd = B_H * B_DH

    def w_copy(p, half, q, m, sem):
        rows = pl.ds(pl.multiple_of(p * PW, PW), PW)
        return pltpu.make_async_copy(w_hbm[m].at[rows, :], stage.at[half, q, m], sem)

    def wa_piece(g, q):
        last = g >= 2 * 3
        return jnp.where(last, 1 + q, g >> 1), jnp.where(last, NT - 1, (g & 1) + 2 * q)

    def wa_copy(c, kt, half, q, sem):
        return pltpu.make_async_copy(
            awqkv_hbm.at[pl.ds(pl.multiple_of(kt * 128, 128), 128),
                         pl.ds(pl.multiple_of(c * D, 128), D)],
            stage.at[half, q, 3, :128], sem)

    def trip_copies(g):
        half = g & 1
        src = jnp.minimum(g, NTRIP - 1)
        cps = []
        for q in range(PP):
            cps += [w_copy((src + 1) * PP + q, half, q, m, sems.at[half]) for m in range(3)]
            cps.append(wa_copy(*wa_piece(src, q), half, q, sems.at[half]))
        return cps

    def start_trip(g):
        for cp in trip_copies(g):
            cp.start(priority=1)

    def wait_trip(g):
        for cp in trip_copies(g):
            cp.wait()

    qr = 2 * hw

    def wo_copy(c):
        src = jnp.minimum(c, hd // (2 * WO_ROWS) - 1)
        rows = pl.ds(pl.multiple_of(src * 2 * WO_ROWS, 2 * WO_ROWS), 2 * WO_ROWS)
        return pltpu.make_async_copy(wo_hbm.at[rows, :], wo_raw.at[lax.rem(c, 3), :, :D],
                                     sems.at[8 + (c & 1)])

    def wo_piece(q, piece, spare, anchor, never):
        half = []
        for k in range(2):
            r = q * qr + k * hw + piece * WX_ROWS
            c = r // WO_ROWS
            slot = jnp.where(spare, 3, lax.rem(c, 3))
            off = jnp.where(spare, 0, 2 * (r - c * WO_ROWS))
            rows = pl.ds(pl.multiple_of(off, 16), 2 * WX_ROWS)
            w = jnp.where(never, anchor, _pack(wo_raw[slot, rows, :D]))
            wo_s[pl.ds(pl.multiple_of(r, 8), WX_ROWS), :D] = w
            half.append(_unpack(w[:, :2 * KH]).astype(F32))
        b11, b12, b21, b22 = [half[k][:, n * KH:(n + 1) * KH] for k in range(2) for n in range(2)]
        for n, v in enumerate((b11 + b22, b12 - b22, b21 - b11, b11 + b12, b21 + b22)):
            wx_s[q, n, pl.ds(pl.multiple_of(piece * WX_ROWS, 8), WX_ROWS), :] = (
                _pack(v.astype(BF16)))

    def x_copies(xr, sem):
        return [pltpu.make_async_copy(ax_hbm.at[xr, :], xa_s.at[xr, :D], sem),
                pltpu.make_async_copy(bx_hbm.at[xr, :], xb_s.at[xr, :D], sem)]

    xpre_cp = pltpu.make_async_copy(bx4_hbm.at[:, 0], xpre_s, sems.at[3])
    late_cps = ([pltpu.make_async_copy(mem0_hbm, mem0_s, sems.at[2])]
                + x_copies(pl.ds(0, X_HEAD), sems.at[2]))
    awo_cps = [
        pltpu.make_async_copy(awo_hbm.at[:, c * 128:(c + 1) * 128], awo_raw.at[c], sems.at[2])
        for c in range(NT)]
    x_rest = x_copies(pl.ds(X_HEAD, S - X_HEAD), sems.at[3])
    tiles = [(m, j) for m in range(3) for j in range(PW // 128)]
    peel = [tiles[sum(PEEL[:n]):sum(PEEL[:n + 1])] for n in range(len(PEEL))]
    peel_cps = [[pltpu.make_async_copy(w_hbm[m].at[pl.ds(q * PW + j * 128, 128), :],
                                       stage.at[1, q, m, pl.ds(j * 128, 128), :], sems.at[4 + n])
                 for m, j in blk for q in range(PP)] for n, blk in enumerate(peel)]
    peel_cps[-1].append(wa_copy(0, NT - 1, 1, 0, sems.at[3 + len(PEEL)]))

    xpre_cp.start()
    for cps in peel_cps:
        for cp in cps:
            cp.start(priority=1)
    start_trip(0)
    for cp in late_cps:
        cp.start(priority=1)
    kv_s[:, :, :A_HALO, :] = jnp.zeros((2, NT, A_HALO, 128), F32)
    wo_raw[3, :2 * WX_ROWS, :D] = jnp.zeros((2 * WX_ROWS, D), BF16)

    def gather_heads(ref):
        rows = []
        for j in range(A_DH // 2):
            u = ref[pl.ds(j, A_H, stride=A_DH // 2), :]
            rows.append(pltpu.bitcast(u << 16, F32))
            rows.append(pltpu.bitcast(u & jnp.uint32(0xFFFF0000), F32))
        return jnp.concatenate(rows, axis=0)

    HR = NSEG * PRE // 2

    def xq(i, k):
        return _unpack(xp_s[i * HR // 2:(i + 1) * HR // 2, k * KH:(k + 1) * KH])

    def strassen_lhs():
        f = lambda i, k: xq(i, k).astype(F32)
        sums = (f(0, 0) + f(1, 1), f(1, 0) + f(1, 1), f(0, 0) + f(0, 1),
                f(1, 0) - f(0, 0), f(0, 1) - f(1, 1))
        for n, v in enumerate(sums):
            xs_s[n] = _pack(v.astype(BF16))

    def pair_prep2(pp, half, m, js=(0, 1, 2), hook=None):
        if SKIP_PROLOGUE:
            return
        p = pp * PP
        for q in range(2):
            lo, hi = js[0] * 128, (js[-1] + 1) * 128
            w_s[p + q, :, m * PW + lo:m * PW + hi] = _pack(stage[half, q, m, lo:hi, :].T)
        nseg = ST_ROWS // PRE
        for j in js:
            rows = slice(j * 128, (j + 1) * 128)
            b = lambda k, q: stage[half, q, m, rows, k * KH:(k + 1) * KH]
            bf = lambda k, q: b(k, q).astype(F32)
            rhs = ((bf(0, 0) + bf(1, 1)).astype(BF16), b(0, 0),
                   (bf(0, 1) - bf(1, 1)).astype(BF16), (bf(1, 0) - bf(0, 0)).astype(BF16),
                   b(1, 1), (bf(0, 0) + bf(0, 1)).astype(BF16),
                   (bf(1, 0) + bf(1, 1)).astype(BF16))
            tail = [stage[half, q, m, rows, 2 * KH:] for q in range(2)]
            for c in range(HR // ST_ROWS):
                r = slice(c * ST_ROWS // 2, (c + 1) * ST_ROWS // 2)
                sm = lambda n: _unpack(xs_s[n, r, :])
                qd = lambda i, k: _unpack(
                    xp_s[(i * HR + c * ST_ROWS) // 2:(i * HR + (c + 1) * ST_ROWS) // 2,
                         k * KH:(k + 1) * KH])
                rest = lambda i: _unpack(
                    xp_s[(i * HR + c * ST_ROWS) // 2:(i * HR + (c + 1) * ST_ROWS) // 2, 2 * KH:])

                def put(i, q, v):
                    s0 = i * (NSEG // 2) + c * nseg
                    col = (3 * q + m) * PW + j * 128
                    pre_s[s0:s0 + nseg, pp, :, col:col + 128] = v.reshape(nseg, PRE, 128)
                    if hook is not None:
                        hook(v)

                m5 = _nt_dot(sm(2), rhs[4])
                m3 = _nt_dot(qd(0, 0), rhs[2])
                put(0, 1, _nt_dot(rest(0), tail[1]) + m3 + m5)
                m1 = _nt_dot(sm(0), rhs[0])
                m4 = _nt_dot(qd(1, 1), rhs[3])
                put(0, 0, _nt_dot(rest(0), tail[0]) + _nt_dot(sm(4), rhs[6]) + (m1 + m4 - m5))
                m2 = _nt_dot(sm(1), rhs[1])
                put(1, 0, _nt_dot(rest(1), tail[0]) + m2 + m4)
                put(1, 1, _nt_dot(rest(1), tail[1]) + _nt_dot(sm(3), rhs[5]) + (m1 - m2 + m3))

    def wa_prep(c, kt, half, q):
        t1_s[q] = _pack(stage[half, q, 3, :128].T)
        g = gather_heads(t1_s.at[q])
        wa_s[c, pl.ds(pl.multiple_of(kt * 64, 64), 64), :] = _pack(g.astype(BF16).T)
        return g

    def wa_trip(g, half):
        lo, hi = [wa_prep(*wa_piece(g, q), half, q) for q in range(2)]
        for t in range(2):
            b11, b12 = lo[2 * t * 128:(2 * t + 1) * 128], lo[(2 * t + 1) * 128:(2 * t + 2) * 128]
            b21, b22 = hi[2 * t * 128:(2 * t + 1) * 128], hi[(2 * t + 1) * 128:(2 * t + 2) * 128]
            sums = cat([b11 + b22, b12 - b22, b21 - b11, b11 + b12, b21 + b22])
            wc_s[g, t] = _pack(sums.astype(BF16).T)

    xpre_cp.wait()
    xp_s[...] = _pack(xpre_s[...].reshape(NSEG * PRE, D))
    strassen_lhs()
    for blk, cps in zip(peel, peel_cps):
        for cp in cps:
            cp.wait()
        for m in range(3):
            js = tuple(j for mm, j in blk if mm == m)
            if js:
                pair_prep2(0, 1, m, js)
    wa_prep(0, NT - 1, 1, 0)
    wo_copy(0).start(priority=1)
    start_trip(1)

    def prologue(g, carry):
        half = g & 1

        @pl.when(g > 0)
        def _():
            wo_copy(g - 1).wait()

        @pl.when(g == NTRIP - 1)
        def _():
            for cp in awo_cps:
                cp.start()

        wait_trip(g)
        calls = [0]
        per = hw // WX_ROWS
        done = [x // WX_ROWS for x in WX_DONE]
        total = max(b - a for a, b in zip(done, done[1:]))
        todo = list(range(total))
        first, stop = NQ * per, (NQ + 1) * per
        for trip in range(1, NTRIP):
            first = jnp.where(g == trip, done[trip - 1], first)
            stop = jnp.where(g == trip, done[trip], stop)

        def hook(v):
            calls[0] += 1
            want = (calls[0] - WX_SKIP) * total // (36 - WX_SKIP - WX_TAIL)
            t = 0
            while todo and todo[0] < want:
                k = jnp.minimum(first + todo.pop(0), stop - 1)
                q = k // per
                anchor = jnp.concatenate(
                    [v[(NT * t + c) * WX_ROWS:(NT * t + c + 1) * WX_ROWS] for c in range(NT)],
                    axis=1)
                wo_piece(q, k % per, g == 0, pltpu.bitcast(anchor, U32), g > NSEG)
                t += 1

        for m in range(3):
            pair_prep2(g + 1, half, m, hook=hook)
            if m == 0:
                wa_trip(g, half)
        wo_copy(g + 1).start(priority=1)
        start_trip(g + 2)
        return carry

    lax.fori_loop(0, NTRIP, prologue, 0)

    for cp in late_cps + awo_cps:
        cp.wait()
    for cp in x_rest:
        cp.start()

    for c in range(NT):
        t1_s[c] = _pack(awo_raw[c])
        awo_s[:, c * 128:(c + 1) * 128] = _pack(gather_heads(t1_s.at[c]).astype(BF16))

    def out_copy(row, n, half):
        r = pl.ds(row, n)
        c = slice(half * D, (half + 1) * D)
        return pltpu.make_async_copy(out_s.at[r, c], out_hbm.at[r, c], sems.at[7])

    def segment(s, mem, u):
        last = u == SPT - 1
        row0 = pl.multiple_of(s * SEG, SEG)
        ninf = jnp.float32(-jnp.inf)

        qi = lax.broadcasted_iota(jnp.int32, (SEG, 128), 0)
        kl = lax.broadcasted_iota(jnp.int32, (SEG, 128), 1)
        is_a = kl < L
        a80 = lax.broadcasted_iota(jnp.int32, (SEG, 2 * L), 1) < L
        real = kl < 2 * L
        kpos = jnp.where(is_a, kl, kl - L)
        allowed = ((qi >= FRESH) | (qi + MEM + PRE >= kpos)) & real
        fill = jnp.where(real, NEG, ninf)
        pi = lax.broadcasted_iota(jnp.int32, (GP * PRE, 128), 0)
        pk = lax.broadcasted_iota(jnp.int32, (GP * PRE, 128), 1)
        p_own = (pk // SEG) == (pi // PRE)
        p_allowed = (pk % (MEM + PRE)) <= (pi % PRE) + MEM
        p_first = (pk % SEG) < MEM + PRE
        p_allowed = p_allowed & p_own
        p_fill = jnp.where(p_own, NEG, ninf)
        col_a = lax.broadcasted_iota(jnp.int32, (1, PW), 1) < B_DH
        col128_a = lax.broadcasted_iota(jnp.int32, (1, 128), 1) < (B_DH - 128)

        xb = xb_s[pl.ds(row0, SEG), :D].astype(F32)
        h = jnp.concatenate([xb[PRE:], mem], axis=0).astype(BF16)

        def proj(p, m):
            return _dot(h, _unpack(w_s[p, :, m * PW:(m + 1) * PW]))

        def pre(p, m):
            col = (3 * (p % PP) + m) * PW
            return pre_s[s, p // PP, :, col:col + PW]

        def block_diag(p, m):
            f = proj(p, m)
            full = jnp.concatenate([f[FRESH:], pre(p, m), f[:FRESH]], axis=0)
            z = jnp.zeros_like(full)
            return jnp.where(col_a, full, z), jnp.where(col_a, z, full)

        def keys_t(blocks):
            fold = cat([jnp.concatenate([x[:, :128] if i % 2 == 0 else x[:, 256:], x[:, 128:256]],
                                        axis=1) for i, x in enumerate(blocks)])
            t = fold.T
            return t[:128].astype(BF16), t[128:].astype(BF16)

        def qk(q, kt, lane_a):
            outer = _dot(cat([q[:, :128], q[:, 256:]]).astype(BF16), kt[0])
            sc = (jnp.where(lane_a, outer[:SEG], outer[SEG:])
                  + _dot(q[:, 128:256].astype(BF16), kt[1]))
            if sc.shape[1] < 128:
                sc = jnp.concatenate([sc, jnp.zeros((SEG, 128 - sc.shape[1]), F32)], axis=1)
            return sc

        def row_max(raw, ok, other, first):
            sc = jnp.where(ok, raw * b_scale, other)
            ma = jnp.max(jnp.where(first, sc, ninf), axis=1, keepdims=True)
            mb = jnp.max(jnp.where(first, ninf, sc), axis=1, keepdims=True)
            return sc, ma, mb

        def probs(mx, first, late_norm):
            sc, ma, mb = mx
            e = jnp.exp2(sc - jnp.where(first, ma, mb))
            ea, eb = jnp.where(first, e, 0.0), jnp.where(first, 0.0, e)
            sa = jnp.sum(ea, axis=1, keepdims=True)
            sb = jnp.sum(eb, axis=1, keepdims=True)
            if late_norm:
                return e.astype(BF16), _recip(sa), _recip(sb)
            return (e * _recip(jnp.where(first, sa, sb))).astype(BF16), None, None

        def apply_v(e, blocks):
            pad = 128 - sum(x.shape[0] for x in blocks)
            rows = list(blocks) + ([jnp.zeros((pad, PW), F32)] if pad else [])
            return _dot(e, cat(rows).astype(BF16))

        def pv(sm, vbd):
            e, ra, rb = sm
            o = apply_v(e, vbd)
            if ra is not None:
                o = jnp.concatenate([
                    o[:, :128] * ra,
                    o[:, 128:256] * jnp.where(col128_a, ra, rb),
                    o[:, 256:] * rb], axis=1)
            return o

        def pre_pv(g, pr, vbds):
            o = apply_v(pr, [x[:MEM + PRE] for vb in vbds for x in vb])
            if not last:
                odef_s[u, g] = o
            return o

        def wout(p, o, acc):
            contrib = _dot(o.astype(BF16), _unpack(wo_s[p * hw:(p + 1) * hw, :D]))
            return contrib if acc is None else acc + contrib

        def deferred(p):
            r = slice((p % GP) * PRE, (p % GP + 1) * PRE)
            return cat([odef_s[v, p // GP, r, :] for v in range(SPT - 1)]
                       + [val["PPV", p // GP][r]])

        def wout_strassen(kind, q):
            a11, a21 = val["PV", 2 * q], deferred(2 * q)
            if kind != "XA":
                a12, a22 = val["PV", 2 * q + 1], deferred(2 * q + 1)
            blk = lambda k, n: _unpack(
                wo_s[q * qr + k * hw:q * qr + (k + 1) * hw, n * KH:(n + 1) * KH])
            sm = lambda n: _unpack(wx_s[q, n])
            if kind == "XA":
                terms = {3: (a11, sm(1)), 6: (a21 - a11, sm(3))}
            elif kind == "XB":
                terms = {1: (a11 + a22, sm(0)), 4: (a22, sm(2)), 5: (a11 + a12, blk(1, 1)),
                         7: (a12 - a22, sm(4))}
            elif kind == "XC":
                terms = {2: (a21 + a22, blk(0, 0))}
            else:
                lhs = jnp.concatenate([cat([a11, a21]), cat([a12, a22])], axis=1)
                terms = {0: (lhs, _unpack(wo_s[q * qr:(q + 1) * qr, 2 * KH:D]))}
            for n, (x, w) in terms.items():
                r = _dot(x.astype(BF16), w)
                val["acc", n] = val["acc", n] + r if ("acc", n) in val else r

        arow0 = pl.multiple_of((s - u % 2) * SEG, 2 * SEG)

        def a_put(m, j, r):
            if m == 0:
                qa_s[j] = _round(r)
            else:
                kv_s[m - 1, j, A_HALO:A_HALO + 2 * SEG, :] = _round(r) if m == 1 else r

        def a_proj(idx):
            m, j = divmod(idx, NT)
            if "xa" not in val:
                val["xa"] = xa_s[pl.ds(arow0, 2 * SEG), :D]
            if m < 2 or j == NT - 1:
                a_put(m, j, _dot(val["xa"], _unpack(wa_s[m, :, j * 128:(j + 1) * 128])))
                return
            t = j // 2
            if "xs" not in val:
                xf = val["xa"].astype(F32)
                f = lambda i, k: xf[i * SEG:(i + 1) * SEG, k * KH:(k + 1) * KH]
                val["xs"] = [v.astype(BF16) for v in (
                    f(0, 0) + f(1, 1), f(1, 0) + f(1, 1), f(0, 0), f(1, 1), f(0, 0) + f(0, 1),
                    f(1, 0) - f(0, 0), f(0, 1) - f(1, 1))]
                val["xr"] = xf[:, 2 * KH:].astype(BF16)
            sm = lambda n: _unpack(cat([wc_s[2 * m + k, t, :, n * 128:(n + 1) * 128]
                                        for k in range(2)]))
            blk = lambda k, j: _unpack(wa_s[m, k * KH // 2:(k + 1) * KH // 2,
                                            (2 * t + j) * 128:(2 * t + j + 1) * 128])
            rhs = (sm(0), blk(0, 0), sm(1), sm(2), blk(1, 1), sm(3), sm(4))
            mm = lambda n: _dot(val["xs"][n], rhs[n])
            tail = [_dot(val["xr"], _unpack(wa_s[m, KH:, (2 * t + j) * 128:(2 * t + j + 1) * 128]))
                    for j in range(2)]
            m1, m2, m3, m4, m5 = [mm(n) for n in range(5)]
            a_put(m, 2 * t, tail[0] + cat([mm(6) + (m1 + m4 - m5), m2 + m4]))
            a_put(m, 2 * t + 1, tail[1] + cat([m3 + m5, mm(5) + (m1 - m2 + m3)]))

        def window(m, j, w, hf):
            lo = A_HALO + hf * SEG - A_DIL * w
            return kv_s[m, j, lo:lo + SEG, :]

        def local_softmax(hf):
            pos = arow0 + hf * SEG + lax.broadcasted_iota(jnp.int32, (SEG, 128), 0)
            rows = slice(hf * SEG, (hf + 1) * SEG)
            logits = []
            for w in range(A_W):
                t = qa_s[0, rows, :] * window(0, 0, w, hf)
                for j in range(1, NT):
                    t = t + qa_s[j, rows, :] * window(0, j, w, hf)
                t = t + pltpu.roll(t, 64, 1)
                t = t + pltpu.roll(t, 32, 1)
                t = _round(_round(t) * a_scale)
                if w > 0 and hf == 0:
                    t = jnp.where(pos >= A_DIL * w, t, -1000000000.0)
                logits.append(t)
            mx = functools.reduce(jnp.maximum, logits)
            es = [jnp.exp(l - mx) for l in logits]
            inv = _recip(functools.reduce(lambda x, y: x + y, es))
            return es, inv

        def local_pv(j, hf):
            es, inv = val["LA", hf]
            o = es[0] * window(1, j, 0, hf)
            for w in range(1, A_W):
                o = o + es[w] * window(1, j, w, hf)
            return o * inv

        def local_out(j, acc):
            wj = _unpack(awo_s[j * 64:(j + 1) * 64, :])
            r = _dot(cat([local_pv(j, 0), local_pv(j, 1)]).astype(BF16), wj)
            for m in range(2):
                kv_s[m, j, :A_HALO, :] = kv_s[m, j, 2 * SEG:2 * SEG + A_HALO, :]
            return r if acc is None else acc + r

        val = {}
        acc = None
        oa = None
        for kind, t in _order(u):
            if kind == "K":
                val[kind, t] = block_diag(t, 1)
            elif kind == "V":
                val[kind, t] = block_diag(t, 2)
            elif kind == "Q":
                val[kind, t] = proj(t, 0)
            elif kind == "T":
                val[kind, t] = keys_t(val["K", t])
            elif kind == "S":
                val[kind, t] = qk(val["Q", t], val["T", t], a80)
            elif kind == "M":
                val[kind, t] = row_max(val["S", t], allowed, fill, is_a)
            elif kind == "E":
                val[kind, t] = probs(val["M", t], is_a, t >= LATE_FROM)
            elif kind == "PV":
                val[kind, t] = pv(val["E", t], val["V", t])
            elif kind == "TG":
                val[kind, t] = keys_t([x[:MEM + PRE] for r in range(GP)
                                       for x in val["K", GP * t + r]])
            elif kind == "PS":
                q = cat([pre(GP * t + r, 0) for r in range(GP)])
                val[kind, t] = qk(q, val["TG", t], p_first)
            elif kind == "MG":
                val[kind, t] = row_max(val["PS", t], p_allowed, p_fill, p_first)
            elif kind == "EG":
                val[kind, t] = probs(val["MG", t], p_first, False)[0]
            elif kind == "PPV":
                val[kind, t] = pre_pv(t, val["EG", t], [val["V", GP * t + r] for r in range(GP)])
            elif kind == "W":
                acc = wout(t, val["PV", t], acc)
            elif kind in ("XA", "XB", "XC", "Y"):
                wout_strassen(kind, t)
            elif kind == "LA":
                val[kind, t] = local_softmax(t)
            elif kind == "AP":
                a_proj(t)
            elif kind == "AO":
                oa = local_out(t, oa)
                if t == NT - 1:
                    out_s[pl.ds(arow0, 2 * SEG), :D] = oa.astype(BF16)
                    out_copy(arow0, 2 * SEG, 0).start()
        if last:
            m = lambda n: val["acc", n]
            acc = jnp.concatenate([
                cat([m(1) + m(4) - m(5) + m(7), m(2) + m(4)]),
                cat([m(3) + m(5), m(1) - m(2) + m(3) + m(6)]), m(0)], axis=1)
        return acc

    def steps(i, mem):
        @pl.when(i == 1)
        def _():
            for cp in x_rest:
                cp.wait()

        accs = []
        for u in range(SPT):
            accs.append(segment(i * SPT + u, mem, u))
            mem = accs[-1][FRESH:SEG]
        res = cat([x for u in range(SPT) for x in (
            accs[-1][SEG + u * PRE:SEG + (u + 1) * PRE], accs[u][:FRESH])])
        row = pl.multiple_of(i * SPT * SEG, SPT * SEG)
        out_s[pl.ds(row, SPT * SEG), D:2 * D] = res.astype(BF16)
        out_copy(row, SPT * SEG, 1).start()
        return mem

    lax.fori_loop(0, N_STEPS, steps, mem0_s[...].astype(F32))

    wo_copy(NTRIP - 1).wait()
    wo_copy(NTRIP).wait()
    wait_trip(NTRIP)
    wait_trip(NTRIP + 1)

    done = N_STEPS * SPT * SEG
    pltpu.make_async_copy(out_s.at[:done, :], out_hbm.at[:done, :], sems.at[7]).wait()


@jax.jit
def pallas_concat_heads__sliding_local_dilated__memory_aug_recurrent_mem_tr__prompt_kernel(
    A_x: jax.Array,
    A_wqkv: jax.Array,
    A_wo: jax.Array,
    B_x: jax.Array,
    B_mem0: jax.Array,
    B_Wq: jax.Array,
    B_Wk: jax.Array,
    B_Wv: jax.Array,
    B_Wo: jax.Array,
    B_seg_len,
):
    del B_seg_len
    assert A_x.shape == (1, S, D) and B_x.shape == (1, S, D)
    hd = B_H * B_DH
    wq_t = jnp.transpose(B_Wq, (1, 2, 0)).reshape(hd, D)
    wk_t = jnp.transpose(B_Wk, (1, 2, 0)).reshape(hd, D)
    wv_t = jnp.transpose(B_Wv, (1, 2, 0)).reshape(hd, D)
    wo = B_Wo.reshape(hd, D)

    any_spec = pl.BlockSpec(memory_space=pl.ANY)
    out = pl.pallas_call(
        _kernel,
        out_shape=jax.ShapeDtypeStruct((S, 2 * D), BF16),
        in_specs=[any_spec] * 10,
        out_specs=any_spec,
        scratch_shapes=[
            pltpu.VMEM((2, PP, 4, PW, D), BF16),
            pltpu.VMEM((NT, D, 128), BF16),
            pltpu.VMEM((4, 2 * WO_ROWS, WO_W), BF16),
            pltpu.VMEM((NP, D // 2, 3 * PW), U32),
            pltpu.VMEM((hd // 2 + PW, WO_W), U32),
            pltpu.VMEM((NQ + 1, 5, PW // 2, KH), U32),
            pltpu.VMEM((NSEG, NP // PP, PRE, PRE_W), F32),
            pltpu.VMEM((SPT - 1, NG, GP * PRE, PW), F32),
            pltpu.VMEM((S, 2 * D), BF16),
            pltpu.VMEM((S, X_W), BF16),
            pltpu.VMEM((S, X_W), BF16),
            pltpu.VMEM((NSEG, PRE, D), BF16),
            pltpu.VMEM((NSEG * PRE // 2, D), U32),
            pltpu.VMEM((5, NSEG * PRE // 4, 256), U32),
            pltpu.VMEM((MEM, D), BF16),
            pltpu.VMEM((3, D // 2, D), U32),
            pltpu.VMEM((NTRIP, 2, 64, D), U32),
            pltpu.VMEM((D // 2, D), U32),
            pltpu.VMEM((NT, D // 2, 128), U32),
            pltpu.VMEM((NT, 2 * SEG, 128), F32),
            pltpu.VMEM((2, NT, A_HALO + 2 * SEG, 128), F32),
            pltpu.SemaphoreType.DMA((10,)),
        ],
        compiler_params=pltpu.CompilerParams(vmem_limit_bytes=120 * 1024 * 1024,
                                             disable_bounds_checks=True),
    )(A_x.reshape(S, D), A_wqkv, A_wo, B_x.reshape(S, D), B_x.reshape(NSEG, SEG // PRE, PRE, D),
      B_mem0.reshape(MEM, D), wq_t, wk_t, wv_t, wo)
    return out.reshape(1, S, 2 * D)
```

```python
import functools

import jax
import jax.numpy as jnp
from jax import lax
import jax.experimental.pallas as pl
import jax.experimental.pallas.tpu as pltpu

F32 = jnp.float32
BF16 = jnp.bfloat16
U32 = jnp.uint32

S = 2048
D = 640
NT = D // 128
A_H = 32
A_DH = D // A_H
A_W = 8
A_DIL = 2
A_HALO = 16
B_H = 32
B_DH = 192
MEM = 8
SEG = 32
NSEG = S // SEG
NP = B_H // 2
PW = 2 * B_DH
PRE = 8
FRESH = SEG - PRE
L = MEM + SEG
GP = 4
NG = NP // GP
LOG2E = 1.4426950408889634
NEG = -1000000000.0 * LOG2E
PP = 2
NTRIP = NP // PP - 1
PEEL = (2, 2, 5)
KH = 256
WO_ROWS = 512
WX_DONE = (0, 192, 448, 768, 960, 1216, 1536)
WX_ROWS = 16
WX_SKIP, WX_TAIL = 2, 2
ST_ROWS = 256
X_HEAD = 128
X_W = 768
WO_W = 768
SPT = 4
N_STEPS = NSEG // SPT
NQ = NP // 2

LAT_MM, LAT_X, LAT_T, LAT_N, LAT_N_LATE = 190, 190, 380, 230, 100
LATE_FROM = NP - 2
AP_AFTER = (6, 12, 18, 24, 30)
AO_AFTER = (30, 40)
TAIL_FILL = (2, 2, 2, 0)
HOLD_W = (0, 3, 0, 0)


def _segment_order(u):
    odd, last = u % 2 == 1, u == SPT - 1
    proj = []
    for g in range(NG):
        proj += [("K", GP * g + r) for r in range(GP)]
        for r in range(GP):
            proj += [("V", GP * g + r), ("Q", GP * g + r)]
    dur = {"K": 120, "V": 120, "Q": 120, "S": 24, "PV": 24, "PS": 24, "PPV": 24,
           "W": 120, "XA": 96, "XB": 192, "XC": 48, "Y": 96, "AO": 80, "AP": 90,
           "T": 0, "M": 0, "E": 0, "TG": 0, "MG": 0, "EG": 0}
    end = {}

    def ready(task):
        k, i = task
        if k == "T":
            deps = [(("K", i), LAT_MM)]
        elif k == "S":
            deps = [(("Q", i), LAT_MM), (("T", i), LAT_T)]
        elif k == "M":
            deps = [(("S", i), LAT_MM - 40)]
        elif k == "E":
            deps = [(("M", i), LAT_X)]
        elif k == "PV":
            deps = [(("E", i), LAT_N_LATE if i >= LATE_FROM else LAT_N), (("V", i), LAT_MM)]
        elif k == "TG":
            deps = [(("K", GP * i + r), LAT_MM) for r in range(GP)]
        elif k == "PS":
            deps = [(("TG", i), LAT_T)]
        elif k == "MG":
            deps = [(("PS", i), LAT_MM - 40)]
        elif k == "EG":
            deps = [(("MG", i), LAT_X)]
        elif k == "PPV":
            deps = [(("EG", i), LAT_N), (("V", GP * i + GP - 1), LAT_MM)]
        elif k == "W":
            deps = [(("PV", i), LAT_MM)]
        else:
            deps = [(("PV", 2 * i), LAT_MM), (("PPV", 2 * i // GP), LAT_MM)]
            if k != "XA":
                deps.append((("PV", 2 * i + 1), LAT_MM))
        if any(d not in end for d, _ in deps):
            return None
        return max(end[d] + lat for d, lat in deps)

    pend = ([(k, p) for k in ("E", "M", "T") for p in range(NP)]
            + [(k, g) for k in ("EG", "MG", "TG") for g in range(NG)]
            + ([(k, q) for q in range(NQ) for k in ("XA", "XB", "Y", "XC")] if last
               else [("W", p) for p in range(NP)])
            + [("PPV", g) for g in range(NG)]
            + [("PV", p) for p in range(NP)] + [("PS", g) for g in range(NG)]
            + [("S", p) for p in range(NP)])
    fill = [("AO", j) for j in range(NT)] if odd else [("AP", j) for j in (5, 6, 7, 8, 9, 0, 1, 2, 3, 4, 10, 12, 14)]
    order = []
    now = [0]

    def emit(task):
        order.append(task)
        now[0] += dur[task[0]]
        end[task] = now[0]

    nproj = 0
    while pend:
        cand = [x for x in pend if ready(x) is not None and ready(x) <= now[0]]
        if proj:
            cand = [x for x in cand if not (x[0] == "W" and x[1] >= NP - GP - HOLD_W[u])]
        if cand:
            if not proj:
                cand = [x for x in cand if x[0] not in ("W", "XA", "XB", "XC", "Y")] or cand
            pend.remove(cand[0])
            emit(cand[0])
        elif proj:
            emit(proj.pop(0))
            nproj += 1
            if odd and nproj == GP:
                order += [("LA", 0), ("LA", 1)]
            if nproj in (AO_AFTER if odd else AP_AFTER):
                emit(fill.pop(0))
        elif len(fill) > TAIL_FILL[u]:
            emit(fill.pop(0))
        else:
            now[0] = min(ready(x) for x in pend if ready(x) is not None)
    return order + fill


ORDERS = (
    "K0 T0 K1 K3 K2 V0 T1 T2 Q1 T3 Q0 AP5 Q2 AP6 S0 TG0 M0 PS0 V1 V2 V3 E0 MG0 S1 S2 M1 Q3 EG0 "
    "PV0 K4 K5 E1 M2 S3 K6 T4 W0 E2 M3 T5 PPV0 PV1 K7 AP7 AP8 E3 T6 W1 T7 TG1 PV2 PV3 Q4 W2 V4 W3 "
    "PS1 Q5 S4 V5 M4 MG1 V6 Q7 Q6 E4 S5 EG1 V7 M5 PV4 S6 K8 PPV1 E5 S7 M6 W4 K9 E6 M7 T8 K10 PV5 "
    "AP9 T9 K11 E7 W5 T10 TG2 PV6 V8 T11 PV7 Q8 W7 S8 W6 PS2 V10 V9 Q9 M8 MG2 Q10 E8 EG2 V11 S9 "
    "Q11 M9 PV8 S10 K12 T12 PPV2 E9 S11 M10 W8 E10 M11 PV9 K14 K13 K15 E11 T13 W9 PV10 V12 T14 "
    "T15 TG3 PV11 Q12 W10 W11 PS3 S12 Q13 V13 M12 MG3 V15 V14 E12 Q14 EG3 Q15 S13 M13 PV12 S14 "
    "AP0 AP1 PPV3 E13 W12 S15 M14 AP2 AP3 E14 PV13 M15 AP4 AP10 PV14 W13 E15 PV15 W14 W15 AP14 "
    "AP12 ",
    "K0 K2 K1 T0 K3 LA0 LA1 Q0 V1 T1 V0 T2 T3 TG0 Q1 S0 V2 PS0 Q2 M0 S1 V3 MG0 Q3 M1 S2 K4 EG0 K5 "
    "E0 E1 M2 PV0 S3 K6 T4 K7 PPV0 E2 T5 M3 W0 T6 PV1 PV2 V4 E3 T7 TG1 Q4 W1 W2 PV3 PS1 S4 V5 Q5 "
    "M4 MG1 W3 AO0 S5 V6 E4 EG1 Q6 M5 V7 PV4 Q7 E5 S6 K8 W4 M6 PPV1 PV5 S7 K9 T8 E6 W5 K10 M7 PV6 "
    "T9 K11 E7 T10 V8 W6 T11 TG2 PV7 Q8 AO1 W7 S8 V9 PS2 Q9 M8 V10 MG2 Q10 E8 S9 V11 EG2 Q11 PV8 "
    "M9 S10 K12 PPV2 E9 S11 M10 K13 W8 E10 M11 T12 PV9 K14 K15 E11 T13 T14 PV10 AO2 V12 T15 TG3 "
    "Q12 PV11 V13 Q13 PS3 S12 V14 Q14 M12 S13 MG3 V15 Q15 E12 M13 EG3 S14 W9 E13 M14 PPV3 W10 "
    "PV12 S15 W11 E14 M15 PV13 W12 PV14 E15 W13 PV15 W14 W15 AO3 AO4 ",
    "K0 K1 T0 K3 T1 AP5 K2 AP6 V0 Q0 TG0 T3 T2 V1 S0 Q1 PS0 Q2 V2 M0 S1 V3 E0 MG0 Q3 M1 K4 S2 EG0 "
    "PV0 K5 E1 M2 PPV0 S3 K6 T4 W0 E2 M3 T5 AP7 AP8 PV1 K7 E3 W1 T6 T7 TG1 PV2 V4 PV3 Q4 W2 W3 "
    "PS1 S4 V5 M4 Q5 MG1 V6 S5 Q6 EG1 E4 V7 Q7 M5 PV4 S6 K8 PPV1 E5 S7 M6 W4 AP9 K9 E6 M7 T8 PV5 "
    "K10 T9 K11 E7 W5 T10 PV6 V8 T11 TG2 Q8 PV7 W6 W7 S8 PS2 Q9 M8 MG2 V10 V9 Q10 E8 EG2 S9 V11 "
    "Q11 M9 PV8 S10 K12 PPV2 E9 W8 S11 M10 K13 E10 M11 T12 PV9 K14 K15 E11 T13 W9 PV11 T14 PV10 "
    "V12 T15 TG3 Q12 W10 V13 W11 PS3 S12 Q13 MG3 M12 V14 Q14 E12 EG3 S13 V15 Q15 M13 PV12 S14 E13 "
    "AP0 AP1 PPV3 S15 M14 W12 AP2 AP3 M15 AP4 E14 PV14 PV13 AP10 E15 W13 PV15 W14 W15 AP12 AP14 ",
    "K1 K0 K2 T0 K3 LA0 LA1 T1 V0 T2 Q0 T3 TG0 V1 Q1 S0 PS0 M0 V2 Q2 V3 MG0 Q3 S1 E0 M1 S2 EG0 K4 "
    "K5 M2 T4 PV0 E1 AO0 PPV0 S3 K6 E2 T5 K7 M3 XA0 T6 PV1 PV2 Y0 V4 E3 T7 TG1 Q4 XB0 XC0 XA1 PV3 "
    "PS1 S4 V5 Q5 M4 MG1 XB1 E4 Y1 XC1 EG1 S5 Q6 V6 M5 V7 S6 PV4 AO1 Q7 E5 PPV1 K8 S7 M6 XA2 K9 "
    "M7 T8 PV5 K10 E6 T9 XB2 E7 T10 Y2 K11 TG2 T11 XC2 PV6 PV7 V8 Y3 Q8 XA3 XB3 PS2 S8 V9 Q9 M8 "
    "MG2 V10 Q10 AO2 E8 EG2 S9 V11 S10 M9 PV8 K12 Q11 M10 PPV2 K13 E9 K14 S11 E10 T12 M11 T13 K15 "
    "PV10 PV9 XA4 T14 V12 E11 XB4 T15 TG3 XA5 Y4 Q12 AO3 PV11 XB5 PS3 S12 V13 Q13 MG3 V14 M12 Q14 "
    "EG3 S13 V15 E12 M13 PV12 Q15 S14 AO4 PPV3 E13 S15 M14 E14 XA6 M15 XC3 XC4 XC5 PV13 E15 Y5 "
    "PV14 XB6 PV15 Y6 XA7 XB7 XC6 Y7 XC7 ",
)
SKIP_PROLOGUE = False


def _order(u):
    if ORDERS is None or ORDERS[u] is None:
        return _segment_order(u)
    return [(t.rstrip("0123456789"), int(t.lstrip("ABCDEFGHIJKLMNOPQRSTUVWXYZ")))
            for t in ORDERS[u].split()]


def _nt_dot(a, b):
    return lax.dot_general(a, b, (((1,), (1,)), ((), ())), preferred_element_type=F32)


def _dot(a, b):
    return jnp.dot(a, b, preferred_element_type=F32)


def _pack(x):
    return pltpu.bitcast(x, U32)


def _unpack(x):
    return pltpu.bitcast(x, BF16)


def cat(parts):
    return jnp.concatenate(parts, axis=0)


def _round(x):
    return x.astype(BF16).astype(F32)


def _recip(x):
    r = pl.reciprocal(x, approx=True)
    return r * (2.0 - x * r)


def _kernel(ax_hbm, awqkv_hbm, awo_hbm, bx_hbm, bx4_hbm, mem0_hbm, wq_hbm, wk_hbm, wv_hbm, wo_hbm,
            out_hbm,
            stage, awo_raw, wo_raw, w_s, wo_s, wx_s, pre_s, odef_s, out_s,
            xa_s, xb_s, xpre_s, xp_s, xs_s, mem0_s, wa_s, wc_s, awo_s, t1_s, qa_s, kv_s,
            sems):
    b_scale = 0.072265625 * LOG2E
    a_scale = 0.2236328125

    w_hbm = (wq_hbm, wk_hbm, wv_hbm)
    hw = PW // 2
    hd = B_H * B_DH

    def w_copy(p, half, q, m, sem):
        rows = pl.ds(pl.multiple_of(p * PW, PW), PW)
        return pltpu.make_async_copy(w_hbm[m].at[rows, :], stage.at[half, q, m], sem)

    def wa_piece(g, q):
        last = g >= 2 * 3
        return jnp.where(last, 1 + q, g >> 1), jnp.where(last, NT - 1, (g & 1) + 2 * q)

    def wa_copy(c, kt, half, q, sem):
        return pltpu.make_async_copy(
            awqkv_hbm.at[pl.ds(pl.multiple_of(kt * 128, 128), 128),
                         pl.ds(pl.multiple_of(c * D, 128), D)],
            stage.at[half, q, 3, :128], sem)

    def trip_copies(g):
        half = g & 1
        src = jnp.minimum(g, NTRIP - 1)
        cps = []
        for q in range(PP):
            cps += [w_copy((src + 1) * PP + q, half, q, m, sems.at[half]) for m in range(3)]
            cps.append(wa_copy(*wa_piece(src, q), half, q, sems.at[half]))
        return cps

    def start_trip(g):
        for cp in trip_copies(g):
            cp.start(priority=1)

    def wait_trip(g):
        for cp in trip_copies(g):
            cp.wait()

    qr = 2 * hw

    def wo_copy(c):
        src = jnp.minimum(c, hd // (2 * WO_ROWS) - 1)
        rows = pl.ds(pl.multiple_of(src * 2 * WO_ROWS, 2 * WO_ROWS), 2 * WO_ROWS)
        return pltpu.make_async_copy(wo_hbm.at[rows, :], wo_raw.at[lax.rem(c, 3), :, :D],
                                     sems.at[8 + (c & 1)])

    def wo_piece(q, piece, spare, anchor, never):
        half = []
        for k in range(2):
            r = q * qr + k * hw + piece * WX_ROWS
            c = r // WO_ROWS
            slot = jnp.where(spare, 3, lax.rem(c, 3))
            off = jnp.where(spare, 0, 2 * (r - c * WO_ROWS))
            rows = pl.ds(pl.multiple_of(off, 16), 2 * WX_ROWS)
            w = jnp.where(never, anchor, _pack(wo_raw[slot, rows, :D]))
            wo_s[pl.ds(pl.multiple_of(r, 8), WX_ROWS), :D] = w
            half.append(_unpack(w[:, :2 * KH]).astype(F32))
        b11, b12, b21, b22 = [half[k][:, n * KH:(n + 1) * KH] for k in range(2) for n in range(2)]
        for n, v in enumerate((b11 + b22, b12 - b22, b21 - b11, b11 + b12, b21 + b22)):
            wx_s[q, n, pl.ds(pl.multiple_of(piece * WX_ROWS, 8), WX_ROWS), :] = (
                _pack(v.astype(BF16)))

    def x_copies(xr, sem):
        return [pltpu.make_async_copy(ax_hbm.at[xr, :], xa_s.at[xr, :D], sem),
                pltpu.make_async_copy(bx_hbm.at[xr, :], xb_s.at[xr, :D], sem)]

    xpre_cp = pltpu.make_async_copy(bx4_hbm.at[:, 0], xpre_s, sems.at[3])
    late_cps = ([pltpu.make_async_copy(mem0_hbm, mem0_s, sems.at[2])]
                + x_copies(pl.ds(0, X_HEAD), sems.at[2]))
    awo_cps = [
        pltpu.make_async_copy(awo_hbm.at[:, c * 128:(c + 1) * 128], awo_raw.at[c], sems.at[2])
        for c in range(NT)]
    x_rest = x_copies(pl.ds(X_HEAD, S - X_HEAD), sems.at[3])
    tiles = [(m, j) for m in range(3) for j in range(PW // 128)]
    peel = [tiles[sum(PEEL[:n]):sum(PEEL[:n + 1])] for n in range(len(PEEL))]
    peel_cps = [[pltpu.make_async_copy(w_hbm[m].at[pl.ds(q * PW + j * 128, 128), :],
                                       stage.at[1, q, m, pl.ds(j * 128, 128), :], sems.at[4 + n])
                 for m, j in blk for q in range(PP)] for n, blk in enumerate(peel)]
    peel_cps[-1].append(wa_copy(0, NT - 1, 1, 0, sems.at[3 + len(PEEL)]))

    xpre_cp.start()
    for cps in peel_cps:
        for cp in cps:
            cp.start(priority=1)
    start_trip(0)
    for cp in late_cps:
        cp.start(priority=1)
    kv_s[:, :, :A_HALO, :] = jnp.zeros((2, NT, A_HALO, 128), F32)
    wo_raw[3, :2 * WX_ROWS, :D] = jnp.zeros((2 * WX_ROWS, D), BF16)

    def gather_heads(ref):
        rows = []
        for j in range(A_DH // 2):
            u = ref[pl.ds(j, A_H, stride=A_DH // 2), :]
            rows.append(pltpu.bitcast(u << 16, F32))
            rows.append(pltpu.bitcast(u & jnp.uint32(0xFFFF0000), F32))
        return jnp.concatenate(rows, axis=0)

    HR = NSEG * PRE // 2

    def xq(i, k):
        return _unpack(xp_s[i * HR // 2:(i + 1) * HR // 2, k * KH:(k + 1) * KH])

    def strassen_lhs():
        f = lambda i, k: xq(i, k).astype(F32)
        sums = (f(0, 0) + f(1, 1), f(1, 0) + f(1, 1), f(0, 0) + f(0, 1),
                f(1, 0) - f(0, 0), f(0, 1) - f(1, 1))
        for n, v in enumerate(sums):
            xs_s[n] = _pack(v.astype(BF16))

    def pair_prep2(pp, half, m, js=(0, 1, 2), hook=None):
        if SKIP_PROLOGUE:
            return
        p = pp * PP
        for q in range(2):
            lo, hi = js[0] * 128, (js[-1] + 1) * 128
            w_s[p + q, :, m * PW + lo:m * PW + hi] = _pack(stage[half, q, m, lo:hi, :].T)
        nseg = ST_ROWS // PRE
        for j in js:
            rows = slice(j * 128, (j + 1) * 128)
            b = lambda k, q: stage[half, q, m, rows, k * KH:(k + 1) * KH]
            bf = lambda k, q: b(k, q).astype(F32)
            rhs = ((bf(0, 0) + bf(1, 1)).astype(BF16), b(0, 0),
                   (bf(0, 1) - bf(1, 1)).astype(BF16), (bf(1, 0) - bf(0, 0)).astype(BF16),
                   b(1, 1), (bf(0, 0) + bf(0, 1)).astype(BF16),
                   (bf(1, 0) + bf(1, 1)).astype(BF16))
            tail = [stage[half, q, m, rows, 2 * KH:] for q in range(2)]
            for c in range(HR // ST_ROWS):
                r = slice(c * ST_ROWS // 2, (c + 1) * ST_ROWS // 2)
                sm = lambda n: _unpack(xs_s[n, r, :])
                qd = lambda i, k: _unpack(
                    xp_s[(i * HR + c * ST_ROWS) // 2:(i * HR + (c + 1) * ST_ROWS) // 2,
                         k * KH:(k + 1) * KH])
                rest = lambda i: _unpack(
                    xp_s[(i * HR + c * ST_ROWS) // 2:(i * HR + (c + 1) * ST_ROWS) // 2, 2 * KH:])

                def put(i, q, v):
                    s0 = i * (NSEG // 2) + c * nseg
                    col = (3 * q + m) * PW + j * 128
                    pre_s[s0:s0 + nseg, pp, :, col:col + 128] = v.reshape(nseg, PRE, 128)
                    if hook is not None:
                        hook(v)

                m5 = _nt_dot(sm(2), rhs[4])
                m3 = _nt_dot(qd(0, 0), rhs[2])
                put(0, 1, _nt_dot(rest(0), tail[1]) + m3 + m5)
                m1 = _nt_dot(sm(0), rhs[0])
                m4 = _nt_dot(qd(1, 1), rhs[3])
                put(0, 0, _nt_dot(rest(0), tail[0]) + _nt_dot(sm(4), rhs[6]) + (m1 + m4 - m5))
                m2 = _nt_dot(sm(1), rhs[1])
                put(1, 0, _nt_dot(rest(1), tail[0]) + m2 + m4)
                put(1, 1, _nt_dot(rest(1), tail[1]) + _nt_dot(sm(3), rhs[5]) + (m1 - m2 + m3))

    def wa_prep(c, kt, half, q):
        t1_s[q] = _pack(stage[half, q, 3, :128].T)
        g = gather_heads(t1_s.at[q])
        wa_s[c, pl.ds(pl.multiple_of(kt * 64, 64), 64), :] = _pack(g.astype(BF16).T)
        return g

    def wa_trip(g, half):
        lo, hi = [wa_prep(*wa_piece(g, q), half, q) for q in range(2)]
        slot = jnp.where((g >> 1) == 2, g & 1, 2)
        for t in range(2):
            b11, b12 = lo[2 * t * 128:(2 * t + 1) * 128], lo[(2 * t + 1) * 128:(2 * t + 2) * 128]
            b21, b22 = hi[2 * t * 128:(2 * t + 1) * 128], hi[(2 * t + 1) * 128:(2 * t + 2) * 128]
            sums = cat([b11 + b22, b12 - b22, b21 - b11, b11 + b12, b21 + b22])
            wc_s[slot, t] = _pack(sums.astype(BF16).T)

    xpre_cp.wait()
    xp_s[...] = _pack(xpre_s[...].reshape(NSEG * PRE, D))
    strassen_lhs()
    for blk, cps in zip(peel, peel_cps):
        for cp in cps:
            cp.wait()
        for m in range(3):
            js = tuple(j for mm, j in blk if mm == m)
            if js:
                pair_prep2(0, 1, m, js)
    wa_prep(0, NT - 1, 1, 0)
    wo_copy(0).start(priority=1)
    start_trip(1)

    def prologue(g, carry):
        half = g & 1

        @pl.when(g > 0)
        def _():
            wo_copy(g - 1).wait()

        @pl.when(g == NTRIP - 1)
        def _():
            for cp in awo_cps:
                cp.start()

        wait_trip(g)
        calls = [0]
        per = hw // WX_ROWS
        done = [x // WX_ROWS for x in WX_DONE]
        total = max(b - a for a, b in zip(done, done[1:]))
        todo = list(range(total))
        first, stop = NQ * per, (NQ + 1) * per
        for trip in range(1, NTRIP):
            first = jnp.where(g == trip, done[trip - 1], first)
            stop = jnp.where(g == trip, done[trip], stop)

        def hook(v):
            calls[0] += 1
            want = (calls[0] - WX_SKIP) * total // (36 - WX_SKIP - WX_TAIL)
            t = 0
            while todo and todo[0] < want:
                k = jnp.minimum(first + todo.pop(0), stop - 1)
                q = k // per
                anchor = jnp.concatenate(
                    [v[(NT * t + c) * WX_ROWS:(NT * t + c + 1) * WX_ROWS] for c in range(NT)],
                    axis=1)
                wo_piece(q, k % per, g == 0, pltpu.bitcast(anchor, U32), g > NSEG)
                t += 1

        for m in range(3):
            pair_prep2(g + 1, half, m, hook=hook)
            if m == 0:
                wa_trip(g, half)
        wo_copy(g + 1).start(priority=1)
        start_trip(g + 2)
        return carry

    lax.fori_loop(0, NTRIP, prologue, 0)

    for cp in late_cps + awo_cps:
        cp.wait()
    for cp in x_rest:
        cp.start()

    for c in range(NT):
        t1_s[c] = _pack(awo_raw[c])
        awo_s[:, c * 128:(c + 1) * 128] = _pack(gather_heads(t1_s.at[c]).astype(BF16))

    def out_copy(row, n, half):
        r = pl.ds(row, n)
        c = slice(half * D, (half + 1) * D)
        return pltpu.make_async_copy(out_s.at[r, c], out_hbm.at[r, c], sems.at[7])

    def segment(s, mem, u):
        last = u == SPT - 1
        row0 = pl.multiple_of(s * SEG, SEG)
        ninf = jnp.float32(-jnp.inf)

        qi = lax.broadcasted_iota(jnp.int32, (SEG, 128), 0)
        kl = lax.broadcasted_iota(jnp.int32, (SEG, 128), 1)
        is_a = kl < L
        a80 = lax.broadcasted_iota(jnp.int32, (SEG, 2 * L), 1) < L
        real = kl < 2 * L
        kpos = jnp.where(is_a, kl, kl - L)
        allowed = ((qi >= FRESH) | (qi + MEM + PRE >= kpos)) & real
        fill = jnp.where(real, NEG, ninf)
        pi = lax.broadcasted_iota(jnp.int32, (GP * PRE, 128), 0)
        pk = lax.broadcasted_iota(jnp.int32, (GP * PRE, 128), 1)
        p_own = (pk // SEG) == (pi // PRE)
        p_allowed = (pk % (MEM + PRE)) <= (pi % PRE) + MEM
        p_first = (pk % SEG) < MEM + PRE
        p_allowed = p_allowed & p_own
        p_fill = jnp.where(p_own, NEG, ninf)
        col_a = lax.broadcasted_iota(jnp.int32, (1, PW), 1) < B_DH
        col128_a = lax.broadcasted_iota(jnp.int32, (1, 128), 1) < (B_DH - 128)

        xb = xb_s[pl.ds(row0, SEG), :D].astype(F32)
        h = jnp.concatenate([xb[PRE:], mem], axis=0).astype(BF16)

        def proj(p, m):
            return _dot(h, _unpack(w_s[p, :, m * PW:(m + 1) * PW]))

        def pre(p, m):
            col = (3 * (p % PP) + m) * PW
            return pre_s[s, p // PP, :, col:col + PW]

        def block_diag(p, m):
            f = proj(p, m)
            full = jnp.concatenate([f[FRESH:], pre(p, m), f[:FRESH]], axis=0)
            z = jnp.zeros_like(full)
            return jnp.where(col_a, full, z), jnp.where(col_a, z, full)

        def keys_t(blocks):
            fold = cat([jnp.concatenate([x[:, :128] if i % 2 == 0 else x[:, 256:], x[:, 128:256]],
                                        axis=1) for i, x in enumerate(blocks)])
            t = fold.T
            return t[:128].astype(BF16), t[128:].astype(BF16)

        def qk(q, kt, lane_a):
            outer = _dot(cat([q[:, :128], q[:, 256:]]).astype(BF16), kt[0])
            sc = (jnp.where(lane_a, outer[:SEG], outer[SEG:])
                  + _dot(q[:, 128:256].astype(BF16), kt[1]))
            if sc.shape[1] < 128:
                sc = jnp.concatenate([sc, jnp.zeros((SEG, 128 - sc.shape[1]), F32)], axis=1)
            return sc

        def row_max(raw, ok, other, first):
            sc = jnp.where(ok, raw * b_scale, other)
            ma = jnp.max(jnp.where(first, sc, ninf), axis=1, keepdims=True)
            mb = jnp.max(jnp.where(first, ninf, sc), axis=1, keepdims=True)
            return sc, ma, mb

        def probs(mx, first, late_norm):
            sc, ma, mb = mx
            e = jnp.exp2(sc - jnp.where(first, ma, mb))
            ea, eb = jnp.where(first, e, 0.0), jnp.where(first, 0.0, e)
            sa = jnp.sum(ea, axis=1, keepdims=True)
            sb = jnp.sum(eb, axis=1, keepdims=True)
            if late_norm:
                return e.astype(BF16), _recip(sa), _recip(sb)
            return (e * _recip(jnp.where(first, sa, sb))).astype(BF16), None, None

        def apply_v(e, blocks):
            pad = 128 - sum(x.shape[0] for x in blocks)
            rows = list(blocks) + ([jnp.zeros((pad, PW), F32)] if pad else [])
            return _dot(e, cat(rows).astype(BF16))

        def pv(sm, vbd):
            e, ra, rb = sm
            o = apply_v(e, vbd)
            if ra is not None:
                o = jnp.concatenate([
                    o[:, :128] * ra,
                    o[:, 128:256] * jnp.where(col128_a, ra, rb),
                    o[:, 256:] * rb], axis=1)
            return o

        def pre_pv(g, pr, vbds):
            o = apply_v(pr, [x[:MEM + PRE] for vb in vbds for x in vb])
            if not last:
                odef_s[u, g] = o
            return o

        def wout(p, o, acc):
            contrib = _dot(o.astype(BF16), _unpack(wo_s[p * hw:(p + 1) * hw, :D]))
            return contrib if acc is None else acc + contrib

        def deferred(p):
            r = slice((p % GP) * PRE, (p % GP + 1) * PRE)
            return cat([odef_s[v, p // GP, r, :] for v in range(SPT - 1)]
                       + [val["PPV", p // GP][r]])

        def wout_strassen(kind, q):
            a11, a21 = val["PV", 2 * q], deferred(2 * q)
            if kind != "XA":
                a12, a22 = val["PV", 2 * q + 1], deferred(2 * q + 1)
            blk = lambda k, n: _unpack(
                wo_s[q * qr + k * hw:q * qr + (k + 1) * hw, n * KH:(n + 1) * KH])
            sm = lambda n: _unpack(wx_s[q, n])
            if kind == "XA":
                terms = {3: (a11, sm(1)), 6: (a21 - a11, sm(3))}
            elif kind == "XB":
                terms = {1: (a11 + a22, sm(0)), 4: (a22, sm(2)), 5: (a11 + a12, blk(1, 1)),
                         7: (a12 - a22, sm(4))}
            elif kind == "XC":
                terms = {2: (a21 + a22, blk(0, 0))}
            else:
                lhs = jnp.concatenate([cat([a11, a21]), cat([a12, a22])], axis=1)
                terms = {0: (lhs, _unpack(wo_s[q * qr:(q + 1) * qr, 2 * KH:D]))}
            for n, (x, w) in terms.items():
                r = _dot(x.astype(BF16), w)
                val["acc", n] = val["acc", n] + r if ("acc", n) in val else r

        arow0 = pl.multiple_of((s - u % 2) * SEG, 2 * SEG)

        def a_put(m, j, r):
            if m == 0:
                qa_s[j] = _round(r)
            else:
                kv_s[m - 1, j, A_HALO:A_HALO + 2 * SEG, :] = _round(r) if m == 1 else r

        def a_proj(idx):
            m, j = divmod(idx, NT)
            if "xa" not in val:
                val["xa"] = xa_s[pl.ds(arow0, 2 * SEG), :D]
            if m < 2 or j == NT - 1:
                a_put(m, j, _dot(val["xa"], _unpack(wa_s[m, :, j * 128:(j + 1) * 128])))
                return
            t = j // 2
            if "xs" not in val:
                xf = val["xa"].astype(F32)
                f = lambda i, k: xf[i * SEG:(i + 1) * SEG, k * KH:(k + 1) * KH]
                val["xs"] = [v.astype(BF16) for v in (
                    f(0, 0) + f(1, 1), f(1, 0) + f(1, 1), f(0, 0), f(1, 1), f(0, 0) + f(0, 1),
                    f(1, 0) - f(0, 0), f(0, 1) - f(1, 1))]
                val["xr"] = xf[:, 2 * KH:].astype(BF16)
            sm = lambda n: _unpack(cat([wc_s[k, t, :, n * 128:(n + 1) * 128]
                                        for k in range(2)]))
            blk = lambda k, j: _unpack(wa_s[m, k * KH // 2:(k + 1) * KH // 2,
                                            (2 * t + j) * 128:(2 * t + j + 1) * 128])
            rhs = (sm(0), blk(0, 0), sm(1), sm(2), blk(1, 1), sm(3), sm(4))
            mm = lambda n: _dot(val["xs"][n], rhs[n])
            tail = [_dot(val["xr"], _unpack(wa_s[m, KH:, (2 * t + j) * 128:(2 * t + j + 1) * 128]))
                    for j in range(2)]
            m1, m2, m3, m4, m5 = [mm(n) for n in range(5)]
            a_put(m, 2 * t, tail[0] + cat([mm(6) + (m1 + m4 - m5), m2 + m4]))
            a_put(m, 2 * t + 1, tail[1] + cat([m3 + m5, mm(5) + (m1 - m2 + m3)]))

        def window(m, j, w, hf):
            lo = A_HALO + hf * SEG - A_DIL * w
            return kv_s[m, j, lo:lo + SEG, :]

        def local_softmax(hf):
            pos = arow0 + hf * SEG + lax.broadcasted_iota(jnp.int32, (SEG, 128), 0)
            rows = slice(hf * SEG, (hf + 1) * SEG)
            logits = []
            for w in range(A_W):
                t = qa_s[0, rows, :] * window(0, 0, w, hf)
                for j in range(1, NT):
                    t = t + qa_s[j, rows, :] * window(0, j, w, hf)
                t = t + pltpu.roll(t, 64, 1)
                t = t + pltpu.roll(t, 32, 1)
                t = _round(_round(t) * a_scale)
                if w > 0 and hf == 0:
                    t = jnp.where(pos >= A_DIL * w, t, -1000000000.0)
                logits.append(t)
            mx = functools.reduce(jnp.maximum, logits)
            es = [jnp.exp(l - mx) for l in logits]
            inv = _recip(functools.reduce(lambda x, y: x + y, es))
            return es, inv

        def local_pv(j, hf):
            es, inv = val["LA", hf]
            o = es[0] * window(1, j, 0, hf)
            for w in range(1, A_W):
                o = o + es[w] * window(1, j, w, hf)
            return o * inv

        def local_out(j, acc):
            wj = _unpack(awo_s[j * 64:(j + 1) * 64, :])
            r = _dot(cat([local_pv(j, 0), local_pv(j, 1)]).astype(BF16), wj)
            for m in range(2):
                kv_s[m, j, :A_HALO, :] = kv_s[m, j, 2 * SEG:2 * SEG + A_HALO, :]
            return r if acc is None else acc + r

        val = {}
        acc = None
        oa = None
        for kind, t in _order(u):
            if kind == "K":
                val[kind, t] = block_diag(t, 1)
            elif kind == "V":
                val[kind, t] = block_diag(t, 2)
            elif kind == "Q":
                val[kind, t] = proj(t, 0)
            elif kind == "T":
                val[kind, t] = keys_t(val["K", t])
            elif kind == "S":
                val[kind, t] = qk(val["Q", t], val["T", t], a80)
            elif kind == "M":
                val[kind, t] = row_max(val["S", t], allowed, fill, is_a)
            elif kind == "E":
                val[kind, t] = probs(val["M", t], is_a, t >= LATE_FROM)
            elif kind == "PV":
                val[kind, t] = pv(val["E", t], val["V", t])
            elif kind == "TG":
                val[kind, t] = keys_t([x[:MEM + PRE] for r in range(GP)
                                       for x in val["K", GP * t + r]])
            elif kind == "PS":
                q = cat([pre(GP * t + r, 0) for r in range(GP)])
                val[kind, t] = qk(q, val["TG", t], p_first)
            elif kind == "MG":
                val[kind, t] = row_max(val["PS", t], p_allowed, p_fill, p_first)
            elif kind == "EG":
                val[kind, t] = probs(val["MG", t], p_first, False)[0]
            elif kind == "PPV":
                val[kind, t] = pre_pv(t, val["EG", t], [val["V", GP * t + r] for r in range(GP)])
            elif kind == "W":
                acc = wout(t, val["PV", t], acc)
            elif kind in ("XA", "XB", "XC", "Y"):
                wout_strassen(kind, t)
            elif kind == "LA":
                val[kind, t] = local_softmax(t)
            elif kind == "AP":
                a_proj(t)
            elif kind == "AO":
                oa = local_out(t, oa)
                if t == NT - 1:
                    out_s[pl.ds(arow0, 2 * SEG), :D] = oa.astype(BF16)
                    out_copy(arow0, 2 * SEG, 0).start()
        if last:
            m = lambda n: val["acc", n]
            acc = jnp.concatenate([
                cat([m(1) + m(4) - m(5) + m(7), m(2) + m(4)]),
                cat([m(3) + m(5), m(1) - m(2) + m(3) + m(6)]), m(0)], axis=1)
        return acc

    def steps(i, mem):
        @pl.when(i == 1)
        def _():
            for cp in x_rest:
                cp.wait()

        accs = []
        for u in range(SPT):
            accs.append(segment(i * SPT + u, mem, u))
            mem = accs[-1][FRESH:SEG]
        res = cat([x for u in range(SPT) for x in (
            accs[-1][SEG + u * PRE:SEG + (u + 1) * PRE], accs[u][:FRESH])])
        row = pl.multiple_of(i * SPT * SEG, SPT * SEG)
        out_s[pl.ds(row, SPT * SEG), D:2 * D] = res.astype(BF16)
        out_copy(row, SPT * SEG, 1).start()
        return mem

    lax.fori_loop(0, N_STEPS, steps, mem0_s[...].astype(F32))

    wo_copy(NTRIP - 1).wait()
    wo_copy(NTRIP).wait()
    wait_trip(NTRIP)
    wait_trip(NTRIP + 1)

    done = N_STEPS * SPT * SEG
    pltpu.make_async_copy(out_s.at[:done, :], out_hbm.at[:done, :], sems.at[7]).wait()


@jax.jit
def pallas_concat_heads__sliding_local_dilated__memory_aug_recurrent_mem_tr__prompt_kernel(
    A_x: jax.Array,
    A_wqkv: jax.Array,
    A_wo: jax.Array,
    B_x: jax.Array,
    B_mem0: jax.Array,
    B_Wq: jax.Array,
    B_Wk: jax.Array,
    B_Wv: jax.Array,
    B_Wo: jax.Array,
    B_seg_len,
):
    del B_seg_len
    assert A_x.shape == (1, S, D) and B_x.shape == (1, S, D)
    hd = B_H * B_DH
    wq_t = jnp.transpose(B_Wq, (1, 2, 0)).reshape(hd, D)
    wk_t = jnp.transpose(B_Wk, (1, 2, 0)).reshape(hd, D)
    wv_t = jnp.transpose(B_Wv, (1, 2, 0)).reshape(hd, D)
    wo = B_Wo.reshape(hd, D)

    any_spec = pl.BlockSpec(memory_space=pl.ANY)
    out = pl.pallas_call(
        _kernel,
        out_shape=jax.ShapeDtypeStruct((S, 2 * D), BF16),
        in_specs=[any_spec] * 10,
        out_specs=any_spec,
        scratch_shapes=[
            pltpu.VMEM((2, PP, 4, PW, D), BF16),
            pltpu.VMEM((NT, D, 128), BF16),
            pltpu.VMEM((4, 2 * WO_ROWS, WO_W), BF16),
            pltpu.VMEM((NP, D // 2, 3 * PW), U32),
            pltpu.VMEM((hd // 2 + PW, WO_W), U32),
            pltpu.VMEM((NQ + 1, 5, PW // 2, KH), U32),
            pltpu.VMEM((NSEG, NP // PP, PRE, 3 * PP * PW), F32),
            pltpu.VMEM((SPT - 1, NG, GP * PRE, PW), F32),
            pltpu.VMEM((S, 2 * D), BF16),
            pltpu.VMEM((S, X_W), BF16),
            pltpu.VMEM((S, X_W), BF16),
            pltpu.VMEM((NSEG, PRE, D), BF16),
            pltpu.VMEM((NSEG * PRE // 2, D), U32),
            pltpu.VMEM((5, NSEG * PRE // 4, 256), U32),
            pltpu.VMEM((MEM, D), BF16),
            pltpu.VMEM((3, D // 2, D), U32),
            pltpu.VMEM((3, 2, 64, D), U32),
            pltpu.VMEM((D // 2, D), U32),
            pltpu.VMEM((NT, D // 2, 128), U32),
            pltpu.VMEM((NT, 2 * SEG, 128), F32),
            pltpu.VMEM((2, NT, A_HALO + 2 * SEG, 128), F32),
            pltpu.SemaphoreType.DMA((10,)),
        ],
        compiler_params=pltpu.CompilerParams(vmem_limit_bytes=120 * 1024 * 1024,
                                             disable_bounds_checks=True),
    )(A_x.reshape(S, D), A_wqkv, A_wo, B_x.reshape(S, D), B_x.reshape(NSEG, SEG // PRE, PRE, D),
      B_mem0.reshape(MEM, D), wq_t, wk_t, wv_t, wo)
    return out.reshape(1, S, 2 * D)
```
